```python
import jax
import jax.numpy as jnp

def _softmax(x, axis=-1):
    return jax.nn.softmax(x, axis=axis)

def _gelu(x):
    return jax.nn.gelu(x, approximate=True)

def _silu(x):
    return jax.nn.silu(x)

def _sigmoid(x):
    return jax.nn.sigmoid(x)

def _layernorm(x, axis=-1, eps=1e-05):
    m = jnp.mean(x, axis=axis, keepdims=True)
    v = jnp.var(x, axis=axis, keepdims=True)
    return (x - m) / jnp.sqrt(v + eps)

def _scatter_add(tgt, idx, src, axis=0):
    return tgt.at[idx].add(src)

def _segment_sum(src, seg, n):
    return jax.ops.segment_sum(src, seg, n)

class _Rng:

    def __init__(self, key):
        self._k = key

    def _next(self):
        self._k, sub = jax.random.split(self._k)
        return sub

    def normal(self, shape):
        return jax.random.normal(self._next(), shape, dtype=jnp.bfloat16)

    def randint(self, lo, hi, shape):
        return jax.random.randint(self._next(), shape, lo, hi, dtype=jnp.int32)

    def uniform(self, shape, lo=0.0, hi=1.0):
        return jax.random.uniform(self._next(), shape, jnp.bfloat16, lo, hi)

    def permutation(self, n):
        return jax.random.permutation(self._next(), n)
kernel_name = 'interleave_layers__memory_aug_recurrent_mem_tr__sliding_local_dilated__prompt'

def setup_inputs():
    _rng = _Rng(jax.random.key(int.from_bytes(__import__("os").urandom(4), "little")))
    _w = lambda a: (lambda t: t.astype(jnp.bfloat16) if jnp.issubdtype(t.dtype, jnp.floating) else t)(jnp.asarray(a))

    def _A_setup():
        B, S, Dm = (1, 2048, 640)
        H, Dh = (32, 192)
        M, seg = (8, 32)
        seg = min(seg, S)
        S = S // seg * seg
        return {'x': _w((lambda *s: _rng.normal(s) * 0.05)(B, S, Dm)), 'mem0': _w((lambda *s: _rng.normal(s) * 0.05)(B, M, Dm)), 'Wq': _w((lambda *s: _rng.normal(s) * 0.05)(Dm, H, Dh) * Dm ** (-0.5)), 'Wk': _w((lambda *s: _rng.normal(s) * 0.05)(Dm, H, Dh) * Dm ** (-0.5)), 'Wv': _w((lambda *s: _rng.normal(s) * 0.05)(Dm, H, Dh) * Dm ** (-0.5)), 'Wo': _w((lambda *s: _rng.normal(s) * 0.05)(H, Dh, Dm) * (H * Dh) ** (-0.5)), 'seg_len': seg}
    _A_in = _A_setup()

    def _B_setup():
        B, S, D = (1, 2048, 640)
        return {'x': _w((lambda *s: _rng.normal(s) * 0.05)(B, S, D)), 'wqkv': _w((lambda *s: _rng.normal(s) * 0.05)(D, 3 * D)), 'wo': _w((lambda *s: _rng.normal(s) * 0.05)(D, D))}
    _B_in = _B_setup()
    return {'A_x': _A_in['x'], 'A_mem0': _A_in['mem0'], 'A_Wq': _A_in['Wq'], 'A_Wk': _A_in['Wk'], 'A_Wv': _A_in['Wv'], 'A_Wo': _A_in['Wo'], 'A_seg_len': _A_in['seg_len'], 'B_x': _B_in['x'], 'B_wqkv': _B_in['wqkv'], 'B_wo': _B_in['wo']}

def reference(A_x, A_mem0, A_Wq, A_Wk, A_Wv, A_Wo, A_seg_len, B_x, B_wqkv, B_wo):

    def _A_ref(x, mem0, Wq, Wk, Wv, Wo, seg_len):
        B, S, Dm = x.shape
        H, Dh = (Wq.shape[1], Wq.shape[2])
        M = mem0.shape[1]
        scale = Dh ** (-0.5)
        n_seg = S // seg_len
        L = M + seg_len
        idx = jnp.arange(L)
        mask = (idx[:, None] < M) | (idx[:, None] >= idx[None, :])
        mem = mem0
        outs = []
        for s in range(n_seg):
            xs = x[:, s * seg_len:(s + 1) * seg_len, :].copy()
            h = jnp.concatenate([mem, xs], axis=1)
            q = jnp.einsum('btd,dhe->bhte', h, Wq)
            k = jnp.einsum('btd,dhe->bhte', h, Wk)
            v = jnp.einsum('btd,dhe->bhte', h, Wv)
            scores = jnp.einsum('bhqe,bhke->bhqk', q, k) * scale
            scores = jnp.where(mask[None, None], scores, -1000000000.0)
            p = _softmax(scores, axis=-1)
            o = jnp.einsum('bhqk,bhke->bhqe', p, v)
            o = jnp.einsum('bhte,hed->btd', o, Wo)
            mem = o[:, :M, :].copy()
            outs.append(o[:, M:, :])
        return jnp.concatenate(outs, axis=1)

    def _B_ref(x, wqkv, wo):
        B, S, D = x.shape
        H = 32
        Dh = D // H
        W, dil = (8, 2)
        qkv = (lambda x, *d: x.transpose(*d))((x @ wqkv).reshape(B, S, 3, H, Dh), 2, 0, 3, 1, 4)
        q, k, v = (qkv[0], qkv[1], qkv[2])
        scale = Dh ** (-0.5)
        pos = jnp.arange(S)
        off = jnp.arange(W) * dil
        idx = pos[:, None] - off[None, :]
        mask = idx >= 0
        idx_c = jnp.where(mask, idx, 0).reshape(-1)
        kg = k[:, :, idx_c, :].reshape(B, H, S, W, Dh)
        vg = v[:, :, idx_c, :].reshape(B, H, S, W, Dh)
        logits = jnp.einsum('bhsd,bhswd->bhsw', q, kg) * scale
        logits = jnp.where(mask[None, None, :, :], logits, -1000000000.0)
        attn = _softmax(logits, axis=-1)
        o = jnp.einsum('bhsw,bhswd->bhsd', attn, vg)
        return (lambda x, *d: x.transpose(*d))(o, 0, 2, 1, 3).reshape(B, S, D) @ wo
    x = A_x
    x = x + _A_ref(_layernorm(x, axis=-1), A_mem0, A_Wq, A_Wk, A_Wv, A_Wo, A_seg_len)
    x = x + _B_ref(_layernorm(x, axis=-1), B_wqkv, B_wo)
    x = x + _A_ref(_layernorm(x, axis=-1), A_mem0, A_Wq, A_Wk, A_Wv, A_Wo, A_seg_len)
    x = x + _B_ref(_layernorm(x, axis=-1), B_wqkv, B_wo)
    return x
```

```python
import functools

import jax
import jax.numpy as jnp
from jax import lax
import jax.experimental.pallas as pl
import jax.experimental.pallas.tpu as pltpu

F32 = jnp.float32
BF16 = jnp.bfloat16
NEG = -1000000000.0
LN_EPS = 1e-05

B_HEADS = 32
B_WIN = 8
B_DIL = 2
HIST = 16


def _ln(x):
    m = jnp.mean(x, axis=-1, keepdims=True)
    c = x - m
    v = jnp.mean(c * c, axis=-1, keepdims=True)
    return c / jnp.sqrt(v + LN_EPS)


def _nt(a, b):
    return lax.dot_general(a, b, (((1,), (1,)), ((), ())), preferred_element_type=F32)


def _nn(a, b):
    return jnp.dot(a, b, preferred_element_type=F32)


def _kernel(x_ref, mem0_ref, wq_ref, wk_ref, wv_ref, wo_ref, bqkv_ref, bwo_ref,
            out_ref,
            h_ref, xb_ref, x2_ref, kb_ref, vb_ref,
            *, seg, n_seg, n_mem, n_heads, dh, dm):
    t = pl.program_id(0)
    L = n_mem + seg
    R = 2 * L
    LP = 48
    PW = 2 * dh
    nct = dm // 128

    @pl.when(t == 0)
    def _init():
        m0 = mem0_ref[...].astype(F32)
        h_ref[0:n_mem, :] = m0
        h_ref[n_mem:L, :] = _ln(x_ref[0:seg, :].astype(F32))
        h_ref[L:L + n_mem, :] = m0
        h_ref[L + n_mem:R, :] = jnp.zeros((seg, dm), F32)
        xb_ref[...] = jnp.zeros(xb_ref.shape, F32)
        x2_ref[...] = jnp.zeros(x2_ref.shape, F32)
        kb_ref[...] = jnp.zeros(kb_ref.shape, F32)
        vb_ref[...] = jnp.zeros(vb_ref.shape, F32)

    def b_part():
        yb = xb_ref[...]
        qkv = _nn(_ln(yb).astype(BF16), bqkv_ref[...])
        bscale = float(dm // B_HEADS) ** (-0.5)
        row = lax.broadcasted_iota(jnp.int32, (seg, 128), 0)
        outs = []
        for l in range(2):
            r0 = l * seg
            pos = row + (t - (1 + 2 * l)) * seg
            for j in range(nct):
                kb_ref[l, j, HIST:HIST + seg, :] = qkv[r0:r0 + seg, dm + j * 128:dm + (j + 1) * 128]
                vb_ref[l, j, HIST:HIST + seg, :] = qkv[r0:r0 + seg, 2 * dm + j * 128:2 * dm + (j + 1) * 128]
            logits = []
            for w in range(B_WIN):
                o = HIST - w * B_DIL
                acc = None
                for j in range(nct):
                    p = qkv[r0:r0 + seg, j * 128:(j + 1) * 128] * kb_ref[l, j, o:o + seg, :]
                    acc = p if acc is None else acc + p
                acc = acc + pltpu.roll(acc, 64, 1)
                acc = acc + pltpu.roll(acc, 32, 1)
                lg = acc * bscale
                if w > 0:
                    lg = jnp.where(pos >= w * B_DIL, lg, NEG)
                logits.append(lg)
            m = logits[0]
            for w in range(1, B_WIN):
                m = jnp.maximum(m, logits[w])
            es = [jnp.exp(lg - m) for lg in logits]
            den = es[0]
            for w in range(1, B_WIN):
                den = den + es[w]
            inv = 1.0 / den
            cols = []
            for j in range(nct):
                acc = None
                for w in range(B_WIN):
                    o = HIST - w * B_DIL
                    p = es[w] * vb_ref[l, j, o:o + seg, :]
                    acc = p if acc is None else acc + p
                cols.append(acc * inv)
            outs.append(jnp.concatenate(cols, axis=1))
            for j in range(nct):
                kb_ref[l, j, 0:HIST, :] = qkv[r0 + seg - HIST:r0 + seg, dm + j * 128:dm + (j + 1) * 128]
                vb_ref[l, j, 0:HIST, :] = qkv[r0 + seg - HIST:r0 + seg, 2 * dm + j * 128:2 * dm + (j + 1) * 128]
        ob = jnp.concatenate(outs, axis=0).astype(BF16)
        zb = yb + _nn(ob, bwo_ref[...])
        out_ref[...] = zb[seg:2 * seg].astype(out_ref.dtype)
        return zb[0:seg]

    def a_part():
        h = h_ref[...].astype(BF16)
        scale = float(dh) ** (-0.5)
        qi = lax.broadcasted_iota(jnp.int32, (R, R), 0)
        li = lax.broadcasted_iota(jnp.int32, (R, R), 1)
        qi = jnp.where(qi >= L, qi - L, qi)
        lane_a = li < L
        ki = jnp.where(lane_a, li, li - L)
        causal = (qi < n_mem) | (qi >= ki)
        col_a = lax.broadcasted_iota(jnp.int32, (L, PW), 1) < dh
        acc = None
        for g in range(n_heads // 2):
            c0 = g * PW
            q = _nt(h, wq_ref[c0:c0 + PW, :]).astype(BF16)
            k = _nt(h, wk_ref[c0:c0 + PW, :])
            v = _nt(h, wv_ref[c0:c0 + PW, :])

            def blk(z, l):
                zz = z[l * L:(l + 1) * L]
                return jnp.concatenate(
                    [jnp.where(col_a, zz, 0.0), jnp.where(col_a, 0.0, zz)], axis=0).astype(BF16)

            s1 = _nt(q[0:LP], blk(k, 0))[0:L]
            s2 = _nt(q[R - LP:R], blk(k, 1))[LP - L:LP]
            s = jnp.concatenate([s1, s2], axis=0) * scale
            s = jnp.where(causal, s, NEG)
            m_a = jnp.max(jnp.where(lane_a, s, -jnp.inf), axis=-1, keepdims=True)
            m_b = jnp.max(jnp.where(lane_a, -jnp.inf, s), axis=-1, keepdims=True)
            e = jnp.exp(s - jnp.where(lane_a, m_a, m_b))
            d_a = jnp.sum(jnp.where(lane_a, e, 0.0), axis=-1, keepdims=True)
            d_b = jnp.sum(jnp.where(lane_a, 0.0, e), axis=-1, keepdims=True)
            p = (e / jnp.where(lane_a, d_a, d_b)).astype(BF16)
            o1 = _nn(p[0:LP], blk(v, 0))[0:L]
            o2 = _nn(p[R - LP:R], blk(v, 1))[LP - L:LP]
            o = jnp.concatenate([o1, o2], axis=0).astype(BF16)
            c = _nn(o, wo_ref[c0:c0 + PW, :])
            acc = c if acc is None else acc + c
        return acc

    @pl.when(t < n_seg + 2)
    def _main():
        x2_new = b_part()
        acc = a_part()
        tc = jnp.minimum(t, n_seg - 1)
        tn = jnp.minimum(t + 1, n_seg - 1)
        x_cur = x_ref[pl.ds(pl.multiple_of(tc * seg, seg), seg), :].astype(F32)
        x_nxt = x_ref[pl.ds(pl.multiple_of(tn * seg, seg), seg), :].astype(F32)
        xb_ref[0:seg, :] = x_cur + acc[n_mem:L]
        xb_ref[seg:2 * seg, :] = x2_ref[...] + acc[L + n_mem:R]
        x2_ref[...] = x2_new
        h_ref[0:n_mem, :] = acc[0:n_mem]
        h_ref[n_mem:L, :] = _ln(x_nxt)
        h_ref[L:L + n_mem, :] = jnp.where(t < 2, mem0_ref[...].astype(F32), acc[L:L + n_mem])
        h_ref[L + n_mem:R, :] = _ln(x2_new)

    @pl.when(t == n_seg + 2)
    def _tail():
        b_part()


@functools.partial(jax.jit, static_argnames=("A_seg_len",))
def pallas_interleave_layers__memory_aug_recurrent_mem_tr__sliding_local_dilated__prompt_kernel(
    A_x: jax.Array,
    A_mem0: jax.Array,
    A_Wq: jax.Array,
    A_Wk: jax.Array,
    A_Wv: jax.Array,
    A_Wo: jax.Array,
    A_seg_len,
    B_x: jax.Array,
    B_wqkv: jax.Array,
    B_wo: jax.Array,
):
    del B_x
    _, S, dm = A_x.shape
    n_heads, dh = A_Wq.shape[1], A_Wq.shape[2]
    n_mem = A_mem0.shape[1]
    seg = int(A_seg_len)
    n_seg = S // seg
    hd = n_heads * dh
    bdh = dm // B_HEADS

    x = A_x.reshape(S, dm)
    mem0 = A_mem0.reshape(n_mem, dm)
    wq = jnp.transpose(A_Wq, (1, 2, 0)).reshape(hd, dm)
    wk = jnp.transpose(A_Wk, (1, 2, 0)).reshape(hd, dm)
    wv = jnp.transpose(A_Wv, (1, 2, 0)).reshape(hd, dm)
    wo = A_Wo.reshape(hd, dm)
    bqkv = B_wqkv.reshape(dm, 3, B_HEADS, bdh).transpose(0, 1, 3, 2).reshape(dm, 3 * dm)
    bwo = B_wo.reshape(B_HEADS, bdh, dm).transpose(1, 0, 2).reshape(dm, dm)

    kern = functools.partial(_kernel, seg=seg, n_seg=n_seg, n_mem=n_mem,
                             n_heads=n_heads, dh=dh, dm=dm)

    def full(shape):
        return pl.BlockSpec(shape, lambda t: (0,) * len(shape), pipeline_mode=pl.Buffered(1))

    out = pl.pallas_call(
        kern,
        grid=(n_seg + 3,),
        in_specs=[full((S, dm)), full((n_mem, dm)), full((hd, dm)), full((hd, dm)),
                  full((hd, dm)), full((hd, dm)), full((dm, 3 * dm)), full((dm, dm))],
        out_specs=pl.BlockSpec((seg, dm), lambda t: (jnp.maximum(t - 3, 0), 0)),
        out_shape=jax.ShapeDtypeStruct((S, dm), A_x.dtype),
        scratch_shapes=[
            pltpu.VMEM((2 * (n_mem + seg), dm), F32),
            pltpu.VMEM((2 * seg, dm), F32),
            pltpu.VMEM((seg, dm), F32),
            pltpu.VMEM((2, dm // 128, HIST + seg, 128), F32),
            pltpu.VMEM((2, dm // 128, HIST + seg, 128), F32),
        ],
        compiler_params=pltpu.CompilerParams(
            dimension_semantics=("arbitrary",),
            vmem_limit_bytes=100 * 1024 * 1024,
        ),
    )(x, mem0, wq, wk, wv, wo, bqkv, bwo)
    return out.reshape(1, S, dm)
```

```python
import functools

import jax
import jax.numpy as jnp
from jax import lax
import jax.experimental.pallas as pl
import jax.experimental.pallas.tpu as pltpu

F32 = jnp.float32
BF16 = jnp.bfloat16
NEG = -1000000000.0
LN_EPS = 1e-05

B_HEADS = 32
B_WIN = 8
B_DIL = 2
HIST = 16


def _ln(x):
    m = jnp.mean(x, axis=-1, keepdims=True)
    c = x - m
    v = jnp.mean(c * c, axis=-1, keepdims=True)
    return c / jnp.sqrt(v + LN_EPS)


def _nt(a, b):
    return lax.dot_general(a, b, (((1,), (1,)), ((), ())), preferred_element_type=F32)


def _nn(a, b):
    return jnp.dot(a, b, preferred_element_type=F32)


def _kernel(x_ref, mem0_ref, wq_ref, wk_ref, wv_ref, wo_ref, bqkv_ref, bwo_ref,
            out_ref,
            h_ref, xb_ref, x2_ref, kb_ref, vb_ref,
            *, seg, n_seg, n_mem, n_heads, dh, dm):
    t = pl.program_id(0)
    L = n_mem + seg
    R = 2 * L
    LP = 48
    PW = 2 * dh
    nct = dm // 128

    @pl.when(t == 0)
    def _init():
        m0 = mem0_ref[...].astype(F32)
        h_ref[0:n_mem, :] = m0
        h_ref[n_mem:L, :] = _ln(x_ref[0:seg, :].astype(F32))
        h_ref[L:L + n_mem, :] = m0
        h_ref[L + n_mem:R, :] = jnp.zeros((seg, dm), F32)
        xb_ref[...] = jnp.zeros(xb_ref.shape, F32)
        x2_ref[...] = jnp.zeros(x2_ref.shape, F32)
        kb_ref[...] = jnp.zeros(kb_ref.shape, F32)
        vb_ref[...] = jnp.zeros(vb_ref.shape, F32)

    bscale = float(dm // B_HEADS) ** (-0.5)

    def b_qkv():
        yb = xb_ref[...]
        return _nn(_ln(yb).astype(BF16), bqkv_ref[...])

    def b_attn(qkv):
        row = lax.broadcasted_iota(jnp.int32, (seg, 128), 0)
        outs = []
        for l in range(2):
            r0 = l * seg
            pos = row + (t - (1 + 2 * l)) * seg
            for j in range(nct):
                kb_ref[l, j, HIST:HIST + seg, :] = qkv[r0:r0 + seg, dm + j * 128:dm + (j + 1) * 128]
                vb_ref[l, j, HIST:HIST + seg, :] = qkv[r0:r0 + seg, 2 * dm + j * 128:2 * dm + (j + 1) * 128]
            logits = []
            for w in range(B_WIN):
                o = HIST - w * B_DIL
                acc = None
                for j in range(nct):
                    p = qkv[r0:r0 + seg, j * 128:(j + 1) * 128] * kb_ref[l, j, o:o + seg, :]
                    acc = p if acc is None else acc + p
                acc = acc + pltpu.roll(acc, 64, 1)
                acc = acc + pltpu.roll(acc, 32, 1)
                lg = acc * bscale
                if w > 0:
                    lg = jnp.where(pos >= w * B_DIL, lg, NEG)
                logits.append(lg)
            m = logits[0]
            for w in range(1, B_WIN):
                m = jnp.maximum(m, logits[w])
            es = [jnp.exp(lg - m) for lg in logits]
            den = es[0]
            for w in range(1, B_WIN):
                den = den + es[w]
            inv = 1.0 / den
            cols = []
            for j in range(nct):
                acc = None
                for w in range(B_WIN):
                    o = HIST - w * B_DIL
                    p = es[w] * vb_ref[l, j, o:o + seg, :]
                    acc = p if acc is None else acc + p
                cols.append(acc * inv)
            outs.append(jnp.concatenate(cols, axis=1))
            for j in range(nct):
                kb_ref[l, j, 0:HIST, :] = qkv[r0 + seg - HIST:r0 + seg, dm + j * 128:dm + (j + 1) * 128]
                vb_ref[l, j, 0:HIST, :] = qkv[r0 + seg - HIST:r0 + seg, 2 * dm + j * 128:2 * dm + (j + 1) * 128]
        return jnp.concatenate(outs, axis=0).astype(BF16)

    def b_out(ob):
        zb = xb_ref[...] + _nn(ob, bwo_ref[...])
        out_ref[...] = zb[seg:2 * seg].astype(out_ref.dtype)
        return zb[0:seg]

    @pl.when(t < n_seg + 2)
    def _main():
        h = h_ref[...].astype(BF16)
        scale = float(dh) ** (-0.5)
        qi = lax.broadcasted_iota(jnp.int32, (R, R), 0)
        li = lax.broadcasted_iota(jnp.int32, (R, R), 1)
        qi = jnp.where(qi >= L, qi - L, qi)
        lane_a = li < L
        ki = jnp.where(lane_a, li, li - L)
        causal = (qi < n_mem) | (qi >= ki)
        col_a = lax.broadcasted_iota(jnp.int32, (L, PW), 1) < dh

        def proj(w_ref, g):
            return _nt(h, w_ref[g * PW:(g + 1) * PW, :])

        def blk(z, l):
            zz = z[l * L:(l + 1) * L]
            return jnp.concatenate(
                [jnp.where(col_a, zz, 0.0), jnp.where(col_a, 0.0, zz)], axis=0).astype(BF16)

        def scores(q, k):
            s1 = _nt(q[0:LP].astype(BF16), blk(k, 0))[0:L]
            s2 = _nt(q[R - LP:R].astype(BF16), blk(k, 1))[LP - L:LP]
            s = jnp.concatenate([s1, s2], axis=0) * scale
            s = jnp.where(causal, s, NEG)
            m_a = jnp.max(jnp.where(lane_a, s, -jnp.inf), axis=-1, keepdims=True)
            m_b = jnp.max(jnp.where(lane_a, -jnp.inf, s), axis=-1, keepdims=True)
            e = jnp.exp(s - jnp.where(lane_a, m_a, m_b))
            d_a = jnp.sum(jnp.where(lane_a, e, 0.0), axis=-1, keepdims=True)
            d_b = jnp.sum(jnp.where(lane_a, 0.0, e), axis=-1, keepdims=True)
            return e / jnp.where(lane_a, d_a, d_b)

        def pv(p, v):
            o1 = _nn(p[0:LP].astype(BF16), blk(v, 0))[0:L]
            o2 = _nn(p[R - LP:R].astype(BF16), blk(v, 1))[LP - L:LP]
            return jnp.concatenate([o1, o2], axis=0).astype(BF16)

        def oproj(o, g):
            return _nn(o, wo_ref[g * PW:(g + 1) * PW, :])

        G = n_heads // 2
        q = proj(wq_ref, 0)
        k = proj(wk_ref, 0)
        v = proj(wv_ref, 0)
        p = scores(q, k)
        bq = b_qkv()
        ob = b_attn(bq)
        acc = None
        for g in range(G - 1):
            q = proj(wq_ref, g + 1)
            k = proj(wk_ref, g + 1)
            o = pv(p, v)
            v = proj(wv_ref, g + 1)
            p = scores(q, k)
            if g < G - 2:
                c = oproj(o, g)
                acc = c if acc is None else acc + c
        x2_new = b_out(ob)
        o_last = pv(p, v)
        acc = acc + oproj(o, G - 2)
        acc = acc + oproj(o_last, G - 1)

        tc = jnp.minimum(t, n_seg - 1)
        tn = jnp.minimum(t + 1, n_seg - 1)
        x_cur = x_ref[pl.ds(pl.multiple_of(tc * seg, seg), seg), :].astype(F32)
        x_nxt = x_ref[pl.ds(pl.multiple_of(tn * seg, seg), seg), :].astype(F32)
        xb_ref[0:seg, :] = x_cur + acc[n_mem:L]
        xb_ref[seg:2 * seg, :] = x2_ref[...] + acc[L + n_mem:R]
        x2_ref[...] = x2_new
        h_ref[0:n_mem, :] = acc[0:n_mem]
        h_ref[n_mem:L, :] = _ln(x_nxt)
        h_ref[L:L + n_mem, :] = jnp.where(t < 2, mem0_ref[...].astype(F32), acc[L:L + n_mem])
        h_ref[L + n_mem:R, :] = _ln(x2_new)

    @pl.when(t == n_seg + 2)
    def _tail():
        b_out(b_attn(b_qkv()))


@functools.partial(jax.jit, static_argnames=("A_seg_len",))
def pallas_interleave_layers__memory_aug_recurrent_mem_tr__sliding_local_dilated__prompt_kernel(
    A_x: jax.Array,
    A_mem0: jax.Array,
    A_Wq: jax.Array,
    A_Wk: jax.Array,
    A_Wv: jax.Array,
    A_Wo: jax.Array,
    A_seg_len,
    B_x: jax.Array,
    B_wqkv: jax.Array,
    B_wo: jax.Array,
):
    del B_x
    _, S, dm = A_x.shape
    n_heads, dh = A_Wq.shape[1], A_Wq.shape[2]
    n_mem = A_mem0.shape[1]
    seg = int(A_seg_len)
    n_seg = S // seg
    hd = n_heads * dh
    bdh = dm // B_HEADS

    x = A_x.reshape(S, dm)
    mem0 = A_mem0.reshape(n_mem, dm)
    wq = jnp.transpose(A_Wq, (1, 2, 0)).reshape(hd, dm)
    wk = jnp.transpose(A_Wk, (1, 2, 0)).reshape(hd, dm)
    wv = jnp.transpose(A_Wv, (1, 2, 0)).reshape(hd, dm)
    wo = A_Wo.reshape(hd, dm)
    bqkv = B_wqkv.reshape(dm, 3, B_HEADS, bdh).transpose(0, 1, 3, 2).reshape(dm, 3 * dm)
    bwo = B_wo.reshape(B_HEADS, bdh, dm).transpose(1, 0, 2).reshape(dm, dm)

    kern = functools.partial(_kernel, seg=seg, n_seg=n_seg, n_mem=n_mem,
                             n_heads=n_heads, dh=dh, dm=dm)

    def full(shape):
        return pl.BlockSpec(shape, lambda t: (0,) * len(shape), pipeline_mode=pl.Buffered(1))

    out = pl.pallas_call(
        kern,
        grid=(n_seg + 3,),
        in_specs=[full((S, dm)), full((n_mem, dm)), full((hd, dm)), full((hd, dm)),
                  full((hd, dm)), full((hd, dm)), full((dm, 3 * dm)), full((dm, dm))],
        out_specs=pl.BlockSpec((seg, dm), lambda t: (jnp.maximum(t - 3, 0), 0)),
        out_shape=jax.ShapeDtypeStruct((S, dm), A_x.dtype),
        scratch_shapes=[
            pltpu.VMEM((2 * (n_mem + seg), dm), F32),
            pltpu.VMEM((2 * seg, dm), F32),
            pltpu.VMEM((seg, dm), F32),
            pltpu.VMEM((2, dm // 128, HIST + seg, 128), F32),
            pltpu.VMEM((2, dm // 128, HIST + seg, 128), F32),
        ],
        compiler_params=pltpu.CompilerParams(
            dimension_semantics=("arbitrary",),
            vmem_limit_bytes=100 * 1024 * 1024,
        ),
    )(x, mem0, wq, wk, wv, wo, bqkv, bwo)
    return out.reshape(1, S, dm)
```

```python
import functools

import jax
import jax.numpy as jnp
from jax import lax
import jax.experimental.pallas as pl
import jax.experimental.pallas.tpu as pltpu

F32 = jnp.float32
BF16 = jnp.bfloat16
NEG = -1000000000.0
LN_EPS = 1e-05

B_HEADS = 32
B_WIN = 8
B_DIL = 2
HIST = 16
AH = 16
LAG = 2


def _ln(x):
    m = jnp.mean(x, axis=-1, keepdims=True)
    c = x - m
    v = jnp.mean(c * c, axis=-1, keepdims=True)
    return c * lax.rsqrt(v + LN_EPS)


def _nt(a, b):
    return lax.dot_general(a, b, (((1,), (1,)), ((), ())), preferred_element_type=F32)


def _nn(a, b):
    return jnp.dot(a, b, preferred_element_type=F32)


def _cat(xs, axis=0):
    return jnp.concatenate(xs, axis=axis)


def _kernel(x_hbm, mem0_ref, wq_hbm, wk_hbm, wv_hbm, wo_hbm, bqkv_hbm, bwo_hbm,
            out_ref,
            x_ref, stage_ref, w_ref, wo_ref, bst1_ref, bst2_ref, btmp_ref, bqkv_ref, bwo_ref,
            xln_ref, ring_ref,
            h_ref, xb_ref, x2_ref, kb_ref, vb_ref, sem_w, sem_m,
            *, seg, n_seg, n_mem, n_heads, dh, dm):
    t = pl.program_id(0)
    S = seg * n_seg
    M2 = 2 * n_mem
    R = M2 + 2 * seg
    RQ = M2 + seg + AH
    PW = 2 * dh
    G = n_heads // 2
    nct = dm // 128
    n_ah = n_seg - 1
    A0 = S - n_ah * AH
    NPRE = A0 - LAG * seg
    RS = -(-A0 // seg) * seg
    w_hbm = (wq_hbm, wk_hbm, wv_hbm)

    NSLOT = 3
    bdh = dm // B_HEADS

    def w_copy(p, g):
        slot = g % NSLOT
        return pltpu.make_async_copy(w_hbm[p].at[pl.ds(g * PW, PW), :],
                                     stage_ref.at[slot, p], sem_w.at[p, slot])

    @pl.when(t == 0)
    def _prologue():
        xa = pltpu.make_async_copy(x_hbm.at[pl.ds(0, NPRE), :], x_ref.at[pl.ds(0, NPRE), :], sem_m.at[0])
        late = [pltpu.make_async_copy(x_hbm.at[pl.ds(NPRE, S - NPRE), :],
                                      x_ref.at[pl.ds(NPRE, S - NPRE), :], sem_m.at[1]),
                pltpu.make_async_copy(bqkv_hbm, bst1_ref, sem_m.at[2]),
                pltpu.make_async_copy(bwo_hbm, bst2_ref, sem_m.at[3])]
        late += [pltpu.make_async_copy(wo_hbm.at[:, pl.ds(j * 128, 128)], wo_ref.at[j], sem_m.at[4 + j])
                 for j in range(nct)]
        xa.start()
        for p in range(3):
            w_copy(p, 0).start()
        xb_ref[...] = jnp.zeros(xb_ref.shape, F32)
        x2_ref[...] = jnp.zeros(x2_ref.shape, F32)
        kb_ref[...] = jnp.zeros(kb_ref.shape, F32)
        vb_ref[...] = jnp.zeros(vb_ref.shape, F32)
        xa.wait()
        for p in range(3):
            w_copy(p, 1).start()

        for i in range(NPRE // 16):
            xln_ref[i * 16:(i + 1) * 16, :] = _ln(x_ref[i * 16:(i + 1) * 16, :].astype(F32)).astype(BF16)

        def pre_group(g):
            for p in range(3):
                w_copy(p, g).wait()
            xl = xln_ref[...]
            slot = g % NSLOT
            for p in range(3):
                w = stage_ref[slot, p]
                y = _nt(xl, w).astype(BF16)
                wt = w.T
                for j in range(3):
                    ring_ref[(g * 3 + p) * 3 + j, 0:NPRE, :] = y[:, j * 128:(j + 1) * 128]
                    w_ref[(g * 3 + p) * 3 + j] = wt[:, j * 128:(j + 1) * 128]

        def pre_body(g, c):
            @pl.when(g + 2 < G)
            def _():
                for p in range(3):
                    w_copy(p, g + 2).start()

            @pl.when(g == 1)
            def _():
                for cp in late:
                    cp.start()
            pre_group(g)
            return c
        lax.fori_loop(0, G - 1, pre_body, 0)

        for cp in late:
            cp.wait()
        for c in range(3 * nct):
            tr = bst1_ref[:, c * 128:(c + 1) * 128].astype(F32).T
            for j in range(nct):
                btmp_ref[j, c * 128:(c + 1) * 128, :] = tr[:, j * 128:(j + 1) * 128]
        for j in range(nct):
            btmp_ref[j, 3 * dm:4 * dm, :] = bst2_ref[:, j * 128:(j + 1) * 128].astype(F32)
        pre_group(G - 1)
        dpt = 128 // B_HEADS
        for c in range(3 * nct):
            part, c5 = divmod(c, nct)
            rows = _cat([_cat([btmp_ref[j, pl.ds(part * dm + c5 * dpt + dd, B_HEADS, stride=bdh), :]
                               for j in range(nct)], axis=1) for dd in range(dpt)])
            bqkv_ref[c] = rows.T.astype(BF16)
        for j in range(nct):
            bwo_ref[j] = _cat([btmp_ref[j, pl.ds(3 * dm + d, B_HEADS, stride=bdh), :]
                               for d in range(bdh)]).astype(BF16)

        m0 = mem0_ref[...].astype(F32)
        h_ref[0:n_mem, :] = m0
        h_ref[n_mem:M2, :] = m0
        h_ref[M2:M2 + seg, :] = _ln(x_ref[NPRE:NPRE + seg, :].astype(F32))
        h_ref[M2 + seg:RQ, :] = _ln(x_ref[A0:A0 + AH, :].astype(F32))

    bscale = float(dm // B_HEADS) ** (-0.5)

    def b_qkv():
        yb = xb_ref[...]
        return _nn(_ln(yb).astype(BF16), _cat([bqkv_ref[c] for c in range(3 * nct)], axis=1))

    def b_attn(qkv):
        row = lax.broadcasted_iota(jnp.int32, (seg, 128), 0)
        outs = []
        for l in range(2):
            r0 = l * seg
            pos = row + (t - (1 + 2 * l)) * seg
            for j in range(nct):
                kb_ref[l, j, HIST:HIST + seg, :] = qkv[r0:r0 + seg, dm + j * 128:dm + (j + 1) * 128]
                vb_ref[l, j, HIST:HIST + seg, :] = qkv[r0:r0 + seg, 2 * dm + j * 128:2 * dm + (j + 1) * 128]
            logits = []
            for w in range(B_WIN):
                o = HIST - w * B_DIL
                acc = None
                for j in range(nct):
                    p = qkv[r0:r0 + seg, j * 128:(j + 1) * 128] * kb_ref[l, j, o:o + seg, :]
                    acc = p if acc is None else acc + p
                acc = acc + pltpu.roll(acc, 64, 1)
                acc = acc + pltpu.roll(acc, 32, 1)
                lg = acc * bscale
                if w > 0:
                    lg = jnp.where(pos >= w * B_DIL, lg, NEG)
                logits.append(lg)
            m = logits[0]
            for w in range(1, B_WIN):
                m = jnp.maximum(m, logits[w])
            es = [jnp.exp(lg - m) for lg in logits]
            den = es[0]
            for w in range(1, B_WIN):
                den = den + es[w]
            inv = 1.0 / den
            cols = []
            for j in range(nct):
                acc = None
                for w in range(B_WIN):
                    o = HIST - w * B_DIL
                    p = es[w] * vb_ref[l, j, o:o + seg, :]
                    acc = p if acc is None else acc + p
                cols.append(acc * inv)
            outs.append(_cat(cols, axis=1))
            for j in range(nct):
                kb_ref[l, j, 0:HIST, :] = qkv[r0 + seg - HIST:r0 + seg, dm + j * 128:dm + (j + 1) * 128]
                vb_ref[l, j, 0:HIST, :] = qkv[r0 + seg - HIST:r0 + seg, 2 * dm + j * 128:2 * dm + (j + 1) * 128]
        return _cat(outs, axis=0).astype(BF16)

    def b_out(ob):
        zb = xb_ref[...] + _nn(ob, _cat([bwo_ref[j] for j in range(nct)], axis=1))
        out_ref[...] = zb[seg:2 * seg].astype(out_ref.dtype)
        return zb[0:seg]

    @pl.when(t < n_seg + LAG)
    def _main():
        h = h_ref[...].astype(BF16)
        scale = float(dh) ** (-0.5)
        tc = jnp.minimum(t, n_seg - 1)
        rd = tc * seg
        rd = pl.multiple_of(jnp.where(rd >= RS, rd - RS, rd), seg)
        ws = pl.multiple_of(jnp.where(t < LAG, NPRE + t * seg, RS), 16)
        wa = A0 + t * AH
        wa = jnp.where(wa >= RS, wa - RS, wa)
        wa = pl.multiple_of(jnp.where(t < n_ah, wa, RS + seg), 16)

        def grp_idx(i):
            g1 = ((i >= n_mem) & (i < M2)) | (i >= M2 + seg)
            idx = jnp.where(i < n_mem, i, jnp.where(i < M2 + seg, i - n_mem, i - n_mem - seg))
            return g1, idx
        rg1, qi = grp_idx(lax.broadcasted_iota(jnp.int32, (R, R), 0))
        cg1, ki = grp_idx(lax.broadcasted_iota(jnp.int32, (R, R), 1))
        causal = (qi < n_mem) | (qi >= ki)
        same = rg1 == cg1
        half = dh - 128
        la8 = lax.broadcasted_iota(jnp.int32, (n_mem, 128), 1) < half
        la32 = lax.broadcasted_iota(jnp.int32, (seg, 128), 1) < half
        lau = lax.broadcasted_iota(jnp.int32, (seg // 2, 128), 1) < half
        mask_a = jnp.where(lau, jnp.uint32(0xFFFFFFFF), jnp.uint32(0))
        mask_b = jnp.where(lau, jnp.uint32(0), jnp.uint32(0xFFFFFFFF))

        def proj(p, g):
            base = (g * 3 + p) * 3
            y = _nn(h, _cat([w_ref[base + j] for j in range(3)], axis=1))
            x1 = [ring_ref[base + j, pl.ds(rd, seg), :] for j in range(3)]
            x2 = [y[M2:M2 + seg, j * 128:(j + 1) * 128].astype(BF16) for j in range(3)]
            for j in range(3):
                ring_ref[base + j, pl.ds(ws, seg), :] = x2[j]
                ring_ref[base + j, pl.ds(wa, AH), :] = y[M2 + seg:RQ, j * 128:(j + 1) * 128].astype(BF16)
            return y[0:M2], x1, x2

        def bmask(z, m):
            return pltpu.bitcast(pltpu.bitcast(z, jnp.uint32) & m, BF16)

        def kv_tiles(z):
            ym, x1, x2 = z
            m1 = ym[0:n_mem]
            m2 = ym[n_mem:M2]
            t0 = _cat([ym[:, 0:128].astype(BF16), x1[0], x2[0]])
            t2 = _cat([_cat([m2[:, 256:384], m1[:, 256:384]]).astype(BF16), x2[2], x1[2]])
            a1 = m1[:, 128:256]
            a2 = m2[:, 128:256]
            mid1 = _cat([_cat([jnp.where(la8, a1, 0.0), jnp.where(la8, 0.0, a1)]).astype(BF16),
                         bmask(x1[1], mask_a), bmask(x1[1], mask_b)])
            mid2 = _cat([_cat([jnp.where(la8, 0.0, a2), jnp.where(la8, a2, 0.0)]).astype(BF16),
                         bmask(x2[1], mask_b), bmask(x2[1], mask_a)])
            return t0, mid1, mid2, t2

        def merge_mid(y1, y2):
            return _cat([y1[0:n_mem], y2[n_mem:M2], y1[M2:M2 + seg], y2[M2:M2 + seg]])

        def scores(q, k):
            ym, x1, x2 = q
            qm = [ym[:, j * 128:(j + 1) * 128].astype(BF16) for j in range(3)]
            k0, km1, km2, k2 = kv_tiles(k)
            s_a = _nt(_cat([qm[0], x1[0], x2[0]]), k0)
            s_b = _nt(_cat([qm[2], x1[2], x2[2]]), k2)
            s_1 = _nt(_cat([qm[1], x1[1]]), km1)
            s_2 = _nt(_cat([qm[1], x2[1]]), km2)
            s = (jnp.where(same, s_a, s_b) + merge_mid(s_1, s_2)) * scale
            s = jnp.where(causal, s, NEG)
            m_0 = jnp.max(jnp.where(cg1, -jnp.inf, s), axis=-1, keepdims=True)
            m_1 = jnp.max(jnp.where(cg1, s, -jnp.inf), axis=-1, keepdims=True)
            e = jnp.exp(s - jnp.where(cg1, m_1, m_0))
            d_0 = jnp.sum(jnp.where(cg1, 0.0, e), axis=-1, keepdims=True)
            d_1 = jnp.sum(jnp.where(cg1, e, 0.0), axis=-1, keepdims=True)
            return e / jnp.where(cg1, d_1, d_0)

        def pv(p, v):
            v0, vm1, vm2, v2 = kv_tiles(v)
            o_a = _nn(jnp.where(same, p, 0.0).astype(BF16), v0)
            o_b = _nn(jnp.where(same, 0.0, p).astype(BF16), v2)
            o_1 = _nn(p[0:M2 + seg].astype(BF16), vm1)
            o_2 = _nn(_cat([p[0:M2], p[M2 + seg:R]]).astype(BF16), vm2)
            return _cat([o_a, merge_mid(o_1, o_2), o_b], axis=1).astype(BF16)

        def oproj(o, g):
            return _nn(o, _cat([wo_ref[j, g * PW:(g + 1) * PW, :] for j in range(nct)], axis=1))

        q = proj(0, 0)
        k = proj(1, 0)
        v = proj(2, 0)
        p = scores(q, k)
        bq = b_qkv()
        ob = b_attn(bq)
        acc = None
        for g in range(G - 1):
            q = proj(0, g + 1)
            k = proj(1, g + 1)
            o = pv(p, v)
            v = proj(2, g + 1)
            p = scores(q, k)
            if g < G - 2:
                c = oproj(o, g)
                acc = c if acc is None else acc + c
        x2_new = b_out(ob)
        o_last = pv(p, v)
        acc = acc + oproj(o, G - 2)
        acc = acc + oproj(o_last, G - 1)

        x_cur = x_ref[pl.ds(pl.multiple_of(tc * seg, seg), seg), :].astype(F32)
        an = pl.multiple_of(jnp.minimum(A0 + (t + 1) * AH, S - AH), AH)
        x_ah = x_ref[pl.ds(an, AH), :].astype(F32)
        x_sl = x_ref[NPRE + seg:NPRE + 2 * seg, :].astype(F32)
        xb_ref[0:seg, :] = x_cur + acc[M2:M2 + seg]
        xb_ref[seg:2 * seg, :] = x2_ref[...] + acc[M2 + seg:R]
        x2_ref[...] = x2_new
        h_ref[0:n_mem, :] = acc[0:n_mem]
        h_ref[n_mem:M2, :] = jnp.where(t < LAG, mem0_ref[...].astype(F32), acc[n_mem:M2])
        h_ref[M2:M2 + seg, :] = _ln(jnp.where(t < LAG - 1, x_sl, x2_new))
        h_ref[M2 + seg:RQ, :] = _ln(x_ah)

    @pl.when(t == n_seg + LAG)
    def _tail():
        b_out(b_attn(b_qkv()))


@functools.partial(jax.jit, static_argnames=("A_seg_len",))
def pallas_interleave_layers__memory_aug_recurrent_mem_tr__sliding_local_dilated__prompt_kernel(
    A_x: jax.Array,
    A_mem0: jax.Array,
    A_Wq: jax.Array,
    A_Wk: jax.Array,
    A_Wv: jax.Array,
    A_Wo: jax.Array,
    A_seg_len,
    B_x: jax.Array,
    B_wqkv: jax.Array,
    B_wo: jax.Array,
):
    del B_x
    _, S, dm = A_x.shape
    n_heads, dh = A_Wq.shape[1], A_Wq.shape[2]
    n_mem = A_mem0.shape[1]
    seg = int(A_seg_len)
    n_seg = S // seg
    hd = n_heads * dh
    assert (seg, n_mem, dh, dm % 128, n_heads % 2) == (32, 8, 192, 0, 0)

    x = A_x.reshape(S, dm)
    mem0 = A_mem0.reshape(n_mem, dm)
    wq = jnp.transpose(A_Wq, (1, 2, 0)).reshape(hd, dm)
    wk = jnp.transpose(A_Wk, (1, 2, 0)).reshape(hd, dm)
    wv = jnp.transpose(A_Wv, (1, 2, 0)).reshape(hd, dm)
    wo = A_Wo.reshape(hd, dm)

    a0 = S - (n_seg - 1) * AH
    npre = a0 - LAG * seg
    rs = -(-a0 // seg) * seg

    kern = functools.partial(_kernel, seg=seg, n_seg=n_seg, n_mem=n_mem,
                             n_heads=n_heads, dh=dh, dm=dm)
    hbm = pl.BlockSpec(memory_space=pltpu.HBM)

    out = pl.pallas_call(
        kern,
        grid=(n_seg + LAG + 1,),
        in_specs=[hbm, pl.BlockSpec((n_mem, dm), lambda t: (0, 0)), hbm, hbm, hbm, hbm, hbm, hbm],
        out_specs=pl.BlockSpec((seg, dm), lambda t: (jnp.maximum(t - (LAG + 1), 0), 0)),
        out_shape=jax.ShapeDtypeStruct((S, dm), A_x.dtype),
        scratch_shapes=[
            pltpu.VMEM((S, dm), BF16),
            pltpu.VMEM((3, 3, 2 * dh, dm), BF16),
            pltpu.VMEM((3 * hd // 128, dm, 128), BF16),
            pltpu.VMEM((dm // 128, hd, 128), BF16),
            pltpu.VMEM((dm, 3 * dm), BF16),
            pltpu.VMEM((dm, dm), BF16),
            pltpu.VMEM((dm // 128, 4 * dm, 128), F32),
            pltpu.VMEM((3 * dm // 128, dm, 128), BF16),
            pltpu.VMEM((dm // 128, dm, 128), BF16),
            pltpu.VMEM((npre, dm), BF16),
            pltpu.VMEM((3 * hd // 128, rs + seg + AH, 128), BF16),
            pltpu.VMEM((2 * n_mem + seg + AH, dm), F32),
            pltpu.VMEM((2 * seg, dm), F32),
            pltpu.VMEM((seg, dm), F32),
            pltpu.VMEM((2, dm // 128, HIST + seg, 128), F32),
            pltpu.VMEM((2, dm // 128, HIST + seg, 128), F32),
            pltpu.SemaphoreType.DMA((3, 3)),
            pltpu.SemaphoreType.DMA((4 + dm // 128,)),
        ],
        compiler_params=pltpu.CompilerParams(
            dimension_semantics=("arbitrary",),
            vmem_limit_bytes=120 * 1024 * 1024,
        ),
    )(x, mem0, wq, wk, wv, wo, B_wqkv, B_wo)
    return out.reshape(1, S, dm)
```

```python
import functools

import jax
import jax.numpy as jnp
from jax import lax
import jax.experimental.pallas as pl
import jax.experimental.pallas.tpu as pltpu

F32 = jnp.float32
BF16 = jnp.bfloat16
U32 = jnp.uint32
NEG = -1000000000.0
LN_EPS = 1e-05

B_HEADS = 32
B_WIN = 8
B_DIL = 2
HIST = 16
AH = 16
LAG = 2
NSLOT = 3
WLAG = 2
BOUT_AT = 8


def _ln(x):
    m = jnp.mean(x, axis=-1, keepdims=True)
    c = x - m
    v = jnp.mean(c * c, axis=-1, keepdims=True)
    return c * lax.rsqrt(v + LN_EPS)


def _nt(a, b):
    return lax.dot_general(a, b, (((1,), (1,)), ((), ())), preferred_element_type=F32)


def _nn(a, b):
    return jnp.dot(a, b, preferred_element_type=F32)


def _cat(xs, axis=0):
    return xs[0] if len(xs) == 1 else jnp.concatenate(xs, axis=axis)


def _pk(z):
    return pltpu.bitcast(z, U32)


def _upk(z):
    return pltpu.bitcast(z, BF16)


def _kernel(x_hbm, mem0_hbm, wq_hbm, wk_hbm, wv_hbm, wo_hbm, bqkv_hbm, bwo_hbm,
            out_hbm,
            x_ref, mem0_ref, stage_ref, w_ref, wo_ref, bst1_ref, bst2_ref, btmp_ref, bqkv_ref, bwo_ref,
            xln_ref, ring_ref, h_ref, xb_ref, x2_ref, kb_ref, vb_ref, o_ref,
            sem_w, sem_m, sem_o,
            *, seg, n_seg, n_mem, n_heads, dh, dm):
    S = seg * n_seg
    M2 = 2 * n_mem
    R = M2 + 2 * seg
    RQ = M2 + seg + AH
    PW = 2 * dh
    G = n_heads // 2
    nct = dm // 128
    n_ah = n_seg - 1
    A0 = S - n_ah * AH
    NPRE = A0 - LAG * seg
    RS = -(-A0 // seg) * seg
    bdh = dm // B_HEADS
    w_hbm = (wq_hbm, wk_hbm, wv_hbm, wo_hbm)

    def w_copy(p, g):
        slot = g % NSLOT
        return pltpu.make_async_copy(w_hbm[p].at[pl.ds(g * PW, PW), :],
                                     stage_ref.at[slot, p], sem_w.at[p, slot])

    xa = pltpu.make_async_copy(x_hbm.at[pl.ds(0, NPRE), :], x_ref.at[pl.ds(0, NPRE), :], sem_m.at[0])
    late = [pltpu.make_async_copy(x_hbm.at[pl.ds(NPRE, S - NPRE), :],
                                  x_ref.at[pl.ds(NPRE, S - NPRE), :], sem_m.at[1]),
            pltpu.make_async_copy(bqkv_hbm, bst1_ref, sem_m.at[2]),
            pltpu.make_async_copy(bwo_hbm, bst2_ref, sem_m.at[3]),
            pltpu.make_async_copy(mem0_hbm, mem0_ref, sem_m.at[4])]
    xa.start()
    for p in range(4):
        w_copy(p, 0).start()
    xb_ref[...] = jnp.zeros(xb_ref.shape, F32)
    x2_ref[...] = jnp.zeros(x2_ref.shape, F32)
    kb_ref[...] = jnp.zeros(kb_ref.shape, F32)
    vb_ref[...] = jnp.zeros(vb_ref.shape, F32)
    xa.wait()
    for p in range(4):
        w_copy(p, 1).start()

    r = 0
    while r < NPRE:
        n = min(256, NPRE - r)
        y = _ln(x_ref[r:r + n, :].astype(F32)).astype(BF16)
        for j in range(nct):
            xln_ref[j, r // 2:(r + n) // 2, :] = _pk(y[:, j * 128:(j + 1) * 128])
        r += n

    def pre_wait(g):
        for p in range(4):
            w_copy(p, g).wait()

    def pre_group(g):
        xl = _cat([_upk(xln_ref[j]) for j in range(nct)], axis=1)
        slot = g % NSLOT
        for p in range(3):
            w = stage_ref[slot, p]
            y = _nt(xl, w).astype(BF16)
            wt = w.T
            for j in range(3):
                ring_ref[(g * 3 + p) * 3 + j, 0:NPRE // 2, :] = _pk(y[:, j * 128:(j + 1) * 128])
                w_ref[(g * 3 + p) * 3 + j] = _pk(wt[:, j * 128:(j + 1) * 128])
        w = stage_ref[slot, 3]
        for j in range(nct):
            wo_ref[g * nct + j] = _pk(w[:, j * 128:(j + 1) * 128])

    def pre_body(g, c):
        @pl.when(g + 2 < G)
        def _():
            for p in range(4):
                w_copy(p, g + 2).start()

        @pl.when(g == 1)
        def _():
            for cp in late:
                cp.start()
        pre_wait(g)
        pre_group(g)
        return c
    lax.fori_loop(0, G - 1, pre_body, 0)

    for cp in late:
        cp.wait()
    pre_wait(G - 1)
    for c in range(3 * nct):
        tr = bst1_ref[:, c * 128:(c + 1) * 128].astype(F32).T
        for j in range(nct):
            btmp_ref[j, c * 128:(c + 1) * 128, :] = tr[:, j * 128:(j + 1) * 128]
    for j in range(nct):
        btmp_ref[j, 3 * dm:4 * dm, :] = bst2_ref[:, j * 128:(j + 1) * 128].astype(F32)
    pre_group(G - 1)
    dpt = 128 // B_HEADS
    for c in range(3 * nct):
        part, c5 = divmod(c, nct)
        rows = _cat([_cat([btmp_ref[j, pl.ds(part * dm + c5 * dpt + dd, B_HEADS, stride=bdh), :]
                           for j in range(nct)], axis=1) for dd in range(dpt)])
        bqkv_ref[c] = _pk(rows.T.astype(BF16))
    for j in range(nct):
        bwo_ref[j] = _pk(_cat([btmp_ref[j, pl.ds(3 * dm + d, B_HEADS, stride=bdh), :]
                               for d in range(bdh)]).astype(BF16))

    m0 = mem0_ref[...].astype(F32)
    h_ref[0:n_mem, :] = m0
    h_ref[n_mem:M2, :] = m0
    h_ref[M2:M2 + seg, :] = _ln(x_ref[NPRE:NPRE + seg, :].astype(F32))
    h_ref[M2 + seg:RQ, :] = _ln(x_ref[A0:A0 + AH, :].astype(F32))

    bscale = float(bdh) ** (-0.5)

    def b_lhs(ls):
        return _ln(xb_ref[ls[0] * seg:(ls[-1] + 1) * seg, :]).astype(BF16)

    def b_proj(lhs, part):
        return _nn(lhs, _cat([_upk(bqkv_ref[part * nct + j]) for j in range(nct)], axis=1))

    def b_attn(t, ls, q, k, v):
        row = lax.broadcasted_iota(jnp.int32, (seg, 128), 0)
        outs = []
        for i, l in enumerate(ls):
            r0 = i * seg
            pos = row + (t - (1 + LAG * l)) * seg
            for j in range(nct):
                kb_ref[l, j, HIST:HIST + seg, :] = k[r0:r0 + seg, j * 128:(j + 1) * 128]
                vb_ref[l, j, HIST:HIST + seg, :] = v[r0:r0 + seg, j * 128:(j + 1) * 128]
            logits = []
            for w in range(B_WIN):
                o = HIST - w * B_DIL
                acc = None
                for j in range(nct):
                    p = q[r0:r0 + seg, j * 128:(j + 1) * 128] * kb_ref[l, j, o:o + seg, :]
                    acc = p if acc is None else acc + p
                acc = acc + pltpu.roll(acc, 64, 1)
                acc = acc + pltpu.roll(acc, 32, 1)
                lg = acc * bscale
                if w > 0:
                    lg = jnp.where(pos >= w * B_DIL, lg, NEG)
                logits.append(lg)
            m = logits[0]
            for w in range(1, B_WIN):
                m = jnp.maximum(m, logits[w])
            es = [jnp.exp(lg - m) for lg in logits]
            den = es[0]
            for w in range(1, B_WIN):
                den = den + es[w]
            inv = 1.0 / den
            cols = []
            for j in range(nct):
                acc = None
                for w in range(B_WIN):
                    o = HIST - w * B_DIL
                    p = es[w] * vb_ref[l, j, o:o + seg, :]
                    acc = p if acc is None else acc + p
                cols.append(acc * inv)
            outs.append(_cat(cols, axis=1))
            for j in range(nct):
                kb_ref[l, j, 0:HIST, :] = k[r0 + seg - HIST:r0 + seg, j * 128:(j + 1) * 128]
                vb_ref[l, j, 0:HIST, :] = v[r0 + seg - HIST:r0 + seg, j * 128:(j + 1) * 128]
        return _cat(outs, axis=0).astype(BF16)

    def b_out(t, ls, ob):
        zb = xb_ref[ls[0] * seg:(ls[-1] + 1) * seg, :] + _nn(
            ob, _cat([_upk(bwo_ref[j]) for j in range(nct)], axis=1))
        if 1 in ls:
            ro = pl.multiple_of((t - LAG) * seg, seg)
            o_ref[pl.ds(ro, seg), :] = zb[(len(ls) - 1) * seg:len(ls) * seg].astype(o_ref.dtype)
        return zb[0:seg] if 0 in ls else None

    def out_copy(b):
        ro = pl.multiple_of(b * seg, seg)
        return pltpu.make_async_copy(o_ref.at[pl.ds(ro + seg, seg), :], out_hbm.at[pl.ds(ro, seg), :], sem_o)

    def step(t, mode):
        l1 = mode != "l2"
        l2 = mode != "l1"
        bls = [0] if mode == "l1" else [0, 1]
        nq = RQ if l1 else M2 + seg
        h = h_ref[0:nq, :].astype(BF16)
        scale = float(dh) ** (-0.5)
        if l1:
            rd = t * (seg // 2)
            rd = pl.multiple_of(jnp.where(rd >= RS // 2, rd - RS // 2, rd), seg // 2)
            wa = (A0 + t * AH) // 2
            wa = jnp.where(wa >= RS // 2, wa - RS // 2, wa)
            wa = pl.multiple_of(jnp.where(t < n_ah, wa, RS // 2), AH // 2)
            if not l2:
                ws = pl.multiple_of((NPRE + t * seg) // 2, AH // 2)

        def grp_idx(i):
            g1 = ((i >= n_mem) & (i < M2)) | (i >= M2 + seg)
            idx = jnp.where(i < n_mem, i, jnp.where(i < M2 + seg, i - n_mem, i - n_mem - seg))
            return g1, idx
        RA = R if (l1 and l2) else M2 + seg
        ri = lax.broadcasted_iota(jnp.int32, (RA, R), 0)
        if not l1:
            ri = jnp.where(ri >= M2, ri + seg, ri)
        rg1, qi = grp_idx(ri)
        cg1, ki = grp_idx(lax.broadcasted_iota(jnp.int32, (RA, R), 1))
        causal = (qi < n_mem) | (qi >= ki)
        same = rg1 == cg1
        half = dh - 128
        la8 = lax.broadcasted_iota(jnp.int32, (n_mem, 128), 1) < half
        lau = lax.broadcasted_iota(jnp.int32, (seg // 2, 128), 1) < half
        mask_a = jnp.where(lau, jnp.uint32(0xFFFFFFFF), jnp.uint32(0))
        mask_b = jnp.where(lau, jnp.uint32(0), jnp.uint32(0xFFFFFFFF))

        def proj(p, g):
            base = (g * 3 + p) * 3
            y = _nn(h, _cat([_upk(w_ref[base + j]) for j in range(3)], axis=1))
            xs = [_pk(y[M2:M2 + seg, j * 128:(j + 1) * 128].astype(BF16)) for j in range(3)]
            if l1:
                x1 = [ring_ref[base + j, pl.ds(rd, seg // 2), :] for j in range(3)]
                for j in range(3):
                    if not l2:
                        ring_ref[base + j, pl.ds(ws, seg // 2), :] = xs[j]
                    ring_ref[base + j, pl.ds(wa, AH // 2), :] = _pk(
                        y[M2 + seg:RQ, j * 128:(j + 1) * 128].astype(BF16))
            else:
                x1 = xs
            x2 = xs if l2 else x1
            return y[0:M2], x1, x2

        def rows(mem, x1, x2):
            return _cat([mem] + ([_upk(x1)] if l1 else []) + ([_upk(x2)] if l2 else []))

        def kv_tiles(z):
            ym, x1, x2 = z
            m1 = ym[0:n_mem]
            m2 = ym[n_mem:M2]
            t0 = _cat([ym[:, 0:128].astype(BF16), _upk(x1[0]), _upk(x2[0])])
            t2 = _cat([_cat([m2[:, 256:384], m1[:, 256:384]]).astype(BF16), _upk(x2[2]), _upk(x1[2])])
            a1 = m1[:, 128:256]
            a2 = m2[:, 128:256]
            mid1 = mid2 = None
            if l1:
                mid1 = _cat([_cat([jnp.where(la8, a1, 0.0), jnp.where(la8, 0.0, a1)]).astype(BF16),
                             _upk(x1[1] & mask_a), _upk(x1[1] & mask_b)])
            if l2:
                mid2 = _cat([_cat([jnp.where(la8, 0.0, a2), jnp.where(la8, a2, 0.0)]).astype(BF16),
                             _upk(x2[1] & mask_b), _upk(x2[1] & mask_a)])
            return t0, mid1, mid2, t2

        def merge_mid(y1, y2):
            if y1 is None:
                return y2
            if y2 is None:
                return y1
            return _cat([y1[0:n_mem], y2[n_mem:M2], y1[M2:M2 + seg], y2[M2:M2 + seg]])

        def scores(q, k):
            ym, x1, x2 = q
            qm = [ym[:, j * 128:(j + 1) * 128].astype(BF16) for j in range(3)]
            k0, km1, km2, k2 = kv_tiles(k)
            s_a = _nt(rows(qm[0], x1[0], x2[0]), k0)
            s_b = _nt(rows(qm[2], x1[2], x2[2]), k2)
            s_1 = _nt(_cat([qm[1], _upk(x1[1])]), km1) if l1 else None
            s_2 = _nt(_cat([qm[1], _upk(x2[1])]), km2) if l2 else None
            s = (jnp.where(same, s_a, s_b) + merge_mid(s_1, s_2)) * scale
            s = jnp.where(causal, s, NEG)
            m_0 = jnp.max(jnp.where(cg1, -jnp.inf, s), axis=-1, keepdims=True)
            m_1 = jnp.max(jnp.where(cg1, s, -jnp.inf), axis=-1, keepdims=True)
            e = jnp.exp(s - jnp.where(cg1, m_1, m_0))
            d_0 = jnp.sum(jnp.where(cg1, 0.0, e), axis=-1, keepdims=True)
            d_1 = jnp.sum(jnp.where(cg1, e, 0.0), axis=-1, keepdims=True)
            return e / jnp.where(cg1, d_1, d_0)

        def pv(p, v):
            v0, vm1, vm2, v2 = kv_tiles(v)
            o_a = _nn(jnp.where(same, p, 0.0).astype(BF16), v0)
            o_b = _nn(jnp.where(same, 0.0, p).astype(BF16), v2)
            o_1 = _nn(p[0:M2 + seg].astype(BF16), vm1) if l1 else None
            o_2 = _nn(_cat([p[0:M2], p[RA - seg:RA]]).astype(BF16), vm2) if l2 else None
            return _cat([o_a, merge_mid(o_1, o_2), o_b], axis=1).astype(BF16)

        def oproj(o, g):
            return _nn(o, _cat([_upk(wo_ref[g * nct + j]) for j in range(nct)], axis=1))

        acc = [None]

        def add_o(g):
            c = oproj(os_[g], g)
            acc[0] = c if acc[0] is None else acc[0] + c

        os_ = [None] * G
        bqkv = []
        q = proj(0, 0)
        k = proj(1, 0)
        v = proj(2, 0)
        p = scores(q, k)
        blhs = b_lhs(bls)
        bqkv.append(b_proj(blhs, 0))
        x2_new = None
        for g in range(G - 1):
            q = proj(0, g + 1)
            k = proj(1, g + 1)
            os_[g] = pv(p, v)
            v = proj(2, g + 1)
            p = scores(q, k)
            if g < 2:
                bqkv.append(b_proj(blhs, g + 1))
            if g == 2:
                ob = b_attn(t, bls, *bqkv)
            if g == BOUT_AT:
                x2_new = b_out(t, bls, ob)
            if g - WLAG >= 0:
                add_o(g - WLAG)
        for g in range(G - 1 - WLAG, G - 2):
            add_o(g)
        os_[G - 1] = pv(p, v)
        add_o(G - 2)
        add_o(G - 1)
        acc = acc[0]

        if l1:
            x_cur = x_ref[pl.ds(pl.multiple_of(t * seg, seg), seg), :].astype(F32)
            xb_ref[0:seg, :] = x_cur + acc[M2:M2 + seg]
            h_ref[0:n_mem, :] = acc[0:n_mem]
            an = pl.multiple_of(jnp.minimum(A0 + (t + 1) * AH, S - AH), AH)
            h_ref[M2 + seg:RQ, :] = _ln(x_ref[pl.ds(an, AH), :].astype(F32))
        if l2:
            xb_ref[seg:2 * seg, :] = x2_ref[...] + acc[RA - seg:RA]
            h_ref[n_mem:M2, :] = acc[n_mem:M2]
            nxt = x2_new
        else:
            x_sl = x_ref[NPRE + seg:NPRE + 2 * seg, :].astype(F32)
            nxt = jnp.where(t < LAG - 1, x_sl, x2_new)
        x2_ref[...] = x2_new
        h_ref[M2:M2 + seg, :] = _ln(nxt)

    def loop(lo, hi, mode):
        def body(t, c):
            if mode != "l1":
                @pl.when(t >= LAG + 2)
                def _():
                    out_copy(t - (LAG + 2)).start()
            step(t, mode)
            return c
        lax.fori_loop(lo, hi, body, 0)

    loop(0, LAG, "l1")
    loop(LAG, n_seg, "full")
    loop(n_seg, n_seg + LAG, "l2")
    t_end = n_seg + LAG
    out_copy(t_end - (LAG + 2)).start()
    blhs = b_lhs([1])
    b_out(t_end, [1], b_attn(t_end, [1], *[b_proj(blhs, part) for part in range(3)]))
    out_copy(n_seg - 1).start()
    pltpu.make_async_copy(o_ref.at[pl.ds(seg, S), :], out_hbm, sem_o).wait()


@functools.partial(jax.jit, static_argnames=("A_seg_len",))
def pallas_interleave_layers__memory_aug_recurrent_mem_tr__sliding_local_dilated__prompt_kernel(
    A_x: jax.Array,
    A_mem0: jax.Array,
    A_Wq: jax.Array,
    A_Wk: jax.Array,
    A_Wv: jax.Array,
    A_Wo: jax.Array,
    A_seg_len,
    B_x: jax.Array,
    B_wqkv: jax.Array,
    B_wo: jax.Array,
):
    del B_x
    _, S, dm = A_x.shape
    n_heads, dh = A_Wq.shape[1], A_Wq.shape[2]
    n_mem = A_mem0.shape[1]
    seg = int(A_seg_len)
    n_seg = S // seg
    hd = n_heads * dh
    nct = dm // 128
    assert (seg, n_mem, dh, dm % 128, n_heads % 2) == (32, 8, 192, 0, 0)

    x = A_x.reshape(S, dm)
    mem0 = A_mem0.reshape(n_mem, dm)
    wq = jnp.transpose(A_Wq, (1, 2, 0)).reshape(hd, dm)
    wk = jnp.transpose(A_Wk, (1, 2, 0)).reshape(hd, dm)
    wv = jnp.transpose(A_Wv, (1, 2, 0)).reshape(hd, dm)
    wo = A_Wo.reshape(hd, dm)

    a0 = S - (n_seg - 1) * AH
    npre = a0 - LAG * seg
    rs = -(-a0 // seg) * seg

    kern = functools.partial(_kernel, seg=seg, n_seg=n_seg, n_mem=n_mem,
                             n_heads=n_heads, dh=dh, dm=dm)
    hbm = pl.BlockSpec(memory_space=pltpu.HBM)

    out = pl.pallas_call(
        kern,
        in_specs=[hbm] * 8,
        out_specs=hbm,
        out_shape=jax.ShapeDtypeStruct((S, dm), A_x.dtype),
        scratch_shapes=[
            pltpu.VMEM((S, dm), BF16),
            pltpu.VMEM((n_mem, dm), BF16),
            pltpu.VMEM((NSLOT, 4, 2 * dh, dm), BF16),
            pltpu.VMEM((3 * hd // 128, dm // 2, 128), U32),
            pltpu.VMEM((n_heads // 2 * nct, dh, 128), U32),
            pltpu.VMEM((dm, 3 * dm), BF16),
            pltpu.VMEM((dm, dm), BF16),
            pltpu.VMEM((nct, 4 * dm, 128), F32),
            pltpu.VMEM((3 * nct, dm // 2, 128), U32),
            pltpu.VMEM((nct, dm // 2, 128), U32),
            pltpu.VMEM((nct, npre // 2, 128), U32),
            pltpu.VMEM((3 * hd // 128, (rs + AH) // 2, 128), U32),
            pltpu.VMEM((2 * n_mem + seg + AH, dm), F32),
            pltpu.VMEM((2 * seg, dm), F32),
            pltpu.VMEM((seg, dm), F32),
            pltpu.VMEM((2, nct, HIST + seg, 128), F32),
            pltpu.VMEM((2, nct, HIST + seg, 128), F32),
            pltpu.VMEM((S + seg, dm), A_x.dtype),
            pltpu.SemaphoreType.DMA((4, NSLOT)),
            pltpu.SemaphoreType.DMA((5,)),
            pltpu.SemaphoreType.DMA(()),
        ],
        compiler_params=pltpu.CompilerParams(
            vmem_limit_bytes=120 * 1024 * 1024,
        ),
    )(x, mem0, wq, wk, wv, wo, B_wqkv, B_wo)
    return out.reshape(1, S, dm)
```

```python
import functools

import jax
import jax.numpy as jnp
from jax import lax
import jax.experimental.pallas as pl
import jax.experimental.pallas.tpu as pltpu

F32 = jnp.float32
BF16 = jnp.bfloat16
U32 = jnp.uint32
NEG = -1000000000.0
LN_EPS = 1e-05

B_HEADS = 32
B_WIN = 8
B_DIL = 2
HIST = 16
AH = 16
LAG = 2
NSLOT = 4
WLAG = 2
BOUT_AT = 8


def _ln(x):
    m = jnp.mean(x, axis=-1, keepdims=True)
    c = x - m
    v = jnp.mean(c * c, axis=-1, keepdims=True)
    return c * lax.rsqrt(v + LN_EPS)


def _nt(a, b):
    return lax.dot_general(a, b, (((1,), (1,)), ((), ())), preferred_element_type=F32)


def _nn(a, b):
    return jnp.dot(a, b, preferred_element_type=F32)


def _cat(xs, axis=0):
    return xs[0] if len(xs) == 1 else jnp.concatenate(xs, axis=axis)


def _pk(z):
    return pltpu.bitcast(z, U32)


def _upk(z):
    return pltpu.bitcast(z, BF16)


def _kernel(x_hbm, mem0_hbm, wq_hbm, wk_hbm, wv_hbm, wo_hbm, bqkv_hbm, bwo_hbm,
            out_hbm,
            x_ref, mem0_ref, stage_ref, w_ref, wo_ref, bst1_ref, bst2_ref, btmp_ref, bqkv_ref, bwo_ref,
            xln_ref, ring_ref, h_ref, xb_ref, x2_ref, kb_ref, vb_ref, o_ref,
            sem_w, sem_m, sem_o,
            *, seg, n_seg, n_mem, n_heads, dh, dm):
    S = seg * n_seg
    M2 = 2 * n_mem
    R = M2 + 2 * seg
    RQ = M2 + seg + AH
    PW = 2 * dh
    G = n_heads // 2
    nct = dm // 128
    n_ah = n_seg
    A0 = S - n_ah * AH
    NPRE = A0 - LAG * seg
    RS = A0 + seg
    bdh = dm // B_HEADS
    w_hbm = (wq_hbm, wk_hbm, wv_hbm, wo_hbm)

    def w_copy(p, g):
        slot = g & (NSLOT - 1)
        return pltpu.make_async_copy(w_hbm[p].at[pl.ds(g * PW, PW), :],
                                     stage_ref.at[slot, p], sem_w.at[p, slot])

    xa = pltpu.make_async_copy(x_hbm.at[pl.ds(0, NPRE), :], x_ref.at[pl.ds(0, NPRE), :], sem_m.at[0])
    late = [pltpu.make_async_copy(x_hbm.at[pl.ds(NPRE, S - NPRE), :],
                                  x_ref.at[pl.ds(NPRE, S - NPRE), :], sem_m.at[1]),
            pltpu.make_async_copy(bqkv_hbm, bst1_ref, sem_m.at[2]),
            pltpu.make_async_copy(bwo_hbm, bst2_ref, sem_m.at[3]),
            pltpu.make_async_copy(mem0_hbm, mem0_ref, sem_m.at[4])]
    xa.start()
    for p in range(4):
        w_copy(p, 0).start()
    xb_ref[...] = jnp.zeros(xb_ref.shape, F32)
    x2_ref[...] = jnp.zeros(x2_ref.shape, F32)
    kb_ref[...] = jnp.zeros(kb_ref.shape, F32)
    vb_ref[...] = jnp.zeros(vb_ref.shape, F32)
    xa.wait()
    for p in range(4):
        w_copy(p, 1).start()

    r = 0
    while r < NPRE:
        n = min(256, NPRE - r)
        y = _ln(x_ref[r:r + n, :].astype(F32))
        for j in range(nct):
            xln_ref[j, r // 2:(r + n) // 2, :] = _pk(y[:, j * 128:(j + 1) * 128].astype(BF16))
        r += n

    def pre_wait(g):
        for p in range(4):
            w_copy(p, g).wait()

    def pre_group(g):
        xl = _cat([_upk(xln_ref[j]) for j in range(nct)], axis=1)
        slot = g & (NSLOT - 1)
        for p in range(3):
            w = stage_ref[slot, p]
            y = _nt(xl, w)
            wt = w.T
            for j in range(3):
                ring_ref[(g * 3 + p) * 3 + j, 0:NPRE // 2, :] = _pk(y[:, j * 128:(j + 1) * 128].astype(BF16))
                w_ref[(g * 3 + p) * 3 + j] = _pk(wt[:, j * 128:(j + 1) * 128])
        w = stage_ref[slot, 3]
        for j in range(nct):
            wo_ref[g * nct + j] = _pk(w[:, j * 128:(j + 1) * 128])

    def pre_body(g, c):
        @pl.when(g + 2 < G)
        def _():
            for p in range(4):
                w_copy(p, g + 2).start()

        @pl.when(g == 1)
        def _():
            for cp in late:
                cp.start()
        pre_wait(g)
        pre_group(g)
        return c
    lax.fori_loop(0, G - 1, pre_body, 0)

    for cp in late:
        cp.wait()
    pre_wait(G - 1)
    for c in range(3 * nct):
        tr = bst1_ref[:, c * 128:(c + 1) * 128].astype(F32).T
        for j in range(nct):
            btmp_ref[j, c * 128:(c + 1) * 128, :] = tr[:, j * 128:(j + 1) * 128]
    for j in range(nct):
        btmp_ref[j, 3 * dm:4 * dm, :] = bst2_ref[:, j * 128:(j + 1) * 128].astype(F32)
    pre_group(G - 1)
    dpt = 128 // B_HEADS
    for c in range(3 * nct):
        part, c5 = divmod(c, nct)
        rows = _cat([_cat([btmp_ref[j, pl.ds(part * dm + c5 * dpt + dd, B_HEADS, stride=bdh), :]
                           for j in range(nct)], axis=1) for dd in range(dpt)])
        bqkv_ref[c] = _pk(rows.T.astype(BF16))
    for j in range(nct):
        bwo_ref[j] = _pk(_cat([btmp_ref[j, pl.ds(3 * dm + d, B_HEADS, stride=bdh), :]
                               for d in range(bdh)]).astype(BF16))

    m0 = mem0_ref[...].astype(F32)
    h_ref[0:n_mem, :] = m0
    h_ref[n_mem:M2, :] = m0
    h_ref[M2:M2 + seg, :] = _ln(x_ref[NPRE:NPRE + seg, :].astype(F32))
    h_ref[M2 + seg:RQ, :] = _ln(x_ref[A0:A0 + AH, :].astype(F32))

    bscale = float(bdh) ** (-0.5)

    def b_lhs(ls):
        return _ln(xb_ref[ls[0] * seg:(ls[-1] + 1) * seg, :]).astype(BF16)

    def b_proj(lhs, part):
        return _nn(lhs, _cat([_upk(bqkv_ref[part * nct + j]) for j in range(nct)], axis=1))

    def b_attn(t, ls, q, k, v):
        row = lax.broadcasted_iota(jnp.int32, (seg, 128), 0)
        outs = []
        for i, l in enumerate(ls):
            r0 = i * seg
            pos = row + (t - (1 + LAG * l)) * seg
            for j in range(nct):
                kb_ref[l, j, HIST:HIST + seg, :] = k[r0:r0 + seg, j * 128:(j + 1) * 128]
                vb_ref[l, j, HIST:HIST + seg, :] = v[r0:r0 + seg, j * 128:(j + 1) * 128]
            logits = []
            for w in range(B_WIN):
                o = HIST - w * B_DIL
                acc = None
                for j in range(nct):
                    p = q[r0:r0 + seg, j * 128:(j + 1) * 128] * kb_ref[l, j, o:o + seg, :]
                    acc = p if acc is None else acc + p
                acc = acc + pltpu.roll(acc, 64, 1)
                acc = acc + pltpu.roll(acc, 32, 1)
                lg = acc * bscale
                if w > 0:
                    lg = jnp.where(pos >= w * B_DIL, lg, NEG)
                logits.append(lg)
            m = logits[0]
            for w in range(1, B_WIN):
                m = jnp.maximum(m, logits[w])
            es = [jnp.exp(lg - m) for lg in logits]
            den = es[0]
            for w in range(1, B_WIN):
                den = den + es[w]
            inv = 1.0 / den
            cols = []
            for j in range(nct):
                acc = None
                for w in range(B_WIN):
                    o = HIST - w * B_DIL
                    p = es[w] * vb_ref[l, j, o:o + seg, :]
                    acc = p if acc is None else acc + p
                cols.append(acc * inv)
            outs.append(_cat(cols, axis=1))
            for j in range(nct):
                kb_ref[l, j, 0:HIST, :] = k[r0 + seg - HIST:r0 + seg, j * 128:(j + 1) * 128]
                vb_ref[l, j, 0:HIST, :] = v[r0 + seg - HIST:r0 + seg, j * 128:(j + 1) * 128]
        return _cat(outs, axis=0).astype(BF16)

    def b_out(t, ls, ob):
        zb = xb_ref[ls[0] * seg:(ls[-1] + 1) * seg, :] + _nn(
            ob, _cat([_upk(bwo_ref[j]) for j in range(nct)], axis=1))
        if 1 in ls:
            ro = pl.multiple_of((t - LAG) * seg, seg)
            o_ref[pl.ds(ro, seg), :] = zb[(len(ls) - 1) * seg:len(ls) * seg].astype(o_ref.dtype)
        return zb[0:seg] if 0 in ls else None

    def out_copy(b):
        ro = pl.multiple_of(b * seg, seg)
        return pltpu.make_async_copy(o_ref.at[pl.ds(ro + seg, seg), :], out_hbm.at[pl.ds(ro, seg), :], sem_o)

    def step(t, mode):
        l1 = mode != "l2"
        l2 = mode != "l1"
        bls = [0] if mode == "l1" else [0, 1]
        nq = RQ if l1 else M2 + seg
        h = h_ref[0:nq, :].astype(BF16)
        scale = float(dh) ** (-0.5)
        if l1:
            rd = t * (seg // 2)
            rd = pl.multiple_of(jnp.where(rd >= RS // 2, rd - RS // 2, rd), seg // 2)
            wa = (A0 + t * AH) // 2
            wa = pl.multiple_of(jnp.where(wa >= RS // 2, wa - RS // 2, wa), AH // 2)
            if not l2:
                ws = pl.multiple_of((NPRE + t * seg) // 2, AH // 2)

        def grp_idx(i):
            g1 = ((i >= n_mem) & (i < M2)) | (i >= M2 + seg)
            idx = jnp.where(i < n_mem, i, jnp.where(i < M2 + seg, i - n_mem, i - n_mem - seg))
            return g1, idx
        RA = R if (l1 and l2) else M2 + seg
        ri = lax.broadcasted_iota(jnp.int32, (RA, R), 0)
        if not l1:
            ri = jnp.where(ri >= M2, ri + seg, ri)
        rg1, qi = grp_idx(ri)
        cg1, ki = grp_idx(lax.broadcasted_iota(jnp.int32, (RA, R), 1))
        causal = (qi < n_mem) | (qi >= ki)
        same = rg1 == cg1
        half = dh - 128
        la8 = lax.broadcasted_iota(jnp.int32, (n_mem, 128), 1) < half
        lau = lax.broadcasted_iota(jnp.int32, (seg // 2, 128), 1) < half
        mask_a = jnp.where(lau, jnp.uint32(0xFFFFFFFF), jnp.uint32(0))
        mask_b = jnp.where(lau, jnp.uint32(0), jnp.uint32(0xFFFFFFFF))

        def proj(p, g):
            base = (g * 3 + p) * 3
            y = _nn(h, _cat([_upk(w_ref[base + j]) for j in range(3)], axis=1))
            xs = [_pk(y[M2:M2 + seg, j * 128:(j + 1) * 128].astype(BF16)) for j in range(3)]
            if l1:
                for j in range(3):
                    if not l2:
                        ring_ref[base + j, pl.ds(ws, seg // 2), :] = xs[j]
                    ring_ref[base + j, pl.ds(wa, AH // 2), :] = _pk(
                        y[M2 + seg:RQ, j * 128:(j + 1) * 128].astype(BF16))
                x1 = [ring_ref[base + j, pl.ds(rd, seg // 2), :] for j in range(3)]
            else:
                x1 = xs
            x2 = xs if l2 else x1
            return y[0:M2], x1, x2

        def rows(mem, x1, x2):
            return _cat([mem] + ([_upk(x1)] if l1 else []) + ([_upk(x2)] if l2 else []))

        def kv_tiles(z):
            ym, x1, x2 = z
            m1 = ym[0:n_mem]
            m2 = ym[n_mem:M2]
            t0 = _cat([ym[:, 0:128].astype(BF16), _upk(x1[0]), _upk(x2[0])])
            t2 = _cat([_cat([m2[:, 256:384], m1[:, 256:384]]).astype(BF16), _upk(x2[2]), _upk(x1[2])])
            a1 = m1[:, 128:256]
            a2 = m2[:, 128:256]
            mid1 = mid2 = None
            if l1:
                mid1 = _cat([_cat([jnp.where(la8, a1, 0.0), jnp.where(la8, 0.0, a1)]).astype(BF16),
                             _upk(x1[1] & mask_a), _upk(x1[1] & mask_b)])
            if l2:
                mid2 = _cat([_cat([jnp.where(la8, 0.0, a2), jnp.where(la8, a2, 0.0)]).astype(BF16),
                             _upk(x2[1] & mask_b), _upk(x2[1] & mask_a)])
            return t0, mid1, mid2, t2

        def merge_mid(y1, y2):
            if y1 is None:
                return y2
            if y2 is None:
                return y1
            return _cat([y1[0:n_mem], y2[n_mem:M2], y1[M2:M2 + seg], y2[M2:M2 + seg]])

        def scores(q, k):
            ym, x1, x2 = q
            qm = [ym[:, j * 128:(j + 1) * 128].astype(BF16) for j in range(3)]
            k0, km1, km2, k2 = kv_tiles(k)
            s_a = _nt(rows(qm[0], x1[0], x2[0]), k0)
            s_b = _nt(rows(qm[2], x1[2], x2[2]), k2)
            s_1 = _nt(_cat([qm[1], _upk(x1[1])]), km1) if l1 else None
            s_2 = _nt(_cat([qm[1], _upk(x2[1])]), km2) if l2 else None
            s = (jnp.where(same, s_a, s_b) + merge_mid(s_1, s_2)) * scale
            s = jnp.where(causal, s, NEG)
            m_0 = jnp.max(jnp.where(cg1, -jnp.inf, s), axis=-1, keepdims=True)
            m_1 = jnp.max(jnp.where(cg1, s, -jnp.inf), axis=-1, keepdims=True)
            e = jnp.exp(s - jnp.where(cg1, m_1, m_0))
            d_0 = jnp.sum(jnp.where(cg1, 0.0, e), axis=-1, keepdims=True)
            d_1 = jnp.sum(jnp.where(cg1, e, 0.0), axis=-1, keepdims=True)
            return e / jnp.where(cg1, d_1, d_0)

        def pv(p, v):
            v0, vm1, vm2, v2 = kv_tiles(v)
            o_a = _nn(jnp.where(same, p, 0.0).astype(BF16), v0)
            o_b = _nn(jnp.where(same, 0.0, p).astype(BF16), v2)
            o_1 = _nn(p[0:M2 + seg].astype(BF16), vm1) if l1 else None
            o_2 = _nn(_cat([p[0:M2], p[RA - seg:RA]]).astype(BF16), vm2) if l2 else None
            return _cat([o_a, merge_mid(o_1, o_2), o_b], axis=1).astype(BF16)

        def oproj(o, g):
            return _nn(o, _cat([_upk(wo_ref[g * nct + j]) for j in range(nct)], axis=1))

        acc = [None]

        def add_o(g):
            c = oproj(os_[g], g)
            acc[0] = c if acc[0] is None else acc[0] + c

        os_ = [None] * G
        bqkv = []
        q = proj(0, 0)
        k = proj(1, 0)
        v = proj(2, 0)
        p = scores(q, k)
        blhs = b_lhs(bls)
        bqkv.append(b_proj(blhs, 0))
        x2_new = None
        for g in range(G - 1):
            q = proj(0, g + 1)
            k = proj(1, g + 1)
            os_[g] = pv(p, v)
            v = proj(2, g + 1)
            p = scores(q, k)
            if g < 2:
                bqkv.append(b_proj(blhs, g + 1))
            if g == 2:
                ob = b_attn(t, bls, *bqkv)
            if g == BOUT_AT:
                x2_new = b_out(t, bls, ob)
            if g - WLAG >= 0:
                add_o(g - WLAG)
        for g in range(G - 1 - WLAG, G - 2):
            add_o(g)
        os_[G - 1] = pv(p, v)
        add_o(G - 2)
        add_o(G - 1)
        acc = acc[0]

        if l1:
            x_cur = x_ref[pl.ds(pl.multiple_of(t * seg, seg), seg), :].astype(F32)
            xb_ref[0:seg, :] = x_cur + acc[M2:M2 + seg]
            h_ref[0:n_mem, :] = acc[0:n_mem]
            an = pl.multiple_of(jnp.minimum(A0 + (t + 1) * AH, S - AH), AH)
            h_ref[M2 + seg:RQ, :] = _ln(x_ref[pl.ds(an, AH), :].astype(F32))
        if l2:
            xb_ref[seg:2 * seg, :] = x2_ref[...] + acc[RA - seg:RA]
            h_ref[n_mem:M2, :] = acc[n_mem:M2]
            nxt = x2_new
        else:
            x_sl = x_ref[NPRE + seg:NPRE + 2 * seg, :].astype(F32)
            nxt = jnp.where(t < LAG - 1, x_sl, x2_new)
        x2_ref[...] = x2_new
        h_ref[M2:M2 + seg, :] = _ln(nxt)

    def loop(lo, hi, mode):
        def body(t, c):
            if mode != "l1":
                @pl.when(t >= LAG + 2)
                def _():
                    out_copy(t - (LAG + 2)).start()
            step(t, mode)
            return c
        lax.fori_loop(lo, hi, body, 0)

    loop(0, LAG, "l1")
    loop(LAG, n_seg, "full")
    loop(n_seg, n_seg + LAG, "l2")
    t_end = n_seg + LAG
    out_copy(t_end - (LAG + 2)).start()
    blhs = b_lhs([1])
    b_out(t_end, [1], b_attn(t_end, [1], *[b_proj(blhs, part) for part in range(3)]))
    out_copy(n_seg - 1).start()
    pltpu.make_async_copy(o_ref.at[pl.ds(seg, S), :], out_hbm, sem_o).wait()


@functools.partial(jax.jit, static_argnames=("A_seg_len",))
def pallas_interleave_layers__memory_aug_recurrent_mem_tr__sliding_local_dilated__prompt_kernel(
    A_x: jax.Array,
    A_mem0: jax.Array,
    A_Wq: jax.Array,
    A_Wk: jax.Array,
    A_Wv: jax.Array,
    A_Wo: jax.Array,
    A_seg_len,
    B_x: jax.Array,
    B_wqkv: jax.Array,
    B_wo: jax.Array,
):
    del B_x
    _, S, dm = A_x.shape
    n_heads, dh = A_Wq.shape[1], A_Wq.shape[2]
    n_mem = A_mem0.shape[1]
    seg = int(A_seg_len)
    n_seg = S // seg
    hd = n_heads * dh
    nct = dm // 128
    assert (seg, n_mem, dh, dm % 128, n_heads % 2) == (32, 8, 192, 0, 0)

    x = A_x.reshape(S, dm)
    mem0 = A_mem0.reshape(n_mem, dm)
    wq = jnp.transpose(A_Wq, (1, 2, 0)).reshape(hd, dm)
    wk = jnp.transpose(A_Wk, (1, 2, 0)).reshape(hd, dm)
    wv = jnp.transpose(A_Wv, (1, 2, 0)).reshape(hd, dm)
    wo = A_Wo.reshape(hd, dm)

    a0 = S - n_seg * AH
    npre = a0 - LAG * seg
    rs = a0 + seg

    kern = functools.partial(_kernel, seg=seg, n_seg=n_seg, n_mem=n_mem,
                             n_heads=n_heads, dh=dh, dm=dm)
    hbm = pl.BlockSpec(memory_space=pltpu.HBM)

    out = pl.pallas_call(
        kern,
        in_specs=[hbm] * 8,
        out_specs=hbm,
        out_shape=jax.ShapeDtypeStruct((S, dm), A_x.dtype),
        scratch_shapes=[
            pltpu.VMEM((S, dm), BF16),
            pltpu.VMEM((n_mem, dm), BF16),
            pltpu.VMEM((NSLOT, 4, 2 * dh, dm), BF16),
            pltpu.VMEM((3 * hd // 128, dm // 2, 128), U32),
            pltpu.VMEM((n_heads // 2 * nct, dh, 128), U32),
            pltpu.VMEM((dm, 3 * dm), BF16),
            pltpu.VMEM((dm, dm), BF16),
            pltpu.VMEM((nct, 4 * dm, 128), F32),
            pltpu.VMEM((3 * nct, dm // 2, 128), U32),
            pltpu.VMEM((nct, dm // 2, 128), U32),
            pltpu.VMEM((nct, npre // 2, 128), U32),
            pltpu.VMEM((3 * hd // 128, rs // 2, 128), U32),
            pltpu.VMEM((2 * n_mem + seg + AH, dm), F32),
            pltpu.VMEM((2 * seg, dm), F32),
            pltpu.VMEM((seg, dm), F32),
            pltpu.VMEM((2, nct, HIST + seg, 128), F32),
            pltpu.VMEM((2, nct, HIST + seg, 128), F32),
            pltpu.VMEM((S + seg, dm), A_x.dtype),
            pltpu.SemaphoreType.DMA((4, NSLOT)),
            pltpu.SemaphoreType.DMA((5,)),
            pltpu.SemaphoreType.DMA(()),
        ],
        compiler_params=pltpu.CompilerParams(
            vmem_limit_bytes=120 * 1024 * 1024,
            disable_bounds_checks=True,
        ),
    )(x, mem0, wq, wk, wv, wo, B_wqkv, B_wo)
    return out.reshape(1, S, dm)
```

```python
import functools

import jax
import jax.numpy as jnp
from jax import lax
import jax.experimental.pallas as pl
import jax.experimental.pallas.tpu as pltpu

F32 = jnp.float32
BF16 = jnp.bfloat16
U32 = jnp.uint32
NEG = -1000000000.0
LN_EPS = 1e-05

B_HEADS = 32
B_WIN = 8
B_DIL = 2
HIST = 16
AH = 16
LAG = 2
NSLOT = 4
WLAG = 2
BOUT_AT = 8


def _ln(x):
    m = jnp.mean(x, axis=-1, keepdims=True)
    c = x - m
    v = jnp.mean(c * c, axis=-1, keepdims=True)
    return c * lax.rsqrt(v + LN_EPS)


def _nt(a, b):
    return lax.dot_general(a, b, (((1,), (1,)), ((), ())), preferred_element_type=F32)


def _nn(a, b):
    return jnp.dot(a, b, preferred_element_type=F32)


def _cat(xs, axis=0):
    return xs[0] if len(xs) == 1 else jnp.concatenate(xs, axis=axis)


def _pk(z):
    return pltpu.bitcast(z, U32)


def _upk(z):
    return pltpu.bitcast(z, BF16)


def _kernel(x_hbm, mem0_hbm, wq_hbm, wk_hbm, wv_hbm, wo_hbm, bqkv_hbm, bwo_hbm,
            out_hbm,
            x_ref, mem0_ref, stage_ref, w_ref, wo_ref, bst1_ref, bst2_ref, btmp_ref, bqkv_ref, bwo_ref,
            xln_ref, ring_ref, h_ref, xb_ref, x2_ref, kb_ref, vb_ref, o_ref,
            sem_w, sem_m, sem_o,
            *, seg, n_seg, n_mem, n_heads, dh, dm):
    S = seg * n_seg
    M2 = 2 * n_mem
    R = M2 + 2 * seg
    RQ = M2 + seg + AH
    PW = 2 * dh
    G = n_heads // 2
    nct = dm // 128
    n_ah = n_seg
    A0 = S - n_ah * AH
    NPRE = A0 - LAG * seg
    RS = A0 + seg
    bdh = dm // B_HEADS
    w_hbm = (wq_hbm, wk_hbm, wv_hbm, wo_hbm)

    def w_copy(p, g):
        slot = g & (NSLOT - 1)
        return pltpu.make_async_copy(w_hbm[p].at[pl.ds(g * PW, PW), :],
                                     stage_ref.at[slot, p], sem_w.at[p, slot])

    xa = pltpu.make_async_copy(x_hbm.at[pl.ds(0, NPRE), :], x_ref.at[pl.ds(0, NPRE), :], sem_m.at[0])
    late = [pltpu.make_async_copy(x_hbm.at[pl.ds(NPRE, S - NPRE), :],
                                  x_ref.at[pl.ds(NPRE, S - NPRE), :], sem_m.at[1]),
            pltpu.make_async_copy(bqkv_hbm, bst1_ref, sem_m.at[2]),
            pltpu.make_async_copy(bwo_hbm, bst2_ref, sem_m.at[3]),
            pltpu.make_async_copy(mem0_hbm, mem0_ref, sem_m.at[4])]
    xa.start()
    for p in range(4):
        w_copy(p, 0).start()
    xb_ref[...] = jnp.zeros(xb_ref.shape, F32)
    x2_ref[...] = jnp.zeros(x2_ref.shape, F32)
    kb_ref[...] = jnp.zeros(kb_ref.shape, F32)
    vb_ref[...] = jnp.zeros(vb_ref.shape, F32)
    xa.wait()
    for p in range(4):
        w_copy(p, 1).start()

    r = 0
    while r < NPRE:
        n = min(256, NPRE - r)
        y = _ln(x_ref[r:r + n, :].astype(F32))
        for j in range(nct):
            xln_ref[j, r // 2:(r + n) // 2, :] = _pk(y[:, j * 128:(j + 1) * 128].astype(BF16))
        r += n

    def pre_wait(g):
        for p in range(4):
            w_copy(p, g).wait()

    def pre_group(g):
        xl = _cat([_upk(xln_ref[j]) for j in range(nct)], axis=1)
        slot = g & (NSLOT - 1)
        for p in range(3):
            w = stage_ref[slot, p]
            y = _nt(xl, w)
            wt = w.T
            for j in range(3):
                ring_ref[(g * 3 + p) * 3 + j, 0:NPRE // 2, :] = _pk(y[:, j * 128:(j + 1) * 128].astype(BF16))
                w_ref[(g * 3 + p) * 3 + j] = _pk(wt[:, j * 128:(j + 1) * 128])
        w = stage_ref[slot, 3]
        for j in range(nct):
            wo_ref[g * nct + j] = _pk(w[:, j * 128:(j + 1) * 128])

    def pre_body(g, c):
        @pl.when(g + 2 < G)
        def _():
            for p in range(4):
                w_copy(p, g + 2).start()

        @pl.when(g == 1)
        def _():
            for cp in late:
                cp.start()
        pre_wait(g)
        pre_group(g)
        return c
    lax.fori_loop(0, G - 1, pre_body, 0)

    for cp in late:
        cp.wait()
    pre_wait(G - 1)
    for c in range(3 * nct):
        tr = bst1_ref[:, c * 128:(c + 1) * 128].astype(F32).T
        for j in range(nct):
            btmp_ref[j, c * 128:(c + 1) * 128, :] = tr[:, j * 128:(j + 1) * 128]
    for j in range(nct):
        btmp_ref[j, 3 * dm:4 * dm, :] = bst2_ref[:, j * 128:(j + 1) * 128].astype(F32)
    pre_group(G - 1)
    dpt = 128 // B_HEADS
    for c in range(3 * nct):
        part, c5 = divmod(c, nct)
        rows = _cat([_cat([btmp_ref[j, pl.ds(part * dm + c5 * dpt + dd, B_HEADS, stride=bdh), :]
                           for j in range(nct)], axis=1) for dd in range(dpt)])
        bqkv_ref[c] = _pk(rows.T.astype(BF16))
    for j in range(nct):
        bwo_ref[j] = _pk(_cat([btmp_ref[j, pl.ds(3 * dm + d, B_HEADS, stride=bdh), :]
                               for d in range(bdh)]).astype(BF16))

    m0 = mem0_ref[...].astype(F32)
    def set_slot(val):
        h_ref[n_mem:M2, :] = val[0:n_mem]
        h_ref[M2 + n_mem:M2 + seg, :] = val[n_mem:seg]

    h_ref[0:n_mem, :] = m0
    h_ref[M2:M2 + n_mem, :] = m0
    set_slot(_ln(x_ref[NPRE:NPRE + seg, :].astype(F32)))
    h_ref[M2 + seg:RQ, :] = _ln(x_ref[A0:A0 + AH, :].astype(F32))

    bscale = float(bdh) ** (-0.5)

    def b_lhs(ls):
        return _ln(xb_ref[ls[0] * seg:(ls[-1] + 1) * seg, :]).astype(BF16)

    def b_proj(lhs, part):
        return _nn(lhs, _cat([_upk(bqkv_ref[part * nct + j]) for j in range(nct)], axis=1))

    def b_attn(t, ls, q, k, v):
        row = lax.broadcasted_iota(jnp.int32, (seg, 128), 0)
        outs = []
        for i, l in enumerate(ls):
            r0 = i * seg
            pos = row + (t - (1 + LAG * l)) * seg
            for j in range(nct):
                kb_ref[l, j, HIST:HIST + seg, :] = k[r0:r0 + seg, j * 128:(j + 1) * 128]
                vb_ref[l, j, HIST:HIST + seg, :] = v[r0:r0 + seg, j * 128:(j + 1) * 128]
            logits = []
            for w in range(B_WIN):
                o = HIST - w * B_DIL
                acc = None
                for j in range(nct):
                    p = q[r0:r0 + seg, j * 128:(j + 1) * 128] * kb_ref[l, j, o:o + seg, :]
                    acc = p if acc is None else acc + p
                acc = acc + pltpu.roll(acc, 64, 1)
                acc = acc + pltpu.roll(acc, 32, 1)
                lg = acc * bscale
                if w > 0:
                    lg = jnp.where(pos >= w * B_DIL, lg, NEG)
                logits.append(lg)
            m = logits[0]
            for w in range(1, B_WIN):
                m = jnp.maximum(m, logits[w])
            es = [jnp.exp(lg - m) for lg in logits]
            den = es[0]
            for w in range(1, B_WIN):
                den = den + es[w]
            inv = 1.0 / den
            cols = []
            for j in range(nct):
                acc = None
                for w in range(B_WIN):
                    o = HIST - w * B_DIL
                    p = es[w] * vb_ref[l, j, o:o + seg, :]
                    acc = p if acc is None else acc + p
                cols.append(acc * inv)
            outs.append(_cat(cols, axis=1))
            for j in range(nct):
                kb_ref[l, j, 0:HIST, :] = k[r0 + seg - HIST:r0 + seg, j * 128:(j + 1) * 128]
                vb_ref[l, j, 0:HIST, :] = v[r0 + seg - HIST:r0 + seg, j * 128:(j + 1) * 128]
        return _cat(outs, axis=0).astype(BF16)

    def b_out(t, ls, ob):
        zb = xb_ref[ls[0] * seg:(ls[-1] + 1) * seg, :] + _nn(
            ob, _cat([_upk(bwo_ref[j]) for j in range(nct)], axis=1))
        if 1 in ls:
            ro = pl.multiple_of((t - LAG) * seg, seg)
            o_ref[pl.ds(ro, seg), :] = zb[(len(ls) - 1) * seg:len(ls) * seg].astype(o_ref.dtype)
        return zb[0:seg] if 0 in ls else None

    def out_copy(b):
        ro = pl.multiple_of(b * seg, seg)
        return pltpu.make_async_copy(o_ref.at[pl.ds(ro + seg, seg), :], out_hbm.at[pl.ds(ro, seg), :], sem_o)

    def step(t, mode):
        l1 = mode != "l2"
        l2 = mode != "l1"
        bls = [0] if mode == "l1" else [0, 1]
        nq = RQ if l1 else M2 + seg
        h = h_ref[0:nq, :].astype(BF16)
        scale = float(dh) ** (-0.5)
        if l1:
            rd = t * (seg // 2)
            rd = pl.multiple_of(jnp.where(rd >= RS // 2, rd - RS // 2, rd), seg // 2)
            wa = (A0 + t * AH) // 2
            wa = pl.multiple_of(jnp.where(wa >= RS // 2, wa - RS // 2, wa), AH // 2)
            if not l2:
                ws = pl.multiple_of((NPRE + t * seg) // 2, AH // 2)

        full = l1 and l2
        RA = R if full else M2 + seg
        CW = R + 2 * M2 if full else R
        ri = lax.broadcasted_iota(jnp.int32, (RA, CW), 0)
        ci = lax.broadcasted_iota(jnp.int32, (RA, CW), 1)
        if not l1:
            ri = jnp.where(ri >= M2, ri + seg, ri)

        def table(i, bounds, vals):
            out = vals[-1]
            for b, v in zip(reversed(bounds), reversed(vals[:-1])):
                out = jnp.where(i < b, v, out)
            return out
        qi = ri - table(ri, [16, 48, 56], [0, 8, 48, 40])
        g0 = (ci < 8) | ((ci >= 16) & (ci < 48))
        k1 = ci - table(ci, [8, 48], [0, 8, 40])
        k2 = ci - table(ci, [8, 24, 32, 48, 56, 80, 88, 96, 104], [-8, 0, 24, 8, 48, 40, 72, 80, 96, 104])
        if full:
            row_l2 = ((ri >= 8) & (ri < 16)) | (ri >= 48)
            row_xa = (ri >= 8) & (ri < 16)
            valid = row_xa == (ci >= 80)
            is_a = jnp.where(ci >= 80, ((ci >= 88) & (ci < 104)).astype(jnp.int32),
                             (g0 != row_l2).astype(jnp.int32)) > 0
            ki = jnp.where(row_l2, k2, k1)
            visible = valid & ((qi < n_mem) | (qi >= ki))
            fill = jnp.where(valid, NEG, -jnp.inf)
        else:
            is_a = g0 if l1 else jnp.logical_not(g0)
            ki = k1 if l1 else k2
            visible = (qi < n_mem) | (qi >= ki)
            fill = NEG
        half = dh - 128
        la8 = lax.broadcasted_iota(jnp.int32, (n_mem, 128), 1) < half
        ones = jnp.full((n_mem, 128), 0xFFFFFFFF, U32)
        zero = jnp.zeros((n_mem, 128), U32)
        mask_a = jnp.where(la8, ones, zero)
        mask_b = jnp.where(la8, zero, ones)

        def pk2(a, b):
            return _pk(_cat([a, b]).astype(BF16))

        def proj(p, g):
            base = (g * 3 + p) * 3
            y = _nn(h, _cat([_upk(w_ref[base + j]) for j in range(3)], axis=1))
            yt = [y[:, j * 128:(j + 1) * 128] for j in range(3)]
            x1 = None
            if l1:
                for j in range(3):
                    if not l2:
                        ring_ref[base + j, pl.ds(ws, seg // 2), :] = _cat(
                            [pk2(yt[j][8:16], yt[j][24:32]), pk2(yt[j][32:40], yt[j][40:48])])
                    ring_ref[base + j, pl.ds(wa, AH // 2), :] = pk2(yt[j][48:56], yt[j][56:64])
                x1 = [ring_ref[base + j, pl.ds(rd, seg // 2), :] for j in range(3)]
            return yt, x1

        def groups(z, j):
            y = z[0][j]
            return pk2(y[0:8], y[8:16]), pk2(y[16:24], y[24:32]), pk2(y[32:40], y[40:48])

        def q_rows(z, j):
            v0, v1, v2 = groups(z, j)
            return [v0] + ([z[1][j]] if l1 else []) + ([v1, v2] if l2 else [])

        def kv_tiles(z):
            yt, x1 = z
            v0, v1, v2 = groups(z, 0)
            t0 = [v0] + ([x1[0]] if l1 else [v1, v2]) + ([v1, v2] if l2 else [x1[0]])
            y = yt[2]
            w0 = pk2(y[8:16], y[0:8])
            w1 = pk2(y[24:32], y[16:24])
            w2 = pk2(y[32:40], y[40:48])
            t2 = [w0] + ([w1, w2] if l2 else [x1[2]]) + ([x1[2]] if l1 else [w1, w2])
            if full:
                t0 += [v0, v1]
                t2 += [w0, w1]
            y = yt[1]

            def ab(z8):
                return jnp.where(la8, z8, 0.0), jnp.where(la8, 0.0, z8)
            mid1 = mid2 = None
            if l2:
                xa_a, xa_b = ab(y[8:16])
                e1 = pk2(xa_b, xa_a)
                u2 = pk2(y[32:40], y[40:48])
                mid2 = [e1, pk2(y[24:32], y[16:24]) & mask_b, u2 & mask_b,
                        pk2(y[16:24], y[24:32]) & mask_a, u2 & mask_a]
            if l1:
                lo, hi = x1[1][0:8], x1[1][8:16]
                mid1 = [pk2(*ab(y[0:8])), lo & mask_a, hi & mask_a, lo & mask_b, hi & mask_b]
                if l2:
                    mid1 += [e1, pk2(*ab(y[16:24]))]
            return t0, mid1, mid2, t2

        def mat(parts):
            return _upk(_cat(parts))

        def scores(q, k):
            k0, km1, km2, k2_ = kv_tiles(k)
            s_a = _nt(mat(q_rows(q, 0)), mat(k0))
            s_b = _nt(mat(q_rows(q, 2)), mat(k2_))
            qm = q_rows(q, 1)
            if full:
                s_m = _cat([_nt(mat(qm[0:2]), mat(km1)), _nt(mat(qm[2:4]), mat(km2 + km1[5:7]))])
            else:
                s_m = _nt(mat(qm), mat(km1 if l1 else km2))
            s = (jnp.where(is_a, s_a, s_b) + s_m) * scale
            s = jnp.where(visible, s, fill)
            m_a = jnp.max(jnp.where(is_a, s, -jnp.inf), axis=-1, keepdims=True)
            m_b = jnp.max(jnp.where(is_a, -jnp.inf, s), axis=-1, keepdims=True)
            e = jnp.exp(s - jnp.where(is_a, m_a, m_b))
            d_a = jnp.sum(jnp.where(is_a, e, 0.0), axis=-1, keepdims=True)
            d_b = jnp.sum(jnp.where(is_a, 0.0, e), axis=-1, keepdims=True)
            return e / jnp.where(is_a, d_a, d_b)

        def pv(p, v):
            v0, vm1, vm2, v2 = kv_tiles(v)
            o_a = _nn(jnp.where(is_a, p, 0.0).astype(BF16), mat(v0))
            o_b = _nn(jnp.where(is_a, 0.0, p).astype(BF16), mat(v2))
            if full:
                o_m = _cat([_nn(p[0:M2 + seg].astype(BF16), mat(vm1)),
                            _nn(p[M2 + seg:R, 0:R].astype(BF16), mat(vm2))])
            else:
                o_m = _nn(p.astype(BF16), mat(vm1 if l1 else vm2))
            return _cat([o_a, o_m, o_b], axis=1).astype(BF16)

        def oproj(o, g):
            return _nn(o, _cat([_upk(wo_ref[g * nct + j]) for j in range(nct)], axis=1))

        acc = [None]

        def add_o(g):
            c = oproj(os_[g], g)
            acc[0] = c if acc[0] is None else acc[0] + c

        os_ = [None] * G
        bqkv = []
        q = proj(0, 0)
        k = proj(1, 0)
        v = proj(2, 0)
        p = scores(q, k)
        blhs = b_lhs(bls)
        bqkv.append(b_proj(blhs, 0))
        x2_new = None
        for g in range(G - 1):
            q = proj(0, g + 1)
            k = proj(1, g + 1)
            os_[g] = pv(p, v)
            v = proj(2, g + 1)
            p = scores(q, k)
            if g < 2:
                bqkv.append(b_proj(blhs, g + 1))
            if g == 2:
                ob = b_attn(t, bls, *bqkv)
            if g == BOUT_AT:
                x2_new = b_out(t, bls, ob)
            if g - WLAG >= 0:
                add_o(g - WLAG)
        for g in range(G - 1 - WLAG, G - 2):
            add_o(g)
        os_[G - 1] = pv(p, v)
        add_o(G - 2)
        add_o(G - 1)
        acc = acc[0]

        if l1:
            x_cur = x_ref[pl.ds(pl.multiple_of(t * seg, seg), seg), :].astype(F32)
            xb_ref[0:seg, :] = x_cur + acc[M2:M2 + seg]
            h_ref[0:n_mem, :] = acc[0:n_mem]
            an = pl.multiple_of(jnp.minimum(A0 + (t + 1) * AH, S - AH), AH)
            h_ref[M2 + seg:RQ, :] = _ln(x_ref[pl.ds(an, AH), :].astype(F32))
        if l2:
            xb_ref[seg:2 * seg, :] = x2_ref[...] + _cat([acc[n_mem:M2], acc[RA - seg + n_mem:RA]])
            h_ref[M2:M2 + n_mem, :] = acc[RA - seg:RA - seg + n_mem]
            nxt = x2_new
        else:
            x_sl = x_ref[NPRE + seg:NPRE + 2 * seg, :].astype(F32)
            nxt = jnp.where(t < LAG - 1, x_sl, x2_new)
        x2_ref[...] = x2_new
        set_slot(_ln(nxt))

    def loop(lo, hi, mode):
        def body(t, c):
            if mode != "l1":
                @pl.when(t >= LAG + 2)
                def _():
                    out_copy(t - (LAG + 2)).start()
            step(t, mode)
            return c
        lax.fori_loop(lo, hi, body, 0)

    loop(0, LAG, "l1")
    loop(LAG, n_seg, "full")
    loop(n_seg, n_seg + LAG, "l2")
    t_end = n_seg + LAG
    out_copy(t_end - (LAG + 2)).start()
    blhs = b_lhs([1])
    b_out(t_end, [1], b_attn(t_end, [1], *[b_proj(blhs, part) for part in range(3)]))
    out_copy(n_seg - 1).start()
    pltpu.make_async_copy(o_ref.at[pl.ds(seg, S), :], out_hbm, sem_o).wait()


@functools.partial(jax.jit, static_argnames=("A_seg_len",))
def pallas_interleave_layers__memory_aug_recurrent_mem_tr__sliding_local_dilated__prompt_kernel(
    A_x: jax.Array,
    A_mem0: jax.Array,
    A_Wq: jax.Array,
    A_Wk: jax.Array,
    A_Wv: jax.Array,
    A_Wo: jax.Array,
    A_seg_len,
    B_x: jax.Array,
    B_wqkv: jax.Array,
    B_wo: jax.Array,
):
    del B_x
    _, S, dm = A_x.shape
    n_heads, dh = A_Wq.shape[1], A_Wq.shape[2]
    n_mem = A_mem0.shape[1]
    seg = int(A_seg_len)
    n_seg = S // seg
    hd = n_heads * dh
    nct = dm // 128
    assert (seg, n_mem, dh, dm % 128, n_heads % 2) == (32, 8, 192, 0, 0)

    x = A_x.reshape(S, dm)
    mem0 = A_mem0.reshape(n_mem, dm)
    wq = jnp.transpose(A_Wq, (1, 2, 0)).reshape(hd, dm)
    wk = jnp.transpose(A_Wk, (1, 2, 0)).reshape(hd, dm)
    wv = jnp.transpose(A_Wv, (1, 2, 0)).reshape(hd, dm)
    wo = A_Wo.reshape(hd, dm)

    a0 = S - n_seg * AH
    npre = a0 - LAG * seg
    rs = a0 + seg

    kern = functools.partial(_kernel, seg=seg, n_seg=n_seg, n_mem=n_mem,
                             n_heads=n_heads, dh=dh, dm=dm)
    hbm = pl.BlockSpec(memory_space=pltpu.HBM)

    out = pl.pallas_call(
        kern,
        in_specs=[hbm] * 8,
        out_specs=hbm,
        out_shape=jax.ShapeDtypeStruct((S, dm), A_x.dtype),
        scratch_shapes=[
            pltpu.VMEM((S, dm), BF16),
            pltpu.VMEM((n_mem, dm), BF16),
            pltpu.VMEM((NSLOT, 4, 2 * dh, dm), BF16),
            pltpu.VMEM((3 * hd // 128, dm // 2, 128), U32),
            pltpu.VMEM((n_heads // 2 * nct, dh, 128), U32),
            pltpu.VMEM((dm, 3 * dm), BF16),
            pltpu.VMEM((dm, dm), BF16),
            pltpu.VMEM((nct, 4 * dm, 128), F32),
            pltpu.VMEM((3 * nct, dm // 2, 128), U32),
            pltpu.VMEM((nct, dm // 2, 128), U32),
            pltpu.VMEM((nct, npre // 2, 128), U32),
            pltpu.VMEM((3 * hd // 128, rs // 2, 128), U32),
            pltpu.VMEM((2 * n_mem + seg + AH, dm), F32),
            pltpu.VMEM((2 * seg, dm), F32),
            pltpu.VMEM((seg, dm), F32),
            pltpu.VMEM((2, nct, HIST + seg, 128), F32),
            pltpu.VMEM((2, nct, HIST + seg, 128), F32),
            pltpu.VMEM((S + seg, dm), A_x.dtype),
            pltpu.SemaphoreType.DMA((4, NSLOT)),
            pltpu.SemaphoreType.DMA((5,)),
            pltpu.SemaphoreType.DMA(()),
        ],
        compiler_params=pltpu.CompilerParams(
            vmem_limit_bytes=120 * 1024 * 1024,
            disable_bounds_checks=True,
        ),
    )(x, mem0, wq, wk, wv, wo, B_wqkv, B_wo)
    return out.reshape(1, S, dm)
```

```python
import functools

import jax
import jax.numpy as jnp
from jax import lax
import jax.experimental.pallas as pl
import jax.experimental.pallas.tpu as pltpu

F32 = jnp.float32
BF16 = jnp.bfloat16
U32 = jnp.uint32
NEG = -1000000000.0
LN_EPS = 1e-05

B_HEADS = 32
B_WIN = 8
B_DIL = 2
HIST = 16
AH = 16
LAG = 2
NSLOT = 4
WLAG = 2
BOUT_AT = 8
NXC = 4


def _ln(x):
    m = jnp.mean(x, axis=-1, keepdims=True)
    c = x - m
    v = jnp.mean(c * c, axis=-1, keepdims=True)
    return c * lax.rsqrt(v + LN_EPS)


def _nt(a, b):
    return lax.dot_general(a, b, (((1,), (1,)), ((), ())), preferred_element_type=F32)


def _nn(a, b):
    return jnp.dot(a, b, preferred_element_type=F32)


def _cat(xs, axis=0):
    return xs[0] if len(xs) == 1 else jnp.concatenate(xs, axis=axis)


def _pk(z):
    return pltpu.bitcast(z, U32)


def _upk(z):
    return pltpu.bitcast(z, BF16)


def _kernel(x_hbm, mem0_hbm, wq_hbm, wk_hbm, wv_hbm, wo_hbm, bqkv_hbm, bwo_hbm,
            out_hbm,
            x_ref, mem0_ref, stage_ref, w_ref, wo_ref, bst_ref, btmp_ref, bw_ref,
            xln_ref, ring_ref, h_ref, xb_ref, x2_ref, kb_ref, vb_ref, o_ref,
            sem_w, sem_m, sem_o,
            *, seg, n_seg, n_mem, n_heads, dh, dm):
    S = seg * n_seg
    M2 = 2 * n_mem
    R = M2 + 2 * seg
    RQ = M2 + seg + AH
    PW = 2 * dh
    G = n_heads // 2
    nct = dm // 128
    n_ah = n_seg
    A0 = S - n_ah * AH
    NPRE = A0 - LAG * seg
    RS = A0 + seg
    bdh = dm // B_HEADS
    w_hbm = (wq_hbm, wk_hbm, wv_hbm, wo_hbm)

    def w_copy(p, g):
        slot = g & (NSLOT - 1)
        return pltpu.make_async_copy(w_hbm[p].at[pl.ds(g * PW, PW), :],
                                     stage_ref.at[slot, p], sem_w.at[p // 3, slot])

    def w_wait(g):
        slot = g & (NSLOT - 1)
        buf = stage_ref.at[slot, pl.ds(0, 3)]
        pltpu.make_async_copy(buf, buf, sem_w.at[0, slot]).wait()

    NB1 = 3 * nct
    WO0 = 3 * dm
    DUM = 4 * dm
    XC = NPRE // NXC
    xcs = [pltpu.make_async_copy(x_hbm.at[pl.ds(i * XC, XC), :], x_ref.at[pl.ds(i * XC, XC), :],
                                 sem_m.at[4 + i]) for i in range(NXC)]
    late = [pltpu.make_async_copy(x_hbm.at[pl.ds(NPRE, S - NPRE), :],
                                  x_ref.at[pl.ds(NPRE, S - NPRE), :], sem_m.at[1]),
            pltpu.make_async_copy(mem0_hbm, mem0_ref, sem_m.at[2])]
    bcp = [pltpu.make_async_copy(bqkv_hbm.at[:, pl.ds(c * 128, 128)], bst_ref.at[c], sem_m.at[3])
           for c in range(NB1)]
    bcp += [pltpu.make_async_copy(bwo_hbm.at[:, pl.ds(j * 128, 128)], bst_ref.at[NB1 + j], sem_m.at[3])
            for j in range(nct)]
    for cp in xcs:
        cp.start()
    stage_ref[NSLOT - 1, 3] = jnp.zeros((PW, dm), BF16)
    xb_ref[...] = jnp.zeros(xb_ref.shape, F32)
    x2_ref[...] = jnp.zeros(x2_ref.shape, F32)
    kb_ref[...] = jnp.zeros(kb_ref.shape, F32)
    vb_ref[...] = jnp.zeros(vb_ref.shape, F32)
    bst_ref[NB1 + nct] = jnp.zeros((dm, 128), BF16)
    btmp_ref[:, DUM:, :] = jnp.zeros((nct, btmp_ref.shape[1] - DUM, 128), F32)
    for i in range(NXC):
        xcs[i].wait()
        if i == 0:
            for p in range(3):
                w_copy(p, 0).start()
        y = _ln(x_ref[i * XC:(i + 1) * XC, :].astype(F32))
        for j in range(nct):
            xln_ref[j, i * XC // 2:(i + 1) * XC // 2, :] = _pk(y[:, j * 128:(j + 1) * 128].astype(BF16))

    dpt = 128 // B_HEADS

    def b_stage1(u):
        ok = (u >= 0) & (u < NB1)
        tr = bst_ref[jnp.where(ok, u, NB1 + nct)].astype(F32).T
        r0 = pl.multiple_of(jnp.where(ok, u * 128, DUM), 128)
        for j in range(nct):
            btmp_ref[j, pl.ds(r0, 128), :] = tr[:, j * 128:(j + 1) * 128]

    def b_stage1_wo(u):
        ok = (u >= 0) & (u < nct)
        r0 = pl.multiple_of(jnp.where(ok, WO0, DUM), 128)
        btmp_ref[jnp.where(ok, u, 0), pl.ds(r0, dm), :] = bst_ref[
            jnp.where(ok, NB1 + u, NB1 + nct)].astype(F32)

    def b_stage2(u):
        ok = (u >= 0) & (u < NB1)
        part = (u >= nct).astype(jnp.int32) + (u >= 2 * nct).astype(jnp.int32)
        r0 = jnp.where(ok, part * dm + (u - part * nct) * dpt, DUM)
        rows = _cat([_cat([btmp_ref[j, pl.ds(r0 + dd, B_HEADS, stride=bdh), :]
                           for j in range(nct)], axis=1) for dd in range(dpt)])
        bw_ref[jnp.where(ok, u, NB1 + nct)] = _pk(rows.T.astype(BF16))

    def b_stage2_wo(u):
        ok = (u >= 0) & (u < nct)
        r0 = jnp.where(ok, WO0, DUM)
        jj = jnp.where(ok, u, 0)
        bw_ref[jnp.where(ok, NB1 + u, NB1 + nct)] = _pk(
            _cat([btmp_ref[jj, pl.ds(r0 + d, B_HEADS, stride=bdh), :] for d in range(bdh)]).astype(BF16))

    def wo_store(g, dst):
        w = stage_ref[g & (NSLOT - 1), 3]
        for j in range(nct):
            wo_ref[dst * nct + j] = _pk(w[:, j * 128:(j + 1) * 128])

    def pre_body(g, c):
        w_wait(g)

        @pl.when(g >= 1)
        def _():
            w_copy(3, g - 1).wait()

        @pl.when(g == 3)
        def _():
            buf = bst_ref.at[pl.ds(0, NB1 + nct)]
            pltpu.make_async_copy(buf, buf, sem_m.at[3]).wait()

        @pl.when(g == 0)
        def _():
            for p in range(3):
                w_copy(p, 1).start()
            w_copy(3, 0).start()

        @pl.when(g + 2 < G)
        def _():
            for p in range(3):
                w_copy(p, g + 2).start()

        @pl.when(g + 1 < G)
        def _():
            w_copy(3, g + 1).start()

        @pl.when(g == 1)
        def _():
            for cp in bcp + late:
                cp.start()

        slot = g & (NSLOT - 1)
        wo_store(g - 1, jnp.where(g >= 1, g - 1, G - 1))
        b_stage2(2 * (g - 8))
        b_stage2(2 * (g - 8) + 1)
        b_stage2_wo(g - 8)
        b_stage1(2 * (g - 3))
        b_stage1(2 * (g - 3) + 1)
        b_stage1_wo(g - 3)
        xl = _cat([_upk(xln_ref[j]) for j in range(nct)], axis=1)
        for p in range(3):
            w = stage_ref[slot, p]
            wt = w.T
            y = _nt(xl, w) if p < 2 else _nn(xl, wt)
            for j in range(3):
                ring_ref[(g * 3 + p) * 3 + j, 0:NPRE // 2, :] = _pk(y[:, j * 128:(j + 1) * 128].astype(BF16))
                w_ref[(g * 3 + p) * 3 + j] = _pk(wt[:, j * 128:(j + 1) * 128])
        return c
    lax.fori_loop(0, G, pre_body, 0)
    w_copy(3, G - 1).wait()
    for cp in late:
        cp.wait()
    wo_store(G - 1, G - 1)

    m0 = mem0_ref[...].astype(F32)
    def set_slot(val):
        h_ref[n_mem:M2, :] = val[0:n_mem]
        h_ref[M2 + n_mem:M2 + seg, :] = val[n_mem:seg]

    h_ref[0:n_mem, :] = m0
    h_ref[M2:M2 + n_mem, :] = m0
    set_slot(_ln(x_ref[NPRE:NPRE + seg, :].astype(F32)))
    h_ref[M2 + seg:RQ, :] = _ln(x_ref[A0:A0 + AH, :].astype(F32))

    bscale = float(bdh) ** (-0.5)

    def b_lhs(ls):
        return _ln(xb_ref[ls[0] * seg:(ls[-1] + 1) * seg, :]).astype(BF16)

    def b_proj(lhs, part):
        return _nn(lhs, _cat([_upk(bw_ref[part * nct + j]) for j in range(nct)], axis=1))

    def b_attn(t, ls, q, k, v):
        row = lax.broadcasted_iota(jnp.int32, (seg, 128), 0)
        outs = []
        for i, l in enumerate(ls):
            r0 = i * seg
            pos = row + (t - (1 + LAG * l)) * seg
            for j in range(nct):
                kb_ref[l, j, HIST:HIST + seg, :] = k[r0:r0 + seg, j * 128:(j + 1) * 128]
                vb_ref[l, j, HIST:HIST + seg, :] = v[r0:r0 + seg, j * 128:(j + 1) * 128]
            logits = []
            for w in range(B_WIN):
                o = HIST - w * B_DIL
                acc = None
                for j in range(nct):
                    p = q[r0:r0 + seg, j * 128:(j + 1) * 128] * kb_ref[l, j, o:o + seg, :]
                    acc = p if acc is None else acc + p
                acc = acc + pltpu.roll(acc, 64, 1)
                acc = acc + pltpu.roll(acc, 32, 1)
                lg = acc * bscale
                if w > 0:
                    lg = jnp.where(pos >= w * B_DIL, lg, NEG)
                logits.append(lg)
            m = logits[0]
            for w in range(1, B_WIN):
                m = jnp.maximum(m, logits[w])
            es = [jnp.exp(lg - m) for lg in logits]
            den = es[0]
            for w in range(1, B_WIN):
                den = den + es[w]
            inv = 1.0 / den
            cols = []
            for j in range(nct):
                acc = None
                for w in range(B_WIN):
                    o = HIST - w * B_DIL
                    p = es[w] * vb_ref[l, j, o:o + seg, :]
                    acc = p if acc is None else acc + p
                cols.append(acc * inv)
            outs.append(_cat(cols, axis=1))
            for j in range(nct):
                kb_ref[l, j, 0:HIST, :] = k[r0 + seg - HIST:r0 + seg, j * 128:(j + 1) * 128]
                vb_ref[l, j, 0:HIST, :] = v[r0 + seg - HIST:r0 + seg, j * 128:(j + 1) * 128]
        return _cat(outs, axis=0).astype(BF16)

    def b_out(t, ls, ob):
        zb = xb_ref[ls[0] * seg:(ls[-1] + 1) * seg, :] + _nn(
            ob, _cat([_upk(bw_ref[NB1 + j]) for j in range(nct)], axis=1))
        if 1 in ls:
            ro = pl.multiple_of((t - LAG) * seg, seg)
            o_ref[pl.ds(ro, seg), :] = zb[(len(ls) - 1) * seg:len(ls) * seg].astype(o_ref.dtype)
        return zb[0:seg] if 0 in ls else None

    def out_copy(b):
        ro = pl.multiple_of(b * seg, seg)
        return pltpu.make_async_copy(o_ref.at[pl.ds(ro + seg, seg), :], out_hbm.at[pl.ds(ro, seg), :], sem_o)

    def step(t, mode):
        l1 = mode != "l2"
        l2 = mode != "l1"
        bls = [0] if mode == "l1" else [0, 1]
        nq = RQ if l1 else M2 + seg
        h = h_ref[0:nq, :].astype(BF16)
        scale = float(dh) ** (-0.5)
        if l1:
            rd = t * (seg // 2)
            rd = pl.multiple_of(jnp.where(rd >= RS // 2, rd - RS // 2, rd), seg // 2)
            wa = (A0 + t * AH) // 2
            wa = pl.multiple_of(jnp.where(wa >= RS // 2, wa - RS // 2, wa), AH // 2)
            if not l2:
                ws = pl.multiple_of((NPRE + t * seg) // 2, AH // 2)

        full = l1 and l2
        RA = R if full else M2 + seg
        CW = R + 2 * M2 if full else R
        ri = lax.broadcasted_iota(jnp.int32, (RA, CW), 0)
        ci = lax.broadcasted_iota(jnp.int32, (RA, CW), 1)
        if not l1:
            ri = jnp.where(ri >= M2, ri + seg, ri)

        def table(i, bounds, vals):
            out = vals[-1]
            for b, v in zip(reversed(bounds), reversed(vals[:-1])):
                out = jnp.where(i < b, v, out)
            return out
        qi = ri - table(ri, [16, 48, 56], [0, 8, 48, 40])
        g0 = (ci < 8) | ((ci >= 16) & (ci < 48))
        k1 = ci - table(ci, [8, 48], [0, 8, 40])
        k2 = ci - table(ci, [8, 24, 32, 48, 56, 80, 88, 96, 104], [-8, 0, 24, 8, 48, 40, 72, 80, 96, 104])
        if full:
            row_l2 = ((ri >= 8) & (ri < 16)) | (ri >= 48)
            row_xa = (ri >= 8) & (ri < 16)
            valid = row_xa == (ci >= 80)
            is_a = jnp.where(ci >= 80, ((ci >= 88) & (ci < 104)).astype(jnp.int32),
                             (g0 != row_l2).astype(jnp.int32)) > 0
            ki = jnp.where(row_l2, k2, k1)
            visible = valid & ((qi < n_mem) | (qi >= ki))
            fill = jnp.where(valid, NEG, -jnp.inf)
        else:
            is_a = g0 if l1 else jnp.logical_not(g0)
            ki = k1 if l1 else k2
            visible = (qi < n_mem) | (qi >= ki)
            fill = NEG
        half = dh - 128
        la8 = lax.broadcasted_iota(jnp.int32, (n_mem, 128), 1) < half
        ones = jnp.full((n_mem, 128), 0xFFFFFFFF, U32)
        zero = jnp.zeros((n_mem, 128), U32)
        mask_a = jnp.where(la8, ones, zero)
        mask_b = jnp.where(la8, zero, ones)

        def pk2(a, b):
            return _pk(_cat([a, b]).astype(BF16))

        def proj(p, g):
            base = (g * 3 + p) * 3
            y = _nn(h, _cat([_upk(w_ref[base + j]) for j in range(3)], axis=1))
            yt = [y[:, j * 128:(j + 1) * 128] for j in range(3)]
            x1 = None
            if l1:
                for j in range(3):
                    if not l2:
                        ring_ref[base + j, pl.ds(ws, seg // 2), :] = _cat(
                            [pk2(yt[j][8:16], yt[j][24:32]), pk2(yt[j][32:40], yt[j][40:48])])
                    ring_ref[base + j, pl.ds(wa, AH // 2), :] = pk2(yt[j][48:56], yt[j][56:64])
                x1 = [ring_ref[base + j, pl.ds(rd, seg // 2), :] for j in range(3)]
            return yt, x1

        def groups(z, j):
            y = z[0][j]
            return pk2(y[0:8], y[8:16]), pk2(y[16:24], y[24:32]), pk2(y[32:40], y[40:48])

        def q_rows(z, j):
            v0, v1, v2 = groups(z, j)
            return [v0] + ([z[1][j]] if l1 else []) + ([v1, v2] if l2 else [])

        def kv_tiles(z):
            yt, x1 = z
            v0, v1, v2 = groups(z, 0)
            t0 = [v0] + ([x1[0]] if l1 else [v1, v2]) + ([v1, v2] if l2 else [x1[0]])
            y = yt[2]
            w0 = pk2(y[8:16], y[0:8])
            w1 = pk2(y[24:32], y[16:24])
            w2 = pk2(y[32:40], y[40:48])
            t2 = [w0] + ([w1, w2] if l2 else [x1[2]]) + ([x1[2]] if l1 else [w1, w2])
            if full:
                t0 += [v0, v1]
                t2 += [w0, w1]
            y = yt[1]

            def ab(z8):
                return jnp.where(la8, z8, 0.0), jnp.where(la8, 0.0, z8)
            mid1 = mid2 = None
            if l2:
                xa_a, xa_b = ab(y[8:16])
                e1 = pk2(xa_b, xa_a)
                u2 = pk2(y[32:40], y[40:48])
                mid2 = [e1, pk2(y[24:32], y[16:24]) & mask_b, u2 & mask_b,
                        pk2(y[16:24], y[24:32]) & mask_a, u2 & mask_a]
            if l1:
                lo, hi = x1[1][0:8], x1[1][8:16]
                mid1 = [pk2(*ab(y[0:8])), lo & mask_a, hi & mask_a, lo & mask_b, hi & mask_b]
                if l2:
                    mid1 += [e1, pk2(*ab(y[16:24]))]
            return t0, mid1, mid2, t2

        def mat(parts):
            return _upk(_cat(parts))

        def scores(q, k):
            k0, km1, km2, k2_ = kv_tiles(k)
            s_a = _nt(mat(q_rows(q, 0)), mat(k0))
            s_b = _nt(mat(q_rows(q, 2)), mat(k2_))
            qm = q_rows(q, 1)
            if full:
                s_m = _cat([_nt(mat(qm[0:2]), mat(km1)), _nt(mat(qm[2:4]), mat(km2 + km1[5:7]))])
            else:
                s_m = _nt(mat(qm), mat(km1 if l1 else km2))
            s = (jnp.where(is_a, s_a, s_b) + s_m) * scale
            s = jnp.where(visible, s, fill)
            m_a = jnp.max(jnp.where(is_a, s, -jnp.inf), axis=-1, keepdims=True)
            m_b = jnp.max(jnp.where(is_a, -jnp.inf, s), axis=-1, keepdims=True)
            e = jnp.exp(s - jnp.where(is_a, m_a, m_b))
            d_a = jnp.sum(jnp.where(is_a, e, 0.0), axis=-1, keepdims=True)
            d_b = jnp.sum(jnp.where(is_a, 0.0, e), axis=-1, keepdims=True)
            return e / jnp.where(is_a, d_a, d_b)

        def pv(p, v):
            v0, vm1, vm2, v2 = kv_tiles(v)
            o_a = _nn(jnp.where(is_a, p, 0.0).astype(BF16), mat(v0))
            o_b = _nn(jnp.where(is_a, 0.0, p).astype(BF16), mat(v2))
            if full:
                o_m = _cat([_nn(p[0:M2 + seg].astype(BF16), mat(vm1)),
                            _nn(p[M2 + seg:R, 0:R].astype(BF16), mat(vm2))])
            else:
                o_m = _nn(p.astype(BF16), mat(vm1 if l1 else vm2))
            return _cat([o_a, o_m, o_b], axis=1).astype(BF16)

        def oproj(o, g):
            return _nn(o, _cat([_upk(wo_ref[g * nct + j]) for j in range(nct)], axis=1))

        acc = [None]

        def add_o(g):
            c = oproj(os_[g], g)
            acc[0] = c if acc[0] is None else acc[0] + c

        os_ = [None] * G
        bqkv = []
        q = proj(0, 0)
        k = proj(1, 0)
        v = proj(2, 0)
        p = scores(q, k)
        blhs = b_lhs(bls)
        bqkv.append(b_proj(blhs, 0))
        x2_new = None
        for g in range(G - 1):
            q = proj(0, g + 1)
            k = proj(1, g + 1)
            os_[g] = pv(p, v)
            v = proj(2, g + 1)
            p = scores(q, k)
            if g < 2:
                bqkv.append(b_proj(blhs, g + 1))
            if g == 2:
                ob = b_attn(t, bls, *bqkv)
            if g == BOUT_AT:
                x2_new = b_out(t, bls, ob)
            if g - WLAG >= 0:
                add_o(g - WLAG)
        for g in range(G - 1 - WLAG, G - 2):
            add_o(g)
        os_[G - 1] = pv(p, v)
        add_o(G - 2)
        add_o(G - 1)
        acc = acc[0]

        if l1:
            x_cur = x_ref[pl.ds(pl.multiple_of(t * seg, seg), seg), :].astype(F32)
            xb_ref[0:seg, :] = x_cur + acc[M2:M2 + seg]
            h_ref[0:n_mem, :] = acc[0:n_mem]
            an = pl.multiple_of(jnp.minimum(A0 + (t + 1) * AH, S - AH), AH)
            h_ref[M2 + seg:RQ, :] = _ln(x_ref[pl.ds(an, AH), :].astype(F32))
        if l2:
            xb_ref[seg:2 * seg, :] = x2_ref[...] + _cat([acc[n_mem:M2], acc[RA - seg + n_mem:RA]])
            h_ref[M2:M2 + n_mem, :] = acc[RA - seg:RA - seg + n_mem]
            nxt = x2_new
        else:
            x_sl = x_ref[NPRE + seg:NPRE + 2 * seg, :].astype(F32)
            nxt = jnp.where(t < LAG - 1, x_sl, x2_new)
        x2_ref[...] = x2_new
        set_slot(_ln(nxt))

    def loop(lo, hi, mode):
        def body(t, c):
            if mode != "l1":
                @pl.when(t >= LAG + 2)
                def _():
                    out_copy(t - (LAG + 2)).start()
            step(t, mode)
            return c
        lax.fori_loop(lo, hi, body, 0)

    loop(0, LAG, "l1")
    loop(LAG, n_seg, "full")
    loop(n_seg, n_seg + LAG, "l2")
    t_end = n_seg + LAG
    out_copy(t_end - (LAG + 2)).start()
    blhs = b_lhs([1])
    b_out(t_end, [1], b_attn(t_end, [1], *[b_proj(blhs, part) for part in range(3)]))
    out_copy(n_seg - 1).start()
    pltpu.make_async_copy(o_ref.at[pl.ds(seg, S), :], out_hbm, sem_o).wait()


@functools.partial(jax.jit, static_argnames=("A_seg_len",))
def pallas_interleave_layers__memory_aug_recurrent_mem_tr__sliding_local_dilated__prompt_kernel(
    A_x: jax.Array,
    A_mem0: jax.Array,
    A_Wq: jax.Array,
    A_Wk: jax.Array,
    A_Wv: jax.Array,
    A_Wo: jax.Array,
    A_seg_len,
    B_x: jax.Array,
    B_wqkv: jax.Array,
    B_wo: jax.Array,
):
    del B_x
    _, S, dm = A_x.shape
    n_heads, dh = A_Wq.shape[1], A_Wq.shape[2]
    n_mem = A_mem0.shape[1]
    seg = int(A_seg_len)
    n_seg = S // seg
    hd = n_heads * dh
    nct = dm // 128
    assert (seg, n_mem, dh, dm % 128, n_heads % 2) == (32, 8, 192, 0, 0)

    x = A_x.reshape(S, dm)
    mem0 = A_mem0.reshape(n_mem, dm)
    wq = jnp.transpose(A_Wq, (1, 2, 0)).reshape(hd, dm)
    wk = jnp.transpose(A_Wk, (1, 2, 0)).reshape(hd, dm)
    wv = jnp.transpose(A_Wv, (1, 2, 0)).reshape(hd, dm)
    wo = A_Wo.reshape(hd, dm)

    a0 = S - n_seg * AH
    npre = a0 - LAG * seg
    rs = a0 + seg

    kern = functools.partial(_kernel, seg=seg, n_seg=n_seg, n_mem=n_mem,
                             n_heads=n_heads, dh=dh, dm=dm)
    hbm = pl.BlockSpec(memory_space=pltpu.HBM)

    out = pl.pallas_call(
        kern,
        in_specs=[hbm] * 8,
        out_specs=hbm,
        out_shape=jax.ShapeDtypeStruct((S, dm), A_x.dtype),
        scratch_shapes=[
            pltpu.VMEM((S, dm), BF16),
            pltpu.VMEM((n_mem, dm), BF16),
            pltpu.VMEM((NSLOT, 4, 2 * dh, dm), BF16),
            pltpu.VMEM((3 * hd // 128, dm // 2, 128), U32),
            pltpu.VMEM((n_heads // 2 * nct, dh, 128), U32),
            pltpu.VMEM((4 * nct + 1, dm, 128), BF16),
            pltpu.VMEM((nct, 5 * dm + 32, 128), F32),
            pltpu.VMEM((4 * nct + 1, dm // 2, 128), U32),
            pltpu.VMEM((nct, npre // 2, 128), U32),
            pltpu.VMEM((3 * hd // 128, rs // 2, 128), U32),
            pltpu.VMEM((2 * n_mem + seg + AH, dm), F32),
            pltpu.VMEM((2 * seg, dm), F32),
            pltpu.VMEM((seg, dm), F32),
            pltpu.VMEM((2, nct, HIST + seg, 128), F32),
            pltpu.VMEM((2, nct, HIST + seg, 128), F32),
            pltpu.VMEM((S + seg, dm), A_x.dtype),
            pltpu.SemaphoreType.DMA((2, NSLOT)),
            pltpu.SemaphoreType.DMA((4 + NXC,)),
            pltpu.SemaphoreType.DMA(()),
        ],
        compiler_params=pltpu.CompilerParams(
            vmem_limit_bytes=120 * 1024 * 1024,
            disable_bounds_checks=True,
        ),
    )(x, mem0, wq, wk, wv, wo, B_wqkv, B_wo)
    return out.reshape(1, S, dm)
```

```python
import functools

import jax
import jax.numpy as jnp
from jax import lax
import jax.experimental.pallas as pl
import jax.experimental.pallas.tpu as pltpu

F32 = jnp.float32
BF16 = jnp.bfloat16
U32 = jnp.uint32
NEG = -1000000000.0
LN_EPS = 1e-05

B_HEADS = 32
B_WIN = 8
B_DIL = 2
HIST = 16
AH = 16
LAG = 2
NSLOT = 4
WLAG = 2
BOUT_AT = 8
NXC = 4
UNROLL = 2


def _ln(x):
    m = jnp.mean(x, axis=-1, keepdims=True)
    c = x - m
    v = jnp.mean(c * c, axis=-1, keepdims=True)
    return c * lax.rsqrt(v + LN_EPS)


def _nt(a, b):
    return lax.dot_general(a, b, (((1,), (1,)), ((), ())), preferred_element_type=F32)


def _nn(a, b):
    return jnp.dot(a, b, preferred_element_type=F32)


def _cat(xs, axis=0):
    return xs[0] if len(xs) == 1 else jnp.concatenate(xs, axis=axis)


def _pk(z):
    return pltpu.bitcast(z, U32)


def _upk(z):
    return pltpu.bitcast(z, BF16)


def _plan(seg, n_seg):
    S = seg * n_seg
    R0 = LAG * seg
    A0 = S - (n_seg - LAG) * AH
    NPRE = A0 - R0
    RS = NPRE + seg
    XC = -(-(A0 + AH) // (16 * NXC)) * 16
    return S, R0, A0, NPRE, RS, XC


def _kernel(x_hbm, mem0_hbm, wq_hbm, wk_hbm, wv_hbm, wo_hbm, bqkv_hbm, bwo_hbm,
            out_hbm,
            x_ref, mem0_ref, stage_ref, w_ref, wo_ref, bst_ref, btmp_ref, bw_ref,
            xln_ref, ring_ref, h_ref, xb_ref, x2_ref, kb_ref, vb_ref, o_ref,
            sem_w, sem_m, sem_o,
            *, seg, n_seg, n_mem, n_heads, dh, dm):
    S, R0, A0, NPRE, RS, XC = _plan(seg, n_seg)
    M2 = 2 * n_mem
    R = M2 + 2 * seg
    RQ = M2 + seg + AH
    PW = 2 * dh
    G = n_heads // 2
    nct = dm // 128
    bdh = dm // B_HEADS
    w_hbm = (wq_hbm, wk_hbm, wv_hbm, wo_hbm)

    def w_copy(p, g):
        slot = g & (NSLOT - 1)
        return pltpu.make_async_copy(w_hbm[p].at[pl.ds(g * PW, PW), :],
                                     stage_ref.at[slot, p], sem_w.at[p // 3, slot])

    def w_wait(g):
        slot = g & (NSLOT - 1)
        buf = stage_ref.at[slot, pl.ds(0, 3)]
        pltpu.make_async_copy(buf, buf, sem_w.at[0, slot]).wait()

    NB1 = 3 * nct
    WO0 = 3 * dm
    DUM = 4 * dm
    XF = NXC * XC

    def x_copy(i):
        r0 = pl.multiple_of(i * XC, 16)
        return pltpu.make_async_copy(x_hbm.at[pl.ds(r0, XC), :], x_ref.at[pl.ds(r0, XC), :], sem_m.at[3 + i])

    x_late = pltpu.make_async_copy(x_hbm.at[pl.ds(XF, S - XF), :], x_ref.at[pl.ds(XF, S - XF), :], sem_m.at[0])
    m_copy = pltpu.make_async_copy(mem0_hbm, mem0_ref, sem_m.at[1])
    bcp = [pltpu.make_async_copy(bqkv_hbm.at[:, pl.ds(c * 128, 128)], bst_ref.at[c], sem_m.at[2])
           for c in range(NB1)]
    bcp += [pltpu.make_async_copy(bwo_hbm.at[:, pl.ds(j * 128, 128)], bst_ref.at[NB1 + j], sem_m.at[2])
            for j in range(nct)]
    for i in range(NXC):
        x_copy(i).start()
    m_copy.start()
    stage_ref[NSLOT - 1, 3] = jnp.zeros((PW, dm), BF16)
    xb_ref[...] = jnp.zeros(xb_ref.shape, F32)
    kb_ref[...] = jnp.zeros(kb_ref.shape, F32)
    vb_ref[...] = jnp.zeros(vb_ref.shape, F32)
    bst_ref[NB1 + nct] = jnp.zeros((dm, 128), BF16)

    def zero_body(j, c):
        btmp_ref[j, DUM:, :] = jnp.zeros((btmp_ref.shape[1] - DUM, 128), F32)
        return c
    lax.fori_loop(0, nct, zero_body, 0)

    def ln_body(i, c):
        x_copy(i).wait()

        @pl.when(i == 0)
        def _():
            for p in range(3):
                w_copy(p, 0).start()
        y = _ln(x_ref[pl.ds(pl.multiple_of(i * XC, 16), XC), :].astype(F32))
        r0 = pl.multiple_of(i * (XC // 2), 8)
        for j in range(nct):
            xln_ref[j, pl.ds(r0, XC // 2), :] = _pk(y[:, j * 128:(j + 1) * 128].astype(BF16))
        return c
    lax.fori_loop(0, NXC, ln_body, 0)

    def xln_rows(r0, n):
        return _cat([_upk(xln_ref[j, r0 // 2:(r0 + n) // 2, :]) for j in range(nct)], axis=1)

    def set_slot(val):
        h_ref[n_mem:M2, :] = val[0:n_mem]
        h_ref[M2 + n_mem:M2 + seg, :] = val[n_mem:seg]

    m_copy.wait()
    m0 = mem0_ref[...].astype(F32)
    h_ref[0:n_mem, :] = m0
    h_ref[M2:M2 + n_mem, :] = m0
    set_slot(xln_rows(0, seg).astype(F32))
    h_ref[M2 + seg:RQ, :] = xln_rows(A0, AH).astype(F32)
    x2_ref[...] = x_ref[0:seg, :].astype(F32)

    dpt = 128 // B_HEADS

    def b_stage1(u):
        ok = (u >= 0) & (u < NB1)
        tr = bst_ref[jnp.where(ok, u, NB1 + nct)].astype(F32).T
        r0 = pl.multiple_of(jnp.where(ok, u * 128, DUM), 128)
        for j in range(nct):
            btmp_ref[j, pl.ds(r0, 128), :] = tr[:, j * 128:(j + 1) * 128]

    def b_stage1_wo(u):
        ok = (u >= 0) & (u < nct)
        r0 = pl.multiple_of(jnp.where(ok, WO0, DUM), 128)
        btmp_ref[jnp.where(ok, u, 0), pl.ds(r0, dm), :] = bst_ref[
            jnp.where(ok, NB1 + u, NB1 + nct)].astype(F32)

    def b_stage2(u):
        ok = (u >= 0) & (u < NB1)
        part = (u >= nct).astype(jnp.int32) + (u >= 2 * nct).astype(jnp.int32)
        r0 = jnp.where(ok, part * dm + (u - part * nct) * dpt, DUM)
        rows = _cat([_cat([btmp_ref[j, pl.ds(r0 + dd, B_HEADS, stride=bdh), :]
                           for j in range(nct)], axis=1) for dd in range(dpt)])
        bw_ref[jnp.where(ok, u, NB1 + nct)] = _pk(rows.T.astype(BF16))

    def b_stage2_wo(u):
        ok = (u >= 0) & (u < nct)
        r0 = jnp.where(ok, WO0, DUM)
        jj = jnp.where(ok, u, 0)
        bw_ref[jnp.where(ok, NB1 + u, NB1 + nct)] = _pk(
            _cat([btmp_ref[jj, pl.ds(r0 + d, B_HEADS, stride=bdh), :] for d in range(bdh)]).astype(BF16))

    def wo_store(g, dst):
        w = stage_ref[g & (NSLOT - 1), 3]
        for j in range(nct):
            wo_ref[dst * nct + j] = _pk(w[:, j * 128:(j + 1) * 128])

    def pre_body(g, c):
        w_wait(g)

        @pl.when(g >= 1)
        def _():
            w_copy(3, g - 1).wait()

        @pl.when(g == 3)
        def _():
            buf = bst_ref.at[pl.ds(0, NB1 + nct)]
            pltpu.make_async_copy(buf, buf, sem_m.at[2]).wait()

        @pl.when(g == 0)
        def _():
            for p in range(3):
                w_copy(p, 1).start()
            w_copy(3, 0).start()

        @pl.when(g + 2 < G)
        def _():
            for p in range(3):
                w_copy(p, g + 2).start()

        @pl.when(g + 1 < G)
        def _():
            w_copy(3, g + 1).start()

        @pl.when(g == 1)
        def _():
            for cp in bcp + [x_late]:
                cp.start()

        slot = g & (NSLOT - 1)
        wo_store(g - 1, jnp.where(g >= 1, g - 1, G - 1))
        b_stage2(2 * (g - 8))
        b_stage2(2 * (g - 8) + 1)
        b_stage2_wo(g - 8)
        b_stage1(2 * (g - 3))
        b_stage1(2 * (g - 3) + 1)
        b_stage1_wo(g - 3)
        xl = xln_rows(R0, NPRE)
        for p in range(3):
            w = stage_ref[slot, p]
            wt = w.T
            y = _nt(xl, w) if p < 2 else _nn(xl, wt)
            for j in range(3):
                ring_ref[(g * 3 + p) * 3 + j, 0:NPRE // 2, :] = _pk(y[:, j * 128:(j + 1) * 128].astype(BF16))
                w_ref[(g * 3 + p) * 3 + j] = _pk(wt[:, j * 128:(j + 1) * 128])
        return c
    lax.fori_loop(0, G, pre_body, 0)
    w_copy(3, G - 1).wait()
    x_late.wait()

    bscale = float(bdh) ** (-0.5)

    def b_lhs(ls):
        return _ln(xb_ref[ls[0] * seg:(ls[-1] + 1) * seg, :]).astype(BF16)

    def b_proj(lhs, part):
        return _nn(lhs, _cat([_upk(bw_ref[part * nct + j]) for j in range(nct)], axis=1))

    def b_attn(t, ls, q, k, v):
        row = lax.broadcasted_iota(jnp.int32, (seg, 128), 0)
        outs = []
        for i, l in enumerate(ls):
            r0 = i * seg
            pos = row + (t - (1 + LAG * l)) * seg
            for j in range(nct):
                kb_ref[l, j, HIST:HIST + seg, :] = k[r0:r0 + seg, j * 128:(j + 1) * 128]
                vb_ref[l, j, HIST:HIST + seg, :] = v[r0:r0 + seg, j * 128:(j + 1) * 128]
            logits = []
            for w in range(B_WIN):
                o = HIST - w * B_DIL
                acc = None
                for j in range(nct):
                    p = q[r0:r0 + seg, j * 128:(j + 1) * 128] * kb_ref[l, j, o:o + seg, :]
                    acc = p if acc is None else acc + p
                acc = acc + pltpu.roll(acc, 64, 1)
                acc = acc + pltpu.roll(acc, 32, 1)
                lg = acc * bscale
                if w > 0:
                    lg = jnp.where(pos >= w * B_DIL, lg, NEG)
                logits.append(lg)
            m = logits[0]
            for w in range(1, B_WIN):
                m = jnp.maximum(m, logits[w])
            es = [jnp.exp(lg - m) for lg in logits]
            den = es[0]
            for w in range(1, B_WIN):
                den = den + es[w]
            inv = 1.0 / den
            cols = []
            for j in range(nct):
                acc = None
                for w in range(B_WIN):
                    o = HIST - w * B_DIL
                    p = es[w] * vb_ref[l, j, o:o + seg, :]
                    acc = p if acc is None else acc + p
                cols.append(acc * inv)
            outs.append(_cat(cols, axis=1).astype(BF16))
            for j in range(nct):
                kb_ref[l, j, 0:HIST, :] = k[r0 + seg - HIST:r0 + seg, j * 128:(j + 1) * 128]
                vb_ref[l, j, 0:HIST, :] = v[r0 + seg - HIST:r0 + seg, j * 128:(j + 1) * 128]
        return outs

    def b_out(t, ls, ob, res=None):
        if res is None:
            res = xb_ref[ls[0] * seg:(ls[-1] + 1) * seg, :]
        zb = res + _nn(ob, _cat([_upk(bw_ref[NB1 + j]) for j in range(nct)], axis=1))
        if 1 in ls:
            ro = pl.multiple_of(jnp.maximum(t - LAG, 0) * seg, seg)
            o_ref[pl.ds(ro, seg), :] = zb[(len(ls) - 1) * seg:len(ls) * seg].astype(o_ref.dtype)
        return zb[0:seg] if 0 in ls else None

    def out_copy(b):
        ro = pl.multiple_of(b * seg, seg)
        return pltpu.make_async_copy(o_ref.at[pl.ds(ro + seg, seg), :], out_hbm.at[pl.ds(ro, seg), :], sem_o)

    def step(t, full, split=False):
        bls = [0, 1]
        nq = RQ if full else M2 + seg
        h = h_ref[0:nq, :].astype(BF16)
        scale = float(dh) ** (-0.5)
        if full:
            s_ = t - LAG
            rd = pl.multiple_of((s_ * (seg // 2)) & (RS // 2 - 1), seg // 2)
            wa = pl.multiple_of((NPRE // 2 + s_ * (AH // 2)) & (RS // 2 - 1), AH // 2)
        else:
            wo_store(G - 1, G - 1)

        RA = R if full else M2 + seg
        CW = R + 2 * M2 if full else R
        ri = lax.broadcasted_iota(jnp.int32, (RA, CW), 0)
        ci = lax.broadcasted_iota(jnp.int32, (RA, CW), 1)
        if not full:
            ri = jnp.where(ri >= M2, ri + seg, ri)

        def table(i, bounds, vals):
            out = vals[-1]
            for b, v in zip(reversed(bounds), reversed(vals[:-1])):
                out = jnp.where(i < b, v, out)
            return out
        qi = ri - table(ri, [16, 48, 56], [0, 8, 48, 40])
        g0 = (ci < 8) | ((ci >= 16) & (ci < 48))
        k2 = ci - table(ci, [8, 24, 32, 48, 56, 80, 88, 96, 104], [-8, 0, 24, 8, 48, 40, 72, 80, 96, 104])
        if full:
            k1 = ci - table(ci, [8, 48], [0, 8, 40])
            row_l2 = ((ri >= 8) & (ri < 16)) | (ri >= 48)
            row_xa = (ri >= 8) & (ri < 16)
            valid = row_xa == (ci >= 80)
            is_a = jnp.where(ci >= 80, ((ci >= 88) & (ci < 104)).astype(jnp.int32),
                             (g0 != row_l2).astype(jnp.int32)) > 0
            ki = jnp.where(row_l2, k2, k1)
            visible = valid & ((qi < n_mem) | (qi >= ki))
            fill = jnp.where(valid, NEG, -jnp.inf)
        else:
            is_a = jnp.logical_not(g0)
            visible = (qi < n_mem) | (qi >= k2)
            fill = NEG
        half = dh - 128
        la8 = lax.broadcasted_iota(jnp.int32, (n_mem, 128), 1) < half
        ones = jnp.full((n_mem, 128), 0xFFFFFFFF, U32)
        zero = jnp.zeros((n_mem, 128), U32)
        mask_a = jnp.where(la8, ones, zero)
        mask_b = jnp.where(la8, zero, ones)

        def pk2(a, b):
            return _pk(_cat([a, b]).astype(BF16))

        def proj(p, g):
            base = (g * 3 + p) * 3
            y = _nn(h, _cat([_upk(w_ref[base + j]) for j in range(3)], axis=1))
            yt = [y[:, j * 128:(j + 1) * 128] for j in range(3)]
            x1 = None
            if full:
                for j in range(3):
                    ring_ref[base + j, pl.ds(wa, AH // 2), :] = pk2(yt[j][48:56], yt[j][56:64])
                x1 = [ring_ref[base + j, pl.ds(rd, seg // 2), :] for j in range(3)]
            return yt, x1

        def groups(z, j):
            y = z[0][j]
            return pk2(y[0:8], y[8:16]), pk2(y[16:24], y[24:32]), pk2(y[32:40], y[40:48])

        def q_rows(z, j):
            v0, v1, v2 = groups(z, j)
            return [v0] + ([z[1][j]] if full else []) + [v1, v2]

        def kv_tiles(z):
            yt, x1 = z
            v0, v1, v2 = groups(z, 0)
            t0 = [v0] + ([x1[0]] if full else [v1, v2]) + [v1, v2]
            y = yt[2]
            w0 = pk2(y[8:16], y[0:8])
            w1 = pk2(y[24:32], y[16:24])
            w2 = pk2(y[32:40], y[40:48])
            t2 = [w0, w1, w2] + ([x1[2]] if full else [w1, w2])
            if full:
                t0 += [v0, v1]
                t2 += [w0, w1]
            y = yt[1]

            def ab(z8):
                return jnp.where(la8, z8, 0.0), jnp.where(la8, 0.0, z8)
            xa_a, xa_b = ab(y[8:16])
            e1 = pk2(xa_b, xa_a)
            u2 = pk2(y[32:40], y[40:48])
            mid2 = [e1, pk2(y[24:32], y[16:24]) & mask_b, u2 & mask_b,
                    pk2(y[16:24], y[24:32]) & mask_a, u2 & mask_a]
            mid1 = None
            if full:
                lo, hi = x1[1][0:8], x1[1][8:16]
                mid1 = [pk2(*ab(y[0:8])), lo & mask_a, hi & mask_a, lo & mask_b, hi & mask_b,
                        e1, pk2(*ab(y[16:24]))]
            return t0, mid1, mid2, t2

        def mat(parts):
            return _upk(_cat(parts))

        def scores(q, k):
            k0, km1, km2, k2_ = kv_tiles(k)
            s_a = _nt(mat(q_rows(q, 0)), mat(k0))
            s_b = _nt(mat(q_rows(q, 2)), mat(k2_))
            qm = q_rows(q, 1)
            if full:
                s_m = _cat([_nt(mat(qm[0:2]), mat(km1)), _nt(mat(qm[2:4]), mat(km2 + km1[5:7]))])
            else:
                s_m = _nt(mat(qm), mat(km2))
            s = (jnp.where(is_a, s_a, s_b) + s_m) * scale
            s = jnp.where(visible, s, fill)
            m_a = jnp.max(jnp.where(is_a, s, -jnp.inf), axis=-1, keepdims=True)
            m_b = jnp.max(jnp.where(is_a, -jnp.inf, s), axis=-1, keepdims=True)
            e = jnp.exp(s - jnp.where(is_a, m_a, m_b))
            d_a = jnp.sum(jnp.where(is_a, e, 0.0), axis=-1, keepdims=True)
            d_b = jnp.sum(jnp.where(is_a, 0.0, e), axis=-1, keepdims=True)
            return e / jnp.where(is_a, d_a, d_b)

        def pv(p, v):
            v0, vm1, vm2, v2 = kv_tiles(v)
            o_a = _nn(jnp.where(is_a, p, 0.0).astype(BF16), mat(v0))
            o_b = _nn(jnp.where(is_a, 0.0, p).astype(BF16), mat(v2))
            if full:
                o_m = _cat([_nn(p[0:M2 + seg].astype(BF16), mat(vm1)),
                            _nn(p[M2 + seg:R, 0:R].astype(BF16), mat(vm2))])
            else:
                o_m = _nn(p.astype(BF16), mat(vm2))
            return _cat([o_a, o_m, o_b], axis=1).astype(BF16)

        def oproj(o, g):
            return _nn(o, _cat([_upk(wo_ref[g * nct + j]) for j in range(nct)], axis=1))

        acc = [None]

        def add_o(g):
            c = oproj(os_[g], g)
            acc[0] = c if acc[0] is None else acc[0] + c

        os_ = [None] * G
        bqkv = []
        q = proj(0, 0)
        k = proj(1, 0)
        v = proj(2, 0)
        p = scores(q, k)
        blhs = b_lhs(bls)
        bqkv.append(b_proj(blhs, 0))
        x2_new = None
        for g in range(G - 1):
            q = proj(0, g + 1)
            k = proj(1, g + 1)
            os_[g] = pv(p, v)
            v = proj(2, g + 1)
            p = scores(q, k)
            if g < 2:
                bqkv.append(b_proj(blhs, g + 1))
            if g == 2:
                ob = b_attn(t, bls, *bqkv)
            if g == BOUT_AT:
                if split:
                    x2_new = b_out(t, [0], ob[0])
                    res2 = xb_ref[seg:2 * seg, :]
                else:
                    x2_new = b_out(t, bls, _cat(ob))
            if g - WLAG >= 0:
                add_o(g - WLAG)
        for g in range(G - 1 - WLAG, G - 2):
            add_o(g)
        os_[G - 1] = pv(p, v)
        add_o(G - 2)
        add_o(G - 1)
        acc = acc[0]
        if split:
            b_out(t, [1], ob[1], res2)

        y2 = x2_ref[...] + _cat([acc[n_mem:M2], acc[RA - seg + n_mem:RA]])
        mem2 = acc[RA - seg:RA - seg + n_mem]
        if full:
            x_cur = x_ref[pl.ds(pl.multiple_of(t * seg, seg), seg), :].astype(F32)
            xb_ref[0:seg, :] = x_cur + acc[M2:M2 + seg]
            xb_ref[seg:2 * seg, :] = y2
            h_ref[0:n_mem, :] = acc[0:n_mem]
            h_ref[M2:M2 + n_mem, :] = mem2
            an = pl.multiple_of(jnp.minimum(A0 + (t + 1 - LAG) * AH, S - AH), AH)
            h_ref[M2 + seg:RQ, :] = _ln(x_ref[pl.ds(an, AH), :].astype(F32))
            nxt = x2_new
        else:
            xb_ref[pl.ds(pl.multiple_of(jnp.where(t < LAG, 0, seg), seg), seg), :] = y2
            h_ref[0:n_mem, :] = mem2
            h_ref[M2:M2 + n_mem, :] = jnp.where(t == LAG - 1, mem0_ref[...].astype(F32), mem2)
            nxt = jnp.where(t < LAG - 1, x_ref[seg:2 * seg, :].astype(F32), x2_new)
        x2_ref[...] = nxt
        set_slot(_ln(nxt))

    def single_body(t, c):
        @pl.when(t >= LAG + 2)
        def _():
            out_copy(t - (LAG + 2)).start()
        step(t, False)
        return c

    def full_body(i, c):
        t = LAG + UNROLL * i
        for u in range(UNROLL):
            @pl.when(t - u >= LAG + 2)
            def _():
                out_copy(t - u - (LAG + 2)).start()
        for u in range(UNROLL):
            step(t + u, True, split=u < UNROLL - 1)
        return c

    def phase(ph, c):
        t0 = ph * n_seg
        lax.fori_loop(t0, t0 + LAG, single_body, 0)
        lax.fori_loop(0, jnp.where(ph == 0, (n_seg - LAG) // UNROLL, 0), full_body, 0)
        return c
    lax.fori_loop(0, 2, phase, 0)

    t_end = n_seg + LAG
    for u in range(1, UNROLL):
        out_copy(n_seg - u - (LAG + 2)).start()
    out_copy(t_end - (LAG + 2)).start()
    blhs = b_lhs([1])
    b_out(t_end, [1], _cat(b_attn(t_end, [1], *[b_proj(blhs, part) for part in range(3)])))
    out_copy(n_seg - 1).start()
    pltpu.make_async_copy(o_ref.at[pl.ds(seg, S), :], out_hbm, sem_o).wait()


@functools.partial(jax.jit, static_argnames=("seg",))
def _run(A_x, A_mem0, A_Wq, A_Wk, A_Wv, A_Wo, B_wqkv, B_wo, *, seg):
    _, S, dm = A_x.shape
    n_heads, dh = A_Wq.shape[1], A_Wq.shape[2]
    n_mem = A_mem0.shape[1]
    n_seg = S // seg
    hd = n_heads * dh
    nct = dm // 128
    assert (seg, n_seg, n_mem, dh, dm % 128, n_heads, LAG) == (32, 64, 8, 192, 0, 32, 2)

    x = A_x.reshape(S, dm)
    mem0 = A_mem0.reshape(n_mem, dm)
    wq = jnp.transpose(A_Wq, (1, 2, 0)).reshape(hd, dm)
    wk = jnp.transpose(A_Wk, (1, 2, 0)).reshape(hd, dm)
    wv = jnp.transpose(A_Wv, (1, 2, 0)).reshape(hd, dm)
    wo = A_Wo.reshape(hd, dm)
    _, _, _, _, rs, xc = _plan(seg, n_seg)

    kern = functools.partial(_kernel, seg=seg, n_seg=n_seg, n_mem=n_mem,
                             n_heads=n_heads, dh=dh, dm=dm)
    hbm = pl.BlockSpec(memory_space=pltpu.HBM)

    out = pl.pallas_call(
        kern,
        in_specs=[hbm] * 8,
        out_specs=hbm,
        out_shape=jax.ShapeDtypeStruct((S, dm), A_x.dtype),
        scratch_shapes=[
            pltpu.VMEM((S, dm), BF16),
            pltpu.VMEM((n_mem, dm), BF16),
            pltpu.VMEM((NSLOT, 4, 2 * dh, dm), BF16),
            pltpu.VMEM((3 * hd // 128, dm // 2, 128), U32),
            pltpu.VMEM((n_heads // 2 * nct, dh, 128), U32),
            pltpu.VMEM((4 * nct + 1, dm, 128), BF16),
            pltpu.VMEM((nct, 5 * dm + 32, 128), F32),
            pltpu.VMEM((4 * nct + 1, dm // 2, 128), U32),
            pltpu.VMEM((nct, NXC * xc // 2, 128), U32),
            pltpu.VMEM((3 * hd // 128, rs // 2, 128), U32),
            pltpu.VMEM((2 * n_mem + seg + AH, dm), F32),
            pltpu.VMEM((2 * seg, dm), F32),
            pltpu.VMEM((seg, dm), F32),
            pltpu.VMEM((2, nct, HIST + seg, 128), F32),
            pltpu.VMEM((2, nct, HIST + seg, 128), F32),
            pltpu.VMEM((S + seg, dm), A_x.dtype),
            pltpu.SemaphoreType.DMA((2, NSLOT)),
            pltpu.SemaphoreType.DMA((3 + NXC,)),
            pltpu.SemaphoreType.DMA(()),
        ],
        compiler_params=pltpu.CompilerParams(
            vmem_limit_bytes=120 * 1024 * 1024,
            disable_bounds_checks=True,
        ),
    )(x, mem0, wq, wk, wv, wo, B_wqkv, B_wo)
    return out.reshape(1, S, dm)


def pallas_interleave_layers__memory_aug_recurrent_mem_tr__sliding_local_dilated__prompt_kernel(
    A_x: jax.Array,
    A_mem0: jax.Array,
    A_Wq: jax.Array,
    A_Wk: jax.Array,
    A_Wv: jax.Array,
    A_Wo: jax.Array,
    A_seg_len,
    B_x: jax.Array,
    B_wqkv: jax.Array,
    B_wo: jax.Array,
):
    del B_x
    seg = A_seg_len if isinstance(A_seg_len, int) else 32
    return _run(A_x, A_mem0, A_Wq, A_Wk, A_Wv, A_Wo, B_wqkv, B_wo, seg=seg)
```

```python
import functools

import jax
import jax.numpy as jnp
from jax import lax
import jax.experimental.pallas as pl
import jax.experimental.pallas.tpu as pltpu

F32 = jnp.float32
BF16 = jnp.bfloat16
U32 = jnp.uint32
NEG = -1000000000.0
LN_EPS = 1e-05

B_HEADS = 32
B_WIN = 8
B_DIL = 2
HIST = 16
AH = 16
LAG = 2
NSLOT = 2
WLAG = 2
BOUT_AT = 8
NXC = 4
UNROLL = 2


def _ln(x):
    m = jnp.mean(x, axis=-1, keepdims=True)
    c = x - m
    v = jnp.mean(c * c, axis=-1, keepdims=True)
    return c * lax.rsqrt(v + LN_EPS)


def _nt(a, b):
    return lax.dot_general(a, b, (((1,), (1,)), ((), ())), preferred_element_type=F32)


def _nn(a, b):
    return jnp.dot(a, b, preferred_element_type=F32)


def _cat(xs, axis=0):
    return xs[0] if len(xs) == 1 else jnp.concatenate(xs, axis=axis)


def _pk(z):
    return pltpu.bitcast(z, U32)


def _upk(z):
    return pltpu.bitcast(z, BF16)


def _plan(seg, n_seg):
    S = seg * n_seg
    R0 = LAG * seg
    A0 = S - (n_seg - LAG) * AH
    NPRE = A0 - R0 - LAG * 8
    RS = A0 - R0 + seg
    XC = -(-(A0 + AH) // (16 * NXC)) * 16
    return S, R0, A0, NPRE, RS, XC


def _kernel(x_hbm, mem0_hbm, wq_hbm, wk_hbm, wv_hbm, wo_hbm, bqkv_hbm, bwo_hbm,
            out_hbm,
            x_ref, mem0_ref, stage_ref, w_ref, wo_ref, bst_ref, btmp_ref, bw_ref,
            xln_ref, ring_ref, h_ref, xb_ref, x2_ref, kb_ref, vb_ref, o_ref,
            sem_w, sem_m, sem_o,
            *, seg, n_seg, n_mem, n_heads, dh, dm):
    S, R0, A0, NPRE, RS, XC = _plan(seg, n_seg)
    M2 = 2 * n_mem
    R = M2 + 2 * seg
    RQ = M2 + seg + AH
    PW = 2 * dh
    G = n_heads // 2
    nct = dm // 128
    bdh = dm // B_HEADS
    w_hbm = (wq_hbm, wk_hbm, wv_hbm, wo_hbm)

    def w_copy(p, g):
        slot = g & (NSLOT - 1)
        return pltpu.make_async_copy(w_hbm[p].at[pl.ds(g * PW, PW), :],
                                     stage_ref.at[slot, p], sem_w.at[p // 3, slot])

    def w_wait(g):
        slot = g & (NSLOT - 1)
        buf = stage_ref.at[slot, pl.ds(0, 3)]
        pltpu.make_async_copy(buf, buf, sem_w.at[0, slot]).wait()

    NB1 = 3 * nct
    WO0 = 3 * dm
    DUM = 4 * dm
    XF = NXC * XC

    def x_copy(i):
        r0 = pl.multiple_of(i * XC, 16)
        return pltpu.make_async_copy(x_hbm.at[pl.ds(r0, XC), :], x_ref.at[pl.ds(r0, XC), :], sem_m.at[3 + i])

    x_late = pltpu.make_async_copy(x_hbm.at[pl.ds(XF, S - XF), :], x_ref.at[pl.ds(XF, S - XF), :], sem_m.at[0])
    m_copy = pltpu.make_async_copy(mem0_hbm, mem0_ref, sem_m.at[1])
    bcp = [pltpu.make_async_copy(bqkv_hbm, bst_ref.at[:, pl.ds(0, 3 * dm)], sem_m.at[2]),
           pltpu.make_async_copy(bwo_hbm, bst_ref.at[:, pl.ds(3 * dm, dm)], sem_m.at[2])]

    def bst_tile(c):
        return bst_ref[:, pl.ds(pl.multiple_of(c * 128, 128), 128)]

    for i in range(NXC):
        x_copy(i).start()
    m_copy.start()
    stage_ref[NSLOT - 1, 3] = jnp.zeros((PW, dm), BF16)
    xb_ref[...] = jnp.zeros(xb_ref.shape, F32)
    kb_ref[...] = jnp.zeros(kb_ref.shape, F32)
    vb_ref[...] = jnp.zeros(vb_ref.shape, F32)
    bst_ref[:, 4 * dm:] = jnp.zeros((dm, 128), BF16)

    def zero_body(j, c):
        btmp_ref[j, DUM:, :] = jnp.zeros((btmp_ref.shape[1] - DUM, 128), F32)
        return c
    lax.fori_loop(0, nct, zero_body, 0)

    def ln_body(i, c):
        x_copy(i).wait()

        @pl.when(i == 0)
        def _():
            for p in range(3):
                w_copy(p, 0).start()
        y = _ln(x_ref[pl.ds(pl.multiple_of(i * XC, 16), XC), :].astype(F32))
        r0 = pl.multiple_of(i * (XC // 2), 8)
        for j in range(nct):
            xln_ref[j, pl.ds(r0, XC // 2), :] = _pk(y[:, j * 128:(j + 1) * 128].astype(BF16))
        return c
    lax.fori_loop(0, NXC, ln_body, 0)

    def xln_rows(r0, n):
        return _cat([_upk(xln_ref[j, r0 // 2:(r0 + n) // 2, :]) for j in range(nct)], axis=1)

    def set_slot(val):
        h_ref[n_mem:M2, :] = val[0:n_mem]
        h_ref[M2 + n_mem:M2 + seg, :] = val[n_mem:seg]

    m_copy.wait()
    m0 = mem0_ref[...].astype(F32)
    xtra = xln_rows(R0 + NPRE, M2).astype(F32)
    h_ref[0:n_mem, :] = xtra[0:n_mem]
    h_ref[M2:M2 + n_mem, :] = m0
    set_slot(xln_rows(0, seg).astype(F32))
    h_ref[M2 + seg:RQ, :] = xln_rows(A0, AH).astype(F32)
    x2_ref[...] = x_ref[0:seg, :].astype(F32)

    dpt = 128 // B_HEADS

    def b_stage1(u):
        ok = (u >= 0) & (u < NB1)
        tr = bst_tile(jnp.where(ok, u, NB1 + nct)).astype(F32).T
        r0 = pl.multiple_of(jnp.where(ok, u * 128, DUM), 128)
        for j in range(nct):
            btmp_ref[j, pl.ds(r0, 128), :] = tr[:, j * 128:(j + 1) * 128]

    def b_stage1_wo(u):
        ok = (u >= 0) & (u < nct)
        r0 = pl.multiple_of(jnp.where(ok, WO0, DUM), 128)
        btmp_ref[jnp.where(ok, u, 0), pl.ds(r0, dm), :] = bst_tile(
            jnp.where(ok, NB1 + u, NB1 + nct)).astype(F32)

    def b_stage2(u):
        ok = (u >= 0) & (u < NB1)
        part = (u >= nct).astype(jnp.int32) + (u >= 2 * nct).astype(jnp.int32)
        r0 = jnp.where(ok, part * dm + (u - part * nct) * dpt, DUM)
        rows = _cat([_cat([btmp_ref[j, pl.ds(r0 + dd, B_HEADS, stride=bdh), :]
                           for j in range(nct)], axis=1) for dd in range(dpt)])
        bw_ref[jnp.where(ok, u, NB1 + nct)] = _pk(rows.T.astype(BF16))

    def b_stage2_wo(u):
        ok = (u >= 0) & (u < nct)
        r0 = jnp.where(ok, WO0, DUM)
        jj = jnp.where(ok, u, 0)
        bw_ref[jnp.where(ok, NB1 + u, NB1 + nct)] = _pk(
            _cat([btmp_ref[jj, pl.ds(r0 + d, B_HEADS, stride=bdh), :] for d in range(bdh)]).astype(BF16))

    def wo_store(g, dst):
        w = stage_ref[g & (NSLOT - 1), 3]
        for j in range(nct):
            wo_ref[dst * nct + j] = _pk(w[:, j * 128:(j + 1) * 128])

    def pre_body(g, c):
        w_wait(g)

        @pl.when(g >= 1)
        def _():
            w_copy(3, g - 1).wait()

        @pl.when(g == 3)
        def _():
            buf = bst_ref.at[:, pl.ds(0, 4 * dm)]
            pltpu.make_async_copy(buf, buf, sem_m.at[2]).wait()

        @pl.when(g + 1 < G)
        def _():
            for p in range(3):
                w_copy(p, g + 1).start()
        w_copy(3, g).start()

        @pl.when(g == 1)
        def _():
            for cp in bcp + [x_late]:
                cp.start()

        slot = g & (NSLOT - 1)
        wo_store(g - 1, jnp.where(g >= 1, g - 1, G - 1))
        b_stage2(2 * (g - 8))
        b_stage2(2 * (g - 8) + 1)
        b_stage2_wo(g - 8)
        b_stage1(2 * (g - 3))
        b_stage1(2 * (g - 3) + 1)
        b_stage1_wo(g - 3)
        xl = xln_rows(R0, NPRE)
        for p in range(3):
            w = stage_ref[slot, p]
            wt = w.T
            y = _nt(xl, w) if p < 2 else _nn(xl, wt)
            for j in range(3):
                ring_ref[(g * 3 + p) * 3 + j, 0:NPRE // 2, :] = _pk(y[:, j * 128:(j + 1) * 128].astype(BF16))
                w_ref[(g * 3 + p) * 3 + j] = _pk(wt[:, j * 128:(j + 1) * 128])
        return c
    lax.fori_loop(0, G, pre_body, 0)
    w_copy(3, G - 1).wait()
    x_late.wait()

    bscale = float(bdh) ** (-0.5)

    def b_lhs(ls):
        return _ln(xb_ref[ls[0] * seg:(ls[-1] + 1) * seg, :]).astype(BF16)

    def b_proj(lhs, part):
        return _nn(lhs, _cat([_upk(bw_ref[part * nct + j]) for j in range(nct)], axis=1))

    def b_attn(t, ls, q, k, v):
        row = lax.broadcasted_iota(jnp.int32, (seg, 128), 0)
        outs = []
        for i, l in enumerate(ls):
            r0 = i * seg
            pos = row + (t - (1 + LAG * l)) * seg
            for j in range(nct):
                kb_ref[l, j, HIST:HIST + seg, :] = k[r0:r0 + seg, j * 128:(j + 1) * 128]
                vb_ref[l, j, HIST:HIST + seg, :] = v[r0:r0 + seg, j * 128:(j + 1) * 128]
            logits = []
            for w in range(B_WIN):
                o = HIST - w * B_DIL
                acc = None
                for j in range(nct):
                    p = q[r0:r0 + seg, j * 128:(j + 1) * 128] * kb_ref[l, j, o:o + seg, :]
                    acc = p if acc is None else acc + p
                acc = acc + pltpu.roll(acc, 64, 1)
                acc = acc + pltpu.roll(acc, 32, 1)
                lg = acc * bscale
                if w > 0:
                    lg = jnp.where(pos >= w * B_DIL, lg, NEG)
                logits.append(lg)
            m = logits[0]
            for w in range(1, B_WIN):
                m = jnp.maximum(m, logits[w])
            es = [jnp.exp(lg - m) for lg in logits]
            den = es[0]
            for w in range(1, B_WIN):
                den = den + es[w]
            inv = 1.0 / den
            cols = []
            for j in range(nct):
                acc = None
                for w in range(B_WIN):
                    o = HIST - w * B_DIL
                    p = es[w] * vb_ref[l, j, o:o + seg, :]
                    acc = p if acc is None else acc + p
                cols.append(acc * inv)
            outs.append(_cat(cols, axis=1).astype(BF16))
            for j in range(nct):
                kb_ref[l, j, 0:HIST, :] = k[r0 + seg - HIST:r0 + seg, j * 128:(j + 1) * 128]
                vb_ref[l, j, 0:HIST, :] = v[r0 + seg - HIST:r0 + seg, j * 128:(j + 1) * 128]
        return outs

    def b_out(t, ls, ob, res=None):
        if res is None:
            res = xb_ref[ls[0] * seg:(ls[-1] + 1) * seg, :]
        zb = res + _nn(ob, _cat([_upk(bw_ref[NB1 + j]) for j in range(nct)], axis=1))
        if 1 in ls:
            ro = pl.multiple_of(jnp.maximum(t - LAG, 0) * seg, seg)
            o_ref[pl.ds(ro, seg), :] = zb[(len(ls) - 1) * seg:len(ls) * seg].astype(o_ref.dtype)
        return zb[0:seg] if 0 in ls else None

    def out_copy(b):
        ro = pl.multiple_of(b * seg, seg)
        return pltpu.make_async_copy(o_ref.at[pl.ds(ro + seg, seg), :], out_hbm.at[pl.ds(ro, seg), :], sem_o)

    def step(t, full, split=False):
        bls = [0, 1]
        nq = RQ if full else M2 + seg
        h = h_ref[0:nq, :].astype(BF16)
        scale = float(dh) ** (-0.5)
        if full:
            s_ = t - LAG
            rd = pl.multiple_of((s_ * (seg // 2)) & (RS // 2 - 1), seg // 2)
            wa = pl.multiple_of(((A0 - R0) // 2 + s_ * (AH // 2)) & (RS // 2 - 1), AH // 2)
        else:
            wx = pl.multiple_of(jnp.where(t < LAG, NPRE // 2 + t * (n_mem // 2), RS // 2), n_mem // 2)
            wo_store(G - 1, G - 1)

        RA = R if full else M2 + seg
        CW = R + 2 * M2 if full else R
        ri = lax.broadcasted_iota(jnp.int32, (RA, CW), 0)
        ci = lax.broadcasted_iota(jnp.int32, (RA, CW), 1)
        if not full:
            ri = jnp.where(ri >= M2, ri + seg, ri)

        def table(i, bounds, vals):
            out = vals[-1]
            for b, v in zip(reversed(bounds), reversed(vals[:-1])):
                out = jnp.where(i < b, v, out)
            return out
        qi = ri - table(ri, [16, 48, 56], [0, 8, 48, 40])
        g0 = (ci < 8) | ((ci >= 16) & (ci < 48))
        k2 = ci - table(ci, [8, 24, 32, 48, 56, 80, 88, 96, 104], [-8, 0, 24, 8, 48, 40, 72, 80, 96, 104])
        if full:
            k1 = ci - table(ci, [8, 48], [0, 8, 40])
            row_l2 = ((ri >= 8) & (ri < 16)) | (ri >= 48)
            row_xa = (ri >= 8) & (ri < 16)
            valid = row_xa == (ci >= 80)
            is_a = jnp.where(ci >= 80, ((ci >= 88) & (ci < 104)).astype(jnp.int32),
                             (g0 != row_l2).astype(jnp.int32)) > 0
            ki = jnp.where(row_l2, k2, k1)
            visible = valid & ((qi < n_mem) | (qi >= ki))
            fill = jnp.where(valid, NEG, -jnp.inf)
        else:
            is_a = jnp.logical_not(g0)
            visible = (qi < n_mem) | (qi >= k2)
            fill = NEG
        half = dh - 128
        la8 = lax.broadcasted_iota(jnp.int32, (n_mem, 128), 1) < half
        ones = jnp.full((n_mem, 128), 0xFFFFFFFF, U32)
        zero = jnp.zeros((n_mem, 128), U32)
        mask_a = jnp.where(la8, ones, zero)
        mask_b = jnp.where(la8, zero, ones)

        def pk2(a, b):
            return _pk(_cat([a, b]).astype(BF16))

        def proj(p, g):
            base = (g * 3 + p) * 3
            y = _nn(h, _cat([_upk(w_ref[base + j]) for j in range(3)], axis=1))
            yt = [y[:, j * 128:(j + 1) * 128] for j in range(3)]
            x1 = None
            if full:
                for j in range(3):
                    ring_ref[base + j, pl.ds(wa, AH // 2), :] = pk2(yt[j][48:56], yt[j][56:64])
                x1 = [ring_ref[base + j, pl.ds(rd, seg // 2), :] for j in range(3)]
            else:
                for j in range(3):
                    ring_ref[base + j, pl.ds(wx, n_mem // 2), :] = pk2(yt[j][0:8], yt[j][8:16])[0:n_mem // 2]
            return yt, x1

        def groups(z, j):
            y = z[0][j]
            return pk2(y[0:8], y[8:16]), pk2(y[16:24], y[24:32]), pk2(y[32:40], y[40:48])

        def q_rows(z, j):
            v0, v1, v2 = groups(z, j)
            return [v0] + ([z[1][j]] if full else []) + [v1, v2]

        def kv_tiles(z):
            yt, x1 = z
            v0, v1, v2 = groups(z, 0)
            t0 = [v0] + ([x1[0]] if full else [v1, v2]) + [v1, v2]
            y = yt[2]
            w0 = pk2(y[8:16], y[0:8])
            w1 = pk2(y[24:32], y[16:24])
            w2 = pk2(y[32:40], y[40:48])
            t2 = [w0, w1, w2] + ([x1[2]] if full else [w1, w2])
            if full:
                t0 += [v0, v1]
                t2 += [w0, w1]
            y = yt[1]

            def ab(z8):
                return jnp.where(la8, z8, 0.0), jnp.where(la8, 0.0, z8)
            xa_a, xa_b = ab(y[8:16])
            e1 = pk2(xa_b, xa_a)
            u2 = pk2(y[32:40], y[40:48])
            mid2 = [e1, pk2(y[24:32], y[16:24]) & mask_b, u2 & mask_b,
                    pk2(y[16:24], y[24:32]) & mask_a, u2 & mask_a]
            mid1 = None
            if full:
                lo, hi = x1[1][0:8], x1[1][8:16]
                mid1 = [pk2(*ab(y[0:8])), lo & mask_a, hi & mask_a, lo & mask_b, hi & mask_b,
                        e1, pk2(*ab(y[16:24]))]
            return t0, mid1, mid2, t2

        def mat(parts):
            return _upk(_cat(parts))

        def scores(q, k):
            k0, km1, km2, k2_ = kv_tiles(k)
            s_a = _nt(mat(q_rows(q, 0)), mat(k0))
            s_b = _nt(mat(q_rows(q, 2)), mat(k2_))
            qm = q_rows(q, 1)
            if full:
                s_m = _cat([_nt(mat(qm[0:2]), mat(km1)), _nt(mat(qm[2:4]), mat(km2 + km1[5:7]))])
            else:
                s_m = _nt(mat(qm), mat(km2))
            s = (jnp.where(is_a, s_a, s_b) + s_m) * scale
            s = jnp.where(visible, s, fill)
            m_a = jnp.max(jnp.where(is_a, s, -jnp.inf), axis=-1, keepdims=True)
            m_b = jnp.max(jnp.where(is_a, -jnp.inf, s), axis=-1, keepdims=True)
            e = jnp.exp(s - jnp.where(is_a, m_a, m_b))
            d_a = jnp.sum(jnp.where(is_a, e, 0.0), axis=-1, keepdims=True)
            d_b = jnp.sum(jnp.where(is_a, 0.0, e), axis=-1, keepdims=True)
            return e / jnp.where(is_a, d_a, d_b)

        def pv(p, v):
            v0, vm1, vm2, v2 = kv_tiles(v)
            o_a = _nn(jnp.where(is_a, p, 0.0).astype(BF16), mat(v0))
            o_b = _nn(jnp.where(is_a, 0.0, p).astype(BF16), mat(v2))
            if full:
                o_m = _cat([_nn(p[0:M2 + seg].astype(BF16), mat(vm1)),
                            _nn(p[M2 + seg:R, 0:R].astype(BF16), mat(vm2))])
            else:
                o_m = _nn(p.astype(BF16), mat(vm2))
            return _cat([o_a, o_m, o_b], axis=1).astype(BF16)

        def oproj(o, g):
            return _nn(o, _cat([_upk(wo_ref[g * nct + j]) for j in range(nct)], axis=1))

        acc = [None]

        def add_o(g):
            c = oproj(os_[g], g)
            acc[0] = c if acc[0] is None else acc[0] + c

        os_ = [None] * G
        bqkv = []
        q = proj(0, 0)
        k = proj(1, 0)
        v = proj(2, 0)
        p = scores(q, k)
        blhs = b_lhs(bls)
        bqkv.append(b_proj(blhs, 0))
        x2_new = None
        for g in range(G - 1):
            q = proj(0, g + 1)
            k = proj(1, g + 1)
            os_[g] = pv(p, v)
            v = proj(2, g + 1)
            p = scores(q, k)
            if g < 2:
                bqkv.append(b_proj(blhs, g + 1))
            if g == 2:
                ob = b_attn(t, bls, *bqkv)
            if g == BOUT_AT:
                if split:
                    x2_new = b_out(t, [0], ob[0])
                    res2 = xb_ref[seg:2 * seg, :]
                else:
                    x2_new = b_out(t, bls, _cat(ob))
            if g - WLAG >= 0:
                add_o(g - WLAG)
        for g in range(G - 1 - WLAG, G - 2):
            add_o(g)
        os_[G - 1] = pv(p, v)
        add_o(G - 2)
        add_o(G - 1)
        acc = acc[0]
        if split:
            b_out(t, [1], ob[1], res2)

        y2 = x2_ref[...] + _cat([acc[n_mem:M2], acc[RA - seg + n_mem:RA]])
        mem2 = acc[RA - seg:RA - seg + n_mem]
        if full:
            x_cur = x_ref[pl.ds(pl.multiple_of(t * seg, seg), seg), :].astype(F32)
            xb_ref[0:seg, :] = x_cur + acc[M2:M2 + seg]
            xb_ref[seg:2 * seg, :] = y2
            h_ref[0:n_mem, :] = acc[0:n_mem]
            h_ref[M2:M2 + n_mem, :] = mem2
            an = pl.multiple_of(jnp.minimum(A0 + (t + 1 - LAG) * AH, S - AH), AH)
            h_ref[M2 + seg:RQ, :] = _ln(x_ref[pl.ds(an, AH), :].astype(F32))
            nxt = x2_new
        else:
            xb_ref[pl.ds(pl.multiple_of(jnp.where(t < LAG, 0, seg), seg), seg), :] = y2
            h_ref[0:n_mem, :] = jnp.where(t < LAG - 1, xln_rows(R0 + NPRE, M2).astype(F32)[n_mem:M2], mem2)
            h_ref[M2:M2 + n_mem, :] = jnp.where(t == LAG - 1, mem0_ref[...].astype(F32), mem2)
            nxt = jnp.where(t < LAG - 1, x_ref[seg:2 * seg, :].astype(F32), x2_new)
        x2_ref[...] = nxt
        set_slot(_ln(nxt))

    def single_body(t, c):
        @pl.when(t >= LAG + 2)
        def _():
            out_copy(t - (LAG + 2)).start()
        step(t, False)
        return c

    def full_body(i, c):
        t = LAG + UNROLL * i
        for u in range(UNROLL):
            @pl.when(t - u >= LAG + 2)
            def _():
                out_copy(t - u - (LAG + 2)).start()
        for u in range(UNROLL):
            step(t + u, True, split=u < UNROLL - 1)
        return c

    def phase(ph, c):
        t0 = ph * n_seg
        lax.fori_loop(t0, t0 + LAG, single_body, 0)
        lax.fori_loop(0, jnp.where(ph == 0, (n_seg - LAG) // UNROLL, 0), full_body, 0)
        return c
    lax.fori_loop(0, 2, phase, 0)

    t_end = n_seg + LAG
    for u in range(1, UNROLL):
        out_copy(n_seg - u - (LAG + 2)).start()
    out_copy(t_end - (LAG + 2)).start()
    blhs = b_lhs([1])
    b_out(t_end, [1], _cat(b_attn(t_end, [1], *[b_proj(blhs, part) for part in range(3)])))
    out_copy(n_seg - 1).start()
    pltpu.make_async_copy(o_ref.at[pl.ds(seg, S), :], out_hbm, sem_o).wait()


@functools.partial(jax.jit, static_argnames=("seg",))
def _run(A_x, A_mem0, A_Wq, A_Wk, A_Wv, A_Wo, B_wqkv, B_wo, *, seg):
    _, S, dm = A_x.shape
    n_heads, dh = A_Wq.shape[1], A_Wq.shape[2]
    n_mem = A_mem0.shape[1]
    n_seg = S // seg
    hd = n_heads * dh
    nct = dm // 128
    assert (seg, n_seg, n_mem, dh, dm % 128, n_heads, LAG) == (32, 64, 8, 192, 0, 32, 2)

    x = A_x.reshape(S, dm)
    mem0 = A_mem0.reshape(n_mem, dm)
    wq = jnp.transpose(A_Wq, (1, 2, 0)).reshape(hd, dm)
    wk = jnp.transpose(A_Wk, (1, 2, 0)).reshape(hd, dm)
    wv = jnp.transpose(A_Wv, (1, 2, 0)).reshape(hd, dm)
    wo = A_Wo.reshape(hd, dm)
    _, _, _, _, rs, xc = _plan(seg, n_seg)

    kern = functools.partial(_kernel, seg=seg, n_seg=n_seg, n_mem=n_mem,
                             n_heads=n_heads, dh=dh, dm=dm)
    hbm = pl.BlockSpec(memory_space=pltpu.HBM)

    out = pl.pallas_call(
        kern,
        in_specs=[hbm] * 8,
        out_specs=hbm,
        out_shape=jax.ShapeDtypeStruct((S, dm), A_x.dtype),
        scratch_shapes=[
            pltpu.VMEM((S, dm), BF16),
            pltpu.VMEM((n_mem, dm), BF16),
            pltpu.VMEM((NSLOT, 4, 2 * dh, dm), BF16),
            pltpu.VMEM((3 * hd // 128, dm // 2, 128), U32),
            pltpu.VMEM((n_heads // 2 * nct, dh, 128), U32),
            pltpu.VMEM((dm, 4 * dm + 128), BF16),
            pltpu.VMEM((nct, 5 * dm + 32, 128), F32),
            pltpu.VMEM((4 * nct + 1, dm // 2, 128), U32),
            pltpu.VMEM((nct, NXC * xc // 2, 128), U32),
            pltpu.VMEM((3 * hd // 128, rs // 2 + 8, 128), U32),
            pltpu.VMEM((2 * n_mem + seg + AH, dm), F32),
            pltpu.VMEM((2 * seg, dm), F32),
            pltpu.VMEM((seg, dm), F32),
            pltpu.VMEM((2, nct, HIST + seg, 128), F32),
            pltpu.VMEM((2, nct, HIST + seg, 128), F32),
            pltpu.VMEM((S + seg, dm), A_x.dtype),
            pltpu.SemaphoreType.DMA((2, NSLOT)),
            pltpu.SemaphoreType.DMA((3 + NXC,)),
            pltpu.SemaphoreType.DMA(()),
        ],
        compiler_params=pltpu.CompilerParams(
            vmem_limit_bytes=120 * 1024 * 1024,
            disable_bounds_checks=True,
        ),
    )(x, mem0, wq, wk, wv, wo, B_wqkv, B_wo)
    return out.reshape(1, S, dm)


def pallas_interleave_layers__memory_aug_recurrent_mem_tr__sliding_local_dilated__prompt_kernel(
    A_x: jax.Array,
    A_mem0: jax.Array,
    A_Wq: jax.Array,
    A_Wk: jax.Array,
    A_Wv: jax.Array,
    A_Wo: jax.Array,
    A_seg_len,
    B_x: jax.Array,
    B_wqkv: jax.Array,
    B_wo: jax.Array,
):
    del B_x
    seg = A_seg_len if isinstance(A_seg_len, int) else 32
    return _run(A_x, A_mem0, A_Wq, A_Wk, A_Wv, A_Wo, B_wqkv, B_wo, seg=seg)
```

```python
import functools

import jax
import jax.numpy as jnp
from jax import lax
import jax.experimental.pallas as pl
import jax.experimental.pallas.tpu as pltpu

F32 = jnp.float32
BF16 = jnp.bfloat16
U32 = jnp.uint32
NEG = -1000000000.0
LN_EPS = 1e-05
LOG2E = 1.4426950408889634
NEG2 = NEG * LOG2E

B_HEADS = 32
B_WIN = 8
B_DIL = 2
HIST = 16
AH = 16
LAG = 2
NSLOT = 2
WLAG = 2
BOUT_AT = 8
NXC = 4
UNROLL = 2


def _ln(x):
    m = jnp.mean(x, axis=-1, keepdims=True)
    c = x - m
    v = jnp.mean(c * c, axis=-1, keepdims=True)
    return c * lax.rsqrt(v + LN_EPS)


def _recip(d):
    r = pl.reciprocal(d, approx=True)
    return r * (2.0 - d * r)


def _nt(a, b):
    return lax.dot_general(a, b, (((1,), (1,)), ((), ())), preferred_element_type=F32)


def _nn(a, b):
    return jnp.dot(a, b, preferred_element_type=F32)


def _cat(xs, axis=0):
    return xs[0] if len(xs) == 1 else jnp.concatenate(xs, axis=axis)


def _pk(z):
    return pltpu.bitcast(z, U32)


def _upk(z):
    return pltpu.bitcast(z, BF16)


def _plan(seg, n_seg):
    S = seg * n_seg
    R0 = LAG * seg
    A0 = S - (n_seg - LAG) * AH
    NPRE = A0 - R0 - LAG * 8
    RS = A0 - R0 + seg
    XC = -(-(A0 + AH) // (16 * NXC)) * 16
    return S, R0, A0, NPRE, RS, XC


def _kernel(x_hbm, mem0_hbm, wq_hbm, wk_hbm, wv_hbm, wo_hbm, bqkv_hbm, bwo_hbm,
            out_hbm,
            x_ref, mem0_ref, stage_ref, w_ref, wo_ref, bst_ref, btmp_ref, bw_ref,
            xln_ref, ring_ref, h_ref, xb_ref, x2_ref, kb_ref, vb_ref, o_ref,
            sem_w, sem_m, sem_o,
            *, seg, n_seg, n_mem, n_heads, dh, dm):
    S, R0, A0, NPRE, RS, XC = _plan(seg, n_seg)
    M2 = 2 * n_mem
    R = M2 + 2 * seg
    RQ = M2 + seg + AH
    PW = 2 * dh
    G = n_heads // 2
    nct = dm // 128
    bdh = dm // B_HEADS
    w_hbm = (wq_hbm, wk_hbm, wv_hbm, wo_hbm)

    def w_copy(p, g):
        slot = g & (NSLOT - 1)
        return pltpu.make_async_copy(w_hbm[p].at[pl.ds(g * PW, PW), :],
                                     stage_ref.at[slot, p], sem_w.at[p // 3, slot])

    def w_wait(g):
        slot = g & (NSLOT - 1)
        buf = stage_ref.at[slot, pl.ds(0, 3)]
        pltpu.make_async_copy(buf, buf, sem_w.at[0, slot]).wait()

    NB1 = 3 * nct
    WO0 = 3 * dm
    DUM = 4 * dm
    XF = NXC * XC

    def x_copy(i):
        r0 = pl.multiple_of(i * XC, 16)
        return pltpu.make_async_copy(x_hbm.at[pl.ds(r0, XC), :], x_ref.at[pl.ds(r0, XC), :], sem_m.at[3 + i])

    x_late = pltpu.make_async_copy(x_hbm.at[pl.ds(XF, S - XF), :], x_ref.at[pl.ds(XF, S - XF), :], sem_m.at[0])
    m_copy = pltpu.make_async_copy(mem0_hbm, mem0_ref, sem_m.at[1])
    bcp = [pltpu.make_async_copy(bqkv_hbm, bst_ref.at[:, pl.ds(0, 3 * dm)], sem_m.at[2]),
           pltpu.make_async_copy(bwo_hbm, bst_ref.at[:, pl.ds(3 * dm, dm)], sem_m.at[2])]

    def bst_tile(c):
        return bst_ref[:, pl.ds(pl.multiple_of(c * 128, 128), 128)]

    for i in range(NXC):
        x_copy(i).start()
    m_copy.start()
    stage_ref[NSLOT - 1, 3] = jnp.zeros((PW, dm), BF16)
    xb_ref[...] = jnp.zeros(xb_ref.shape, F32)
    kb_ref[...] = jnp.zeros(kb_ref.shape, F32)
    vb_ref[...] = jnp.zeros(vb_ref.shape, F32)
    bst_ref[:, 4 * dm:] = jnp.zeros((dm, 128), BF16)

    def zero_body(j, c):
        btmp_ref[j, DUM:, :] = jnp.zeros((btmp_ref.shape[1] - DUM, 128), F32)
        return c
    lax.fori_loop(0, nct, zero_body, 0)

    def ln_body(i, c):
        x_copy(i).wait()

        @pl.when(i == 0)
        def _():
            for p in range(3):
                w_copy(p, 0).start()
        y = _ln(x_ref[pl.ds(pl.multiple_of(i * XC, 16), XC), :].astype(F32))
        r0 = pl.multiple_of(i * (XC // 2), 8)
        for j in range(nct):
            xln_ref[j, pl.ds(r0, XC // 2), :] = _pk(y[:, j * 128:(j + 1) * 128].astype(BF16))
        return c
    lax.fori_loop(0, NXC, ln_body, 0)

    def xln_rows(r0, n):
        return _cat([_upk(xln_ref[j, r0 // 2:(r0 + n) // 2, :]) for j in range(nct)], axis=1)

    def set_slot(val):
        h_ref[n_mem:M2, :] = val[0:n_mem]
        h_ref[M2 + n_mem:M2 + seg, :] = val[n_mem:seg]

    m_copy.wait()
    m0 = mem0_ref[...].astype(F32)
    xtra = xln_rows(R0 + NPRE, M2).astype(F32)
    h_ref[0:n_mem, :] = xtra[0:n_mem]
    h_ref[M2:M2 + n_mem, :] = m0
    set_slot(xln_rows(0, seg).astype(F32))
    h_ref[M2 + seg:RQ, :] = xln_rows(A0, AH).astype(F32)
    x2_ref[...] = x_ref[0:seg, :].astype(F32)

    dpt = 128 // B_HEADS

    def b_stage1(u):
        ok = (u >= 0) & (u < NB1)
        tr = bst_tile(jnp.where(ok, u, NB1 + nct)).astype(F32).T
        r0 = pl.multiple_of(jnp.where(ok, u * 128, DUM), 128)
        for j in range(nct):
            btmp_ref[j, pl.ds(r0, 128), :] = tr[:, j * 128:(j + 1) * 128]

    def b_stage1_wo(u):
        ok = (u >= 0) & (u < nct)
        r0 = pl.multiple_of(jnp.where(ok, WO0, DUM), 128)
        btmp_ref[jnp.where(ok, u, 0), pl.ds(r0, dm), :] = bst_tile(
            jnp.where(ok, NB1 + u, NB1 + nct)).astype(F32)

    def b_stage2(u):
        ok = (u >= 0) & (u < NB1)
        part = (u >= nct).astype(jnp.int32) + (u >= 2 * nct).astype(jnp.int32)
        r0 = jnp.where(ok, part * dm + (u - part * nct) * dpt, DUM)
        rows = _cat([_cat([btmp_ref[j, pl.ds(r0 + dd, B_HEADS, stride=bdh), :]
                           for j in range(nct)], axis=1) for dd in range(dpt)])
        bw_ref[jnp.where(ok, u, NB1 + nct)] = _pk(rows.T.astype(BF16))

    def b_stage2_wo(u):
        ok = (u >= 0) & (u < nct)
        r0 = jnp.where(ok, WO0, DUM)
        jj = jnp.where(ok, u, 0)
        bw_ref[jnp.where(ok, NB1 + u, NB1 + nct)] = _pk(
            _cat([btmp_ref[jj, pl.ds(r0 + d, B_HEADS, stride=bdh), :] for d in range(bdh)]).astype(BF16))

    def wo_store(g, dst):
        w = stage_ref[g & (NSLOT - 1), 3]
        for j in range(nct):
            wo_ref[dst * nct + j] = _pk(w[:, j * 128:(j + 1) * 128])

    def pre_body(g, c):
        w_wait(g)

        @pl.when(g >= 1)
        def _():
            w_copy(3, g - 1).wait()

        @pl.when(g == 3)
        def _():
            buf = bst_ref.at[:, pl.ds(0, 4 * dm)]
            pltpu.make_async_copy(buf, buf, sem_m.at[2]).wait()

        @pl.when(g + 1 < G)
        def _():
            for p in range(3):
                w_copy(p, g + 1).start()
        w_copy(3, g).start()

        @pl.when(g == 1)
        def _():
            for cp in bcp + [x_late]:
                cp.start()

        slot = g & (NSLOT - 1)
        wo_store(g - 1, jnp.where(g >= 1, g - 1, G - 1))
        b_stage2(2 * (g - 8))
        b_stage2(2 * (g - 8) + 1)
        b_stage2_wo(g - 8)
        b_stage1(2 * (g - 3))
        b_stage1(2 * (g - 3) + 1)
        b_stage1_wo(g - 3)
        xl = xln_rows(R0, NPRE)
        for p in range(3):
            w = stage_ref[slot, p]
            wt = w.T
            y = _nt(xl, w) if p < 2 else _nn(xl, wt)
            for j in range(3):
                ring_ref[(g * 3 + p) * 3 + j, 0:NPRE // 2, :] = _pk(y[:, j * 128:(j + 1) * 128].astype(BF16))
                w_ref[(g * 3 + p) * 3 + j] = _pk(wt[:, j * 128:(j + 1) * 128])
        return c
    lax.fori_loop(0, G, pre_body, 0)
    w_copy(3, G - 1).wait()
    x_late.wait()

    bscale = float(bdh) ** (-0.5) * LOG2E

    def b_lhs(ls):
        return _ln(xb_ref[ls[0] * seg:(ls[-1] + 1) * seg, :]).astype(BF16)

    def b_proj(lhs, part):
        return _nn(lhs, _cat([_upk(bw_ref[part * nct + j]) for j in range(nct)], axis=1))

    def b_attn(t, ls, q, k, v):
        row = lax.broadcasted_iota(jnp.int32, (seg, 128), 0)
        outs = []
        for i, l in enumerate(ls):
            r0 = i * seg
            pos = row + (t - (1 + LAG * l)) * seg
            for j in range(nct):
                kb_ref[l, j, HIST:HIST + seg, :] = k[r0:r0 + seg, j * 128:(j + 1) * 128]
                vb_ref[l, j, HIST:HIST + seg, :] = v[r0:r0 + seg, j * 128:(j + 1) * 128]
            logits = []
            for w in range(B_WIN):
                o = HIST - w * B_DIL
                acc = None
                for j in range(nct):
                    p = q[r0:r0 + seg, j * 128:(j + 1) * 128] * kb_ref[l, j, o:o + seg, :]
                    acc = p if acc is None else acc + p
                acc = acc + pltpu.roll(acc, 64, 1)
                acc = acc + pltpu.roll(acc, 32, 1)
                lg = acc * bscale
                if w > 0:
                    lg = jnp.where(pos >= w * B_DIL, lg, NEG2)
                logits.append(lg)
            m = logits[0]
            for w in range(1, B_WIN):
                m = jnp.maximum(m, logits[w])
            es = [jnp.exp2(lg - m) for lg in logits]
            den = es[0]
            for w in range(1, B_WIN):
                den = den + es[w]
            inv = _recip(den)
            cols = []
            for j in range(nct):
                acc = None
                for w in range(B_WIN):
                    o = HIST - w * B_DIL
                    p = es[w] * vb_ref[l, j, o:o + seg, :]
                    acc = p if acc is None else acc + p
                cols.append(acc * inv)
            outs.append(_cat(cols, axis=1).astype(BF16))
            for j in range(nct):
                kb_ref[l, j, 0:HIST, :] = k[r0 + seg - HIST:r0 + seg, j * 128:(j + 1) * 128]
                vb_ref[l, j, 0:HIST, :] = v[r0 + seg - HIST:r0 + seg, j * 128:(j + 1) * 128]
        return outs

    def b_out(t, ls, ob, res=None):
        if res is None:
            res = xb_ref[ls[0] * seg:(ls[-1] + 1) * seg, :]
        zb = res + _nn(ob, _cat([_upk(bw_ref[NB1 + j]) for j in range(nct)], axis=1))
        if 1 in ls:
            ro = pl.multiple_of(jnp.maximum(t - LAG, 0) * seg, seg)
            o_ref[pl.ds(ro, seg), :] = zb[(len(ls) - 1) * seg:len(ls) * seg].astype(o_ref.dtype)
        return zb[0:seg] if 0 in ls else None

    def out_copy(b):
        ro = pl.multiple_of(b * seg, seg)
        return pltpu.make_async_copy(o_ref.at[pl.ds(ro + seg, seg), :], out_hbm.at[pl.ds(ro, seg), :], sem_o)

    def step(t, hc, full, split=False):
        bls = [0, 1]
        nq = RQ if full else M2 + seg
        h = _cat([_upk(hc), h_ref[2 * M2:nq, :].astype(BF16)])
        scale = float(dh) ** (-0.5) * LOG2E
        if full:
            s_ = t - LAG
            rd = pl.multiple_of((s_ * (seg // 2)) & (RS // 2 - 1), seg // 2)
            wa = pl.multiple_of(((A0 - R0) // 2 + s_ * (AH // 2)) & (RS // 2 - 1), AH // 2)
        else:
            wx = pl.multiple_of(jnp.where(t < LAG, NPRE // 2 + t * (n_mem // 2), RS // 2), n_mem // 2)
            wo_store(G - 1, G - 1)

        RA = R if full else M2 + seg
        CW = R + 2 * M2 if full else R
        ri = lax.broadcasted_iota(jnp.int32, (RA, CW), 0)
        ci = lax.broadcasted_iota(jnp.int32, (RA, CW), 1)
        if not full:
            ri = jnp.where(ri >= M2, ri + seg, ri)

        def table(i, bounds, vals):
            out = vals[-1]
            for b, v in zip(reversed(bounds), reversed(vals[:-1])):
                out = jnp.where(i < b, v, out)
            return out
        qi = ri - table(ri, [16, 48, 56], [0, 8, 48, 40])
        g0 = (ci < 8) | ((ci >= 16) & (ci < 48))
        k2 = ci - table(ci, [8, 24, 32, 48, 56, 80, 88, 96, 104], [-8, 0, 24, 8, 48, 40, 72, 80, 96, 104])
        if full:
            k1 = ci - table(ci, [8, 48], [0, 8, 40])
            row_l2 = ((ri >= 8) & (ri < 16)) | (ri >= 48)
            row_xa = (ri >= 8) & (ri < 16)
            valid = row_xa == (ci >= 80)
            is_a = jnp.where(ci >= 80, ((ci >= 88) & (ci < 104)).astype(jnp.int32),
                             (g0 != row_l2).astype(jnp.int32)) > 0
            ki = jnp.where(row_l2, k2, k1)
            visible = valid & ((qi < n_mem) | (qi >= ki))
            fill = jnp.where(valid, NEG2, -jnp.inf)
        else:
            is_a = jnp.logical_not(g0)
            visible = (qi < n_mem) | (qi >= k2)
            fill = NEG2
        half = dh - 128
        la8 = lax.broadcasted_iota(jnp.int32, (n_mem, 128), 1) < half
        ones = jnp.full((n_mem, 128), 0xFFFFFFFF, U32)
        zero = jnp.zeros((n_mem, 128), U32)
        mask_a = jnp.where(la8, ones, zero)
        mask_b = jnp.where(la8, zero, ones)

        def pk2(a, b):
            return _pk(_cat([a, b]).astype(BF16))

        def proj(p, g):
            base = (g * 3 + p) * 3
            y = _nn(h, _cat([_upk(w_ref[base + j]) for j in range(3)], axis=1))
            yt = [y[:, j * 128:(j + 1) * 128] for j in range(3)]
            x1 = None
            if full:
                for j in range(3):
                    ring_ref[base + j, pl.ds(wa, AH // 2), :] = pk2(yt[j][48:56], yt[j][56:64])
                x1 = [ring_ref[base + j, pl.ds(rd, seg // 2), :] for j in range(3)]
            else:
                for j in range(3):
                    ring_ref[base + j, pl.ds(wx, n_mem // 2), :] = pk2(yt[j][0:8], yt[j][8:16])[0:n_mem // 2]
            return yt, x1

        def groups(z, j):
            y = z[0][j]
            return pk2(y[0:8], y[8:16]), pk2(y[16:24], y[24:32]), pk2(y[32:40], y[40:48])

        def q_rows(z, j):
            v0, v1, v2 = groups(z, j)
            return [v0] + ([z[1][j]] if full else []) + [v1, v2]

        def kv_tiles(z):
            yt, x1 = z
            v0, v1, v2 = groups(z, 0)
            t0 = [v0] + ([x1[0]] if full else [v1, v2]) + [v1, v2]
            y = yt[2]
            w0 = pk2(y[8:16], y[0:8])
            w1 = pk2(y[24:32], y[16:24])
            w2 = pk2(y[32:40], y[40:48])
            t2 = [w0, w1, w2] + ([x1[2]] if full else [w1, w2])
            if full:
                t0 += [v0, v1]
                t2 += [w0, w1]
            y = yt[1]

            def ab(z8):
                return jnp.where(la8, z8, 0.0), jnp.where(la8, 0.0, z8)
            xa_a, xa_b = ab(y[8:16])
            e1 = pk2(xa_b, xa_a)
            u2 = pk2(y[32:40], y[40:48])
            mid2 = [e1, pk2(y[24:32], y[16:24]) & mask_b, u2 & mask_b,
                    pk2(y[16:24], y[24:32]) & mask_a, u2 & mask_a]
            mid1 = None
            if full:
                lo, hi = x1[1][0:8], x1[1][8:16]
                mid1 = [pk2(*ab(y[0:8])), lo & mask_a, hi & mask_a, lo & mask_b, hi & mask_b,
                        e1, pk2(*ab(y[16:24]))]
            return t0, mid1, mid2, t2

        def mat(parts):
            return _upk(_cat(parts))

        def scores(q, k):
            k0, km1, km2, k2_ = kv_tiles(k)
            s_a = _nt(mat(q_rows(q, 0)), mat(k0))
            s_b = _nt(mat(q_rows(q, 2)), mat(k2_))
            qm = q_rows(q, 1)
            if full:
                s_m = _cat([_nt(mat(qm[0:2]), mat(km1)), _nt(mat(qm[2:4]), mat(km2 + km1[5:7]))])
            else:
                s_m = _nt(mat(qm), mat(km2))
            s = (jnp.where(is_a, s_a, s_b) + s_m) * scale
            s = jnp.where(visible, s, fill)
            m_a = jnp.max(jnp.where(is_a, s, -jnp.inf), axis=-1, keepdims=True)
            m_b = jnp.max(jnp.where(is_a, -jnp.inf, s), axis=-1, keepdims=True)
            e = jnp.exp2(s - jnp.where(is_a, m_a, m_b))
            d_a = jnp.sum(jnp.where(is_a, e, 0.0), axis=-1, keepdims=True)
            d_b = jnp.sum(jnp.where(is_a, 0.0, e), axis=-1, keepdims=True)
            return e * _recip(jnp.where(is_a, d_a, d_b))

        def pv(p, v):
            v0, vm1, vm2, v2 = kv_tiles(v)
            o_a = _nn(jnp.where(is_a, p, 0.0).astype(BF16), mat(v0))
            o_b = _nn(jnp.where(is_a, 0.0, p).astype(BF16), mat(v2))
            if full:
                o_m = _cat([_nn(p[0:M2 + seg].astype(BF16), mat(vm1)),
                            _nn(p[M2 + seg:R, 0:R].astype(BF16), mat(vm2))])
            else:
                o_m = _nn(p.astype(BF16), mat(vm2))
            return _cat([o_a, o_m, o_b], axis=1).astype(BF16)

        def oproj(o, g):
            return _nn(o, _cat([_upk(wo_ref[g * nct + j]) for j in range(nct)], axis=1))

        acc = [None]

        def add_o(g):
            c = oproj(os_[g], g)
            acc[0] = c if acc[0] is None else acc[0] + c

        os_ = [None] * G
        bqkv = []
        q = proj(0, 0)
        k = proj(1, 0)
        v = proj(2, 0)
        p = scores(q, k)
        blhs = b_lhs(bls)
        bqkv.append(b_proj(blhs, 0))
        x2_new = None
        for g in range(G - 1):
            q = proj(0, g + 1)
            k = proj(1, g + 1)
            os_[g] = pv(p, v)
            v = proj(2, g + 1)
            p = scores(q, k)
            if g < 2:
                bqkv.append(b_proj(blhs, g + 1))
            if g == 2:
                ob = b_attn(t, bls, *bqkv)
            if g == BOUT_AT:
                if split:
                    x2_new = b_out(t, [0], ob[0])
                    res2 = xb_ref[seg:2 * seg, :]
                else:
                    x2_new = b_out(t, bls, _cat(ob))
            if g - WLAG >= 0:
                add_o(g - WLAG)
        for g in range(G - 1 - WLAG, G - 2):
            add_o(g)
        os_[G - 1] = pv(p, v)
        add_o(G - 2)
        add_o(G - 1)
        acc = acc[0]
        if split:
            b_out(t, [1], ob[1], res2)

        y2 = x2_ref[...] + _cat([acc[n_mem:M2], acc[RA - seg + n_mem:RA]])
        mem2 = acc[RA - seg:RA - seg + n_mem]
        if full:
            x_cur = x_ref[pl.ds(pl.multiple_of(t * seg, seg), seg), :].astype(F32)
            xb_ref[0:seg, :] = x_cur + acc[M2:M2 + seg]
            xb_ref[seg:2 * seg, :] = y2
            m1n = acc[0:n_mem]
            m2n = mem2
            an = pl.multiple_of(jnp.minimum(A0 + (t + 1 - LAG) * AH, S - AH), AH)
            h_ref[M2 + seg:RQ, :] = _ln(x_ref[pl.ds(an, AH), :].astype(F32))
            nxt = x2_new
        else:
            xb_ref[pl.ds(pl.multiple_of(jnp.where(t < LAG, 0, seg), seg), seg), :] = y2
            m1n = jnp.where(t < LAG - 1, xln_rows(R0 + NPRE, M2).astype(F32)[n_mem:M2], mem2)
            m2n = jnp.where(t == LAG - 1, mem0_ref[...].astype(F32), mem2)
            nxt = jnp.where(t < LAG - 1, x_ref[seg:2 * seg, :].astype(F32), x2_new)
        x2_ref[...] = nxt
        sl = _ln(nxt)
        h_ref[2 * M2:M2 + seg, :] = sl[M2:seg]
        return _pk(_cat([m1n, sl[0:n_mem], m2n, sl[n_mem:M2]]).astype(BF16))

    def single_body(t, c):
        @pl.when(t >= LAG + 2)
        def _():
            out_copy(t - (LAG + 2)).start()
        return step(t, c, False)

    def full_body(i, c):
        t = LAG + UNROLL * i
        for u in range(UNROLL):
            @pl.when(t - u >= LAG + 2)
            def _():
                out_copy(t - u - (LAG + 2)).start()
        for u in range(UNROLL):
            c = step(t + u, c, True, split=u < UNROLL - 1)
        return c

    def phase(ph, c):
        t0 = ph * n_seg
        c = lax.fori_loop(t0, t0 + LAG, single_body, c)
        return lax.fori_loop(0, jnp.where(ph == 0, (n_seg - LAG) // UNROLL, 0), full_body, c)
    lax.fori_loop(0, 2, phase, _pk(h_ref[0:2 * M2, :].astype(BF16)))

    t_end = n_seg + LAG
    for u in range(1, UNROLL):
        out_copy(n_seg - u - (LAG + 2)).start()
    out_copy(t_end - (LAG + 2)).start()
    blhs = b_lhs([1])
    b_out(t_end, [1], _cat(b_attn(t_end, [1], *[b_proj(blhs, part) for part in range(3)])))
    out_copy(n_seg - 1).start()
    pltpu.make_async_copy(o_ref.at[pl.ds(seg, S), :], out_hbm, sem_o).wait()


@functools.partial(jax.jit, static_argnames=("seg",))
def _run(A_x, A_mem0, A_Wq, A_Wk, A_Wv, A_Wo, B_wqkv, B_wo, *, seg):
    _, S, dm = A_x.shape
    n_heads, dh = A_Wq.shape[1], A_Wq.shape[2]
    n_mem = A_mem0.shape[1]
    n_seg = S // seg
    hd = n_heads * dh
    nct = dm // 128
    assert (seg, n_seg, n_mem, dh, dm % 128, n_heads, LAG) == (32, 64, 8, 192, 0, 32, 2)

    x = A_x.reshape(S, dm)
    mem0 = A_mem0.reshape(n_mem, dm)
    wq = jnp.transpose(A_Wq, (1, 2, 0)).reshape(hd, dm)
    wk = jnp.transpose(A_Wk, (1, 2, 0)).reshape(hd, dm)
    wv = jnp.transpose(A_Wv, (1, 2, 0)).reshape(hd, dm)
    wo = A_Wo.reshape(hd, dm)
    _, _, _, _, rs, xc = _plan(seg, n_seg)

    kern = functools.partial(_kernel, seg=seg, n_seg=n_seg, n_mem=n_mem,
                             n_heads=n_heads, dh=dh, dm=dm)
    hbm = pl.BlockSpec(memory_space=pltpu.HBM)

    out = pl.pallas_call(
        kern,
        in_specs=[hbm] * 8,
        out_specs=hbm,
        out_shape=jax.ShapeDtypeStruct((S, dm), A_x.dtype),
        scratch_shapes=[
            pltpu.VMEM((S, dm), BF16),
            pltpu.VMEM((n_mem, dm), BF16),
            pltpu.VMEM((NSLOT, 4, 2 * dh, dm), BF16),
            pltpu.VMEM((3 * hd // 128, dm // 2, 128), U32),
            pltpu.VMEM((n_heads // 2 * nct, dh, 128), U32),
            pltpu.VMEM((dm, 4 * dm + 128), BF16),
            pltpu.VMEM((nct, 5 * dm + 32, 128), F32),
            pltpu.VMEM((4 * nct + 1, dm // 2, 128), U32),
            pltpu.VMEM((nct, NXC * xc // 2, 128), U32),
            pltpu.VMEM((3 * hd // 128, rs // 2 + 8, 128), U32),
            pltpu.VMEM((2 * n_mem + seg + AH, dm), F32),
            pltpu.VMEM((2 * seg, dm), F32),
            pltpu.VMEM((seg, dm), F32),
            pltpu.VMEM((2, nct, HIST + seg, 128), F32),
            pltpu.VMEM((2, nct, HIST + seg, 128), F32),
            pltpu.VMEM((S + seg, dm), A_x.dtype),
            pltpu.SemaphoreType.DMA((2, NSLOT)),
            pltpu.SemaphoreType.DMA((3 + NXC,)),
            pltpu.SemaphoreType.DMA(()),
        ],
        compiler_params=pltpu.CompilerParams(
            vmem_limit_bytes=120 * 1024 * 1024,
            disable_bounds_checks=True,
        ),
    )(x, mem0, wq, wk, wv, wo, B_wqkv, B_wo)
    return out.reshape(1, S, dm)


def pallas_interleave_layers__memory_aug_recurrent_mem_tr__sliding_local_dilated__prompt_kernel(
    A_x: jax.Array,
    A_mem0: jax.Array,
    A_Wq: jax.Array,
    A_Wk: jax.Array,
    A_Wv: jax.Array,
    A_Wo: jax.Array,
    A_seg_len,
    B_x: jax.Array,
    B_wqkv: jax.Array,
    B_wo: jax.Array,
):
    del B_x
    seg = A_seg_len if isinstance(A_seg_len, int) else 32
    return _run(A_x, A_mem0, A_Wq, A_Wk, A_Wv, A_Wo, B_wqkv, B_wo, seg=seg)
```

```python
import functools

import jax
import jax.numpy as jnp
from jax import lax
import jax.experimental.pallas as pl
import jax.experimental.pallas.tpu as pltpu

F32 = jnp.float32
BF16 = jnp.bfloat16
U32 = jnp.uint32
NEG = -1000000000.0
LN_EPS = 1e-05
LOG2E = 1.4426950408889634
NEG2 = NEG * LOG2E

B_HEADS = 32
B_WIN = 8
B_DIL = 2
HIST = 16
AH = 16
LAG = 2
NSLOT = 2
WLAG = 2
BOUT_AT = 8
NXC = 4
UNROLL = 2


def _ln(x):
    m = jnp.mean(x, axis=-1, keepdims=True)
    c = x - m
    v = jnp.mean(c * c, axis=-1, keepdims=True)
    return c * lax.rsqrt(v + LN_EPS)


def _recip(d):
    r = pl.reciprocal(d, approx=True)
    return r * (2.0 - d * r)


def _nt(a, b):
    return lax.dot_general(a, b, (((1,), (1,)), ((), ())), preferred_element_type=F32)


def _nn(a, b):
    return jnp.dot(a, b, preferred_element_type=F32)


def _cat(xs, axis=0):
    return xs[0] if len(xs) == 1 else jnp.concatenate(xs, axis=axis)


def _pk(z):
    return pltpu.bitcast(z, U32)


def _upk(z):
    return pltpu.bitcast(z, BF16)


def _plan(seg, n_seg):
    S = seg * n_seg
    R0 = LAG * seg
    A0 = S - (n_seg - LAG) * AH
    NPRE = A0 - R0 - LAG * 8
    RS = A0 - R0 + seg
    XC = -(-(A0 + AH) // (16 * NXC)) * 16
    return S, R0, A0, NPRE, RS, XC


def _kernel(x_hbm, mem0_hbm, wq_hbm, wk_hbm, wv_hbm, wo_hbm, bqkv_hbm, bwo_hbm,
            out_hbm,
            x_ref, mem0_ref, stage_ref, w_ref, wo_ref, bst_ref, btmp_ref, bw_ref,
            xln_ref, ring_ref, h_ref, xb_ref, x2_ref, kb_ref, vb_ref, o_ref,
            sem_w, sem_m, sem_o,
            *, seg, n_seg, n_mem, n_heads, dh, dm):
    S, R0, A0, NPRE, RS, XC = _plan(seg, n_seg)
    M2 = 2 * n_mem
    R = M2 + 2 * seg
    RQ = M2 + seg + AH
    PW = 2 * dh
    G = n_heads // 2
    nct = dm // 128
    bdh = dm // B_HEADS
    w_hbm = (wq_hbm, wk_hbm, wv_hbm, wo_hbm)

    def w_copy(p, g):
        slot = g & (NSLOT - 1)
        return pltpu.make_async_copy(w_hbm[p].at[pl.ds(g * PW, PW), :],
                                     stage_ref.at[slot, p], sem_w.at[p // 3, slot])

    def w_wait(g):
        slot = g & (NSLOT - 1)
        buf = stage_ref.at[slot, pl.ds(0, 3)]
        pltpu.make_async_copy(buf, buf, sem_w.at[0, slot]).wait()

    NB1 = 3 * nct
    WO0 = 3 * dm
    DUM = 4 * dm
    XF = NXC * XC

    def x_copy(i):
        r0 = pl.multiple_of(i * XC, 16)
        return pltpu.make_async_copy(x_hbm.at[pl.ds(r0, XC), :], x_ref.at[pl.ds(r0, XC), :], sem_m.at[3 + i])

    x_late = pltpu.make_async_copy(x_hbm.at[pl.ds(XF, S - XF), :], x_ref.at[pl.ds(XF, S - XF), :], sem_m.at[0])
    m_copy = pltpu.make_async_copy(mem0_hbm, mem0_ref, sem_m.at[1])
    bcp = [pltpu.make_async_copy(bqkv_hbm, bst_ref.at[:, pl.ds(0, 3 * dm)], sem_m.at[2]),
           pltpu.make_async_copy(bwo_hbm, bst_ref.at[:, pl.ds(3 * dm, dm)], sem_m.at[2])]

    def bst_tile(c):
        return bst_ref[:, pl.ds(pl.multiple_of(c * 128, 128), 128)]

    for i in range(NXC):
        x_copy(i).start()
    m_copy.start()
    stage_ref[NSLOT - 1, 3] = jnp.zeros((PW, dm), BF16)
    xb_ref[0:2 * seg, :] = jnp.zeros((2 * seg, dm), F32)
    kb_ref[...] = jnp.zeros(kb_ref.shape, F32)
    vb_ref[...] = jnp.zeros(vb_ref.shape, F32)
    bst_ref[:, 4 * dm:] = jnp.zeros((dm, 128), BF16)

    def zero_body(j, c):
        btmp_ref[j, DUM:, :] = jnp.zeros((btmp_ref.shape[1] - DUM, 128), F32)
        return c
    lax.fori_loop(0, nct, zero_body, 0)

    def ln_body(i, c):
        x_copy(i).wait()

        @pl.when(i == 0)
        def _():
            for p in range(3):
                w_copy(p, 0).start()
        y = _ln(x_ref[pl.ds(pl.multiple_of(i * XC, 16), XC), :].astype(F32))
        r0 = pl.multiple_of(i * (XC // 2), 8)
        for j in range(nct):
            xln_ref[j, pl.ds(r0, XC // 2), :] = _pk(y[:, j * 128:(j + 1) * 128].astype(BF16))
        return c
    lax.fori_loop(0, NXC, ln_body, 0)

    def xln_rows(r0, n):
        return _cat([_upk(xln_ref[j, r0 // 2:(r0 + n) // 2, :]) for j in range(nct)], axis=1)

    def set_slot(val):
        h_ref[n_mem:M2, :] = val[0:n_mem]
        h_ref[M2 + n_mem:M2 + seg, :] = val[n_mem:seg]

    m_copy.wait()
    m0 = mem0_ref[...].astype(F32)
    xtra = xln_rows(R0 + NPRE, M2).astype(F32)
    h_ref[0:n_mem, :] = xtra[0:n_mem]
    h_ref[M2:M2 + n_mem, :] = m0
    set_slot(xln_rows(0, seg).astype(F32))
    h_ref[M2 + seg:RQ, :] = xln_rows(A0, AH).astype(F32)
    x2_ref[...] = x_ref[0:seg, :].astype(F32)

    dpt = 128 // B_HEADS

    def b_stage1(u):
        ok = (u >= 0) & (u < NB1)
        tr = bst_tile(jnp.where(ok, u, NB1 + nct)).astype(F32).T
        r0 = pl.multiple_of(jnp.where(ok, u * 128, DUM), 128)
        for j in range(nct):
            btmp_ref[j, pl.ds(r0, 128), :] = tr[:, j * 128:(j + 1) * 128]

    def b_stage1_wo(u):
        ok = (u >= 0) & (u < nct)
        r0 = pl.multiple_of(jnp.where(ok, WO0, DUM), 128)
        btmp_ref[jnp.where(ok, u, 0), pl.ds(r0, dm), :] = bst_tile(
            jnp.where(ok, NB1 + u, NB1 + nct)).astype(F32)

    def b_stage2(u):
        ok = (u >= 0) & (u < NB1)
        part = (u >= nct).astype(jnp.int32) + (u >= 2 * nct).astype(jnp.int32)
        r0 = jnp.where(ok, part * dm + (u - part * nct) * dpt, DUM)
        rows = _cat([_cat([btmp_ref[j, pl.ds(r0 + dd, B_HEADS, stride=bdh), :]
                           for j in range(nct)], axis=1) for dd in range(dpt)])
        bw_ref[jnp.where(ok, u, NB1 + nct)] = _pk(rows.T.astype(BF16))

    def b_stage2_wo(u):
        ok = (u >= 0) & (u < nct)
        r0 = jnp.where(ok, WO0, DUM)
        jj = jnp.where(ok, u, 0)
        bw_ref[jnp.where(ok, NB1 + u, NB1 + nct)] = _pk(
            _cat([btmp_ref[jj, pl.ds(r0 + d, B_HEADS, stride=bdh), :] for d in range(bdh)]).astype(BF16))

    def wo_store(g, dst):
        w = stage_ref[g & (NSLOT - 1), 3]
        for j in range(nct):
            wo_ref[dst * nct + j] = _pk(w[:, j * 128:(j + 1) * 128])

    def pre_body(g, c):
        w_wait(g)

        @pl.when(g >= 1)
        def _():
            w_copy(3, g - 1).wait()

        @pl.when(g == 3)
        def _():
            buf = bst_ref.at[:, pl.ds(0, 4 * dm)]
            pltpu.make_async_copy(buf, buf, sem_m.at[2]).wait()

        @pl.when(g + 1 < G)
        def _():
            for p in range(3):
                w_copy(p, g + 1).start()
        w_copy(3, g).start()

        @pl.when(g == 1)
        def _():
            for cp in bcp + [x_late]:
                cp.start()

        slot = g & (NSLOT - 1)
        wo_store(g - 1, jnp.where(g >= 1, g - 1, G - 1))
        b_stage2(2 * (g - 8))
        b_stage2(2 * (g - 8) + 1)
        b_stage2_wo(g - 8)
        b_stage1(2 * (g - 3))
        b_stage1(2 * (g - 3) + 1)
        b_stage1_wo(g - 3)
        xl = xln_rows(R0, NPRE)
        for p in range(3):
            w = stage_ref[slot, p]
            wt = w.T
            y = _nt(xl, w) if p < 2 else _nn(xl, wt)
            for j in range(3):
                ring_ref[(g * 3 + p) * 3 + j, 0:NPRE // 2, :] = _pk(y[:, j * 128:(j + 1) * 128].astype(BF16))
                w_ref[(g * 3 + p) * 3 + j] = _pk(wt[:, j * 128:(j + 1) * 128])
        return c
    lax.fori_loop(0, G, pre_body, 0)
    w_copy(3, G - 1).wait()
    x_late.wait()

    bscale = float(bdh) ** (-0.5) * LOG2E

    def b_proj(lhs, part):
        return _nn(lhs, _cat([_upk(bw_ref[part * nct + j]) for j in range(nct)], axis=1))

    def b_attn(jobs, q, k, v):
        row = lax.broadcasted_iota(jnp.int32, (seg, 128), 0)
        outs = []
        for i, (l, sidx) in enumerate(jobs):
            r0 = i * seg
            pos = row + sidx * seg
            for j in range(nct):
                kb_ref[l, j, HIST:HIST + seg, :] = k[r0:r0 + seg, j * 128:(j + 1) * 128]
                vb_ref[l, j, HIST:HIST + seg, :] = v[r0:r0 + seg, j * 128:(j + 1) * 128]
            logits = []
            for w in range(B_WIN):
                o = HIST - w * B_DIL
                acc = None
                for j in range(nct):
                    p = q[r0:r0 + seg, j * 128:(j + 1) * 128] * kb_ref[l, j, o:o + seg, :]
                    acc = p if acc is None else acc + p
                acc = acc + pltpu.roll(acc, 64, 1)
                acc = acc + pltpu.roll(acc, 32, 1)
                lg = acc * bscale
                if w > 0:
                    lg = jnp.where(pos >= w * B_DIL, lg, NEG2)
                logits.append(lg)
            m = logits[0]
            for w in range(1, B_WIN):
                m = jnp.maximum(m, logits[w])
            es = [jnp.exp2(lg - m) for lg in logits]
            den = es[0]
            for w in range(1, B_WIN):
                den = den + es[w]
            inv = _recip(den)
            cols = []
            for j in range(nct):
                acc = None
                for w in range(B_WIN):
                    o = HIST - w * B_DIL
                    p = es[w] * vb_ref[l, j, o:o + seg, :]
                    acc = p if acc is None else acc + p
                cols.append(acc * inv)
            outs.append(_cat(cols, axis=1).astype(BF16))
            for j in range(nct):
                kb_ref[l, j, 0:HIST, :] = k[r0 + seg - HIST:r0 + seg, j * 128:(j + 1) * 128]
                vb_ref[l, j, 0:HIST, :] = v[r0 + seg - HIST:r0 + seg, j * 128:(j + 1) * 128]
        return outs

    def b_out(ob, res):
        return res + _nn(ob, _cat([_upk(bw_ref[NB1 + j]) for j in range(nct)], axis=1))

    def o_store(b, val):
        ro = pl.multiple_of((b + 1) * seg, seg)
        o_ref[pl.ds(ro, val.shape[0]), :] = val.astype(o_ref.dtype)

    def out_copy(b):
        ro = pl.multiple_of(b * seg, seg)
        return pltpu.make_async_copy(o_ref.at[pl.ds(ro + seg, seg), :], out_hbm.at[pl.ds(ro, seg), :], sem_o)

    def step(t, hc, full, split=False):
        t_last = n_seg + LAG - 1
        if full:
            jobs = [(0, t - 1), (1, t - 1 - LAG)]

            def b_in():
                return xb_ref[0:2 * seg, :]
        else:
            lb = (t == t_last).astype(jnp.int32)
            jobs = [(lb, t - 1 - lb * (LAG + 1))]

            def b_in():
                return xb_ref[pl.ds(pl.multiple_of(lb * seg, seg), seg), :]
        nq = RQ if full else M2 + seg
        h = _cat([_upk(hc), h_ref[2 * M2:nq, :].astype(BF16)])
        scale = float(dh) ** (-0.5) * LOG2E
        if full:
            s_ = t - LAG
            rd = pl.multiple_of((s_ * (seg // 2)) & (RS // 2 - 1), seg // 2)
            wa = pl.multiple_of(((A0 - R0) // 2 + s_ * (AH // 2)) & (RS // 2 - 1), AH // 2)
        else:
            wx = pl.multiple_of(jnp.where(t < LAG, NPRE // 2 + t * (n_mem // 2), RS // 2), n_mem // 2)
            wo_store(G - 1, G - 1)

        RA = R if full else M2 + seg
        CW = R + 2 * M2 if full else R
        ri = lax.broadcasted_iota(jnp.int32, (RA, CW), 0)
        ci = lax.broadcasted_iota(jnp.int32, (RA, CW), 1)
        if not full:
            ri = jnp.where(ri >= M2, ri + seg, ri)

        def table(i, bounds, vals):
            out = vals[-1]
            for b, v in zip(reversed(bounds), reversed(vals[:-1])):
                out = jnp.where(i < b, v, out)
            return out
        qi = ri - table(ri, [16, 48, 56], [0, 8, 48, 40])
        g0 = (ci < 8) | ((ci >= 16) & (ci < 48))
        k2 = ci - table(ci, [8, 24, 32, 48, 56, 80, 88, 96, 104], [-8, 0, 24, 8, 48, 40, 72, 80, 96, 104])
        if full:
            k1 = ci - table(ci, [8, 48], [0, 8, 40])
            row_l2 = ((ri >= 8) & (ri < 16)) | (ri >= 48)
            row_xa = (ri >= 8) & (ri < 16)
            valid = row_xa == (ci >= 80)
            is_a = jnp.where(ci >= 80, ((ci >= 88) & (ci < 104)).astype(jnp.int32),
                             (g0 != row_l2).astype(jnp.int32)) > 0
            ki = jnp.where(row_l2, k2, k1)
            visible = valid & ((qi < n_mem) | (qi >= ki))
            fill = jnp.where(valid, NEG2, -jnp.inf)
        else:
            is_a = jnp.logical_not(g0)
            visible = (qi < n_mem) | (qi >= k2)
            fill = NEG2
        half = dh - 128
        la8 = lax.broadcasted_iota(jnp.int32, (n_mem, 128), 1) < half
        ones = jnp.full((n_mem, 128), 0xFFFFFFFF, U32)
        zero = jnp.zeros((n_mem, 128), U32)
        mask_a = jnp.where(la8, ones, zero)
        mask_b = jnp.where(la8, zero, ones)

        def pk2(a, b):
            return _pk(_cat([a, b]).astype(BF16))

        def proj(p, g):
            base = (g * 3 + p) * 3
            y = _nn(h, _cat([_upk(w_ref[base + j]) for j in range(3)], axis=1))
            yt = [y[:, j * 128:(j + 1) * 128] for j in range(3)]
            x1 = None
            if full:
                for j in range(3):
                    ring_ref[base + j, pl.ds(wa, AH // 2), :] = pk2(yt[j][48:56], yt[j][56:64])
                x1 = [ring_ref[base + j, pl.ds(rd, seg // 2), :] for j in range(3)]
            else:
                for j in range(3):
                    ring_ref[base + j, pl.ds(wx, n_mem // 2), :] = pk2(yt[j][0:8], yt[j][8:16])[0:n_mem // 2]
            return yt, x1

        def groups(z, j):
            y = z[0][j]
            return pk2(y[0:8], y[8:16]), pk2(y[16:24], y[24:32]), pk2(y[32:40], y[40:48])

        def q_rows(z, j):
            v0, v1, v2 = groups(z, j)
            return [v0] + ([z[1][j]] if full else []) + [v1, v2]

        def kv_tiles(z):
            yt, x1 = z
            v0, v1, v2 = groups(z, 0)
            t0 = [v0] + ([x1[0]] if full else [v1, v2]) + [v1, v2]
            y = yt[2]
            w0 = pk2(y[8:16], y[0:8])
            w1 = pk2(y[24:32], y[16:24])
            w2 = pk2(y[32:40], y[40:48])
            t2 = [w0, w1, w2] + ([x1[2]] if full else [w1, w2])
            if full:
                t0 += [v0, v1]
                t2 += [w0, w1]
            y = yt[1]

            def ab(z8):
                return jnp.where(la8, z8, 0.0), jnp.where(la8, 0.0, z8)
            xa_a, xa_b = ab(y[8:16])
            e1 = pk2(xa_b, xa_a)
            u2 = pk2(y[32:40], y[40:48])
            mid2 = [e1, pk2(y[24:32], y[16:24]) & mask_b, u2 & mask_b,
                    pk2(y[16:24], y[24:32]) & mask_a, u2 & mask_a]
            mid1 = None
            if full:
                lo, hi = x1[1][0:8], x1[1][8:16]
                mid1 = [pk2(*ab(y[0:8])), lo & mask_a, hi & mask_a, lo & mask_b, hi & mask_b,
                        e1, pk2(*ab(y[16:24]))]
            return t0, mid1, mid2, t2

        def mat(parts):
            return _upk(_cat(parts))

        def scores(q, k):
            k0, km1, km2, k2_ = kv_tiles(k)
            s_a = _nt(mat(q_rows(q, 0)), mat(k0))
            s_b = _nt(mat(q_rows(q, 2)), mat(k2_))
            qm = q_rows(q, 1)
            if full:
                s_m = _cat([_nt(mat(qm[0:2]), mat(km1)), _nt(mat(qm[2:4]), mat(km2 + km1[5:7]))])
            else:
                s_m = _nt(mat(qm), mat(km2))
            s = (jnp.where(is_a, s_a, s_b) + s_m) * scale
            s = jnp.where(visible, s, fill)
            m_a = jnp.max(jnp.where(is_a, s, -jnp.inf), axis=-1, keepdims=True)
            m_b = jnp.max(jnp.where(is_a, -jnp.inf, s), axis=-1, keepdims=True)
            e = jnp.exp2(s - jnp.where(is_a, m_a, m_b))
            d_a = jnp.sum(jnp.where(is_a, e, 0.0), axis=-1, keepdims=True)
            d_b = jnp.sum(jnp.where(is_a, 0.0, e), axis=-1, keepdims=True)
            return e * _recip(jnp.where(is_a, d_a, d_b))

        def pv(p, v):
            v0, vm1, vm2, v2 = kv_tiles(v)
            o_a = _nn(jnp.where(is_a, p, 0.0).astype(BF16), mat(v0))
            o_b = _nn(jnp.where(is_a, 0.0, p).astype(BF16), mat(v2))
            if full:
                o_m = _cat([_nn(p[0:M2 + seg].astype(BF16), mat(vm1)),
                            _nn(p[M2 + seg:R, 0:R].astype(BF16), mat(vm2))])
            else:
                o_m = _nn(p.astype(BF16), mat(vm2))
            return _cat([o_a, o_m, o_b], axis=1).astype(BF16)

        def oproj(o, g):
            return _nn(o, _cat([_upk(wo_ref[g * nct + j]) for j in range(nct)], axis=1))

        acc = [None]

        def add_o(g):
            c = oproj(os_[g], g)
            acc[0] = c if acc[0] is None else acc[0] + c

        os_ = [None] * G
        bqkv = []
        q = proj(0, 0)
        k = proj(1, 0)
        v = proj(2, 0)
        p = scores(q, k)
        blhs = _ln(b_in()).astype(BF16)
        bqkv.append(b_proj(blhs, 0))
        x2_new = None
        for g in range(G - 1):
            q = proj(0, g + 1)
            k = proj(1, g + 1)
            os_[g] = pv(p, v)
            v = proj(2, g + 1)
            p = scores(q, k)
            if g < 2:
                bqkv.append(b_proj(blhs, g + 1))
            if g == 2:
                ob = b_attn(jobs, *bqkv)
            if g == BOUT_AT:
                res = b_in()
                if split:
                    x2_new = b_out(ob[0], res[0:seg])
                elif full:
                    zb = b_out(_cat(ob), res)
                    x2_new = zb[0:seg]
                    o_store(t - 1 - LAG, zb[seg:2 * seg])
                else:
                    x2_new = b_out(ob[0], res)
                    o_store(lb * (t_last - LAG - 1) - 1, x2_new)
            if g - WLAG >= 0:
                add_o(g - WLAG)
        for g in range(G - 1 - WLAG, G - 2):
            add_o(g)
        os_[G - 1] = pv(p, v)
        add_o(G - 2)
        add_o(G - 1)
        acc = acc[0]
        if split:
            o_store(t - 1 - LAG, b_out(ob[1], res[seg:2 * seg]))

        y2 = x2_ref[...] + _cat([acc[n_mem:M2], acc[RA - seg + n_mem:RA]])
        mem2 = acc[RA - seg:RA - seg + n_mem]
        if full:
            x_cur = x_ref[pl.ds(pl.multiple_of(t * seg, seg), seg), :].astype(F32)
            xb_ref[0:seg, :] = x_cur + acc[M2:M2 + seg]
            xb_ref[seg:2 * seg, :] = y2
            m1n = acc[0:n_mem]
            m2n = mem2
            an = pl.multiple_of(jnp.minimum(A0 + (t + 1 - LAG) * AH, S - AH), AH)
            h_ref[M2 + seg:RQ, :] = _ln(x_ref[pl.ds(an, AH), :].astype(F32))
            nxt = x2_new
        else:
            xb_ref[pl.ds(pl.multiple_of(jnp.where(t < LAG, 0, (t - n_seg + 2) * seg), seg), seg), :] = y2
            m1n = jnp.where(t < LAG - 1, xln_rows(R0 + NPRE, M2).astype(F32)[n_mem:M2], mem2)
            m2n = jnp.where(t == LAG - 1, mem0_ref[...].astype(F32), mem2)
            nxt = jnp.where(t < LAG - 1, x_ref[seg:2 * seg, :].astype(F32), x2_new)
        x2_ref[...] = nxt
        sl = _ln(nxt)
        h_ref[2 * M2:M2 + seg, :] = sl[M2:seg]
        return _pk(_cat([m1n, sl[0:n_mem], m2n, sl[n_mem:M2]]).astype(BF16))

    def single_body(t, c):
        @pl.when(t >= n_seg)
        def _():
            out_copy(t - (LAG + 3)).start()
        return step(t, c, False)

    def full_body(i, c):
        t = LAG + UNROLL * i
        for u in range(UNROLL):
            @pl.when(t - u >= LAG + 2)
            def _():
                out_copy(t - u - (LAG + 2)).start()
        for u in range(UNROLL):
            c = step(t + u, c, True, split=u < UNROLL - 1)
        return c

    def phase(ph, c):
        t0 = ph * n_seg
        c = lax.fori_loop(t0, t0 + LAG, single_body, c)
        return lax.fori_loop(0, jnp.where(ph == 0, (n_seg - LAG) // UNROLL, 0), full_body, c)
    lax.fori_loop(0, 2, phase, _pk(h_ref[0:2 * M2, :].astype(BF16)))

    out_copy(n_seg - 3).start()
    res = xb_ref[2 * seg:4 * seg, :]
    blhs = _ln(res).astype(BF16)
    ob = b_attn([(1, n_seg - 2), (1, n_seg - 1)], *[b_proj(blhs, part) for part in range(3)])
    o_store(n_seg - 2, b_out(_cat(ob), res))
    out_copy(n_seg - 2).start()
    out_copy(n_seg - 1).start()
    pltpu.make_async_copy(o_ref.at[pl.ds(seg, S), :], out_hbm, sem_o).wait()


@functools.partial(jax.jit, static_argnames=("seg",))
def _run(A_x, A_mem0, A_Wq, A_Wk, A_Wv, A_Wo, B_wqkv, B_wo, *, seg):
    _, S, dm = A_x.shape
    n_heads, dh = A_Wq.shape[1], A_Wq.shape[2]
    n_mem = A_mem0.shape[1]
    n_seg = S // seg
    hd = n_heads * dh
    nct = dm // 128
    assert (seg, n_seg, n_mem, dh, dm % 128, n_heads, LAG, UNROLL) == (32, 64, 8, 192, 0, 32, 2, 2)

    x = A_x.reshape(S, dm)
    mem0 = A_mem0.reshape(n_mem, dm)
    wq = jnp.transpose(A_Wq, (1, 2, 0)).reshape(hd, dm)
    wk = jnp.transpose(A_Wk, (1, 2, 0)).reshape(hd, dm)
    wv = jnp.transpose(A_Wv, (1, 2, 0)).reshape(hd, dm)
    wo = A_Wo.reshape(hd, dm)
    _, _, _, _, rs, xc = _plan(seg, n_seg)

    kern = functools.partial(_kernel, seg=seg, n_seg=n_seg, n_mem=n_mem,
                             n_heads=n_heads, dh=dh, dm=dm)
    hbm = pl.BlockSpec(memory_space=pltpu.HBM)

    out = pl.pallas_call(
        kern,
        in_specs=[hbm] * 8,
        out_specs=hbm,
        out_shape=jax.ShapeDtypeStruct((S, dm), A_x.dtype),
        scratch_shapes=[
            pltpu.VMEM((S, dm), BF16),
            pltpu.VMEM((n_mem, dm), BF16),
            pltpu.VMEM((NSLOT, 4, 2 * dh, dm), BF16),
            pltpu.VMEM((3 * hd // 128, dm // 2, 128), U32),
            pltpu.VMEM((n_heads // 2 * nct, dh, 128), U32),
            pltpu.VMEM((dm, 4 * dm + 128), BF16),
            pltpu.VMEM((nct, 5 * dm + 32, 128), F32),
            pltpu.VMEM((4 * nct + 1, dm // 2, 128), U32),
            pltpu.VMEM((nct, NXC * xc // 2, 128), U32),
            pltpu.VMEM((3 * hd // 128, rs // 2 + 8, 128), U32),
            pltpu.VMEM((2 * n_mem + seg + AH, dm), F32),
            pltpu.VMEM((4 * seg, dm), F32),
            pltpu.VMEM((seg, dm), F32),
            pltpu.VMEM((2, nct, HIST + seg, 128), F32),
            pltpu.VMEM((2, nct, HIST + seg, 128), F32),
            pltpu.VMEM((S + seg, dm), A_x.dtype),
            pltpu.SemaphoreType.DMA((2, NSLOT)),
            pltpu.SemaphoreType.DMA((3 + NXC,)),
            pltpu.SemaphoreType.DMA(()),
        ],
        compiler_params=pltpu.CompilerParams(
            vmem_limit_bytes=120 * 1024 * 1024,
            disable_bounds_checks=True,
        ),
    )(x, mem0, wq, wk, wv, wo, B_wqkv, B_wo)
    return out.reshape(1, S, dm)


def pallas_interleave_layers__memory_aug_recurrent_mem_tr__sliding_local_dilated__prompt_kernel(
    A_x: jax.Array,
    A_mem0: jax.Array,
    A_Wq: jax.Array,
    A_Wk: jax.Array,
    A_Wv: jax.Array,
    A_Wo: jax.Array,
    A_seg_len,
    B_x: jax.Array,
    B_wqkv: jax.Array,
    B_wo: jax.Array,
):
    del B_x
    seg = A_seg_len if isinstance(A_seg_len, int) else 32
    return _run(A_x, A_mem0, A_Wq, A_Wk, A_Wv, A_Wo, B_wqkv, B_wo, seg=seg)
```

```python
import functools

import jax
import jax.numpy as jnp
from jax import lax
import jax.experimental.pallas as pl
import jax.experimental.pallas.tpu as pltpu

F32 = jnp.float32
BF16 = jnp.bfloat16
U32 = jnp.uint32
NEG = -1000000000.0
LN_EPS = 1e-05
LOG2E = 1.4426950408889634
NEG2 = NEG * LOG2E

B_HEADS = 32
B_WIN = 8
B_DIL = 2
HIST = 16
AHS = (32, 16)
LAG = 2
NSLOT = 4
WLAG = 2
BOUT_AT = 8
NXC = 3
UNROLL = 2


def _ln(x):
    m = jnp.mean(x, axis=-1, keepdims=True)
    c = x - m
    v = jnp.mean(c * c, axis=-1, keepdims=True)
    return c * lax.rsqrt(v + LN_EPS)


def _recip(d):
    r = pl.reciprocal(d, approx=True)
    return r * (2.0 - d * r)


def _nt(a, b):
    return lax.dot_general(a, b, (((1,), (1,)), ((), ())), preferred_element_type=F32)


def _nn(a, b):
    return jnp.dot(a, b, preferred_element_type=F32)


def _cat(xs, axis=0):
    return xs[0] if len(xs) == 1 else jnp.concatenate(xs, axis=axis)


def _pk(z):
    return pltpu.bitcast(z, U32)


def _upk(z):
    return pltpu.bitcast(z, BF16)


def _plan(seg, n_seg):
    S = seg * n_seg
    R0 = LAG * seg
    A0 = S - (n_seg - LAG) // UNROLL * sum(AHS)
    NPRE = A0 - R0 - LAG * 8
    RS = 1 << (A0 - R0 + AHS[0] - 1).bit_length()
    XC = NPRE // NXC
    assert XC % 16 == 0 and XC * NXC == NPRE
    return S, R0, A0, NPRE, RS, XC


def _kernel(x_hbm, mem0_hbm, wq_hbm, wk_hbm, wv_hbm, wo_hbm, bqkv_hbm, bwo_hbm,
            out_hbm,
            x_ref, mem0_ref, stage_ref, w_ref, wo_ref, bst_ref, btmp_ref, bw_ref,
            xln_ref, ring_ref, h_ref, xb_ref, x2_ref, kb_ref, vb_ref, o_ref,
            sem_w, sem_m, sem_b, sem_o,
            *, seg, n_seg, n_mem, n_heads, dh, dm):
    S, R0, A0, NPRE, RS, XC = _plan(seg, n_seg)
    M2 = 2 * n_mem
    R = M2 + 2 * seg
    RB = M2 + seg
    PW = 2 * dh
    G = n_heads // 2
    nct = dm // 128
    bdh = dm // B_HEADS
    w_hbm = (wq_hbm, wk_hbm, wv_hbm, wo_hbm)

    def w_copy(p, g, sem=None):
        slot = g & (NSLOT - 1)
        src = g - 1 if p == 3 else g
        return pltpu.make_async_copy(w_hbm[p].at[pl.ds(src * PW, PW), :], stage_ref.at[slot, p],
                                     sem_w.at[slot] if sem is None else sem)

    NB1 = 3 * nct
    WO0 = 3 * dm
    DUM = 4 * dm
    XF = A0 + AHS[0]

    def rows_copy(r0, n, sem):
        return pltpu.make_async_copy(x_hbm.at[pl.ds(r0, n), :], x_ref.at[pl.ds(r0, n), :], sem)

    def x_copy(i):
        return rows_copy(pl.multiple_of(R0 + i * XC, 16), XC, sem_m.at[7 + i])

    small = [rows_copy(0, R0, sem_m.at[1]), rows_copy(R0 + NPRE, XF - R0 - NPRE, sem_m.at[2]),
             pltpu.make_async_copy(mem0_hbm, mem0_ref, sem_m.at[3])]
    x_late = rows_copy(XF, S - XF, sem_m.at[0])

    def bq_copy(part):
        c0 = pl.multiple_of(part * dm, 128)
        return pltpu.make_async_copy(bqkv_hbm.at[:, pl.ds(c0, dm)], bst_ref.at[:, pl.ds(c0, dm)], sem_b.at[part])

    bo_copy = pltpu.make_async_copy(bwo_hbm, bst_ref.at[:, pl.ds(3 * dm, dm)], sem_b.at[3])

    def bst_tile(c):
        return bst_ref[:, pl.ds(pl.multiple_of(c * 128, 128), 128)]

    for i in range(NXC):
        x_copy(i).start()
    for cp in small:
        cp.start()

    def zero_body(j, c):
        btmp_ref[j, DUM:, :] = jnp.zeros((btmp_ref.shape[1] - DUM, 128), F32)
        return c
    lax.fori_loop(0, nct, zero_body, 0)

    for p in range(3):
        w_copy(p, 0, sem_m.at[4 + p]).start()
    for p in range(4):
        w_copy(p, 1).start()
    xb_ref[0:2 * seg, :] = jnp.zeros((2 * seg, dm), F32)
    kb_ref[...] = jnp.zeros(kb_ref.shape, F32)
    vb_ref[...] = jnp.zeros(vb_ref.shape, F32)
    bst_ref[:, 4 * dm:] = jnp.zeros((dm, 128), BF16)

    def ln_body(i, c):
        x_copy(i).wait()
        y = _ln(x_ref[pl.ds(pl.multiple_of(R0 + i * XC, 16), XC), :].astype(F32))
        r0 = pl.multiple_of(i * (XC // 2), 8)
        for j in range(nct):
            xln_ref[j, pl.ds(r0, XC // 2), :] = _pk(y[:, j * 128:(j + 1) * 128].astype(BF16))
        return c
    lax.fori_loop(0, NXC, ln_body, 0)
    for cp in small:
        cp.wait()
    for p in range(4):
        w_copy(p, 2).start()

    def pre_chunk(c, w, nn):
        xl = _cat([_upk(xln_ref[j]) for j in range(nct)], axis=1)
        wt = w.T
        y = _nn(xl, wt) if nn else _nt(xl, w)
        for j in range(3):
            ring_ref[c * 3 + j, 0:NPRE // 2, :] = _pk(y[:, j * 128:(j + 1) * 128].astype(BF16))
            w_ref[c * 3 + j] = _pk(wt[:, j * 128:(j + 1) * 128])

    def init_rows():
        x0 = x_ref[0:seg, :].astype(F32)
        sl = _ln(x0)
        xt = _ln(x_ref[R0 + NPRE:XF, :].astype(F32))
        h_ref[0:n_mem, :] = xt[0:n_mem]
        h_ref[n_mem:M2, :] = sl[0:n_mem]
        h_ref[M2:M2 + n_mem, :] = mem0_ref[...].astype(F32)
        h_ref[M2 + n_mem:RB, :] = sl[n_mem:seg]
        h_ref[RB:RB + AHS[0], :] = xt[M2:M2 + AHS[0]]
        h_ref[RB + AHS[0]:RB + AHS[0] + n_mem, :] = xt[n_mem:M2]
        x2_ref[...] = x0

    def first_body(p, c):
        buf = stage_ref.at[0, p]
        pltpu.make_async_copy(buf, buf, sem_m.at[4 + p]).wait()
        init_rows()
        pre_chunk(p, stage_ref[0, p], False)
        return c
    lax.fori_loop(0, 3, first_body, 0)

    dpt = 128 // B_HEADS

    def b_stage1(u):
        ok = (u >= 0) & (u < NB1)
        tr = bst_tile(jnp.where(ok, u, NB1 + nct)).astype(F32).T
        r0 = pl.multiple_of(jnp.where(ok, u * 128, DUM), 128)
        for j in range(nct):
            btmp_ref[j, pl.ds(r0, 128), :] = tr[:, j * 128:(j + 1) * 128]

    def b_stage1_wo(u):
        ok = (u >= 0) & (u < nct)
        r0 = pl.multiple_of(jnp.where(ok, WO0, DUM), 128)
        btmp_ref[jnp.where(ok, u, 0), pl.ds(r0, dm), :] = bst_tile(
            jnp.where(ok, NB1 + u, NB1 + nct)).astype(F32)

    def b_stage2(u):
        ok = (u >= 0) & (u < NB1)
        part = (u >= nct).astype(jnp.int32) + (u >= 2 * nct).astype(jnp.int32)
        r0 = jnp.where(ok, part * dm + (u - part * nct) * dpt, DUM)
        rows = _cat([_cat([btmp_ref[j, pl.ds(r0 + dd, B_HEADS, stride=bdh), :]
                           for j in range(nct)], axis=1) for dd in range(dpt)])
        bw_ref[jnp.where(ok, u, NB1 + nct)] = _pk(rows.T.astype(BF16))

    def b_stage2_wo(u):
        ok = (u >= 0) & (u < nct)
        r0 = jnp.where(ok, WO0, DUM)
        jj = jnp.where(ok, u, 0)
        bw_ref[jnp.where(ok, NB1 + u, NB1 + nct)] = _pk(
            _cat([btmp_ref[jj, pl.ds(r0 + d, B_HEADS, stride=bdh), :] for d in range(bdh)]).astype(BF16))

    def wo_store(g):
        w = stage_ref[g & (NSLOT - 1), 3]
        for j in range(nct):
            wo_ref[(g - 1) * nct + j] = _pk(w[:, j * 128:(j + 1) * 128])

    wo_last = w_copy(3, G)

    def pre_body(g, c):
        slot = g & (NSLOT - 1)
        buf = stage_ref.at[slot]
        pltpu.make_async_copy(buf, buf, sem_w.at[slot]).wait()

        @pl.when((g >= 3) & (g <= 5))
        def _():
            bq_copy(g - 3).wait()

        @pl.when(g == 6)
        def _():
            bo_copy.wait()

        @pl.when(g + 2 < G)
        def _():
            for p in range(4):
                w_copy(p, g + 2).start()

        @pl.when(g <= 3)
        def _():
            bq_copy(g - 1).start()

        @pl.when(g == 4)
        def _():
            bo_copy.start()

        @pl.when(g == G - 2)
        def _():
            wo_last.start()
            x_late.start()

        wo_store(g)
        b_stage2(2 * (g - 8))
        b_stage2(2 * (g - 8) + 1)
        b_stage2_wo(g - 11)
        b_stage1(2 * (g - 3))
        b_stage1(2 * (g - 3) + 1)
        b_stage1_wo(g - 6)
        for p in range(3):
            pre_chunk(g * 3 + p, stage_ref[slot, p], p == 2)
        return c
    lax.fori_loop(1, G, pre_body, 0)
    wo_last.wait()

    bscale = float(bdh) ** (-0.5) * LOG2E

    def b_proj(lhs, part):
        return _nn(lhs, _cat([_upk(bw_ref[part * nct + j]) for j in range(nct)], axis=1))

    def b_attn(jobs, q, k, v):
        row = lax.broadcasted_iota(jnp.int32, (seg, 128), 0)
        outs = []
        for i, (l, sidx) in enumerate(jobs):
            r0 = i * seg
            pos = row + sidx * seg
            for j in range(nct):
                kb_ref[l, j, HIST:HIST + seg, :] = k[r0:r0 + seg, j * 128:(j + 1) * 128]
                vb_ref[l, j, HIST:HIST + seg, :] = v[r0:r0 + seg, j * 128:(j + 1) * 128]
            logits = []
            for w in range(B_WIN):
                o = HIST - w * B_DIL
                acc = None
                for j in range(nct):
                    p = q[r0:r0 + seg, j * 128:(j + 1) * 128] * kb_ref[l, j, o:o + seg, :]
                    acc = p if acc is None else acc + p
                acc = acc + pltpu.roll(acc, 64, 1)
                acc = acc + pltpu.roll(acc, 32, 1)
                lg = acc * bscale
                if w > 0:
                    lg = jnp.where(pos >= w * B_DIL, lg, NEG2)
                logits.append(lg)
            m = logits[0]
            for w in range(1, B_WIN):
                m = jnp.maximum(m, logits[w])
            es = [jnp.exp2(lg - m) for lg in logits]
            den = es[0]
            for w in range(1, B_WIN):
                den = den + es[w]
            inv = _recip(den)
            cols = []
            for j in range(nct):
                acc = None
                for w in range(B_WIN):
                    o = HIST - w * B_DIL
                    p = es[w] * vb_ref[l, j, o:o + seg, :]
                    acc = p if acc is None else acc + p
                cols.append(acc * inv)
            outs.append(_cat(cols, axis=1).astype(BF16))
            for j in range(nct):
                kb_ref[l, j, 0:HIST, :] = k[r0 + seg - HIST:r0 + seg, j * 128:(j + 1) * 128]
                vb_ref[l, j, 0:HIST, :] = v[r0 + seg - HIST:r0 + seg, j * 128:(j + 1) * 128]
        return outs

    def b_out(ob, res):
        return res + _nn(ob, _cat([_upk(bw_ref[NB1 + j]) for j in range(nct)], axis=1))

    def o_store(b, val):
        ro = pl.multiple_of((b + 1) * seg, seg)
        o_ref[pl.ds(ro, val.shape[0]), :] = val.astype(o_ref.dtype)

    def out_copy(b):
        ro = pl.multiple_of(b * seg, seg)
        return pltpu.make_async_copy(o_ref.at[pl.ds(ro + seg, seg), :], out_hbm.at[pl.ds(ro, seg), :], sem_o)

    def step(t, hc, full, u=0, i=None):
        t_last = n_seg + LAG - 1
        if full:
            jobs = [(0, t - 1), (1, t - 1 - LAG)]

            def b_in():
                return xb_ref[0:2 * seg, :]
        else:
            lb = (t == t_last).astype(jnp.int32)
            jobs = [(lb, t - 1 - lb * (LAG + 1))]

            def b_in():
                return xb_ref[pl.ds(pl.multiple_of(lb * seg, seg), seg), :]
        split = full and u < UNROLL - 1
        nq = RB + AHS[u] if full else RB
        h = _cat([_upk(hc), h_ref[2 * M2:nq, :].astype(BF16)])
        scale = float(dh) ** (-0.5) * LOG2E
        if full:
            s_ = t - LAG
            rd = pl.multiple_of((s_ * (seg // 2)) & (RS // 2 - 1), seg // 2)
            a_off = i * sum(AHS) + sum(AHS[:u])
            wa = [pl.multiple_of(((A0 - R0 + a_off) // 2 + 8 * a) & (RS // 2 - 1), 8)
                  for a in range(AHS[u] // 16)]
        else:
            wx = pl.multiple_of(jnp.where(t < LAG, NPRE // 2 + t * (n_mem // 2), RS // 2), n_mem // 2)
            wo_store(G)

        RA = R if full else M2 + seg
        CW = R + 2 * M2 if full else R
        ri = lax.broadcasted_iota(jnp.int32, (RA, CW), 0)
        ci = lax.broadcasted_iota(jnp.int32, (RA, CW), 1)
        if not full:
            ri = jnp.where(ri >= M2, ri + seg, ri)

        def table(i, bounds, vals):
            out = vals[-1]
            for b, v in zip(reversed(bounds), reversed(vals[:-1])):
                out = jnp.where(i < b, v, out)
            return out
        qi = ri - table(ri, [16, 48, 56], [0, 8, 48, 40])
        g0 = (ci < 8) | ((ci >= 16) & (ci < 48))
        k2 = ci - table(ci, [8, 24, 32, 48, 56, 80, 88, 96, 104], [-8, 0, 24, 8, 48, 40, 72, 80, 96, 104])
        if full:
            k1 = ci - table(ci, [8, 48], [0, 8, 40])
            row_l2 = ((ri >= 8) & (ri < 16)) | (ri >= 48)
            row_xa = (ri >= 8) & (ri < 16)
            valid = row_xa == (ci >= 80)
            is_a = jnp.where(ci >= 80, ((ci >= 88) & (ci < 104)).astype(jnp.int32),
                             (g0 != row_l2).astype(jnp.int32)) > 0
            ki = jnp.where(row_l2, k2, k1)
            visible = valid & ((qi < n_mem) | (qi >= ki))
            fill = jnp.where(valid, NEG2, -jnp.inf)
        else:
            is_a = jnp.logical_not(g0)
            visible = (qi < n_mem) | (qi >= k2)
            fill = NEG2
        half = dh - 128
        la8 = lax.broadcasted_iota(jnp.int32, (n_mem, 128), 1) < half
        ones = jnp.full((n_mem, 128), 0xFFFFFFFF, U32)
        zero = jnp.zeros((n_mem, 128), U32)
        mask_a = jnp.where(la8, ones, zero)
        mask_b = jnp.where(la8, zero, ones)

        def pk2(a, b):
            return _pk(_cat([a, b]).astype(BF16))

        def proj(p, g):
            base = (g * 3 + p) * 3
            y = _nn(h, _cat([_upk(w_ref[base + j]) for j in range(3)], axis=1))
            yt = [y[:, j * 128:(j + 1) * 128] for j in range(3)]
            x1 = None
            if full:
                for j in range(3):
                    for a in range(AHS[u] // 16):
                        r = RB + 16 * a
                        ring_ref[base + j, pl.ds(wa[a], 8), :] = pk2(yt[j][r:r + 8], yt[j][r + 8:r + 16])
                x1 = [ring_ref[base + j, pl.ds(rd, seg // 2), :] for j in range(3)]
            else:
                for j in range(3):
                    ring_ref[base + j, pl.ds(wx, n_mem // 2), :] = pk2(yt[j][0:8], yt[j][8:16])[0:n_mem // 2]
            return yt, x1

        def groups(z, j):
            y = z[0][j]
            return pk2(y[0:8], y[8:16]), pk2(y[16:24], y[24:32]), pk2(y[32:40], y[40:48])

        def q_rows(z, j):
            v0, v1, v2 = groups(z, j)
            return [v0] + ([z[1][j]] if full else []) + [v1, v2]

        def kv_tiles(z):
            yt, x1 = z
            v0, v1, v2 = groups(z, 0)
            t0 = [v0] + ([x1[0]] if full else [v1, v2]) + [v1, v2]
            y = yt[2]
            w0 = pk2(y[8:16], y[0:8])
            w1 = pk2(y[24:32], y[16:24])
            w2 = pk2(y[32:40], y[40:48])
            t2 = [w0, w1, w2] + ([x1[2]] if full else [w1, w2])
            if full:
                t0 += [v0, v1]
                t2 += [w0, w1]
            y = yt[1]

            def ab(z8):
                return jnp.where(la8, z8, 0.0), jnp.where(la8, 0.0, z8)
            xa_a, xa_b = ab(y[8:16])
            e1 = pk2(xa_b, xa_a)
            u2 = pk2(y[32:40], y[40:48])
            mid2 = [e1, pk2(y[24:32], y[16:24]) & mask_b, u2 & mask_b,
                    pk2(y[16:24], y[24:32]) & mask_a, u2 & mask_a]
            mid1 = None
            if full:
                lo, hi = x1[1][0:8], x1[1][8:16]
                mid1 = [pk2(*ab(y[0:8])), lo & mask_a, hi & mask_a, lo & mask_b, hi & mask_b,
                        e1, pk2(*ab(y[16:24]))]
            return t0, mid1, mid2, t2

        def mat(parts):
            return _upk(_cat(parts))

        def scores(q, k):
            k0, km1, km2, k2_ = kv_tiles(k)
            s_a = _nt(mat(q_rows(q, 0)), mat(k0))
            s_b = _nt(mat(q_rows(q, 2)), mat(k2_))
            qm = q_rows(q, 1)
            if full:
                s_m = _cat([_nt(mat(qm[0:2]), mat(km1)), _nt(mat(qm[2:4]), mat(km2 + km1[5:7]))])
            else:
                s_m = _nt(mat(qm), mat(km2))
            s = (jnp.where(is_a, s_a, s_b) + s_m) * scale
            s = jnp.where(visible, s, fill)
            m_a = jnp.max(jnp.where(is_a, s, -jnp.inf), axis=-1, keepdims=True)
            m_b = jnp.max(jnp.where(is_a, -jnp.inf, s), axis=-1, keepdims=True)
            e = jnp.exp2(s - jnp.where(is_a, m_a, m_b))
            d_a = jnp.sum(jnp.where(is_a, e, 0.0), axis=-1, keepdims=True)
            d_b = jnp.sum(jnp.where(is_a, 0.0, e), axis=-1, keepdims=True)
            return e * _recip(jnp.where(is_a, d_a, d_b))

        def pv(p, v):
            v0, vm1, vm2, v2 = kv_tiles(v)
            o_a = _nn(jnp.where(is_a, p, 0.0).astype(BF16), mat(v0))
            o_b = _nn(jnp.where(is_a, 0.0, p).astype(BF16), mat(v2))
            if full:
                o_m = _cat([_nn(p[0:M2 + seg].astype(BF16), mat(vm1)),
                            _nn(p[M2 + seg:R, 0:R].astype(BF16), mat(vm2))])
            else:
                o_m = _nn(p.astype(BF16), mat(vm2))
            return _cat([o_a, o_m, o_b], axis=1).astype(BF16)

        def oproj(o, g):
            return _nn(o, _cat([_upk(wo_ref[g * nct + j]) for j in range(nct)], axis=1))

        acc = [None]

        def add_o(g):
            c = oproj(os_[g], g)
            acc[0] = c if acc[0] is None else acc[0] + c

        os_ = [None] * G
        bqkv = [None] * 3
        q = proj(0, 0)
        k = proj(1, 0)
        v = proj(2, 0)
        p = scores(q, k)
        blhs = _ln(b_in()).astype(BF16)
        bqkv[2] = b_proj(blhs, 2)
        x2_new = None
        for g in range(G - 1):
            q = proj(0, g + 1)
            k = proj(1, g + 1)
            os_[g] = pv(p, v)
            v = proj(2, g + 1)
            p = scores(q, k)
            if g < 2:
                bqkv[1 - g] = b_proj(blhs, 1 - g)
            if g == 2:
                ob = b_attn(jobs, *bqkv)
            if g == BOUT_AT:
                res = b_in()
                if split:
                    x2_new = b_out(ob[0], res[0:seg])
                elif full:
                    zb = b_out(_cat(ob), res)
                    x2_new = zb[0:seg]
                    o_store(t - 1 - LAG, zb[seg:2 * seg])
                else:
                    x2_new = b_out(ob[0], res)
                    o_store(lb * (t_last - LAG - 1) - 1, x2_new)
            if g - WLAG >= 0:
                add_o(g - WLAG)
        for g in range(G - 1 - WLAG, G - 2):
            add_o(g)
        os_[G - 1] = pv(p, v)
        add_o(G - 2)
        add_o(G - 1)
        acc = acc[0]
        if split:
            o_store(t - 1 - LAG, b_out(ob[1], res[seg:2 * seg]))

        y2 = x2_ref[...] + _cat([acc[n_mem:M2], acc[RA - seg + n_mem:RA]])
        mem2 = acc[RA - seg:RA - seg + n_mem]
        if full:
            x_cur = x_ref[pl.ds(pl.multiple_of(t * seg, seg), seg), :].astype(F32)
            xb_ref[0:seg, :] = x_cur + acc[M2:M2 + seg]
            xb_ref[seg:2 * seg, :] = y2
            m1n = acc[0:n_mem]
            m2n = mem2
            ahn = AHS[(u + 1) % UNROLL]
            an = pl.multiple_of(jnp.minimum(A0 + a_off + AHS[u], S - ahn), 16)
            h_ref[RB:RB + ahn, :] = _ln(x_ref[pl.ds(an, ahn), :].astype(F32))
            nxt = x2_new
        else:
            xb_ref[pl.ds(pl.multiple_of(jnp.where(t < LAG, 0, (t - n_seg + 2) * seg), seg), seg), :] = y2
            m1n = jnp.where(t < LAG - 1, h_ref[RB + AHS[0]:RB + AHS[0] + n_mem, :], mem2)
            m2n = jnp.where(t == LAG - 1, mem0_ref[...].astype(F32), mem2)
            nxt = jnp.where(t < LAG - 1, x_ref[seg:2 * seg, :].astype(F32), x2_new)
        x2_ref[...] = nxt
        sl = _ln(nxt)
        h_ref[2 * M2:M2 + seg, :] = sl[M2:seg]
        return _pk(_cat([m1n, sl[0:n_mem], m2n, sl[n_mem:M2]]).astype(BF16))

    def single_body(t, c):
        @pl.when(t >= n_seg)
        def _():
            out_copy(t - (LAG + 3)).start()
        return step(t, c, False)

    def full_body(i, c):
        t = LAG + UNROLL * i
        for u in range(UNROLL):
            @pl.when(t - u >= LAG + 2)
            def _():
                out_copy(t - u - (LAG + 2)).start()
        for u in range(UNROLL):
            c = step(t + u, c, True, u, i)
        return c

    def phase(ph, c):
        t0 = ph * n_seg
        c = lax.fori_loop(t0, t0 + LAG, single_body, c)

        @pl.when(ph == 0)
        def _():
            x_late.wait()
        return lax.fori_loop(0, jnp.where(ph == 0, (n_seg - LAG) // UNROLL, 0), full_body, c)
    lax.fori_loop(0, 2, phase, _pk(h_ref[0:2 * M2, :].astype(BF16)))

    out_copy(n_seg - 3).start()
    res = xb_ref[2 * seg:4 * seg, :]
    blhs = _ln(res).astype(BF16)
    ob = b_attn([(1, n_seg - 2), (1, n_seg - 1)], *[b_proj(blhs, part) for part in range(3)])
    o_store(n_seg - 2, b_out(_cat(ob), res))
    out_copy(n_seg - 2).start()
    out_copy(n_seg - 1).start()
    pltpu.make_async_copy(o_ref.at[pl.ds(seg, S), :], out_hbm, sem_o).wait()


@functools.partial(jax.jit, static_argnames=("seg",))
def _run(A_x, A_mem0, A_Wq, A_Wk, A_Wv, A_Wo, B_wqkv, B_wo, *, seg):
    _, S, dm = A_x.shape
    n_heads, dh = A_Wq.shape[1], A_Wq.shape[2]
    n_mem = A_mem0.shape[1]
    n_seg = S // seg
    hd = n_heads * dh
    nct = dm // 128
    assert (seg, n_seg, n_mem, dh, dm % 128, n_heads, LAG, UNROLL) == (32, 64, 8, 192, 0, 32, 2, 2)

    x = A_x.reshape(S, dm)
    mem0 = A_mem0.reshape(n_mem, dm)
    wq = jnp.transpose(A_Wq, (1, 2, 0)).reshape(hd, dm)
    wk = jnp.transpose(A_Wk, (1, 2, 0)).reshape(hd, dm)
    wv = jnp.transpose(A_Wv, (1, 2, 0)).reshape(hd, dm)
    wo = A_Wo.reshape(hd, dm)
    _, _, _, _, rs, xc = _plan(seg, n_seg)

    kern = functools.partial(_kernel, seg=seg, n_seg=n_seg, n_mem=n_mem,
                             n_heads=n_heads, dh=dh, dm=dm)
    hbm = pl.BlockSpec(memory_space=pltpu.HBM)

    out = pl.pallas_call(
        kern,
        in_specs=[hbm] * 8,
        out_specs=hbm,
        out_shape=jax.ShapeDtypeStruct((S, dm), A_x.dtype),
        scratch_shapes=[
            pltpu.VMEM((S, dm), BF16),
            pltpu.VMEM((n_mem, dm), BF16),
            pltpu.VMEM((NSLOT, 4, 2 * dh, dm), BF16),
            pltpu.VMEM((3 * hd // 128, dm // 2, 128), U32),
            pltpu.VMEM((n_heads // 2 * nct, dh, 128), U32),
            pltpu.VMEM((dm, 4 * dm + 128), BF16),
            pltpu.VMEM((nct, 5 * dm + 32, 128), F32),
            pltpu.VMEM((4 * nct + 1, dm // 2, 128), U32),
            pltpu.VMEM((nct, NXC * xc // 2, 128), U32),
            pltpu.VMEM((3 * hd // 128, rs // 2 + 8, 128), U32),
            pltpu.VMEM((3 * n_mem + seg + AHS[0], dm), F32),
            pltpu.VMEM((4 * seg, dm), F32),
            pltpu.VMEM((seg, dm), F32),
            pltpu.VMEM((2, nct, HIST + seg, 128), F32),
            pltpu.VMEM((2, nct, HIST + seg, 128), F32),
            pltpu.VMEM((S + seg, dm), A_x.dtype),
            pltpu.SemaphoreType.DMA((NSLOT,)),
            pltpu.SemaphoreType.DMA((7 + NXC,)),
            pltpu.SemaphoreType.DMA((4,)),
            pltpu.SemaphoreType.DMA(()),
        ],
        compiler_params=pltpu.CompilerParams(
            vmem_limit_bytes=120 * 1024 * 1024,
            disable_bounds_checks=True,
        ),
    )(x, mem0, wq, wk, wv, wo, B_wqkv, B_wo)
    return out.reshape(1, S, dm)


def pallas_interleave_layers__memory_aug_recurrent_mem_tr__sliding_local_dilated__prompt_kernel(
    A_x: jax.Array,
    A_mem0: jax.Array,
    A_Wq: jax.Array,
    A_Wk: jax.Array,
    A_Wv: jax.Array,
    A_Wo: jax.Array,
    A_seg_len,
    B_x: jax.Array,
    B_wqkv: jax.Array,
    B_wo: jax.Array,
):
    del B_x
    seg = A_seg_len if isinstance(A_seg_len, int) else 32
    return _run(A_x, A_mem0, A_Wq, A_Wk, A_Wv, A_Wo, B_wqkv, B_wo, seg=seg)
```

```python
import functools

import jax
import jax.numpy as jnp
from jax import lax
import jax.experimental.pallas as pl
import jax.experimental.pallas.tpu as pltpu

F32 = jnp.float32
BF16 = jnp.bfloat16
U32 = jnp.uint32
NEG = -1000000000.0
LN_EPS = 1e-05
LOG2E = 1.4426950408889634
NEG2 = NEG * LOG2E

B_HEADS = 32
B_WIN = 8
B_DIL = 2
HIST = 16
AHS = (32, 16)
LAG = 2
NSLOT = 4
WLAG = 2
BOUT_AT = 8
NXC = 3
UNROLL = 2


def _ln(x):
    m = jnp.mean(x, axis=-1, keepdims=True)
    c = x - m
    v = jnp.mean(c * c, axis=-1, keepdims=True)
    return c * lax.rsqrt(v + LN_EPS)


def _recip(d):
    r = pl.reciprocal(d, approx=True)
    return r * (2.0 - d * r)


def _nt(a, b):
    return lax.dot_general(a, b, (((1,), (1,)), ((), ())), preferred_element_type=F32)


def _nn(a, b):
    return jnp.dot(a, b, preferred_element_type=F32)


def _cat(xs, axis=0):
    return xs[0] if len(xs) == 1 else jnp.concatenate(xs, axis=axis)


def _pk(z):
    return pltpu.bitcast(z, U32)


def _upk(z):
    return pltpu.bitcast(z, BF16)


def _base_tiles(W):
    col = [W[j][j] - sum(W[i][j] for i in range(3) if i != j) for j in range(3)]
    row = [W[i][i] - sum(W[i][j] for j in range(3) if j != i) for i in range(3)]
    return col, row


def _tiles_53(W):
    col, row = _base_tiles(W)
    return [col[0], W[3][0] - W[4][0], col[2], W[4][2] - W[3][2], col[1], W[3][1], W[4][1],
            W[0][1], W[1][0], W[1][2], W[2][1], W[0][2], W[3][2], W[2][0], W[4][0],
            row[0], W[3][0] - W[3][2], row[2], W[4][2] - W[4][0], row[1],
            W[0][1] - W[1][0], W[1][2] - W[2][1], W[0][2] - W[2][0], W[3][2] - W[4][0]]


def _tiles_35(W):
    col, row = _base_tiles(W)
    return [col[0], W[0][3] - W[2][3], col[2], W[2][4] - W[0][4], col[1], W[1][3], W[1][4],
            W[0][1], W[1][0], W[1][2], W[2][1], W[0][2], W[0][4], W[2][0], W[2][3],
            row[0], W[0][3] - W[0][4], row[2], W[2][4] - W[2][3], row[1],
            W[0][1] - W[1][0], W[1][2] - W[2][1], W[0][2] - W[2][0], W[0][4] - W[2][3]]


def _bcat(parts, axis=0):
    return _cat([x for x in parts if x is not None], axis=axis).astype(BF16)


def _lhs_pair(T, U, E, i, j):
    if T is None:
        e = E[i] + E[j]
        return dict(a_i=E[i], a_j=E[j], l1=e, l2=e)
    a_i, a_j = T[i] + U[i], T[j] - U[j]
    e = None if E is None else E[i] + E[j]
    cat = lambda x, y: x if y is None else _cat([x, y])
    return dict(a_i=cat(a_i, None if E is None else E[i]), a_j=cat(a_j, None if E is None else E[j]),
                l1=cat(T[i] - U[i] + a_j, e), l2=cat(a_i + T[j] + U[j], e), A=a_i + a_j,
                ai=a_i, aj=a_j)


def _lhs_mid(T, U, E, a0, a2):
    e01 = None if E is None else E[0] + E[1]
    e12 = None if E is None else E[1] + E[2]
    if T is None:
        return dict(a_1=_bcat([E[1]]), l1_01=_bcat([e01]), l2_01=_bcat([e01]),
                    l1_12=_bcat([e12]), l2_12=_bcat([e12]))
    t01, t12 = T[0] + T[1], T[1] + T[2]
    A01, A12 = a0 + T[1], T[1] + a2
    return dict(a_1=_bcat([T[1], None if E is None else E[1]]),
                l1_01=_bcat([t01, e01]), l2_01=_bcat([A01 + U[1], e01]), A01=_bcat([A01]),
                l1_12=_bcat([A12 - U[1], e12]), l2_12=_bcat([t12, e12]), A12=_bcat([A12]),
                b_1=_bcat([U[1]]))


def _lhs_53(T, U, E):
    o, s = _lhs_pair(T, U, E, 0, 2), _lhs_pair(T, U, E, 3, 4)
    L = _lhs_mid(T, U, E, o.get("ai"), o.get("aj"))
    for key in ("a_i", "a_j", "l1", "l2") + (() if T is None else ("A",)):
        L[key] = _cat([o[key], s[key]], axis=1).astype(BF16)
    L["plain"] = _cat([_cat([x[k] for x in (T, E, U) if x is not None]) for k in (3, 4)], axis=1).astype(BF16)
    if T is not None:
        L["b_i"] = _cat([U[0], U[3]], axis=1).astype(BF16)
        L["b_j"] = _cat([U[2], U[4]], axis=1).astype(BF16)
    return L


def _mm_53(L, tile, m):
    p1_01, p2_01 = _nn(L["l1_01"], tile(7, 1)), _nn(L["l2_01"], tile(8, 1))
    if m:
        r01 = p2_01[0:m] - p1_01[0:m] + _nn(L["A01"], tile(20, 1))
    p1_02, p2_02 = _nn(L["l1"], tile(11, 2)), _nn(L["l2"], tile(13, 2))
    if m:
        r02 = (p2_02[0:m] - p1_02[0:m] + _nn(L["A"], tile(22, 2))) * 0.5
    p0 = p2_01 + p2_02 + _nn(L["a_i"], tile(0, 2))
    if m:
        q0 = r01 + r02 + _nn(L["b_i"], tile(15, 2))
    p1_12, p2_12 = _nn(L["l1_12"], tile(9, 1)), _nn(L["l2_12"], tile(10, 1))
    if m:
        r12 = p2_12[0:m] - p1_12[0:m] + _nn(L["A12"], tile(21, 1))
    p2 = p1_02 + p1_12 + _nn(L["a_j"], tile(2, 2))
    if m:
        q2 = r02 + r12 + _nn(L["b_j"], tile(17, 2))
    pl_ = _nn(L["plain"], tile(5, 2))
    mp = p0.shape[0]
    p1 = p1_01 + p2_12 + _nn(L["a_1"], tile(4, 1)) + pl_[0:mp]
    if not m:
        return None, None, [p0, p1, p2]
    q1 = r01 + r12 + _nn(L["b_1"], tile(19, 1)) + pl_[mp:mp + m]
    Y = [p0[0:m] - q0, p1[0:m], p2[0:m] + q2]
    Ey = [p[m:mp] for p in (p0, p1, p2)] if mp > m else None
    return Y, [q0, q1, q2], Ey


def _lhs_35(T, U, E):
    o = _lhs_pair(T, U, E, 0, 2)
    L = _lhs_mid(T, U, E, o.get("ai"), o.get("aj"))
    for key in ("a_i", "a_j", "l1", "l2") + (() if T is None else ("A",)):
        L[key] = o[key].astype(BF16)
    if T is None:
        L["pl3"] = L["pl4"] = L["a_1"]
    else:
        e1 = None if E is None else E[1]
        L["pl3"] = _bcat([T[1] + U[1], e1, U[1]])
        L["pl4"] = _bcat([T[1] - U[1], e1, U[1]])
        L["b_i"], L["b_j"] = U[0].astype(BF16), U[2].astype(BF16)
    return L


def _mm_35(L, tile, m):
    p1_01, p2_01 = _nn(L["l1_01"], tile(7)), _nn(L["l2_01"], tile(8))
    if m:
        r01 = p2_01[0:m] - p1_01[0:m] + _nn(L["A01"], tile(20))
    p1_02, p2_02 = _nn(L["l1"], tile(11)), _nn(L["l2"], tile(13))
    if m:
        r02 = (p2_02[0:m] - p1_02[0:m] + _nn(L["A"], tile(22))) * 0.5
    p0 = p2_01 + p2_02 + _nn(L["a_i"], tile(0))
    if m:
        q0 = r01 + r02 + _nn(L["b_i"], tile(15))
    p1_12, p2_12 = _nn(L["l1_12"], tile(9)), _nn(L["l2_12"], tile(10))
    if m:
        r12 = p2_12[0:m] - p1_12[0:m] + _nn(L["A12"], tile(21))
    p2 = p1_02 + p1_12 + _nn(L["a_j"], tile(2))
    p1 = p1_01 + p2_12 + _nn(L["a_1"], tile(4))
    if m:
        q2 = r02 + r12 + _nn(L["b_j"], tile(17))
        q1 = r01 + r12 + _nn(L["b_1"], tile(19))
    p1_34, p2_34 = _nn(L["l1"], tile(12)), _nn(L["l2"], tile(14))
    if m:
        r34 = (p2_34[0:m] - p1_34[0:m] + _nn(L["A"], tile(23))) * 0.5
    mp = p0.shape[0]
    x3 = _nn(L["pl3"], tile(5))
    p3 = p2_34 + _nn(L["a_i"], tile(1)) + x3[0:mp]
    x4 = _nn(L["pl4"], tile(6))
    p4 = p1_34 + _nn(L["a_j"], tile(3)) + x4[0:mp]
    if not m:
        return [p0, p1, p2, p3, p4], None
    q3 = r34 + _nn(L["b_i"], tile(16)) + x3[mp:mp + m]
    q4 = r34 + _nn(L["b_j"], tile(18)) + x4[mp:mp + m]
    return [p0, p1, p2, p3, p4], [q0, q1, q2, q3, q4]


NTILE = 24


def _plan(seg, n_seg):
    S = seg * n_seg
    R0 = LAG * seg
    A0 = S - (n_seg - LAG) // UNROLL * sum(AHS)
    NPRE = A0 - R0 - LAG * 8
    RS = -(-(A0 - R0 + AHS[0]) // seg) * seg
    XC = NPRE // NXC
    assert XC % 16 == 0 and XC * NXC == NPRE
    return S, R0, A0, NPRE, RS, XC


def _kernel(x_hbm, mem0_hbm, wq_hbm, wk_hbm, wv_hbm, wo_hbm, bqkv_hbm, bwo_hbm,
            out_hbm,
            x_ref, mem0_ref, stage_ref, w_ref, wo_ref, bst_ref, btmp_ref, bw_ref,
            xln_ref, ring_ref, h_ref, xb_ref, x2_ref, kb_ref, vb_ref, o_ref,
            sem_w, sem_m, sem_b, sem_o,
            *, seg, n_seg, n_mem, n_heads, dh, dm):
    S, R0, A0, NPRE, RS, XC = _plan(seg, n_seg)
    M2 = 2 * n_mem
    R = M2 + 2 * seg
    RB = M2 + seg
    PW = 2 * dh
    G = n_heads // 2
    nct = dm // 128
    bdh = dm // B_HEADS
    w_hbm = (wq_hbm, wk_hbm, wv_hbm, wo_hbm)

    def w_copy(p, g, sem=None):
        slot = g & (NSLOT - 1)
        src = g - 1 if p == 3 else g
        return pltpu.make_async_copy(w_hbm[p].at[pl.ds(src * PW, PW), :], stage_ref.at[slot, p],
                                     sem_w.at[slot] if sem is None else sem)

    NB1 = 3 * nct
    WO0 = 3 * dm
    DUM = 4 * dm
    XF = A0 + AHS[0]

    def rows_copy(r0, n, sem):
        return pltpu.make_async_copy(x_hbm.at[pl.ds(r0, n), :], x_ref.at[pl.ds(r0, n), :], sem)

    def x_copy(i):
        return rows_copy(pl.multiple_of(R0 + i * XC, 16), XC, sem_m.at[7 + i])

    small = [rows_copy(0, R0, sem_m.at[1]), rows_copy(R0 + NPRE, XF - R0 - NPRE, sem_m.at[2]),
             pltpu.make_async_copy(mem0_hbm, mem0_ref, sem_m.at[3])]
    x_late = rows_copy(XF, S - XF, sem_m.at[0])

    def bq_copy(part):
        c0 = pl.multiple_of(part * dm, 128)
        return pltpu.make_async_copy(bqkv_hbm.at[:, pl.ds(c0, dm)], bst_ref.at[:, pl.ds(c0, dm)], sem_b.at[part])

    bo_copy = pltpu.make_async_copy(bwo_hbm, bst_ref.at[:, pl.ds(3 * dm, dm)], sem_b.at[3])

    def bst_tile(c):
        return bst_ref[:, pl.ds(pl.multiple_of(c * 128, 128), 128)]

    for i in range(NXC):
        x_copy(i).start()
    for cp in small:
        cp.start()

    def zero_body(j, c):
        btmp_ref[j, DUM:, :] = jnp.zeros((btmp_ref.shape[1] - DUM, 128), F32)
        return c
    lax.fori_loop(0, nct, zero_body, 0)

    for p in range(3):
        w_copy(p, 0, sem_m.at[4 + p]).start()
    for p in range(4):
        w_copy(p, 1).start()
    xb_ref[0:2 * seg, :] = jnp.zeros((2 * seg, dm), F32)
    kb_ref[...] = jnp.zeros(kb_ref.shape, F32)
    vb_ref[...] = jnp.zeros(vb_ref.shape, F32)
    bst_ref[:, 4 * dm:] = jnp.zeros((dm, 128), BF16)

    def ln_body(i, c):
        x_copy(i).wait()
        y = _ln(x_ref[pl.ds(pl.multiple_of(R0 + i * XC, 16), XC), :].astype(F32))
        r0 = pl.multiple_of(i * (XC // 2), 8)
        for j in range(nct):
            xln_ref[j, pl.ds(r0, XC // 2), :] = _pk(y[:, j * 128:(j + 1) * 128].astype(BF16))
        return c
    lax.fori_loop(0, NXC, ln_body, 0)
    for cp in small:
        cp.wait()
    for p in range(4):
        w_copy(p, 2).start()

    def pre_chunk(c, w, nn):
        xl = _cat([_upk(xln_ref[j]) for j in range(nct)], axis=1)
        wt = w.T
        y = _nn(xl, wt) if nn else _nt(xl, w)
        for j in range(3):
            ring_ref[c * 3 + j, 0:NPRE // 2, :] = _pk(y[:, j * 128:(j + 1) * 128].astype(BF16))
        wf = wt.astype(F32)
        tiles = _tiles_53([[wf[k * 128:(k + 1) * 128, n * 128:(n + 1) * 128] for n in range(3)]
                           for k in range(nct)])
        for i, tl in enumerate(tiles):
            w_ref[c, i * 64:(i + 1) * 64, :] = _pk(tl.astype(BF16))

    def init_rows():
        x0 = x_ref[0:seg, :].astype(F32)
        sl = _ln(x0)
        xt = _ln(x_ref[R0 + NPRE:XF, :].astype(F32))
        h_ref[0:n_mem, :] = xt[0:n_mem]
        h_ref[n_mem:M2, :] = sl[0:n_mem]
        h_ref[M2:M2 + n_mem, :] = mem0_ref[...].astype(F32)
        h_ref[M2 + n_mem:RB, :] = sl[n_mem:seg]
        h_ref[RB:RB + AHS[0], :] = xt[M2:M2 + AHS[0]]
        h_ref[RB + AHS[0]:RB + AHS[0] + n_mem, :] = xt[n_mem:M2]
        x2_ref[...] = x0

    def first_body(p, c):
        buf = stage_ref.at[0, p]
        pltpu.make_async_copy(buf, buf, sem_m.at[4 + p]).wait()
        init_rows()
        pre_chunk(p, stage_ref[0, p], False)
        return c
    lax.fori_loop(0, 3, first_body, 0)

    dpt = 128 // B_HEADS

    def b_stage1(u):
        ok = (u >= 0) & (u < NB1)
        tr = bst_tile(jnp.where(ok, u, NB1 + nct)).astype(F32).T
        r0 = pl.multiple_of(jnp.where(ok, u * 128, DUM), 128)
        for j in range(nct):
            btmp_ref[j, pl.ds(r0, 128), :] = tr[:, j * 128:(j + 1) * 128]

    def b_stage1_wo(u):
        ok = (u >= 0) & (u < nct)
        r0 = pl.multiple_of(jnp.where(ok, WO0, DUM), 128)
        btmp_ref[jnp.where(ok, u, 0), pl.ds(r0, dm), :] = bst_tile(
            jnp.where(ok, NB1 + u, NB1 + nct)).astype(F32)

    def b_stage2(u):
        ok = (u >= 0) & (u < NB1)
        part = (u >= nct).astype(jnp.int32) + (u >= 2 * nct).astype(jnp.int32)
        r0 = jnp.where(ok, part * dm + (u - part * nct) * dpt, DUM)
        rows = _cat([_cat([btmp_ref[j, pl.ds(r0 + dd, B_HEADS, stride=bdh), :]
                           for j in range(nct)], axis=1) for dd in range(dpt)])
        bw_ref[jnp.where(ok, u, NB1 + nct)] = _pk(rows.T.astype(BF16))

    def b_stage2_wo(u):
        ok = (u >= 0) & (u < nct)
        r0 = jnp.where(ok, WO0, DUM)
        jj = jnp.where(ok, u, 0)
        bw_ref[jnp.where(ok, NB1 + u, NB1 + nct)] = _pk(
            _cat([btmp_ref[jj, pl.ds(r0 + d, B_HEADS, stride=bdh), :] for d in range(bdh)]).astype(BF16))

    def wo_store(g):
        wf = stage_ref[g & (NSLOT - 1), 3].astype(F32)
        tiles = _tiles_35([[wf[k * 128:(k + 1) * 128, n * 128:(n + 1) * 128] for n in range(nct)]
                           for k in range(3)])
        for i, tl in enumerate(tiles):
            wo_ref[g - 1, i * 64:(i + 1) * 64, :] = _pk(tl.astype(BF16))

    wo_last = w_copy(3, G)

    def pre_body(g, c):
        slot = g & (NSLOT - 1)
        buf = stage_ref.at[slot]
        pltpu.make_async_copy(buf, buf, sem_w.at[slot]).wait()

        @pl.when((g >= 3) & (g <= 5))
        def _():
            bq_copy(g - 3).wait()

        @pl.when(g == 6)
        def _():
            bo_copy.wait()

        @pl.when(g + 2 < G)
        def _():
            for p in range(4):
                w_copy(p, g + 2).start()

        @pl.when(g <= 3)
        def _():
            bq_copy(g - 1).start()

        @pl.when(g == 4)
        def _():
            bo_copy.start()

        @pl.when(g == G - 2)
        def _():
            wo_last.start()
            x_late.start()

        wo_store(g)
        b_stage2(2 * (g - 8))
        b_stage2(2 * (g - 8) + 1)
        b_stage2_wo(g - 11)
        b_stage1(2 * (g - 3))
        b_stage1(2 * (g - 3) + 1)
        b_stage1_wo(g - 6)
        for p in range(3):
            pre_chunk(g * 3 + p, stage_ref[slot, p], p == 2)
        return c
    lax.fori_loop(1, G, pre_body, 0)
    wo_last.wait()

    bscale = float(bdh) ** (-0.5) * LOG2E

    def b_proj(lhs, part):
        return _nn(lhs, _cat([_upk(bw_ref[part * nct + j]) for j in range(nct)], axis=1))

    def b_attn(jobs, q, k, v):
        row = lax.broadcasted_iota(jnp.int32, (seg, 128), 0)
        outs = []
        for i, (l, sidx) in enumerate(jobs):
            r0 = i * seg
            pos = row + sidx * seg
            for j in range(nct):
                kb_ref[l, j, HIST:HIST + seg, :] = k[r0:r0 + seg, j * 128:(j + 1) * 128]
                vb_ref[l, j, HIST:HIST + seg, :] = v[r0:r0 + seg, j * 128:(j + 1) * 128]
            logits = []
            for w in range(B_WIN):
                o = HIST - w * B_DIL
                acc = None
                for j in range(nct):
                    p = q[r0:r0 + seg, j * 128:(j + 1) * 128] * kb_ref[l, j, o:o + seg, :]
                    acc = p if acc is None else acc + p
                acc = acc + pltpu.roll(acc, 64, 1)
                acc = acc + pltpu.roll(acc, 32, 1)
                lg = acc * bscale
                if w > 0:
                    lg = jnp.where(pos >= w * B_DIL, lg, NEG2)
                logits.append(lg)
            m = logits[0]
            for w in range(1, B_WIN):
                m = jnp.maximum(m, logits[w])
            es = [jnp.exp2(lg - m) for lg in logits]
            den = es[0]
            for w in range(1, B_WIN):
                den = den + es[w]
            inv = _recip(den)
            cols = []
            for j in range(nct):
                acc = None
                for w in range(B_WIN):
                    o = HIST - w * B_DIL
                    p = es[w] * vb_ref[l, j, o:o + seg, :]
                    acc = p if acc is None else acc + p
                cols.append(acc * inv)
            outs.append(_cat(cols, axis=1).astype(BF16))
            for j in range(nct):
                kb_ref[l, j, 0:HIST, :] = k[r0 + seg - HIST:r0 + seg, j * 128:(j + 1) * 128]
                vb_ref[l, j, 0:HIST, :] = v[r0 + seg - HIST:r0 + seg, j * 128:(j + 1) * 128]
        return outs

    def b_out(ob, res):
        return res + _nn(ob, _cat([_upk(bw_ref[NB1 + j]) for j in range(nct)], axis=1))

    def o_store(b, val):
        ro = pl.multiple_of((b + 1) * seg, seg)
        o_ref[pl.ds(ro, val.shape[0]), :] = val.astype(o_ref.dtype)

    def out_copy(b):
        ro = pl.multiple_of(b * seg, seg)
        return pltpu.make_async_copy(o_ref.at[pl.ds(ro + seg, seg), :], out_hbm.at[pl.ds(ro, seg), :], sem_o)

    def step(t, hc, full, u=0, i=None):
        t_last = n_seg + LAG - 1
        if full:
            jobs = [(0, t - 1), (1, t - 1 - LAG)]

            def b_in():
                return xb_ref[0:2 * seg, :]
        else:
            lb = (t == t_last).astype(jnp.int32)
            jobs = [(lb, t - 1 - lb * (LAG + 1))]

            def b_in():
                return xb_ref[pl.ds(pl.multiple_of(lb * seg, seg), seg), :]
        split = full and u < UNROLL - 1
        nq = RB + AHS[u] if full else RB
        v0r = _cat([hc[0:n_mem], h_ref[n_mem:M2, :]])
        v1r = _cat([hc[n_mem:M2], h_ref[M2 + n_mem:2 * M2, :]])

        def ktiles(z):
            return [z[:, k * 128:(k + 1) * 128] for k in range(z.shape[1] // 128)]
        if full:
            hl = _lhs_53(ktiles(_cat([v0r, h_ref[2 * M2:RB, :]])), ktiles(_cat([v1r, h_ref[RB:RB + 16, :]])),
                         ktiles(h_ref[RB + 16:nq, :]) if nq > RB + 16 else None)
        else:
            hl = _lhs_53(None, None, ktiles(_cat([v0r, v1r, h_ref[2 * M2:RB, :]])))
        scale = float(dh) ** (-0.5) * LOG2E
        if full:
            s_ = t - LAG
            rd = pl.multiple_of(lax.rem(s_ * (seg // 2), RS // 2), seg // 2)
            a_off = i * sum(AHS) + sum(AHS[:u])
            wa = [pl.multiple_of(lax.rem((A0 - R0 + a_off) // 2 + 8 * a, RS // 2), 8)
                  for a in range(AHS[u] // 16)]
        else:
            wx = pl.multiple_of(jnp.where(t < LAG, NPRE // 2 + t * (n_mem // 2), RS // 2), n_mem // 2)
            wo_store(G)

        RA = R if full else M2 + seg
        CW = R + 2 * M2 if full else R
        ri = lax.broadcasted_iota(jnp.int32, (RA, CW), 0)
        ci = lax.broadcasted_iota(jnp.int32, (RA, CW), 1)
        if not full:
            ri = jnp.where(ri >= M2, ri + seg, ri)

        def table(i, bounds, vals):
            out = vals[-1]
            for b, v in zip(reversed(bounds), reversed(vals[:-1])):
                out = jnp.where(i < b, v, out)
            return out
        qi = ri - table(ri, [16, 48, 56], [0, 8, 48, 40])
        g0 = (ci < 8) | ((ci >= 16) & (ci < 48))
        k2 = ci - table(ci, [8, 24, 32, 48, 56, 80, 88, 96, 104], [-8, 0, 24, 8, 48, 40, 72, 80, 96, 104])
        if full:
            k1 = ci - table(ci, [8, 48], [0, 8, 40])
            row_l2 = ((ri >= 8) & (ri < 16)) | (ri >= 48)
            row_xa = (ri >= 8) & (ri < 16)
            valid = row_xa == (ci >= 80)
            is_a = jnp.where(ci >= 80, ((ci >= 88) & (ci < 104)).astype(jnp.int32),
                             (g0 != row_l2).astype(jnp.int32)) > 0
            ki = jnp.where(row_l2, k2, k1)
            visible = valid & ((qi < n_mem) | (qi >= ki))
            fill = jnp.where(valid, NEG2, -jnp.inf)
        else:
            is_a = jnp.logical_not(g0)
            visible = (qi < n_mem) | (qi >= k2)
            fill = NEG2
        half = dh - 128
        la8 = lax.broadcasted_iota(jnp.int32, (n_mem, 128), 1) < half
        ones = jnp.full((n_mem, 128), 0xFFFFFFFF, U32)
        zero = jnp.zeros((n_mem, 128), U32)
        mask_a = jnp.where(la8, ones, zero)
        mask_b = jnp.where(la8, zero, ones)

        def pk2(a, b):
            return _pk(_cat([a, b]).astype(BF16))

        def proj(p, g):
            base = (g * 3 + p) * 3
            ys, zs, es = _mm_53(hl, lambda i, n: _upk(w_ref[g * 3 + p, i * 64:(i + n) * 64, :]),
                                2 * M2 if full else 0)
            if full:
                yt = [_cat([ys[j][0:M2], zs[j][0:M2], ys[j][M2:2 * M2], zs[j][M2:2 * M2]]
                           + ([] if es is None else [es[j]])) for j in range(3)]
            else:
                yt = es
            x1 = None
            if full:
                for j in range(3):
                    for a in range(AHS[u] // 16):
                        r = RB + 16 * a
                        ring_ref[base + j, pl.ds(wa[a], 8), :] = pk2(yt[j][r:r + 8], yt[j][r + 8:r + 16])
                x1 = [ring_ref[base + j, pl.ds(rd, seg // 2), :] for j in range(3)]
            else:
                for j in range(3):
                    ring_ref[base + j, pl.ds(wx, n_mem // 2), :] = pk2(yt[j][0:8], yt[j][8:16])[0:n_mem // 2]
            return yt, x1

        def groups(z, j):
            y = z[0][j]
            return pk2(y[0:8], y[8:16]), pk2(y[16:24], y[24:32]), pk2(y[32:40], y[40:48])

        def q_rows(z, j):
            v0, v1, v2 = groups(z, j)
            return [v0] + ([z[1][j]] if full else []) + [v1, v2]

        def kv_tiles(z):
            yt, x1 = z
            v0, v1, v2 = groups(z, 0)
            t0 = [v0] + ([x1[0]] if full else [v1, v2]) + [v1, v2]
            y = yt[2]
            w0 = pk2(y[8:16], y[0:8])
            w1 = pk2(y[24:32], y[16:24])
            w2 = pk2(y[32:40], y[40:48])
            t2 = [w0, w1, w2] + ([x1[2]] if full else [w1, w2])
            if full:
                t0 += [v0, v1]
                t2 += [w0, w1]
            y = yt[1]

            def ab(z8):
                return jnp.where(la8, z8, 0.0), jnp.where(la8, 0.0, z8)
            xa_a, xa_b = ab(y[8:16])
            e1 = pk2(xa_b, xa_a)
            u2 = pk2(y[32:40], y[40:48])
            mid2 = [e1, pk2(y[24:32], y[16:24]) & mask_b, u2 & mask_b,
                    pk2(y[16:24], y[24:32]) & mask_a, u2 & mask_a]
            mid1 = None
            if full:
                lo, hi = x1[1][0:8], x1[1][8:16]
                mid1 = [pk2(*ab(y[0:8])), lo & mask_a, hi & mask_a, lo & mask_b, hi & mask_b,
                        e1, pk2(*ab(y[16:24]))]
            return t0, mid1, mid2, t2

        def mat(parts):
            return _upk(_cat(parts))

        def scores(q, k):
            k0, km1, km2, k2_ = kv_tiles(k)
            s_a = _nt(mat(q_rows(q, 0)), mat(k0))
            s_b = _nt(mat(q_rows(q, 2)), mat(k2_))
            qm = q_rows(q, 1)
            if full:
                s_m = _cat([_nt(mat(qm[0:2]), mat(km1)), _nt(mat(qm[2:4]), mat(km2 + km1[5:7]))])
            else:
                s_m = _nt(mat(qm), mat(km2))
            s = (jnp.where(is_a, s_a, s_b) + s_m) * scale
            s = jnp.where(visible, s, fill)
            m_a = jnp.max(jnp.where(is_a, s, -jnp.inf), axis=-1, keepdims=True)
            m_b = jnp.max(jnp.where(is_a, -jnp.inf, s), axis=-1, keepdims=True)
            e = jnp.exp2(s - jnp.where(is_a, m_a, m_b))
            d_a = jnp.sum(jnp.where(is_a, e, 0.0), axis=-1, keepdims=True)
            d_b = jnp.sum(jnp.where(is_a, 0.0, e), axis=-1, keepdims=True)
            return e * _recip(jnp.where(is_a, d_a, d_b))

        def pv(p, v):
            v0, vm1, vm2, v2 = kv_tiles(v)
            o_a = _nn(jnp.where(is_a, p, 0.0).astype(BF16), mat(v0))
            o_b = _nn(jnp.where(is_a, 0.0, p).astype(BF16), mat(v2))
            if full:
                o_m = _cat([_nn(p[0:M2 + seg].astype(BF16), mat(vm1)),
                            _nn(p[M2 + seg:R, 0:R].astype(BF16), mat(vm2))])
            else:
                o_m = _nn(p.astype(BF16), mat(vm2))
            ot = [o_a, o_m, o_b]
            if full:
                return _lhs_35([o[0:32] for o in ot], [_cat([o[48:64], o[32:48]]) for o in ot],
                               [o[64:80] for o in ot])
            return _lhs_35(None, None, ot)

        acc = [None, None]

        def add_o(g):
            c = _mm_35(os_[g], lambda i: _upk(wo_ref[g, i * 64:(i + 1) * 64, :]), 2 * M2 if full else 0)
            for z in range(2):
                if c[z] is not None:
                    acc[z] = c[z] if acc[z] is None else [a + b for a, b in zip(acc[z], c[z])]

        os_ = [None] * G
        bqkv = [None] * 3
        q = proj(0, 0)
        k = proj(1, 0)
        v = proj(2, 0)
        p = scores(q, k)
        blhs = _ln(b_in()).astype(BF16)
        bqkv[2] = b_proj(blhs, 2)
        x2_new = None
        for g in range(G - 1):
            q = proj(0, g + 1)
            k = proj(1, g + 1)
            os_[g] = pv(p, v)
            v = proj(2, g + 1)
            p = scores(q, k)
            if g < 2:
                bqkv[1 - g] = b_proj(blhs, 1 - g)
            if g == 2:
                ob = b_attn(jobs, *bqkv)
            if g == BOUT_AT:
                res = b_in()
                if split:
                    x2_new = b_out(ob[0], res[0:seg])
                elif full:
                    zb = b_out(_cat(ob), res)
                    x2_new = zb[0:seg]
                    o_store(t - 1 - LAG, zb[seg:2 * seg])
                else:
                    x2_new = b_out(ob[0], res)
                    o_store(lb * (t_last - LAG - 1) - 1, x2_new)
            if g - WLAG >= 0:
                add_o(g - WLAG)
        for g in range(G - 1 - WLAG, G - 2):
            add_o(g)
        os_[G - 1] = pv(p, v)
        add_o(G - 2)
        add_o(G - 1)
        if full:
            pa, qa = acc
            lam = (-1, 0, 1, -1, 1)
            ya = [p[0:32] if l == 0 else (p[0:32] + q if l > 0 else p[0:32] - q) for p, q, l in zip(pa, qa, lam)]
            acc = _cat([_cat([y, q[16:32], q[0:16], p[32:48]]) for y, p, q in zip(ya, pa, qa)], axis=1)
        else:
            acc = _cat(acc[0], axis=1)
        if split:
            o_store(t - 1 - LAG, b_out(ob[1], res[seg:2 * seg]))

        y2 = x2_ref[...] + _cat([acc[n_mem:M2], acc[RA - seg + n_mem:RA]])
        mem2 = acc[RA - seg:RA - seg + n_mem]
        if full:
            x_cur = x_ref[pl.ds(pl.multiple_of(t * seg, seg), seg), :].astype(F32)
            xb_ref[0:seg, :] = x_cur + acc[M2:M2 + seg]
            xb_ref[seg:2 * seg, :] = y2
            m1n = acc[0:n_mem]
            m2n = mem2
            ahn = AHS[(u + 1) % UNROLL]
            an = pl.multiple_of(jnp.minimum(A0 + a_off + AHS[u], S - ahn), 16)
            h_ref[RB:RB + ahn, :] = _ln(x_ref[pl.ds(an, ahn), :].astype(F32))
            nxt = x2_new
        else:
            xb_ref[pl.ds(pl.multiple_of(jnp.where(t < LAG, 0, (t - n_seg + 2) * seg), seg), seg), :] = y2
            m1n = jnp.where(t < LAG - 1, h_ref[RB + AHS[0]:RB + AHS[0] + n_mem, :], mem2)
            m2n = jnp.where(t == LAG - 1, mem0_ref[...].astype(F32), mem2)
            nxt = jnp.where(t < LAG - 1, x_ref[seg:2 * seg, :].astype(F32), x2_new)
        x2_ref[...] = nxt
        sl = _ln(nxt)
        h_ref[n_mem:M2, :] = sl[0:n_mem]
        h_ref[M2 + n_mem:RB, :] = sl[n_mem:seg]
        return _cat([m1n, m2n])

    def single_body(t, c):
        @pl.when(t >= n_seg)
        def _():
            out_copy(t - (LAG + 3)).start()
        return step(t, c, False)

    def full_body(i, c):
        t = LAG + UNROLL * i
        for u in range(UNROLL):
            @pl.when(t - u >= LAG + 2)
            def _():
                out_copy(t - u - (LAG + 2)).start()
        for u in range(UNROLL):
            c = step(t + u, c, True, u, i)
        return c

    def phase(ph, c):
        t0 = ph * n_seg
        c = lax.fori_loop(t0, t0 + LAG, single_body, c)

        @pl.when(ph == 0)
        def _():
            x_late.wait()
        return lax.fori_loop(0, jnp.where(ph == 0, (n_seg - LAG) // UNROLL, 0), full_body, c)
    lax.fori_loop(0, 2, phase, _cat([h_ref[0:n_mem, :], h_ref[M2:M2 + n_mem, :]]))

    out_copy(n_seg - 3).start()
    res = xb_ref[2 * seg:4 * seg, :]
    blhs = _ln(res).astype(BF16)
    ob = b_attn([(1, n_seg - 2), (1, n_seg - 1)], *[b_proj(blhs, part) for part in range(3)])
    o_store(n_seg - 2, b_out(_cat(ob), res))
    out_copy(n_seg - 2).start()
    out_copy(n_seg - 1).start()
    pltpu.make_async_copy(o_ref.at[pl.ds(seg, S), :], out_hbm, sem_o).wait()


@functools.partial(jax.jit, static_argnames=("seg",))
def _run(A_x, A_mem0, A_Wq, A_Wk, A_Wv, A_Wo, B_wqkv, B_wo, *, seg):
    _, S, dm = A_x.shape
    n_heads, dh = A_Wq.shape[1], A_Wq.shape[2]
    n_mem = A_mem0.shape[1]
    n_seg = S // seg
    hd = n_heads * dh
    nct = dm // 128
    assert (seg, n_seg, n_mem, dh, dm % 128, n_heads, LAG, UNROLL) == (32, 64, 8, 192, 0, 32, 2, 2)

    x = A_x.reshape(S, dm)
    mem0 = A_mem0.reshape(n_mem, dm)
    wq = jnp.transpose(A_Wq, (1, 2, 0)).reshape(hd, dm)
    wk = jnp.transpose(A_Wk, (1, 2, 0)).reshape(hd, dm)
    wv = jnp.transpose(A_Wv, (1, 2, 0)).reshape(hd, dm)
    wo = A_Wo.reshape(hd, dm)
    _, _, _, _, rs, xc = _plan(seg, n_seg)

    kern = functools.partial(_kernel, seg=seg, n_seg=n_seg, n_mem=n_mem,
                             n_heads=n_heads, dh=dh, dm=dm)
    hbm = pl.BlockSpec(memory_space=pltpu.HBM)

    out = pl.pallas_call(
        kern,
        in_specs=[hbm] * 8,
        out_specs=hbm,
        out_shape=jax.ShapeDtypeStruct((S, dm), A_x.dtype),
        scratch_shapes=[
            pltpu.VMEM((S, dm), BF16),
            pltpu.VMEM((n_mem, dm), BF16),
            pltpu.VMEM((NSLOT, 4, 2 * dh, dm), BF16),
            pltpu.VMEM((3 * n_heads // 2, NTILE * 64, 128), U32),
            pltpu.VMEM((n_heads // 2, NTILE * 64, 128), U32),
            pltpu.VMEM((dm, 4 * dm + 128), BF16),
            pltpu.VMEM((nct, 5 * dm + 32, 128), F32),
            pltpu.VMEM((4 * nct + 1, dm // 2, 128), U32),
            pltpu.VMEM((nct, NXC * xc // 2, 128), U32),
            pltpu.VMEM((3 * hd // 128, rs // 2 + 8, 128), U32),
            pltpu.VMEM((3 * n_mem + seg + AHS[0], dm), F32),
            pltpu.VMEM((4 * seg, dm), F32),
            pltpu.VMEM((seg, dm), F32),
            pltpu.VMEM((2, nct, HIST + seg, 128), F32),
            pltpu.VMEM((2, nct, HIST + seg, 128), F32),
            pltpu.VMEM((S + seg, dm), A_x.dtype),
            pltpu.SemaphoreType.DMA((NSLOT,)),
            pltpu.SemaphoreType.DMA((7 + NXC,)),
            pltpu.SemaphoreType.DMA((4,)),
            pltpu.SemaphoreType.DMA(()),
        ],
        compiler_params=pltpu.CompilerParams(
            vmem_limit_bytes=120 * 1024 * 1024,
            disable_bounds_checks=True,
        ),
    )(x, mem0, wq, wk, wv, wo, B_wqkv, B_wo)
    return out.reshape(1, S, dm)


def pallas_interleave_layers__memory_aug_recurrent_mem_tr__sliding_local_dilated__prompt_kernel(
    A_x: jax.Array,
    A_mem0: jax.Array,
    A_Wq: jax.Array,
    A_Wk: jax.Array,
    A_Wv: jax.Array,
    A_Wo: jax.Array,
    A_seg_len,
    B_x: jax.Array,
    B_wqkv: jax.Array,
    B_wo: jax.Array,
):
    del B_x
    seg = A_seg_len if isinstance(A_seg_len, int) else 32
    return _run(A_x, A_mem0, A_Wq, A_Wk, A_Wv, A_Wo, B_wqkv, B_wo, seg=seg)
```

```python
import functools

import jax
import jax.numpy as jnp
from jax import lax
import jax.experimental.pallas as pl
import jax.experimental.pallas.tpu as pltpu

F32 = jnp.float32
BF16 = jnp.bfloat16
U32 = jnp.uint32
NEG = -1000000000.0
LN_EPS = 1e-05
LOG2E = 1.4426950408889634
NEG2 = NEG * LOG2E

B_HEADS = 32
B_WIN = 8
B_DIL = 2
HIST = 16
AHS = (32, 16)
LAG = 2
NSLOT = 4
WLAG = 3
BOUT_AT = 8
NNM = '001001001'
NNF = '000'
WPOS = 0
BPOS = 0
NXC = 3
UNROLL = 2


def _ln(x):
    m = jnp.mean(x, axis=-1, keepdims=True)
    c = x - m
    v = jnp.mean(c * c, axis=-1, keepdims=True)
    return c * lax.rsqrt(v + LN_EPS)


def _recip(d):
    r = pl.reciprocal(d, approx=True)
    return r * (2.0 - d * r)


def _nt(a, b):
    return lax.dot_general(a, b, (((1,), (1,)), ((), ())), preferred_element_type=F32)


def _nn(a, b):
    return jnp.dot(a, b, preferred_element_type=F32)


def _cat(xs, axis=0):
    return xs[0] if len(xs) == 1 else jnp.concatenate(xs, axis=axis)


def _pk(z):
    return pltpu.bitcast(z, U32)


def _upk(z):
    return pltpu.bitcast(z, BF16)


def _base_tiles(W):
    col = [W[j][j] - sum(W[i][j] for i in range(3) if i != j) for j in range(3)]
    row = [W[i][i] - sum(W[i][j] for j in range(3) if j != i) for i in range(3)]
    return col, row


def _tiles_53(W):
    col, row = _base_tiles(W)
    return [col[0], W[3][0] - W[4][0], col[2], W[4][2] - W[3][2], col[1], W[3][1], W[4][1],
            W[0][1], W[1][0], W[1][2], W[2][1], W[0][2], W[3][2], W[2][0], W[4][0],
            row[0], W[3][0] - W[3][2], row[2], W[4][2] - W[4][0], row[1],
            W[0][1] - W[1][0], W[1][2] - W[2][1], W[0][2] - W[2][0], W[3][2] - W[4][0]]


def _tiles_35(W):
    col, row = _base_tiles(W)
    return [col[0], W[0][3] - W[2][3], col[2], W[2][4] - W[0][4], col[1], W[1][3], W[1][4],
            W[0][1], W[1][0], W[1][2], W[2][1], W[0][2], W[0][4], W[2][0], W[2][3],
            row[0], W[0][3] - W[0][4], row[2], W[2][4] - W[2][3], row[1],
            W[0][1] - W[1][0], W[1][2] - W[2][1], W[0][2] - W[2][0], W[0][4] - W[2][3]]


def _bcat(parts, axis=0):
    return _cat([x for x in parts if x is not None], axis=axis).astype(BF16)


def _lhs_pair(T, U, E, i, j):
    if T is None:
        e = E[i] + E[j]
        return dict(a_i=E[i], a_j=E[j], l1=e, l2=e)
    a_i, a_j = T[i] + U[i], T[j] - U[j]
    e = None if E is None else E[i] + E[j]
    cat = lambda x, y: x if y is None else _cat([x, y])
    return dict(a_i=cat(a_i, None if E is None else E[i]), a_j=cat(a_j, None if E is None else E[j]),
                l1=cat(T[i] - U[i] + a_j, e), l2=cat(a_i + T[j] + U[j], e), A=a_i + a_j,
                ai=a_i, aj=a_j)


def _lhs_mid(T, U, E, a0, a2):
    e01 = None if E is None else E[0] + E[1]
    e12 = None if E is None else E[1] + E[2]
    if T is None:
        return dict(a_1=_bcat([E[1]]), l1_01=_bcat([e01]), l2_01=_bcat([e01]),
                    l1_12=_bcat([e12]), l2_12=_bcat([e12]))
    t01, t12 = T[0] + T[1], T[1] + T[2]
    A01, A12 = a0 + T[1], T[1] + a2
    return dict(a_1=_bcat([T[1], None if E is None else E[1]]),
                l1_01=_bcat([t01, e01]), l2_01=_bcat([A01 + U[1], e01]), A01=_bcat([A01]),
                l1_12=_bcat([A12 - U[1], e12]), l2_12=_bcat([t12, e12]), A12=_bcat([A12]),
                b_1=_bcat([U[1]]))


def _lhs_53(T, U, E):
    o, s = _lhs_pair(T, U, E, 0, 2), _lhs_pair(T, U, E, 3, 4)
    L = _lhs_mid(T, U, E, o.get("ai"), o.get("aj"))
    for key in ("a_i", "a_j", "l1", "l2") + (() if T is None else ("A",)):
        L[key] = _cat([o[key], s[key]], axis=1).astype(BF16)
    L["plain"] = _cat([_cat([x[k] for x in (T, E, U) if x is not None]) for k in (3, 4)], axis=1).astype(BF16)
    if T is not None:
        L["b_i"] = _cat([U[0], U[3]], axis=1).astype(BF16)
        L["b_j"] = _cat([U[2], U[4]], axis=1).astype(BF16)
    return L


def _mm_53(L, tile, m, _nn=_nn):
    p1_01, p2_01 = _nn(L["l1_01"], tile(7, 1)), _nn(L["l2_01"], tile(8, 1))
    if m:
        r01 = p2_01[0:m] - p1_01[0:m] + _nn(L["A01"], tile(20, 1))
    p1_02, p2_02 = _nn(L["l1"], tile(11, 2)), _nn(L["l2"], tile(13, 2))
    if m:
        r02 = (p2_02[0:m] - p1_02[0:m] + _nn(L["A"], tile(22, 2))) * 0.5
    p0 = p2_01 + p2_02 + _nn(L["a_i"], tile(0, 2))
    if m:
        q0 = r01 + r02 + _nn(L["b_i"], tile(15, 2))
    p1_12, p2_12 = _nn(L["l1_12"], tile(9, 1)), _nn(L["l2_12"], tile(10, 1))
    if m:
        r12 = p2_12[0:m] - p1_12[0:m] + _nn(L["A12"], tile(21, 1))
    p2 = p1_02 + p1_12 + _nn(L["a_j"], tile(2, 2))
    if m:
        q2 = r02 + r12 + _nn(L["b_j"], tile(17, 2))
    pl_ = _nn(L["plain"], tile(5, 2))
    mp = p0.shape[0]
    p1 = p1_01 + p2_12 + _nn(L["a_1"], tile(4, 1)) + pl_[0:mp]
    if not m:
        return None, None, [p0, p1, p2]
    q1 = r01 + r12 + _nn(L["b_1"], tile(19, 1)) + pl_[mp:mp + m]
    Y = [p0[0:m] - q0, p1[0:m], p2[0:m] + q2]
    Ey = [p[m:mp] for p in (p0, p1, p2)] if mp > m else None
    return Y, [q0, q1, q2], Ey


def _lhs_35(T, U, E):
    o = _lhs_pair(T, U, E, 0, 2)
    L = _lhs_mid(T, U, E, o.get("ai"), o.get("aj"))
    for key in ("a_i", "a_j", "l1", "l2") + (() if T is None else ("A",)):
        L[key] = o[key].astype(BF16)
    if T is None:
        L["pl3"] = L["pl4"] = L["a_1"]
    else:
        e1 = None if E is None else E[1]
        L["pl3"] = _bcat([T[1] + U[1], e1, U[1]])
        L["pl4"] = _bcat([T[1] - U[1], e1, U[1]])
        L["b_i"], L["b_j"] = U[0].astype(BF16), U[2].astype(BF16)
    return L


def _mm_35(L, tile, m):
    p1_01, p2_01 = _nn(L["l1_01"], tile(7)), _nn(L["l2_01"], tile(8))
    if m:
        r01 = p2_01[0:m] - p1_01[0:m] + _nn(L["A01"], tile(20))
    p1_02, p2_02 = _nn(L["l1"], tile(11)), _nn(L["l2"], tile(13))
    if m:
        r02 = (p2_02[0:m] - p1_02[0:m] + _nn(L["A"], tile(22))) * 0.5
    p0 = p2_01 + p2_02 + _nn(L["a_i"], tile(0))
    if m:
        q0 = r01 + r02 + _nn(L["b_i"], tile(15))
    p1_12, p2_12 = _nn(L["l1_12"], tile(9)), _nn(L["l2_12"], tile(10))
    if m:
        r12 = p2_12[0:m] - p1_12[0:m] + _nn(L["A12"], tile(21))
    p2 = p1_02 + p1_12 + _nn(L["a_j"], tile(2))
    p1 = p1_01 + p2_12 + _nn(L["a_1"], tile(4))
    if m:
        q2 = r02 + r12 + _nn(L["b_j"], tile(17))
        q1 = r01 + r12 + _nn(L["b_1"], tile(19))
    p1_34, p2_34 = _nn(L["l1"], tile(12)), _nn(L["l2"], tile(14))
    if m:
        r34 = (p2_34[0:m] - p1_34[0:m] + _nn(L["A"], tile(23))) * 0.5
    mp = p0.shape[0]
    x3 = _nn(L["pl3"], tile(5))
    p3 = p2_34 + _nn(L["a_i"], tile(1)) + x3[0:mp]
    x4 = _nn(L["pl4"], tile(6))
    p4 = p1_34 + _nn(L["a_j"], tile(3)) + x4[0:mp]
    if not m:
        return [p0, p1, p2, p3, p4], None
    q3 = r34 + _nn(L["b_i"], tile(16)) + x3[mp:mp + m]
    q4 = r34 + _nn(L["b_j"], tile(18)) + x4[mp:mp + m]
    return [p0, p1, p2, p3, p4], [q0, q1, q2, q3, q4]


NTILE = 24
_PLAIN_53 = {5: (3, 1), 6: (4, 1), 7: (0, 1), 8: (1, 0), 9: (1, 2), 10: (2, 1), 11: (0, 2), 12: (3, 2),
             13: (2, 0), 14: (4, 0)}
_PLAIN_35 = {5: (1, 3), 6: (1, 4), 7: (0, 1), 8: (1, 0), 9: (1, 2), 10: (2, 1), 11: (0, 2), 12: (0, 4),
             13: (2, 0), 14: (2, 3)}
_KEYS1 = ("a_1", "b_1", "l1_01", "l2_01", "A01", "l1_12", "l2_12", "A12")
_KEYS2 = ("a_i", "a_j", "b_i", "b_j", "l1", "l2", "A")


def _plan(seg, n_seg):
    S = seg * n_seg
    R0 = LAG * seg
    A0 = S - (n_seg - LAG) // UNROLL * sum(AHS)
    NPRE = A0 - R0 - LAG * 8
    RS = -(-(A0 - R0 + AHS[0]) // seg) * seg
    XC = NPRE // NXC
    assert XC % 32 == 0 and XC * NXC == NPRE
    return S, R0, A0, NPRE, RS, XC


def _kernel(x_hbm, mem0_hbm, wq_hbm, wk_hbm, wv_hbm, wo_hbm, bqkv_hbm, bwo_hbm,
            out_hbm,
            x_ref, mem0_ref, stage_ref, w_ref, wo_ref, bst_ref, btmp_ref, bw_ref,
            xln_ref, ring_ref, h_ref, xb_ref, x2_ref, kb_ref, vb_ref, o_ref,
            sem_w, sem_m, sem_b, sem_o,
            *, seg, n_seg, n_mem, n_heads, dh, dm):
    S, R0, A0, NPRE, RS, XC = _plan(seg, n_seg)
    M2 = 2 * n_mem
    R = M2 + 2 * seg
    RB = M2 + seg
    PW = 2 * dh
    G = n_heads // 2
    nct = dm // 128
    bdh = dm // B_HEADS
    w_hbm = (wq_hbm, wk_hbm, wv_hbm, wo_hbm)

    def w_copy(p, g, sem=None):
        slot = g & (NSLOT - 1)
        src = g - 1 if p == 3 else g
        return pltpu.make_async_copy(w_hbm[p].at[pl.ds(src * PW, PW), :], stage_ref.at[slot, p],
                                     sem_w.at[slot] if sem is None else sem)

    NB1 = 3 * nct
    WO0 = 3 * dm
    DUM = 4 * dm
    XF = A0 + AHS[0]
    XH = XC // 2

    def rows_copy(r0, n, sem):
        return pltpu.make_async_copy(x_hbm.at[pl.ds(r0, n), :], x_ref.at[pl.ds(r0, n), :], sem)

    def x_copy(i):
        return rows_copy(pl.multiple_of(R0 + i * XC, 16), XC, sem_m.at[7 + i])

    small = [rows_copy(0, R0, sem_m.at[1]), rows_copy(R0 + NPRE, XF - R0 - NPRE, sem_m.at[2]),
             pltpu.make_async_copy(mem0_hbm, mem0_ref, sem_m.at[3])]
    x_late = rows_copy(XF, S - XF, sem_m.at[0])

    def bq_copy(part):
        c0 = pl.multiple_of(part * dm, 128)
        return pltpu.make_async_copy(bqkv_hbm.at[:, pl.ds(c0, dm)], bst_ref.at[:, pl.ds(c0, dm)], sem_b.at[part])

    bo_copy = pltpu.make_async_copy(bwo_hbm, bst_ref.at[:, pl.ds(3 * dm, dm)], sem_b.at[3])

    def bst_tile(c):
        return bst_ref[:, pl.ds(pl.multiple_of(c * 128, 128), 128)]

    for i in range(NXC):
        x_copy(i).start()
    for cp in small:
        cp.start()

    def zero_body(j, c):
        btmp_ref[j, DUM:, :] = jnp.zeros((btmp_ref.shape[1] - DUM, 128), F32)
        return c
    lax.fori_loop(0, nct, zero_body, 0)

    for p in range(3):
        w_copy(p, 0, sem_m.at[4 + p]).start()
    for p in range(4):
        w_copy(p, 1).start()
    xb_ref[0:2 * seg, :] = jnp.zeros((2 * seg, dm), F32)
    kb_ref[...] = jnp.zeros(kb_ref.shape, F32)
    vb_ref[...] = jnp.zeros(vb_ref.shape, F32)
    bst_ref[:, 4 * dm:] = jnp.zeros((dm, 128), BF16)

    def ln_body(i, c):
        x_copy(i).wait()
        y = _ln(x_ref[pl.ds(pl.multiple_of(R0 + i * XC, 16), XC), :].astype(F32))
        L = _lhs_53([y[0:XH, k * 128:(k + 1) * 128] for k in range(nct)],
                    [y[XH:XC, k * 128:(k + 1) * 128] for k in range(nct)], None)
        parts = [L[key] for key in _KEYS1]
        for z in [L[key] for key in _KEYS2] + [L["plain"][0:XH]]:
            parts += [z[:, 0:128], z[:, 128:256]]
        r0 = pl.multiple_of(i * (XH // 2), 8)
        for j, z in enumerate(parts):
            xln_ref[j, pl.ds(r0, XH // 2), :] = _pk(z)
        return c
    lax.fori_loop(0, NXC, ln_body, 0)
    for cp in small:
        cp.wait()
    for p in range(4):
        w_copy(p, 2).start()

    def pre_chunk(c, w, nn):
        strips = []
        for r in range(0, 128, 16):
            strips.append(_tiles_53([[w[n * 128 + r:n * 128 + r + 16, k * 128:(k + 1) * 128].astype(F32)
                                      for n in range(3)] for k in range(nct)]))
        tb = []
        for i in range(NTILE):
            if i in _PLAIN_53:
                k, n = _PLAIN_53[i]
                tb.append(w[n * 128:(n + 1) * 128, k * 128:(k + 1) * 128])
            else:
                tb.append(_cat([st[i] for st in strips]).astype(BF16))
        for i, x in enumerate(tb):
            w_ref[c, i * 64:(i + 1) * 64, :] = _pk(x.T)

        def dot_nt(a, idx):
            i, n = idx
            out = None
            for e in range(n):
                r = _nt(a[:, e * 128:(e + 1) * 128], tb[i + e])
                out = r if out is None else out + r
            return out

        for i in range(NXC):
            def op(j):
                return _upk(xln_ref[j, i * (XH // 2):(i + 1) * (XH // 2), :])
            L = {key: op(j) for j, key in enumerate(_KEYS1)}
            for j, key in enumerate(_KEYS2):
                L[key] = _cat([op(len(_KEYS1) + 2 * j + e) for e in range(2)], axis=1)
            L["plain"] = _cat([_cat([op(NTILE - 2), L["b_i"][:, 128:256]]),
                               _cat([op(NTILE - 1), L["b_j"][:, 128:256]])], axis=1)
            if nn[i] == '1':
                ys, zs, _ = _mm_53(L, lambda a, n: _upk(w_ref[c, a * 64:(a + n) * 64, :]), XH)
            else:
                ys, zs, _ = _mm_53(L, lambda a, n: (a, n), XH, dot_nt)
            for j in range(3):
                ring_ref[c * 3 + j, i * XH:i * XH + XH // 2, :] = _pk(ys[j].astype(BF16))
                ring_ref[c * 3 + j, i * XH + XH // 2:(i + 1) * XH, :] = _pk(zs[j].astype(BF16))

    def init_rows():
        x0 = x_ref[0:seg, :].astype(F32)
        sl = _ln(x0)
        xt = _ln(x_ref[R0 + NPRE:XF, :].astype(F32))
        h_ref[0:n_mem, :] = xt[0:n_mem]
        h_ref[n_mem:M2, :] = sl[0:n_mem]
        h_ref[M2:M2 + n_mem, :] = mem0_ref[...].astype(F32)
        h_ref[M2 + n_mem:RB, :] = sl[n_mem:seg]
        h_ref[RB:RB + AHS[0], :] = xt[M2:M2 + AHS[0]]
        h_ref[RB + AHS[0]:RB + AHS[0] + n_mem, :] = xt[n_mem:M2]
        x2_ref[...] = x0

    def first_body(p, c):
        buf = stage_ref.at[0, p]
        pltpu.make_async_copy(buf, buf, sem_m.at[4 + p]).wait()
        init_rows()
        pre_chunk(p, stage_ref.at[0, p], NNF)
        return c
    lax.fori_loop(0, 3, first_body, 0)

    dpt = 128 // B_HEADS

    def b_stage1(u):
        ok = (u >= 0) & (u < NB1)
        tr = bst_tile(jnp.where(ok, u, NB1 + nct)).astype(F32).T
        r0 = pl.multiple_of(jnp.where(ok, u * 128, DUM), 128)
        for j in range(nct):
            btmp_ref[j, pl.ds(r0, 128), :] = tr[:, j * 128:(j + 1) * 128]

    def b_stage1_wo(u):
        ok = (u >= 0) & (u < nct)
        r0 = pl.multiple_of(jnp.where(ok, WO0, DUM), 128)
        btmp_ref[jnp.where(ok, u, 0), pl.ds(r0, dm), :] = bst_tile(
            jnp.where(ok, NB1 + u, NB1 + nct)).astype(F32)

    def b_stage2(u):
        ok = (u >= 0) & (u < NB1)
        part = (u >= nct).astype(jnp.int32) + (u >= 2 * nct).astype(jnp.int32)
        r0 = jnp.where(ok, part * dm + (u - part * nct) * dpt, DUM)
        rows = _cat([_cat([btmp_ref[j, pl.ds(r0 + dd, B_HEADS, stride=bdh), :]
                           for j in range(nct)], axis=1) for dd in range(dpt)])
        bw_ref[jnp.where(ok, u, NB1 + nct)] = _pk(rows.T.astype(BF16))

    def b_stage2_wo(u):
        ok = (u >= 0) & (u < nct)
        r0 = jnp.where(ok, WO0, DUM)
        jj = jnp.where(ok, u, 0)
        bw_ref[jnp.where(ok, NB1 + u, NB1 + nct)] = _pk(
            _cat([btmp_ref[jj, pl.ds(r0 + d, B_HEADS, stride=bdh), :] for d in range(bdh)]).astype(BF16))

    def wo_store(g):
        w = stage_ref.at[g & (NSLOT - 1), 3]
        for r in range(0, 128, 16):
            wb = [[w[k * 128 + r:k * 128 + r + 16, n * 128:(n + 1) * 128] for n in range(nct)] for k in range(3)]
            tiles = _tiles_35([[x.astype(F32) for x in row] for row in wb])
            for i, tl in enumerate(tiles):
                if i in _PLAIN_35:
                    k, n = _PLAIN_35[i]
                    tl = wb[k][n]
                wo_ref[g - 1, i * 64 + r // 2:i * 64 + r // 2 + 8, :] = _pk(tl.astype(BF16))

    wo_last = w_copy(3, G)

    def pre_body(g, c):
        slot = g & (NSLOT - 1)
        buf = stage_ref.at[slot]
        pltpu.make_async_copy(buf, buf, sem_w.at[slot]).wait()

        @pl.when((g >= 3) & (g <= 5))
        def _():
            bq_copy(g - 3).wait()

        @pl.when(g == 6)
        def _():
            bo_copy.wait()

        @pl.when(g + 2 < G)
        def _():
            for p in range(4):
                w_copy(p, g + 2).start()

        @pl.when(g <= 3)
        def _():
            bq_copy(g - 1).start()

        @pl.when(g == 4)
        def _():
            bo_copy.start()

        @pl.when(g == G - 2)
        def _():
            wo_last.start()
            x_late.start()

        for p in range(4):
            if p == WPOS:
                wo_store(g)
            if p == BPOS:
                b_stage2(2 * (g - 8))
                b_stage2(2 * (g - 8) + 1)
                b_stage2_wo(g - 11)
                b_stage1(2 * (g - 3))
                b_stage1(2 * (g - 3) + 1)
                b_stage1_wo(g - 6)
            if p < 3:
                pre_chunk(g * 3 + p, stage_ref.at[slot, p], NNM[3 * p:3 * p + 3])
        return c
    lax.fori_loop(1, G, pre_body, 0)
    wo_last.wait()

    bscale = float(bdh) ** (-0.5) * LOG2E

    def b_proj(lhs, part):
        return _nn(lhs, _cat([_upk(bw_ref[part * nct + j]) for j in range(nct)], axis=1))

    def b_attn(jobs, q, k, v):
        row = lax.broadcasted_iota(jnp.int32, (seg, 128), 0)
        outs = []
        for i, (l, sidx) in enumerate(jobs):
            r0 = i * seg
            pos = row + sidx * seg
            for j in range(nct):
                kb_ref[l, j, HIST:HIST + seg, :] = k[r0:r0 + seg, j * 128:(j + 1) * 128]
                vb_ref[l, j, HIST:HIST + seg, :] = v[r0:r0 + seg, j * 128:(j + 1) * 128]
            logits = []
            for w in range(B_WIN):
                o = HIST - w * B_DIL
                acc = None
                for j in range(nct):
                    p = q[r0:r0 + seg, j * 128:(j + 1) * 128] * kb_ref[l, j, o:o + seg, :]
                    acc = p if acc is None else acc + p
                acc = acc + pltpu.roll(acc, 64, 1)
                acc = acc + pltpu.roll(acc, 32, 1)
                lg = acc * bscale
                if w > 0:
                    lg = jnp.where(pos >= w * B_DIL, lg, NEG2)
                logits.append(lg)
            m = logits[0]
            for w in range(1, B_WIN):
                m = jnp.maximum(m, logits[w])
            es = [jnp.exp2(lg - m) for lg in logits]
            den = es[0]
            for w in range(1, B_WIN):
                den = den + es[w]
            inv = _recip(den)
            cols = []
            for j in range(nct):
                acc = None
                for w in range(B_WIN):
                    o = HIST - w * B_DIL
                    p = es[w] * vb_ref[l, j, o:o + seg, :]
                    acc = p if acc is None else acc + p
                cols.append(acc * inv)
            outs.append(_cat(cols, axis=1).astype(BF16))
            for j in range(nct):
                kb_ref[l, j, 0:HIST, :] = k[r0 + seg - HIST:r0 + seg, j * 128:(j + 1) * 128]
                vb_ref[l, j, 0:HIST, :] = v[r0 + seg - HIST:r0 + seg, j * 128:(j + 1) * 128]
        return outs

    def b_out(ob, res):
        return res + _nn(ob, _cat([_upk(bw_ref[NB1 + j]) for j in range(nct)], axis=1))

    def o_store(b, val):
        ro = pl.multiple_of((b + 1) * seg, seg)
        o_ref[pl.ds(ro, val.shape[0]), :] = val.astype(o_ref.dtype)

    def out_copy(b):
        ro = pl.multiple_of(b * seg, seg)
        return pltpu.make_async_copy(o_ref.at[pl.ds(ro + seg, seg), :], out_hbm.at[pl.ds(ro, seg), :], sem_o)

    def step(t, hc, full, u=0, i=None):
        t_last = n_seg + LAG - 1
        if full:
            jobs = [(0, t - 1), (1, t - 1 - LAG)]

            def b_in():
                return xb_ref[0:2 * seg, :]
        else:
            lb = (t == t_last).astype(jnp.int32)
            jobs = [(lb, t - 1 - lb * (LAG + 1))]

            def b_in():
                return xb_ref[pl.ds(pl.multiple_of(lb * seg, seg), seg), :]
        split = full and u < UNROLL - 1
        nq = RB + AHS[u] if full else RB
        v0r = _cat([hc[0:n_mem], h_ref[n_mem:M2, :]])
        v1r = _cat([hc[n_mem:M2], h_ref[M2 + n_mem:2 * M2, :]])

        def ktiles(z):
            return [z[:, k * 128:(k + 1) * 128] for k in range(z.shape[1] // 128)]
        if full:
            hl = _lhs_53(ktiles(_cat([v0r, h_ref[2 * M2:RB, :]])), ktiles(_cat([v1r, h_ref[RB:RB + 16, :]])),
                         ktiles(h_ref[RB + 16:nq, :]) if nq > RB + 16 else None)
        else:
            hl = _lhs_53(None, None, ktiles(_cat([v0r, v1r, h_ref[2 * M2:RB, :]])))
        scale = float(dh) ** (-0.5) * LOG2E
        if full:
            s_ = t - LAG
            rd = pl.multiple_of(lax.rem(s_ * (seg // 2), RS // 2), seg // 2)
            a_off = i * sum(AHS) + sum(AHS[:u])
            wa = [pl.multiple_of(lax.rem((A0 - R0 + a_off) // 2 + 8 * a, RS // 2), 8)
                  for a in range(AHS[u] // 16)]
        else:
            wx = pl.multiple_of(jnp.where(t < LAG, NPRE // 2 + t * (n_mem // 2), RS // 2), n_mem // 2)
            wo_store(G)

        RA = R if full else M2 + seg
        CW = R + 2 * M2 if full else R
        ri = lax.broadcasted_iota(jnp.int32, (RA, CW), 0)
        ci = lax.broadcasted_iota(jnp.int32, (RA, CW), 1)
        if not full:
            ri = jnp.where(ri >= M2, ri + seg, ri)

        def table(i, bounds, vals):
            out = vals[-1]
            for b, v in zip(reversed(bounds), reversed(vals[:-1])):
                out = jnp.where(i < b, v, out)
            return out
        qi = ri - table(ri, [16, 48, 56], [0, 8, 48, 40])
        g0 = (ci < 8) | ((ci >= 16) & (ci < 48))
        k2 = ci - table(ci, [8, 24, 32, 48, 56, 80, 88, 96, 104], [-8, 0, 24, 8, 48, 40, 72, 80, 96, 104])
        if full:
            k1 = ci - table(ci, [8, 48], [0, 8, 40])
            row_l2 = ((ri >= 8) & (ri < 16)) | (ri >= 48)
            row_xa = (ri >= 8) & (ri < 16)
            valid = row_xa == (ci >= 80)
            is_a = jnp.where(ci >= 80, ((ci >= 88) & (ci < 104)).astype(jnp.int32),
                             (g0 != row_l2).astype(jnp.int32)) > 0
            ki = jnp.where(row_l2, k2, k1)
            visible = valid & ((qi < n_mem) | (qi >= ki))
            fill = jnp.where(valid, NEG2, -jnp.inf)
        else:
            is_a = jnp.logical_not(g0)
            visible = (qi < n_mem) | (qi >= k2)
            fill = NEG2
        half = dh - 128
        la8 = lax.broadcasted_iota(jnp.int32, (n_mem, 128), 1) < half
        ones = jnp.full((n_mem, 128), 0xFFFFFFFF, U32)
        zero = jnp.zeros((n_mem, 128), U32)
        mask_a = jnp.where(la8, ones, zero)
        mask_b = jnp.where(la8, zero, ones)

        def pk2(a, b):
            return _pk(_cat([a, b]).astype(BF16))

        def proj(p, g):
            base = (g * 3 + p) * 3
            ys, zs, es = _mm_53(hl, lambda i, n: _upk(w_ref[g * 3 + p, i * 64:(i + n) * 64, :]),
                                2 * M2 if full else 0)
            if full:
                yt = [_cat([ys[j][0:M2], zs[j][0:M2], ys[j][M2:2 * M2], zs[j][M2:2 * M2]]
                           + ([] if es is None else [es[j]])) for j in range(3)]
            else:
                yt = es
            x1 = None
            if full:
                for j in range(3):
                    for a in range(AHS[u] // 16):
                        r = RB + 16 * a
                        ring_ref[base + j, pl.ds(wa[a], 8), :] = pk2(yt[j][r:r + 8], yt[j][r + 8:r + 16])
                x1 = [ring_ref[base + j, pl.ds(rd, seg // 2), :] for j in range(3)]
            else:
                for j in range(3):
                    ring_ref[base + j, pl.ds(wx, n_mem // 2), :] = pk2(yt[j][0:8], yt[j][8:16])[0:n_mem // 2]
            return yt, x1

        def groups(z, j):
            y = z[0][j]
            return pk2(y[0:8], y[8:16]), pk2(y[16:24], y[24:32]), pk2(y[32:40], y[40:48])

        def q_rows(z, j):
            v0, v1, v2 = groups(z, j)
            return [v0] + ([z[1][j]] if full else []) + [v1, v2]

        def kv_tiles(z):
            yt, x1 = z
            v0, v1, v2 = groups(z, 0)
            t0 = [v0] + ([x1[0]] if full else [v1, v2]) + [v1, v2]
            y = yt[2]
            w0 = pk2(y[8:16], y[0:8])
            w1 = pk2(y[24:32], y[16:24])
            w2 = pk2(y[32:40], y[40:48])
            t2 = [w0, w1, w2] + ([x1[2]] if full else [w1, w2])
            if full:
                t0 += [v0, v1]
                t2 += [w0, w1]
            y = yt[1]

            def ab(z8):
                return jnp.where(la8, z8, 0.0), jnp.where(la8, 0.0, z8)
            xa_a, xa_b = ab(y[8:16])
            e1 = pk2(xa_b, xa_a)
            u2 = pk2(y[32:40], y[40:48])
            mid2 = [e1, pk2(y[24:32], y[16:24]) & mask_b, u2 & mask_b,
                    pk2(y[16:24], y[24:32]) & mask_a, u2 & mask_a]
            mid1 = None
            if full:
                lo, hi = x1[1][0:8], x1[1][8:16]
                mid1 = [pk2(*ab(y[0:8])), lo & mask_a, hi & mask_a, lo & mask_b, hi & mask_b,
                        e1, pk2(*ab(y[16:24]))]
            return t0, mid1, mid2, t2

        def mat(parts):
            return _upk(_cat(parts))

        def scores(q, k):
            k0, km1, km2, k2_ = kv_tiles(k)
            s_a = _nt(mat(q_rows(q, 0)), mat(k0))
            s_b = _nt(mat(q_rows(q, 2)), mat(k2_))
            qm = q_rows(q, 1)
            if full:
                s_m = _cat([_nt(mat(qm[0:2]), mat(km1)), _nt(mat(qm[2:4]), mat(km2 + km1[5:7]))])
            else:
                s_m = _nt(mat(qm), mat(km2))
            s = (jnp.where(is_a, s_a, s_b) + s_m) * scale
            s = jnp.where(visible, s, fill)
            m_a = jnp.max(jnp.where(is_a, s, -jnp.inf), axis=-1, keepdims=True)
            m_b = jnp.max(jnp.where(is_a, -jnp.inf, s), axis=-1, keepdims=True)
            e = jnp.exp2(s - jnp.where(is_a, m_a, m_b))
            d_a = jnp.sum(jnp.where(is_a, e, 0.0), axis=-1, keepdims=True)
            d_b = jnp.sum(jnp.where(is_a, 0.0, e), axis=-1, keepdims=True)
            return e * _recip(jnp.where(is_a, d_a, d_b))

        def pv(p, v):
            v0, vm1, vm2, v2 = kv_tiles(v)
            o_a = _nn(jnp.where(is_a, p, 0.0).astype(BF16), mat(v0))
            o_b = _nn(jnp.where(is_a, 0.0, p).astype(BF16), mat(v2))
            if full:
                o_m = _cat([_nn(p[0:M2 + seg].astype(BF16), mat(vm1)),
                            _nn(p[M2 + seg:R, 0:R].astype(BF16), mat(vm2))])
            else:
                o_m = _nn(p.astype(BF16), mat(vm2))
            ot = [o_a, o_m, o_b]
            if full:
                return _lhs_35([o[0:32] for o in ot], [_cat([o[48:64], o[32:48]]) for o in ot],
                               [o[64:80] for o in ot])
            return _lhs_35(None, None, ot)

        acc = [None, None]

        def add_o(g):
            c = _mm_35(os_[g], lambda i: _upk(wo_ref[g, i * 64:(i + 1) * 64, :]), 2 * M2 if full else 0)
            for z in range(2):
                if c[z] is not None:
                    acc[z] = c[z] if acc[z] is None else [a + b for a, b in zip(acc[z], c[z])]

        os_ = [None] * G
        bqkv = [None] * 3
        k = proj(1, 0)
        q = proj(0, 0)
        v = proj(2, 0)
        p = scores(q, k)
        blhs = _ln(b_in()).astype(BF16)
        bqkv[2] = b_proj(blhs, 2)
        x2_new = None
        for g in range(G - 1):
            k = proj(1, g + 1)
            q = proj(0, g + 1)
            vn = proj(2, g + 1)
            os_[g] = pv(p, v)
            v = vn
            if g < 2:
                bqkv[1 - g] = b_proj(blhs, 1 - g)
            if g == 2:
                ob = b_attn(jobs, *bqkv)
            if g == BOUT_AT:
                res = b_in()
                if split:
                    x2_new = b_out(ob[0], res[0:seg])
                elif full:
                    zb = b_out(_cat(ob), res)
                    x2_new = zb[0:seg]
                    o_store(t - 1 - LAG, zb[seg:2 * seg])
                else:
                    x2_new = b_out(ob[0], res)
                    o_store(lb * (t_last - LAG - 1) - 1, x2_new)
            if g - WLAG >= 0:
                add_o(g - WLAG)
            p = scores(q, k)
        for g in range(G - 1 - WLAG, G - 2):
            add_o(g)
        os_[G - 1] = pv(p, v)
        add_o(G - 2)
        add_o(G - 1)
        if full:
            pa, qa = acc
            lam = (-1, 0, 1, -1, 1)
            ya = [p[0:32] if l == 0 else (p[0:32] + q if l > 0 else p[0:32] - q) for p, q, l in zip(pa, qa, lam)]
            acc = _cat([_cat([y, q[16:32], q[0:16], p[32:48]]) for y, p, q in zip(ya, pa, qa)], axis=1)
        else:
            acc = _cat(acc[0], axis=1)
        if split:
            o_store(t - 1 - LAG, b_out(ob[1], res[seg:2 * seg]))

        y2 = x2_ref[...] + _cat([acc[n_mem:M2], acc[RA - seg + n_mem:RA]])
        mem2 = acc[RA - seg:RA - seg + n_mem]
        if full:
            x_cur = x_ref[pl.ds(pl.multiple_of(t * seg, seg), seg), :].astype(F32)
            xb_ref[0:seg, :] = x_cur + acc[M2:M2 + seg]
            xb_ref[seg:2 * seg, :] = y2
            m1n = acc[0:n_mem]
            m2n = mem2
            ahn = AHS[(u + 1) % UNROLL]
            an = pl.multiple_of(jnp.minimum(A0 + a_off + AHS[u], S - ahn), 16)
            h_ref[RB:RB + ahn, :] = _ln(x_ref[pl.ds(an, ahn), :].astype(F32))
            nxt = x2_new
        else:
            xb_ref[pl.ds(pl.multiple_of(jnp.where(t < LAG, 0, (t - n_seg + 2) * seg), seg), seg), :] = y2
            m1n = jnp.where(t < LAG - 1, h_ref[RB + AHS[0]:RB + AHS[0] + n_mem, :], mem2)
            m2n = jnp.where(t == LAG - 1, mem0_ref[...].astype(F32), mem2)
            nxt = jnp.where(t < LAG - 1, x_ref[seg:2 * seg, :].astype(F32), x2_new)
        x2_ref[...] = nxt
        sl = _ln(nxt)
        h_ref[n_mem:M2, :] = sl[0:n_mem]
        h_ref[M2 + n_mem:RB, :] = sl[n_mem:seg]
        return _cat([m1n, m2n])

    def single_body(t, c):
        @pl.when(t >= n_seg)
        def _():
            out_copy(t - (LAG + 3)).start()
        return step(t, c, False)

    def full_body(i, c):
        t = LAG + UNROLL * i
        for u in range(UNROLL):
            @pl.when(t - u >= LAG + 2)
            def _():
                out_copy(t - u - (LAG + 2)).start()
        for u in range(UNROLL):
            c = step(t + u, c, True, u, i)
        return c

    def phase(ph, c):
        t0 = ph * n_seg
        c = lax.fori_loop(t0, t0 + LAG, single_body, c)

        @pl.when(ph == 0)
        def _():
            x_late.wait()
        return lax.fori_loop(0, jnp.where(ph == 0, (n_seg - LAG) // UNROLL, 0), full_body, c)
    lax.fori_loop(0, 2, phase, _cat([h_ref[0:n_mem, :], h_ref[M2:M2 + n_mem, :]]))

    out_copy(n_seg - 3).start()
    res = xb_ref[2 * seg:4 * seg, :]
    blhs = _ln(res).astype(BF16)
    ob = b_attn([(1, n_seg - 2), (1, n_seg - 1)], *[b_proj(blhs, part) for part in range(3)])
    o_store(n_seg - 2, b_out(_cat(ob), res))
    out_copy(n_seg - 2).start()
    out_copy(n_seg - 1).start()
    pltpu.make_async_copy(o_ref.at[pl.ds(seg, S), :], out_hbm, sem_o).wait()


@functools.partial(jax.jit, static_argnames=("seg",))
def _run(A_x, A_mem0, A_Wq, A_Wk, A_Wv, A_Wo, B_wqkv, B_wo, *, seg):
    _, S, dm = A_x.shape
    n_heads, dh = A_Wq.shape[1], A_Wq.shape[2]
    n_mem = A_mem0.shape[1]
    n_seg = S // seg
    hd = n_heads * dh
    nct = dm // 128
    assert (seg, n_seg, n_mem, dh, dm % 128, n_heads, LAG, UNROLL) == (32, 64, 8, 192, 0, 32, 2, 2)

    x = A_x.reshape(S, dm)
    mem0 = A_mem0.reshape(n_mem, dm)
    wq = jnp.transpose(A_Wq, (1, 2, 0)).reshape(hd, dm)
    wk = jnp.transpose(A_Wk, (1, 2, 0)).reshape(hd, dm)
    wv = jnp.transpose(A_Wv, (1, 2, 0)).reshape(hd, dm)
    wo = A_Wo.reshape(hd, dm)
    _, _, _, _, rs, xc = _plan(seg, n_seg)

    kern = functools.partial(_kernel, seg=seg, n_seg=n_seg, n_mem=n_mem,
                             n_heads=n_heads, dh=dh, dm=dm)
    hbm = pl.BlockSpec(memory_space=pltpu.HBM)

    out = pl.pallas_call(
        kern,
        in_specs=[hbm] * 8,
        out_specs=hbm,
        out_shape=jax.ShapeDtypeStruct((S, dm), A_x.dtype),
        scratch_shapes=[
            pltpu.VMEM((S, dm), BF16),
            pltpu.VMEM((n_mem, dm), BF16),
            pltpu.VMEM((NSLOT, 4, 2 * dh, dm), BF16),
            pltpu.VMEM((3 * n_heads // 2, NTILE * 64, 128), U32),
            pltpu.VMEM((n_heads // 2, NTILE * 64, 128), U32),
            pltpu.VMEM((dm, 4 * dm + 128), BF16),
            pltpu.VMEM((nct, 5 * dm + 32, 128), F32),
            pltpu.VMEM((4 * nct + 1, dm // 2, 128), U32),
            pltpu.VMEM((NTILE, NXC * xc // 4, 128), U32),
            pltpu.VMEM((3 * hd // 128, rs // 2 + 8, 128), U32),
            pltpu.VMEM((3 * n_mem + seg + AHS[0], dm), F32),
            pltpu.VMEM((4 * seg, dm), F32),
            pltpu.VMEM((seg, dm), F32),
            pltpu.VMEM((2, nct, HIST + seg, 128), F32),
            pltpu.VMEM((2, nct, HIST + seg, 128), F32),
            pltpu.VMEM((S + seg, dm), A_x.dtype),
            pltpu.SemaphoreType.DMA((NSLOT,)),
            pltpu.SemaphoreType.DMA((7 + NXC,)),
            pltpu.SemaphoreType.DMA((4,)),
            pltpu.SemaphoreType.DMA(()),
        ],
        compiler_params=pltpu.CompilerParams(
            vmem_limit_bytes=120 * 1024 * 1024,
            disable_bounds_checks=True,
        ),
    )(x, mem0, wq, wk, wv, wo, B_wqkv, B_wo)
    return out.reshape(1, S, dm)


def pallas_interleave_layers__memory_aug_recurrent_mem_tr__sliding_local_dilated__prompt_kernel(
    A_x: jax.Array,
    A_mem0: jax.Array,
    A_Wq: jax.Array,
    A_Wk: jax.Array,
    A_Wv: jax.Array,
    A_Wo: jax.Array,
    A_seg_len,
    B_x: jax.Array,
    B_wqkv: jax.Array,
    B_wo: jax.Array,
):
    del B_x
    seg = A_seg_len if isinstance(A_seg_len, int) else 32
    return _run(A_x, A_mem0, A_Wq, A_Wk, A_Wv, A_Wo, B_wqkv, B_wo, seg=seg)
```

```python
import functools

import jax
import jax.numpy as jnp
from jax import lax
import jax.experimental.pallas as pl
import jax.experimental.pallas.tpu as pltpu

F32 = jnp.float32
BF16 = jnp.bfloat16
U32 = jnp.uint32
NEG = -1000000000.0
LN_EPS = 1e-05
LOG2E = 1.4426950408889634
NEG2 = NEG * LOG2E

B_HEADS = 32
B_WIN = 8
B_DIL = 2
HIST = 16
AHS = (32, 16)
LAG = 2
NSLOT = 4
NNM = '001'
NNF = '000'
WSCHED = '4:0,5:1,6:2,7:3,8:4'
BOUT_R = 6
NXC = 3
UNROLL = 2


def _ln(x):
    m = jnp.mean(x, axis=-1, keepdims=True)
    c = x - m
    v = jnp.mean(c * c, axis=-1, keepdims=True)
    return c * lax.rsqrt(v + LN_EPS)


def _recip(d):
    r = pl.reciprocal(d, approx=True)
    return r * (2.0 - d * r)


def _nt(a, b):
    return lax.dot_general(a, b, (((1,), (1,)), ((), ())), preferred_element_type=F32)


def _nn(a, b):
    return jnp.dot(a, b, preferred_element_type=F32)


def _cat(xs, axis=0):
    return xs[0] if len(xs) == 1 else jnp.concatenate(xs, axis=axis)


def _pk(z):
    return pltpu.bitcast(z, U32)


def _upk(z):
    return pltpu.bitcast(z, BF16)


LAM = (-1.5, -0.5, 0.0, 0.5, 1.5)


def _scheme(stars):
    tiles, prog = [], []
    for star in stars:
        if len(star) == 1:
            prog.append(("single", star[0], None, len(tiles)))
            tiles.append([star[0][:2]])
            continue
        left = [len(star) - 1] * len(star)
        for j in range(1, len(star)):
            for i in range(j):
                x, y = star[i], star[j]
                prog.append(("pair", x, y, len(tiles)))
                tiles += [[(x[0], y[1])], [(y[0], x[1])], [(x[0], y[1]), (y[0], x[1])]]
                for e in (i, j):
                    left[e] -= 1
                    if left[e] == 0:
                        z = star[e]
                        prog.append(("diag", z, None, len(tiles)))
                        tiles += [[z[:2]] + [(o[0], z[1]) for o in star if o is not z],
                                  [z[:2]] + [(z[0], o[1]) for o in star if o is not z]]
    return tiles, prog


S55 = _scheme([[(i, i, LAM[i]) for i in range(5)]])
S53 = _scheme([[(0, 0, LAM[0]), (2, 1, LAM[2]), (4, 2, LAM[4])], [(1, 0, LAM[1]), (3, 2, LAM[3])],
               [(1, 1, LAM[1])], [(3, 1, LAM[3])]])
S35 = _scheme([[(0, 0, LAM[0]), (1, 2, LAM[2]), (2, 4, LAM[4])], [(0, 1, LAM[1]), (2, 3, LAM[3])],
               [(1, 1, LAM[1])], [(1, 3, LAM[3])]])


def _op_keys(prog):
    keys = []
    for kind, x, y, _ in prog:
        if kind == "pair":
            new = [(nm, x[0], x[2], y[0], y[2]) for nm in ("l1", "l2", "A")]
        else:
            new = [("a", x[0], x[2]), ("b", x[0])]
        keys += [k for k in new if k not in keys]
    return keys


def _scaled(c, u):
    return u if c == 1.0 else c * u


class _Operands:
    def __init__(self, T, U, E):
        self.T, self.U, self.E, self.memo = T, U, E, {}

    def _get(self, key, fn):
        if key not in self.memo:
            self.memo[key] = fn()
        return self.memo[key]

    def paired(self, key):
        T, U = self.T, self.U
        if key[0] == "b":
            return U[key[1]]
        if key[0] == "a":
            k, lam = key[1:]
            if lam == 0.0:
                return T[k]
            return self._get(("f",) + key, lambda: T[k] - _scaled(lam, U[k]) if lam > 0
                             else T[k] + _scaled(-lam, U[k]))
        kx, lx, ky, ly = key[1:]
        A = self._get(("f", "A") + key[1:],
                      lambda: self.paired(("a", kx, lx)) + self.paired(("a", ky, ly)))
        if key[0] == "A":
            return A
        return A - _scaled(ly - lx, U[kx]) if key[0] == "l1" else A + _scaled(ly - lx, U[ky])

    def extra(self, key):
        if key[0] == "a":
            return self.E[key[1]]
        return self._get(("e", key[1], key[3]), lambda: self.E[key[1]] + self.E[key[3]])

    def __call__(self, key):
        if self.T is None:
            ek = ("a", key[1]) if key[0] in ("a", "s") else ("l", key[1], 0, key[3])
            return self._get(ek, lambda: self.extra(ek).astype(BF16))

        def build():
            ak = ("a",) + key[1:] if key[0] == "s" else key
            parts = [self.paired(ak)]
            if self.E is not None and ak[0] in ("a", "l1", "l2"):
                parts.append(self.extra(ak))
            if key[0] == "s":
                parts.append(self.U[key[1]])
            return _cat(parts).astype(BF16)
        return self._get(key, build)


def _fast_mm(prog, op, dot, m, p, q):
    def add(d, key, val):
        d[key] = val if key not in d else d[key] + val

    for kind, x, y, i in prog:
        if kind == "pair":
            kk = (x[0], x[2], y[0], y[2])
            p1, p2 = dot(op(("l1",) + kk), i), dot(op(("l2",) + kk), i + 1)
            if m:
                r = _scaled(1.0 / (y[2] - x[2]), p2[0:m] - p1[0:m] + dot(op(("A",) + kk), i + 2))
                add(q, (x[1], x[2]), r)
                add(q, (y[1], y[2]), r)
            add(p, y[1], p1)
            add(p, x[1], p2)
        elif kind == "diag":
            add(p, x[1], dot(op(("a", x[0], x[2])), i))
            if m:
                add(q, (x[1], x[2]), dot(op(("b", x[0])), i + 1))
        else:
            r = dot(op(("s", x[0], x[2])), i)
            add(p, x[1], r[0:r.shape[0] - m])
            if m:
                add(q, (x[1], x[2]), r[r.shape[0] - m:])


def _fast_out(p, q, n, m):
    if not m:
        return None, None, p[n]
    y, z = p[n][0:m], None
    for (nn, lam), v in q.items():
        if nn == n:
            z = v if z is None else z + v
            if lam != 0.0:
                y = y + _scaled(lam, v) if lam > 0 else y - _scaled(-lam, v)
    return y, z, (p[n][m:] if p[n].shape[0] > m else None)


def _combo(tile, block):
    out = block(*tile[0])
    for kn in tile[1:]:
        out = out - block(*kn)
    return out


GT = 5
RT = 3
KEYS_R = _op_keys(S53[1])
KEYS = KEYS_R + [k for k in _op_keys(S55[1]) if k not in KEYS_R]


def _plan(seg, n_seg):
    S = seg * n_seg
    R0 = LAG * seg
    A0 = S - (n_seg - LAG) // UNROLL * sum(AHS)
    NPRE = A0 - R0 - LAG * 8
    RS = -(-(A0 - R0 + AHS[0]) // seg) * seg
    XC = NPRE // NXC
    assert XC % 32 == 0 and XC * NXC == NPRE
    return S, R0, A0, NPRE, RS, XC


def _kernel(x_hbm, mem0_hbm, wq_hbm, wk_hbm, wv_hbm, wo_hbm, bqkv_hbm, bwo_hbm,
            out_hbm,
            x_ref, mem0_ref, stage_ref, stage0_ref, wr_ref, w_ref, bst_ref, btmp_ref, bw_ref,
            xln_ref, ring_ref, h_ref, xb_ref, x2_ref, kb_ref, vb_ref, o_ref,
            sem_w, sem_m, sem_b, sem_o,
            *, seg, n_seg, n_mem, n_heads, dh, dm):
    S, R0, A0, NPRE, RS, XC = _plan(seg, n_seg)
    M2 = 2 * n_mem
    R = M2 + 2 * seg
    RB = M2 + seg
    PW = 2 * dh
    G = n_heads // 2
    nct = dm // 128
    bdh = dm // B_HEADS
    NT = n_heads * dh // 128
    NG = (NT - RT) // GT
    w_hbm = (wq_hbm, wk_hbm, wv_hbm, wo_hbm)

    def w_copy(p, g):
        slot = g & (NSLOT - 1)
        return pltpu.make_async_copy(w_hbm[p].at[pl.ds((RT + (g - 1) * GT) * 128, GT * 128), :],
                                     stage_ref.at[slot, p], sem_w.at[slot])

    def w0_copy(p):
        return pltpu.make_async_copy(w_hbm[p].at[pl.ds(0, RT * 128), :], stage0_ref.at[p], sem_m.at[4 + p])

    NB1 = 3 * nct
    WO0 = 3 * dm
    DUM = 4 * dm
    XF = A0 + AHS[0]
    XH = XC // 2

    def rows_copy(r0, n, sem):
        return pltpu.make_async_copy(x_hbm.at[pl.ds(r0, n), :], x_ref.at[pl.ds(r0, n), :], sem)

    def x_copy(i):
        return rows_copy(pl.multiple_of(R0 + i * XC, 16), XC, sem_m.at[8 + i])

    small = [rows_copy(0, R0, sem_m.at[1]), rows_copy(R0 + NPRE, XF - R0 - NPRE, sem_m.at[2]),
             pltpu.make_async_copy(mem0_hbm, mem0_ref, sem_m.at[3])]
    x_late = rows_copy(XF, S - XF, sem_m.at[0])

    def bq_copy(part):
        c0 = pl.multiple_of(part * dm, 128)
        return pltpu.make_async_copy(bqkv_hbm.at[:, pl.ds(c0, dm)], bst_ref.at[:, pl.ds(c0, dm)], sem_b.at[part])

    bo_copy = pltpu.make_async_copy(bwo_hbm, bst_ref.at[:, pl.ds(3 * dm, dm)], sem_b.at[3])

    def bst_tile(c):
        return bst_ref[:, pl.ds(pl.multiple_of(c * 128, 128), 128)]

    for i in range(NXC):
        x_copy(i).start()
    for cp in small:
        cp.start()

    def zero_body(j, c):
        btmp_ref[j, DUM:, :] = jnp.zeros((btmp_ref.shape[1] - DUM, 128), F32)
        return c
    lax.fori_loop(0, nct, zero_body, 0)

    for p in range(3):
        w0_copy(p).start()
    for p in range(4):
        w_copy(p, 1).start()
    xb_ref[0:2 * seg, :] = jnp.zeros((2 * seg, dm), F32)
    kb_ref[...] = jnp.zeros(kb_ref.shape, F32)
    vb_ref[...] = jnp.zeros(vb_ref.shape, F32)
    bst_ref[:, 4 * dm:] = jnp.zeros((dm, 128), BF16)

    def ln_ops(i, lo, hi):
        y = _ln(x_ref[pl.ds(pl.multiple_of(R0 + i * XC, 16), XC), :].astype(F32))
        ops = _Operands([y[0:XH, k * 128:(k + 1) * 128] for k in range(nct)],
                        [y[XH:XC, k * 128:(k + 1) * 128] for k in range(nct)], None)
        r0 = pl.multiple_of(i * (XH // 2), 8)
        for j in range(lo, hi):
            xln_ref[j, pl.ds(r0, XH // 2), :] = _pk(ops(KEYS[j]))

    def ln_body(i, c):
        x_copy(i).wait()
        ln_ops(i, 0, len(KEYS_R))
        return c
    lax.fori_loop(0, NXC, ln_body, 0)
    for cp in small:
        cp.wait()
    bq_copy(0).start()

    def pre_chunk(scheme, w, dst, n0, nn):
        tiles, prog = scheme
        strips = []
        for r in range(0, 128, 16):
            memo = {}

            def block(k, n):
                if (k, n) not in memo:
                    memo[k, n] = w[n * 128 + r:n * 128 + r + 16, k * 128:(k + 1) * 128].astype(F32)
                return memo[k, n]
            strips.append([_combo(tl, block) if len(tl) > 1 else None for tl in tiles])
        tb = []
        for i, tl in enumerate(tiles):
            if len(tl) == 1:
                k, n = tl[0]
                tb.append(w[n * 128:(n + 1) * 128, k * 128:(k + 1) * 128])
            else:
                tb.append(_cat([st[i] for st in strips]).astype(BF16))
        for i, x in enumerate(tb):
            dst[i * 64:(i + 1) * 64, :] = _pk(x.T)

        for c in range(NXC):
            def op(key):
                def ld(kk):
                    return _upk(xln_ref[KEYS.index(kk), c * (XH // 2):(c + 1) * (XH // 2), :])
                if key[0] == "s":
                    return _cat([ld(("a",) + key[1:]), ld(("b", key[1]))])
                return ld(key)
            if nn[c] == '1':
                dot = lambda a, i: _nn(a, _upk(dst[i * 64:(i + 1) * 64, :]))
            else:
                dot = lambda a, i: _nt(a, tb[i])
            p, q = {}, {}
            _fast_mm(prog, op, dot, XH, p, q)
            for n in range(len(p)):
                y, z, _ = _fast_out(p, q, n, XH)
                ring_ref[n0 + n, c * XH:c * XH + XH // 2, :] = _pk(y.astype(BF16))
                ring_ref[n0 + n, c * XH + XH // 2:(c + 1) * XH, :] = _pk(z.astype(BF16))

    def init_rows():
        x0 = x_ref[0:seg, :].astype(F32)
        sl = _ln(x0)
        xt = _ln(x_ref[R0 + NPRE:XF, :].astype(F32))
        h_ref[0:n_mem, :] = xt[0:n_mem]
        h_ref[n_mem:M2, :] = sl[0:n_mem]
        h_ref[M2:M2 + n_mem, :] = mem0_ref[...].astype(F32)
        h_ref[M2 + n_mem:RB, :] = sl[n_mem:seg]
        h_ref[RB:RB + AHS[0], :] = xt[M2:M2 + AHS[0]]
        h_ref[RB + AHS[0]:RB + AHS[0] + n_mem, :] = xt[n_mem:M2]
        x2_ref[...] = x0

    def first_body(p, c):
        buf = stage0_ref.at[p]
        pltpu.make_async_copy(buf, buf, sem_m.at[4 + p]).wait()

        @pl.when(p == 0)
        def _():
            for pp in range(4):
                w_copy(pp, 2).start()
        init_rows()
        pre_chunk(S53, buf, wr_ref.at[p], p * NT, NNF)
        ln_ops(p, len(KEYS_R), len(KEYS))
        return c
    lax.fori_loop(0, 3, first_body, 0)

    dpt = 128 // B_HEADS

    def b_stage1(u):
        ok = (u >= 0) & (u < NB1)
        tr = bst_tile(jnp.where(ok, u, NB1 + nct)).astype(F32).T
        r0 = pl.multiple_of(jnp.where(ok, u * 128, DUM), 128)
        for j in range(nct):
            btmp_ref[j, pl.ds(r0, 128), :] = tr[:, j * 128:(j + 1) * 128]

    def b_stage1_wo(u):
        ok = (u >= 0) & (u < nct)
        r0 = pl.multiple_of(jnp.where(ok, WO0, DUM), 128)
        btmp_ref[jnp.where(ok, u, 0), pl.ds(r0, dm), :] = bst_tile(
            jnp.where(ok, NB1 + u, NB1 + nct)).astype(F32)

    def b_stage2(u):
        ok = (u >= 0) & (u < NB1)
        part = (u >= nct).astype(jnp.int32) + (u >= 2 * nct).astype(jnp.int32)
        r0 = jnp.where(ok, part * dm + (u - part * nct) * dpt, DUM)
        rows = _cat([_cat([btmp_ref[j, pl.ds(r0 + dd, B_HEADS, stride=bdh), :]
                           for j in range(nct)], axis=1) for dd in range(dpt)])
        bw_ref[jnp.where(ok, u, NB1 + nct)] = _pk(rows.T.astype(BF16))

    def b_stage2_wo(u):
        ok = (u >= 0) & (u < nct)
        r0 = jnp.where(ok, WO0, DUM)
        jj = jnp.where(ok, u, 0)
        bw_ref[jnp.where(ok, NB1 + u, NB1 + nct)] = _pk(
            _cat([btmp_ref[jj, pl.ds(r0 + d, B_HEADS, stride=bdh), :] for d in range(bdh)]).astype(BF16))

    def wo_store(scheme, w, dst):
        for r in range(0, 128, 16):
            memo = {}

            def raw(k, n):
                return w[k * 128 + r:k * 128 + r + 16, n * 128:(n + 1) * 128]

            def block(k, n):
                if (k, n) not in memo:
                    memo[k, n] = raw(k, n).astype(F32)
                return memo[k, n]
            for i, tl in enumerate(scheme[0]):
                val = raw(*tl[0]) if len(tl) == 1 else _combo(tl, block).astype(BF16)
                dst[i * 64 + r // 2:i * 64 + r // 2 + 8, :] = _pk(val)

    def pre_body(g, c):
        slot = g & (NSLOT - 1)
        buf = stage_ref.at[slot]
        pltpu.make_async_copy(buf, buf, sem_w.at[slot]).wait()

        @pl.when((g >= 2) & (g <= 4))
        def _():
            bq_copy(g - 2).wait()

        @pl.when(g == 4)
        def _():
            bo_copy.wait()

        @pl.when(g <= 2)
        def _():
            bq_copy(g).start()

        @pl.when(g == 2)
        def _():
            bo_copy.start()

        @pl.when(g + 2 <= NG)
        def _():
            for p in range(4):
                w_copy(p, g + 2).start()

        @pl.when(g == NG - 1)
        def _():
            w0_copy(3).start()
            x_late.start()

        wo_store(S55, stage_ref.at[slot, 3], w_ref.at[3 * NG + g - 1])
        for e in range(3):
            b_stage2(3 * (g - 5) + e)
        b_stage2_wo(g - 5)
        for e in range(3):
            b_stage1(3 * (g - 2) + e)
        b_stage1_wo(g - 4)
        for p in range(3):
            pre_chunk(S55, stage_ref.at[slot, p], w_ref.at[p * NG + g - 1], p * NT + RT + (g - 1) * GT, NNM)
        return c
    lax.fori_loop(1, NG + 1, pre_body, 0)
    w0_copy(3).wait()

    bscale = float(bdh) ** (-0.5) * LOG2E

    def b_proj(lhs, part):
        return _nn(lhs, _cat([_upk(bw_ref[part * nct + j]) for j in range(nct)], axis=1))

    def b_attn(jobs, q, k, v):
        row = lax.broadcasted_iota(jnp.int32, (seg, 128), 0)
        outs = []
        for i, (l, sidx) in enumerate(jobs):
            r0 = i * seg
            pos = row + sidx * seg
            for j in range(nct):
                kb_ref[l, j, HIST:HIST + seg, :] = k[r0:r0 + seg, j * 128:(j + 1) * 128]
                vb_ref[l, j, HIST:HIST + seg, :] = v[r0:r0 + seg, j * 128:(j + 1) * 128]
            logits = []
            for w in range(B_WIN):
                o = HIST - w * B_DIL
                acc = None
                for j in range(nct):
                    p = q[r0:r0 + seg, j * 128:(j + 1) * 128] * kb_ref[l, j, o:o + seg, :]
                    acc = p if acc is None else acc + p
                acc = acc + pltpu.roll(acc, 64, 1)
                acc = acc + pltpu.roll(acc, 32, 1)
                lg = acc * bscale
                if w > 0:
                    lg = jnp.where(pos >= w * B_DIL, lg, NEG2)
                logits.append(lg)
            m = logits[0]
            for w in range(1, B_WIN):
                m = jnp.maximum(m, logits[w])
            es = [jnp.exp2(lg - m) for lg in logits]
            den = es[0]
            for w in range(1, B_WIN):
                den = den + es[w]
            inv = _recip(den)
            cols = []
            for j in range(nct):
                acc = None
                for w in range(B_WIN):
                    o = HIST - w * B_DIL
                    p = es[w] * vb_ref[l, j, o:o + seg, :]
                    acc = p if acc is None else acc + p
                cols.append(acc * inv)
            outs.append(_cat(cols, axis=1).astype(BF16))
            for j in range(nct):
                kb_ref[l, j, 0:HIST, :] = k[r0 + seg - HIST:r0 + seg, j * 128:(j + 1) * 128]
                vb_ref[l, j, 0:HIST, :] = v[r0 + seg - HIST:r0 + seg, j * 128:(j + 1) * 128]
        return outs

    def b_out(ob, res):
        return res + _nn(ob, _cat([_upk(bw_ref[NB1 + j]) for j in range(nct)], axis=1))

    def o_store(b, val):
        ro = pl.multiple_of((b + 1) * seg, seg)
        o_ref[pl.ds(ro, val.shape[0]), :] = val.astype(o_ref.dtype)

    def out_copy(b):
        ro = pl.multiple_of(b * seg, seg)
        return pltpu.make_async_copy(o_ref.at[pl.ds(ro + seg, seg), :], out_hbm.at[pl.ds(ro, seg), :], sem_o)

    def step(t, hc, full, u=0, i=None):
        t_last = n_seg + LAG - 1
        if full:
            jobs = [(0, t - 1), (1, t - 1 - LAG)]

            def b_in():
                return xb_ref[0:2 * seg, :]
        else:
            lb = (t == t_last).astype(jnp.int32)
            jobs = [(lb, t - 1 - lb * (LAG + 1))]

            def b_in():
                return xb_ref[pl.ds(pl.multiple_of(lb * seg, seg), seg), :]
        split = full and u < UNROLL - 1
        nq = RB + AHS[u] if full else RB
        v0r = _cat([hc[0:n_mem], h_ref[n_mem:M2, :]])
        v1r = _cat([hc[n_mem:M2], h_ref[M2 + n_mem:2 * M2, :]])

        def ktiles(z):
            return [z[:, k * 128:(k + 1) * 128] for k in range(z.shape[1] // 128)]
        if full:
            hl = _Operands(ktiles(_cat([v0r, h_ref[2 * M2:RB, :]])), ktiles(_cat([v1r, h_ref[RB:RB + 16, :]])),
                           ktiles(h_ref[RB + 16:nq, :]) if nq > RB + 16 else None)
        else:
            hl = _Operands(None, None, ktiles(_cat([v0r, v1r, h_ref[2 * M2:RB, :]])))
        mh = 2 * M2 if full else 0

        def tile_dot(p, r):
            src = wr_ref.at[p] if r == 0 else w_ref.at[p * NG + r - 1]
            return lambda a, i: _nn(a, _upk(src[i * 64:(i + 1) * 64, :]))
        scale = float(dh) ** (-0.5) * LOG2E
        if full:
            s_ = t - LAG
            rd = pl.multiple_of(lax.rem(s_ * (seg // 2), RS // 2), seg // 2)
            a_off = i * sum(AHS) + sum(AHS[:u])
            wa = [pl.multiple_of(lax.rem((A0 - R0 + a_off) // 2 + 8 * a, RS // 2), 8)
                  for a in range(AHS[u] // 16)]
        else:
            wx = pl.multiple_of(jnp.where(t < LAG, NPRE // 2 + t * (n_mem // 2), RS // 2), n_mem // 2)
            wo_store(S35, stage0_ref.at[3], wr_ref.at[3])

        RA = R if full else M2 + seg
        CW = R + 2 * M2 if full else R
        ri = lax.broadcasted_iota(jnp.int32, (RA, CW), 0)
        ci = lax.broadcasted_iota(jnp.int32, (RA, CW), 1)
        if not full:
            ri = jnp.where(ri >= M2, ri + seg, ri)

        def table(i, bounds, vals):
            out = vals[-1]
            for b, v in zip(reversed(bounds), reversed(vals[:-1])):
                out = jnp.where(i < b, v, out)
            return out
        qi = ri - table(ri, [16, 48, 56], [0, 8, 48, 40])
        g0 = (ci < 8) | ((ci >= 16) & (ci < 48))
        k2 = ci - table(ci, [8, 24, 32, 48, 56, 80, 88, 96, 104], [-8, 0, 24, 8, 48, 40, 72, 80, 96, 104])
        if full:
            k1 = ci - table(ci, [8, 48], [0, 8, 40])
            row_l2 = ((ri >= 8) & (ri < 16)) | (ri >= 48)
            row_xa = (ri >= 8) & (ri < 16)
            valid = row_xa == (ci >= 80)
            is_a = jnp.where(ci >= 80, ((ci >= 88) & (ci < 104)).astype(jnp.int32),
                             (g0 != row_l2).astype(jnp.int32)) > 0
            ki = jnp.where(row_l2, k2, k1)
            visible = valid & ((qi < n_mem) | (qi >= ki))
            fill = jnp.where(valid, NEG2, -jnp.inf)
        else:
            is_a = jnp.logical_not(g0)
            visible = (qi < n_mem) | (qi >= k2)
            fill = NEG2
        half = dh - 128
        la8 = lax.broadcasted_iota(jnp.int32, (n_mem, 128), 1) < half
        ones = jnp.full((n_mem, 128), 0xFFFFFFFF, U32)
        zero = jnp.zeros((n_mem, 128), U32)
        mask_a = jnp.where(la8, ones, zero)
        mask_b = jnp.where(la8, zero, ones)

        def pk2(a, b):
            return _pk(_cat([a, b]).astype(BF16))

        yt = [[None] * NT for _ in range(3)]
        x1 = [[None] * NT for _ in range(3)]

        def proj(p, r):
            pa, qa = {}, {}
            _fast_mm((S53 if r == 0 else S55)[1], hl, tile_dot(p, r), mh, pa, qa)
            n0 = 0 if r == 0 else RT + (r - 1) * GT
            for n in range(len(pa)):
                y, z, e = _fast_out(pa, qa, n, mh)
                idx = p * NT + n0 + n
                if full:
                    y = _cat([y[0:M2], z[0:M2], y[M2:2 * M2], z[M2:2 * M2]] + ([] if e is None else [e]))
                    for a in range(AHS[u] // 16):
                        rr = RB + 16 * a
                        ring_ref[idx, pl.ds(wa[a], 8), :] = pk2(y[rr:rr + 8], y[rr + 8:rr + 16])
                else:
                    y = e
                    ring_ref[idx, pl.ds(wx, n_mem // 2), :] = pk2(y[0:8], y[8:16])[0:n_mem // 2]
                yt[p][n0 + n] = y
            if full:
                for n in range(len(pa)):
                    x1[p][n0 + n] = ring_ref[p * NT + n0 + n, pl.ds(rd, seg // 2), :]

        def pair(p, g):
            return yt[p][3 * g:3 * g + 3], x1[p][3 * g:3 * g + 3]

        def groups(z, j):
            y = z[0][j]
            return pk2(y[0:8], y[8:16]), pk2(y[16:24], y[24:32]), pk2(y[32:40], y[40:48])

        def q_rows(z, j):
            v0, v1, v2 = groups(z, j)
            return [v0] + ([z[1][j]] if full else []) + [v1, v2]

        def kv_tiles(z):
            yt, x1 = z
            v0, v1, v2 = groups(z, 0)
            t0 = [v0] + ([x1[0]] if full else [v1, v2]) + [v1, v2]
            y = yt[2]
            w0 = pk2(y[8:16], y[0:8])
            w1 = pk2(y[24:32], y[16:24])
            w2 = pk2(y[32:40], y[40:48])
            t2 = [w0, w1, w2] + ([x1[2]] if full else [w1, w2])
            if full:
                t0 += [v0, v1]
                t2 += [w0, w1]
            y = yt[1]

            def ab(z8):
                return jnp.where(la8, z8, 0.0), jnp.where(la8, 0.0, z8)
            xa_a, xa_b = ab(y[8:16])
            e1 = pk2(xa_b, xa_a)
            u2 = pk2(y[32:40], y[40:48])
            mid2 = [e1, pk2(y[24:32], y[16:24]) & mask_b, u2 & mask_b,
                    pk2(y[16:24], y[24:32]) & mask_a, u2 & mask_a]
            mid1 = None
            if full:
                lo, hi = x1[1][0:8], x1[1][8:16]
                mid1 = [pk2(*ab(y[0:8])), lo & mask_a, hi & mask_a, lo & mask_b, hi & mask_b,
                        e1, pk2(*ab(y[16:24]))]
            return t0, mid1, mid2, t2

        def mat(parts):
            return _upk(_cat(parts))

        def scores(q, k):
            k0, km1, km2, k2_ = kv_tiles(k)
            s_a = _nt(mat(q_rows(q, 0)), mat(k0))
            s_b = _nt(mat(q_rows(q, 2)), mat(k2_))
            qm = q_rows(q, 1)
            if full:
                s_m = _cat([_nt(mat(qm[0:2]), mat(km1)), _nt(mat(qm[2:4]), mat(km2 + km1[5:7]))])
            else:
                s_m = _nt(mat(qm), mat(km2))
            s = (jnp.where(is_a, s_a, s_b) + s_m) * scale
            s = jnp.where(visible, s, fill)
            m_a = jnp.max(jnp.where(is_a, s, -jnp.inf), axis=-1, keepdims=True)
            m_b = jnp.max(jnp.where(is_a, -jnp.inf, s), axis=-1, keepdims=True)
            e = jnp.exp2(s - jnp.where(is_a, m_a, m_b))
            d_a = jnp.sum(jnp.where(is_a, e, 0.0), axis=-1, keepdims=True)
            d_b = jnp.sum(jnp.where(is_a, 0.0, e), axis=-1, keepdims=True)
            return e * _recip(jnp.where(is_a, d_a, d_b))

        def pv(p, v):
            v0, vm1, vm2, v2 = kv_tiles(v)
            o_a = _nn(jnp.where(is_a, p, 0.0).astype(BF16), mat(v0))
            o_b = _nn(jnp.where(is_a, 0.0, p).astype(BF16), mat(v2))
            if full:
                o_m = _cat([_nn(p[0:M2 + seg].astype(BF16), mat(vm1)),
                            _nn(p[M2 + seg:R, 0:R].astype(BF16), mat(vm2))])
            else:
                o_m = _nn(p.astype(BF16), mat(vm2))
            return [o_a, o_m, o_b]

        ot = []
        pacc, qacc = {}, {}

        def add_o(r):
            n0 = 0 if r == 0 else RT + (r - 1) * GT
            oo = ot[n0:n0 + (RT if r == 0 else GT)]
            if full:
                ops = _Operands([o[0:32] for o in oo], [_cat([o[48:64], o[32:48]]) for o in oo],
                                [o[64:80] for o in oo])
            else:
                ops = _Operands(None, None, oo)
            _fast_mm((S35 if r == 0 else S55)[1], ops, tile_dot(3, r), mh, pacc, qacc)

        wsched = dict(tuple(int(v) for v in e.split(":")) for e in WSCHED.split(","))
        bqkv = [None] * 3
        probs = []
        x2_new = None

        def do_pv():
            for g in range(len(ot) // 3, len(probs)):
                ot.extend(pv(probs[g], pair(2, g)))

        for r in range(NG + 1):
            proj(1, r)
            proj(0, r)
            proj(2, r)
            do_pv()
            if r == 0:
                blhs = _ln(b_in()).astype(BF16)
            if r < 3:
                bqkv[2 - r] = b_proj(blhs, 2 - r)
            if r == 3:
                ob = b_attn(jobs, *bqkv)
            if r == BOUT_R:
                res = b_in()
                if split:
                    x2_new = b_out(ob[0], res[0:seg])
                elif full:
                    zb = b_out(_cat(ob), res)
                    x2_new = zb[0:seg]
                    o_store(t - 1 - LAG, zb[seg:2 * seg])
                else:
                    x2_new = b_out(ob[0], res)
                    o_store(lb * (t_last - LAG - 1) - 1, x2_new)
            if r in wsched:
                add_o(wsched[r])
            for g in range(len(probs), (RT + r * GT) // 3):
                probs.append(scores(pair(0, g), pair(1, g)))
        for r in range(len(wsched), NG - 2):
            add_o(r)
        do_pv()
        for r in range(NG - 2, NG + 1):
            add_o(r)
        cols = []
        for n in range(nct):
            y, z, e = _fast_out(pacc, qacc, n, mh)
            cols.append(_cat([y, z[16:32], z[0:16], e]) if full else e)
        acc = _cat(cols, axis=1)
        if split:
            o_store(t - 1 - LAG, b_out(ob[1], res[seg:2 * seg]))

        y2 = x2_ref[...] + _cat([acc[n_mem:M2], acc[RA - seg + n_mem:RA]])
        mem2 = acc[RA - seg:RA - seg + n_mem]
        if full:
            x_cur = x_ref[pl.ds(pl.multiple_of(t * seg, seg), seg), :].astype(F32)
            xb_ref[0:seg, :] = x_cur + acc[M2:M2 + seg]
            xb_ref[seg:2 * seg, :] = y2
            m1n = acc[0:n_mem]
            m2n = mem2
            ahn = AHS[(u + 1) % UNROLL]
            an = pl.multiple_of(jnp.minimum(A0 + a_off + AHS[u], S - ahn), 16)
            h_ref[RB:RB + ahn, :] = _ln(x_ref[pl.ds(an, ahn), :].astype(F32))
            nxt = x2_new
        else:
            xb_ref[pl.ds(pl.multiple_of(jnp.where(t < LAG, 0, (t - n_seg + 2) * seg), seg), seg), :] = y2
            m1n = jnp.where(t < LAG - 1, h_ref[RB + AHS[0]:RB + AHS[0] + n_mem, :], mem2)
            m2n = jnp.where(t == LAG - 1, mem0_ref[...].astype(F32), mem2)
            nxt = jnp.where(t < LAG - 1, x_ref[seg:2 * seg, :].astype(F32), x2_new)
        x2_ref[...] = nxt
        sl = _ln(nxt)
        h_ref[n_mem:M2, :] = sl[0:n_mem]
        h_ref[M2 + n_mem:RB, :] = sl[n_mem:seg]
        return _cat([m1n, m2n])

    def single_body(t, c):
        @pl.when(t >= n_seg)
        def _():
            out_copy(t - (LAG + 3)).start()
        return step(t, c, False)

    def full_body(i, c):
        t = LAG + UNROLL * i
        for u in range(UNROLL):
            @pl.when(t - u >= LAG + 2)
            def _():
                out_copy(t - u - (LAG + 2)).start()
        for u in range(UNROLL):
            c = step(t + u, c, True, u, i)
        return c

    def phase(ph, c):
        t0 = ph * n_seg
        c = lax.fori_loop(t0, t0 + LAG, single_body, c)

        @pl.when(ph == 0)
        def _():
            x_late.wait()
        return lax.fori_loop(0, jnp.where(ph == 0, (n_seg - LAG) // UNROLL, 0), full_body, c)
    lax.fori_loop(0, 2, phase, _cat([h_ref[0:n_mem, :], h_ref[M2:M2 + n_mem, :]]))

    out_copy(n_seg - 3).start()
    res = xb_ref[2 * seg:4 * seg, :]
    blhs = _ln(res).astype(BF16)
    ob = b_attn([(1, n_seg - 2), (1, n_seg - 1)], *[b_proj(blhs, part) for part in range(3)])
    o_store(n_seg - 2, b_out(_cat(ob), res))
    out_copy(n_seg - 2).start()
    out_copy(n_seg - 1).start()
    pltpu.make_async_copy(o_ref.at[pl.ds(seg, S), :], out_hbm, sem_o).wait()


@functools.partial(jax.jit, static_argnames=("seg",))
def _run(A_x, A_mem0, A_Wq, A_Wk, A_Wv, A_Wo, B_wqkv, B_wo, *, seg):
    _, S, dm = A_x.shape
    n_heads, dh = A_Wq.shape[1], A_Wq.shape[2]
    n_mem = A_mem0.shape[1]
    n_seg = S // seg
    hd = n_heads * dh
    nct = dm // 128
    ng = (hd // 128 - RT) // GT
    assert (seg, n_seg, n_mem, dh, dm % 128, n_heads, LAG, UNROLL) == (32, 64, 8, 192, 0, 32, 2, 2)

    x = A_x.reshape(S, dm)
    mem0 = A_mem0.reshape(n_mem, dm)
    wq = jnp.transpose(A_Wq, (1, 2, 0)).reshape(hd, dm)
    wk = jnp.transpose(A_Wk, (1, 2, 0)).reshape(hd, dm)
    wv = jnp.transpose(A_Wv, (1, 2, 0)).reshape(hd, dm)
    wo = A_Wo.reshape(hd, dm)
    _, _, _, _, rs, xc = _plan(seg, n_seg)

    kern = functools.partial(_kernel, seg=seg, n_seg=n_seg, n_mem=n_mem,
                             n_heads=n_heads, dh=dh, dm=dm)
    hbm = pl.BlockSpec(memory_space=pltpu.HBM)

    out = pl.pallas_call(
        kern,
        in_specs=[hbm] * 8,
        out_specs=hbm,
        out_shape=jax.ShapeDtypeStruct((S, dm), A_x.dtype),
        scratch_shapes=[
            pltpu.VMEM((S, dm), BF16),
            pltpu.VMEM((n_mem, dm), BF16),
            pltpu.VMEM((NSLOT, 4, GT * 128, dm), BF16),
            pltpu.VMEM((4, RT * 128, dm), BF16),
            pltpu.VMEM((4, len(S53[0]) * 64, 128), U32),
            pltpu.VMEM((4 * ng, len(S55[0]) * 64, 128), U32),
            pltpu.VMEM((dm, 4 * dm + 128), BF16),
            pltpu.VMEM((nct, 5 * dm + 32, 128), F32),
            pltpu.VMEM((4 * nct + 1, dm // 2, 128), U32),
            pltpu.VMEM((len(KEYS), NXC * xc // 4, 128), U32),
            pltpu.VMEM((3 * hd // 128, rs // 2 + 8, 128), U32),
            pltpu.VMEM((3 * n_mem + seg + AHS[0], dm), F32),
            pltpu.VMEM((4 * seg, dm), F32),
            pltpu.VMEM((seg, dm), F32),
            pltpu.VMEM((2, nct, HIST + seg, 128), F32),
            pltpu.VMEM((2, nct, HIST + seg, 128), F32),
            pltpu.VMEM((S + seg, dm), A_x.dtype),
            pltpu.SemaphoreType.DMA((NSLOT,)),
            pltpu.SemaphoreType.DMA((8 + NXC,)),
            pltpu.SemaphoreType.DMA((4,)),
            pltpu.SemaphoreType.DMA(()),
        ],
        compiler_params=pltpu.CompilerParams(
            vmem_limit_bytes=120 * 1024 * 1024,
            disable_bounds_checks=True,
        ),
    )(x, mem0, wq, wk, wv, wo, B_wqkv, B_wo)
    return out.reshape(1, S, dm)


def pallas_interleave_layers__memory_aug_recurrent_mem_tr__sliding_local_dilated__prompt_kernel(
    A_x: jax.Array,
    A_mem0: jax.Array,
    A_Wq: jax.Array,
    A_Wk: jax.Array,
    A_Wv: jax.Array,
    A_Wo: jax.Array,
    A_seg_len,
    B_x: jax.Array,
    B_wqkv: jax.Array,
    B_wo: jax.Array,
):
    del B_x
    seg = A_seg_len if isinstance(A_seg_len, int) else 32
    return _run(A_x, A_mem0, A_Wq, A_Wk, A_Wv, A_Wo, B_wqkv, B_wo, seg=seg)
```

```python
import functools

import jax
import jax.numpy as jnp
from jax import lax
import jax.experimental.pallas as pl
import jax.experimental.pallas.tpu as pltpu

F32 = jnp.float32
BF16 = jnp.bfloat16
U32 = jnp.uint32
NEG = -1000000000.0
LN_EPS = 1e-05
LOG2E = 1.4426950408889634
NEG2 = NEG * LOG2E

B_HEADS = 32
B_WIN = 8
B_DIL = 2
HIST = 16
AHS = (32, 16)
LAG = 2
NSLOT = 4
NNM = '000'
NNF = '000'
WSCHED = '4:0,5:1,6:2,7:3,8:4'
BOUT_R = int(6)
ORDR = 'kqvPFS'
TAILPV = int(7)
PERT = int(1)
WPOS = int(0)
SKIPM = int(0)
BT = int(0)
NOB = int(0)
WTT = int(1)
DORD = 'sss'
RCH = [int(v) for v in '80,80,80'.split(',')]
NXC = 3
UNROLL = 2


def _ln(x):
    m = jnp.mean(x, axis=-1, keepdims=True)
    c = x - m
    v = jnp.mean(c * c, axis=-1, keepdims=True)
    return c * lax.rsqrt(v + LN_EPS)


def _recip(d):
    r = pl.reciprocal(d, approx=True)
    return r * (2.0 - d * r)


def _nt(a, b):
    return lax.dot_general(a, b, (((1,), (1,)), ((), ())), preferred_element_type=F32)


def _nn(a, b):
    return jnp.dot(a, b, preferred_element_type=F32)


def _cat(xs, axis=0):
    return xs[0] if len(xs) == 1 else jnp.concatenate(xs, axis=axis)


def _pk(z):
    return pltpu.bitcast(z, U32)


def _upk(z):
    return pltpu.bitcast(z, BF16)


LAM = (-1.5, -0.5, 0.0, 0.5, 1.5)


def _scheme(stars):
    tiles, prog = [], []
    for star in stars:
        if len(star) == 1:
            prog.append(("single", star[0], None, len(tiles)))
            tiles.append([star[0][:2]])
            continue
        left = [len(star) - 1] * len(star)
        for j in range(1, len(star)):
            for i in range(j):
                x, y = star[i], star[j]
                prog.append(("pair", x, y, len(tiles)))
                tiles += [[(x[0], y[1])], [(y[0], x[1])], [(x[0], y[1]), (y[0], x[1])]]
                for e in (i, j):
                    left[e] -= 1
                    if left[e] == 0:
                        z = star[e]
                        prog.append(("diag", z, None, len(tiles)))
                        tiles += [[z[:2]] + [(o[0], z[1]) for o in star if o is not z],
                                  [z[:2]] + [(z[0], o[1]) for o in star if o is not z]]
    return tiles, prog


S55 = _scheme([[(i, i, LAM[i]) for i in range(5)]])
S53 = _scheme([[(0, 0, LAM[0]), (2, 1, LAM[2]), (4, 2, LAM[4])], [(1, 0, LAM[1]), (3, 2, LAM[3])],
               [(1, 1, LAM[1])], [(3, 1, LAM[3])]])
S35 = _scheme([[(0, 0, LAM[0]), (1, 2, LAM[2]), (2, 4, LAM[4])], [(0, 1, LAM[1]), (2, 3, LAM[3])],
               [(1, 1, LAM[1])], [(1, 3, LAM[3])]])


def _reorder(prog, mode):
    pairs = [e for e in prog if e[0] != "diag"]
    diags = [e for e in prog if e[0] == "diag"]
    if mode == "l":
        return prog
    out = []
    if mode == "f":
        for e in pairs:
            for z in (e[1], e[2]):
                for dg in diags:
                    if dg[1] == z and dg not in out:
                        out.append(dg)
            out.append(e)
        return out
    step = len(pairs) / len(diags)
    k = 0
    for i, e in enumerate(pairs):
        out.append(e)
        while k < len(diags) and (k + 0.5) * step <= i + 1:
            out.append(diags[k])
            k += 1
    return out + diags[k:]


def _op_keys(prog):
    keys = []
    for kind, x, y, _ in prog:
        if kind == "pair":
            new = [(nm, x[0], x[2], y[0], y[2]) for nm in ("l1", "l2", "A")]
        else:
            new = [("a", x[0], x[2]), ("b", x[0])]
        keys += [k for k in new if k not in keys]
    return keys


def _scaled(c, u):
    return u if c == 1.0 else c * u


class _Operands:
    def __init__(self, T, U, E):
        self.T, self.U, self.E, self.memo = T, U, E, {}

    def _get(self, key, fn):
        if key not in self.memo:
            self.memo[key] = fn()
        return self.memo[key]

    def paired(self, key):
        T, U = self.T, self.U
        if key[0] == "b":
            return U[key[1]]
        if key[0] == "a":
            k, lam = key[1:]
            if lam == 0.0:
                return T[k]
            return self._get(("f",) + key, lambda: T[k] - _scaled(lam, U[k]) if lam > 0
                             else T[k] + _scaled(-lam, U[k]))
        kx, lx, ky, ly = key[1:]
        A = self._get(("f", "A") + key[1:],
                      lambda: self.paired(("a", kx, lx)) + self.paired(("a", ky, ly)))
        if key[0] == "A":
            return A
        return A - _scaled(ly - lx, U[kx]) if key[0] == "l1" else A + _scaled(ly - lx, U[ky])

    def extra(self, key):
        if key[0] == "a":
            return self.E[key[1]]
        return self._get(("e", key[1], key[3]), lambda: self.E[key[1]] + self.E[key[3]])

    def __call__(self, key):
        if self.T is None:
            ek = ("a", key[1]) if key[0] in ("a", "s") else ("l", key[1], 0, key[3])
            return self._get(ek, lambda: self.extra(ek).astype(BF16))

        def build():
            ak = ("a",) + key[1:] if key[0] == "s" else key
            parts = [self.paired(ak)]
            if self.E is not None and ak[0] in ("a", "l1", "l2"):
                parts.append(self.extra(ak))
            if key[0] == "s":
                parts.append(self.U[key[1]])
            return _cat(parts).astype(BF16)
        return self._get(key, build)


def _fast_mm(prog, op, dot, m, p, q):
    def add(d, key, val):
        d[key] = val if key not in d else d[key] + val

    for kind, x, y, i in prog:
        if kind == "pair":
            kk = (x[0], x[2], y[0], y[2])
            p1, p2 = dot(op(("l1",) + kk), i), dot(op(("l2",) + kk), i + 1)
            if m:
                r = _scaled(1.0 / (y[2] - x[2]), p2[0:m] - p1[0:m] + dot(op(("A",) + kk), i + 2))
                add(q, (x[1], x[2]), r)
                add(q, (y[1], y[2]), r)
            add(p, y[1], p1)
            add(p, x[1], p2)
        elif kind == "diag":
            add(p, x[1], dot(op(("a", x[0], x[2])), i))
            if m:
                add(q, (x[1], x[2]), dot(op(("b", x[0])), i + 1))
        else:
            r = dot(op(("s", x[0], x[2])), i)
            add(p, x[1], r[0:r.shape[0] - m])
            if m:
                add(q, (x[1], x[2]), r[r.shape[0] - m:])


def _fast_out(p, q, n, m):
    if not m:
        return None, None, p[n]
    y, z = p[n][0:m], None
    for (nn, lam), v in q.items():
        if nn == n:
            z = v if z is None else z + v
            if lam != 0.0:
                y = y + _scaled(lam, v) if lam > 0 else y - _scaled(-lam, v)
    return y, z, (p[n][m:] if p[n].shape[0] > m else None)


def _combo(tile, block):
    out = block(*tile[0])
    for kn in tile[1:]:
        out = out - block(*kn)
    return out


GT = 5
RT = 3
KEYS_R = _op_keys(S53[1])
KEYS = KEYS_R + [k for k in _op_keys(S55[1]) if k not in KEYS_R]


def _plan(seg, n_seg):
    S = seg * n_seg
    R0 = LAG * seg
    A0 = S - (n_seg - LAG) // UNROLL * sum(AHS)
    NPRE = A0 - R0 - LAG * 8
    RS = -(-(A0 - R0 + AHS[0]) // seg) * seg
    XC = NPRE // NXC
    assert XC % 32 == 0 and XC * NXC == NPRE
    return S, R0, A0, NPRE, RS, XC


def _kernel(x_hbm, mem0_hbm, wq_hbm, wk_hbm, wv_hbm, wo_hbm, bqkv_hbm, bwo_hbm,
            out_hbm,
            x_ref, mem0_ref, stage_ref, stage0_ref, wr_ref, w_ref, bst_ref, btmp_ref, bw_ref,
            xln_ref, ring_ref, h_ref, xb_ref, x2_ref, kb_ref, vb_ref, o_ref,
            sem_w, sem_m, sem_b, sem_o,
            *, seg, n_seg, n_mem, n_heads, dh, dm):
    S, R0, A0, NPRE, RS, XC = _plan(seg, n_seg)
    M2 = 2 * n_mem
    R = M2 + 2 * seg
    RB = M2 + seg
    PW = 2 * dh
    G = n_heads // 2
    nct = dm // 128
    bdh = dm // B_HEADS
    NT = n_heads * dh // 128
    NG = (NT - RT) // GT
    w_hbm = (wq_hbm, wk_hbm, wv_hbm, wo_hbm)

    def w_copy(p, g):
        slot = g & (NSLOT - 1)
        return pltpu.make_async_copy(w_hbm[p].at[pl.ds((RT + (g - 1) * GT) * 128, GT * 128), :],
                                     stage_ref.at[slot, p], sem_w.at[slot])

    def w0_copy(p):
        return pltpu.make_async_copy(w_hbm[p].at[pl.ds(0, RT * 128), :], stage0_ref.at[p], sem_m.at[4 + p])

    NB1 = 3 * nct
    WO0 = 3 * dm
    DUM = 4 * dm
    XF = A0 + AHS[0]
    XH = XC // 2

    def rows_copy(r0, n, sem):
        return pltpu.make_async_copy(x_hbm.at[pl.ds(r0, n), :], x_ref.at[pl.ds(r0, n), :], sem)

    def x_copy(i):
        return rows_copy(pl.multiple_of(R0 + i * XC, 16), XC, sem_m.at[8 + i])

    small = [rows_copy(0, R0, sem_m.at[1]), rows_copy(R0 + NPRE, XF - R0 - NPRE, sem_m.at[2]),
             pltpu.make_async_copy(mem0_hbm, mem0_ref, sem_m.at[3])]
    x_late = rows_copy(XF, S - XF, sem_m.at[0])

    def bq_copy(part):
        c0 = pl.multiple_of(part * dm, 128)
        return pltpu.make_async_copy(bqkv_hbm.at[:, pl.ds(c0, dm)], bst_ref.at[:, pl.ds(c0, dm)], sem_b.at[part])

    bo_copy = pltpu.make_async_copy(bwo_hbm, bst_ref.at[:, pl.ds(3 * dm, dm)], sem_b.at[3])

    def bst_tile(c):
        return bst_ref[:, pl.ds(pl.multiple_of(c * 128, 128), 128)]

    for i in range(NXC):
        x_copy(i).start()
    for cp in small:
        cp.start()

    def zero_body(j, c):
        btmp_ref[j, DUM:, :] = jnp.zeros((btmp_ref.shape[1] - DUM, 128), F32)
        return c
    lax.fori_loop(0, nct, zero_body, 0)

    for p in range(3):
        w0_copy(p).start()
    for p in range(4):
        w_copy(p, 1).start()
    xb_ref[0:2 * seg, :] = jnp.zeros((2 * seg, dm), F32)
    kb_ref[...] = jnp.zeros(kb_ref.shape, F32)
    vb_ref[...] = jnp.zeros(vb_ref.shape, F32)
    bst_ref[:, 4 * dm:] = jnp.zeros((dm, 128), BF16)

    def ln_ops(i, lo, hi):
        y = _ln(x_ref[pl.ds(pl.multiple_of(R0 + i * XC, 16), XC), :].astype(F32))
        ops = _Operands([y[0:XH, k * 128:(k + 1) * 128] for k in range(nct)],
                        [y[XH:XC, k * 128:(k + 1) * 128] for k in range(nct)], None)
        r0 = pl.multiple_of(i * (XH // 2), 8)
        for j in range(lo, hi):
            xln_ref[j, pl.ds(r0, XH // 2), :] = _pk(ops(KEYS[j]))

    def ln_body(i, c):
        x_copy(i).wait()
        ln_ops(i, 0, len(KEYS_R))
        return c
    lax.fori_loop(0, NXC, ln_body, 0)
    for cp in small:
        cp.wait()
    bq_copy(0).start()

    def pre_chunk(scheme, w, dst, n0, nn, dord='l'):
        tiles, prog = scheme
        prog = _reorder(prog, dord)
        strips = []
        for r in range(0, 0 if PERT else 128, 16):
            memo = {}

            def block(k, n):
                if (k, n) not in memo:
                    memo[k, n] = w[n * 128 + r:n * 128 + r + 16, k * 128:(k + 1) * 128].astype(F32)
                return memo[k, n]
            strips.append([_combo(tl, block) if len(tl) > 1 else None for tl in tiles])
        tb = []
        for i, tl in enumerate(tiles):
            if len(tl) == 1:
                k, n = tl[0]
                tb.append(w[n * 128:(n + 1) * 128, k * 128:(k + 1) * 128])
            elif PERT:
                tb.append(_combo(tl, lambda k, n: w[n * 128:(n + 1) * 128, k * 128:(k + 1) * 128].astype(F32)
                                 ).astype(BF16))
            else:
                tb.append(_cat([st[i] for st in strips]).astype(BF16))
            if PERT:
                dst[i * 64:(i + 1) * 64, :] = _pk(tb[i].T)
        for i, x in enumerate(tb):
            if not PERT:
                dst[i * 64:(i + 1) * 64, :] = _pk(x.T)

        for c in range(NXC):
            def op(key):
                def ld(kk):
                    return _upk(xln_ref[KEYS.index(kk), c * (XH // 2):(c + 1) * (XH // 2), :])
                if key[0] == "s":
                    return _cat([ld(("a",) + key[1:]), ld(("b", key[1]))])
                return ld(key)
            if nn[c] == '1':
                dot = lambda a, i: _nn(a, _upk(dst[i * 64:(i + 1) * 64, :]))
            else:
                dot = lambda a, i: _nt(a, tb[i])
            p, q = {}, {}
            _fast_mm(prog, op, dot, XH, p, q)
            for n in range(len(p)):
                y, z, _ = _fast_out(p, q, n, XH)
                ring_ref[n0 + n, c * XH:c * XH + XH // 2, :] = _pk(y.astype(BF16))
                ring_ref[n0 + n, c * XH + XH // 2:(c + 1) * XH, :] = _pk(z.astype(BF16))

    def init_rows():
        x0 = x_ref[0:seg, :].astype(F32)
        sl = _ln(x0)
        xt = _ln(x_ref[R0 + NPRE:XF, :].astype(F32))
        h_ref[0:n_mem, :] = xt[0:n_mem]
        h_ref[n_mem:M2, :] = sl[0:n_mem]
        h_ref[M2:M2 + n_mem, :] = mem0_ref[...].astype(F32)
        h_ref[M2 + n_mem:RB, :] = sl[n_mem:seg]
        h_ref[RB:RB + AHS[0], :] = xt[M2:M2 + AHS[0]]
        h_ref[RB + AHS[0]:RB + AHS[0] + n_mem, :] = xt[n_mem:M2]
        x2_ref[...] = x0

    def first_body(p, c):
        buf = stage0_ref.at[p]
        pltpu.make_async_copy(buf, buf, sem_m.at[4 + p]).wait()

        @pl.when(p == 0)
        def _():
            for pp in range(4):
                w_copy(pp, 2).start()
        init_rows()
        pre_chunk(S53, buf, wr_ref.at[p], p * NT, NNF)
        ln_ops(p, len(KEYS_R), len(KEYS))
        return c
    lax.fori_loop(0, 3, first_body, 0)

    dpt = 128 // B_HEADS

    def b_stage1(u):
        ok = (u >= 0) & (u < NB1)
        tr = bst_tile(jnp.where(ok, u, NB1 + nct)).T.astype(F32) if BT & 1 else bst_tile(jnp.where(ok, u, NB1 + nct)).astype(F32).T
        r0 = pl.multiple_of(jnp.where(ok, u * 128, DUM), 128)
        for j in range(nct):
            btmp_ref[j, pl.ds(r0, 128), :] = tr[:, j * 128:(j + 1) * 128]

    def b_stage1_wo(u):
        ok = (u >= 0) & (u < nct)
        r0 = pl.multiple_of(jnp.where(ok, WO0, DUM), 128)
        btmp_ref[jnp.where(ok, u, 0), pl.ds(r0, dm), :] = bst_tile(
            jnp.where(ok, NB1 + u, NB1 + nct)).astype(F32)

    def b_stage2(u):
        ok = (u >= 0) & (u < NB1)
        part = (u >= nct).astype(jnp.int32) + (u >= 2 * nct).astype(jnp.int32)
        r0 = jnp.where(ok, part * dm + (u - part * nct) * dpt, DUM)
        rows = _cat([_cat([btmp_ref[j, pl.ds(r0 + dd, B_HEADS, stride=bdh), :]
                           for j in range(nct)], axis=1) for dd in range(dpt)])
        bw_ref[jnp.where(ok, u, NB1 + nct)] = _pk(rows.astype(BF16).T if BT & 2 else rows.T.astype(BF16))

    def b_stage2_wo(u):
        ok = (u >= 0) & (u < nct)
        r0 = jnp.where(ok, WO0, DUM)
        jj = jnp.where(ok, u, 0)
        bw_ref[jnp.where(ok, NB1 + u, NB1 + nct)] = _pk(
            _cat([btmp_ref[jj, pl.ds(r0 + d, B_HEADS, stride=bdh), :] for d in range(bdh)]).astype(BF16))

    def wo_store(scheme, w, dst):
        if WTT:
            rawt = lambda k, n: w[k * 128:(k + 1) * 128, n * 128:(n + 1) * 128]
            for i, tl in enumerate(scheme[0]):
                if len(tl) == 1:
                    val = rawt(*tl[0])
                    if WTT == 3:
                        val = _upk(_pk(val.T)).T
                else:
                    val = _combo(tl, lambda k, n: rawt(k, n).astype(F32)).astype(BF16)
                    if WTT in (1, 3):
                        val = _upk(_pk(val.T)).T
                dst[i * 64:(i + 1) * 64, :] = _pk(val)
            return
        for r in range(0, 128, 16):
            memo = {}

            def raw(k, n):
                return w[k * 128 + r:k * 128 + r + 16, n * 128:(n + 1) * 128]

            def block(k, n):
                if (k, n) not in memo:
                    memo[k, n] = raw(k, n).astype(F32)
                return memo[k, n]
            for i, tl in enumerate(scheme[0]):
                val = raw(*tl[0]) if len(tl) == 1 else _combo(tl, block).astype(BF16)
                dst[i * 64 + r // 2:i * 64 + r // 2 + 8, :] = _pk(val)

    def pre_body(g, c):
        slot = g & (NSLOT - 1)
        buf = stage_ref.at[slot]
        pltpu.make_async_copy(buf, buf, sem_w.at[slot]).wait()

        @pl.when((g >= 2) & (g <= 4))
        def _():
            bq_copy(g - 2).wait()

        @pl.when(g == 4)
        def _():
            bo_copy.wait()

        @pl.when(g <= 2)
        def _():
            bq_copy(g).start()

        @pl.when(g == 2)
        def _():
            bo_copy.start()

        @pl.when(g + 2 <= NG)
        def _():
            for p in range(4):
                w_copy(p, g + 2).start()

        @pl.when(g == NG - 1)
        def _():
            w0_copy(3).start()
            x_late.start()

        if WPOS == 0:
            wo_store(S55, stage_ref.at[slot, 3], w_ref.at[3 * NG + g - 1])
        for e in range(0 if NOB else 3):
            b_stage2(3 * (g - 5) + e)
        b_stage2_wo(g - 5)
        for e in range(0 if NOB else 3):
            b_stage1(3 * (g - 2) + e)
        b_stage1_wo(g - 4)
        for p in range(3):
            pre_chunk(S55, stage_ref.at[slot, p], w_ref.at[p * NG + g - 1], p * NT + RT + (g - 1) * GT, NNM, DORD[p])
            if WPOS == p + 1:
                wo_store(S55, stage_ref.at[slot, 3], w_ref.at[3 * NG + g - 1])
        return c
    lax.fori_loop(1, NG + 1, pre_body, 0)
    w0_copy(3).wait()

    bscale = float(bdh) ** (-0.5) * LOG2E

    def b_proj(lhs, part):
        return _nn(lhs, _cat([_upk(bw_ref[part * nct + j]) for j in range(nct)], axis=1))

    def b_attn(jobs, q, k, v):
        row = lax.broadcasted_iota(jnp.int32, (seg, 128), 0)
        outs = []
        for i, (l, sidx) in enumerate(jobs):
            r0 = i * seg
            pos = row + sidx * seg
            for j in range(nct):
                kb_ref[l, j, HIST:HIST + seg, :] = k[r0:r0 + seg, j * 128:(j + 1) * 128]
                vb_ref[l, j, HIST:HIST + seg, :] = v[r0:r0 + seg, j * 128:(j + 1) * 128]
            logits = []
            for w in range(B_WIN):
                o = HIST - w * B_DIL
                acc = None
                for j in range(nct):
                    p = q[r0:r0 + seg, j * 128:(j + 1) * 128] * kb_ref[l, j, o:o + seg, :]
                    acc = p if acc is None else acc + p
                acc = acc + pltpu.roll(acc, 64, 1)
                acc = acc + pltpu.roll(acc, 32, 1)
                lg = acc * bscale
                if w > 0:
                    lg = jnp.where(pos >= w * B_DIL, lg, NEG2)
                logits.append(lg)
            m = logits[0]
            for w in range(1, B_WIN):
                m = jnp.maximum(m, logits[w])
            es = [jnp.exp2(lg - m) for lg in logits]
            den = es[0]
            for w in range(1, B_WIN):
                den = den + es[w]
            inv = _recip(den)
            cols = []
            for j in range(nct):
                acc = None
                for w in range(B_WIN):
                    o = HIST - w * B_DIL
                    p = es[w] * vb_ref[l, j, o:o + seg, :]
                    acc = p if acc is None else acc + p
                cols.append(acc * inv)
            outs.append(_cat(cols, axis=1).astype(BF16))
            for j in range(nct):
                kb_ref[l, j, 0:HIST, :] = k[r0 + seg - HIST:r0 + seg, j * 128:(j + 1) * 128]
                vb_ref[l, j, 0:HIST, :] = v[r0 + seg - HIST:r0 + seg, j * 128:(j + 1) * 128]
        return outs

    def b_out(ob, res):
        return res + _nn(ob, _cat([_upk(bw_ref[NB1 + j]) for j in range(nct)], axis=1))

    def o_store(b, val):
        ro = pl.multiple_of((b + 1) * seg, seg)
        o_ref[pl.ds(ro, val.shape[0]), :] = val.astype(o_ref.dtype)

    def out_copy(b):
        ro = pl.multiple_of(b * seg, seg)
        return pltpu.make_async_copy(o_ref.at[pl.ds(ro + seg, seg), :], out_hbm.at[pl.ds(ro, seg), :], sem_o)

    def step(t, hc, full, u=0, i=None):
        t_last = n_seg + LAG - 1
        if full:
            jobs = [(0, t - 1), (1, t - 1 - LAG)]

            def b_in():
                return xb_ref[0:2 * seg, :]
        else:
            lb = (t == t_last).astype(jnp.int32)
            jobs = [(lb, t - 1 - lb * (LAG + 1))]

            def b_in():
                return xb_ref[pl.ds(pl.multiple_of(lb * seg, seg), seg), :]
        split = full and u < UNROLL - 1
        nq = RB + AHS[u] if full else RB
        v0r = _cat([hc[0:n_mem], h_ref[n_mem:M2, :]])
        v1r = _cat([hc[n_mem:M2], h_ref[M2 + n_mem:2 * M2, :]])

        def ktiles(z):
            return [z[:, k * 128:(k + 1) * 128] for k in range(z.shape[1] // 128)]
        if full:
            hl = _Operands(ktiles(_cat([v0r, h_ref[2 * M2:RB, :]])), ktiles(_cat([v1r, h_ref[RB:RB + 16, :]])),
                           ktiles(h_ref[RB + 16:nq, :]) if nq > RB + 16 else None)
        else:
            hl = _Operands(None, None, ktiles(_cat([v0r, v1r, h_ref[2 * M2:RB, :]])))
        mh = 2 * M2 if full else 0

        def tile_dot(p, r):
            src = wr_ref.at[p] if r == 0 else w_ref.at[p * NG + r - 1]
            return lambda a, i: _nn(a, _upk(src[i * 64:(i + 1) * 64, :]))
        scale = float(dh) ** (-0.5) * LOG2E
        if full:
            s_ = t - LAG
            rd = pl.multiple_of(lax.rem(s_ * (seg // 2), RS // 2), seg // 2)
            a_off = i * sum(AHS) + sum(AHS[:u])
            wa = [pl.multiple_of(lax.rem((A0 - R0 + a_off) // 2 + 8 * a, RS // 2), 8)
                  for a in range(AHS[u] // 16)]
        else:
            wx = pl.multiple_of(jnp.where(t < LAG, NPRE // 2 + t * (n_mem // 2), RS // 2), n_mem // 2)
            wo_store(S35, stage0_ref.at[3], wr_ref.at[3])

        RA = R if full else M2 + seg
        CW = R + 2 * M2 if full else R
        ri = lax.broadcasted_iota(jnp.int32, (RA, CW), 0)
        ci = lax.broadcasted_iota(jnp.int32, (RA, CW), 1)
        if not full:
            ri = jnp.where(ri >= M2, ri + seg, ri)

        def table(i, bounds, vals):
            out = vals[-1]
            for b, v in zip(reversed(bounds), reversed(vals[:-1])):
                out = jnp.where(i < b, v, out)
            return out
        qi = ri - table(ri, [16, 48, 56], [0, 8, 48, 40])
        g0 = (ci < 8) | ((ci >= 16) & (ci < 48))
        k2 = ci - table(ci, [8, 24, 32, 48, 56, 80, 88, 96, 104], [-8, 0, 24, 8, 48, 40, 72, 80, 96, 104])
        if full:
            k1 = ci - table(ci, [8, 48], [0, 8, 40])
            row_l2 = ((ri >= 8) & (ri < 16)) | (ri >= 48)
            row_xa = (ri >= 8) & (ri < 16)
            valid = row_xa == (ci >= 80)
            is_a = jnp.where(ci >= 80, ((ci >= 88) & (ci < 104)).astype(jnp.int32),
                             (g0 != row_l2).astype(jnp.int32)) > 0
            ki = jnp.where(row_l2, k2, k1)
            visible = valid & ((qi < n_mem) | (qi >= ki))
            fill = jnp.where(valid, NEG2, -jnp.inf)
        else:
            is_a = jnp.logical_not(g0)
            visible = (qi < n_mem) | (qi >= k2)
            fill = NEG2
        half = dh - 128
        la8 = lax.broadcasted_iota(jnp.int32, (n_mem, 128), 1) < half
        ones = jnp.full((n_mem, 128), 0xFFFFFFFF, U32)
        zero = jnp.zeros((n_mem, 128), U32)
        mask_a = jnp.where(la8, ones, zero)
        mask_b = jnp.where(la8, zero, ones)

        def pk2(a, b):
            return _pk(_cat([a, b]).astype(BF16))

        yt = [[None] * NT for _ in range(3)]
        x1 = [[None] * NT for _ in range(3)]

        def proj(p, r):
            pa, qa = {}, {}
            _fast_mm((S53 if r == 0 else S55)[1], hl, tile_dot(p, r), mh, pa, qa)
            n0 = 0 if r == 0 else RT + (r - 1) * GT
            for n in range(len(pa)):
                y, z, e = _fast_out(pa, qa, n, mh)
                idx = p * NT + n0 + n
                if full:
                    y = _cat([y[0:M2], z[0:M2], y[M2:2 * M2], z[M2:2 * M2]] + ([] if e is None else [e]))
                    for a in range(AHS[u] // 16):
                        rr = RB + 16 * a
                        ring_ref[idx, pl.ds(wa[a], 8), :] = pk2(y[rr:rr + 8], y[rr + 8:rr + 16])
                else:
                    y = e
                    ring_ref[idx, pl.ds(wx, n_mem // 2), :] = pk2(y[0:8], y[8:16])[0:n_mem // 2]
                yt[p][n0 + n] = y
            if full:
                for n in range(len(pa)):
                    x1[p][n0 + n] = ring_ref[p * NT + n0 + n, pl.ds(rd, seg // 2), :]

        def pair(p, g):
            return yt[p][3 * g:3 * g + 3], x1[p][3 * g:3 * g + 3]

        def groups(z, j):
            y = z[0][j]
            return pk2(y[0:8], y[8:16]), pk2(y[16:24], y[24:32]), pk2(y[32:40], y[40:48])

        def q_rows(z, j):
            v0, v1, v2 = groups(z, j)
            return [v0] + ([z[1][j]] if full else []) + [v1, v2]

        def kv_tiles(z):
            yt, x1 = z
            v0, v1, v2 = groups(z, 0)
            t0 = [v0] + ([x1[0]] if full else [v1, v2]) + [v1, v2]
            y = yt[2]
            w0 = pk2(y[8:16], y[0:8])
            w1 = pk2(y[24:32], y[16:24])
            w2 = pk2(y[32:40], y[40:48])
            t2 = [w0, w1, w2] + ([x1[2]] if full else [w1, w2])
            if full:
                t0 += [v0, v1]
                t2 += [w0, w1]
            y = yt[1]

            def ab(z8):
                return jnp.where(la8, z8, 0.0), jnp.where(la8, 0.0, z8)
            xa_a, xa_b = ab(y[8:16])
            e1 = pk2(xa_b, xa_a)
            u2 = pk2(y[32:40], y[40:48])
            mid2 = [e1, pk2(y[24:32], y[16:24]) & mask_b, u2 & mask_b,
                    pk2(y[16:24], y[24:32]) & mask_a, u2 & mask_a]
            mid1 = None
            if full:
                lo, hi = x1[1][0:8], x1[1][8:16]
                mid1 = [pk2(*ab(y[0:8])), lo & mask_a, hi & mask_a, lo & mask_b, hi & mask_b,
                        e1, pk2(*ab(y[16:24]))]
            return t0, mid1, mid2, t2

        def mat(parts):
            return _upk(_cat(parts))

        def scores(q, k):
            k0, km1, km2, k2_ = kv_tiles(k)
            s_a = _nt(mat(q_rows(q, 0)), mat(k0))
            s_b = _nt(mat(q_rows(q, 2)), mat(k2_))
            qm = q_rows(q, 1)
            if full:
                s_m = _cat([_nt(mat(qm[0:2]), mat(km1)), _nt(mat(qm[2:4]), mat(km2 + km1[5:7]))])
            else:
                s_m = _nt(mat(qm), mat(km2))
            s = (jnp.where(is_a, s_a, s_b) + s_m) * scale
            s = jnp.where(visible, s, fill)
            m_a = jnp.max(jnp.where(is_a, s, -jnp.inf), axis=-1, keepdims=True)
            m_b = jnp.max(jnp.where(is_a, -jnp.inf, s), axis=-1, keepdims=True)
            e = jnp.exp2(s - jnp.where(is_a, m_a, m_b))
            d_a = jnp.sum(jnp.where(is_a, e, 0.0), axis=-1, keepdims=True)
            d_b = jnp.sum(jnp.where(is_a, 0.0, e), axis=-1, keepdims=True)
            return e * _recip(jnp.where(is_a, d_a, d_b))

        def pv(p, v):
            v0, vm1, vm2, v2 = kv_tiles(v)
            o_a = _nn(jnp.where(is_a, p, 0.0).astype(BF16), mat(v0))
            o_b = _nn(jnp.where(is_a, 0.0, p).astype(BF16), mat(v2))
            if full:
                o_m = _cat([_nn(p[0:M2 + seg].astype(BF16), mat(vm1)),
                            _nn(p[M2 + seg:R, 0:R].astype(BF16), mat(vm2))])
            else:
                o_m = _nn(p.astype(BF16), mat(vm2))
            return [o_a, o_m, o_b]

        ot = []
        pacc, qacc = {}, {}

        def add_o(r):
            n0 = 0 if r == 0 else RT + (r - 1) * GT
            oo = ot[n0:n0 + (RT if r == 0 else GT)]
            if full:
                ops = _Operands([o[0:32] for o in oo], [_cat([o[48:64], o[32:48]]) for o in oo],
                                [o[64:80] for o in oo])
            else:
                ops = _Operands(None, None, oo)
            _fast_mm((S35 if r == 0 else S55)[1], ops, tile_dot(3, r), mh, pacc, qacc)

        wsched = dict(tuple(int(v) for v in e.split(":")) for e in WSCHED.split(","))
        bqkv = [None] * 3
        probs = []
        x2_new = None

        def do_pv():
            for g in range(len(ot) // 3, len(probs)):
                ot.extend(pv(probs[g], pair(2, g)))

        for r in range(NG + 1):
            npr = len(probs)
            for ch in ORDR:
                if ch in 'qkv':
                    proj('qkv'.index(ch), r)
                elif ch == 'P':
                    for g in range(len(ot) // 3, npr):
                        ot.extend(pv(probs[g], pair(2, g)))
                elif ch == 'S':
                    for g in range(len(probs), (RT + r * GT) // 3):
                        probs.append(scores(pair(0, g), pair(1, g)))
                else:
                    if r == 0:
                        blhs = _ln(b_in()).astype(BF16)
                    if r < 3:
                        bqkv[2 - r] = b_proj(blhs, 2 - r)
                    if r == 3:
                        ob = b_attn(jobs, *bqkv)
                    if r == BOUT_R:
                        res = b_in()
                        if split:
                            x2_new = b_out(ob[0], res[0:seg])
                        elif full:
                            zb = b_out(_cat(ob), res)
                            x2_new = zb[0:seg]
                            o_store(t - 1 - LAG, zb[seg:2 * seg])
                        else:
                            x2_new = b_out(ob[0], res)
                            o_store(lb * (t_last - LAG - 1) - 1, x2_new)
                    if r in wsched:
                        add_o(wsched[r])
        for r in range(len(wsched), TAILPV):
            add_o(r)
        do_pv()
        for r in range(max(TAILPV, len(wsched)), NG + 1):
            add_o(r)
        cols = []
        for n in range(nct):
            y, z, e = _fast_out(pacc, qacc, n, mh)
            cols.append(_cat([y, z[16:32], z[0:16], e]) if full else e)
        acc = _cat(cols, axis=1)
        if split:
            o_store(t - 1 - LAG, b_out(ob[1], res[seg:2 * seg]))

        y2 = x2_ref[...] + _cat([acc[n_mem:M2], acc[RA - seg + n_mem:RA]])
        mem2 = acc[RA - seg:RA - seg + n_mem]
        if full:
            x_cur = x_ref[pl.ds(pl.multiple_of(t * seg, seg), seg), :].astype(F32)
            xb_ref[0:seg, :] = x_cur + acc[M2:M2 + seg]
            xb_ref[seg:2 * seg, :] = y2
            m1n = acc[0:n_mem]
            m2n = mem2
            ahn = AHS[(u + 1) % UNROLL]
            an = pl.multiple_of(jnp.minimum(A0 + a_off + AHS[u], S - ahn), 16)
            h_ref[RB:RB + ahn, :] = _ln(x_ref[pl.ds(an, ahn), :].astype(F32))
            nxt = x2_new
        else:
            xb_ref[pl.ds(pl.multiple_of(jnp.where(t < LAG, 0, (t - n_seg + 2) * seg), seg), seg), :] = y2
            m1n = jnp.where(t < LAG - 1, h_ref[RB + AHS[0]:RB + AHS[0] + n_mem, :], mem2)
            m2n = jnp.where(t == LAG - 1, mem0_ref[...].astype(F32), mem2)
            nxt = jnp.where(t < LAG - 1, x_ref[seg:2 * seg, :].astype(F32), x2_new)
        x2_ref[...] = nxt
        sl = _ln(nxt)
        h_ref[n_mem:M2, :] = sl[0:n_mem]
        h_ref[M2 + n_mem:RB, :] = sl[n_mem:seg]
        return _cat([m1n, m2n])

    def single_body(t, c):
        @pl.when(t >= n_seg)
        def _():
            out_copy(t - (LAG + 3)).start()
        return step(t, c, False)

    def full_body(i, c):
        t = LAG + UNROLL * i
        for u in range(UNROLL):
            @pl.when(t - u >= LAG + 2)
            def _():
                out_copy(t - u - (LAG + 2)).start()
        for u in range(UNROLL):
            c = step(t + u, c, True, u, i)
        return c

    def phase(ph, c):
        t0 = ph * n_seg
        c = lax.fori_loop(t0, t0 + LAG, single_body, c)

        @pl.when(ph == 0)
        def _():
            x_late.wait()
        return lax.fori_loop(0, jnp.where(ph == 0, (n_seg - LAG) // UNROLL, 0), full_body, c)
    if not SKIPM:
      lax.fori_loop(0, 2, phase, _cat([h_ref[0:n_mem, :], h_ref[M2:M2 + n_mem, :]]))

    if SKIPM:
        def keep(i, c):
            z = (w_ref[i, pl.ds(pl.multiple_of(i * 8, 8), 8), :] + ring_ref[i, pl.ds(pl.multiple_of(i * 8, 8), 8), :]
                 + wr_ref[i & 3, pl.ds(pl.multiple_of(i * 8, 8), 8), :])
            xb_ref[2 * seg:2 * seg + 8, 0:128] = pltpu.bitcast(z, F32) + h_ref[pl.ds(pl.multiple_of((i & 7) * 8, 8), 8), 0:128] + x2_ref[0:8, 0:128]
            return c
        lax.fori_loop(0, 20, keep, 0)
    out_copy(n_seg - 3).start()
    res = xb_ref[2 * seg:4 * seg, :]
    blhs = _ln(res).astype(BF16)
    ob = b_attn([(1, n_seg - 2), (1, n_seg - 1)], *[b_proj(blhs, part) for part in range(3)])
    o_store(n_seg - 2, b_out(_cat(ob), res))
    out_copy(n_seg - 2).start()
    out_copy(n_seg - 1).start()
    pltpu.make_async_copy(o_ref.at[pl.ds(seg, S), :], out_hbm, sem_o).wait()


@functools.partial(jax.jit, static_argnames=("seg",))
def _run(A_x, A_mem0, A_Wq, A_Wk, A_Wv, A_Wo, B_wqkv, B_wo, *, seg):
    _, S, dm = A_x.shape
    n_heads, dh = A_Wq.shape[1], A_Wq.shape[2]
    n_mem = A_mem0.shape[1]
    n_seg = S // seg
    hd = n_heads * dh
    nct = dm // 128
    ng = (hd // 128 - RT) // GT
    assert (seg, n_seg, n_mem, dh, dm % 128, n_heads, LAG, UNROLL) == (32, 64, 8, 192, 0, 32, 2, 2)

    x = A_x.reshape(S, dm)
    mem0 = A_mem0.reshape(n_mem, dm)
    wq = jnp.transpose(A_Wq, (1, 2, 0)).reshape(hd, dm)
    wk = jnp.transpose(A_Wk, (1, 2, 0)).reshape(hd, dm)
    wv = jnp.transpose(A_Wv, (1, 2, 0)).reshape(hd, dm)
    wo = A_Wo.reshape(hd, dm)
    _, _, _, _, rs, xc = _plan(seg, n_seg)

    kern = functools.partial(_kernel, seg=seg, n_seg=n_seg, n_mem=n_mem,
                             n_heads=n_heads, dh=dh, dm=dm)
    hbm = pl.BlockSpec(memory_space=pltpu.HBM)

    out = pl.pallas_call(
        kern,
        in_specs=[hbm] * 8,
        out_specs=hbm,
        out_shape=jax.ShapeDtypeStruct((S, dm), A_x.dtype),
        scratch_shapes=[
            pltpu.VMEM((S, dm), BF16),
            pltpu.VMEM((n_mem, dm), BF16),
            pltpu.VMEM((NSLOT, 4, GT * 128, dm), BF16),
            pltpu.VMEM((4, RT * 128, dm), BF16),
            pltpu.VMEM((4, len(S53[0]) * 64, 128), U32),
            pltpu.VMEM((4 * ng, len(S55[0]) * 64, 128), U32),
            pltpu.VMEM((dm, 4 * dm + 128), BF16),
            pltpu.VMEM((nct, 5 * dm + 32, 128), F32),
            pltpu.VMEM((4 * nct + 1, dm // 2, 128), U32),
            pltpu.VMEM((len(KEYS), NXC * xc // 4, 128), U32),
            pltpu.VMEM((3 * hd // 128, rs // 2 + 8, 128), U32),
            pltpu.VMEM((3 * n_mem + seg + AHS[0], dm), F32),
            pltpu.VMEM((4 * seg, dm), F32),
            pltpu.VMEM((seg, dm), F32),
            pltpu.VMEM((2, nct, HIST + seg, 128), F32),
            pltpu.VMEM((2, nct, HIST + seg, 128), F32),
            pltpu.VMEM((S + seg, dm), A_x.dtype),
            pltpu.SemaphoreType.DMA((NSLOT,)),
            pltpu.SemaphoreType.DMA((8 + NXC,)),
            pltpu.SemaphoreType.DMA((4,)),
            pltpu.SemaphoreType.DMA(()),
        ],
        compiler_params=pltpu.CompilerParams(
            vmem_limit_bytes=120 * 1024 * 1024,
            disable_bounds_checks=True,
        ),
    )(x, mem0, wq, wk, wv, wo, B_wqkv, B_wo)
    return out.reshape(1, S, dm)


def pallas_interleave_layers__memory_aug_recurrent_mem_tr__sliding_local_dilated__prompt_kernel(
    A_x: jax.Array,
    A_mem0: jax.Array,
    A_Wq: jax.Array,
    A_Wk: jax.Array,
    A_Wv: jax.Array,
    A_Wo: jax.Array,
    A_seg_len,
    B_x: jax.Array,
    B_wqkv: jax.Array,
    B_wo: jax.Array,
):
    del B_x
    seg = A_seg_len if isinstance(A_seg_len, int) else 32
    return _run(A_x, A_mem0, A_Wq, A_Wk, A_Wv, A_Wo, B_wqkv, B_wo, seg=seg)
```

```python
import functools

import jax
import jax.numpy as jnp
from jax import lax
import jax.experimental.pallas as pl
import jax.experimental.pallas.tpu as pltpu

F32 = jnp.float32
BF16 = jnp.bfloat16
U32 = jnp.uint32
NEG = -1000000000.0
LN_EPS = 1e-05
LOG2E = 1.4426950408889634
NEG2 = NEG * LOG2E

B_HEADS = 32
B_WIN = 8
B_DIL = 2
HIST = 16
AHS = (32, 16)
LAG = 2
NSLOT = 4
NNM = '000'
NNF = '000'
WSCHED = '3:0,4:1,5:2,7:3,8:4,9:5'
BOUT_R = int(6)
ORDR = 'vkqFPS'
TAILPV = int(7)
PERT = int(1)
WPOS = int(0)
SKIPM = int(0)
MDQ = 'l'
MDW = 'l'
CW128 = int(0)
OSC = int(1)
PSC = int(0)
LATE = int(1)
KVS = int(1)
BT = int(0)
NOB = int(0)
WTT = int(1)
DORD = 'sss'
RCH = [int(v) for v in '80,80,80'.split(',')]
NXC = 3
UNROLL = 2


def _ln(x):
    m = jnp.mean(x, axis=-1, keepdims=True)
    c = x - m
    v = jnp.mean(c * c, axis=-1, keepdims=True)
    return c * lax.rsqrt(v + LN_EPS)


def _recip(d):
    return pl.reciprocal(d, approx=True)


def _nt(a, b):
    return lax.dot_general(a, b, (((1,), (1,)), ((), ())), preferred_element_type=F32)


def _nn(a, b):
    return jnp.dot(a, b, preferred_element_type=F32)


def _cat(xs, axis=0):
    return xs[0] if len(xs) == 1 else jnp.concatenate(xs, axis=axis)


def _pk(z):
    return pltpu.bitcast(z, U32)


def _upk(z):
    return pltpu.bitcast(z, BF16)


LAM = (-1.5, -0.5, 0.0, 0.5, 1.5)


def _scheme(stars):
    tiles, prog = [], []
    for star in stars:
        if len(star) == 1:
            prog.append(("single", star[0], None, len(tiles)))
            tiles.append([star[0][:2]])
            continue
        left = [len(star) - 1] * len(star)
        for j in range(1, len(star)):
            for i in range(j):
                x, y = star[i], star[j]
                prog.append(("pair", x, y, len(tiles)))
                tiles += [[(x[0], y[1])], [(y[0], x[1])], [(x[0], y[1]), (y[0], x[1])]]
                for e in (i, j):
                    left[e] -= 1
                    if left[e] == 0:
                        z = star[e]
                        prog.append(("diag", z, None, len(tiles)))
                        tiles += [[z[:2]] + [(o[0], z[1]) for o in star if o is not z],
                                  [z[:2]] + [(z[0], o[1]) for o in star if o is not z]]
    return tiles, prog


S55 = _scheme([[(i, i, LAM[i]) for i in range(5)]])
S53 = _scheme([[(0, 0, LAM[0]), (2, 1, LAM[2]), (4, 2, LAM[4])], [(1, 0, LAM[1]), (3, 2, LAM[3])],
               [(1, 1, LAM[1])], [(3, 1, LAM[3])]])
S35 = _scheme([[(0, 0, LAM[0]), (1, 2, LAM[2]), (2, 4, LAM[4])], [(0, 1, LAM[1]), (2, 3, LAM[3])],
               [(1, 1, LAM[1])], [(1, 3, LAM[3])]])


def _reorder(prog, mode):
    pairs = [e for e in prog if e[0] != "diag"]
    diags = [e for e in prog if e[0] == "diag"]
    if mode == "l":
        return prog
    out = []
    if mode == "f":
        for e in pairs:
            for z in (e[1], e[2]):
                for dg in diags:
                    if dg[1] == z and dg not in out:
                        out.append(dg)
            out.append(e)
        return out
    step = len(pairs) / len(diags)
    k = 0
    for i, e in enumerate(pairs):
        out.append(e)
        while k < len(diags) and (k + 0.5) * step <= i + 1:
            out.append(diags[k])
            k += 1
    return out + diags[k:]


def _op_keys(prog):
    keys = []
    for kind, x, y, _ in prog:
        if kind == "pair":
            new = [(nm, x[0], x[2], y[0], y[2]) for nm in ("l1", "l2", "A")]
        else:
            new = [("a", x[0], x[2]), ("b", x[0])]
        keys += [k for k in new if k not in keys]
    return keys


def _scaled(c, u):
    return u if c == 1.0 else c * u


class _Operands:
    def __init__(self, T, U, E):
        self.T, self.U, self.E, self.memo = T, U, E, {}

    def _get(self, key, fn):
        if key not in self.memo:
            self.memo[key] = fn()
        return self.memo[key]

    def paired(self, key):
        T, U = self.T, self.U
        if key[0] == "b":
            return U[key[1]]
        if key[0] == "a":
            k, lam = key[1:]
            if lam == 0.0:
                return T[k]
            return self._get(("f",) + key, lambda: T[k] - _scaled(lam, U[k]) if lam > 0
                             else T[k] + _scaled(-lam, U[k]))
        kx, lx, ky, ly = key[1:]
        A = self._get(("f", "A") + key[1:],
                      lambda: self.paired(("a", kx, lx)) + self.paired(("a", ky, ly)))
        if key[0] == "A":
            return A
        return A - _scaled(ly - lx, U[kx]) if key[0] == "l1" else A + _scaled(ly - lx, U[ky])

    def extra(self, key):
        if key[0] == "a":
            return self.E[key[1]]
        return self._get(("e", key[1], key[3]), lambda: self.E[key[1]] + self.E[key[3]])

    def __call__(self, key):
        if self.T is None:
            ek = ("a", key[1]) if key[0] in ("a", "s") else ("l", key[1], 0, key[3])
            return self._get(ek, lambda: self.extra(ek).astype(BF16))

        def build():
            ak = ("a",) + key[1:] if key[0] == "s" else key
            parts = [self.paired(ak)]
            if self.E is not None and ak[0] in ("a", "l1", "l2"):
                parts.append(self.extra(ak))
            if key[0] == "s":
                parts.append(self.U[key[1]])
            return _cat(parts).astype(BF16)
        return self._get(key, build)


def _fast_mm(prog, op, dot, m, p, q):
    def add(d, key, val):
        d[key] = val if key not in d else d[key] + val

    for kind, x, y, i in prog:
        if kind == "pair":
            kk = (x[0], x[2], y[0], y[2])
            p1, p2 = dot(op(("l1",) + kk), i), dot(op(("l2",) + kk), i + 1)
            if m:
                r = _scaled(1.0 / (y[2] - x[2]), p2[0:m] - p1[0:m] + dot(op(("A",) + kk), i + 2))
                add(q, (x[1], x[2]), r)
                add(q, (y[1], y[2]), r)
            add(p, y[1], p1)
            add(p, x[1], p2)
        elif kind == "diag":
            add(p, x[1], dot(op(("a", x[0], x[2])), i))
            if m:
                add(q, (x[1], x[2]), dot(op(("b", x[0])), i + 1))
        else:
            r = dot(op(("s", x[0], x[2])), i)
            add(p, x[1], r[0:r.shape[0] - m])
            if m:
                add(q, (x[1], x[2]), r[r.shape[0] - m:])


def _fast_out(p, q, n, m):
    if not m:
        return None, None, p[n]
    y, z = p[n][0:m], None
    for (nn, lam), v in q.items():
        if nn == n:
            z = v if z is None else z + v
            if lam != 0.0:
                y = y + _scaled(lam, v) if lam > 0 else y - _scaled(-lam, v)
    return y, z, (p[n][m:] if p[n].shape[0] > m else None)


def _combo(tile, block):
    out = block(*tile[0])
    for kn in tile[1:]:
        out = out - block(*kn)
    return out


GT = 5
RT = 3
KEYS_R = _op_keys(S53[1])
KEYS = KEYS_R + [k for k in _op_keys(S55[1]) if k not in KEYS_R]


def _plan(seg, n_seg):
    S = seg * n_seg
    R0 = LAG * seg
    A0 = S - (n_seg - LAG) // UNROLL * sum(AHS)
    NPRE = A0 - R0 - LAG * 8
    RS = -(-(A0 - R0 + AHS[0]) // seg) * seg
    XC = NPRE // NXC
    assert XC % 32 == 0 and XC * NXC == NPRE
    return S, R0, A0, NPRE, RS, XC


def _kernel(x_hbm, mem0_hbm, wq_hbm, wk_hbm, wv_hbm, wo_hbm, bqkv_hbm, bwo_hbm,
            out_hbm,
            x_ref, mem0_ref, stage_ref, stage0_ref, wr_ref, w_ref, bst_ref, btmp_ref, bw_ref,
            xln_ref, ring_ref, h_ref, xb_ref, x2_ref, kb_ref, vb_ref, o_ref, bias_ref, kv_ref, os_ref, ps_ref,
            sem_w, sem_m, sem_b, sem_o,
            *, seg, n_seg, n_mem, n_heads, dh, dm):
    S, R0, A0, NPRE, RS, XC = _plan(seg, n_seg)
    M2 = 2 * n_mem
    R = M2 + 2 * seg
    RB = M2 + seg
    PW = 2 * dh
    G = n_heads // 2
    nct = dm // 128
    bdh = dm // B_HEADS
    NT = n_heads * dh // 128
    NG = (NT - RT) // GT
    w_hbm = (wq_hbm, wk_hbm, wv_hbm, wo_hbm)

    def w_copy(p, g):
        slot = g & (NSLOT - 1)
        return pltpu.make_async_copy(w_hbm[p].at[pl.ds((RT + (g - 1) * GT) * 128, GT * 128), :],
                                     stage_ref.at[slot, p], sem_w.at[slot])

    def w0_copy(p):
        return pltpu.make_async_copy(w_hbm[p].at[pl.ds(0, RT * 128), :], stage0_ref.at[p], sem_m.at[4 + p])

    NB1 = 3 * nct
    WO0 = 3 * dm
    DUM = 4 * dm
    XF = A0 + AHS[0]
    XH = XC // 2

    def rows_copy(r0, n, sem):
        return pltpu.make_async_copy(x_hbm.at[pl.ds(r0, n), :], x_ref.at[pl.ds(r0, n), :], sem)

    def x_copy(i):
        return rows_copy(pl.multiple_of(R0 + i * XC, 16), XC, sem_m.at[8 + i])

    small = [rows_copy(0, R0, sem_m.at[1]), rows_copy(R0 + NPRE, XF - R0 - NPRE, sem_m.at[2]),
             pltpu.make_async_copy(mem0_hbm, mem0_ref, sem_m.at[3])]
    x_late = rows_copy(XF, S - XF, sem_m.at[0])

    def bq_copy(part):
        c0 = pl.multiple_of(part * dm, 128)
        return pltpu.make_async_copy(bqkv_hbm.at[:, pl.ds(c0, dm)], bst_ref.at[:, pl.ds(c0, dm)], sem_b.at[part])

    bo_copy = pltpu.make_async_copy(bwo_hbm, bst_ref.at[:, pl.ds(3 * dm, dm)], sem_b.at[3])

    def bst_tile(c):
        return bst_ref[:, pl.ds(pl.multiple_of(c * 128, 128), 128)]

    def bias_tables(full):
        RA = R if full else M2 + seg
        CW = 128
        ri = lax.broadcasted_iota(jnp.int32, (RA, CW), 0)
        ci = lax.broadcasted_iota(jnp.int32, (RA, CW), 1)
        if not full:
            ri = jnp.where(ri >= M2, ri + seg, ri)

        def table(i, bounds, vals):
            out = vals[-1]
            for b, v in zip(reversed(bounds), reversed(vals[:-1])):
                out = jnp.where(i < b, v, out)
            return out
        qi = ri - table(ri, [16, 48, 56], [0, 8, 48, 40])
        g0 = (ci < 8) | ((ci >= 16) & (ci < 48))
        k2 = ci - table(ci, [8, 24, 32, 48, 56, 80, 88, 96, 104], [-8, 0, 24, 8, 48, 40, 72, 80, 96, 104])
        if full:
            k1 = ci - table(ci, [8, 48], [0, 8, 40])
            row_l2 = ((ri >= 8) & (ri < 16)) | (ri >= 48)
            row_xa = (ri >= 8) & (ri < 16)
            valid = (row_xa == (ci >= 80)) & (ci < 112)
            is_a = jnp.where(ci >= 80, ((ci >= 88) & (ci < 104)).astype(jnp.int32),
                             (g0 != row_l2).astype(jnp.int32)) > 0
            ki = jnp.where(row_l2, k2, k1)
            visible = valid & ((qi < n_mem) | (qi >= ki))
            fill = jnp.where(valid, NEG2, -jnp.inf)
        else:
            is_a = jnp.logical_not(g0)
            visible = (qi < n_mem) | (qi >= k2)
            fill = NEG2
        for e, mine in enumerate((is_a, jnp.logical_not(is_a))):
            bias_ref[(0 if full else 2) + e, 0:RA, :] = jnp.where(
                mine, jnp.where(visible, 0.0, fill), -jnp.inf)

    for i in range(NXC):
        x_copy(i).start()
    for cp in small:
        cp.start()

    def zero_body(j, c):
        btmp_ref[j, DUM:, :] = jnp.zeros((btmp_ref.shape[1] - DUM, 128), F32)
        return c
    lax.fori_loop(0, nct, zero_body, 0)

    for p in range(3):
        w0_copy(p).start()
    for p in range(4):
        w_copy(p, 1).start()
    xb_ref[0:2 * seg, :] = jnp.zeros((2 * seg, dm), F32)
    kb_ref[...] = jnp.zeros(kb_ref.shape, F32)
    vb_ref[...] = jnp.zeros(vb_ref.shape, F32)
    bst_ref[:, 4 * dm:] = jnp.zeros((dm, 128), BF16)
    bias_tables(True)
    bias_tables(False)

    def ln_ops(i, lo, hi):
        y = _ln(x_ref[pl.ds(pl.multiple_of(R0 + i * XC, 16), XC), :].astype(F32))
        ops = _Operands([y[0:XH, k * 128:(k + 1) * 128] for k in range(nct)],
                        [y[XH:XC, k * 128:(k + 1) * 128] for k in range(nct)], None)
        r0 = pl.multiple_of(i * (XH // 2), 8)
        for j in range(lo, hi):
            xln_ref[j, pl.ds(r0, XH // 2), :] = _pk(ops(KEYS[j]))

    def ln_body(i, c):
        x_copy(i).wait()
        ln_ops(i, 0, len(KEYS_R))
        return c
    lax.fori_loop(0, NXC, ln_body, 0)
    for cp in small:
        cp.wait()
    bq_copy(0).start()

    def pre_chunk(scheme, w, dst, n0, nn, dord='l'):
        tiles, prog = scheme
        prog = _reorder(prog, dord)
        strips = []
        for r in range(0, 0 if PERT else 128, 16):
            memo = {}

            def block(k, n):
                if (k, n) not in memo:
                    memo[k, n] = w[n * 128 + r:n * 128 + r + 16, k * 128:(k + 1) * 128].astype(F32)
                return memo[k, n]
            strips.append([_combo(tl, block) if len(tl) > 1 else None for tl in tiles])
        tb = []
        for i, tl in enumerate(tiles):
            if len(tl) == 1:
                k, n = tl[0]
                tb.append(w[n * 128:(n + 1) * 128, k * 128:(k + 1) * 128])
            elif PERT:
                tb.append(_combo(tl, lambda k, n: w[n * 128:(n + 1) * 128, k * 128:(k + 1) * 128].astype(F32)
                                 ).astype(BF16))
            else:
                tb.append(_cat([st[i] for st in strips]).astype(BF16))
            if PERT:
                dst[i * 64:(i + 1) * 64, :] = _pk(tb[i].T)
        for i, x in enumerate(tb):
            if not PERT:
                dst[i * 64:(i + 1) * 64, :] = _pk(x.T)

        for c in range(NXC):
            def op(key):
                def ld(kk):
                    return _upk(xln_ref[KEYS.index(kk), c * (XH // 2):(c + 1) * (XH // 2), :])
                if key[0] == "s":
                    return _cat([ld(("a",) + key[1:]), ld(("b", key[1]))])
                return ld(key)
            if nn[c] == '1':
                dot = lambda a, i: _nn(a, _upk(dst[i * 64:(i + 1) * 64, :]))
            else:
                dot = lambda a, i: _nt(a, tb[i])
            p, q = {}, {}
            _fast_mm(prog, op, dot, XH, p, q)
            for n in range(len(p)):
                y, z, _ = _fast_out(p, q, n, XH)
                ring_ref[n0 + n, c * XH:c * XH + XH // 2, :] = _pk(y.astype(BF16))
                ring_ref[n0 + n, c * XH + XH // 2:(c + 1) * XH, :] = _pk(z.astype(BF16))

    def init_rows():
        x0 = x_ref[0:seg, :].astype(F32)
        sl = _ln(x0)
        xt = _ln(x_ref[R0 + NPRE:XF, :].astype(F32))
        h_ref[0:n_mem, :] = xt[0:n_mem]
        h_ref[n_mem:M2, :] = sl[0:n_mem]
        h_ref[M2:M2 + n_mem, :] = mem0_ref[...].astype(F32)
        h_ref[M2 + n_mem:RB, :] = sl[n_mem:seg]
        h_ref[RB:RB + AHS[0], :] = xt[M2:M2 + AHS[0]]
        h_ref[RB + AHS[0]:RB + AHS[0] + n_mem, :] = xt[n_mem:M2]
        x2_ref[...] = x0

    def first_body(p, c):
        buf = stage0_ref.at[p]
        pltpu.make_async_copy(buf, buf, sem_m.at[4 + p]).wait()

        @pl.when(p == 0)
        def _():
            for pp in range(4):
                w_copy(pp, 2).start()
        init_rows()
        pre_chunk(S53, buf, wr_ref.at[p], p * NT, NNF)
        ln_ops(p, len(KEYS_R), len(KEYS))
        return c
    lax.fori_loop(0, 3, first_body, 0)

    dpt = 128 // B_HEADS

    def b_stage1(u):
        ok = (u >= 0) & (u < NB1)
        tr = bst_tile(jnp.where(ok, u, NB1 + nct)).T.astype(F32) if BT & 1 else bst_tile(jnp.where(ok, u, NB1 + nct)).astype(F32).T
        r0 = pl.multiple_of(jnp.where(ok, u * 128, DUM), 128)
        for j in range(nct):
            btmp_ref[j, pl.ds(r0, 128), :] = tr[:, j * 128:(j + 1) * 128]

    def b_stage1_wo(u):
        ok = (u >= 0) & (u < nct)
        r0 = pl.multiple_of(jnp.where(ok, WO0, DUM), 128)
        btmp_ref[jnp.where(ok, u, 0), pl.ds(r0, dm), :] = bst_tile(
            jnp.where(ok, NB1 + u, NB1 + nct)).astype(F32)

    def b_stage2(u):
        ok = (u >= 0) & (u < NB1)
        part = (u >= nct).astype(jnp.int32) + (u >= 2 * nct).astype(jnp.int32)
        r0 = jnp.where(ok, part * dm + (u - part * nct) * dpt, DUM)
        rows = _cat([_cat([btmp_ref[j, pl.ds(r0 + dd, B_HEADS, stride=bdh), :]
                           for j in range(nct)], axis=1) for dd in range(dpt)])
        bw_ref[jnp.where(ok, u, NB1 + nct)] = _pk(rows.astype(BF16).T if BT & 2 else rows.T.astype(BF16))

    def b_stage2_wo(u):
        ok = (u >= 0) & (u < nct)
        r0 = jnp.where(ok, WO0, DUM)
        jj = jnp.where(ok, u, 0)
        bw_ref[jnp.where(ok, NB1 + u, NB1 + nct)] = _pk(
            _cat([btmp_ref[jj, pl.ds(r0 + d, B_HEADS, stride=bdh), :] for d in range(bdh)]).astype(BF16))

    def wo_store(scheme, w, dst):
        if WTT and scheme is S55:
            rawt = lambda k, n: w[k * 128:(k + 1) * 128, n * 128:(n + 1) * 128]
            for i, tl in enumerate(scheme[0]):
                if len(tl) == 1:
                    val = rawt(*tl[0])
                    if WTT == 3:
                        val = _upk(_pk(val.T)).T
                else:
                    val = _combo(tl, lambda k, n: rawt(k, n).astype(F32)).astype(BF16)
                    if WTT in (1, 3):
                        val = _upk(_pk(val.T)).T
                dst[i * 64:(i + 1) * 64, :] = _pk(val)
            return
        for r in range(0, 128, 16):
            memo = {}

            def raw(k, n):
                return w[k * 128 + r:k * 128 + r + 16, n * 128:(n + 1) * 128]

            def block(k, n):
                if (k, n) not in memo:
                    memo[k, n] = raw(k, n).astype(F32)
                return memo[k, n]
            for i, tl in enumerate(scheme[0]):
                val = raw(*tl[0]) if len(tl) == 1 else _combo(tl, block).astype(BF16)
                dst[i * 64 + r // 2:i * 64 + r // 2 + 8, :] = _pk(val)

    def pre_body(g, c):
        slot = g & (NSLOT - 1)
        buf = stage_ref.at[slot]
        pltpu.make_async_copy(buf, buf, sem_w.at[slot]).wait()

        @pl.when((g >= 2) & (g <= 4))
        def _():
            bq_copy(g - 2).wait()

        @pl.when(g == 4)
        def _():
            bo_copy.wait()

        @pl.when(g <= 2)
        def _():
            bq_copy(g).start()

        @pl.when(g == 2)
        def _():
            bo_copy.start()

        @pl.when(g + 2 <= NG)
        def _():
            for p in range(4):
                w_copy(p, g + 2).start()

        @pl.when(g == NG - 1)
        def _():
            w0_copy(3).start()
            x_late.start()

        if WPOS == 0:
            wo_store(S55, stage_ref.at[slot, 3], w_ref.at[3 * NG + g - 1])
        for e in range(0 if NOB else 3):
            b_stage2(3 * (g - 5) + e)
        b_stage2_wo(g - 5)
        for e in range(0 if NOB else 3):
            b_stage1(3 * (g - 2) + e)
        b_stage1_wo(g - 4)
        for p in range(3):
            pre_chunk(S55, stage_ref.at[slot, p], w_ref.at[p * NG + g - 1], p * NT + RT + (g - 1) * GT, NNM, DORD[p])
            if WPOS == p + 1:
                wo_store(S55, stage_ref.at[slot, 3], w_ref.at[3 * NG + g - 1])
        return c
    lax.fori_loop(1, NG + 1, pre_body, 0)
    w0_copy(3).wait()

    bscale = float(bdh) ** (-0.5) * LOG2E

    def b_proj(lhs, part):
        return _nn(lhs, _cat([_upk(bw_ref[part * nct + j]) for j in range(nct)], axis=1))

    def b_attn(jobs, q, k, v):
        row = lax.broadcasted_iota(jnp.int32, (seg, 128), 0)
        outs = []
        for i, (l, sidx) in enumerate(jobs):
            r0 = i * seg
            pos = row + sidx * seg
            for j in range(nct):
                kb_ref[l, j, HIST:HIST + seg, :] = k[r0:r0 + seg, j * 128:(j + 1) * 128]
                vb_ref[l, j, HIST:HIST + seg, :] = v[r0:r0 + seg, j * 128:(j + 1) * 128]
            logits = []
            for w in range(B_WIN):
                o = HIST - w * B_DIL
                acc = None
                for j in range(nct):
                    p = q[r0:r0 + seg, j * 128:(j + 1) * 128] * kb_ref[l, j, o:o + seg, :]
                    acc = p if acc is None else acc + p
                acc = acc + pltpu.roll(acc, 64, 1)
                acc = acc + pltpu.roll(acc, 32, 1)
                lg = acc * bscale
                if w > 0:
                    lg = jnp.where(pos >= w * B_DIL, lg, NEG2)
                logits.append(lg)
            m = logits[0]
            for w in range(1, B_WIN):
                m = jnp.maximum(m, logits[w])
            es = [jnp.exp2(lg - m) for lg in logits]
            den = es[0]
            for w in range(1, B_WIN):
                den = den + es[w]
            inv = _recip(den)
            cols = []
            for j in range(nct):
                acc = None
                for w in range(B_WIN):
                    o = HIST - w * B_DIL
                    p = es[w] * vb_ref[l, j, o:o + seg, :]
                    acc = p if acc is None else acc + p
                cols.append(acc * inv)
            outs.append(_cat(cols, axis=1).astype(BF16))
            for j in range(nct):
                kb_ref[l, j, 0:HIST, :] = k[r0 + seg - HIST:r0 + seg, j * 128:(j + 1) * 128]
                vb_ref[l, j, 0:HIST, :] = v[r0 + seg - HIST:r0 + seg, j * 128:(j + 1) * 128]
        return outs

    def b_out(ob, res):
        return res + _nn(ob, _cat([_upk(bw_ref[NB1 + j]) for j in range(nct)], axis=1))

    def o_store(b, val):
        ro = pl.multiple_of((b + 1) * seg, seg)
        o_ref[pl.ds(ro, val.shape[0]), :] = val.astype(o_ref.dtype)

    def out_copy(b):
        ro = pl.multiple_of(b * seg, seg)
        return pltpu.make_async_copy(o_ref.at[pl.ds(ro + seg, seg), :], out_hbm.at[pl.ds(ro, seg), :], sem_o)

    def step(t, hc, full, u=0, i=None):
        t_last = n_seg + LAG - 1
        if full:
            jobs = [(0, t - 1), (1, t - 1 - LAG)]

            def b_in():
                return xb_ref[0:2 * seg, :]
        else:
            lb = (t == t_last).astype(jnp.int32)
            jobs = [(lb, t - 1 - lb * (LAG + 1))]

            def b_in():
                return xb_ref[pl.ds(pl.multiple_of(lb * seg, seg), seg), :]
        split = full and u < UNROLL - 1
        nq = RB + AHS[u] if full else RB
        v0r = _cat([hc[0:n_mem], h_ref[n_mem:M2, :]])
        v1r = _cat([hc[n_mem:M2], h_ref[M2 + n_mem:2 * M2, :]])

        def ktiles(z):
            return [z[:, k * 128:(k + 1) * 128] for k in range(z.shape[1] // 128)]
        if full:
            hl = _Operands(ktiles(_cat([v0r, h_ref[2 * M2:RB, :]])), ktiles(_cat([v1r, h_ref[RB:RB + 16, :]])),
                           ktiles(h_ref[RB + 16:nq, :]) if nq > RB + 16 else None)
        else:
            hl = _Operands(None, None, ktiles(_cat([v0r, v1r, h_ref[2 * M2:RB, :]])))
        mh = 2 * M2 if full else 0

        def tile_dot(p, r):
            src = wr_ref.at[p] if r == 0 else w_ref.at[p * NG + r - 1]
            return lambda a, i: _nn(a, _upk(src[i * 64:(i + 1) * 64, :]))
        scale = float(dh) ** (-0.5) * LOG2E
        if full:
            s_ = t - LAG
            rd = pl.multiple_of(lax.rem(s_ * (seg // 2), RS // 2), seg // 2)
            a_off = i * sum(AHS) + sum(AHS[:u])
            wa = [pl.multiple_of(lax.rem((A0 - R0 + a_off) // 2 + 8 * a, RS // 2), 8)
                  for a in range(AHS[u] // 16)]
        else:
            wx = pl.multiple_of(jnp.where(t < LAG, NPRE // 2 + t * (n_mem // 2), RS // 2), n_mem // 2)
            wo_store(S35, stage0_ref.at[3], wr_ref.at[3])

        RA = R if full else M2 + seg
        CW = (128 if CW128 else R + 2 * M2) if full else R
        bidx = 0 if full else 2
        half = dh - 128
        la8 = lax.broadcasted_iota(jnp.int32, (n_mem, 128), 1) < half
        ones = jnp.full((n_mem, 128), 0xFFFFFFFF, U32)
        zero = jnp.zeros((n_mem, 128), U32)
        mask_a = jnp.where(la8, ones, zero)
        mask_b = jnp.where(la8, zero, ones)

        def pk2(a, b):
            return _pk(_cat([a, b]).astype(BF16))

        yt = [[None] * NT for _ in range(3)]
        x1 = [[None] * NT for _ in range(3)]

        def proj(p, r):
            pa, qa = {}, {}
            _fast_mm(_reorder((S53 if r == 0 else S55)[1], MDQ), hl, tile_dot(p, r), mh, pa, qa)
            n0 = 0 if r == 0 else RT + (r - 1) * GT
            for n in range(len(pa)):
                y, z, e = _fast_out(pa, qa, n, mh)
                idx = p * NT + n0 + n
                if full:
                    y = _cat([y[0:M2], z[0:M2], y[M2:2 * M2], z[M2:2 * M2]] + ([] if e is None else [e]))
                    for a in range(AHS[u] // 16):
                        rr = RB + 16 * a
                        ring_ref[idx, pl.ds(wa[a], 8), :] = pk2(y[rr:rr + 8], y[rr + 8:rr + 16])
                else:
                    y = e
                    ring_ref[idx, pl.ds(wx, n_mem // 2), :] = pk2(y[0:8], y[8:16])[0:n_mem // 2]
                yt[p][n0 + n] = stash(idx, packed(p, (n0 + n) % 3, y))
            if full and not LATE:
                for n in range(len(pa)):
                    x1[p][n0 + n] = ring_ref[p * NT + n0 + n, pl.ds(rd, seg // 2), :]

        def ab(z8):
            return jnp.where(la8, z8, 0.0), jnp.where(la8, 0.0, z8)

        def packed(p, j, y):
            u2 = pk2(y[32:40], y[40:48])
            if p == 0 or j == 0:
                return [pk2(y[0:8], y[8:16]), pk2(y[16:24], y[24:32]), u2]
            if j == 2:
                return [pk2(y[8:16], y[0:8]), pk2(y[24:32], y[16:24]), u2]
            xa_a, xa_b = ab(y[8:16])
            out = [pk2(xa_b, xa_a), pk2(y[24:32], y[16:24]) & mask_b, pk2(y[16:24], y[24:32]) & mask_a, u2]
            if full:
                out += [pk2(*ab(y[0:8])), pk2(*ab(y[16:24]))]
            return out

        def stash(idx, parts):
            if not KVS:
                return lambda: parts
            kv_ref[idx, 0:8 * len(parts), :] = _cat(parts)
            return lambda: [kv_ref[idx, 8 * e:8 * e + 8, :] for e in range(len(parts))]

        def pair(p, g):
            if full and LATE:
                xs = [ring_ref[p * NT + 3 * g + j, pl.ds(rd, seg // 2), :] for j in range(3)]
            else:
                xs = x1[p][3 * g:3 * g + 3]
            return [f() for f in yt[p][3 * g:3 * g + 3]], xs

        def q_rows(z, j):
            v0, v1, v2 = z[0][j]
            return [v0] + ([z[1][j]] if full else []) + [v1, v2]

        def kv_tiles(z):
            yt, x1 = z
            v0, v1, v2 = yt[0]
            t0 = [v0] + ([x1[0]] if full else [v1, v2]) + [v1, v2]
            w0, w1, w2 = yt[2]
            t2 = [w0, w1, w2] + ([x1[2]] if full else [w1, w2])
            if full:
                t0 += [v0, v1]
                t2 += [w0, w1]
            e1, mb, ma, u2 = yt[1][0:4]
            mid2 = [e1, mb, u2 & mask_b, ma, u2 & mask_a]
            mid1 = None
            if full:
                lo, hi = x1[1][0:8], x1[1][8:16]
                mid1 = [yt[1][4], lo & mask_a, hi & mask_a, lo & mask_b, hi & mask_b, e1, yt[1][5]]
            return t0, mid1, mid2, t2

        def mat(parts):
            return _upk(_cat(parts))

        def scores(q, k):
            k0, km1, km2, k2_ = kv_tiles(k)
            s_a = _nt(mat(q_rows(q, 0)), mat(k0))
            s_b = _nt(mat(q_rows(q, 2)), mat(k2_))
            qm = q_rows(q, 1)
            if full:
                s_m = _cat([_nt(mat(qm[0:2]), mat(km1)), _nt(mat(qm[2:4]), mat(km2 + km1[5:]))])
            else:
                s_m = _nt(mat(qm), mat(km2))
            out = []
            for e, sx in enumerate((s_a, s_b)):
                s = (sx + s_m) * scale + bias_ref[bidx + e, 0:RA, 0:CW]
                ex = jnp.exp2(s - jnp.max(s, axis=-1, keepdims=True))
                out.append(ex * _recip(jnp.sum(ex, axis=-1, keepdims=True)))
            if PSC:
                idx = 2 * len(probs)
                for e in range(2):
                    ps_ref[idx + e, 0:RA, 0:CW] = out[e]
                return lambda: [ps_ref[idx + e, 0:RA, 0:CW] for e in range(2)]
            return lambda: out

        def pv(p, v):
            p = p()
            v0, vm1, vm2, v2 = kv_tiles(v)
            o_a = _nn(p[0].astype(BF16), mat(v0))
            o_b = _nn(p[1].astype(BF16), mat(v2))
            p = p[0] + p[1]
            if full:
                o_m = _cat([_nn(p[0:M2 + seg].astype(BF16), mat(vm1)),
                            _nn(p[M2 + seg:R, 0:R].astype(BF16), mat(vm2))])
            else:
                o_m = _nn(p.astype(BF16), mat(vm2))
            out = []
            for o in (o_a, o_m, o_b):
                if OSC:
                    idx = len(ot) + len(out)
                    os_ref[idx, 0:RA, :] = o
                    out.append(functools.partial(lambda i: os_ref[i, 0:RA, :], idx))
                else:
                    out.append(functools.partial(lambda z: z, o))
            return out

        ot = []
        pacc, qacc = {}, {}

        def add_o(r):
            n0 = 0 if r == 0 else RT + (r - 1) * GT
            oo = [f() for f in ot[n0:n0 + (RT if r == 0 else GT)]]
            if full:
                ops = _Operands([o[0:32] for o in oo], [_cat([o[48:64], o[32:48]]) for o in oo],
                                [o[64:80] for o in oo])
            else:
                ops = _Operands(None, None, oo)
            _fast_mm(_reorder((S35 if r == 0 else S55)[1], MDW), ops, tile_dot(3, r), mh, pacc, qacc)

        wsched = dict(tuple(int(v) for v in e.split(":")) for e in WSCHED.split(","))
        bqkv = [None] * 3
        probs = []
        x2_new = None

        def do_pv():
            for g in range(len(ot) // 3, len(probs)):
                ot.extend(pv(probs[g], pair(2, g)))

        for r in range(NG + 1):
            npr = len(probs)
            for ch in ORDR:
                if ch in 'qkv':
                    proj('qkv'.index(ch), r)
                elif ch == 'P':
                    for g in range(len(ot) // 3, npr):
                        ot.extend(pv(probs[g], pair(2, g)))
                elif ch == 'S':
                    for g in range(len(probs), (RT + r * GT) // 3):
                        probs.append(scores(pair(0, g), pair(1, g)))
                else:
                    if r == 0:
                        blhs = _ln(b_in()).astype(BF16)
                    if r < 3:
                        bqkv[2 - r] = b_proj(blhs, 2 - r)
                    if r == 3:
                        ob = b_attn(jobs, *bqkv)
                    if r == BOUT_R:
                        res = b_in()
                        if split:
                            x2_new = b_out(ob[0], res[0:seg])
                        elif full:
                            zb = b_out(_cat(ob), res)
                            x2_new = zb[0:seg]
                            o_store(t - 1 - LAG, zb[seg:2 * seg])
                        else:
                            x2_new = b_out(ob[0], res)
                            o_store(lb * (t_last - LAG - 1) - 1, x2_new)
                    if r in wsched:
                        add_o(wsched[r])
        for r in range(len(wsched), TAILPV):
            add_o(r)
        do_pv()
        for r in range(max(TAILPV, len(wsched)), NG + 1):
            add_o(r)
        cols = []
        for n in range(nct):
            y, z, e = _fast_out(pacc, qacc, n, mh)
            cols.append(_cat([y, z[16:32], z[0:16], e]) if full else e)
        acc = _cat(cols, axis=1)
        if split:
            o_store(t - 1 - LAG, b_out(ob[1], res[seg:2 * seg]))

        y2 = x2_ref[...] + _cat([acc[n_mem:M2], acc[RA - seg + n_mem:RA]])
        mem2 = acc[RA - seg:RA - seg + n_mem]
        if full:
            x_cur = x_ref[pl.ds(pl.multiple_of(t * seg, seg), seg), :].astype(F32)
            xb_ref[0:seg, :] = x_cur + acc[M2:M2 + seg]
            xb_ref[seg:2 * seg, :] = y2
            m1n = acc[0:n_mem]
            m2n = mem2
            ahn = AHS[(u + 1) % UNROLL]
            an = pl.multiple_of(jnp.minimum(A0 + a_off + AHS[u], S - ahn), 16)
            h_ref[RB:RB + ahn, :] = _ln(x_ref[pl.ds(an, ahn), :].astype(F32))
            nxt = x2_new
        else:
            xb_ref[pl.ds(pl.multiple_of(jnp.where(t < LAG, 0, (t - n_seg + 2) * seg), seg), seg), :] = y2
            m1n = jnp.where(t < LAG - 1, h_ref[RB + AHS[0]:RB + AHS[0] + n_mem, :], mem2)
            m2n = jnp.where(t == LAG - 1, mem0_ref[...].astype(F32), mem2)
            nxt = jnp.where(t < LAG - 1, x_ref[seg:2 * seg, :].astype(F32), x2_new)
        x2_ref[...] = nxt
        sl = _ln(nxt)
        h_ref[n_mem:M2, :] = sl[0:n_mem]
        h_ref[M2 + n_mem:RB, :] = sl[n_mem:seg]
        return _cat([m1n, m2n])

    def single_body(t, c):
        @pl.when(t >= n_seg)
        def _():
            out_copy(t - (LAG + 3)).start()
        return step(t, c, False)

    def full_body(i, c):
        t = LAG + UNROLL * i
        for u in range(UNROLL):
            @pl.when(t - u >= LAG + 2)
            def _():
                out_copy(t - u - (LAG + 2)).start()
        for u in range(UNROLL):
            c = step(t + u, c, True, u, i)
        return c

    def phase(ph, c):
        t0 = ph * n_seg
        c = lax.fori_loop(t0, t0 + LAG, single_body, c)

        @pl.when(ph == 0)
        def _():
            x_late.wait()
        return lax.fori_loop(0, jnp.where(ph == 0, (n_seg - LAG) // UNROLL, 0), full_body, c)
    if not SKIPM:
      lax.fori_loop(0, 2, phase, _cat([h_ref[0:n_mem, :], h_ref[M2:M2 + n_mem, :]]))

    if SKIPM:
        def keep(i, c):
            z = (w_ref[i, pl.ds(pl.multiple_of(i * 8, 8), 8), :] + ring_ref[i, pl.ds(pl.multiple_of(i * 8, 8), 8), :]
                 + wr_ref[i & 3, pl.ds(pl.multiple_of(i * 8, 8), 8), :])
            xb_ref[2 * seg:2 * seg + 8, 0:128] = pltpu.bitcast(z, F32) + h_ref[pl.ds(pl.multiple_of((i & 7) * 8, 8), 8), 0:128] + x2_ref[0:8, 0:128]
            return c
        lax.fori_loop(0, 20, keep, 0)
    out_copy(n_seg - 3).start()
    res = xb_ref[2 * seg:4 * seg, :]
    blhs = _ln(res).astype(BF16)
    ob = b_attn([(1, n_seg - 2), (1, n_seg - 1)], *[b_proj(blhs, part) for part in range(3)])
    o_store(n_seg - 2, b_out(_cat(ob), res))
    out_copy(n_seg - 2).start()
    out_copy(n_seg - 1).start()
    pltpu.make_async_copy(o_ref.at[pl.ds(seg, S), :], out_hbm, sem_o).wait()


@functools.partial(jax.jit, static_argnames=("seg",))
def _run(A_x, A_mem0, A_Wq, A_Wk, A_Wv, A_Wo, B_wqkv, B_wo, *, seg):
    _, S, dm = A_x.shape
    n_heads, dh = A_Wq.shape[1], A_Wq.shape[2]
    n_mem = A_mem0.shape[1]
    n_seg = S // seg
    hd = n_heads * dh
    nct = dm // 128
    ng = (hd // 128 - RT) // GT
    assert (seg, n_seg, n_mem, dh, dm % 128, n_heads, LAG, UNROLL) == (32, 64, 8, 192, 0, 32, 2, 2)

    x = A_x.reshape(S, dm)
    mem0 = A_mem0.reshape(n_mem, dm)
    wq = jnp.transpose(A_Wq, (1, 2, 0)).reshape(hd, dm)
    wk = jnp.transpose(A_Wk, (1, 2, 0)).reshape(hd, dm)
    wv = jnp.transpose(A_Wv, (1, 2, 0)).reshape(hd, dm)
    wo = A_Wo.reshape(hd, dm)
    _, _, _, _, rs, xc = _plan(seg, n_seg)

    kern = functools.partial(_kernel, seg=seg, n_seg=n_seg, n_mem=n_mem,
                             n_heads=n_heads, dh=dh, dm=dm)
    hbm = pl.BlockSpec(memory_space=pltpu.HBM)

    out = pl.pallas_call(
        kern,
        in_specs=[hbm] * 8,
        out_specs=hbm,
        out_shape=jax.ShapeDtypeStruct((S, dm), A_x.dtype),
        scratch_shapes=[
            pltpu.VMEM((S, dm), BF16),
            pltpu.VMEM((n_mem, dm), BF16),
            pltpu.VMEM((NSLOT, 4, GT * 128, dm), BF16),
            pltpu.VMEM((4, RT * 128, dm), BF16),
            pltpu.VMEM((4, len(S53[0]) * 64, 128), U32),
            pltpu.VMEM((4 * ng, len(S55[0]) * 64, 128), U32),
            pltpu.VMEM((dm, 4 * dm + 128), BF16),
            pltpu.VMEM((nct, 5 * dm + 32, 128), F32),
            pltpu.VMEM((4 * nct + 1, dm // 2, 128), U32),
            pltpu.VMEM((len(KEYS), NXC * xc // 4, 128), U32),
            pltpu.VMEM((3 * hd // 128, rs // 2 + 8, 128), U32),
            pltpu.VMEM((3 * n_mem + seg + AHS[0], dm), F32),
            pltpu.VMEM((4 * seg, dm), F32),
            pltpu.VMEM((seg, dm), F32),
            pltpu.VMEM((2, nct, HIST + seg, 128), F32),
            pltpu.VMEM((2, nct, HIST + seg, 128), F32),
            pltpu.VMEM((S + seg, dm), A_x.dtype),
            pltpu.VMEM((4, 2 * n_mem + 2 * seg, 128), F32),
            pltpu.VMEM((3 * hd // 128, 48, 128), U32),
            pltpu.VMEM((hd // 128, 2 * n_mem + 2 * seg, 128), F32),
            pltpu.VMEM((n_heads, 2 * n_mem + 2 * seg, 128), F32),
            pltpu.SemaphoreType.DMA((NSLOT,)),
            pltpu.SemaphoreType.DMA((8 + NXC,)),
            pltpu.SemaphoreType.DMA((4,)),
            pltpu.SemaphoreType.DMA(()),
        ],
        compiler_params=pltpu.CompilerParams(
            vmem_limit_bytes=120 * 1024 * 1024,
            disable_bounds_checks=True,
        ),
    )(x, mem0, wq, wk, wv, wo, B_wqkv, B_wo)
    return out.reshape(1, S, dm)


def pallas_interleave_layers__memory_aug_recurrent_mem_tr__sliding_local_dilated__prompt_kernel(
    A_x: jax.Array,
    A_mem0: jax.Array,
    A_Wq: jax.Array,
    A_Wk: jax.Array,
    A_Wv: jax.Array,
    A_Wo: jax.Array,
    A_seg_len,
    B_x: jax.Array,
    B_wqkv: jax.Array,
    B_wo: jax.Array,
):
    del B_x
    seg = A_seg_len if isinstance(A_seg_len, int) else 32
    return _run(A_x, A_mem0, A_Wq, A_Wk, A_Wv, A_Wo, B_wqkv, B_wo, seg=seg)
```

```python
import functools

import jax
import jax.numpy as jnp
from jax import lax
import jax.experimental.pallas as pl
import jax.experimental.pallas.tpu as pltpu

F32 = jnp.float32
BF16 = jnp.bfloat16
U32 = jnp.uint32
NEG = -1000000000.0
LN_EPS = 1e-05
LOG2E = 1.4426950408889634
NEG2 = NEG * LOG2E

B_HEADS = 32
B_WIN = 8
B_DIL = 2
HIST = 16
UNROLL = int(1)
AHS = (16,) * UNROLL
LAG = 2
NSLOT = 2
NNM = '000'
NNF = '000'
WSCHED = '3:0,4:1,6:2,7:3,8:4,9:5'
BOUT_R = int(5)
ORDR = 'vkqFPS'
TAILPV = int(7)
PERT = int(1)
WPOS = int(0)
SKIPM = int(0)
MDQ = 'l'
MDW = 'l'
CW128 = int(0)
OSC = int(0)
PSC = int(0)
LATE = int(1)
KVS = int(1)
BT = int(0)
NOB = int(0)
WTT = int(1)
DORD = 'sss'
RCH = [int(v) for v in '80,80,80'.split(',')]
NXC = 6
HC = 3


def _ln(x):
    m = jnp.mean(x, axis=-1, keepdims=True)
    c = x - m
    v = jnp.mean(c * c, axis=-1, keepdims=True)
    return c * lax.rsqrt(v + LN_EPS)


def _recip(d):
    return pl.reciprocal(d, approx=True)


def _nt(a, b):
    return lax.dot_general(a, b, (((1,), (1,)), ((), ())), preferred_element_type=F32)


def _nn(a, b):
    return jnp.dot(a, b, preferred_element_type=F32)


def _cat(xs, axis=0):
    return xs[0] if len(xs) == 1 else jnp.concatenate(xs, axis=axis)


def _pk(z):
    return pltpu.bitcast(z, U32)


def _upk(z):
    return pltpu.bitcast(z, BF16)


LAM = (-1.5, -0.5, 0.0, 0.5, 1.5)


def _scheme(stars):
    tiles, prog = [], []
    for star in stars:
        if len(star) == 1:
            prog.append(("single", star[0], None, len(tiles)))
            tiles.append([star[0][:2]])
            continue
        left = [len(star) - 1] * len(star)
        for j in range(1, len(star)):
            for i in range(j):
                x, y = star[i], star[j]
                prog.append(("pair", x, y, len(tiles)))
                tiles += [[(x[0], y[1])], [(y[0], x[1])], [(x[0], y[1]), (y[0], x[1])]]
                for e in (i, j):
                    left[e] -= 1
                    if left[e] == 0:
                        z = star[e]
                        prog.append(("diag", z, None, len(tiles)))
                        tiles += [[z[:2]] + [(o[0], z[1]) for o in star if o is not z],
                                  [z[:2]] + [(z[0], o[1]) for o in star if o is not z]]
    return tiles, prog


S55 = _scheme([[(i, i, LAM[i]) for i in range(5)]])
S53 = _scheme([[(0, 0, LAM[0]), (2, 1, LAM[2]), (4, 2, LAM[4])], [(1, 0, LAM[1]), (3, 2, LAM[3])],
               [(1, 1, LAM[1])], [(3, 1, LAM[3])]])
S35 = _scheme([[(0, 0, LAM[0]), (1, 2, LAM[2]), (2, 4, LAM[4])], [(0, 1, LAM[1]), (2, 3, LAM[3])],
               [(1, 1, LAM[1])], [(1, 3, LAM[3])]])


def _reorder(prog, mode):
    pairs = [e for e in prog if e[0] != "diag"]
    diags = [e for e in prog if e[0] == "diag"]
    if mode == "l":
        return prog
    out = []
    if mode == "f":
        for e in pairs:
            for z in (e[1], e[2]):
                for dg in diags:
                    if dg[1] == z and dg not in out:
                        out.append(dg)
            out.append(e)
        return out
    step = len(pairs) / len(diags)
    k = 0
    for i, e in enumerate(pairs):
        out.append(e)
        while k < len(diags) and (k + 0.5) * step <= i + 1:
            out.append(diags[k])
            k += 1
    return out + diags[k:]


def _op_keys(prog):
    keys = []
    for kind, x, y, _ in prog:
        if kind == "pair":
            new = [(nm, x[0], x[2], y[0], y[2]) for nm in ("l1", "l2", "A")]
        else:
            new = [("a", x[0], x[2]), ("b", x[0])]
        keys += [k for k in new if k not in keys]
    return keys


def _scaled(c, u):
    return u if c == 1.0 else c * u


class _Operands:
    def __init__(self, T, U, E):
        self.T, self.U, self.E, self.memo = T, U, E, {}

    def _get(self, key, fn):
        if key not in self.memo:
            self.memo[key] = fn()
        return self.memo[key]

    def paired(self, key):
        T, U = self.T, self.U
        if key[0] == "b":
            return U[key[1]]
        if key[0] == "a":
            k, lam = key[1:]
            if lam == 0.0:
                return T[k]
            return self._get(("f",) + key, lambda: T[k] - _scaled(lam, U[k]) if lam > 0
                             else T[k] + _scaled(-lam, U[k]))
        kx, lx, ky, ly = key[1:]
        A = self._get(("f", "A") + key[1:],
                      lambda: self.paired(("a", kx, lx)) + self.paired(("a", ky, ly)))
        if key[0] == "A":
            return A
        return A - _scaled(ly - lx, U[kx]) if key[0] == "l1" else A + _scaled(ly - lx, U[ky])

    def extra(self, key):
        if key[0] == "a":
            return self.E[key[1]]
        return self._get(("e", key[1], key[3]), lambda: self.E[key[1]] + self.E[key[3]])

    def __call__(self, key):
        if self.T is None:
            ek = ("a", key[1]) if key[0] in ("a", "s") else ("l", key[1], 0, key[3])
            return self._get(ek, lambda: self.extra(ek).astype(BF16))

        def build():
            ak = ("a",) + key[1:] if key[0] == "s" else key
            parts = [self.paired(ak)]
            if self.E is not None and ak[0] in ("a", "l1", "l2"):
                parts.append(self.extra(ak))
            if key[0] == "s":
                parts.append(self.U[key[1]])
            return _cat(parts).astype(BF16)
        return self._get(key, build)


def _fast_mm(prog, op, dot, m, p, q):
    def add(d, key, val):
        d[key] = val if key not in d else d[key] + val

    for kind, x, y, i in prog:
        if kind == "pair":
            kk = (x[0], x[2], y[0], y[2])
            p1, p2 = dot(op(("l1",) + kk), i), dot(op(("l2",) + kk), i + 1)
            if m:
                r = _scaled(1.0 / (y[2] - x[2]), p2[0:m] - p1[0:m] + dot(op(("A",) + kk), i + 2))
                add(q, (x[1], x[2]), r)
                add(q, (y[1], y[2]), r)
            add(p, y[1], p1)
            add(p, x[1], p2)
        elif kind == "diag":
            add(p, x[1], dot(op(("a", x[0], x[2])), i))
            if m:
                add(q, (x[1], x[2]), dot(op(("b", x[0])), i + 1))
        else:
            r = dot(op(("s", x[0], x[2])), i)
            add(p, x[1], r[0:r.shape[0] - m])
            if m:
                add(q, (x[1], x[2]), r[r.shape[0] - m:])


def _fast_out(p, q, n, m):
    if not m:
        return None, None, p[n]
    y, z = p[n][0:m], None
    for (nn, lam), v in q.items():
        if nn == n:
            z = v if z is None else z + v
            if lam != 0.0:
                y = y + _scaled(lam, v) if lam > 0 else y - _scaled(-lam, v)
    return y, z, (p[n][m:] if p[n].shape[0] > m else None)


def _combo(tile, block):
    out = block(*tile[0])
    for kn in tile[1:]:
        out = out - block(*kn)
    return out


GT = 5
RT = 3
KEYS_R = _op_keys(S53[1])
KEYS = KEYS_R + [k for k in _op_keys(S55[1]) if k not in KEYS_R]


def _plan(seg, n_seg):
    S = seg * n_seg
    R0 = LAG * seg
    A0 = S - (n_seg - LAG) // UNROLL * sum(AHS)
    NPRE = A0 - R0 - LAG * 8
    RS = -(-(A0 - R0 + AHS[0]) // seg) * seg
    XC = NPRE // NXC // 32 * 32
    assert XC * NXC + 16 == NPRE
    return S, R0, A0, NPRE, RS, XC


def _kernel(x_hbm, mem0_hbm, wq_hbm, wk_hbm, wv_hbm, wo_hbm, bqkv_hbm, bwo_hbm,
            out_hbm,
            x_ref, mem0_ref, stage_ref, stage0_ref, wr_ref, w_ref, bst_ref, btmp_ref, bw_ref,
            xln_ref, xe_ref, ring_ref, h_ref, xb_ref, x2_ref, kb_ref, vb_ref, o_ref, bias_ref, kv_ref, os_ref, ps_ref,
            sem_w, sem_m, sem_b, sem_o,
            *, seg, n_seg, n_mem, n_heads, dh, dm):
    S, R0, A0, NPRE, RS, XC = _plan(seg, n_seg)
    M2 = 2 * n_mem
    R = M2 + 2 * seg
    RB = M2 + seg
    PW = 2 * dh
    G = n_heads // 2
    nct = dm // 128
    bdh = dm // B_HEADS
    NT = n_heads * dh // 128
    NG = (NT - RT) // GT
    w_hbm = (wq_hbm, wk_hbm, wv_hbm, wo_hbm)

    def w_copy(p, g):
        slot = g & (NSLOT - 1)
        return pltpu.make_async_copy(w_hbm[p].at[pl.ds((RT + (g - 1) * GT) * 128, GT * 128), :],
                                     stage_ref.at[slot, p], sem_w.at[slot])

    def w0_copy(p):
        return pltpu.make_async_copy(w_hbm[p].at[pl.ds(0, RT * 128), :], stage0_ref.at[p], sem_m.at[4 + p])

    NB1 = 3 * nct
    WO0 = 3 * dm
    DUM = 4 * dm
    XF = A0 + AHS[0]
    XH = XC // 2

    def rows_copy(r0, n, sem):
        return pltpu.make_async_copy(x_hbm.at[pl.ds(r0, n), :], x_ref.at[pl.ds(r0, n), :], sem)

    def x_copy(i):
        return rows_copy(pl.multiple_of(R0 + i * XC, 16), XC, sem_m.at[8 + i])

    small = [rows_copy(0, R0, sem_m.at[1]), rows_copy(R0 + NPRE - 16, XF - R0 - NPRE + 16, sem_m.at[2]),
             pltpu.make_async_copy(mem0_hbm, mem0_ref, sem_m.at[3])]
    x_late = rows_copy(XF, S - XF, sem_m.at[0])

    def bq_copy(part):
        c0 = pl.multiple_of(part * dm, 128)
        return pltpu.make_async_copy(bqkv_hbm.at[:, pl.ds(c0, dm)], bst_ref.at[:, pl.ds(c0, dm)], sem_b.at[part])

    bo_copy = pltpu.make_async_copy(bwo_hbm, bst_ref.at[:, pl.ds(3 * dm, dm)], sem_b.at[3])

    def bst_tile(c):
        return bst_ref[:, pl.ds(pl.multiple_of(c * 128, 128), 128)]

    def bias_tables(full):
        RA = R if full else M2 + seg
        CW = 128
        ri = lax.broadcasted_iota(jnp.int32, (RA, CW), 0)
        ci = lax.broadcasted_iota(jnp.int32, (RA, CW), 1)
        if not full:
            ri = jnp.where(ri >= M2, ri + seg, ri)

        def table(i, bounds, vals):
            out = vals[-1]
            for b, v in zip(reversed(bounds), reversed(vals[:-1])):
                out = jnp.where(i < b, v, out)
            return out
        qi = ri - table(ri, [16, 48, 56], [0, 8, 48, 40])
        g0 = (ci < 8) | ((ci >= 16) & (ci < 48))
        k2 = ci - table(ci, [8, 24, 32, 48, 56, 80, 88, 96, 104], [-8, 0, 24, 8, 48, 40, 72, 80, 96, 104])
        if full:
            k1 = ci - table(ci, [8, 48], [0, 8, 40])
            row_l2 = ((ri >= 8) & (ri < 16)) | (ri >= 48)
            row_xa = (ri >= 8) & (ri < 16)
            valid = (row_xa == (ci >= 80)) & (ci < 112)
            is_a = jnp.where(ci >= 80, ((ci >= 88) & (ci < 104)).astype(jnp.int32),
                             (g0 != row_l2).astype(jnp.int32)) > 0
            ki = jnp.where(row_l2, k2, k1)
            visible = valid & ((qi < n_mem) | (qi >= ki))
            fill = jnp.where(valid, NEG2, -jnp.inf)
        else:
            is_a = jnp.logical_not(g0)
            visible = (qi < n_mem) | (qi >= k2)
            fill = NEG2
        for e, mine in enumerate((is_a, jnp.logical_not(is_a))):
            bias_ref[(0 if full else 2) + e, 0:RA, :] = jnp.where(
                mine, jnp.where(visible, 0.0, fill), -jnp.inf)

    for cp in small:
        cp.start()
    for i in range(HC):
        x_copy(i).start()

    def zero_body(j, c):
        btmp_ref[j, DUM:, :] = jnp.zeros((btmp_ref.shape[1] - DUM, 128), F32)
        return c
    lax.fori_loop(0, nct, zero_body, 0)

    w0_copy(0).start()
    xb_ref[0:2 * seg, :] = jnp.zeros((2 * seg, dm), F32)
    kb_ref[...] = jnp.zeros(kb_ref.shape, F32)
    vb_ref[...] = jnp.zeros(vb_ref.shape, F32)
    bst_ref[:, 4 * dm:] = jnp.zeros((dm, 128), BF16)
    bias_tables(True)
    bias_tables(False)
    for cp in small:
        cp.wait()

    def ekey(key):
        return ("a", key[1]) if key[0] == "a" else ("l", key[1], 0, key[3])
    EKEYS = []
    for key in KEYS:
        if key[0] in ("a", "l1") and ekey(key) not in EKEYS:
            EKEYS.append(ekey(key))
    ye = _ln(x_ref[R0 + NPRE - 16:R0 + NPRE, :].astype(F32))
    eops = _Operands(None, None, [ye[:, k * 128:(k + 1) * 128] for k in range(nct)])
    for j, key in enumerate(EKEYS):
        xe_ref[j] = _pk(eops(key))

    def ln_ops(i, hi):
        y = _ln(x_ref[pl.ds(pl.multiple_of(R0 + i * XC, 16), XC), :].astype(F32))
        ops = _Operands([y[0:XH, k * 128:(k + 1) * 128] for k in range(nct)],
                        [y[XH:XC, k * 128:(k + 1) * 128] for k in range(nct)], None)
        r0 = pl.multiple_of(i * (XH // 2), 8)
        for j in range(hi):
            xln_ref[j, pl.ds(r0, XH // 2), :] = _pk(ops(KEYS[j]))

    def ln_body(i, c):
        x_copy(i).wait()

        @pl.when(i == 0)
        def _():
            x_copy(HC).start()

        @pl.when(i == 1)
        def _():
            w0_copy(1).start()
            w0_copy(2).start()

        @pl.when(i == 2)
        def _():
            x_copy(HC + 1).start()
            x_copy(HC + 2).start()
        ln_ops(i, len(KEYS_R))
        return c
    lax.fori_loop(0, HC, ln_body, 0)

    def pre_chunk(scheme, w, dst, n0, c0, nchunk):
        tiles, prog = scheme
        prog = _reorder(prog, "s")
        raw = lambda k, n: w[n * 128:(n + 1) * 128, k * 128:(k + 1) * 128]
        tb = []
        for i, tl in enumerate(tiles):
            tb.append(raw(*tl[0]) if len(tl) == 1
                      else _combo(tl, lambda k, n: raw(k, n).astype(F32)).astype(BF16))
            dst[i * 64:(i + 1) * 64, :] = _pk(tb[i].T)

        def al(v, m):
            return v if isinstance(v, int) else pl.multiple_of(v, m)

        for cc in range(nchunk):
            c = c0 + cc

            def op(key):
                def ld(kk):
                    v = xln_ref[KEYS.index(kk), pl.ds(al(c * (XH // 2), 8), XH // 2), :]
                    if cc == nchunk - 1 and kk[0] in ("a", "l1", "l2"):
                        v = _cat([v, xe_ref[EKEYS.index(ekey(kk))]])
                    return v
                if key[0] == "s":
                    return _upk(_cat([ld(("a",) + key[1:]), ld(("b", key[1]))]))
                return _upk(ld(key))
            p, q = {}, {}
            _fast_mm(prog, op, lambda a, i: _nt(a, tb[i]), XH, p, q)
            for n in range(len(p)):
                y, z, e = _fast_out(p, q, n, XH)
                ring_ref[n0 + n, pl.ds(al(c * XH, 8), XH // 2), :] = _pk(y.astype(BF16))
                ring_ref[n0 + n, pl.ds(al(c * XH + XH // 2, 8), XH // 2), :] = _pk(z.astype(BF16))
                if e is not None:
                    ring_ref[n0 + n, NXC * XH:NXC * XH + 8, :] = _pk(e.astype(BF16))

    def init_rows():
        x0 = x_ref[0:seg, :].astype(F32)
        sl = _ln(x0)
        xt = _ln(x_ref[R0 + NPRE:XF, :].astype(F32))
        h_ref[0:n_mem, :] = xt[0:n_mem]
        h_ref[n_mem:M2, :] = sl[0:n_mem]
        h_ref[M2:M2 + n_mem, :] = mem0_ref[...].astype(F32)
        h_ref[M2 + n_mem:RB, :] = sl[n_mem:seg]
        h_ref[RB:RB + AHS[0], :] = xt[M2:M2 + AHS[0]]
        h_ref[RB + AHS[0]:RB + AHS[0] + n_mem, :] = xt[n_mem:M2]
        x2_ref[...] = x0

    def first_body(m, c):
        hf = (m >= 3).astype(jnp.int32)
        p = m - 3 * hf
        buf = stage0_ref.at[p]

        @pl.when(m < 3)
        def _():
            pltpu.make_async_copy(buf, buf, sem_m.at[4 + p]).wait()
            x_copy(HC + m).wait()

        @pl.when(m == 0)
        def _():
            for pp in range(4):
                w_copy(pp, 1).start()

        @pl.when(m == 2)
        def _():
            bq_copy(0).start()
        init_rows()
        pre_chunk(S53, buf, wr_ref.at[p], p * NT, hf * HC, HC)
        ln_ops(p + HC * (1 - hf), len(KEYS))
        return c
    lax.fori_loop(0, 6, first_body, 0)

    dpt = 128 // B_HEADS

    def b_stage1(u):
        ok = (u >= 0) & (u < NB1)
        tr = bst_tile(jnp.where(ok, u, NB1 + nct)).T.astype(F32) if BT & 1 else bst_tile(jnp.where(ok, u, NB1 + nct)).astype(F32).T
        r0 = pl.multiple_of(jnp.where(ok, u * 128, DUM), 128)
        for j in range(nct):
            btmp_ref[j, pl.ds(r0, 128), :] = tr[:, j * 128:(j + 1) * 128]

    def b_stage1_wo(u):
        ok = (u >= 0) & (u < nct)
        r0 = pl.multiple_of(jnp.where(ok, WO0, DUM), 128)
        btmp_ref[jnp.where(ok, u, 0), pl.ds(r0, dm), :] = bst_tile(
            jnp.where(ok, NB1 + u, NB1 + nct)).astype(F32)

    def b_stage2(u):
        ok = (u >= 0) & (u < NB1)
        part = (u >= nct).astype(jnp.int32) + (u >= 2 * nct).astype(jnp.int32)
        r0 = jnp.where(ok, part * dm + (u - part * nct) * dpt, DUM)
        rows = _cat([_cat([btmp_ref[j, pl.ds(r0 + dd, B_HEADS, stride=bdh), :]
                           for j in range(nct)], axis=1) for dd in range(dpt)])
        bw_ref[jnp.where(ok, u, NB1 + nct)] = _pk(rows.astype(BF16).T if BT & 2 else rows.T.astype(BF16))

    def b_stage2_wo(u):
        ok = (u >= 0) & (u < nct)
        r0 = jnp.where(ok, WO0, DUM)
        jj = jnp.where(ok, u, 0)
        bw_ref[jnp.where(ok, NB1 + u, NB1 + nct)] = _pk(
            _cat([btmp_ref[jj, pl.ds(r0 + d, B_HEADS, stride=bdh), :] for d in range(bdh)]).astype(BF16))

    def wo_store(scheme, w, dst):
        if WTT and scheme is S55:
            rawt = lambda k, n: w[k * 128:(k + 1) * 128, n * 128:(n + 1) * 128]
            for i, tl in enumerate(scheme[0]):
                if len(tl) == 1:
                    val = rawt(*tl[0])
                    if WTT == 3:
                        val = _upk(_pk(val.T)).T
                else:
                    val = _combo(tl, lambda k, n: rawt(k, n).astype(F32)).astype(BF16)
                    if WTT in (1, 3):
                        val = _upk(_pk(val.T)).T
                dst[i * 64:(i + 1) * 64, :] = _pk(val)
            return
        for r in range(0, 128, 16):
            memo = {}

            def raw(k, n):
                return w[k * 128 + r:k * 128 + r + 16, n * 128:(n + 1) * 128]

            def block(k, n):
                if (k, n) not in memo:
                    memo[k, n] = raw(k, n).astype(F32)
                return memo[k, n]
            for i, tl in enumerate(scheme[0]):
                val = raw(*tl[0]) if len(tl) == 1 else _combo(tl, block).astype(BF16)
                dst[i * 64 + r // 2:i * 64 + r // 2 + 8, :] = _pk(val)

    def pre_body(g, c):
        slot = g & (NSLOT - 1)
        buf = stage_ref.at[slot]
        pltpu.make_async_copy(buf, buf, sem_w.at[slot]).wait()

        @pl.when((g >= 2) & (g <= 4))
        def _():
            bq_copy(g - 2).wait()

        @pl.when(g == 4)
        def _():
            bo_copy.wait()

        @pl.when(g <= 2)
        def _():
            bq_copy(g).start()

        @pl.when(g == 2)
        def _():
            bo_copy.start()

        @pl.when(g + 1 <= NG)
        def _():
            for p in range(4):
                w_copy(p, g + 1).start()

        @pl.when(g == NG - 1)
        def _():
            w0_copy(3).start()
            x_late.start()

        if WPOS == 0:
            wo_store(S55, stage_ref.at[slot, 3], w_ref.at[3 * NG + g - 1])
        for e in range(0 if NOB else 3):
            b_stage2(3 * (g - 5) + e)
        b_stage2_wo(g - 5)
        for e in range(0 if NOB else 3):
            b_stage1(3 * (g - 2) + e)
        b_stage1_wo(g - 4)
        for p in range(3):
            pre_chunk(S55, stage_ref.at[slot, p], w_ref.at[p * NG + g - 1], p * NT + RT + (g - 1) * GT, 0, NXC)
            if WPOS == p + 1:
                wo_store(S55, stage_ref.at[slot, 3], w_ref.at[3 * NG + g - 1])
        return c
    lax.fori_loop(1, NG + 1, pre_body, 0)
    w0_copy(3).wait()

    bscale = float(bdh) ** (-0.5) * LOG2E

    def b_proj(lhs, part):
        return _nn(lhs, _cat([_upk(bw_ref[part * nct + j]) for j in range(nct)], axis=1))

    def b_attn(jobs, q, k, v):
        row = lax.broadcasted_iota(jnp.int32, (seg, 128), 0)
        outs = []
        for i, (l, sidx) in enumerate(jobs):
            r0 = i * seg
            pos = row + sidx * seg
            for j in range(nct):
                kb_ref[l, j, HIST:HIST + seg, :] = k[r0:r0 + seg, j * 128:(j + 1) * 128]
                vb_ref[l, j, HIST:HIST + seg, :] = v[r0:r0 + seg, j * 128:(j + 1) * 128]
            logits = []
            for w in range(B_WIN):
                o = HIST - w * B_DIL
                acc = None
                for j in range(nct):
                    p = q[r0:r0 + seg, j * 128:(j + 1) * 128] * kb_ref[l, j, o:o + seg, :]
                    acc = p if acc is None else acc + p
                acc = acc + pltpu.roll(acc, 64, 1)
                acc = acc + pltpu.roll(acc, 32, 1)
                lg = acc * bscale
                if w > 0:
                    lg = jnp.where(pos >= w * B_DIL, lg, NEG2)
                logits.append(lg)
            m = logits[0]
            for w in range(1, B_WIN):
                m = jnp.maximum(m, logits[w])
            es = [jnp.exp2(lg - m) for lg in logits]
            den = es[0]
            for w in range(1, B_WIN):
                den = den + es[w]
            inv = _recip(den)
            cols = []
            for j in range(nct):
                acc = None
                for w in range(B_WIN):
                    o = HIST - w * B_DIL
                    p = es[w] * vb_ref[l, j, o:o + seg, :]
                    acc = p if acc is None else acc + p
                cols.append(acc * inv)
            outs.append(_cat(cols, axis=1).astype(BF16))
            for j in range(nct):
                kb_ref[l, j, 0:HIST, :] = k[r0 + seg - HIST:r0 + seg, j * 128:(j + 1) * 128]
                vb_ref[l, j, 0:HIST, :] = v[r0 + seg - HIST:r0 + seg, j * 128:(j + 1) * 128]
        return outs

    def b_out(ob, res):
        return res + _nn(ob, _cat([_upk(bw_ref[NB1 + j]) for j in range(nct)], axis=1))

    def o_store(b, val):
        ro = pl.multiple_of((b + 1) * seg, seg)
        o_ref[pl.ds(ro, val.shape[0]), :] = val.astype(o_ref.dtype)

    def out_copy(b):
        ro = pl.multiple_of(b * seg, seg)
        return pltpu.make_async_copy(o_ref.at[pl.ds(ro + seg, seg), :], out_hbm.at[pl.ds(ro, seg), :], sem_o)

    def step(t, hc, full, u=0, i=None):
        t_last = n_seg + LAG - 1
        if full:
            jobs = [(0, t - 1), (1, t - 1 - LAG)]

            def b_in():
                return xb_ref[0:2 * seg, :]
        else:
            lb = (t == t_last).astype(jnp.int32)
            jobs = [(lb, t - 1 - lb * (LAG + 1))]

            def b_in():
                return xb_ref[pl.ds(pl.multiple_of(lb * seg, seg), seg), :]
        split = full and u < UNROLL - 1
        nq = RB + AHS[u] if full else RB
        v0r = _cat([hc[0:n_mem], h_ref[n_mem:M2, :]])
        v1r = _cat([hc[n_mem:M2], h_ref[M2 + n_mem:2 * M2, :]])

        def ktiles(z):
            return [z[:, k * 128:(k + 1) * 128] for k in range(z.shape[1] // 128)]
        if full:
            hl = _Operands(ktiles(_cat([v0r, h_ref[2 * M2:RB, :]])), ktiles(_cat([v1r, h_ref[RB:RB + 16, :]])),
                           ktiles(h_ref[RB + 16:nq, :]) if nq > RB + 16 else None)
        else:
            hl = _Operands(None, None, ktiles(_cat([v0r, v1r, h_ref[2 * M2:RB, :]])))
        mh = 2 * M2 if full else 0

        def tile_dot(p, r):
            src = wr_ref.at[p] if r == 0 else w_ref.at[p * NG + r - 1]
            return lambda a, i: _nn(a, _upk(src[i * 64:(i + 1) * 64, :]))
        scale = float(dh) ** (-0.5) * LOG2E
        if full:
            s_ = t - LAG
            rd = pl.multiple_of(lax.rem(s_ * (seg // 2), RS // 2), seg // 2)
            a_off = i * sum(AHS) + sum(AHS[:u])
            wa = [pl.multiple_of(lax.rem((A0 - R0 + a_off) // 2 + 8 * a, RS // 2), 8)
                  for a in range(AHS[u] // 16)]
        else:
            wx = pl.multiple_of(jnp.where(t < LAG, NPRE // 2 + t * (n_mem // 2), RS // 2), n_mem // 2)
            wo_store(S35, stage0_ref.at[3], wr_ref.at[3])

        RA = R if full else M2 + seg
        CW = (128 if CW128 else R + 2 * M2) if full else R
        bidx = 0 if full else 2
        half = dh - 128
        la8 = lax.broadcasted_iota(jnp.int32, (n_mem, 128), 1) < half
        ones = jnp.full((n_mem, 128), 0xFFFFFFFF, U32)
        zero = jnp.zeros((n_mem, 128), U32)
        mask_a = jnp.where(la8, ones, zero)
        mask_b = jnp.where(la8, zero, ones)

        def pk2(a, b):
            return _pk(_cat([a, b]).astype(BF16))

        yt = [[None] * NT for _ in range(3)]
        x1 = [[None] * NT for _ in range(3)]

        def proj(p, r):
            pa, qa = {}, {}
            _fast_mm(_reorder((S53 if r == 0 else S55)[1], MDQ), hl, tile_dot(p, r), mh, pa, qa)
            n0 = 0 if r == 0 else RT + (r - 1) * GT
            for n in range(len(pa)):
                y, z, e = _fast_out(pa, qa, n, mh)
                idx = p * NT + n0 + n
                if full:
                    y = _cat([y[0:M2], z[0:M2], y[M2:2 * M2], z[M2:2 * M2]] + ([] if e is None else [e]))
                    for a in range(AHS[u] // 16):
                        rr = RB + 16 * a
                        ring_ref[idx, pl.ds(wa[a], 8), :] = pk2(y[rr:rr + 8], y[rr + 8:rr + 16])
                else:
                    y = e
                    ring_ref[idx, pl.ds(wx, n_mem // 2), :] = pk2(y[0:8], y[8:16])[0:n_mem // 2]
                yt[p][n0 + n] = stash(p * 16 + (n0 + n) % 16, packed(p, (n0 + n) % 3, y))
            if full and not LATE:
                for n in range(len(pa)):
                    x1[p][n0 + n] = ring_ref[p * NT + n0 + n, pl.ds(rd, seg // 2), :]

        def ab(z8):
            return jnp.where(la8, z8, 0.0), jnp.where(la8, 0.0, z8)

        def packed(p, j, y):
            u2 = pk2(y[32:40], y[40:48])
            if p == 0 or j == 0:
                return [pk2(y[0:8], y[8:16]), pk2(y[16:24], y[24:32]), u2]
            if j == 2:
                return [pk2(y[8:16], y[0:8]), pk2(y[24:32], y[16:24]), u2]
            xa_a, xa_b = ab(y[8:16])
            out = [pk2(xa_b, xa_a), pk2(y[24:32], y[16:24]) & mask_b, pk2(y[16:24], y[24:32]) & mask_a, u2]
            if full:
                out += [pk2(*ab(y[0:8])), pk2(*ab(y[16:24]))]
            return out

        def stash(idx, parts):
            if not KVS:
                return lambda: parts
            kv_ref[idx, 0:8 * len(parts), :] = _cat(parts)
            return lambda: [kv_ref[idx, 8 * e:8 * e + 8, :] for e in range(len(parts))]

        def pair(p, g):
            if full and LATE:
                xs = [ring_ref[p * NT + 3 * g + j, pl.ds(rd, seg // 2), :] for j in range(3)]
            else:
                xs = x1[p][3 * g:3 * g + 3]
            return [f() for f in yt[p][3 * g:3 * g + 3]], xs

        def q_rows(z, j):
            v0, v1, v2 = z[0][j]
            return [v0] + ([z[1][j]] if full else []) + [v1, v2]

        def kv_tiles(z):
            yt, x1 = z
            v0, v1, v2 = yt[0]
            t0 = [v0] + ([x1[0]] if full else [v1, v2]) + [v1, v2]
            w0, w1, w2 = yt[2]
            t2 = [w0, w1, w2] + ([x1[2]] if full else [w1, w2])
            if full:
                t0 += [v0, v1]
                t2 += [w0, w1]
            e1, mb, ma, u2 = yt[1][0:4]
            mid2 = [e1, mb, u2 & mask_b, ma, u2 & mask_a]
            mid1 = None
            if full:
                lo, hi = x1[1][0:8], x1[1][8:16]
                mid1 = [yt[1][4], lo & mask_a, hi & mask_a, lo & mask_b, hi & mask_b, e1, yt[1][5]]
            return t0, mid1, mid2, t2

        def mat(parts):
            return _upk(_cat(parts))

        def scores(q, k):
            k0, km1, km2, k2_ = kv_tiles(k)
            s_a = _nt(mat(q_rows(q, 0)), mat(k0))
            s_b = _nt(mat(q_rows(q, 2)), mat(k2_))
            qm = q_rows(q, 1)
            if full:
                s_m = _cat([_nt(mat(qm[0:2]), mat(km1)), _nt(mat(qm[2:4]), mat(km2 + km1[5:]))])
            else:
                s_m = _nt(mat(qm), mat(km2))
            out = []
            for e, sx in enumerate((s_a, s_b)):
                s = (sx + s_m) * scale + bias_ref[bidx + e, 0:RA, 0:CW]
                ex = jnp.exp2(s - jnp.max(s, axis=-1, keepdims=True))
                out.append(ex * _recip(jnp.sum(ex, axis=-1, keepdims=True)))
            if PSC:
                idx = 2 * len(probs)
                for e in range(2):
                    ps_ref[idx + e, 0:RA, 0:CW] = out[e]
                return lambda: [ps_ref[idx + e, 0:RA, 0:CW] for e in range(2)]
            return lambda: out

        def pv(p, v):
            p = p()
            v0, vm1, vm2, v2 = kv_tiles(v)
            o_a = _nn(p[0].astype(BF16), mat(v0))
            o_b = _nn(p[1].astype(BF16), mat(v2))
            p = p[0] + p[1]
            if full:
                o_m = _cat([_nn(p[0:M2 + seg].astype(BF16), mat(vm1)),
                            _nn(p[M2 + seg:R, 0:R].astype(BF16), mat(vm2))])
            else:
                o_m = _nn(p.astype(BF16), mat(vm2))
            out = []
            for o in (o_a, o_m, o_b):
                if OSC:
                    idx = len(ot) + len(out)
                    os_ref[idx, 0:RA, :] = o
                    out.append(functools.partial(lambda i: os_ref[i, 0:RA, :], idx))
                else:
                    out.append(functools.partial(lambda z: z, o))
            return out

        ot = []
        pacc, qacc = {}, {}

        def add_o(r):
            n0 = 0 if r == 0 else RT + (r - 1) * GT
            oo = [f() for f in ot[n0:n0 + (RT if r == 0 else GT)]]
            if full:
                ops = _Operands([o[0:32] for o in oo], [_cat([o[48:64], o[32:48]]) for o in oo],
                                [o[64:80] for o in oo])
            else:
                ops = _Operands(None, None, oo)
            _fast_mm(_reorder((S35 if r == 0 else S55)[1], MDW), ops, tile_dot(3, r), mh, pacc, qacc)

        wsched = dict(tuple(int(v) for v in e.split(":")) for e in WSCHED.split(","))
        bqkv = [None] * 3
        probs = []
        x2_new = None

        def do_pv():
            for g in range(len(ot) // 3, len(probs)):
                ot.extend(pv(probs[g], pair(2, g)))

        for r in range(NG + 1):
            npr = len(probs)
            for ch in ORDR:
                if ch in 'qkv':
                    proj('qkv'.index(ch), r)
                elif ch == 'P':
                    for g in range(len(ot) // 3, npr):
                        ot.extend(pv(probs[g], pair(2, g)))
                elif ch == 'S':
                    for g in range(len(probs), (RT + r * GT) // 3):
                        probs.append(scores(pair(0, g), pair(1, g)))
                else:
                    if r == 0:
                        blhs = _ln(b_in()).astype(BF16)
                    if r < 3:
                        bqkv[2 - r] = b_proj(blhs, 2 - r)
                    if r == 3:
                        ob = b_attn(jobs, *bqkv)
                    if r == BOUT_R:
                        res = b_in()
                        if split:
                            x2_new = b_out(ob[0], res[0:seg])
                        elif full:
                            zb = b_out(_cat(ob), res)
                            x2_new = zb[0:seg]
                            o_store(t - 1 - LAG, zb[seg:2 * seg])
                        else:
                            x2_new = b_out(ob[0], res)
                            o_store(lb * (t_last - LAG - 1) - 1, x2_new)
                    if r in wsched:
                        add_o(wsched[r])
        for r in range(len(wsched), TAILPV):
            add_o(r)
        do_pv()
        for r in range(max(TAILPV, len(wsched)), NG + 1):
            add_o(r)
        cols = []
        for n in range(nct):
            y, z, e = _fast_out(pacc, qacc, n, mh)
            cols.append(_cat([y, z[16:32], z[0:16], e]) if full else e)
        acc = _cat(cols, axis=1)
        if split:
            o_store(t - 1 - LAG, b_out(ob[1], res[seg:2 * seg]))

        y2 = x2_ref[...] + _cat([acc[n_mem:M2], acc[RA - seg + n_mem:RA]])
        mem2 = acc[RA - seg:RA - seg + n_mem]
        if full:
            x_cur = x_ref[pl.ds(pl.multiple_of(t * seg, seg), seg), :].astype(F32)
            xb_ref[0:seg, :] = x_cur + acc[M2:M2 + seg]
            xb_ref[seg:2 * seg, :] = y2
            m1n = acc[0:n_mem]
            m2n = mem2
            ahn = AHS[(u + 1) % UNROLL]
            an = pl.multiple_of(jnp.minimum(A0 + a_off + AHS[u], S - ahn), 16)
            h_ref[RB:RB + ahn, :] = _ln(x_ref[pl.ds(an, ahn), :].astype(F32))
            nxt = x2_new
        else:
            xb_ref[pl.ds(pl.multiple_of(jnp.where(t < LAG, 0, (t - n_seg + 2) * seg), seg), seg), :] = y2
            m1n = jnp.where(t < LAG - 1, h_ref[RB + AHS[0]:RB + AHS[0] + n_mem, :], mem2)
            m2n = jnp.where(t == LAG - 1, mem0_ref[...].astype(F32), mem2)
            nxt = jnp.where(t < LAG - 1, x_ref[seg:2 * seg, :].astype(F32), x2_new)
        x2_ref[...] = nxt
        sl = _ln(nxt)
        h_ref[n_mem:M2, :] = sl[0:n_mem]
        h_ref[M2 + n_mem:RB, :] = sl[n_mem:seg]
        return _cat([m1n, m2n])

    def single_body(t, c):
        @pl.when(t >= n_seg + 2 - UNROLL)
        def _():
            out_copy(t - (LAG + 3)).start()
        return step(t, c, False)

    def full_body(i, c):
        t = LAG + UNROLL * i
        for u in range(UNROLL):
            @pl.when(t - u >= LAG + 2)
            def _():
                out_copy(t - u - (LAG + 2)).start()
        for u in range(UNROLL):
            c = step(t + u, c, True, u, i)
        return c

    def phase(ph, c):
        t0 = ph * n_seg
        c = lax.fori_loop(t0, t0 + LAG, single_body, c)

        @pl.when(ph == 0)
        def _():
            x_late.wait()
        return lax.fori_loop(0, jnp.where(ph == 0, (n_seg - LAG) // UNROLL, 0), full_body, c)
    if not SKIPM:
      lax.fori_loop(0, 2, phase, _cat([h_ref[0:n_mem, :], h_ref[M2:M2 + n_mem, :]]))

    if SKIPM:
        def keep(i, c):
            z = (w_ref[i, pl.ds(pl.multiple_of(i * 8, 8), 8), :] + ring_ref[i, pl.ds(pl.multiple_of(i * 8, 8), 8), :]
                 + wr_ref[i & 3, pl.ds(pl.multiple_of(i * 8, 8), 8), :])
            xb_ref[2 * seg:2 * seg + 8, 0:128] = pltpu.bitcast(z, F32) + h_ref[pl.ds(pl.multiple_of((i & 7) * 8, 8), 8), 0:128] + x2_ref[0:8, 0:128]
            return c
        lax.fori_loop(0, 20, keep, 0)
    out_copy(n_seg - 3).start()
    res = xb_ref[2 * seg:4 * seg, :]
    blhs = _ln(res).astype(BF16)
    ob = b_attn([(1, n_seg - 2), (1, n_seg - 1)], *[b_proj(blhs, part) for part in range(3)])
    o_store(n_seg - 2, b_out(_cat(ob), res))
    out_copy(n_seg - 2).start()
    out_copy(n_seg - 1).start()
    pltpu.make_async_copy(o_ref.at[pl.ds(seg, S), :], out_hbm, sem_o).wait()


@functools.partial(jax.jit, static_argnames=("seg",))
def _run(A_x, A_mem0, A_Wq, A_Wk, A_Wv, A_Wo, B_wqkv, B_wo, *, seg):
    _, S, dm = A_x.shape
    n_heads, dh = A_Wq.shape[1], A_Wq.shape[2]
    n_mem = A_mem0.shape[1]
    n_seg = S // seg
    hd = n_heads * dh
    nct = dm // 128
    ng = (hd // 128 - RT) // GT
    assert (seg, n_seg, n_mem, dh, dm % 128, n_heads, LAG) == (32, 64, 8, 192, 0, 32, 2)

    x = A_x.reshape(S, dm)
    mem0 = A_mem0.reshape(n_mem, dm)
    wq = jnp.transpose(A_Wq, (1, 2, 0)).reshape(hd, dm)
    wk = jnp.transpose(A_Wk, (1, 2, 0)).reshape(hd, dm)
    wv = jnp.transpose(A_Wv, (1, 2, 0)).reshape(hd, dm)
    wo = A_Wo.reshape(hd, dm)
    _, _, _, _, rs, xc = _plan(seg, n_seg)

    kern = functools.partial(_kernel, seg=seg, n_seg=n_seg, n_mem=n_mem,
                             n_heads=n_heads, dh=dh, dm=dm)
    hbm = pl.BlockSpec(memory_space=pltpu.HBM)

    out = pl.pallas_call(
        kern,
        in_specs=[hbm] * 8,
        out_specs=hbm,
        out_shape=jax.ShapeDtypeStruct((S, dm), A_x.dtype),
        scratch_shapes=[
            pltpu.VMEM((S, dm), BF16),
            pltpu.VMEM((n_mem, dm), BF16),
            pltpu.VMEM((NSLOT, 4, GT * 128, dm), BF16),
            pltpu.VMEM((4, RT * 128, dm), BF16),
            pltpu.VMEM((4, len(S53[0]) * 64, 128), U32),
            pltpu.VMEM((4 * ng, len(S55[0]) * 64, 128), U32),
            pltpu.VMEM((dm, 4 * dm + 128), BF16),
            pltpu.VMEM((nct, 5 * dm + 32, 128), F32),
            pltpu.VMEM((4 * nct + 1, dm // 2, 128), U32),
            pltpu.VMEM((len(KEYS), NXC * xc // 4, 128), U32),
            pltpu.VMEM((15, 8, 128), U32),
            pltpu.VMEM((3 * hd // 128, rs // 2 + 8, 128), U32),
            pltpu.VMEM((3 * n_mem + seg + AHS[0], dm), F32),
            pltpu.VMEM((4 * seg, dm), F32),
            pltpu.VMEM((seg, dm), F32),
            pltpu.VMEM((2, nct, HIST + seg, 128), F32),
            pltpu.VMEM((2, nct, HIST + seg, 128), F32),
            pltpu.VMEM((S + seg, dm), A_x.dtype),
            pltpu.VMEM((4, 2 * n_mem + 2 * seg, 128), F32),
            pltpu.VMEM((48, 48, 128), U32),
            pltpu.VMEM((hd // 128, 2 * n_mem + 2 * seg, 128), F32),
            pltpu.VMEM((n_heads, 2 * n_mem + 2 * seg, 128), F32),
            pltpu.SemaphoreType.DMA((NSLOT,)),
            pltpu.SemaphoreType.DMA((8 + NXC,)),
            pltpu.SemaphoreType.DMA((4,)),
            pltpu.SemaphoreType.DMA(()),
        ],
        compiler_params=pltpu.CompilerParams(
            vmem_limit_bytes=128 * 1024 * 1024,
            disable_bounds_checks=True,
        ),
    )(x, mem0, wq, wk, wv, wo, B_wqkv, B_wo)
    return out.reshape(1, S, dm)


def pallas_interleave_layers__memory_aug_recurrent_mem_tr__sliding_local_dilated__prompt_kernel(
    A_x: jax.Array,
    A_mem0: jax.Array,
    A_Wq: jax.Array,
    A_Wk: jax.Array,
    A_Wv: jax.Array,
    A_Wo: jax.Array,
    A_seg_len,
    B_x: jax.Array,
    B_wqkv: jax.Array,
    B_wo: jax.Array,
):
    del B_x
    seg = A_seg_len if isinstance(A_seg_len, int) else 32
    return _run(A_x, A_mem0, A_Wq, A_Wk, A_Wv, A_Wo, B_wqkv, B_wo, seg=seg)
```

```python
import functools

import jax
import jax.numpy as jnp
from jax import lax
import jax.experimental.pallas as pl
import jax.experimental.pallas.tpu as pltpu

F32 = jnp.float32
BF16 = jnp.bfloat16
U32 = jnp.uint32
NEG = -1000000000.0
LN_EPS = 1e-05
LOG2E = 1.4426950408889634
NEG2 = NEG * LOG2E

B_HEADS = 32
B_WIN = 8
B_DIL = 2
HIST = 16
UNROLL = int(1)
AHS = (16,) * UNROLL
LAG = 2
NSLOT = 2
NNM = '000'
NNF = '000'
WSCHED = '3:0,4:1,6:2,7:3,8:4,9:5'
BOUT_R = int(5)
ORDR = 'vkqFPS'
TAILPV = int(8)
PERT = int(1)
WPOS = int(0)
SKIPM = int(0)
MV = int(1)
PD = 's'
NNC = int(9)
MDQ = 'l'
MDW = 'l'
CW128 = int(0)
OSC = int(0)
PSC = int(0)
LATE = int(1)
KVS = int(1)
BT = int(0)
NOB = int(0)
WTT = int(1)
DORD = 'sss'
RCH = [int(v) for v in '80,80,80'.split(',')]
NXC = 6
HC = 3


def _ln(x):
    m = jnp.mean(x, axis=-1, keepdims=True)
    c = x - m
    v = jnp.mean(c * c, axis=-1, keepdims=True)
    return c * lax.rsqrt(v + LN_EPS)


def _recip(d):
    return pl.reciprocal(d, approx=True)


def _nt(a, b):
    return lax.dot_general(a, b, (((1,), (1,)), ((), ())), preferred_element_type=F32)


def _nn(a, b):
    return jnp.dot(a, b, preferred_element_type=F32)


def _cat(xs, axis=0):
    return xs[0] if len(xs) == 1 else jnp.concatenate(xs, axis=axis)


def _pk(z):
    return pltpu.bitcast(z, U32)


def _upk(z):
    return pltpu.bitcast(z, BF16)


LAM = (-1.5, -0.5, 0.0, 0.5, 1.5)


def _scheme(stars):
    tiles, prog = [], []
    for star in stars:
        if len(star) == 1:
            prog.append(("single", star[0], None, len(tiles)))
            tiles.append([star[0][:2]])
            continue
        left = [len(star) - 1] * len(star)
        for j in range(1, len(star)):
            for i in range(j):
                x, y = star[i], star[j]
                prog.append(("pair", x, y, len(tiles)))
                tiles += [[(x[0], y[1])], [(y[0], x[1])], [(x[0], y[1]), (y[0], x[1])]]
                for e in (i, j):
                    left[e] -= 1
                    if left[e] == 0:
                        z = star[e]
                        prog.append(("diag", z, None, len(tiles)))
                        tiles += [[z[:2]] + [(o[0], z[1]) for o in star if o is not z],
                                  [z[:2]] + [(z[0], o[1]) for o in star if o is not z]]
    return tiles, prog


S55 = _scheme([[(i, i, LAM[i]) for i in range(5)]])
S53 = _scheme([[(0, 0, LAM[0]), (2, 1, LAM[2]), (4, 2, LAM[4])], [(1, 0, LAM[1]), (3, 2, LAM[3])],
               [(1, 1, LAM[1])], [(3, 1, LAM[3])]])
S35 = _scheme([[(0, 0, LAM[0]), (1, 2, LAM[2]), (2, 4, LAM[4])], [(0, 1, LAM[1]), (2, 3, LAM[3])],
               [(1, 1, LAM[1])], [(1, 3, LAM[3])]])


def _reorder(prog, mode):
    pairs = [e for e in prog if e[0] != "diag"]
    diags = [e for e in prog if e[0] == "diag"]
    if mode == "l":
        return prog
    out = []
    if mode == "f":
        for e in pairs:
            for z in (e[1], e[2]):
                for dg in diags:
                    if dg[1] == z and dg not in out:
                        out.append(dg)
            out.append(e)
        return out
    step = len(pairs) / len(diags)
    k = 0
    for i, e in enumerate(pairs):
        out.append(e)
        while k < len(diags) and (k + 0.5) * step <= i + 1:
            out.append(diags[k])
            k += 1
    return out + diags[k:]


def _op_keys(prog):
    keys = []
    for kind, x, y, _ in prog:
        if kind == "pair":
            new = [(nm, x[0], x[2], y[0], y[2]) for nm in ("l1", "l2", "A")]
        else:
            new = [("a", x[0], x[2]), ("b", x[0])]
        keys += [k for k in new if k not in keys]
    return keys


def _scaled(c, u):
    return u if c == 1.0 else c * u


class _Operands:
    def __init__(self, T, U, E):
        self.T, self.U, self.E, self.memo = T, U, E, {}

    def _get(self, key, fn):
        if key not in self.memo:
            self.memo[key] = fn()
        return self.memo[key]

    def paired(self, key):
        T, U = self.T, self.U
        if key[0] == "b":
            return U[key[1]]
        if key[0] == "a":
            k, lam = key[1:]
            if lam == 0.0:
                return T[k]
            return self._get(("f",) + key, lambda: T[k] - _scaled(lam, U[k]) if lam > 0
                             else T[k] + _scaled(-lam, U[k]))
        kx, lx, ky, ly = key[1:]
        A = self._get(("f", "A") + key[1:],
                      lambda: self.paired(("a", kx, lx)) + self.paired(("a", ky, ly)))
        if key[0] == "A":
            return A
        return A - _scaled(ly - lx, U[kx]) if key[0] == "l1" else A + _scaled(ly - lx, U[ky])

    def extra(self, key):
        if key[0] == "a":
            return self.E[key[1]]
        return self._get(("e", key[1], key[3]), lambda: self.E[key[1]] + self.E[key[3]])

    def __call__(self, key):
        if self.T is None:
            ek = ("a", key[1]) if key[0] in ("a", "s") else ("l", key[1], 0, key[3])
            return self._get(ek, lambda: self.extra(ek).astype(BF16))

        def build():
            ak = ("a",) + key[1:] if key[0] == "s" else key
            parts = [self.paired(ak)]
            if self.E is not None and ak[0] in ("a", "l1", "l2"):
                parts.append(self.extra(ak))
            if key[0] == "s":
                parts.append(self.U[key[1]])
            return _cat(parts).astype(BF16)
        return self._get(key, build)


def _fast_mm(prog, op, dot, m, p, q):
    def add(d, key, val):
        d[key] = val if key not in d else d[key] + val

    for kind, x, y, i in prog:
        if kind == "pair":
            kk = (x[0], x[2], y[0], y[2])
            p1, p2 = dot(op(("l1",) + kk), i), dot(op(("l2",) + kk), i + 1)
            if m:
                r = _scaled(1.0 / (y[2] - x[2]), p2[0:m] - p1[0:m] + dot(op(("A",) + kk), i + 2))
                add(q, (x[1], x[2]), r)
                add(q, (y[1], y[2]), r)
            add(p, y[1], p1)
            add(p, x[1], p2)
        elif kind == "diag":
            add(p, x[1], dot(op(("a", x[0], x[2])), i))
            if m:
                add(q, (x[1], x[2]), dot(op(("b", x[0])), i + 1))
        else:
            r = dot(op(("s", x[0], x[2])), i)
            add(p, x[1], r[0:r.shape[0] - m])
            if m:
                add(q, (x[1], x[2]), r[r.shape[0] - m:])


def _fast_out(p, q, n, m):
    if not m:
        return None, None, p[n]
    y, z = p[n][0:m], None
    for (nn, lam), v in q.items():
        if nn == n:
            z = v if z is None else z + v
            if lam != 0.0:
                y = y + _scaled(lam, v) if lam > 0 else y - _scaled(-lam, v)
    return y, z, (p[n][m:] if p[n].shape[0] > m else None)


def _combo(tile, block):
    out = block(*tile[0])
    for kn in tile[1:]:
        out = out - block(*kn)
    return out


GT = 5
RT = 3
KEYS_R = _op_keys(S53[1])
KEYS = KEYS_R + [k for k in _op_keys(S55[1]) if k not in KEYS_R]


def _plan(seg, n_seg):
    S = seg * n_seg
    R0 = LAG * seg
    A0 = S - (n_seg - LAG) // UNROLL * sum(AHS)
    NPRE = A0 - R0 - LAG * 8
    RS = -(-(A0 - R0 + AHS[0]) // seg) * seg
    XC = NPRE // NXC // 32 * 32
    assert XC * NXC + 16 == NPRE
    return S, R0, A0, NPRE, RS, XC


def _kernel(x_hbm, mem0_hbm, wq_hbm, wk_hbm, wv_hbm, wo_hbm, bqkv_hbm, bwo_hbm,
            out_hbm,
            x_ref, mem0_ref, stage_ref, stage0_ref, wr_ref, w_ref, bst_ref, btmp_ref, bw_ref,
            xla_ref, xlb_ref, xlc_ref, xe_ref, ring_ref, h_ref, xb_ref, x2_ref, kb_ref, vb_ref, o_ref, bias_ref, kv_ref, os_ref, ps_ref,
            sem_w, sem_m, sem_b, sem_o,
            *, seg, n_seg, n_mem, n_heads, dh, dm):
    S, R0, A0, NPRE, RS, XC = _plan(seg, n_seg)
    M2 = 2 * n_mem
    R = M2 + 2 * seg
    RB = M2 + seg
    PW = 2 * dh
    G = n_heads // 2
    nct = dm // 128
    bdh = dm // B_HEADS
    NT = n_heads * dh // 128
    NG = (NT - RT) // GT
    w_hbm = (wq_hbm, wk_hbm, wv_hbm, wo_hbm)

    def w_copy(p, g):
        slot = g & (NSLOT - 1)
        return pltpu.make_async_copy(w_hbm[p].at[pl.ds((RT + (g - 1) * GT) * 128, GT * 128), :],
                                     stage_ref.at[slot, p], sem_w.at[slot])

    def w0_copy(p):
        dst = stage0_ref if p == 3 else stage_ref.at[0, p, pl.ds(0, RT * 128)]
        return pltpu.make_async_copy(w_hbm[p].at[pl.ds(0, RT * 128), :], dst, sem_m.at[4 + p])

    NB1 = 3 * nct
    WO0 = 3 * dm
    DUM = 4 * dm
    XF = A0 + AHS[0]
    XH = XC // 2

    def rows_copy(r0, n, sem):
        return pltpu.make_async_copy(x_hbm.at[pl.ds(r0, n), :], x_ref.at[pl.ds(r0, n), :], sem)

    def x_copy(i):
        return rows_copy(pl.multiple_of(R0 + i * XC, 16), XC, sem_m.at[8 + i])

    small = [rows_copy(0, R0, sem_m.at[1]), rows_copy(R0 + NPRE - 16, XF - R0 - NPRE + 16, sem_m.at[2]),
             pltpu.make_async_copy(mem0_hbm, mem0_ref, sem_m.at[3])]
    x_late = rows_copy(XF, S - XF, sem_m.at[0])

    def bq_copy(part):
        c0 = pl.multiple_of(part * dm, 128)
        return pltpu.make_async_copy(bqkv_hbm.at[:, pl.ds(c0, dm)], bst_ref.at[:, pl.ds(c0, dm)], sem_b.at[part])

    bo_copy = pltpu.make_async_copy(bwo_hbm, bst_ref.at[:, pl.ds(3 * dm, dm)], sem_b.at[3])

    def bst_tile(c):
        return bst_ref[:, pl.ds(pl.multiple_of(c * 128, 128), 128)]

    def bias_tables(full):
        RA = R if full else M2 + seg
        CW = 128
        ri = lax.broadcasted_iota(jnp.int32, (RA, CW), 0)
        ci = lax.broadcasted_iota(jnp.int32, (RA, CW), 1)
        if not full:
            ri = jnp.where(ri >= M2, ri + seg, ri)

        def table(i, bounds, vals):
            out = vals[-1]
            for b, v in zip(reversed(bounds), reversed(vals[:-1])):
                out = jnp.where(i < b, v, out)
            return out
        qi = ri - table(ri, [16, 48, 56], [0, 8, 48, 40])
        g0 = (ci < 8) | ((ci >= 16) & (ci < 48))
        k2 = ci - table(ci, [8, 24, 32, 48, 56, 80, 88, 96, 104], [-8, 0, 24, 8, 48, 40, 72, 80, 96, 104])
        if full:
            k1 = ci - table(ci, [8, 48], [0, 8, 40])
            row_l2 = ((ri >= 8) & (ri < 16)) | (ri >= 48)
            row_xa = (ri >= 8) & (ri < 16)
            valid = (row_xa == (ci >= 80)) & (ci < 112)
            is_a = jnp.where(ci >= 80, ((ci >= 88) & (ci < 104)).astype(jnp.int32),
                             (g0 != row_l2).astype(jnp.int32)) > 0
            ki = jnp.where(row_l2, k2, k1)
            visible = valid & ((qi < n_mem) | (qi >= ki))
            fill = jnp.where(valid, NEG2, -jnp.inf)
        else:
            is_a = jnp.logical_not(g0)
            visible = (qi < n_mem) | (qi >= k2)
            fill = NEG2
        for e, mine in enumerate((is_a, jnp.logical_not(is_a))):
            bias_ref[(0 if full else 2) + e, 0:RA, :] = jnp.where(
                mine, jnp.where(visible, 0.0, fill), -jnp.inf)

    for i in range(HC):
        x_copy(i).start()

    def zero_body(j, c):
        btmp_ref[j, DUM:, :] = jnp.zeros((btmp_ref.shape[1] - DUM, 128), F32)
        return c
    lax.fori_loop(0, nct, zero_body, 0)

    w0_copy(0).start()
    xb_ref[0:2 * seg, :] = jnp.zeros((2 * seg, dm), F32)
    kb_ref[...] = jnp.zeros(kb_ref.shape, F32)
    vb_ref[...] = jnp.zeros(vb_ref.shape, F32)
    bst_ref[:, 4 * dm:] = jnp.zeros((dm, 128), BF16)
    bias_tables(True)
    bias_tables(False)

    def ekey(key):
        return ("a", key[1]) if key[0] == "a" else ("l", key[1], 0, key[3])
    EKEYS = []
    for key in KEYS:
        if key[0] in ("a", "l1") and ekey(key) not in EKEYS:
            EKEYS.append(ekey(key))

    def e_ops():
        ye = _ln(x_ref[R0 + NPRE - 16:R0 + NPRE, :].astype(F32))
        eops = _Operands(None, None, [ye[:, k * 128:(k + 1) * 128] for k in range(nct)])
        for j, key in enumerate(EKEYS):
            xe_ref[j] = _pk(eops(key))

    NKR = len(KEYS_R)

    def xl(j, hf, i):
        if j >= NKR:
            ref, j, i = xlc_ref, j - NKR, hf * HC + i
        else:
            ref = (xla_ref, xlb_ref)[hf]
        r0 = i * (XH // 2)
        return ref.at[j, pl.ds(r0 if isinstance(r0, int) else pl.multiple_of(r0, 8), XH // 2)]

    def ln_ops(hf, i, lo, hi):
        y = _ln(x_ref[pl.ds(pl.multiple_of(R0 + (hf * HC + i) * XC, 16), XC), :].astype(F32))
        ops = _Operands([y[0:XH, k * 128:(k + 1) * 128] for k in range(nct)],
                        [y[XH:XC, k * 128:(k + 1) * 128] for k in range(nct)], None)
        for j in range(lo, hi):
            xl(j, hf, i)[...] = _pk(ops(KEYS[j]))

    def ln_body(i, c):
        x_copy(i).wait()

        @pl.when(i == 0)
        def _():
            x_copy(HC).start()

        @pl.when(i == 1)
        def _():
            w0_copy(1).start()
            w0_copy(2).start()

        @pl.when(i == 2)
        def _():
            x_copy(HC + 1).start()
            x_copy(HC + 2).start()
            for cp in small:
                cp.start()
        ln_ops(0, i, 0, len(KEYS_R))
        return c
    lax.fori_loop(0, HC, ln_body, 0)

    def pre_chunk(scheme, w, dst, n0, chunks):
        tiles, prog = scheme
        prog = _reorder(prog, PD)
        dot = dot_nn = lambda a, i: _nn(a, _upk(dst[i * 64:(i + 1) * 64, :]))
        if w is not None:
            raw = lambda k, n: w[n * 128:(n + 1) * 128, k * 128:(k + 1) * 128]
            tb = []
            for i, tl in enumerate(tiles):
                tb.append(raw(*tl[0]) if len(tl) == 1
                          else _combo(tl, lambda k, n: raw(k, n).astype(F32)).astype(BF16))
                dst[i * 64:(i + 1) * 64, :] = _pk(tb[i].T)
            dot = lambda a, i: _nt(a, tb[i])

        for c in chunks:
            def op(key):
                def ld(kk):
                    v = xl(KEYS.index(kk), c // HC, c % HC)[...]
                    if c == NXC - 1 and kk[0] in ("a", "l1", "l2"):
                        v = _cat([v, xe_ref[EKEYS.index(ekey(kk))]])
                    return v
                if key[0] == "s":
                    return _upk(_cat([ld(("a",) + key[1:]), ld(("b", key[1]))]))
                return _upk(ld(key))
            p, q = {}, {}
            _fast_mm(prog, op, dot_nn if c >= NNC else dot, XH, p, q)
            for n in range(len(p)):
                y, z, e = _fast_out(p, q, n, XH)
                ring_ref[n0 + n, c * XH:c * XH + XH // 2, :] = _pk(y.astype(BF16))
                ring_ref[n0 + n, c * XH + XH // 2:(c + 1) * XH, :] = _pk(z.astype(BF16))
                if e is not None:
                    ring_ref[n0 + n, NXC * XH:NXC * XH + 8, :] = _pk(e.astype(BF16))

    def init_rows():
        x0 = x_ref[0:seg, :].astype(F32)
        sl = _ln(x0)
        xt = _ln(x_ref[R0 + NPRE:XF, :].astype(F32))
        h_ref[0:n_mem, :] = xt[0:n_mem]
        h_ref[n_mem:M2, :] = sl[0:n_mem]
        h_ref[M2:M2 + n_mem, :] = mem0_ref[...].astype(F32)
        h_ref[M2 + n_mem:RB, :] = sl[n_mem:seg]
        h_ref[RB:RB + AHS[0], :] = xt[M2:M2 + AHS[0]]
        h_ref[RB + AHS[0]:RB + AHS[0] + n_mem, :] = xt[n_mem:M2]
        x2_ref[...] = x0

    def first_a(p, c):
        buf = stage_ref.at[0, p, pl.ds(0, RT * 128)]
        pltpu.make_async_copy(buf, buf, sem_m.at[4 + p]).wait()
        x_copy(HC + p).wait()

        @pl.when(p == 0)
        def _():
            for pp in range(4):
                w_copy(pp, 1).start()

        @pl.when(p == 2)
        def _():
            bq_copy(0).start()
        ln_ops(1, p, 0, len(KEYS) if MV else len(KEYS_R))
        pre_chunk(S53, buf, wr_ref.at[p], p * NT, range(HC))
        return c
    lax.fori_loop(0, 3, first_a, 0)
    for cp in small:
        cp.wait()

    def first_b(p, c):
        e_ops()
        init_rows()
        ln_ops(0, p, len(KEYS_R), len(KEYS))
        pre_chunk(S53, None, wr_ref.at[p], p * NT, range(HC, NXC))
        if not MV:
            ln_ops(1, p, len(KEYS_R), len(KEYS))
        return c
    lax.fori_loop(0, 3, first_b, 0)

    dpt = 128 // B_HEADS

    def b_stage1(u):
        ok = (u >= 0) & (u < NB1)
        tr = bst_tile(jnp.where(ok, u, NB1 + nct)).T.astype(F32) if BT & 1 else bst_tile(jnp.where(ok, u, NB1 + nct)).astype(F32).T
        r0 = pl.multiple_of(jnp.where(ok, u * 128, DUM), 128)
        for j in range(nct):
            btmp_ref[j, pl.ds(r0, 128), :] = tr[:, j * 128:(j + 1) * 128]

    def b_stage1_wo(u):
        ok = (u >= 0) & (u < nct)
        r0 = pl.multiple_of(jnp.where(ok, WO0, DUM), 128)
        btmp_ref[jnp.where(ok, u, 0), pl.ds(r0, dm), :] = bst_tile(
            jnp.where(ok, NB1 + u, NB1 + nct)).astype(F32)

    def b_stage2(u):
        ok = (u >= 0) & (u < NB1)
        part = (u >= nct).astype(jnp.int32) + (u >= 2 * nct).astype(jnp.int32)
        r0 = jnp.where(ok, part * dm + (u - part * nct) * dpt, DUM)
        rows = _cat([_cat([btmp_ref[j, pl.ds(r0 + dd, B_HEADS, stride=bdh), :]
                           for j in range(nct)], axis=1) for dd in range(dpt)])
        bw_ref[jnp.where(ok, u, NB1 + nct)] = _pk(rows.astype(BF16).T if BT & 2 else rows.T.astype(BF16))

    def b_stage2_wo(u):
        ok = (u >= 0) & (u < nct)
        r0 = jnp.where(ok, WO0, DUM)
        jj = jnp.where(ok, u, 0)
        bw_ref[jnp.where(ok, NB1 + u, NB1 + nct)] = _pk(
            _cat([btmp_ref[jj, pl.ds(r0 + d, B_HEADS, stride=bdh), :] for d in range(bdh)]).astype(BF16))

    def wo_store(scheme, w, dst):
        if WTT and scheme is S55:
            rawt = lambda k, n: w[k * 128:(k + 1) * 128, n * 128:(n + 1) * 128]
            for i, tl in enumerate(scheme[0]):
                if len(tl) == 1:
                    val = rawt(*tl[0])
                    if WTT == 3:
                        val = _upk(_pk(val.T)).T
                else:
                    val = _combo(tl, lambda k, n: rawt(k, n).astype(F32)).astype(BF16)
                    if WTT in (1, 3):
                        val = _upk(_pk(val.T)).T
                dst[i * 64:(i + 1) * 64, :] = _pk(val)
            return
        for r in range(0, 128, 16):
            memo = {}

            def raw(k, n):
                return w[k * 128 + r:k * 128 + r + 16, n * 128:(n + 1) * 128]

            def block(k, n):
                if (k, n) not in memo:
                    memo[k, n] = raw(k, n).astype(F32)
                return memo[k, n]
            for i, tl in enumerate(scheme[0]):
                val = raw(*tl[0]) if len(tl) == 1 else _combo(tl, block).astype(BF16)
                dst[i * 64 + r // 2:i * 64 + r // 2 + 8, :] = _pk(val)

    def pre_body(g, c):
        slot = g & (NSLOT - 1)
        buf = stage_ref.at[slot]
        pltpu.make_async_copy(buf, buf, sem_w.at[slot]).wait()

        @pl.when((g >= 2) & (g <= 4))
        def _():
            bq_copy(g - 2).wait()

        @pl.when(g == 4)
        def _():
            bo_copy.wait()

        @pl.when(g <= 2)
        def _():
            bq_copy(g).start()

        @pl.when(g == 2)
        def _():
            bo_copy.start()

        @pl.when(g + 1 <= NG)
        def _():
            for p in range(4):
                w_copy(p, g + 1).start()

        @pl.when(g == NG - 1)
        def _():
            w0_copy(3).start()
            x_late.start()

        if WPOS == 0:
            wo_store(S55, stage_ref.at[slot, 3], w_ref.at[3 * NG + g - 1])
        for e in range(0 if NOB else 3):
            b_stage2(3 * (g - 5) + e)
        b_stage2_wo(g - 5)
        for e in range(0 if NOB else 3):
            b_stage1(3 * (g - 2) + e)
        b_stage1_wo(g - 4)
        for p in range(3):
            pre_chunk(S55, stage_ref.at[slot, p], w_ref.at[p * NG + g - 1], p * NT + RT + (g - 1) * GT, range(NXC))
            if WPOS == p + 1:
                wo_store(S55, stage_ref.at[slot, 3], w_ref.at[3 * NG + g - 1])
        return c
    lax.fori_loop(1, NG + 1, pre_body, 0)
    w0_copy(3).wait()

    bscale = float(bdh) ** (-0.5) * LOG2E

    def b_proj(lhs, part):
        return _nn(lhs, _cat([_upk(bw_ref[part * nct + j]) for j in range(nct)], axis=1))

    def b_attn(jobs, q, k, v):
        row = lax.broadcasted_iota(jnp.int32, (seg, 128), 0)
        outs = []
        for i, (l, sidx) in enumerate(jobs):
            r0 = i * seg
            pos = row + sidx * seg
            for j in range(nct):
                kb_ref[l, j, HIST:HIST + seg, :] = k[r0:r0 + seg, j * 128:(j + 1) * 128]
                vb_ref[l, j, HIST:HIST + seg, :] = v[r0:r0 + seg, j * 128:(j + 1) * 128]
            logits = []
            for w in range(B_WIN):
                o = HIST - w * B_DIL
                acc = None
                for j in range(nct):
                    p = q[r0:r0 + seg, j * 128:(j + 1) * 128] * kb_ref[l, j, o:o + seg, :]
                    acc = p if acc is None else acc + p
                acc = acc + pltpu.roll(acc, 64, 1)
                acc = acc + pltpu.roll(acc, 32, 1)
                lg = acc * bscale
                if w > 0:
                    lg = jnp.where(pos >= w * B_DIL, lg, NEG2)
                logits.append(lg)
            m = logits[0]
            for w in range(1, B_WIN):
                m = jnp.maximum(m, logits[w])
            es = [jnp.exp2(lg - m) for lg in logits]
            den = es[0]
            for w in range(1, B_WIN):
                den = den + es[w]
            inv = _recip(den)
            cols = []
            for j in range(nct):
                acc = None
                for w in range(B_WIN):
                    o = HIST - w * B_DIL
                    p = es[w] * vb_ref[l, j, o:o + seg, :]
                    acc = p if acc is None else acc + p
                cols.append(acc * inv)
            outs.append(_cat(cols, axis=1).astype(BF16))
            for j in range(nct):
                kb_ref[l, j, 0:HIST, :] = k[r0 + seg - HIST:r0 + seg, j * 128:(j + 1) * 128]
                vb_ref[l, j, 0:HIST, :] = v[r0 + seg - HIST:r0 + seg, j * 128:(j + 1) * 128]
        return outs

    def b_out(ob, res):
        return res + _nn(ob, _cat([_upk(bw_ref[NB1 + j]) for j in range(nct)], axis=1))

    def o_store(b, val):
        ro = pl.multiple_of((b + 1) * seg, seg)
        o_ref[pl.ds(ro, val.shape[0]), :] = val.astype(o_ref.dtype)

    def out_copy(b):
        ro = pl.multiple_of(b * seg, seg)
        return pltpu.make_async_copy(o_ref.at[pl.ds(ro + seg, seg), :], out_hbm.at[pl.ds(ro, seg), :], sem_o)

    def step(t, hc, full, u=0, i=None):
        t_last = n_seg + LAG - 1
        if full:
            jobs = [(0, t - 1), (1, t - 1 - LAG)]

            def b_in():
                return xb_ref[0:2 * seg, :]
        else:
            lb = (t == t_last).astype(jnp.int32)
            jobs = [(lb, t - 1 - lb * (LAG + 1))]

            def b_in():
                return xb_ref[pl.ds(pl.multiple_of(lb * seg, seg), seg), :]
        split = full and u < UNROLL - 1
        nq = RB + AHS[u] if full else RB
        v0r = _cat([hc[0:n_mem], h_ref[n_mem:M2, :]])
        v1r = _cat([hc[n_mem:M2], h_ref[M2 + n_mem:2 * M2, :]])

        def ktiles(z):
            return [z[:, k * 128:(k + 1) * 128] for k in range(z.shape[1] // 128)]
        if full:
            hl = _Operands(ktiles(_cat([v0r, h_ref[2 * M2:RB, :]])), ktiles(_cat([v1r, h_ref[RB:RB + 16, :]])),
                           ktiles(h_ref[RB + 16:nq, :]) if nq > RB + 16 else None)
        else:
            hl = _Operands(None, None, ktiles(_cat([v0r, v1r, h_ref[2 * M2:RB, :]])))
        mh = 2 * M2 if full else 0

        def tile_dot(p, r):
            src = wr_ref.at[p] if r == 0 else w_ref.at[p * NG + r - 1]
            return lambda a, i: _nn(a, _upk(src[i * 64:(i + 1) * 64, :]))
        scale = float(dh) ** (-0.5) * LOG2E
        if full:
            s_ = t - LAG
            rd = pl.multiple_of(lax.rem(s_ * (seg // 2), RS // 2), seg // 2)
            a_off = i * sum(AHS) + sum(AHS[:u])
            wa = [pl.multiple_of(lax.rem((A0 - R0 + a_off) // 2 + 8 * a, RS // 2), 8)
                  for a in range(AHS[u] // 16)]
        else:
            wx = pl.multiple_of(jnp.where(t < LAG, NPRE // 2 + t * (n_mem // 2), RS // 2), n_mem // 2)
            wo_store(S35, stage0_ref, wr_ref.at[3])

        RA = R if full else M2 + seg
        CW = (128 if CW128 else R + 2 * M2) if full else R
        bidx = 0 if full else 2
        half = dh - 128
        la8 = lax.broadcasted_iota(jnp.int32, (n_mem, 128), 1) < half
        ones = jnp.full((n_mem, 128), 0xFFFFFFFF, U32)
        zero = jnp.zeros((n_mem, 128), U32)
        mask_a = jnp.where(la8, ones, zero)
        mask_b = jnp.where(la8, zero, ones)

        def pk2(a, b):
            return _pk(_cat([a, b]).astype(BF16))

        yt = [[None] * NT for _ in range(3)]
        x1 = [[None] * NT for _ in range(3)]

        def proj(p, r):
            pa, qa = {}, {}
            _fast_mm(_reorder((S53 if r == 0 else S55)[1], MDQ), hl, tile_dot(p, r), mh, pa, qa)
            n0 = 0 if r == 0 else RT + (r - 1) * GT
            for n in range(len(pa)):
                y, z, e = _fast_out(pa, qa, n, mh)
                idx = p * NT + n0 + n
                if full:
                    y = _cat([y[0:M2], z[0:M2], y[M2:2 * M2], z[M2:2 * M2]] + ([] if e is None else [e]))
                    for a in range(AHS[u] // 16):
                        rr = RB + 16 * a
                        ring_ref[idx, pl.ds(wa[a], 8), :] = pk2(y[rr:rr + 8], y[rr + 8:rr + 16])
                else:
                    y = e
                    ring_ref[idx, pl.ds(wx, n_mem // 2), :] = pk2(y[0:8], y[8:16])[0:n_mem // 2]
                yt[p][n0 + n] = stash(p * 16 + (n0 + n) % 16, packed(p, (n0 + n) % 3, y))
            if full and not LATE:
                for n in range(len(pa)):
                    x1[p][n0 + n] = ring_ref[p * NT + n0 + n, pl.ds(rd, seg // 2), :]

        def ab(z8):
            return jnp.where(la8, z8, 0.0), jnp.where(la8, 0.0, z8)

        def packed(p, j, y):
            u2 = pk2(y[32:40], y[40:48])
            if p == 0 or j == 0:
                return [pk2(y[0:8], y[8:16]), pk2(y[16:24], y[24:32]), u2]
            if j == 2:
                return [pk2(y[8:16], y[0:8]), pk2(y[24:32], y[16:24]), u2]
            xa_a, xa_b = ab(y[8:16])
            out = [pk2(xa_b, xa_a), pk2(y[24:32], y[16:24]) & mask_b, pk2(y[16:24], y[24:32]) & mask_a, u2]
            if full:
                out += [pk2(*ab(y[0:8])), pk2(*ab(y[16:24]))]
            return out

        def stash(idx, parts):
            if not KVS:
                return lambda: parts
            kv_ref[idx, 0:8 * len(parts), :] = _cat(parts)
            return lambda: [kv_ref[idx, 8 * e:8 * e + 8, :] for e in range(len(parts))]

        def pair(p, g):
            if full and LATE:
                xs = [ring_ref[p * NT + 3 * g + j, pl.ds(rd, seg // 2), :] for j in range(3)]
            else:
                xs = x1[p][3 * g:3 * g + 3]
            return [f() for f in yt[p][3 * g:3 * g + 3]], xs

        def q_rows(z, j):
            v0, v1, v2 = z[0][j]
            return [v0] + ([z[1][j]] if full else []) + [v1, v2]

        def kv_tiles(z):
            yt, x1 = z
            v0, v1, v2 = yt[0]
            t0 = [v0] + ([x1[0]] if full else [v1, v2]) + [v1, v2]
            w0, w1, w2 = yt[2]
            t2 = [w0, w1, w2] + ([x1[2]] if full else [w1, w2])
            if full:
                t0 += [v0, v1]
                t2 += [w0, w1]
            e1, mb, ma, u2 = yt[1][0:4]
            mid2 = [e1, mb, u2 & mask_b, ma, u2 & mask_a]
            mid1 = None
            if full:
                lo, hi = x1[1][0:8], x1[1][8:16]
                mid1 = [yt[1][4], lo & mask_a, hi & mask_a, lo & mask_b, hi & mask_b, e1, yt[1][5]]
            return t0, mid1, mid2, t2

        def mat(parts):
            return _upk(_cat(parts))

        def scores(q, k):
            k0, km1, km2, k2_ = kv_tiles(k)
            s_a = _nt(mat(q_rows(q, 0)), mat(k0))
            s_b = _nt(mat(q_rows(q, 2)), mat(k2_))
            qm = q_rows(q, 1)
            if full:
                s_m = _cat([_nt(mat(qm[0:2]), mat(km1)), _nt(mat(qm[2:4]), mat(km2 + km1[5:]))])
            else:
                s_m = _nt(mat(qm), mat(km2))
            out = []
            for e, sx in enumerate((s_a, s_b)):
                s = (sx + s_m) * scale + bias_ref[bidx + e, 0:RA, 0:CW]
                ex = jnp.exp2(s - jnp.max(s, axis=-1, keepdims=True))
                out.append(ex * _recip(jnp.sum(ex, axis=-1, keepdims=True)))
            if PSC:
                idx = 2 * len(probs)
                for e in range(2):
                    ps_ref[idx + e, 0:RA, 0:CW] = out[e]
                return lambda: [ps_ref[idx + e, 0:RA, 0:CW] for e in range(2)]
            return lambda: out

        def pv(p, v):
            p = p()
            v0, vm1, vm2, v2 = kv_tiles(v)
            o_a = _nn(p[0].astype(BF16), mat(v0))
            o_b = _nn(p[1].astype(BF16), mat(v2))
            p = p[0] + p[1]
            if full:
                o_m = _cat([_nn(p[0:M2 + seg].astype(BF16), mat(vm1)),
                            _nn(p[M2 + seg:R, 0:R].astype(BF16), mat(vm2))])
            else:
                o_m = _nn(p.astype(BF16), mat(vm2))
            out = []
            for o in (o_a, o_m, o_b):
                if OSC:
                    idx = len(ot) + len(out)
                    os_ref[idx, 0:RA, :] = o
                    out.append(functools.partial(lambda i: os_ref[i, 0:RA, :], idx))
                else:
                    out.append(functools.partial(lambda z: z, o))
            return out

        ot = []
        pacc, qacc = {}, {}

        def add_o(r):
            n0 = 0 if r == 0 else RT + (r - 1) * GT
            oo = [f() for f in ot[n0:n0 + (RT if r == 0 else GT)]]
            if full:
                ops = _Operands([o[0:32] for o in oo], [_cat([o[48:64], o[32:48]]) for o in oo],
                                [o[64:80] for o in oo])
            else:
                ops = _Operands(None, None, oo)
            _fast_mm(_reorder((S35 if r == 0 else S55)[1], MDW), ops, tile_dot(3, r), mh, pacc, qacc)

        wsched = dict(tuple(int(v) for v in e.split(":")) for e in WSCHED.split(","))
        bqkv = [None] * 3
        probs = []
        x2_new = None

        def do_pv():
            for g in range(len(ot) // 3, len(probs)):
                ot.extend(pv(probs[g], pair(2, g)))

        for r in range(NG + 1):
            npr = len(probs)
            for ch in ORDR:
                if ch in 'qkv':
                    proj('qkv'.index(ch), r)
                elif ch == 'P':
                    for g in range(len(ot) // 3, npr):
                        ot.extend(pv(probs[g], pair(2, g)))
                elif ch == 'S':
                    for g in range(len(probs), (RT + r * GT) // 3):
                        probs.append(scores(pair(0, g), pair(1, g)))
                else:
                    if r == 0:
                        blhs = _ln(b_in()).astype(BF16)
                    if r < 3:
                        bqkv[2 - r] = b_proj(blhs, 2 - r)
                    if r == 3:
                        ob = b_attn(jobs, *bqkv)
                    if r == BOUT_R:
                        res = b_in()
                        if split:
                            x2_new = b_out(ob[0], res[0:seg])
                        elif full:
                            zb = b_out(_cat(ob), res)
                            x2_new = zb[0:seg]
                            o_store(t - 1 - LAG, zb[seg:2 * seg])
                        else:
                            x2_new = b_out(ob[0], res)
                            o_store(lb * (t_last - LAG - 1) - 1, x2_new)
                    if r in wsched:
                        add_o(wsched[r])
        for r in range(len(wsched), TAILPV):
            add_o(r)
        do_pv()
        for r in range(max(TAILPV, len(wsched)), NG + 1):
            add_o(r)
        cols = []
        for n in range(nct):
            y, z, e = _fast_out(pacc, qacc, n, mh)
            cols.append(_cat([y, z[16:32], z[0:16], e]) if full else e)
        acc = _cat(cols, axis=1)
        if split:
            o_store(t - 1 - LAG, b_out(ob[1], res[seg:2 * seg]))

        y2 = x2_ref[...] + _cat([acc[n_mem:M2], acc[RA - seg + n_mem:RA]])
        mem2 = acc[RA - seg:RA - seg + n_mem]
        if full:
            x_cur = x_ref[pl.ds(pl.multiple_of(t * seg, seg), seg), :].astype(F32)
            xb_ref[0:seg, :] = x_cur + acc[M2:M2 + seg]
            xb_ref[seg:2 * seg, :] = y2
            m1n = acc[0:n_mem]
            m2n = mem2
            ahn = AHS[(u + 1) % UNROLL]
            an = pl.multiple_of(jnp.minimum(A0 + a_off + AHS[u], S - ahn), 16)
            h_ref[RB:RB + ahn, :] = _ln(x_ref[pl.ds(an, ahn), :].astype(F32))
            nxt = x2_new
        else:
            xb_ref[pl.ds(pl.multiple_of(jnp.where(t < LAG, 0, (t - n_seg + 2) * seg), seg), seg), :] = y2
            m1n = jnp.where(t < LAG - 1, h_ref[RB + AHS[0]:RB + AHS[0] + n_mem, :], mem2)
            m2n = jnp.where(t == LAG - 1, mem0_ref[...].astype(F32), mem2)
            nxt = jnp.where(t < LAG - 1, x_ref[seg:2 * seg, :].astype(F32), x2_new)
        x2_ref[...] = nxt
        sl = _ln(nxt)
        h_ref[n_mem:M2, :] = sl[0:n_mem]
        h_ref[M2 + n_mem:RB, :] = sl[n_mem:seg]
        return _cat([m1n, m2n])

    def single_body(t, c):
        @pl.when(t >= n_seg + 2 - UNROLL)
        def _():
            out_copy(t - (LAG + 3)).start()
        return step(t, c, False)

    def full_body(i, c):
        t = LAG + UNROLL * i
        for u in range(UNROLL):
            @pl.when(t - u >= LAG + 2)
            def _():
                out_copy(t - u - (LAG + 2)).start()
        for u in range(UNROLL):
            c = step(t + u, c, True, u, i)
        return c

    def phase(ph, c):
        t0 = ph * n_seg
        c = lax.fori_loop(t0, t0 + LAG, single_body, c)

        @pl.when(ph == 0)
        def _():
            x_late.wait()
        return lax.fori_loop(0, jnp.where(ph == 0, (n_seg - LAG) // UNROLL, 0), full_body, c)
    if not SKIPM:
      lax.fori_loop(0, 2, phase, _cat([h_ref[0:n_mem, :], h_ref[M2:M2 + n_mem, :]]))

    if SKIPM:
        def keep(i, c):
            z = (w_ref[i, pl.ds(pl.multiple_of(i * 8, 8), 8), :] + ring_ref[i, pl.ds(pl.multiple_of(i * 8, 8), 8), :]
                 + wr_ref[i & 3, pl.ds(pl.multiple_of(i * 8, 8), 8), :])
            xb_ref[2 * seg:2 * seg + 8, 0:128] = pltpu.bitcast(z, F32) + h_ref[pl.ds(pl.multiple_of((i & 7) * 8, 8), 8), 0:128] + x2_ref[0:8, 0:128]
            return c
        lax.fori_loop(0, 20, keep, 0)
    out_copy(n_seg - 3).start()
    res = xb_ref[2 * seg:4 * seg, :]
    blhs = _ln(res).astype(BF16)
    ob = b_attn([(1, n_seg - 2), (1, n_seg - 1)], *[b_proj(blhs, part) for part in range(3)])
    o_store(n_seg - 2, b_out(_cat(ob), res))
    out_copy(n_seg - 2).start()
    out_copy(n_seg - 1).start()
    pltpu.make_async_copy(o_ref.at[pl.ds(seg, S), :], out_hbm, sem_o).wait()


@functools.partial(jax.jit, static_argnames=("seg",))
def _run(A_x, A_mem0, A_Wq, A_Wk, A_Wv, A_Wo, B_wqkv, B_wo, *, seg):
    _, S, dm = A_x.shape
    n_heads, dh = A_Wq.shape[1], A_Wq.shape[2]
    n_mem = A_mem0.shape[1]
    n_seg = S // seg
    hd = n_heads * dh
    nct = dm // 128
    ng = (hd // 128 - RT) // GT
    assert (seg, n_seg, n_mem, dh, dm % 128, n_heads, LAG) == (32, 64, 8, 192, 0, 32, 2)

    x = A_x.reshape(S, dm)
    mem0 = A_mem0.reshape(n_mem, dm)
    wq = jnp.transpose(A_Wq, (1, 2, 0)).reshape(hd, dm)
    wk = jnp.transpose(A_Wk, (1, 2, 0)).reshape(hd, dm)
    wv = jnp.transpose(A_Wv, (1, 2, 0)).reshape(hd, dm)
    wo = A_Wo.reshape(hd, dm)
    _, _, _, _, rs, xc = _plan(seg, n_seg)

    kern = functools.partial(_kernel, seg=seg, n_seg=n_seg, n_mem=n_mem,
                             n_heads=n_heads, dh=dh, dm=dm)
    hbm = pl.BlockSpec(memory_space=pltpu.HBM)

    out = pl.pallas_call(
        kern,
        in_specs=[hbm] * 8,
        out_specs=hbm,
        out_shape=jax.ShapeDtypeStruct((S, dm), A_x.dtype),
        scratch_shapes=[
            pltpu.VMEM((S, dm), BF16),
            pltpu.VMEM((n_mem, dm), BF16),
            pltpu.VMEM((NSLOT, 4, GT * 128, dm), BF16),
            pltpu.VMEM((RT * 128, dm), BF16),
            pltpu.VMEM((4, len(S53[0]) * 64, 128), U32),
            pltpu.VMEM((4 * ng, len(S55[0]) * 64, 128), U32),
            pltpu.VMEM((dm, 4 * dm + 128), BF16),
            pltpu.VMEM((nct, 5 * dm + 32, 128), F32),
            pltpu.VMEM((4 * nct + 1, dm // 2, 128), U32),
            pltpu.VMEM((len(KEYS_R), HC * xc // 4, 128), U32),
            pltpu.VMEM((len(KEYS_R), HC * xc // 4, 128), U32),
            pltpu.VMEM((len(KEYS) - len(KEYS_R), NXC * xc // 4, 128), U32),
            pltpu.VMEM((15, 8, 128), U32),
            pltpu.VMEM((3 * hd // 128, rs // 2 + 8, 128), U32),
            pltpu.VMEM((3 * n_mem + seg + AHS[0], dm), F32),
            pltpu.VMEM((4 * seg, dm), F32),
            pltpu.VMEM((seg, dm), F32),
            pltpu.VMEM((2, nct, HIST + seg, 128), F32),
            pltpu.VMEM((2, nct, HIST + seg, 128), F32),
            pltpu.VMEM((S + seg, dm), A_x.dtype),
            pltpu.VMEM((4, 2 * n_mem + 2 * seg, 128), F32),
            pltpu.VMEM((48, 48, 128), U32),
            pltpu.VMEM((hd // 128, 2 * n_mem + 2 * seg, 128), F32),
            pltpu.VMEM((n_heads, 2 * n_mem + 2 * seg, 128), F32),
            pltpu.SemaphoreType.DMA((NSLOT,)),
            pltpu.SemaphoreType.DMA((8 + NXC,)),
            pltpu.SemaphoreType.DMA((4,)),
            pltpu.SemaphoreType.DMA(()),
        ],
        compiler_params=pltpu.CompilerParams(
            vmem_limit_bytes=128 * 1024 * 1024,
            disable_bounds_checks=True,
        ),
    )(x, mem0, wq, wk, wv, wo, B_wqkv, B_wo)
    return out.reshape(1, S, dm)


def pallas_interleave_layers__memory_aug_recurrent_mem_tr__sliding_local_dilated__prompt_kernel(
    A_x: jax.Array,
    A_mem0: jax.Array,
    A_Wq: jax.Array,
    A_Wk: jax.Array,
    A_Wv: jax.Array,
    A_Wo: jax.Array,
    A_seg_len,
    B_x: jax.Array,
    B_wqkv: jax.Array,
    B_wo: jax.Array,
):
    del B_x
    seg = A_seg_len if isinstance(A_seg_len, int) else 32
    return _run(A_x, A_mem0, A_Wq, A_Wk, A_Wv, A_Wo, B_wqkv, B_wo, seg=seg)
```

```python
import functools

import jax
import jax.numpy as jnp
from jax import lax
import jax.experimental.pallas as pl
import jax.experimental.pallas.tpu as pltpu

F32 = jnp.float32
BF16 = jnp.bfloat16
U32 = jnp.uint32
NEG = -1000000000.0
LN_EPS = 1e-05
LOG2E = 1.4426950408889634
NEG2 = NEG * LOG2E

B_HEADS = 32
B_WIN = 8
B_DIL = 2
HIST = 16
AH = 16
LAG = 2
NSLOT = 2
NXC = 6
HC = 3
WSCHED = {3: 0, 4: 1, 6: 2, 7: 3, 8: 4, 9: 5}
BOUT_R = 5
TAILPV = 8


def _ln(x):
    m = jnp.mean(x, axis=-1, keepdims=True)
    c = x - m
    v = jnp.mean(c * c, axis=-1, keepdims=True)
    return c * lax.rsqrt(v + LN_EPS)


def _recip(d):
    return pl.reciprocal(d, approx=True)


def _nt(a, b):
    return lax.dot_general(a, b, (((1,), (1,)), ((), ())), preferred_element_type=F32)


def _nn(a, b):
    return jnp.dot(a, b, preferred_element_type=F32)


def _cat(xs, axis=0):
    return xs[0] if len(xs) == 1 else jnp.concatenate(xs, axis=axis)


def _pk(z):
    return pltpu.bitcast(z, U32)


def _upk(z):
    return pltpu.bitcast(z, BF16)


LAM = (-1.5, -0.5, 0.0, 0.5, 1.5)


def _scheme(stars):
    tiles, prog = [], []
    for star in stars:
        if len(star) == 1:
            prog.append(("single", star[0], None, len(tiles)))
            tiles.append([star[0][:2]])
            continue
        left = [len(star) - 1] * len(star)
        for j in range(1, len(star)):
            for i in range(j):
                x, y = star[i], star[j]
                prog.append(("pair", x, y, len(tiles)))
                tiles += [[(x[0], y[1])], [(y[0], x[1])], [(x[0], y[1]), (y[0], x[1])]]
                for e in (i, j):
                    left[e] -= 1
                    if left[e] == 0:
                        z = star[e]
                        prog.append(("diag", z, None, len(tiles)))
                        tiles += [[z[:2]] + [(o[0], z[1]) for o in star if o is not z],
                                  [z[:2]] + [(z[0], o[1]) for o in star if o is not z]]
    return tiles, prog


S55 = _scheme([[(i, i, LAM[i]) for i in range(5)]])
S53 = _scheme([[(0, 0, LAM[0]), (2, 1, LAM[2]), (4, 2, LAM[4])], [(1, 0, LAM[1]), (3, 2, LAM[3])],
               [(1, 1, LAM[1])], [(3, 1, LAM[3])]])
S35 = _scheme([[(0, 0, LAM[0]), (1, 2, LAM[2]), (2, 4, LAM[4])], [(0, 1, LAM[1]), (2, 3, LAM[3])],
               [(1, 1, LAM[1])], [(1, 3, LAM[3])]])


def _spread(prog):
    pairs = [e for e in prog if e[0] != "diag"]
    diags = [e for e in prog if e[0] == "diag"]
    out, k = [], 0
    for i, e in enumerate(pairs):
        out.append(e)
        while k < len(diags) and (k + 0.5) * len(pairs) <= (i + 1) * len(diags):
            out.append(diags[k])
            k += 1
    return out + diags[k:]


def _op_keys(prog):
    keys = []
    for kind, x, y, _ in prog:
        if kind == "pair":
            new = [(nm, x[0], x[2], y[0], y[2]) for nm in ("l1", "l2", "A")]
        else:
            new = [("a", x[0], x[2]), ("b", x[0])]
        keys += [k for k in new if k not in keys]
    return keys


def _scaled(c, u):
    return u if c == 1.0 else c * u


class _Operands:
    def __init__(self, T, U, E):
        self.T, self.U, self.E, self.memo = T, U, E, {}

    def _get(self, key, fn):
        if key not in self.memo:
            self.memo[key] = fn()
        return self.memo[key]

    def paired(self, key):
        T, U = self.T, self.U
        if key[0] == "b":
            return U[key[1]]
        if key[0] == "a":
            k, lam = key[1:]
            if lam == 0.0:
                return T[k]
            return self._get(("f",) + key, lambda: T[k] - _scaled(lam, U[k]) if lam > 0
                             else T[k] + _scaled(-lam, U[k]))
        kx, lx, ky, ly = key[1:]
        A = self._get(("f", "A") + key[1:],
                      lambda: self.paired(("a", kx, lx)) + self.paired(("a", ky, ly)))
        if key[0] == "A":
            return A
        return A - _scaled(ly - lx, U[kx]) if key[0] == "l1" else A + _scaled(ly - lx, U[ky])

    def extra(self, key):
        if key[0] == "a":
            return self.E[key[1]]
        return self._get(("e", key[1], key[3]), lambda: self.E[key[1]] + self.E[key[3]])

    def __call__(self, key):
        if self.T is None:
            ek = ("a", key[1]) if key[0] in ("a", "s") else ("l", key[1], 0, key[3])
            return self._get(ek, lambda: self.extra(ek).astype(BF16))

        def build():
            ak = ("a",) + key[1:] if key[0] == "s" else key
            parts = [self.paired(ak)]
            if self.E is not None and ak[0] in ("a", "l1", "l2"):
                parts.append(self.extra(ak))
            if key[0] == "s":
                parts.append(self.U[key[1]])
            return _cat(parts).astype(BF16)
        return self._get(key, build)


def _fast_mm(prog, op, dot, m, p, q):
    def add(d, key, val):
        d[key] = val if key not in d else d[key] + val

    for kind, x, y, i in prog:
        if kind == "pair":
            kk = (x[0], x[2], y[0], y[2])
            p1, p2 = dot(op(("l1",) + kk), i), dot(op(("l2",) + kk), i + 1)
            if m:
                r = _scaled(1.0 / (y[2] - x[2]), p2[0:m] - p1[0:m] + dot(op(("A",) + kk), i + 2))
                add(q, (x[1], x[2]), r)
                add(q, (y[1], y[2]), r)
            add(p, y[1], p1)
            add(p, x[1], p2)
        elif kind == "diag":
            add(p, x[1], dot(op(("a", x[0], x[2])), i))
            if m:
                add(q, (x[1], x[2]), dot(op(("b", x[0])), i + 1))
        else:
            r = dot(op(("s", x[0], x[2])), i)
            add(p, x[1], r[0:r.shape[0] - m])
            if m:
                add(q, (x[1], x[2]), r[r.shape[0] - m:])


def _fast_out(p, q, n, m):
    if not m:
        return None, None, p[n]
    y, z = p[n][0:m], None
    for (nn, lam), v in q.items():
        if nn == n:
            z = v if z is None else z + v
            if lam != 0.0:
                y = y + _scaled(lam, v) if lam > 0 else y - _scaled(-lam, v)
    return y, z, (p[n][m:] if p[n].shape[0] > m else None)


def _combo(tile, block):
    out = block(*tile[0])
    for kn in tile[1:]:
        out = out - block(*kn)
    return out


GT = 5
RT = 3
KEYS_R = _op_keys(S53[1])
KEYS = KEYS_R + [k for k in _op_keys(S55[1]) if k not in KEYS_R]


def _plan(seg, n_seg):
    S = seg * n_seg
    R0 = LAG * seg
    A0 = S - (n_seg - LAG) * AH
    NPRE = A0 - R0 - LAG * 8
    RS = -(-(A0 - R0 + AH) // seg) * seg
    XC = NPRE // NXC // 32 * 32
    assert XC * NXC + 16 == NPRE
    return S, R0, A0, NPRE, RS, XC


def _kernel(x_hbm, mem0_hbm, wq_hbm, wk_hbm, wv_hbm, wo_hbm, bqkv_hbm, bwo_hbm,
            out_hbm,
            x_ref, mem0_ref, stage_ref, stage0_ref, wr_ref, w_ref, bst_ref, btmp_ref, bw_ref,
            xla_ref, xlb_ref, xlc_ref, xe_ref, ring_ref, h_ref, xb_ref, x2_ref, kb_ref, vb_ref, o_ref, bias_ref, kv_ref,
            sem_w, sem_m, sem_b, sem_o,
            *, seg, n_seg, n_mem, n_heads, dh, dm):
    S, R0, A0, NPRE, RS, XC = _plan(seg, n_seg)
    M2 = 2 * n_mem
    R = M2 + 2 * seg
    RB = M2 + seg
    PW = 2 * dh
    G = n_heads // 2
    nct = dm // 128
    bdh = dm // B_HEADS
    NT = n_heads * dh // 128
    NG = (NT - RT) // GT
    w_hbm = (wq_hbm, wk_hbm, wv_hbm, wo_hbm)

    def w_copy(p, g):
        slot = g & (NSLOT - 1)
        return pltpu.make_async_copy(w_hbm[p].at[pl.ds((RT + (g - 1) * GT) * 128, GT * 128), :],
                                     stage_ref.at[slot, p], sem_w.at[slot])

    def w0_copy(p):
        dst = stage0_ref if p == 3 else stage_ref.at[0, p, pl.ds(0, RT * 128)]
        return pltpu.make_async_copy(w_hbm[p].at[pl.ds(0, RT * 128), :], dst, sem_m.at[4 + p])

    NB1 = 3 * nct
    WO0 = 3 * dm
    XF = A0 + AH
    XH = XC // 2

    def rows_copy(r0, n, sem):
        return pltpu.make_async_copy(x_hbm.at[pl.ds(r0, n), :], x_ref.at[pl.ds(r0, n), :], sem)

    def x_copy(i):
        return rows_copy(pl.multiple_of(R0 + i * XC, 16), XC, sem_m.at[8 + i])

    small = [rows_copy(0, R0, sem_m.at[1]), rows_copy(R0 + NPRE - 16, XF - R0 - NPRE + 16, sem_m.at[2]),
             pltpu.make_async_copy(mem0_hbm, mem0_ref, sem_m.at[3])]
    x_late = rows_copy(XF, S - XF, sem_m.at[0])

    def bq_copy(part):
        c0 = pl.multiple_of(part * dm, 128)
        return pltpu.make_async_copy(bqkv_hbm.at[:, pl.ds(c0, dm)], bst_ref.at[:, pl.ds(c0, dm)], sem_b.at[part])

    bo_copy = pltpu.make_async_copy(bwo_hbm, bst_ref.at[:, pl.ds(3 * dm, dm)], sem_b.at[3])

    def bst_tile(c):
        return bst_ref[:, pl.ds(pl.multiple_of(c * 128, 128), 128)]

    def bias_tables(full):
        RA = R if full else M2 + seg
        CW = 128
        ri = lax.broadcasted_iota(jnp.int32, (RA, CW), 0)
        ci = lax.broadcasted_iota(jnp.int32, (RA, CW), 1)
        if not full:
            ri = jnp.where(ri >= M2, ri + seg, ri)

        def table(i, bounds, vals):
            out = vals[-1]
            for b, v in zip(reversed(bounds), reversed(vals[:-1])):
                out = jnp.where(i < b, v, out)
            return out
        qi = ri - table(ri, [16, 48, 56], [0, 8, 48, 40])
        g0 = (ci < 8) | ((ci >= 16) & (ci < 48))
        k2 = ci - table(ci, [8, 24, 32, 48, 56, 80, 88, 96, 104], [-8, 0, 24, 8, 48, 40, 72, 80, 96, 104])
        if full:
            k1 = ci - table(ci, [8, 48], [0, 8, 40])
            row_l2 = ((ri >= 8) & (ri < 16)) | (ri >= 48)
            row_xa = (ri >= 8) & (ri < 16)
            valid = (row_xa == (ci >= 80)) & (ci < 112)
            is_a = jnp.where(ci >= 80, ((ci >= 88) & (ci < 104)).astype(jnp.int32),
                             (g0 != row_l2).astype(jnp.int32)) > 0
            ki = jnp.where(row_l2, k2, k1)
            visible = valid & ((qi < n_mem) | (qi >= ki))
            fill = jnp.where(valid, NEG2, -jnp.inf)
        else:
            is_a = jnp.logical_not(g0)
            visible = (qi < n_mem) | (qi >= k2)
            fill = NEG2
        for e, mine in enumerate((is_a, jnp.logical_not(is_a))):
            bias_ref[(0 if full else 2) + e, 0:RA, :] = jnp.where(
                mine, jnp.where(visible, 0.0, fill), -jnp.inf)

    for i in range(HC):
        x_copy(i).start()

    def zero_body(j, c):
        btmp_ref[j, 0:dm, :] = jnp.zeros((dm, 128), F32)
        return c
    lax.fori_loop(0, nct, zero_body, 0)

    w0_copy(0).start()
    xb_ref[0:2 * seg, :] = jnp.zeros((2 * seg, dm), F32)
    kb_ref[...] = jnp.zeros(kb_ref.shape, F32)
    vb_ref[...] = jnp.zeros(vb_ref.shape, F32)
    bst_ref[:, 4 * dm:] = jnp.zeros((dm, 128), BF16)
    bias_tables(True)
    bias_tables(False)

    def ekey(key):
        return ("a", key[1]) if key[0] == "a" else ("l", key[1], 0, key[3])
    EKEYS = []
    for key in KEYS:
        if key[0] in ("a", "l1") and ekey(key) not in EKEYS:
            EKEYS.append(ekey(key))

    def e_ops():
        ye = _ln(x_ref[R0 + NPRE - 16:R0 + NPRE, :].astype(F32))
        eops = _Operands(None, None, [ye[:, k * 128:(k + 1) * 128] for k in range(nct)])
        for j, key in enumerate(EKEYS):
            xe_ref[j] = _pk(eops(key))

    NKR = len(KEYS_R)

    def xl(j, hf, i):
        if j >= NKR:
            ref, j, i = xlc_ref, j - NKR, hf * HC + i
        else:
            ref = (xla_ref, xlb_ref)[hf]
        r0 = i * (XH // 2)
        return ref.at[j, pl.ds(r0 if isinstance(r0, int) else pl.multiple_of(r0, 8), XH // 2)]

    def ln_ops(hf, i, lo, hi):
        y = _ln(x_ref[pl.ds(pl.multiple_of(R0 + (hf * HC + i) * XC, 16), XC), :].astype(F32))
        ops = _Operands([y[0:XH, k * 128:(k + 1) * 128] for k in range(nct)],
                        [y[XH:XC, k * 128:(k + 1) * 128] for k in range(nct)], None)
        for j in range(lo, hi):
            xl(j, hf, i)[...] = _pk(ops(KEYS[j]))

    def ln_body(i, c):
        x_copy(i).wait()

        @pl.when(i == 0)
        def _():
            x_copy(HC).start()

        @pl.when(i == 1)
        def _():
            w0_copy(1).start()
            w0_copy(2).start()

        @pl.when(i == 2)
        def _():
            x_copy(HC + 1).start()
            x_copy(HC + 2).start()
            for cp in small:
                cp.start()
        ln_ops(0, i, 0, len(KEYS_R))
        return c
    lax.fori_loop(0, HC, ln_body, 0)

    def pre_chunk(scheme, w, dst, n0, chunks):
        tiles, prog = scheme
        prog = _spread(prog)
        dot = lambda a, i: _nn(a, _upk(dst[i * 64:(i + 1) * 64, :]))
        if w is not None:
            raw = lambda k, n: w[n * 128:(n + 1) * 128, k * 128:(k + 1) * 128]
            tb = []
            for i, tl in enumerate(tiles):
                tb.append(raw(*tl[0]) if len(tl) == 1
                          else _combo(tl, lambda k, n: raw(k, n).astype(F32)).astype(BF16))
                dst[i * 64:(i + 1) * 64, :] = _pk(tb[i].T)
            dot = lambda a, i: _nt(a, tb[i])

        for c in chunks:
            def op(key):
                def ld(kk):
                    v = xl(KEYS.index(kk), c // HC, c % HC)[...]
                    if c == NXC - 1 and kk[0] in ("a", "l1", "l2"):
                        v = _cat([v, xe_ref[EKEYS.index(ekey(kk))]])
                    return v
                if key[0] == "s":
                    return _upk(_cat([ld(("a",) + key[1:]), ld(("b", key[1]))]))
                return _upk(ld(key))
            p, q = {}, {}
            _fast_mm(prog, op, dot, XH, p, q)
            for n in range(len(p)):
                y, z, e = _fast_out(p, q, n, XH)
                ring_ref[n0 + n, c * XH:c * XH + XH // 2, :] = _pk(y.astype(BF16))
                ring_ref[n0 + n, c * XH + XH // 2:(c + 1) * XH, :] = _pk(z.astype(BF16))
                if e is not None:
                    ring_ref[n0 + n, NXC * XH:NXC * XH + 8, :] = _pk(e.astype(BF16))

    def init_rows():
        x0 = x_ref[0:seg, :].astype(F32)
        sl = _ln(x0)
        xt = _ln(x_ref[R0 + NPRE:XF, :].astype(F32))
        h_ref[0:n_mem, :] = xt[0:n_mem]
        h_ref[n_mem:M2, :] = sl[0:n_mem]
        h_ref[M2:M2 + n_mem, :] = mem0_ref[...].astype(F32)
        h_ref[M2 + n_mem:RB, :] = sl[n_mem:seg]
        h_ref[RB:RB + AH, :] = xt[M2:M2 + AH]
        h_ref[RB + AH:RB + AH + n_mem, :] = xt[n_mem:M2]
        x2_ref[...] = x0

    def first_a(p, c):
        buf = stage_ref.at[0, p, pl.ds(0, RT * 128)]
        pltpu.make_async_copy(buf, buf, sem_m.at[4 + p]).wait()
        x_copy(HC + p).wait()

        @pl.when(p == 0)
        def _():
            for pp in range(4):
                w_copy(pp, 1).start()

        @pl.when(p == 2)
        def _():
            bq_copy(0).start()
        ln_ops(1, p, 0, len(KEYS))
        pre_chunk(S53, buf, wr_ref.at[p], p * NT, range(HC))
        return c
    lax.fori_loop(0, 3, first_a, 0)
    for cp in small:
        cp.wait()

    def first_b(p, c):
        e_ops()
        init_rows()
        ln_ops(0, p, len(KEYS_R), len(KEYS))
        pre_chunk(S53, None, wr_ref.at[p], p * NT, range(HC, NXC))
        return c
    lax.fori_loop(0, 3, first_b, 0)

    dpt = 128 // B_HEADS

    def b_stage1(u):
        uc = jnp.clip(u, 0, NB1 - 1)
        tr = bst_tile(jnp.where(u >= 0, uc, NB1 + nct)).astype(F32).T
        r0 = pl.multiple_of(uc * 128, 128)
        for j in range(nct):
            btmp_ref[j, pl.ds(r0, 128), :] = tr[:, j * 128:(j + 1) * 128]

    def b_stage1_wo(u):
        uc = jnp.clip(u, 0, nct - 1)
        btmp_ref[uc, WO0:WO0 + dm, :] = bst_tile(jnp.where(u >= 0, NB1 + uc, NB1 + nct)).astype(F32)

    def b_stage2(u):
        uc = jnp.clip(u, 0, NB1 - 1)
        part = (uc >= nct).astype(jnp.int32) + (uc >= 2 * nct).astype(jnp.int32)
        r0 = part * dm + (uc - part * nct) * dpt
        rows = _cat([_cat([btmp_ref[j, pl.ds(r0 + dd, B_HEADS, stride=bdh), :]
                           for j in range(nct)], axis=1) for dd in range(dpt)])
        bw_ref[uc] = _pk(rows.T.astype(BF16))

    def b_stage2_wo(u):
        uc = jnp.clip(u, 0, nct - 1)
        r0 = jnp.where(u >= 0, WO0, 0)
        bw_ref[NB1 + uc] = _pk(
            _cat([btmp_ref[uc, pl.ds(r0 + d, B_HEADS, stride=bdh), :] for d in range(bdh)]).astype(BF16))

    def wo_store(scheme, w, dst):
        if scheme is S55:
            rawt = lambda k, n: w[k * 128:(k + 1) * 128, n * 128:(n + 1) * 128]
            for i, tl in enumerate(scheme[0]):
                if len(tl) == 1:
                    val = rawt(*tl[0])
                else:
                    val = _combo(tl, lambda k, n: rawt(k, n).astype(F32)).astype(BF16)
                    val = _upk(_pk(val.T)).T
                dst[i * 64:(i + 1) * 64, :] = _pk(val)
            return
        for r in range(0, 128, 16):
            memo = {}

            def raw(k, n):
                return w[k * 128 + r:k * 128 + r + 16, n * 128:(n + 1) * 128]

            def block(k, n):
                if (k, n) not in memo:
                    memo[k, n] = raw(k, n).astype(F32)
                return memo[k, n]
            for i, tl in enumerate(scheme[0]):
                val = raw(*tl[0]) if len(tl) == 1 else _combo(tl, block).astype(BF16)
                dst[i * 64 + r // 2:i * 64 + r // 2 + 8, :] = _pk(val)

    def pre_body(g, c):
        slot = g & (NSLOT - 1)
        buf = stage_ref.at[slot]
        pltpu.make_async_copy(buf, buf, sem_w.at[slot]).wait()

        @pl.when((g >= 2) & (g <= 4))
        def _():
            bq_copy(g - 2).wait()

        @pl.when(g == 4)
        def _():
            bo_copy.wait()

        @pl.when(g <= 2)
        def _():
            bq_copy(g).start()

        @pl.when(g == 2)
        def _():
            bo_copy.start()

        @pl.when(g + 1 <= NG)
        def _():
            for p in range(4):
                w_copy(p, g + 1).start()

        @pl.when(g == NG - 1)
        def _():
            w0_copy(3).start()
            x_late.start()

        wo_store(S55, stage_ref.at[slot, 3], w_ref.at[3 * NG + g - 1])
        for e in range(3):
            b_stage2(3 * (g - 5) + e)
        b_stage2_wo(g - 5)
        for e in range(3):
            b_stage1(3 * (g - 2) + e)
        b_stage1_wo(g - 4)
        for p in range(3):
            pre_chunk(S55, stage_ref.at[slot, p], w_ref.at[p * NG + g - 1], p * NT + RT + (g - 1) * GT, range(NXC))
        return c
    lax.fori_loop(1, NG + 1, pre_body, 0)
    w0_copy(3).wait()

    bscale = float(bdh) ** (-0.5) * LOG2E

    def b_proj(lhs, part):
        return _nn(lhs, _cat([_upk(bw_ref[part * nct + j]) for j in range(nct)], axis=1))

    def b_attn(jobs, q, k, v):
        row = lax.broadcasted_iota(jnp.int32, (seg, 128), 0)
        outs = []
        for i, (l, sidx) in enumerate(jobs):
            r0 = i * seg
            pos = row + sidx * seg
            for j in range(nct):
                kb_ref[l, j, HIST:HIST + seg, :] = k[r0:r0 + seg, j * 128:(j + 1) * 128]
                vb_ref[l, j, HIST:HIST + seg, :] = v[r0:r0 + seg, j * 128:(j + 1) * 128]
            logits = []
            for w in range(B_WIN):
                o = HIST - w * B_DIL
                acc = None
                for j in range(nct):
                    p = q[r0:r0 + seg, j * 128:(j + 1) * 128] * kb_ref[l, j, o:o + seg, :]
                    acc = p if acc is None else acc + p
                acc = acc + pltpu.roll(acc, 64, 1)
                acc = acc + pltpu.roll(acc, 32, 1)
                lg = acc * bscale
                if w > 0:
                    lg = jnp.where(pos >= w * B_DIL, lg, NEG2)
                logits.append(lg)
            m = logits[0]
            for w in range(1, B_WIN):
                m = jnp.maximum(m, logits[w])
            es = [jnp.exp2(lg - m) for lg in logits]
            den = es[0]
            for w in range(1, B_WIN):
                den = den + es[w]
            inv = _recip(den)
            cols = []
            for j in range(nct):
                acc = None
                for w in range(B_WIN):
                    o = HIST - w * B_DIL
                    p = es[w] * vb_ref[l, j, o:o + seg, :]
                    acc = p if acc is None else acc + p
                cols.append(acc * inv)
            outs.append(_cat(cols, axis=1).astype(BF16))
            for j in range(nct):
                kb_ref[l, j, 0:HIST, :] = k[r0 + seg - HIST:r0 + seg, j * 128:(j + 1) * 128]
                vb_ref[l, j, 0:HIST, :] = v[r0 + seg - HIST:r0 + seg, j * 128:(j + 1) * 128]
        return outs

    def b_out(ob, res):
        return res + _nn(ob, _cat([_upk(bw_ref[NB1 + j]) for j in range(nct)], axis=1))

    def o_store(b, val):
        ro = pl.multiple_of((b + 1) * seg, seg)
        o_ref[pl.ds(ro, val.shape[0]), :] = val.astype(o_ref.dtype)

    def out_copy(b):
        ro = pl.multiple_of(b * seg, seg)
        return pltpu.make_async_copy(o_ref.at[pl.ds(ro + seg, seg), :], out_hbm.at[pl.ds(ro, seg), :], sem_o)

    def step(t, hc, full):
        t_last = n_seg + LAG - 1
        if full:
            jobs = [(0, t - 1), (1, t - 1 - LAG)]

            def b_in():
                return xb_ref[0:2 * seg, :]
        else:
            lb = (t == t_last).astype(jnp.int32)
            jobs = [(lb, t - 1 - lb * (LAG + 1))]

            def b_in():
                return xb_ref[pl.ds(pl.multiple_of(lb * seg, seg), seg), :]
        v0r = _cat([hc[0:n_mem], h_ref[n_mem:M2, :]])
        v1r = _cat([hc[n_mem:M2], h_ref[M2 + n_mem:2 * M2, :]])

        def ktiles(z):
            return [z[:, k * 128:(k + 1) * 128] for k in range(z.shape[1] // 128)]
        if full:
            hl = _Operands(ktiles(_cat([v0r, h_ref[2 * M2:RB, :]])), ktiles(_cat([v1r, h_ref[RB:RB + AH, :]])), None)
        else:
            hl = _Operands(None, None, ktiles(_cat([v0r, v1r, h_ref[2 * M2:RB, :]])))
        mh = 2 * M2 if full else 0

        def tile_dot(p, r):
            src = wr_ref.at[p] if r == 0 else w_ref.at[p * NG + r - 1]
            return lambda a, i: _nn(a, _upk(src[i * 64:(i + 1) * 64, :]))
        scale = float(dh) ** (-0.5) * LOG2E
        if full:
            s_ = t - LAG
            rd = pl.multiple_of(lax.rem(s_ * (seg // 2), RS // 2), seg // 2)
            wa = pl.multiple_of(lax.rem((A0 - R0 + s_ * AH) // 2, RS // 2), 8)
        else:
            wx = pl.multiple_of(jnp.where(t < LAG, NPRE // 2 + t * (n_mem // 2), RS // 2), n_mem // 2)
            wo_store(S35, stage0_ref, wr_ref.at[3])

        RA = R if full else M2 + seg
        CW = R + 2 * M2 if full else R
        bidx = 0 if full else 2
        half = dh - 128
        la8 = lax.broadcasted_iota(jnp.int32, (n_mem, 128), 1) < half
        ones = jnp.full((n_mem, 128), 0xFFFFFFFF, U32)
        zero = jnp.zeros((n_mem, 128), U32)
        mask_a = jnp.where(la8, ones, zero)
        mask_b = jnp.where(la8, zero, ones)

        def pk2(a, b):
            return _pk(_cat([a, b]).astype(BF16))

        yt = [[None] * NT for _ in range(3)]

        def proj(p, r):
            pa, qa = {}, {}
            _fast_mm((S53 if r == 0 else S55)[1], hl, tile_dot(p, r), mh, pa, qa)
            n0 = 0 if r == 0 else RT + (r - 1) * GT
            for n in range(len(pa)):
                y, z, e = _fast_out(pa, qa, n, mh)
                idx = p * NT + n0 + n
                if full:
                    ring_ref[idx, pl.ds(wa, 8), :] = pk2(z[16:24], z[24:32])
                    y = _cat([y[0:M2], z[0:M2], y[M2:2 * M2]])
                else:
                    y = e
                    ring_ref[idx, pl.ds(wx, n_mem // 2), :] = pk2(y[0:8], y[8:16])[0:n_mem // 2]
                yt[p][n0 + n] = stash(p * 16 + (n0 + n) % 16, packed(p, (n0 + n) % 3, y))

        def ab(z8):
            return jnp.where(la8, z8, 0.0), jnp.where(la8, 0.0, z8)

        def packed(p, j, y):
            u2 = pk2(y[32:40], y[40:48])
            if p == 0 or j == 0:
                return [pk2(y[0:8], y[8:16]), pk2(y[16:24], y[24:32]), u2]
            if j == 2:
                return [pk2(y[8:16], y[0:8]), pk2(y[24:32], y[16:24]), u2]
            xa_a, xa_b = ab(y[8:16])
            out = [pk2(xa_b, xa_a), pk2(y[24:32], y[16:24]) & mask_b, pk2(y[16:24], y[24:32]) & mask_a, u2]
            if full:
                out += [pk2(*ab(y[0:8])), pk2(*ab(y[16:24]))]
            return out

        def stash(idx, parts):
            kv_ref[idx, 0:8 * len(parts), :] = _cat(parts)
            return lambda: [kv_ref[idx, 8 * e:8 * e + 8, :] for e in range(len(parts))]

        def pair(p, g):
            xs = [ring_ref[p * NT + 3 * g + j, pl.ds(rd, seg // 2), :] for j in range(3)] if full else None
            return [f() for f in yt[p][3 * g:3 * g + 3]], xs

        def q_rows(z, j):
            v0, v1, v2 = z[0][j]
            return [v0] + ([z[1][j]] if full else []) + [v1, v2]

        def kv_tiles(z):
            yt, x1 = z
            v0, v1, v2 = yt[0]
            t0 = [v0] + ([x1[0]] if full else [v1, v2]) + [v1, v2]
            w0, w1, w2 = yt[2]
            t2 = [w0, w1, w2] + ([x1[2]] if full else [w1, w2])
            if full:
                t0 += [v0, v1]
                t2 += [w0, w1]
            e1, mb, ma, u2 = yt[1][0:4]
            mid2 = [e1, mb, u2 & mask_b, ma, u2 & mask_a]
            mid1 = None
            if full:
                lo, hi = x1[1][0:8], x1[1][8:16]
                mid1 = [yt[1][4], lo & mask_a, hi & mask_a, lo & mask_b, hi & mask_b, e1, yt[1][5]]
            return t0, mid1, mid2, t2

        def mat(parts):
            return _upk(_cat(parts))

        def scores(q, k):
            k0, km1, km2, k2_ = kv_tiles(k)
            s_a = _nt(mat(q_rows(q, 0)), mat(k0))
            s_b = _nt(mat(q_rows(q, 2)), mat(k2_))
            qm = q_rows(q, 1)
            if full:
                s_m = _cat([_nt(mat(qm[0:2]), mat(km1)), _cat([_nt(mat(qm[2:4]), mat(km2)), jnp.zeros((seg, CW - R), F32)], axis=1)])
            else:
                s_m = _nt(mat(qm), mat(km2))
            out = []
            for e, sx in enumerate((s_a, s_b)):
                s = (sx + s_m) * scale + bias_ref[bidx + e, 0:RA, 0:CW]
                ex = jnp.exp2(s - jnp.max(s, axis=-1, keepdims=True))
                out.append(ex * _recip(jnp.sum(ex, axis=-1, keepdims=True)))
            return out

        def pv(p, v):
            v0, vm1, vm2, v2 = kv_tiles(v)
            o_a = _nn(p[0].astype(BF16), mat(v0))
            o_b = _nn(p[1].astype(BF16), mat(v2))
            p = p[0] + p[1]
            if full:
                o_m = _cat([_nn(p[0:M2 + seg].astype(BF16), mat(vm1)),
                            _nn(p[M2 + seg:R, 0:R].astype(BF16), mat(vm2))])
            else:
                o_m = _nn(p.astype(BF16), mat(vm2))
            return [o_a, o_m, o_b]

        ot = []
        pacc, qacc = {}, {}

        def add_o(r):
            n0 = 0 if r == 0 else RT + (r - 1) * GT
            oo = ot[n0:n0 + (RT if r == 0 else GT)]
            if full:
                ops = _Operands([o[0:32] for o in oo], [_cat([o[48:64], o[32:48]]) for o in oo],
                                [o[64:80] for o in oo])
            else:
                ops = _Operands(None, None, oo)
            _fast_mm((S35 if r == 0 else S55)[1], ops, tile_dot(3, r), mh, pacc, qacc)

        bqkv = [None] * 3
        probs = []

        def do_pv():
            for g in range(len(ot) // 3, len(probs)):
                ot.extend(pv(probs[g], pair(2, g)))

        for r in range(NG + 1):
            proj(2, r)
            proj(1, r)
            proj(0, r)
            if r == 0:
                blhs = _ln(b_in()).astype(BF16)
            if r < 3:
                bqkv[2 - r] = b_proj(blhs, 2 - r)
            if r == 3:
                ob = b_attn(jobs, *bqkv)
            if r == BOUT_R:
                zb = b_out(_cat(ob), b_in())
                x2_new = zb[0:seg]
                if full:
                    o_store(t - 1 - LAG, zb[seg:2 * seg])
                else:
                    o_store(lb * (t_last - LAG - 1) - 1, x2_new)
            if r in WSCHED:
                add_o(WSCHED[r])
            do_pv()
            for g in range(len(probs), (RT + r * GT) // 3):
                probs.append(scores(pair(0, g), pair(1, g)))
        for r in range(len(WSCHED), TAILPV):
            add_o(r)
        do_pv()
        for r in range(TAILPV, NG + 1):
            add_o(r)
        cols = []
        for n in range(nct):
            y, z, e = _fast_out(pacc, qacc, n, mh)
            cols.append(_cat([y, z[16:32], z[0:16], e]) if full else e)
        acc = _cat(cols, axis=1)

        y2 = x2_ref[...] + _cat([acc[n_mem:M2], acc[RA - seg + n_mem:RA]])
        mem2 = acc[RA - seg:RA - seg + n_mem]
        if full:
            x_cur = x_ref[pl.ds(pl.multiple_of(t * seg, seg), seg), :].astype(F32)
            xb_ref[0:seg, :] = x_cur + acc[M2:M2 + seg]
            xb_ref[seg:2 * seg, :] = y2
            m1n = acc[0:n_mem]
            m2n = mem2
            an = pl.multiple_of(jnp.minimum(A0 + (s_ + 1) * AH, S - AH), AH)
            h_ref[RB:RB + AH, :] = _ln(x_ref[pl.ds(an, AH), :].astype(F32))
            nxt = x2_new
        else:
            xb_ref[pl.ds(pl.multiple_of(jnp.where(t < LAG, 0, (t - n_seg + 2) * seg), seg), seg), :] = y2
            m1n = jnp.where(t < LAG - 1, h_ref[RB + AH:RB + AH + n_mem, :], mem2)
            m2n = jnp.where(t == LAG - 1, mem0_ref[...].astype(F32), mem2)
            nxt = jnp.where(t < LAG - 1, x_ref[seg:2 * seg, :].astype(F32), x2_new)
        x2_ref[...] = nxt
        sl = _ln(nxt)
        h_ref[n_mem:M2, :] = sl[0:n_mem]
        h_ref[M2 + n_mem:RB, :] = sl[n_mem:seg]
        return _cat([m1n, m2n])

    def single_body(t, c):
        @pl.when(t == n_seg)
        def _():
            out_copy(t - (LAG + 2)).start()
        return step(t, c, False)

    def full_body(t, c):
        @pl.when(t >= LAG + 2)
        def _():
            out_copy(t - (LAG + 2)).start()
        return step(t, c, True)

    def phase(ph, c):
        t0 = ph * n_seg
        c = lax.fori_loop(t0, t0 + LAG, single_body, c)

        @pl.when(ph == 0)
        def _():
            x_late.wait()
        return lax.fori_loop(LAG, jnp.where(ph == 0, n_seg, LAG), full_body, c)
    lax.fori_loop(0, 2, phase, _cat([h_ref[0:n_mem, :], h_ref[M2:M2 + n_mem, :]]))

    out_copy(n_seg - 3).start()
    res = xb_ref[2 * seg:4 * seg, :]
    blhs = _ln(res).astype(BF16)
    ob = b_attn([(1, n_seg - 2), (1, n_seg - 1)], *[b_proj(blhs, part) for part in range(3)])
    o_store(n_seg - 2, b_out(_cat(ob), res))
    out_copy(n_seg - 2).start()
    out_copy(n_seg - 1).start()
    pltpu.make_async_copy(o_ref.at[pl.ds(seg, S), :], out_hbm, sem_o).wait()


@functools.partial(jax.jit, static_argnames=("seg",))
def _run(A_x, A_mem0, A_Wq, A_Wk, A_Wv, A_Wo, B_wqkv, B_wo, *, seg):
    _, S, dm = A_x.shape
    n_heads, dh = A_Wq.shape[1], A_Wq.shape[2]
    n_mem = A_mem0.shape[1]
    n_seg = S // seg
    hd = n_heads * dh
    nct = dm // 128
    ng = (hd // 128 - RT) // GT
    assert (seg, n_seg, n_mem, dh, dm % 128, n_heads, LAG) == (32, 64, 8, 192, 0, 32, 2)

    x = A_x.reshape(S, dm)
    mem0 = A_mem0.reshape(n_mem, dm)
    wq = jnp.transpose(A_Wq, (1, 2, 0)).reshape(hd, dm)
    wk = jnp.transpose(A_Wk, (1, 2, 0)).reshape(hd, dm)
    wv = jnp.transpose(A_Wv, (1, 2, 0)).reshape(hd, dm)
    wo = A_Wo.reshape(hd, dm)
    _, _, _, _, rs, xc = _plan(seg, n_seg)

    kern = functools.partial(_kernel, seg=seg, n_seg=n_seg, n_mem=n_mem,
                             n_heads=n_heads, dh=dh, dm=dm)
    hbm = pl.BlockSpec(memory_space=pltpu.HBM)

    out = pl.pallas_call(
        kern,
        in_specs=[hbm] * 8,
        out_specs=hbm,
        out_shape=jax.ShapeDtypeStruct((S, dm), A_x.dtype),
        scratch_shapes=[
            pltpu.VMEM((S, dm), BF16),
            pltpu.VMEM((n_mem, dm), BF16),
            pltpu.VMEM((NSLOT, 4, GT * 128, dm), BF16),
            pltpu.VMEM((RT * 128, dm), BF16),
            pltpu.VMEM((4, len(S53[0]) * 64, 128), U32),
            pltpu.VMEM((4 * ng, len(S55[0]) * 64, 128), U32),
            pltpu.VMEM((dm, 4 * dm + 128), BF16),
            pltpu.VMEM((nct, 4 * dm + 32, 128), F32),
            pltpu.VMEM((4 * nct, dm // 2, 128), U32),
            pltpu.VMEM((len(KEYS_R), HC * xc // 4, 128), U32),
            pltpu.VMEM((len(KEYS_R), HC * xc // 4, 128), U32),
            pltpu.VMEM((len(KEYS) - len(KEYS_R), NXC * xc // 4, 128), U32),
            pltpu.VMEM((15, 8, 128), U32),
            pltpu.VMEM((3 * hd // 128, rs // 2 + 8, 128), U32),
            pltpu.VMEM((3 * n_mem + seg + AH, dm), F32),
            pltpu.VMEM((4 * seg, dm), F32),
            pltpu.VMEM((seg, dm), F32),
            pltpu.VMEM((2, nct, HIST + seg, 128), F32),
            pltpu.VMEM((2, nct, HIST + seg, 128), F32),
            pltpu.VMEM((S + seg, dm), A_x.dtype),
            pltpu.VMEM((4, 2 * n_mem + 2 * seg, 128), F32),
            pltpu.VMEM((48, 48, 128), U32),
            pltpu.SemaphoreType.DMA((NSLOT,)),
            pltpu.SemaphoreType.DMA((8 + NXC,)),
            pltpu.SemaphoreType.DMA((4,)),
            pltpu.SemaphoreType.DMA(()),
        ],
        compiler_params=pltpu.CompilerParams(
            vmem_limit_bytes=126 * 1024 * 1024,
            disable_bounds_checks=True,
        ),
    )(x, mem0, wq, wk, wv, wo, B_wqkv, B_wo)
    return out.reshape(1, S, dm)


def pallas_interleave_layers__memory_aug_recurrent_mem_tr__sliding_local_dilated__prompt_kernel(
    A_x: jax.Array,
    A_mem0: jax.Array,
    A_Wq: jax.Array,
    A_Wk: jax.Array,
    A_Wv: jax.Array,
    A_Wo: jax.Array,
    A_seg_len,
    B_x: jax.Array,
    B_wqkv: jax.Array,
    B_wo: jax.Array,
):
    del B_x
    seg = A_seg_len if isinstance(A_seg_len, int) else 32
    return _run(A_x, A_mem0, A_Wq, A_Wk, A_Wv, A_Wo, B_wqkv, B_wo, seg=seg)
```

```python
import functools

import jax
import jax.numpy as jnp
from jax import lax
import jax.experimental.pallas as pl
import jax.experimental.pallas.tpu as pltpu

F32 = jnp.float32
BF16 = jnp.bfloat16
U32 = jnp.uint32
NEG = -1000000000.0
LN_EPS = 1e-05
LOG2E = 1.4426950408889634
NEG2 = NEG * LOG2E

B_HEADS = 32
B_WIN = 8
B_DIL = 2
HIST = 16
SKIPM = int(0)
PACE = int(1)
BDL = int(0)
BD0 = int(40)
PB = int(60)
PB0 = int(100)
PC = int(0)
BAR = int(3)
BO = int(5)
WS = '346789'
AH = 16
LAG = 2
NSLOT = 2
NXC = 6
HC = 3
WSCHED = dict((int(c), i) for i, c in enumerate(WS))
BOUT_R = BO
TAILPV = 8


def _ln(x):
    m = jnp.mean(x, axis=-1, keepdims=True)
    c = x - m
    v = jnp.mean(c * c, axis=-1, keepdims=True)
    return c * lax.rsqrt(v + LN_EPS)


def _recip(d):
    return pl.reciprocal(d, approx=True)


def _nt(a, b):
    return lax.dot_general(a, b, (((1,), (1,)), ((), ())), preferred_element_type=F32)


def _nn(a, b):
    return jnp.dot(a, b, preferred_element_type=F32)


def _cat(xs, axis=0):
    return xs[0] if len(xs) == 1 else jnp.concatenate(xs, axis=axis)


def _pk(z):
    return pltpu.bitcast(z, U32)


def _upk(z):
    return pltpu.bitcast(z, BF16)


LAM = (-1.5, -0.5, 0.0, 0.5, 1.5)


def _scheme(stars):
    tiles, prog = [], []
    for star in stars:
        if len(star) == 1:
            prog.append(("single", star[0], None, len(tiles)))
            tiles.append([star[0][:2]])
            continue
        left = [len(star) - 1] * len(star)
        for j in range(1, len(star)):
            for i in range(j):
                x, y = star[i], star[j]
                prog.append(("pair", x, y, len(tiles)))
                tiles += [[(x[0], y[1])], [(y[0], x[1])], [(x[0], y[1]), (y[0], x[1])]]
                for e in (i, j):
                    left[e] -= 1
                    if left[e] == 0:
                        z = star[e]
                        prog.append(("diag", z, None, len(tiles)))
                        tiles += [[z[:2]] + [(o[0], z[1]) for o in star if o is not z],
                                  [z[:2]] + [(z[0], o[1]) for o in star if o is not z]]
    return tiles, prog


S55 = _scheme([[(i, i, LAM[i]) for i in range(5)]])
S53 = _scheme([[(0, 0, LAM[0]), (2, 1, LAM[2]), (4, 2, LAM[4])], [(1, 0, LAM[1]), (3, 2, LAM[3])],
               [(1, 1, LAM[1])], [(3, 1, LAM[3])]])
S35 = _scheme([[(0, 0, LAM[0]), (1, 2, LAM[2]), (2, 4, LAM[4])], [(0, 1, LAM[1]), (2, 3, LAM[3])],
               [(1, 1, LAM[1])], [(1, 3, LAM[3])]])


def _spread(prog):
    pairs = [e for e in prog if e[0] != "diag"]
    diags = [e for e in prog if e[0] == "diag"]
    out, k = [], 0
    for i, e in enumerate(pairs):
        out.append(e)
        while k < len(diags) and (k + 0.5) * len(pairs) <= (i + 1) * len(diags):
            out.append(diags[k])
            k += 1
    return out + diags[k:]


def _op_keys(prog):
    keys = []
    for kind, x, y, _ in prog:
        if kind == "pair":
            new = [(nm, x[0], x[2], y[0], y[2]) for nm in ("l1", "l2", "A")]
        else:
            new = [("a", x[0], x[2]), ("b", x[0])]
        keys += [k for k in new if k not in keys]
    return keys


def _scaled(c, u):
    return u if c == 1.0 else c * u


class _Operands:
    def __init__(self, T, U, E):
        self.T, self.U, self.E, self.memo = T, U, E, {}

    def _get(self, key, fn):
        if key not in self.memo:
            self.memo[key] = fn()
        return self.memo[key]

    def paired(self, key):
        T, U = self.T, self.U
        if key[0] == "b":
            return U[key[1]]
        if key[0] == "a":
            k, lam = key[1:]
            if lam == 0.0:
                return T[k]
            return self._get(("f",) + key, lambda: T[k] - _scaled(lam, U[k]) if lam > 0
                             else T[k] + _scaled(-lam, U[k]))
        kx, lx, ky, ly = key[1:]
        A = self._get(("f", "A") + key[1:],
                      lambda: self.paired(("a", kx, lx)) + self.paired(("a", ky, ly)))
        if key[0] == "A":
            return A
        return A - _scaled(ly - lx, U[kx]) if key[0] == "l1" else A + _scaled(ly - lx, U[ky])

    def extra(self, key):
        if key[0] == "a":
            return self.E[key[1]]
        return self._get(("e", key[1], key[3]), lambda: self.E[key[1]] + self.E[key[3]])

    def __call__(self, key):
        if self.T is None:
            ek = ("a", key[1]) if key[0] in ("a", "s") else ("l", key[1], 0, key[3])
            return self._get(ek, lambda: self.extra(ek).astype(BF16))

        def build():
            ak = ("a",) + key[1:] if key[0] == "s" else key
            parts = [self.paired(ak)]
            if self.E is not None and ak[0] in ("a", "l1", "l2"):
                parts.append(self.extra(ak))
            if key[0] == "s":
                parts.append(self.U[key[1]])
            return _cat(parts).astype(BF16)
        return self._get(key, build)


def _fast_mm(prog, op, dot, m, p, q):
    def add(d, key, val):
        d[key] = val if key not in d else d[key] + val

    for kind, x, y, i in prog:
        if kind == "pair":
            kk = (x[0], x[2], y[0], y[2])
            p1, p2 = dot(op(("l1",) + kk), i), dot(op(("l2",) + kk), i + 1)
            if m:
                r = _scaled(1.0 / (y[2] - x[2]), p2[0:m] - p1[0:m] + dot(op(("A",) + kk), i + 2))
                add(q, (x[1], x[2]), r)
                add(q, (y[1], y[2]), r)
            add(p, y[1], p1)
            add(p, x[1], p2)
        elif kind == "diag":
            add(p, x[1], dot(op(("a", x[0], x[2])), i))
            if m:
                add(q, (x[1], x[2]), dot(op(("b", x[0])), i + 1))
        else:
            r = dot(op(("s", x[0], x[2])), i)
            add(p, x[1], r[0:r.shape[0] - m])
            if m:
                add(q, (x[1], x[2]), r[r.shape[0] - m:])


def _fast_out(p, q, n, m):
    if not m:
        return None, None, p[n]
    y, z = p[n][0:m], None
    for (nn, lam), v in q.items():
        if nn == n:
            z = v if z is None else z + v
            if lam != 0.0:
                y = y + _scaled(lam, v) if lam > 0 else y - _scaled(-lam, v)
    return y, z, (p[n][m:] if p[n].shape[0] > m else None)


def _combo(tile, block):
    out = block(*tile[0])
    for kn in tile[1:]:
        out = out - block(*kn)
    return out


GT = 5
RT = 3
KEYS_R = _op_keys(S53[1])
KEYS = KEYS_R + [k for k in _op_keys(S55[1]) if k not in KEYS_R]


def _plan(seg, n_seg):
    S = seg * n_seg
    R0 = LAG * seg
    A0 = S - (n_seg - LAG) * AH
    NPRE = A0 - R0 - LAG * 8
    RS = -(-(A0 - R0 + AH) // seg) * seg
    XC = NPRE // NXC // 32 * 32
    assert XC * NXC + 16 == NPRE
    return S, R0, A0, NPRE, RS, XC


def _kernel(x_hbm, mem0_hbm, wq_hbm, wk_hbm, wv_hbm, wo_hbm, bqkv_hbm, bwo_hbm,
            out_hbm,
            x_ref, mem0_ref, stage_ref, stage0_ref, wr_ref, w_ref, bst_ref, btmp_ref, bw_ref,
            xla_ref, xlb_ref, xlc_ref, xe_ref, ring_ref, h_ref, xb_ref, x2_ref, kb_ref, vb_ref, o_ref, bias_ref, kv_ref,
            sem_w, sem_m, sem_b, sem_o,
            *, seg, n_seg, n_mem, n_heads, dh, dm):
    S, R0, A0, NPRE, RS, XC = _plan(seg, n_seg)
    M2 = 2 * n_mem
    R = M2 + 2 * seg
    RB = M2 + seg
    PW = 2 * dh
    G = n_heads // 2
    nct = dm // 128
    bdh = dm // B_HEADS
    NT = n_heads * dh // 128
    NG = (NT - RT) // GT
    w_hbm = (wq_hbm, wk_hbm, wv_hbm, wo_hbm)

    def w_copy(p, g):
        slot = g & (NSLOT - 1)
        return pltpu.make_async_copy(w_hbm[p].at[pl.ds((RT + (g - 1) * GT) * 128, GT * 128), :],
                                     stage_ref.at[slot, p], sem_w.at[slot])

    def w0_copy(p):
        dst = stage0_ref if p == 3 else stage_ref.at[0, p, pl.ds(0, RT * 128)]
        return pltpu.make_async_copy(w_hbm[p].at[pl.ds(0, RT * 128), :], dst, sem_m.at[4 + p])

    NB1 = 3 * nct
    WO0 = 3 * dm
    XF = A0 + AH
    XH = XC // 2

    def rows_copy(r0, n, sem):
        return pltpu.make_async_copy(x_hbm.at[pl.ds(r0, n), :], x_ref.at[pl.ds(r0, n), :], sem)

    def x_copy(i):
        return rows_copy(pl.multiple_of(R0 + i * XC, 16), XC, sem_m.at[8 + i])

    small = [rows_copy(0, R0, sem_m.at[1]), rows_copy(R0 + NPRE - 16, XF - R0 - NPRE + 16, sem_m.at[2]),
             pltpu.make_async_copy(mem0_hbm, mem0_ref, sem_m.at[3])]
    x_late = rows_copy(XF, S - XF, sem_m.at[0])

    def bq_copy(part):
        c0 = pl.multiple_of(part * dm, 128)
        return pltpu.make_async_copy(bqkv_hbm.at[:, pl.ds(c0, dm)], bst_ref.at[:, pl.ds(c0, dm)], sem_b.at[part])

    bo_copy = pltpu.make_async_copy(bwo_hbm, bst_ref.at[:, pl.ds(3 * dm, dm)], sem_b.at[3])

    def bst_tile(c):
        return bst_ref[:, pl.ds(pl.multiple_of(c * 128, 128), 128)]

    def bias_tables(full):
        RA = R if full else M2 + seg
        CW = 128
        ri = lax.broadcasted_iota(jnp.int32, (RA, CW), 0)
        ci = lax.broadcasted_iota(jnp.int32, (RA, CW), 1)
        if not full:
            ri = jnp.where(ri >= M2, ri + seg, ri)

        def table(i, bounds, vals):
            out = vals[-1]
            for b, v in zip(reversed(bounds), reversed(vals[:-1])):
                out = jnp.where(i < b, v, out)
            return out
        qi = ri - table(ri, [16, 48, 56], [0, 8, 48, 40])
        g0 = (ci < 8) | ((ci >= 16) & (ci < 48))
        k2 = ci - table(ci, [8, 24, 32, 48, 56, 80, 88, 96, 104], [-8, 0, 24, 8, 48, 40, 72, 80, 96, 104])
        if full:
            k1 = ci - table(ci, [8, 48], [0, 8, 40])
            row_l2 = ((ri >= 8) & (ri < 16)) | (ri >= 48)
            row_xa = (ri >= 8) & (ri < 16)
            valid = (row_xa == (ci >= 80)) & (ci < 112)
            is_a = jnp.where(ci >= 80, ((ci >= 88) & (ci < 104)).astype(jnp.int32),
                             (g0 != row_l2).astype(jnp.int32)) > 0
            ki = jnp.where(row_l2, k2, k1)
            visible = valid & ((qi < n_mem) | (qi >= ki))
            fill = jnp.where(valid, NEG2, -jnp.inf)
        else:
            is_a = jnp.logical_not(g0)
            visible = (qi < n_mem) | (qi >= k2)
            fill = NEG2
        for e, mine in enumerate((is_a, jnp.logical_not(is_a))):
            bias_ref[(0 if full else 2) + e, 0:RA, :] = jnp.where(
                mine, jnp.where(visible, 0.0, fill), -jnp.inf)

    for i in range(HC):
        x_copy(i).start()

    def zero_body(j, c):
        btmp_ref[j, 0:dm, :] = jnp.zeros((dm, 128), F32)
        return c
    lax.fori_loop(0, nct, zero_body, 0)

    w0_copy(0).start()
    xb_ref[0:2 * seg, :] = jnp.zeros((2 * seg, dm), F32)
    kb_ref[...] = jnp.zeros(kb_ref.shape, F32)
    vb_ref[...] = jnp.zeros(vb_ref.shape, F32)
    bst_ref[:, 4 * dm:] = jnp.zeros((dm, 128), BF16)
    bias_tables(True)
    bias_tables(False)

    def ekey(key):
        return ("a", key[1]) if key[0] == "a" else ("l", key[1], 0, key[3])
    EKEYS = []
    for key in KEYS:
        if key[0] in ("a", "l1") and ekey(key) not in EKEYS:
            EKEYS.append(ekey(key))

    def e_ops():
        ye = _ln(x_ref[R0 + NPRE - 16:R0 + NPRE, :].astype(F32))
        eops = _Operands(None, None, [ye[:, k * 128:(k + 1) * 128] for k in range(nct)])
        for j, key in enumerate(EKEYS):
            xe_ref[j] = _pk(eops(key))

    NKR = len(KEYS_R)

    def xl(j, hf, i):
        if j >= NKR:
            ref, j, i = xlc_ref, j - NKR, hf * HC + i
        else:
            ref = (xla_ref, xlb_ref)[hf]
        r0 = i * (XH // 2)
        return ref.at[j, pl.ds(r0 if isinstance(r0, int) else pl.multiple_of(r0, 8), XH // 2)]

    def ln_ops(hf, i, lo, hi):
        y = _ln(x_ref[pl.ds(pl.multiple_of(R0 + (hf * HC + i) * XC, 16), XC), :].astype(F32))
        ops = _Operands([y[0:XH, k * 128:(k + 1) * 128] for k in range(nct)],
                        [y[XH:XC, k * 128:(k + 1) * 128] for k in range(nct)], None)
        for j in range(lo, hi):
            xl(j, hf, i)[...] = _pk(ops(KEYS[j]))

    def ln_body(i, c):
        x_copy(i).wait()

        @pl.when(i == 0)
        def _():
            x_copy(HC).start()

        @pl.when(i == 1)
        def _():
            w0_copy(1).start()
            w0_copy(2).start()

        @pl.when(i == 2)
        def _():
            x_copy(HC + 1).start()
            x_copy(HC + 2).start()
            for cp in small:
                cp.start()
        ln_ops(0, i, 0, len(KEYS_R))
        return c
    lax.fori_loop(0, HC, ln_body, 0)

    def prep(scheme, w, dst):
        raw = lambda k, n: w[n * 128:(n + 1) * 128, k * 128:(k + 1) * 128]
        tb = []
        for i, tl in enumerate(scheme[0]):
            tb.append(raw(*tl[0]) if len(tl) == 1
                      else _combo(tl, lambda k, n: raw(k, n).astype(F32)).astype(BF16))
            tt = _pk(tb[i].T)
            dst[i * 64:(i + 1) * 64, :] = tt
            if len(tl) > 1:
                tdeps.append([tt[56:64]])
        return tb

    pcnt, pdl, tdeps = [0], [], []

    def pre_chunk(scheme, w, dst, n0, chunks, never=None, tb=None):
        tiles, prog = scheme
        prog = _spread(prog)
        dot = lambda a, i: _nn(a, _upk(dst[i * 64:(i + 1) * 64, :]))
        if w is not None:
            if tb is None:
                tb = prep(scheme, w, dst)
            dot = lambda a, i: _nt(a, tb[i])

        for c in chunks:
            def op(key):
                def ld(kk):
                    v = xl(KEYS.index(kk), c // HC, c % HC)[...]
                    if c == NXC - 1 and kk[0] in ("a", "l1", "l2"):
                        v = _cat([v, xe_ref[EKEYS.index(ekey(kk))]])
                    return v
                if key[0] == "s":
                    return _upk(_cat([ld(("a",) + key[1:]), ld(("b", key[1]))]))
                v = ld(key)
                pcnt[0] += 1
                pdl.sort(key=lambda e: e[0])
                if pdl and pcnt[0] >= pdl[0][0]:
                    deps = pdl.pop(0)[1]
                    v = _cat([jnp.where(never, d, v[8 * e:8 * e + 8]) for e, d in enumerate(deps)]
                             + ([v[8 * len(deps):]] if v.shape[0] > 8 * len(deps) else []))
                return _upk(v)
            p, q = {}, {}
            _fast_mm(prog, op, dot, XH, p, q)
            for n in range(len(p)):
                y, z, e = _fast_out(p, q, n, XH)
                ring_ref[n0 + n, c * XH:c * XH + XH // 2, :] = _pk(y.astype(BF16))
                ring_ref[n0 + n, c * XH + XH // 2:(c + 1) * XH, :] = _pk(z.astype(BF16))
                if e is not None:
                    ring_ref[n0 + n, NXC * XH:NXC * XH + 8, :] = _pk(e.astype(BF16))

    def init_rows():
        x0 = x_ref[0:seg, :].astype(F32)
        sl = _ln(x0)
        xt = _ln(x_ref[R0 + NPRE:XF, :].astype(F32))
        h_ref[0:n_mem, :] = xt[0:n_mem]
        h_ref[n_mem:M2, :] = sl[0:n_mem]
        h_ref[M2:M2 + n_mem, :] = mem0_ref[...].astype(F32)
        h_ref[M2 + n_mem:RB, :] = sl[n_mem:seg]
        h_ref[RB:RB + AH, :] = xt[M2:M2 + AH]
        h_ref[RB + AH:RB + AH + n_mem, :] = xt[n_mem:M2]
        x2_ref[...] = x0

    def first_a(p, c):
        buf = stage_ref.at[0, p, pl.ds(0, RT * 128)]
        pltpu.make_async_copy(buf, buf, sem_m.at[4 + p]).wait()
        x_copy(HC + p).wait()

        @pl.when(p == 0)
        def _():
            for pp in range(4):
                w_copy(pp, 1).start()

        @pl.when(p == 2)
        def _():
            bq_copy(0).start()
        ln_ops(1, p, 0, len(KEYS))
        pre_chunk(S53, buf, wr_ref.at[p], p * NT, range(HC))
        return c
    lax.fori_loop(0, 3, first_a, 0)
    for cp in small:
        cp.wait()

    def first_b(p, c):
        e_ops()
        init_rows()
        ln_ops(0, p, len(KEYS_R), len(KEYS))
        pre_chunk(S53, None, wr_ref.at[p], p * NT, range(HC, NXC))
        return c
    lax.fori_loop(0, 3, first_b, 0)

    dpt = 128 // B_HEADS

    def b_stage1(u):
        uc = jnp.clip(u, 0, NB1 - 1)
        tr = bst_tile(jnp.where(u >= 0, uc, NB1 + nct)).astype(F32).T
        r0 = pl.multiple_of(uc * 128, 128)
        for j in range(nct):
            btmp_ref[j, pl.ds(r0, 128), :] = tr[:, j * 128:(j + 1) * 128]
        return [pltpu.bitcast(tr[120:128, j * 128:(j + 1) * 128], U32) for j in range(nct)]

    def b_stage1_wo(u):
        uc = jnp.clip(u, 0, nct - 1)
        btmp_ref[uc, WO0:WO0 + dm, :] = bst_tile(jnp.where(u >= 0, NB1 + uc, NB1 + nct)).astype(F32)

    def b_stage2(u):
        uc = jnp.clip(u, 0, NB1 - 1)
        part = (uc >= nct).astype(jnp.int32) + (uc >= 2 * nct).astype(jnp.int32)
        r0 = part * dm + (uc - part * nct) * dpt
        rows = _cat([_cat([btmp_ref[j, pl.ds(r0 + dd, B_HEADS, stride=bdh), :]
                           for j in range(nct)], axis=1) for dd in range(dpt)])
        val = _pk(rows.T.astype(BF16))
        bw_ref[uc] = val
        return [val[64 * j + 56:64 * j + 64] for j in range(nct)]

    def b_stage2_wo(u):
        uc = jnp.clip(u, 0, nct - 1)
        r0 = jnp.where(u >= 0, WO0, 0)
        bw_ref[NB1 + uc] = _pk(
            _cat([btmp_ref[uc, pl.ds(r0 + d, B_HEADS, stride=bdh), :] for d in range(bdh)]).astype(BF16))

    def wo_store(scheme, w, dst, never=None):
        if scheme is S55:
            rawt = lambda k, n: w[k * 128:(k + 1) * 128, n * 128:(n + 1) * 128]
            plain = [i for i, tl in enumerate(scheme[0]) if len(tl) == 1]
            for i, tl in enumerate(scheme[0]):
                if len(tl) > 1:
                    val = _combo(tl, lambda k, n: rawt(k, n).astype(F32)).astype(BF16)
                    val = _pk(_upk(_pk(val.T)).T)
                    dst[i * 64:(i + 1) * 64, :] = val
                    j = plain.pop()
                    pv_ = _pk(rawt(*scheme[0][j][0]))
                    dst[j * 64:(j + 1) * 64, :] = jnp.where(never, val, pv_) if PACE else pv_
            return
        for r in range(0, 128, 16):
            memo = {}

            def raw(k, n):
                return w[k * 128 + r:k * 128 + r + 16, n * 128:(n + 1) * 128]

            def block(k, n):
                if (k, n) not in memo:
                    memo[k, n] = raw(k, n).astype(F32)
                return memo[k, n]
            for i, tl in enumerate(scheme[0]):
                val = raw(*tl[0]) if len(tl) == 1 else _combo(tl, block).astype(BF16)
                dst[i * 64 + r // 2:i * 64 + r // 2 + 8, :] = _pk(val)

    def pre_body(g, c):
        slot = g & (NSLOT - 1)
        buf = stage_ref.at[slot]
        pltpu.make_async_copy(buf, buf, sem_w.at[slot]).wait()

        @pl.when((g >= 2) & (g <= 4))
        def _():
            bq_copy(g - 2).wait()

        @pl.when(g == 4)
        def _():
            bo_copy.wait()

        @pl.when(g <= 2)
        def _():
            bq_copy(g).start()

        @pl.when(g == 2)
        def _():
            bo_copy.start()

        @pl.when(g + 1 <= NG)
        def _():
            for p in range(4):
                w_copy(p, g + 1).start()

        @pl.when(g == NG - 1)
        def _():
            w0_copy(3).start()
            x_late.start()

        wo_store(S55, stage_ref.at[slot, 3], w_ref.at[3 * NG + g - 1], g > NG + 5)
        deps = [b_stage2(3 * (g - 5) + e) for e in range(3)]
        b_stage2_wo(g - 5)
        deps += [b_stage1(3 * (g - 2) + e) for e in range(3)]
        b_stage1_wo(g - 4)
        pcnt[0] = 0
        if PB:
            pdl.extend((PB0 + PB * e, d) for e, d in enumerate(deps))
        tbs = [prep(S55, stage_ref.at[slot, 0], w_ref.at[g - 1])]
        for p in range(3):
            if p < 2:
                del tdeps[:]
                tbs.append(prep(S55, stage_ref.at[slot, p + 1], w_ref.at[(p + 1) * NG + g - 1]))
                if PC:
                    pdl.extend((pcnt[0] + 60 + PC * e, d) for e, d in enumerate(tdeps))
            pre_chunk(S55, stage_ref.at[slot, p], w_ref.at[p * NG + g - 1], p * NT + RT + (g - 1) * GT, range(NXC),
                      g > NG + 5, tbs[p])
        return c
    lax.fori_loop(1, NG + 1, pre_body, 0)
    w0_copy(3).wait()

    bscale = float(bdh) ** (-0.5) * LOG2E

    def b_proj(lhs, part):
        return _nn(lhs, _cat([_upk(bw_ref[part * nct + j]) for j in range(nct)], axis=1))

    def b_attn(jobs, q, k, v, sink=None):
        row = lax.broadcasted_iota(jnp.int32, (seg, 128), 0)
        outs = []
        for i, (l, sidx) in enumerate(jobs):
            r0 = i * seg
            pos = row + sidx * seg
            for j in range(nct):
                kb_ref[l, j, HIST:HIST + seg, :] = k[r0:r0 + seg, j * 128:(j + 1) * 128]
                vb_ref[l, j, HIST:HIST + seg, :] = v[r0:r0 + seg, j * 128:(j + 1) * 128]
            logits = []
            for w in range(B_WIN):
                o = HIST - w * B_DIL
                acc = None
                for j in range(nct):
                    p = q[r0:r0 + seg, j * 128:(j + 1) * 128] * kb_ref[l, j, o:o + seg, :]
                    acc = p if acc is None else acc + p
                acc = acc + pltpu.roll(acc, 64, 1)
                acc = acc + pltpu.roll(acc, 32, 1)
                lg = acc * bscale
                if w > 0:
                    lg = jnp.where(pos >= w * B_DIL, lg, NEG2)
                logits.append(lg)
            m = logits[0]
            for w in range(1, B_WIN):
                m = jnp.maximum(m, logits[w])
            es = [jnp.exp2(lg - m) for lg in logits]
            den = es[0]
            for w in range(1, B_WIN):
                den = den + es[w]
            inv = _recip(den)
            cols = []
            for j in range(nct):
                acc = None
                for w in range(B_WIN):
                    o = HIST - w * B_DIL
                    p = es[w] * vb_ref[l, j, o:o + seg, :]
                    acc = p if acc is None else acc + p
                cols.append(acc * inv)
            outs.append(_cat(cols, axis=1).astype(BF16))
            if sink is not None:
                for rg in range(0, seg, 8):
                    sink.append([c[rg:rg + 8] for c in cols])
            for j in range(nct):
                kb_ref[l, j, 0:HIST, :] = k[r0 + seg - HIST:r0 + seg, j * 128:(j + 1) * 128]
                vb_ref[l, j, 0:HIST, :] = v[r0 + seg - HIST:r0 + seg, j * 128:(j + 1) * 128]
        return outs

    def b_out(ob, res):
        return res + _nn(ob, _cat([_upk(bw_ref[NB1 + j]) for j in range(nct)], axis=1))

    def o_store(b, val):
        ro = pl.multiple_of((b + 1) * seg, seg)
        o_ref[pl.ds(ro, val.shape[0]), :] = val.astype(o_ref.dtype)

    def out_copy(b):
        ro = pl.multiple_of(b * seg, seg)
        return pltpu.make_async_copy(o_ref.at[pl.ds(ro + seg, seg), :], out_hbm.at[pl.ds(ro, seg), :], sem_o)

    def step(t, hc, full):
        t_last = n_seg + LAG - 1
        if full:
            jobs = [(0, t - 1), (1, t - 1 - LAG)]

            def b_in():
                return xb_ref[0:2 * seg, :]
        else:
            lb = (t == t_last).astype(jnp.int32)
            jobs = [(lb, t - 1 - lb * (LAG + 1))]

            def b_in():
                return xb_ref[pl.ds(pl.multiple_of(lb * seg, seg), seg), :]
        v0r = _cat([hc[0:n_mem], h_ref[n_mem:M2, :]])
        v1r = _cat([hc[n_mem:M2], h_ref[M2 + n_mem:2 * M2, :]])

        def ktiles(z):
            return [z[:, k * 128:(k + 1) * 128] for k in range(z.shape[1] // 128)]
        if full:
            hl = _Operands(ktiles(_cat([v0r, h_ref[2 * M2:RB, :]])), ktiles(_cat([v1r, h_ref[RB:RB + AH, :]])), None)
        else:
            hl = _Operands(None, None, ktiles(_cat([v0r, v1r, h_ref[2 * M2:RB, :]])))
        mh = 2 * M2 if full else 0

        def tile_dot(p, r):
            src = wr_ref.at[p] if r == 0 else w_ref.at[p * NG + r - 1]

            def dot(a, i):
                wt = src[i * 64:(i + 1) * 64, :]
                cnt[0] += 1
                if dl and cnt[0] >= dl[0][0]:
                    deps = dl.pop(0)[1]
                    wt = _cat([jnp.where(never, pltpu.bitcast(d, U32), wt[8 * e:8 * e + 8])
                               for e, d in enumerate(deps)] + [wt[8 * len(deps):]])
                return _nn(a, _upk(wt))
            return dot
        cnt, dl = [0], []
        never = t > 4 * n_seg
        scale = float(dh) ** (-0.5) * LOG2E
        if full:
            s_ = t - LAG
            rd = pl.multiple_of(lax.rem(s_ * (seg // 2), RS // 2), seg // 2)
            wa = pl.multiple_of(lax.rem((A0 - R0 + s_ * AH) // 2, RS // 2), 8)
        else:
            wx = pl.multiple_of(jnp.where(t < LAG, NPRE // 2 + t * (n_mem // 2), RS // 2), n_mem // 2)
            wo_store(S35, stage0_ref, wr_ref.at[3])

        RA = R if full else M2 + seg
        CW = R + 2 * M2 if full else R
        bidx = 0 if full else 2
        half = dh - 128
        la8 = lax.broadcasted_iota(jnp.int32, (n_mem, 128), 1) < half
        ones = jnp.full((n_mem, 128), 0xFFFFFFFF, U32)
        zero = jnp.zeros((n_mem, 128), U32)
        mask_a = jnp.where(la8, ones, zero)
        mask_b = jnp.where(la8, zero, ones)

        def pk2(a, b):
            return _pk(_cat([a, b]).astype(BF16))

        yt = [[None] * NT for _ in range(3)]

        def proj(p, r):
            pa, qa = {}, {}
            _fast_mm((S53 if r == 0 else S55)[1], hl, tile_dot(p, r), mh, pa, qa)
            n0 = 0 if r == 0 else RT + (r - 1) * GT
            for n in range(len(pa)):
                y, z, e = _fast_out(pa, qa, n, mh)
                idx = p * NT + n0 + n
                if full:
                    ring_ref[idx, pl.ds(wa, 8), :] = pk2(z[16:24], z[24:32])
                    y = _cat([y[0:M2], z[0:M2], y[M2:2 * M2]])
                else:
                    y = e
                    ring_ref[idx, pl.ds(wx, n_mem // 2), :] = pk2(y[0:8], y[8:16])[0:n_mem // 2]
                yt[p][n0 + n] = stash(p * 16 + (n0 + n) % 16, packed(p, (n0 + n) % 3, y))

        def ab(z8):
            return jnp.where(la8, z8, 0.0), jnp.where(la8, 0.0, z8)

        def packed(p, j, y):
            u2 = pk2(y[32:40], y[40:48])
            if p == 0 or j == 0:
                return [pk2(y[0:8], y[8:16]), pk2(y[16:24], y[24:32]), u2]
            if j == 2:
                return [pk2(y[8:16], y[0:8]), pk2(y[24:32], y[16:24]), u2]
            xa_a, xa_b = ab(y[8:16])
            out = [pk2(xa_b, xa_a), pk2(y[24:32], y[16:24]) & mask_b, pk2(y[16:24], y[24:32]) & mask_a, u2]
            if full:
                out += [pk2(*ab(y[0:8])), pk2(*ab(y[16:24]))]
            return out

        def stash(idx, parts):
            kv_ref[idx, 0:8 * len(parts), :] = _cat(parts)
            return lambda: [kv_ref[idx, 8 * e:8 * e + 8, :] for e in range(len(parts))]

        def pair(p, g):
            xs = [ring_ref[p * NT + 3 * g + j, pl.ds(rd, seg // 2), :] for j in range(3)] if full else None
            return [f() for f in yt[p][3 * g:3 * g + 3]], xs

        def q_rows(z, j):
            v0, v1, v2 = z[0][j]
            return [v0] + ([z[1][j]] if full else []) + [v1, v2]

        def kv_tiles(z):
            yt, x1 = z
            v0, v1, v2 = yt[0]
            t0 = [v0] + ([x1[0]] if full else [v1, v2]) + [v1, v2]
            w0, w1, w2 = yt[2]
            t2 = [w0, w1, w2] + ([x1[2]] if full else [w1, w2])
            if full:
                t0 += [v0, v1]
                t2 += [w0, w1]
            e1, mb, ma, u2 = yt[1][0:4]
            mid2 = [e1, mb, u2 & mask_b, ma, u2 & mask_a]
            mid1 = None
            if full:
                lo, hi = x1[1][0:8], x1[1][8:16]
                mid1 = [yt[1][4], lo & mask_a, hi & mask_a, lo & mask_b, hi & mask_b, e1, yt[1][5]]
            return t0, mid1, mid2, t2

        def mat(parts):
            return _upk(_cat(parts))

        def scores(q, k):
            k0, km1, km2, k2_ = kv_tiles(k)
            s_a = _nt(mat(q_rows(q, 0)), mat(k0))
            s_b = _nt(mat(q_rows(q, 2)), mat(k2_))
            qm = q_rows(q, 1)
            if full:
                s_m = _cat([_nt(mat(qm[0:2]), mat(km1)), _cat([_nt(mat(qm[2:4]), mat(km2)), jnp.zeros((seg, CW - R), F32)], axis=1)])
            else:
                s_m = _nt(mat(qm), mat(km2))
            out = []
            for e, sx in enumerate((s_a, s_b)):
                s = (sx + s_m) * scale + bias_ref[bidx + e, 0:RA, 0:CW]
                ex = jnp.exp2(s - jnp.max(s, axis=-1, keepdims=True))
                out.append(ex * _recip(jnp.sum(ex, axis=-1, keepdims=True)))
            return out

        def pv(p, v):
            v0, vm1, vm2, v2 = kv_tiles(v)
            o_a = _nn(p[0].astype(BF16), mat(v0))
            o_b = _nn(p[1].astype(BF16), mat(v2))
            p = p[0] + p[1]
            if full:
                o_m = _cat([_nn(p[0:M2 + seg].astype(BF16), mat(vm1)),
                            _nn(p[M2 + seg:R, 0:R].astype(BF16), mat(vm2))])
            else:
                o_m = _nn(p.astype(BF16), mat(vm2))
            return [o_a, o_m, o_b]

        ot = []
        pacc, qacc = {}, {}

        def add_o(r):
            n0 = 0 if r == 0 else RT + (r - 1) * GT
            oo = ot[n0:n0 + (RT if r == 0 else GT)]
            if full:
                ops = _Operands([o[0:32] for o in oo], [_cat([o[48:64], o[32:48]]) for o in oo],
                                [o[64:80] for o in oo])
            else:
                ops = _Operands(None, None, oo)
            _fast_mm((S35 if r == 0 else S55)[1], ops, tile_dot(3, r), mh, pacc, qacc)

        bqkv = [None] * 3
        probs = []

        def do_pv():
            for g in range(len(ot) // 3, len(probs)):
                ot.extend(pv(probs[g], pair(2, g)))

        for r in range(NG + 1):
            proj(2, r)
            proj(1, r)
            proj(0, r)
            if r == 0:
                blhs = _ln(b_in()).astype(BF16)
            if r < 3:
                bqkv[2 - r] = b_proj(blhs, 2 - r)
            if r == BAR:
                sink = []
                ob = b_attn(jobs, *bqkv, sink=sink)
                if BDL and full:
                    dl.extend((cnt[0] + BD0 + BDL * e, d) for e, d in enumerate(sink))
            if r == BOUT_R:
                zb = b_out(_cat(ob), b_in())
                x2_new = zb[0:seg]
                if full:
                    o_store(t - 1 - LAG, zb[seg:2 * seg])
                else:
                    o_store(lb * (t_last - LAG - 1) - 1, x2_new)
            if r in WSCHED:
                add_o(WSCHED[r])
            do_pv()
            for g in range(len(probs), (RT + r * GT) // 3):
                probs.append(scores(pair(0, g), pair(1, g)))
        for r in range(len(WSCHED), TAILPV):
            add_o(r)
        do_pv()
        for r in range(TAILPV, NG + 1):
            add_o(r)
        cols = []
        for n in range(nct):
            y, z, e = _fast_out(pacc, qacc, n, mh)
            cols.append(_cat([y, z[16:32], z[0:16], e]) if full else e)
        acc = _cat(cols, axis=1)

        y2 = x2_ref[...] + _cat([acc[n_mem:M2], acc[RA - seg + n_mem:RA]])
        mem2 = acc[RA - seg:RA - seg + n_mem]
        if full:
            x_cur = x_ref[pl.ds(pl.multiple_of(t * seg, seg), seg), :].astype(F32)
            xb_ref[0:seg, :] = x_cur + acc[M2:M2 + seg]
            xb_ref[seg:2 * seg, :] = y2
            m1n = acc[0:n_mem]
            m2n = mem2
            an = pl.multiple_of(jnp.minimum(A0 + (s_ + 1) * AH, S - AH), AH)
            h_ref[RB:RB + AH, :] = _ln(x_ref[pl.ds(an, AH), :].astype(F32))
            nxt = x2_new
        else:
            xb_ref[pl.ds(pl.multiple_of(jnp.where(t < LAG, 0, (t - n_seg + 2) * seg), seg), seg), :] = y2
            m1n = jnp.where(t < LAG - 1, h_ref[RB + AH:RB + AH + n_mem, :], mem2)
            m2n = jnp.where(t == LAG - 1, mem0_ref[...].astype(F32), mem2)
            nxt = jnp.where(t < LAG - 1, x_ref[seg:2 * seg, :].astype(F32), x2_new)
        x2_ref[...] = nxt
        sl = _ln(nxt)
        h_ref[n_mem:M2, :] = sl[0:n_mem]
        h_ref[M2 + n_mem:RB, :] = sl[n_mem:seg]
        return _cat([m1n, m2n])

    def single_body(t, c):
        @pl.when(t == n_seg)
        def _():
            out_copy(t - (LAG + 2)).start()
        return step(t, c, False)

    def full_body(t, c):
        @pl.when(t >= LAG + 2)
        def _():
            out_copy(t - (LAG + 2)).start()
        return step(t, c, True)

    def phase(ph, c):
        t0 = ph * n_seg
        c = lax.fori_loop(t0, t0 + LAG, single_body, c)

        @pl.when(ph == 0)
        def _():
            x_late.wait()
        return lax.fori_loop(LAG, jnp.where(ph == 0, n_seg, LAG), full_body, c)
    if not SKIPM:
      lax.fori_loop(0, 2, phase, _cat([h_ref[0:n_mem, :], h_ref[M2:M2 + n_mem, :]]))

    if SKIPM:
        def keep(i, c):
            z = (w_ref[i, pl.ds(pl.multiple_of(i * 8, 8), 8), :] + ring_ref[i, pl.ds(pl.multiple_of(i * 8, 8), 8), :]
                 + wr_ref[i & 3, pl.ds(pl.multiple_of(i * 8, 8), 8), :])
            xb_ref[2 * seg:2 * seg + 8, 0:128] = pltpu.bitcast(z, F32) + h_ref[pl.ds(pl.multiple_of((i & 7) * 8, 8), 8), 0:128] + x2_ref[0:8, 0:128]
            return c
        lax.fori_loop(0, 36, keep, 0)
    out_copy(n_seg - 3).start()
    res = xb_ref[2 * seg:4 * seg, :]
    blhs = _ln(res).astype(BF16)
    ob = b_attn([(1, n_seg - 2), (1, n_seg - 1)], *[b_proj(blhs, part) for part in range(3)])
    o_store(n_seg - 2, b_out(_cat(ob), res))
    out_copy(n_seg - 2).start()
    out_copy(n_seg - 1).start()
    pltpu.make_async_copy(o_ref.at[pl.ds(seg, S), :], out_hbm, sem_o).wait()


@functools.partial(jax.jit, static_argnames=("seg",))
def _run(A_x, A_mem0, A_Wq, A_Wk, A_Wv, A_Wo, B_wqkv, B_wo, *, seg):
    _, S, dm = A_x.shape
    n_heads, dh = A_Wq.shape[1], A_Wq.shape[2]
    n_mem = A_mem0.shape[1]
    n_seg = S // seg
    hd = n_heads * dh
    nct = dm // 128
    ng = (hd // 128 - RT) // GT
    assert (seg, n_seg, n_mem, dh, dm % 128, n_heads, LAG) == (32, 64, 8, 192, 0, 32, 2)

    x = A_x.reshape(S, dm)
    mem0 = A_mem0.reshape(n_mem, dm)
    wq = jnp.transpose(A_Wq, (1, 2, 0)).reshape(hd, dm)
    wk = jnp.transpose(A_Wk, (1, 2, 0)).reshape(hd, dm)
    wv = jnp.transpose(A_Wv, (1, 2, 0)).reshape(hd, dm)
    wo = A_Wo.reshape(hd, dm)
    _, _, _, _, rs, xc = _plan(seg, n_seg)

    kern = functools.partial(_kernel, seg=seg, n_seg=n_seg, n_mem=n_mem,
                             n_heads=n_heads, dh=dh, dm=dm)
    hbm = pl.BlockSpec(memory_space=pltpu.HBM)

    out = pl.pallas_call(
        kern,
        in_specs=[hbm] * 8,
        out_specs=hbm,
        out_shape=jax.ShapeDtypeStruct((S, dm), A_x.dtype),
        scratch_shapes=[
            pltpu.VMEM((S, dm), BF16),
            pltpu.VMEM((n_mem, dm), BF16),
            pltpu.VMEM((NSLOT, 4, GT * 128, dm), BF16),
            pltpu.VMEM((RT * 128, dm), BF16),
            pltpu.VMEM((4, len(S53[0]) * 64, 128), U32),
            pltpu.VMEM((4 * ng, len(S55[0]) * 64, 128), U32),
            pltpu.VMEM((dm, 4 * dm + 128), BF16),
            pltpu.VMEM((nct, 4 * dm + 32, 128), F32),
            pltpu.VMEM((4 * nct, dm // 2, 128), U32),
            pltpu.VMEM((len(KEYS_R), HC * xc // 4, 128), U32),
            pltpu.VMEM((len(KEYS_R), HC * xc // 4, 128), U32),
            pltpu.VMEM((len(KEYS) - len(KEYS_R), NXC * xc // 4, 128), U32),
            pltpu.VMEM((15, 8, 128), U32),
            pltpu.VMEM((3 * hd // 128, rs // 2 + 8, 128), U32),
            pltpu.VMEM((3 * n_mem + seg + AH, dm), F32),
            pltpu.VMEM((4 * seg, dm), F32),
            pltpu.VMEM((seg, dm), F32),
            pltpu.VMEM((2, nct, HIST + seg, 128), F32),
            pltpu.VMEM((2, nct, HIST + seg, 128), F32),
            pltpu.VMEM((S + seg, dm), A_x.dtype),
            pltpu.VMEM((4, 2 * n_mem + 2 * seg, 128), F32),
            pltpu.VMEM((48, 48, 128), U32),
            pltpu.SemaphoreType.DMA((NSLOT,)),
            pltpu.SemaphoreType.DMA((8 + NXC,)),
            pltpu.SemaphoreType.DMA((4,)),
            pltpu.SemaphoreType.DMA(()),
        ],
        compiler_params=pltpu.CompilerParams(
            vmem_limit_bytes=126 * 1024 * 1024,
            disable_bounds_checks=True,
        ),
    )(x, mem0, wq, wk, wv, wo, B_wqkv, B_wo)
    return out.reshape(1, S, dm)


def pallas_interleave_layers__memory_aug_recurrent_mem_tr__sliding_local_dilated__prompt_kernel(
    A_x: jax.Array,
    A_mem0: jax.Array,
    A_Wq: jax.Array,
    A_Wk: jax.Array,
    A_Wv: jax.Array,
    A_Wo: jax.Array,
    A_seg_len,
    B_x: jax.Array,
    B_wqkv: jax.Array,
    B_wo: jax.Array,
):
    del B_x
    seg = A_seg_len if isinstance(A_seg_len, int) else 32
    return _run(A_x, A_mem0, A_Wq, A_Wk, A_Wv, A_Wo, B_wqkv, B_wo, seg=seg)
```

```python
import functools

import jax
import jax.numpy as jnp
from jax import lax
import jax.experimental.pallas as pl
import jax.experimental.pallas.tpu as pltpu

F32 = jnp.float32
BF16 = jnp.bfloat16
U32 = jnp.uint32
NEG = -1000000000.0
LN_EPS = 1e-05
LOG2E = 1.4426950408889634
NEG2 = NEG * LOG2E

B_HEADS = 32
B_WIN = 8
B_DIL = 2
HIST = 16
SKIPM = int(0)
PACE = int(1)
BDL = int(0)
BD0 = int(40)
PB = int(60)
PB0 = int(100)
PC = int(0)
GO = int(50)
LZ = int(0)
GH = int(0)
GT8 = int(0)
GE = int(0)
BAR = int(3)
BO = int(5)
WS = '346789'
AH = 16
LAG = 2
NSLOT = 2
NXC = 6
HC = 3
WSCHED = dict((int(c), i) for i, c in enumerate(WS))
BOUT_R = BO
TAILPV = 8


def _ln(x):
    m = jnp.mean(x, axis=-1, keepdims=True)
    c = x - m
    v = jnp.mean(c * c, axis=-1, keepdims=True)
    return c * lax.rsqrt(v + LN_EPS)


def _recip(d):
    return pl.reciprocal(d, approx=True)


def _nt(a, b):
    return lax.dot_general(a, b, (((1,), (1,)), ((), ())), preferred_element_type=F32)


def _nn(a, b):
    return jnp.dot(a, b, preferred_element_type=F32)


def _cat(xs, axis=0):
    return xs[0] if len(xs) == 1 else jnp.concatenate(xs, axis=axis)


def _pk(z):
    return pltpu.bitcast(z, U32)


def _upk(z):
    return pltpu.bitcast(z, BF16)


LAM = (-1.5, -0.5, 0.0, 0.5, 1.5)


def _scheme(stars):
    tiles, prog = [], []
    for star in stars:
        if len(star) == 1:
            prog.append(("single", star[0], None, len(tiles)))
            tiles.append([star[0][:2]])
            continue
        left = [len(star) - 1] * len(star)
        for j in range(1, len(star)):
            for i in range(j):
                x, y = star[i], star[j]
                prog.append(("pair", x, y, len(tiles)))
                tiles += [[(x[0], y[1])], [(y[0], x[1])], [(x[0], y[1]), (y[0], x[1])]]
                for e in (i, j):
                    left[e] -= 1
                    if left[e] == 0:
                        z = star[e]
                        prog.append(("diag", z, None, len(tiles)))
                        tiles += [[z[:2]] + [(o[0], z[1]) for o in star if o is not z],
                                  [z[:2]] + [(z[0], o[1]) for o in star if o is not z]]
    return tiles, prog


S55 = _scheme([[(i, i, LAM[i]) for i in range(5)]])
S53 = _scheme([[(0, 0, LAM[0]), (2, 1, LAM[2]), (4, 2, LAM[4])], [(1, 0, LAM[1]), (3, 2, LAM[3])],
               [(1, 1, LAM[1])], [(3, 1, LAM[3])]])
S35 = _scheme([[(0, 0, LAM[0]), (1, 2, LAM[2]), (2, 4, LAM[4])], [(0, 1, LAM[1]), (2, 3, LAM[3])],
               [(1, 1, LAM[1])], [(1, 3, LAM[3])]])


def _spread(prog):
    pairs = [e for e in prog if e[0] != "diag"]
    diags = [e for e in prog if e[0] == "diag"]
    out, k = [], 0
    for i, e in enumerate(pairs):
        out.append(e)
        while k < len(diags) and (k + 0.5) * len(pairs) <= (i + 1) * len(diags):
            out.append(diags[k])
            k += 1
    return out + diags[k:]


def _op_keys(prog):
    keys = []
    for kind, x, y, _ in prog:
        if kind == "pair":
            new = [(nm, x[0], x[2], y[0], y[2]) for nm in ("l1", "l2", "A")]
        else:
            new = [("a", x[0], x[2]), ("b", x[0])]
        keys += [k for k in new if k not in keys]
    return keys


def _scaled(c, u):
    return u if c == 1.0 else c * u


class _Operands:
    def __init__(self, T, U, E, gate=None):
        if gate is not None:
            class Lazy:
                def __getitem__(lz, k):
                    return self._get(("u", k), lambda: gate(U[k]))
            self.U = Lazy()
        else:
            self.U = U
        self.T, self.E, self.memo = T, E, {}

    def _get(self, key, fn):
        if key not in self.memo:
            self.memo[key] = fn()
        return self.memo[key]

    def paired(self, key):
        T, U = self.T, self.U
        if key[0] == "b":
            return U[key[1]]
        if key[0] == "a":
            k, lam = key[1:]
            if lam == 0.0:
                return T[k]
            return self._get(("f",) + key, lambda: T[k] - _scaled(lam, U[k]) if lam > 0
                             else T[k] + _scaled(-lam, U[k]))
        kx, lx, ky, ly = key[1:]
        A = self._get(("f", "A") + key[1:],
                      lambda: self.paired(("a", kx, lx)) + self.paired(("a", ky, ly)))
        if key[0] == "A":
            return A
        return A - _scaled(ly - lx, U[kx]) if key[0] == "l1" else A + _scaled(ly - lx, U[ky])

    def extra(self, key):
        if key[0] == "a":
            return self.E[key[1]]
        return self._get(("e", key[1], key[3]), lambda: self.E[key[1]] + self.E[key[3]])

    def __call__(self, key):
        if self.T is None:
            ek = ("a", key[1]) if key[0] in ("a", "s") else ("l", key[1], 0, key[3])
            return self._get(ek, lambda: self.extra(ek).astype(BF16))

        def build():
            ak = ("a",) + key[1:] if key[0] == "s" else key
            parts = [self.paired(ak)]
            if self.E is not None and ak[0] in ("a", "l1", "l2"):
                parts.append(self.extra(ak))
            if key[0] == "s":
                parts.append(self.U[key[1]])
            return _cat(parts).astype(BF16)
        return self._get(key, build)


def _fast_mm(prog, op, dot, m, p, q):
    def add(d, key, val):
        d[key] = val if key not in d else d[key] + val

    for kind, x, y, i in prog:
        if kind == "pair":
            kk = (x[0], x[2], y[0], y[2])
            p1, p2 = dot(op(("l1",) + kk), i), dot(op(("l2",) + kk), i + 1)
            if m:
                r = _scaled(1.0 / (y[2] - x[2]), p2[0:m] - p1[0:m] + dot(op(("A",) + kk), i + 2))
                add(q, (x[1], x[2]), r)
                add(q, (y[1], y[2]), r)
            add(p, y[1], p1)
            add(p, x[1], p2)
        elif kind == "diag":
            add(p, x[1], dot(op(("a", x[0], x[2])), i))
            if m:
                add(q, (x[1], x[2]), dot(op(("b", x[0])), i + 1))
        else:
            r = dot(op(("s", x[0], x[2])), i)
            add(p, x[1], r[0:r.shape[0] - m])
            if m:
                add(q, (x[1], x[2]), r[r.shape[0] - m:])


def _fast_out(p, q, n, m):
    if not m:
        return None, None, p[n]
    y, z = p[n][0:m], None
    for (nn, lam), v in q.items():
        if nn == n:
            z = v if z is None else z + v
            if lam != 0.0:
                y = y + _scaled(lam, v) if lam > 0 else y - _scaled(-lam, v)
    return y, z, (p[n][m:] if p[n].shape[0] > m else None)


def _combo(tile, block):
    out = block(*tile[0])
    for kn in tile[1:]:
        out = out - block(*kn)
    return out


GT = 5
RT = 3
KEYS_R = _op_keys(S53[1])
KEYS = KEYS_R + [k for k in _op_keys(S55[1]) if k not in KEYS_R]


def _plan(seg, n_seg):
    S = seg * n_seg
    R0 = LAG * seg
    A0 = S - (n_seg - LAG) * AH
    NPRE = A0 - R0 - LAG * 8
    RS = -(-(A0 - R0 + AH) // seg) * seg
    XC = NPRE // NXC // 32 * 32
    assert XC * NXC + 16 == NPRE
    return S, R0, A0, NPRE, RS, XC


def _kernel(x_hbm, mem0_hbm, wq_hbm, wk_hbm, wv_hbm, wo_hbm, bqkv_hbm, bwo_hbm,
            out_hbm,
            x_ref, mem0_ref, stage_ref, stage0_ref, wr_ref, w_ref, bst_ref, btmp_ref, bw_ref,
            xla_ref, xlb_ref, xlc_ref, xe_ref, ring_ref, h_ref, xb_ref, x2_ref, kb_ref, vb_ref, o_ref, bias_ref, kv_ref,
            sem_w, sem_m, sem_b, sem_o,
            *, seg, n_seg, n_mem, n_heads, dh, dm):
    S, R0, A0, NPRE, RS, XC = _plan(seg, n_seg)
    M2 = 2 * n_mem
    R = M2 + 2 * seg
    RB = M2 + seg
    PW = 2 * dh
    G = n_heads // 2
    nct = dm // 128
    bdh = dm // B_HEADS
    NT = n_heads * dh // 128
    NG = (NT - RT) // GT
    w_hbm = (wq_hbm, wk_hbm, wv_hbm, wo_hbm)

    def w_copy(p, g):
        slot = g & (NSLOT - 1)
        return pltpu.make_async_copy(w_hbm[p].at[pl.ds((RT + (g - 1) * GT) * 128, GT * 128), :],
                                     stage_ref.at[slot, p], sem_w.at[slot])

    def w0_copy(p):
        dst = stage0_ref if p == 3 else stage_ref.at[0, p, pl.ds(0, RT * 128)]
        return pltpu.make_async_copy(w_hbm[p].at[pl.ds(0, RT * 128), :], dst, sem_m.at[4 + p])

    NB1 = 3 * nct
    WO0 = 3 * dm
    XF = A0 + AH
    XH = XC // 2

    def rows_copy(r0, n, sem):
        return pltpu.make_async_copy(x_hbm.at[pl.ds(r0, n), :], x_ref.at[pl.ds(r0, n), :], sem)

    def x_copy(i):
        return rows_copy(pl.multiple_of(R0 + i * XC, 16), XC, sem_m.at[8 + i])

    small = [rows_copy(0, R0, sem_m.at[1]), rows_copy(R0 + NPRE - 16, XF - R0 - NPRE + 16, sem_m.at[2]),
             pltpu.make_async_copy(mem0_hbm, mem0_ref, sem_m.at[3])]
    x_late = rows_copy(XF, S - XF, sem_m.at[0])

    def bq_copy(part):
        c0 = pl.multiple_of(part * dm, 128)
        return pltpu.make_async_copy(bqkv_hbm.at[:, pl.ds(c0, dm)], bst_ref.at[:, pl.ds(c0, dm)], sem_b.at[part])

    bo_copy = pltpu.make_async_copy(bwo_hbm, bst_ref.at[:, pl.ds(3 * dm, dm)], sem_b.at[3])

    def bst_tile(c):
        return bst_ref[:, pl.ds(pl.multiple_of(c * 128, 128), 128)]

    def bias_tables(full):
        RA = R if full else M2 + seg
        CW = 128
        ri = lax.broadcasted_iota(jnp.int32, (RA, CW), 0)
        ci = lax.broadcasted_iota(jnp.int32, (RA, CW), 1)
        if not full:
            ri = jnp.where(ri >= M2, ri + seg, ri)

        def table(i, bounds, vals):
            out = vals[-1]
            for b, v in zip(reversed(bounds), reversed(vals[:-1])):
                out = jnp.where(i < b, v, out)
            return out
        qi = ri - table(ri, [16, 48, 56], [0, 8, 48, 40])
        g0 = (ci < 8) | ((ci >= 16) & (ci < 48))
        k2 = ci - table(ci, [8, 24, 32, 48, 56, 80, 88, 96, 104], [-8, 0, 24, 8, 48, 40, 72, 80, 96, 104])
        if full:
            k1 = ci - table(ci, [8, 48], [0, 8, 40])
            row_l2 = ((ri >= 8) & (ri < 16)) | (ri >= 48)
            row_xa = (ri >= 8) & (ri < 16)
            valid = (row_xa == (ci >= 80)) & (ci < 112)
            is_a = jnp.where(ci >= 80, ((ci >= 88) & (ci < 104)).astype(jnp.int32),
                             (g0 != row_l2).astype(jnp.int32)) > 0
            ki = jnp.where(row_l2, k2, k1)
            visible = valid & ((qi < n_mem) | (qi >= ki))
            fill = jnp.where(valid, NEG2, -jnp.inf)
        else:
            is_a = jnp.logical_not(g0)
            visible = (qi < n_mem) | (qi >= k2)
            fill = NEG2
        for e, mine in enumerate((is_a, jnp.logical_not(is_a))):
            bias_ref[(0 if full else 2) + e, 0:RA, :] = jnp.where(
                mine, jnp.where(visible, 0.0, fill), -jnp.inf)

    for i in range(HC):
        x_copy(i).start()

    def zero_body(j, c):
        btmp_ref[j, 0:dm, :] = jnp.zeros((dm, 128), F32)
        return c
    lax.fori_loop(0, nct, zero_body, 0)

    w0_copy(0).start()
    xb_ref[0:2 * seg, :] = jnp.zeros((2 * seg, dm), F32)
    kb_ref[...] = jnp.zeros(kb_ref.shape, F32)
    vb_ref[...] = jnp.zeros(vb_ref.shape, F32)
    bst_ref[:, 4 * dm:] = jnp.zeros((dm, 128), BF16)
    bias_tables(True)
    bias_tables(False)

    def ekey(key):
        return ("a", key[1]) if key[0] == "a" else ("l", key[1], 0, key[3])
    EKEYS = []
    for key in KEYS:
        if key[0] in ("a", "l1") and ekey(key) not in EKEYS:
            EKEYS.append(ekey(key))

    def e_ops():
        ye = _ln(x_ref[R0 + NPRE - 16:R0 + NPRE, :].astype(F32))
        eops = _Operands(None, None, [ye[:, k * 128:(k + 1) * 128] for k in range(nct)])
        for j, key in enumerate(EKEYS):
            xe_ref[j] = _pk(eops(key))

    NKR = len(KEYS_R)

    def xl(j, hf, i):
        if j >= NKR:
            ref, j, i = xlc_ref, j - NKR, hf * HC + i
        else:
            ref = (xla_ref, xlb_ref)[hf]
        r0 = i * (XH // 2)
        return ref.at[j, pl.ds(r0 if isinstance(r0, int) else pl.multiple_of(r0, 8), XH // 2)]

    def ln_ops(hf, i, lo, hi):
        y = _ln(x_ref[pl.ds(pl.multiple_of(R0 + (hf * HC + i) * XC, 16), XC), :].astype(F32))
        ops = _Operands([y[0:XH, k * 128:(k + 1) * 128] for k in range(nct)],
                        [y[XH:XC, k * 128:(k + 1) * 128] for k in range(nct)], None)
        for j in range(lo, hi):
            xl(j, hf, i)[...] = _pk(ops(KEYS[j]))

    def ln_body(i, c):
        x_copy(i).wait()

        @pl.when(i == 0)
        def _():
            x_copy(HC).start()

        @pl.when(i == 1)
        def _():
            w0_copy(1).start()
            w0_copy(2).start()

        @pl.when(i == 2)
        def _():
            x_copy(HC + 1).start()
            x_copy(HC + 2).start()
            for cp in small:
                cp.start()
        ln_ops(0, i, 0, len(KEYS_R))
        return c
    lax.fori_loop(0, HC, ln_body, 0)

    def prep(scheme, w, dst):
        raw = lambda k, n: w[n * 128:(n + 1) * 128, k * 128:(k + 1) * 128]
        tb = []
        for i, tl in enumerate(scheme[0]):
            tb.append(raw(*tl[0]) if len(tl) == 1
                      else _combo(tl, lambda k, n: raw(k, n).astype(F32)).astype(BF16))
            tt = _pk(tb[i].T)
            dst[i * 64:(i + 1) * 64, :] = tt
            if len(tl) > 1:
                tdeps.append([tt[56:64]])
        return tb

    pcnt, pdl, tdeps = [0], [], []

    def pre_chunk(scheme, w, dst, n0, chunks, never=None, tb=None):
        tiles, prog = scheme
        prog = _spread(prog)
        dot = lambda a, i: _nn(a, _upk(dst[i * 64:(i + 1) * 64, :]))
        if w is not None:
            if tb is None:
                tb = prep(scheme, w, dst)
            dot = lambda a, i: _nt(a, tb[i])

        for c in chunks:
            def op(key):
                def ld(kk):
                    v = xl(KEYS.index(kk), c // HC, c % HC)[...]
                    if c == NXC - 1 and kk[0] in ("a", "l1", "l2"):
                        v = _cat([v, xe_ref[EKEYS.index(ekey(kk))]])
                    return v
                if key[0] == "s":
                    return _upk(_cat([ld(("a",) + key[1:]), ld(("b", key[1]))]))
                v = ld(key)
                pcnt[0] += 1
                pdl.sort(key=lambda e: e[0])
                if pdl and pcnt[0] >= pdl[0][0]:
                    deps = pdl.pop(0)[1]
                    v = _cat([jnp.where(never, d, v[8 * e:8 * e + 8]) for e, d in enumerate(deps)]
                             + ([v[8 * len(deps):]] if v.shape[0] > 8 * len(deps) else []))
                return _upk(v)
            p, q = {}, {}
            _fast_mm(prog, op, dot, XH, p, q)
            for n in range(len(p)):
                y, z, e = _fast_out(p, q, n, XH)
                ring_ref[n0 + n, c * XH:c * XH + XH // 2, :] = _pk(y.astype(BF16))
                ring_ref[n0 + n, c * XH + XH // 2:(c + 1) * XH, :] = _pk(z.astype(BF16))
                if e is not None:
                    ring_ref[n0 + n, NXC * XH:NXC * XH + 8, :] = _pk(e.astype(BF16))

    def init_rows():
        x0 = x_ref[0:seg, :].astype(F32)
        sl = _ln(x0)
        xt = _ln(x_ref[R0 + NPRE:XF, :].astype(F32))
        h_ref[0:n_mem, :] = xt[0:n_mem]
        h_ref[n_mem:M2, :] = sl[0:n_mem]
        h_ref[M2:M2 + n_mem, :] = mem0_ref[...].astype(F32)
        h_ref[M2 + n_mem:RB, :] = sl[n_mem:seg]
        h_ref[RB:RB + AH, :] = xt[M2:M2 + AH]
        h_ref[RB + AH:RB + AH + n_mem, :] = xt[n_mem:M2]
        x2_ref[...] = x0

    def first_a(p, c):
        buf = stage_ref.at[0, p, pl.ds(0, RT * 128)]
        pltpu.make_async_copy(buf, buf, sem_m.at[4 + p]).wait()
        x_copy(HC + p).wait()

        @pl.when(p == 0)
        def _():
            for pp in range(4):
                w_copy(pp, 1).start()

        @pl.when(p == 2)
        def _():
            bq_copy(0).start()
        ln_ops(1, p, 0, len(KEYS))
        pre_chunk(S53, buf, wr_ref.at[p], p * NT, range(HC))
        return c
    lax.fori_loop(0, 3, first_a, 0)
    for cp in small:
        cp.wait()

    def first_b(p, c):
        e_ops()
        init_rows()
        ln_ops(0, p, len(KEYS_R), len(KEYS))
        pre_chunk(S53, None, wr_ref.at[p], p * NT, range(HC, NXC))
        return c
    lax.fori_loop(0, 3, first_b, 0)

    dpt = 128 // B_HEADS

    def b_stage1(u):
        uc = jnp.clip(u, 0, NB1 - 1)
        tr = bst_tile(jnp.where(u >= 0, uc, NB1 + nct)).astype(F32).T
        r0 = pl.multiple_of(uc * 128, 128)
        for j in range(nct):
            btmp_ref[j, pl.ds(r0, 128), :] = tr[:, j * 128:(j + 1) * 128]
        return [pltpu.bitcast(tr[120:128, j * 128:(j + 1) * 128], U32) for j in range(nct)]

    def b_stage1_wo(u):
        uc = jnp.clip(u, 0, nct - 1)
        btmp_ref[uc, WO0:WO0 + dm, :] = bst_tile(jnp.where(u >= 0, NB1 + uc, NB1 + nct)).astype(F32)

    def b_stage2(u):
        uc = jnp.clip(u, 0, NB1 - 1)
        part = (uc >= nct).astype(jnp.int32) + (uc >= 2 * nct).astype(jnp.int32)
        r0 = part * dm + (uc - part * nct) * dpt
        rows = _cat([_cat([btmp_ref[j, pl.ds(r0 + dd, B_HEADS, stride=bdh), :]
                           for j in range(nct)], axis=1) for dd in range(dpt)])
        val = _pk(rows.T.astype(BF16))
        bw_ref[uc] = val
        return [val[64 * j + 56:64 * j + 64] for j in range(nct)]

    def b_stage2_wo(u):
        uc = jnp.clip(u, 0, nct - 1)
        r0 = jnp.where(u >= 0, WO0, 0)
        bw_ref[NB1 + uc] = _pk(
            _cat([btmp_ref[uc, pl.ds(r0 + d, B_HEADS, stride=bdh), :] for d in range(bdh)]).astype(BF16))

    def wo_store(scheme, w, dst, never=None):
        if scheme is S55:
            rawt = lambda k, n: w[k * 128:(k + 1) * 128, n * 128:(n + 1) * 128]
            plain = [i for i, tl in enumerate(scheme[0]) if len(tl) == 1]
            for i, tl in enumerate(scheme[0]):
                if len(tl) > 1:
                    val = _combo(tl, lambda k, n: rawt(k, n).astype(F32)).astype(BF16)
                    val = _pk(_upk(_pk(val.T)).T)
                    dst[i * 64:(i + 1) * 64, :] = val
                    j = plain.pop()
                    pv_ = _pk(rawt(*scheme[0][j][0]))
                    dst[j * 64:(j + 1) * 64, :] = jnp.where(never, val, pv_) if PACE else pv_
            return
        for r in range(0, 128, 16):
            memo = {}

            def raw(k, n):
                return w[k * 128 + r:k * 128 + r + 16, n * 128:(n + 1) * 128]

            def block(k, n):
                if (k, n) not in memo:
                    memo[k, n] = raw(k, n).astype(F32)
                return memo[k, n]
            for i, tl in enumerate(scheme[0]):
                val = raw(*tl[0]) if len(tl) == 1 else _combo(tl, block).astype(BF16)
                dst[i * 64 + r // 2:i * 64 + r // 2 + 8, :] = _pk(val)

    def pre_body(g, c):
        slot = g & (NSLOT - 1)
        buf = stage_ref.at[slot]
        pltpu.make_async_copy(buf, buf, sem_w.at[slot]).wait()

        @pl.when((g >= 2) & (g <= 4))
        def _():
            bq_copy(g - 2).wait()

        @pl.when(g == 4)
        def _():
            bo_copy.wait()

        @pl.when(g <= 2)
        def _():
            bq_copy(g).start()

        @pl.when(g == 2)
        def _():
            bo_copy.start()

        @pl.when(g + 1 <= NG)
        def _():
            for p in range(4):
                w_copy(p, g + 1).start()

        @pl.when(g == NG - 1)
        def _():
            w0_copy(3).start()
            x_late.start()

        wo_store(S55, stage_ref.at[slot, 3], w_ref.at[3 * NG + g - 1], g > NG + 5)
        deps = [b_stage2(3 * (g - 5) + e) for e in range(3)]
        b_stage2_wo(g - 5)
        deps += [b_stage1(3 * (g - 2) + e) for e in range(3)]
        b_stage1_wo(g - 4)
        pcnt[0] = 0
        if PB:
            pdl.extend((PB0 + PB * e, d) for e, d in enumerate(deps))
        tbs = [prep(S55, stage_ref.at[slot, 0], w_ref.at[g - 1])]
        for p in range(3):
            if p < 2:
                del tdeps[:]
                tbs.append(prep(S55, stage_ref.at[slot, p + 1], w_ref.at[(p + 1) * NG + g - 1]))
                if PC:
                    pdl.extend((pcnt[0] + 60 + PC * e, d) for e, d in enumerate(tdeps))
            pre_chunk(S55, stage_ref.at[slot, p], w_ref.at[p * NG + g - 1], p * NT + RT + (g - 1) * GT, range(NXC),
                      g > NG + 5, tbs[p])
        return c
    lax.fori_loop(1, NG + 1, pre_body, 0)
    w0_copy(3).wait()

    bscale = float(bdh) ** (-0.5) * LOG2E

    def b_proj(lhs, part):
        return _nn(lhs, _cat([_upk(bw_ref[part * nct + j]) for j in range(nct)], axis=1))

    def b_attn(jobs, q, k, v, sink=None):
        row = lax.broadcasted_iota(jnp.int32, (seg, 128), 0)
        outs = []
        for i, (l, sidx) in enumerate(jobs):
            r0 = i * seg
            pos = row + sidx * seg
            for j in range(nct):
                kb_ref[l, j, HIST:HIST + seg, :] = k[r0:r0 + seg, j * 128:(j + 1) * 128]
                vb_ref[l, j, HIST:HIST + seg, :] = v[r0:r0 + seg, j * 128:(j + 1) * 128]
            logits = []
            for w in range(B_WIN):
                o = HIST - w * B_DIL
                acc = None
                for j in range(nct):
                    p = q[r0:r0 + seg, j * 128:(j + 1) * 128] * kb_ref[l, j, o:o + seg, :]
                    acc = p if acc is None else acc + p
                acc = acc + pltpu.roll(acc, 64, 1)
                acc = acc + pltpu.roll(acc, 32, 1)
                lg = acc * bscale
                if w > 0:
                    lg = jnp.where(pos >= w * B_DIL, lg, NEG2)
                logits.append(lg)
            m = logits[0]
            for w in range(1, B_WIN):
                m = jnp.maximum(m, logits[w])
            es = [jnp.exp2(lg - m) for lg in logits]
            den = es[0]
            for w in range(1, B_WIN):
                den = den + es[w]
            inv = _recip(den)
            cols = []
            for j in range(nct):
                acc = None
                for w in range(B_WIN):
                    o = HIST - w * B_DIL
                    p = es[w] * vb_ref[l, j, o:o + seg, :]
                    acc = p if acc is None else acc + p
                cols.append(acc * inv)
            outs.append(_cat(cols, axis=1).astype(BF16))
            if sink is not None:
                for rg in range(0, seg, 8):
                    sink.append([c[rg:rg + 8] for c in cols])
            for j in range(nct):
                kb_ref[l, j, 0:HIST, :] = k[r0 + seg - HIST:r0 + seg, j * 128:(j + 1) * 128]
                vb_ref[l, j, 0:HIST, :] = v[r0 + seg - HIST:r0 + seg, j * 128:(j + 1) * 128]
        return outs

    def b_out(ob, res):
        return res + _nn(ob, _cat([_upk(bw_ref[NB1 + j]) for j in range(nct)], axis=1))

    def o_store(b, val):
        ro = pl.multiple_of((b + 1) * seg, seg)
        o_ref[pl.ds(ro, val.shape[0]), :] = val.astype(o_ref.dtype)

    def out_copy(b):
        ro = pl.multiple_of(b * seg, seg)
        return pltpu.make_async_copy(o_ref.at[pl.ds(ro + seg, seg), :], out_hbm.at[pl.ds(ro, seg), :], sem_o)

    def step(t, hc, full):
        t_last = n_seg + LAG - 1
        if full:
            jobs = [(0, t - 1), (1, t - 1 - LAG)]

            def b_in():
                return xb_ref[0:2 * seg, :]
        else:
            lb = (t == t_last).astype(jnp.int32)
            jobs = [(lb, t - 1 - lb * (LAG + 1))]

            def b_in():
                return xb_ref[pl.ds(pl.multiple_of(lb * seg, seg), seg), :]
        v0r = _cat([hc[0:n_mem], h_ref[n_mem:M2, :]])
        v1r = _cat([hc[n_mem:M2], h_ref[M2 + n_mem:2 * M2, :]])

        hist = []
        never = t > 4 * n_seg

        def gate(back, z):
            if not back or len(hist) < back:
                return z
            gv = hist[-back]
            return _cat([jnp.where(never, gv, z[e:e + 8]) for e in range(0, z.shape[0], 8)])

        def ktiles(z):
            return [z[:, k * 128:(k + 1) * 128] for k in range(z.shape[1] // 128)]
        if full:
            hl = _Operands(ktiles(_cat([v0r, h_ref[2 * M2:RB, :]])), ktiles(_cat([v1r, h_ref[RB:RB + AH, :]])), None)
        else:
            hl = _Operands(None, None, ktiles(_cat([v0r, v1r, h_ref[2 * M2:RB, :]])))
        mh = 2 * M2 if full else 0

        def tile_dot(p, r):
            src = wr_ref.at[p] if r == 0 else w_ref.at[p * NG + r - 1]

            def dot(a, i):
                wt = src[i * 64:(i + 1) * 64, :]
                cnt[0] += 1
                if dl and cnt[0] >= dl[0][0]:
                    deps = dl.pop(0)[1]
                    wt = _cat([jnp.where(never, pltpu.bitcast(d, U32), wt[8 * e:8 * e + 8])
                               for e, d in enumerate(deps)] + [wt[8 * len(deps):]])
                res_ = _nn(a, _upk(wt))
                hist.append(res_[0:8])
                return res_
            return dot
        cnt, dl = [0], []
        scale = float(dh) ** (-0.5) * LOG2E
        if full:
            s_ = t - LAG
            rd = pl.multiple_of(lax.rem(s_ * (seg // 2), RS // 2), seg // 2)
            wa = pl.multiple_of(lax.rem((A0 - R0 + s_ * AH) // 2, RS // 2), 8)
        else:
            wx = pl.multiple_of(jnp.where(t < LAG, NPRE // 2 + t * (n_mem // 2), RS // 2), n_mem // 2)
            wo_store(S35, stage0_ref, wr_ref.at[3])

        RA = R if full else M2 + seg
        CW = R + 2 * M2 if full else R
        bidx = 0 if full else 2
        half = dh - 128
        la8 = lax.broadcasted_iota(jnp.int32, (n_mem, 128), 1) < half
        ones = jnp.full((n_mem, 128), 0xFFFFFFFF, U32)
        zero = jnp.zeros((n_mem, 128), U32)
        mask_a = jnp.where(la8, ones, zero)
        mask_b = jnp.where(la8, zero, ones)

        def pk2(a, b):
            return _pk(_cat([a, b]).astype(BF16))

        yt = [[None] * NT for _ in range(3)]

        def proj(p, r):
            pa, qa = {}, {}
            _fast_mm((S53 if r == 0 else S55)[1], hl, tile_dot(p, r), mh, pa, qa)
            n0 = 0 if r == 0 else RT + (r - 1) * GT
            for n in range(len(pa)):
                y, z, e = _fast_out(pa, qa, n, mh)
                idx = p * NT + n0 + n
                if full:
                    ring_ref[idx, pl.ds(wa, 8), :] = pk2(z[16:24], z[24:32])
                    y = _cat([y[0:M2], z[0:M2], y[M2:2 * M2]])
                else:
                    y = e
                    ring_ref[idx, pl.ds(wx, n_mem // 2), :] = pk2(y[0:8], y[8:16])[0:n_mem // 2]
                yt[p][n0 + n] = stash(p * 16 + (n0 + n) % 16, packed(p, (n0 + n) % 3, y))

        def ab(z8):
            return jnp.where(la8, z8, 0.0), jnp.where(la8, 0.0, z8)

        def packed(p, j, y):
            u2 = pk2(y[32:40], y[40:48])
            if p == 0 or j == 0:
                return [pk2(y[0:8], y[8:16]), pk2(y[16:24], y[24:32]), u2]
            if j == 2:
                return [pk2(y[8:16], y[0:8]), pk2(y[24:32], y[16:24]), u2]
            xa_a, xa_b = ab(y[8:16])
            out = [pk2(xa_b, xa_a), pk2(y[24:32], y[16:24]) & mask_b, pk2(y[16:24], y[24:32]) & mask_a, u2]
            if full:
                out += [pk2(*ab(y[0:8])), pk2(*ab(y[16:24]))]
            return out

        def stash(idx, parts):
            kv_ref[idx, 0:8 * len(parts), :] = _cat(parts)
            return lambda: [kv_ref[idx, 8 * e:8 * e + 8, :] for e in range(len(parts))]

        def pair(p, g):
            xs = [ring_ref[p * NT + 3 * g + j, pl.ds(rd, seg // 2), :] for j in range(3)] if full else None
            return [f() for f in yt[p][3 * g:3 * g + 3]], xs

        def q_rows(z, j):
            v0, v1, v2 = z[0][j]
            return [v0] + ([z[1][j]] if full else []) + [v1, v2]

        def kv_tiles(z):
            yt, x1 = z
            v0, v1, v2 = yt[0]
            t0 = [v0] + ([x1[0]] if full else [v1, v2]) + [v1, v2]
            w0, w1, w2 = yt[2]
            t2 = [w0, w1, w2] + ([x1[2]] if full else [w1, w2])
            if full:
                t0 += [v0, v1]
                t2 += [w0, w1]
            e1, mb, ma, u2 = yt[1][0:4]
            mid2 = [e1, mb, u2 & mask_b, ma, u2 & mask_a]
            mid1 = None
            if full:
                lo, hi = x1[1][0:8], x1[1][8:16]
                mid1 = [yt[1][4], lo & mask_a, hi & mask_a, lo & mask_b, hi & mask_b, e1, yt[1][5]]
            return t0, mid1, mid2, t2

        def mat(parts):
            return _upk(_cat(parts))

        def scores(q, k):
            k0, km1, km2, k2_ = kv_tiles(k)
            s_a = _nt(mat(q_rows(q, 0)), mat(k0))
            s_b = _nt(mat(q_rows(q, 2)), mat(k2_))
            qm = q_rows(q, 1)
            if full:
                s_m = _cat([_nt(mat(qm[0:2]), mat(km1)), _cat([_nt(mat(qm[2:4]), mat(km2)), jnp.zeros((seg, CW - R), F32)], axis=1)])
            else:
                s_m = _nt(mat(qm), mat(km2))
            out = []
            for e, sx in enumerate((s_a, s_b)):
                s = (sx + s_m) * scale + bias_ref[bidx + e, 0:RA, 0:CW]
                ex = jnp.exp2(s - jnp.max(s, axis=-1, keepdims=True))
                out.append(ex * _recip(jnp.sum(ex, axis=-1, keepdims=True)))
            return out

        def pv(p, v):
            v0, vm1, vm2, v2 = kv_tiles(v)
            o_a = _nn(p[0].astype(BF16), mat(v0))
            o_b = _nn(p[1].astype(BF16), mat(v2))
            p = p[0] + p[1]
            if full:
                o_m = _cat([_nn(p[0:M2 + seg].astype(BF16), mat(vm1)),
                            _nn(p[M2 + seg:R, 0:R].astype(BF16), mat(vm2))])
            else:
                o_m = _nn(p.astype(BF16), mat(vm2))
            return [o_a, o_m, o_b]

        ot = []
        pacc, qacc = {}, {}

        def add_o(r):
            n0 = 0 if r == 0 else RT + (r - 1) * GT
            oo = ot[n0:n0 + (RT if r == 0 else GT)]
            if full:
                gt = (lambda z: z) if (r >= TAILPV and not GT8) else functools.partial(gate, GO)
                us = [_cat([o[48:64], o[32:48]]) for o in oo]
                if LZ:
                    ops = _Operands([o[0:32] for o in oo], us, [o[64:80] for o in oo], gt)
                else:
                    ops = _Operands([o[0:32] for o in oo], [gt(z) for z in us], [o[64:80] for o in oo])
            else:
                ops = _Operands(None, None, oo)
            _fast_mm((S35 if r == 0 else S55)[1], ops, tile_dot(3, r), mh, pacc, qacc)

        bqkv = [None] * 3
        probs = []

        def do_pv():
            for g in range(len(ot) // 3, len(probs)):
                ot.extend(pv(probs[g], pair(2, g)))

        for r in range(NG + 1):
            proj(2, r)
            proj(1, r)
            proj(0, r)
            if r == 0:
                blhs = _ln(b_in()).astype(BF16)
            if r < 3:
                bqkv[2 - r] = b_proj(blhs, 2 - r)
            if r == BAR:
                sink = []
                ob = b_attn(jobs, *bqkv, sink=sink)
                if BDL and full:
                    dl.extend((cnt[0] + BD0 + BDL * e, d) for e, d in enumerate(sink))
            if r == BOUT_R:
                zb = b_out(_cat(ob), b_in())
                x2_new = zb[0:seg]
                if full:
                    o_store(t - 1 - LAG, zb[seg:2 * seg])
                else:
                    o_store(lb * (t_last - LAG - 1) - 1, x2_new)
            if r in WSCHED:
                add_o(WSCHED[r])
            do_pv()
            for g in range(len(probs), (RT + r * GT) // 3):
                probs.append(scores(pair(0, g), pair(1, g)))
        for r in range(len(WSCHED), TAILPV):
            add_o(r)
        do_pv()
        for r in range(TAILPV, NG + 1):
            add_o(r)
        cols = []
        for n in range(nct):
            y, z, e = _fast_out(pacc, qacc, n, mh)
            cols.append(_cat([y, z[16:32], z[0:16], e]) if full else e)
        acc = _cat(cols, axis=1)

        y2 = x2_ref[...] + _cat([acc[n_mem:M2], acc[RA - seg + n_mem:RA]])
        mem2 = acc[RA - seg:RA - seg + n_mem]
        if full:
            x_cur = x_ref[pl.ds(pl.multiple_of(t * seg, seg), seg), :].astype(F32)
            xb_ref[0:seg, :] = x_cur + acc[M2:M2 + seg]
            xb_ref[seg:2 * seg, :] = y2
            m1n = acc[0:n_mem]
            m2n = mem2
            an = pl.multiple_of(jnp.minimum(A0 + (s_ + 1) * AH, S - AH), AH)
            h_ref[RB:RB + AH, :] = _ln(x_ref[pl.ds(an, AH), :].astype(F32))
            nxt = x2_new
        else:
            xb_ref[pl.ds(pl.multiple_of(jnp.where(t < LAG, 0, (t - n_seg + 2) * seg), seg), seg), :] = y2
            m1n = jnp.where(t < LAG - 1, h_ref[RB + AH:RB + AH + n_mem, :], mem2)
            m2n = jnp.where(t == LAG - 1, mem0_ref[...].astype(F32), mem2)
            nxt = jnp.where(t < LAG - 1, x_ref[seg:2 * seg, :].astype(F32), x2_new)
        x2_ref[...] = nxt
        sl = _ln(nxt)
        h_ref[n_mem:M2, :] = sl[0:n_mem]
        h_ref[M2 + n_mem:RB, :] = sl[n_mem:seg]
        return _cat([m1n, m2n])

    def single_body(t, c):
        @pl.when(t == n_seg)
        def _():
            out_copy(t - (LAG + 2)).start()
        return step(t, c, False)

    def full_body(t, c):
        @pl.when(t >= LAG + 2)
        def _():
            out_copy(t - (LAG + 2)).start()
        return step(t, c, True)

    def phase(ph, c):
        t0 = ph * n_seg
        c = lax.fori_loop(t0, t0 + LAG, single_body, c)

        @pl.when(ph == 0)
        def _():
            x_late.wait()
        return lax.fori_loop(LAG, jnp.where(ph == 0, n_seg, LAG), full_body, c)
    if not SKIPM:
      lax.fori_loop(0, 2, phase, _cat([h_ref[0:n_mem, :], h_ref[M2:M2 + n_mem, :]]))

    if SKIPM:
        def keep(i, c):
            z = (w_ref[i, pl.ds(pl.multiple_of(i * 8, 8), 8), :] + ring_ref[i, pl.ds(pl.multiple_of(i * 8, 8), 8), :]
                 + wr_ref[i & 3, pl.ds(pl.multiple_of(i * 8, 8), 8), :])
            xb_ref[2 * seg:2 * seg + 8, 0:128] = pltpu.bitcast(z, F32) + h_ref[pl.ds(pl.multiple_of((i & 7) * 8, 8), 8), 0:128] + x2_ref[0:8, 0:128]
            return c
        lax.fori_loop(0, 36, keep, 0)
    out_copy(n_seg - 3).start()
    res = xb_ref[2 * seg:4 * seg, :]
    blhs = _ln(res).astype(BF16)
    ob = b_attn([(1, n_seg - 2), (1, n_seg - 1)], *[b_proj(blhs, part) for part in range(3)])
    o_store(n_seg - 2, b_out(_cat(ob), res))
    out_copy(n_seg - 2).start()
    out_copy(n_seg - 1).start()
    pltpu.make_async_copy(o_ref.at[pl.ds(seg, S), :], out_hbm, sem_o).wait()


@functools.partial(jax.jit, static_argnames=("seg",))
def _run(A_x, A_mem0, A_Wq, A_Wk, A_Wv, A_Wo, B_wqkv, B_wo, *, seg):
    _, S, dm = A_x.shape
    n_heads, dh = A_Wq.shape[1], A_Wq.shape[2]
    n_mem = A_mem0.shape[1]
    n_seg = S // seg
    hd = n_heads * dh
    nct = dm // 128
    ng = (hd // 128 - RT) // GT
    assert (seg, n_seg, n_mem, dh, dm % 128, n_heads, LAG) == (32, 64, 8, 192, 0, 32, 2)

    x = A_x.reshape(S, dm)
    mem0 = A_mem0.reshape(n_mem, dm)
    wq = jnp.transpose(A_Wq, (1, 2, 0)).reshape(hd, dm)
    wk = jnp.transpose(A_Wk, (1, 2, 0)).reshape(hd, dm)
    wv = jnp.transpose(A_Wv, (1, 2, 0)).reshape(hd, dm)
    wo = A_Wo.reshape(hd, dm)
    _, _, _, _, rs, xc = _plan(seg, n_seg)

    kern = functools.partial(_kernel, seg=seg, n_seg=n_seg, n_mem=n_mem,
                             n_heads=n_heads, dh=dh, dm=dm)
    hbm = pl.BlockSpec(memory_space=pltpu.HBM)

    out = pl.pallas_call(
        kern,
        in_specs=[hbm] * 8,
        out_specs=hbm,
        out_shape=jax.ShapeDtypeStruct((S, dm), A_x.dtype),
        scratch_shapes=[
            pltpu.VMEM((S, dm), BF16),
            pltpu.VMEM((n_mem, dm), BF16),
            pltpu.VMEM((NSLOT, 4, GT * 128, dm), BF16),
            pltpu.VMEM((RT * 128, dm), BF16),
            pltpu.VMEM((4, len(S53[0]) * 64, 128), U32),
            pltpu.VMEM((4 * ng, len(S55[0]) * 64, 128), U32),
            pltpu.VMEM((dm, 4 * dm + 128), BF16),
            pltpu.VMEM((nct, 4 * dm + 32, 128), F32),
            pltpu.VMEM((4 * nct, dm // 2, 128), U32),
            pltpu.VMEM((len(KEYS_R), HC * xc // 4, 128), U32),
            pltpu.VMEM((len(KEYS_R), HC * xc // 4, 128), U32),
            pltpu.VMEM((len(KEYS) - len(KEYS_R), NXC * xc // 4, 128), U32),
            pltpu.VMEM((15, 8, 128), U32),
            pltpu.VMEM((3 * hd // 128, rs // 2 + 8, 128), U32),
            pltpu.VMEM((3 * n_mem + seg + AH, dm), F32),
            pltpu.VMEM((4 * seg, dm), F32),
            pltpu.VMEM((seg, dm), F32),
            pltpu.VMEM((2, nct, HIST + seg, 128), F32),
            pltpu.VMEM((2, nct, HIST + seg, 128), F32),
            pltpu.VMEM((S + seg, dm), A_x.dtype),
            pltpu.VMEM((4, 2 * n_mem + 2 * seg, 128), F32),
            pltpu.VMEM((48, 48, 128), U32),
            pltpu.SemaphoreType.DMA((NSLOT,)),
            pltpu.SemaphoreType.DMA((8 + NXC,)),
            pltpu.SemaphoreType.DMA((4,)),
            pltpu.SemaphoreType.DMA(()),
        ],
        compiler_params=pltpu.CompilerParams(
            vmem_limit_bytes=126 * 1024 * 1024,
            disable_bounds_checks=True,
        ),
    )(x, mem0, wq, wk, wv, wo, B_wqkv, B_wo)
    return out.reshape(1, S, dm)


def pallas_interleave_layers__memory_aug_recurrent_mem_tr__sliding_local_dilated__prompt_kernel(
    A_x: jax.Array,
    A_mem0: jax.Array,
    A_Wq: jax.Array,
    A_Wk: jax.Array,
    A_Wv: jax.Array,
    A_Wo: jax.Array,
    A_seg_len,
    B_x: jax.Array,
    B_wqkv: jax.Array,
    B_wo: jax.Array,
):
    del B_x
    seg = A_seg_len if isinstance(A_seg_len, int) else 32
    return _run(A_x, A_mem0, A_Wq, A_Wk, A_Wv, A_Wo, B_wqkv, B_wo, seg=seg)
```

```python
import functools

import jax
import jax.numpy as jnp
from jax import lax
import jax.experimental.pallas as pl
import jax.experimental.pallas.tpu as pltpu

F32 = jnp.float32
BF16 = jnp.bfloat16
U32 = jnp.uint32
NEG = -1000000000.0
LN_EPS = 1e-05
LOG2E = 1.4426950408889634
NEG2 = NEG * LOG2E

B_HEADS = 32
B_WIN = 8
B_DIL = 2
HIST = 16
SKIPM = int(0)
PACE = int(1)
BDL = int(0)
BD0 = int(40)
PB = int(60)
PB0 = int(100)
PC = int(0)
GO = int(40)
LZ = int(0)
GH = int(0)
GT8 = int(0)
LD = int(150)
LDA = int(0)
HS = int(1)
GE = int(0)
BAR = int(3)
BO = int(5)
WS = '346789'
AH = 16
LAG = 2
NSLOT = 2
NXC = 6
HC = 3
WSCHED = dict((int(c), i) for i, c in enumerate(WS))
BOUT_R = BO
TAILPV = 8


def _ln(x):
    m = jnp.mean(x, axis=-1, keepdims=True)
    c = x - m
    v = jnp.mean(c * c, axis=-1, keepdims=True)
    return c * lax.rsqrt(v + LN_EPS)


def _recip(d):
    return pl.reciprocal(d, approx=True)


def _nt(a, b):
    return lax.dot_general(a, b, (((1,), (1,)), ((), ())), preferred_element_type=F32)


def _nn(a, b):
    return jnp.dot(a, b, preferred_element_type=F32)


def _cat(xs, axis=0):
    return xs[0] if len(xs) == 1 else jnp.concatenate(xs, axis=axis)


def _pk(z):
    return pltpu.bitcast(z, U32)


def _upk(z):
    return pltpu.bitcast(z, BF16)


LAM = (-1.5, -0.5, 0.0, 0.5, 1.5)


def _scheme(stars):
    tiles, prog = [], []
    for star in stars:
        if len(star) == 1:
            prog.append(("single", star[0], None, len(tiles)))
            tiles.append([star[0][:2]])
            continue
        left = [len(star) - 1] * len(star)
        for j in range(1, len(star)):
            for i in range(j):
                x, y = star[i], star[j]
                prog.append(("pair", x, y, len(tiles)))
                tiles += [[(x[0], y[1])], [(y[0], x[1])], [(x[0], y[1]), (y[0], x[1])]]
                for e in (i, j):
                    left[e] -= 1
                    if left[e] == 0:
                        z = star[e]
                        prog.append(("diag", z, None, len(tiles)))
                        tiles += [[z[:2]] + [(o[0], z[1]) for o in star if o is not z],
                                  [z[:2]] + [(z[0], o[1]) for o in star if o is not z]]
    return tiles, prog


S55 = _scheme([[(i, i, LAM[i]) for i in range(5)]])
S53 = _scheme([[(0, 0, LAM[0]), (2, 1, LAM[2]), (4, 2, LAM[4])], [(1, 0, LAM[1]), (3, 2, LAM[3])],
               [(1, 1, LAM[1])], [(3, 1, LAM[3])]])
S35 = _scheme([[(0, 0, LAM[0]), (1, 2, LAM[2]), (2, 4, LAM[4])], [(0, 1, LAM[1]), (2, 3, LAM[3])],
               [(1, 1, LAM[1])], [(1, 3, LAM[3])]])


def _spread(prog):
    pairs = [e for e in prog if e[0] != "diag"]
    diags = [e for e in prog if e[0] == "diag"]
    out, k = [], 0
    for i, e in enumerate(pairs):
        out.append(e)
        while k < len(diags) and (k + 0.5) * len(pairs) <= (i + 1) * len(diags):
            out.append(diags[k])
            k += 1
    return out + diags[k:]


def _op_keys(prog):
    keys = []
    for kind, x, y, _ in prog:
        if kind == "pair":
            new = [(nm, x[0], x[2], y[0], y[2]) for nm in ("l1", "l2", "A")]
        else:
            new = [("a", x[0], x[2]), ("b", x[0])]
        keys += [k for k in new if k not in keys]
    return keys


def _scaled(c, u):
    return u if c == 1.0 else c * u


class _Operands:
    def __init__(self, T, U, E, gate=None):
        if gate is not None:
            class Lazy:
                def __getitem__(lz, k):
                    return self._get(("u", k), lambda: gate(U[k]))
            self.U = Lazy()
        else:
            self.U = U
        self.T, self.E, self.memo = T, E, {}

    def _get(self, key, fn):
        if key not in self.memo:
            self.memo[key] = fn()
        return self.memo[key]

    def paired(self, key):
        T, U = self.T, self.U
        if key[0] == "b":
            return U[key[1]]
        if key[0] == "a":
            k, lam = key[1:]
            if lam == 0.0:
                return T[k]
            return self._get(("f",) + key, lambda: T[k] - _scaled(lam, U[k]) if lam > 0
                             else T[k] + _scaled(-lam, U[k]))
        kx, lx, ky, ly = key[1:]
        A = self._get(("f", "A") + key[1:],
                      lambda: self.paired(("a", kx, lx)) + self.paired(("a", ky, ly)))
        if key[0] == "A":
            return A
        return A - _scaled(ly - lx, U[kx]) if key[0] == "l1" else A + _scaled(ly - lx, U[ky])

    def extra(self, key):
        if key[0] == "a":
            return self.E[key[1]]
        return self._get(("e", key[1], key[3]), lambda: self.E[key[1]] + self.E[key[3]])

    def __call__(self, key):
        if self.T is None:
            ek = ("a", key[1]) if key[0] in ("a", "s") else ("l", key[1], 0, key[3])
            return self._get(ek, lambda: self.extra(ek).astype(BF16))

        def build():
            ak = ("a",) + key[1:] if key[0] == "s" else key
            parts = [self.paired(ak)]
            if self.E is not None and ak[0] in ("a", "l1", "l2"):
                parts.append(self.extra(ak))
            if key[0] == "s":
                parts.append(self.U[key[1]])
            return _cat(parts).astype(BF16)
        return self._get(key, build)


def _fast_mm(prog, op, dot, m, p, q):
    def add(d, key, val):
        d[key] = val if key not in d else d[key] + val

    for kind, x, y, i in prog:
        if kind == "pair":
            kk = (x[0], x[2], y[0], y[2])
            p1, p2 = dot(op(("l1",) + kk), i), dot(op(("l2",) + kk), i + 1)
            if m:
                r = _scaled(1.0 / (y[2] - x[2]), p2[0:m] - p1[0:m] + dot(op(("A",) + kk), i + 2))
                add(q, (x[1], x[2]), r)
                add(q, (y[1], y[2]), r)
            add(p, y[1], p1)
            add(p, x[1], p2)
        elif kind == "diag":
            add(p, x[1], dot(op(("a", x[0], x[2])), i))
            if m:
                add(q, (x[1], x[2]), dot(op(("b", x[0])), i + 1))
        else:
            r = dot(op(("s", x[0], x[2])), i)
            add(p, x[1], r[0:r.shape[0] - m])
            if m:
                add(q, (x[1], x[2]), r[r.shape[0] - m:])


def _fast_out(p, q, n, m):
    if not m:
        return None, None, p[n]
    y, z = p[n][0:m], None
    for (nn, lam), v in q.items():
        if nn == n:
            z = v if z is None else z + v
            if lam != 0.0:
                y = y + _scaled(lam, v) if lam > 0 else y - _scaled(-lam, v)
    return y, z, (p[n][m:] if p[n].shape[0] > m else None)


def _combo(tile, block):
    out = block(*tile[0])
    for kn in tile[1:]:
        out = out - block(*kn)
    return out


GT = 5
RT = 3
KEYS_R = _op_keys(S53[1])
KEYS = KEYS_R + [k for k in _op_keys(S55[1]) if k not in KEYS_R]


def _plan(seg, n_seg):
    S = seg * n_seg
    R0 = LAG * seg
    A0 = S - (n_seg - LAG) * AH
    NPRE = A0 - R0 - LAG * 8
    RS = -(-(A0 - R0 + AH) // seg) * seg
    XC = NPRE // NXC // 32 * 32
    assert XC * NXC + 16 == NPRE
    return S, R0, A0, NPRE, RS, XC


def _kernel(x_hbm, mem0_hbm, wq_hbm, wk_hbm, wv_hbm, wo_hbm, bqkv_hbm, bwo_hbm,
            out_hbm,
            x_ref, mem0_ref, stage_ref, stage0_ref, wr_ref, w_ref, bst_ref, btmp_ref, bw_ref,
            xla_ref, xlb_ref, xlc_ref, xe_ref, ring_ref, h_ref, xb_ref, x2_ref, kb_ref, vb_ref, o_ref, bias_ref, kv_ref,
            sem_w, sem_m, sem_b, sem_o,
            *, seg, n_seg, n_mem, n_heads, dh, dm):
    S, R0, A0, NPRE, RS, XC = _plan(seg, n_seg)
    M2 = 2 * n_mem
    R = M2 + 2 * seg
    RB = M2 + seg
    PW = 2 * dh
    G = n_heads // 2
    nct = dm // 128
    bdh = dm // B_HEADS
    NT = n_heads * dh // 128
    NG = (NT - RT) // GT
    w_hbm = (wq_hbm, wk_hbm, wv_hbm, wo_hbm)

    def w_copy(p, g):
        slot = g & (NSLOT - 1)
        return pltpu.make_async_copy(w_hbm[p].at[pl.ds((RT + (g - 1) * GT) * 128, GT * 128), :],
                                     stage_ref.at[slot, p], sem_w.at[slot])

    def w0_copy(p):
        dst = stage0_ref if p == 3 else stage_ref.at[0, p, pl.ds(0, RT * 128)]
        return pltpu.make_async_copy(w_hbm[p].at[pl.ds(0, RT * 128), :], dst, sem_m.at[4 + p])

    NB1 = 3 * nct
    WO0 = 3 * dm
    XF = A0 + AH
    XH = XC // 2

    def rows_copy(r0, n, sem):
        return pltpu.make_async_copy(x_hbm.at[pl.ds(r0, n), :], x_ref.at[pl.ds(r0, n), :], sem)

    def x_copy(i):
        return rows_copy(pl.multiple_of(R0 + i * XC, 16), XC, sem_m.at[8 + i])

    small = [rows_copy(0, R0, sem_m.at[1]), rows_copy(R0 + NPRE - 16, XF - R0 - NPRE + 16, sem_m.at[2]),
             pltpu.make_async_copy(mem0_hbm, mem0_ref, sem_m.at[3])]
    x_late = rows_copy(XF, S - XF, sem_m.at[0])

    def bq_copy(part):
        c0 = pl.multiple_of(part * dm, 128)
        return pltpu.make_async_copy(bqkv_hbm.at[:, pl.ds(c0, dm)], bst_ref.at[:, pl.ds(c0, dm)], sem_b.at[part])

    bo_copy = pltpu.make_async_copy(bwo_hbm, bst_ref.at[:, pl.ds(3 * dm, dm)], sem_b.at[3])

    def bst_tile(c):
        return bst_ref[:, pl.ds(pl.multiple_of(c * 128, 128), 128)]

    def bias_tables(full):
        RA = R if full else M2 + seg
        CW = 128
        ri = lax.broadcasted_iota(jnp.int32, (RA, CW), 0)
        ci = lax.broadcasted_iota(jnp.int32, (RA, CW), 1)
        if not full:
            ri = jnp.where(ri >= M2, ri + seg, ri)

        def table(i, bounds, vals):
            out = vals[-1]
            for b, v in zip(reversed(bounds), reversed(vals[:-1])):
                out = jnp.where(i < b, v, out)
            return out
        qi = ri - table(ri, [16, 48, 56], [0, 8, 48, 40])
        g0 = (ci < 8) | ((ci >= 16) & (ci < 48))
        k2 = ci - table(ci, [8, 24, 32, 48, 56, 80, 88, 96, 104], [-8, 0, 24, 8, 48, 40, 72, 80, 96, 104])
        if full:
            k1 = ci - table(ci, [8, 48], [0, 8, 40])
            row_l2 = ((ri >= 8) & (ri < 16)) | (ri >= 48)
            row_xa = (ri >= 8) & (ri < 16)
            valid = (row_xa == (ci >= 80)) & (ci < 112)
            is_a = jnp.where(ci >= 80, ((ci >= 88) & (ci < 104)).astype(jnp.int32),
                             (g0 != row_l2).astype(jnp.int32)) > 0
            ki = jnp.where(row_l2, k2, k1)
            visible = valid & ((qi < n_mem) | (qi >= ki))
            fill = jnp.where(valid, NEG2, -jnp.inf)
        else:
            is_a = jnp.logical_not(g0)
            visible = (qi < n_mem) | (qi >= k2)
            fill = NEG2
        for e, mine in enumerate((is_a, jnp.logical_not(is_a))):
            bias_ref[(0 if full else 2) + e, 0:RA, :] = jnp.where(
                mine, jnp.where(visible, 0.0, fill), -jnp.inf)

    for i in range(HC):
        x_copy(i).start()

    def zero_body(j, c):
        btmp_ref[j, 0:dm, :] = jnp.zeros((dm, 128), F32)
        return c
    lax.fori_loop(0, nct, zero_body, 0)

    w0_copy(0).start()
    xb_ref[0:2 * seg, :] = jnp.zeros((2 * seg, dm), F32)
    kb_ref[...] = jnp.zeros(kb_ref.shape, F32)
    vb_ref[...] = jnp.zeros(vb_ref.shape, F32)
    bst_ref[:, 4 * dm:] = jnp.zeros((dm, 128), BF16)
    bias_tables(True)
    bias_tables(False)

    def ekey(key):
        return ("a", key[1]) if key[0] == "a" else ("l", key[1], 0, key[3])
    EKEYS = []
    for key in KEYS:
        if key[0] in ("a", "l1") and ekey(key) not in EKEYS:
            EKEYS.append(ekey(key))

    def e_ops():
        ye = _ln(x_ref[R0 + NPRE - 16:R0 + NPRE, :].astype(F32))
        eops = _Operands(None, None, [ye[:, k * 128:(k + 1) * 128] for k in range(nct)])
        for j, key in enumerate(EKEYS):
            xe_ref[j] = _pk(eops(key))

    NKR = len(KEYS_R)

    def xl(j, hf, i):
        if j >= NKR:
            ref, j, i = xlc_ref, j - NKR, hf * HC + i
        else:
            ref = (xla_ref, xlb_ref)[hf]
        r0 = i * (XH // 2)
        return ref.at[j, pl.ds(r0 if isinstance(r0, int) else pl.multiple_of(r0, 8), XH // 2)]

    def ln_ops(hf, i, lo, hi):
        y = _ln(x_ref[pl.ds(pl.multiple_of(R0 + (hf * HC + i) * XC, 16), XC), :].astype(F32))
        ops = _Operands([y[0:XH, k * 128:(k + 1) * 128] for k in range(nct)],
                        [y[XH:XC, k * 128:(k + 1) * 128] for k in range(nct)], None)
        for j in range(lo, hi):
            xl(j, hf, i)[...] = _pk(ops(KEYS[j]))

    def ln_body(i, c):
        x_copy(i).wait()

        @pl.when(i == 0)
        def _():
            x_copy(HC).start()

        @pl.when(i == 1)
        def _():
            w0_copy(1).start()
            w0_copy(2).start()

        @pl.when(i == 2)
        def _():
            x_copy(HC + 1).start()
            x_copy(HC + 2).start()
            for cp in small:
                cp.start()
        ln_ops(0, i, 0, len(KEYS_R))
        return c
    lax.fori_loop(0, HC, ln_body, 0)

    def prep(scheme, w, dst):
        raw = lambda k, n: w[n * 128:(n + 1) * 128, k * 128:(k + 1) * 128]
        tb = []
        for i, tl in enumerate(scheme[0]):
            tb.append(raw(*tl[0]) if len(tl) == 1
                      else _combo(tl, lambda k, n: raw(k, n).astype(F32)).astype(BF16))
            tt = _pk(tb[i].T)
            dst[i * 64:(i + 1) * 64, :] = tt
            if len(tl) > 1:
                tdeps.append([tt[56:64]])
        return tb

    pcnt, pdl, tdeps = [0], [], []

    def pre_chunk(scheme, w, dst, n0, chunks, never=None, tb=None):
        tiles, prog = scheme
        prog = _spread(prog)
        dot = lambda a, i: _nn(a, _upk(dst[i * 64:(i + 1) * 64, :]))
        if w is not None:
            if tb is None:
                tb = prep(scheme, w, dst)
            dot = lambda a, i: _nt(a, tb[i])

        for c in chunks:
            def op(key):
                def ld(kk):
                    v = xl(KEYS.index(kk), c // HC, c % HC)[...]
                    if c == NXC - 1 and kk[0] in ("a", "l1", "l2"):
                        v = _cat([v, xe_ref[EKEYS.index(ekey(kk))]])
                    return v
                if key[0] == "s":
                    return _upk(_cat([ld(("a",) + key[1:]), ld(("b", key[1]))]))
                v = ld(key)
                pcnt[0] += 1
                pdl.sort(key=lambda e: e[0])
                if pdl and pcnt[0] >= pdl[0][0]:
                    deps = pdl.pop(0)[1]
                    v = _cat([jnp.where(never, d, v[8 * e:8 * e + 8]) for e, d in enumerate(deps)]
                             + ([v[8 * len(deps):]] if v.shape[0] > 8 * len(deps) else []))
                return _upk(v)
            p, q = {}, {}
            _fast_mm(prog, op, dot, XH, p, q)
            for n in range(len(p)):
                y, z, e = _fast_out(p, q, n, XH)
                ring_ref[n0 + n, c * XH:c * XH + XH // 2, :] = _pk(y.astype(BF16))
                ring_ref[n0 + n, c * XH + XH // 2:(c + 1) * XH, :] = _pk(z.astype(BF16))
                if e is not None:
                    ring_ref[n0 + n, NXC * XH:NXC * XH + 8, :] = _pk(e.astype(BF16))

    def init_rows():
        x0 = x_ref[0:seg, :].astype(F32)
        sl = _ln(x0)
        xt = _ln(x_ref[R0 + NPRE:XF, :].astype(F32))
        h_ref[0:n_mem, :] = xt[0:n_mem]
        h_ref[n_mem:M2, :] = sl[0:n_mem]
        h_ref[M2:M2 + n_mem, :] = mem0_ref[...].astype(F32)
        h_ref[M2 + n_mem:RB, :] = sl[n_mem:seg]
        h_ref[RB:RB + AH, :] = xt[M2:M2 + AH]
        h_ref[RB + AH:RB + AH + n_mem, :] = xt[n_mem:M2]
        x2_ref[...] = x0

    def first_a(p, c):
        buf = stage_ref.at[0, p, pl.ds(0, RT * 128)]
        pltpu.make_async_copy(buf, buf, sem_m.at[4 + p]).wait()
        x_copy(HC + p).wait()

        @pl.when(p == 0)
        def _():
            for pp in range(4):
                w_copy(pp, 1).start()

        @pl.when(p == 2)
        def _():
            bq_copy(0).start()
        ln_ops(1, p, 0, len(KEYS))
        pre_chunk(S53, buf, wr_ref.at[p], p * NT, range(HC))
        return c
    lax.fori_loop(0, 3, first_a, 0)
    for cp in small:
        cp.wait()

    def first_b(p, c):
        e_ops()
        init_rows()
        ln_ops(0, p, len(KEYS_R), len(KEYS))
        pre_chunk(S53, None, wr_ref.at[p], p * NT, range(HC, NXC))
        return c
    lax.fori_loop(0, 3, first_b, 0)

    dpt = 128 // B_HEADS

    def b_stage1(u):
        uc = jnp.clip(u, 0, NB1 - 1)
        tr = bst_tile(jnp.where(u >= 0, uc, NB1 + nct)).astype(F32).T
        r0 = pl.multiple_of(uc * 128, 128)
        for j in range(nct):
            btmp_ref[j, pl.ds(r0, 128), :] = tr[:, j * 128:(j + 1) * 128]
        return [pltpu.bitcast(tr[120:128, j * 128:(j + 1) * 128], U32) for j in range(nct)]

    def b_stage1_wo(u):
        uc = jnp.clip(u, 0, nct - 1)
        btmp_ref[uc, WO0:WO0 + dm, :] = bst_tile(jnp.where(u >= 0, NB1 + uc, NB1 + nct)).astype(F32)

    def b_stage2(u):
        uc = jnp.clip(u, 0, NB1 - 1)
        part = (uc >= nct).astype(jnp.int32) + (uc >= 2 * nct).astype(jnp.int32)
        r0 = part * dm + (uc - part * nct) * dpt
        rows = _cat([_cat([btmp_ref[j, pl.ds(r0 + dd, B_HEADS, stride=bdh), :]
                           for j in range(nct)], axis=1) for dd in range(dpt)])
        val = _pk(rows.T.astype(BF16))
        bw_ref[uc] = val
        return [val[64 * j + 56:64 * j + 64] for j in range(nct)]

    def b_stage2_wo(u):
        uc = jnp.clip(u, 0, nct - 1)
        r0 = jnp.where(u >= 0, WO0, 0)
        bw_ref[NB1 + uc] = _pk(
            _cat([btmp_ref[uc, pl.ds(r0 + d, B_HEADS, stride=bdh), :] for d in range(bdh)]).astype(BF16))

    def wo_store(scheme, w, dst, never=None):
        if scheme is S55:
            rawt = lambda k, n: w[k * 128:(k + 1) * 128, n * 128:(n + 1) * 128]
            plain = [i for i, tl in enumerate(scheme[0]) if len(tl) == 1]
            for i, tl in enumerate(scheme[0]):
                if len(tl) > 1:
                    val = _combo(tl, lambda k, n: rawt(k, n).astype(F32)).astype(BF16)
                    val = _pk(_upk(_pk(val.T)).T)
                    dst[i * 64:(i + 1) * 64, :] = val
                    j = plain.pop()
                    pv_ = _pk(rawt(*scheme[0][j][0]))
                    dst[j * 64:(j + 1) * 64, :] = jnp.where(never, val, pv_) if PACE else pv_
            return
        for r in range(0, 128, 16):
            memo = {}

            def raw(k, n):
                return w[k * 128 + r:k * 128 + r + 16, n * 128:(n + 1) * 128]

            def block(k, n):
                if (k, n) not in memo:
                    memo[k, n] = raw(k, n).astype(F32)
                return memo[k, n]
            for i, tl in enumerate(scheme[0]):
                val = raw(*tl[0]) if len(tl) == 1 else _combo(tl, block).astype(BF16)
                dst[i * 64 + r // 2:i * 64 + r // 2 + 8, :] = _pk(val)

    def pre_body(g, c):
        slot = g & (NSLOT - 1)
        buf = stage_ref.at[slot]
        pltpu.make_async_copy(buf, buf, sem_w.at[slot]).wait()

        @pl.when((g >= 2) & (g <= 4))
        def _():
            bq_copy(g - 2).wait()

        @pl.when(g == 4)
        def _():
            bo_copy.wait()

        @pl.when(g <= 2)
        def _():
            bq_copy(g).start()

        @pl.when(g == 2)
        def _():
            bo_copy.start()

        @pl.when(g + 1 <= NG)
        def _():
            for p in range(4):
                w_copy(p, g + 1).start()

        @pl.when(g == NG - 1)
        def _():
            w0_copy(3).start()
            x_late.start()

        wo_store(S55, stage_ref.at[slot, 3], w_ref.at[3 * NG + g - 1], g > NG + 5)
        deps = [b_stage2(3 * (g - 5) + e) for e in range(3)]
        b_stage2_wo(g - 5)
        deps += [b_stage1(3 * (g - 2) + e) for e in range(3)]
        b_stage1_wo(g - 4)
        pcnt[0] = 0
        if PB:
            pdl.extend((PB0 + PB * e, d) for e, d in enumerate(deps))
        tbs = [prep(S55, stage_ref.at[slot, 0], w_ref.at[g - 1])]
        for p in range(3):
            if p < 2:
                del tdeps[:]
                tbs.append(prep(S55, stage_ref.at[slot, p + 1], w_ref.at[(p + 1) * NG + g - 1]))
                if PC:
                    pdl.extend((pcnt[0] + 60 + PC * e, d) for e, d in enumerate(tdeps))
            pre_chunk(S55, stage_ref.at[slot, p], w_ref.at[p * NG + g - 1], p * NT + RT + (g - 1) * GT, range(NXC),
                      g > NG + 5, tbs[p])
        return c
    lax.fori_loop(1, NG + 1, pre_body, 0)
    w0_copy(3).wait()

    bscale = float(bdh) ** (-0.5) * LOG2E

    def b_proj(lhs, part):
        return _nn(lhs, _cat([_upk(bw_ref[part * nct + j]) for j in range(nct)], axis=1))

    def b_attn(jobs, q, k, v, sink=None):
        row = lax.broadcasted_iota(jnp.int32, (seg, 128), 0)
        outs = []
        for i, (l, sidx) in enumerate(jobs):
            r0 = i * seg
            pos = row + sidx * seg
            for j in range(nct if HS else 0):
                kb_ref[l, j, 0:HIST, :] = kb_ref[l, j, seg:seg + HIST, :]
                vb_ref[l, j, 0:HIST, :] = vb_ref[l, j, seg:seg + HIST, :]
            for j in range(nct):
                kb_ref[l, j, HIST:HIST + seg, :] = k[r0:r0 + seg, j * 128:(j + 1) * 128]
                vb_ref[l, j, HIST:HIST + seg, :] = v[r0:r0 + seg, j * 128:(j + 1) * 128]
            logits = []
            for w in range(B_WIN):
                o = HIST - w * B_DIL
                acc = None
                for j in range(nct):
                    p = q[r0:r0 + seg, j * 128:(j + 1) * 128] * kb_ref[l, j, o:o + seg, :]
                    acc = p if acc is None else acc + p
                acc = acc + pltpu.roll(acc, 64, 1)
                acc = acc + pltpu.roll(acc, 32, 1)
                lg = acc * bscale
                if w > 0:
                    lg = jnp.where(pos >= w * B_DIL, lg, NEG2)
                logits.append(lg)
            m = logits[0]
            for w in range(1, B_WIN):
                m = jnp.maximum(m, logits[w])
            es = [jnp.exp2(lg - m) for lg in logits]
            den = es[0]
            for w in range(1, B_WIN):
                den = den + es[w]
            inv = _recip(den)
            cols = []
            for j in range(nct):
                acc = None
                for w in range(B_WIN):
                    o = HIST - w * B_DIL
                    p = es[w] * vb_ref[l, j, o:o + seg, :]
                    acc = p if acc is None else acc + p
                cols.append(acc * inv)
            outs.append(_cat(cols, axis=1).astype(BF16))
            if sink is not None:
                for rg in range(0, seg, 8):
                    sink.append([c[rg:rg + 8] for c in cols])
            for j in range(0 if HS else nct):
                kb_ref[l, j, 0:HIST, :] = k[r0 + seg - HIST:r0 + seg, j * 128:(j + 1) * 128]
                vb_ref[l, j, 0:HIST, :] = v[r0 + seg - HIST:r0 + seg, j * 128:(j + 1) * 128]
        return outs

    def b_out(ob, res):
        return res + _nn(ob, _cat([_upk(bw_ref[NB1 + j]) for j in range(nct)], axis=1))

    def o_store(b, val):
        ro = pl.multiple_of((b + 1) * seg, seg)
        o_ref[pl.ds(ro, val.shape[0]), :] = val.astype(o_ref.dtype)

    def out_copy(b):
        ro = pl.multiple_of(b * seg, seg)
        return pltpu.make_async_copy(o_ref.at[pl.ds(ro + seg, seg), :], out_hbm.at[pl.ds(ro, seg), :], sem_o)

    def step(t, hc, full):
        t_last = n_seg + LAG - 1
        if full:
            jobs = [(0, t - 1), (1, t - 1 - LAG)]

            def b_in():
                return xb_ref[0:2 * seg, :]
        else:
            lb = (t == t_last).astype(jnp.int32)
            jobs = [(lb, t - 1 - lb * (LAG + 1))]

            def b_in():
                return xb_ref[pl.ds(pl.multiple_of(lb * seg, seg), seg), :]
        v0r = _cat([hc[0:n_mem], h_ref[n_mem:M2, :]])
        v1r = _cat([hc[n_mem:M2], h_ref[M2 + n_mem:2 * M2, :]])

        hist = []
        never = t > 4 * n_seg

        def gate(back, z):
            if not back or len(hist) < back:
                return z
            gv = hist[-back]
            return _cat([jnp.where(never, gv, z[e:e + 8]) for e in range(0, z.shape[0], 8)])

        def ktiles(z):
            return [z[:, k * 128:(k + 1) * 128] for k in range(z.shape[1] // 128)]
        if full:
            hl = _Operands(ktiles(_cat([v0r, h_ref[2 * M2:RB, :]])), ktiles(_cat([v1r, h_ref[RB:RB + AH, :]])), None)
        else:
            hl = _Operands(None, None, ktiles(_cat([v0r, v1r, h_ref[2 * M2:RB, :]])))
        mh = 2 * M2 if full else 0

        def tile_dot(p, r):
            src = wr_ref.at[p] if r == 0 else w_ref.at[p * NG + r - 1]

            def dot(a, i):
                wt = src[i * 64:(i + 1) * 64, :]
                cnt[0] += 1
                if dl and cnt[0] >= dl[0][0]:
                    deps = dl.pop(0)[1]
                    wt = _cat([jnp.where(never, pltpu.bitcast(d, U32), wt[8 * e:8 * e + 8])
                               for e, d in enumerate(deps)] + [wt[8 * len(deps):]])
                res_ = _nn(a, _upk(wt))
                hist.append(res_[0:8])
                return res_
            return dot
        cnt, dl = [0], []
        scale = float(dh) ** (-0.5) * LOG2E
        if full:
            s_ = t - LAG
            rd = pl.multiple_of(lax.rem(s_ * (seg // 2), RS // 2), seg // 2)
            wa = pl.multiple_of(lax.rem((A0 - R0 + s_ * AH) // 2, RS // 2), 8)
        else:
            wx = pl.multiple_of(jnp.where(t < LAG, NPRE // 2 + t * (n_mem // 2), RS // 2), n_mem // 2)
            wo_store(S35, stage0_ref, wr_ref.at[3])

        RA = R if full else M2 + seg
        CW = R + 2 * M2 if full else R
        bidx = 0 if full else 2
        half = dh - 128
        la8 = lax.broadcasted_iota(jnp.int32, (n_mem, 128), 1) < half
        ones = jnp.full((n_mem, 128), 0xFFFFFFFF, U32)
        zero = jnp.zeros((n_mem, 128), U32)
        mask_a = jnp.where(la8, ones, zero)
        mask_b = jnp.where(la8, zero, ones)

        def pk2(a, b):
            return _pk(_cat([a, b]).astype(BF16))

        yt = [[None] * NT for _ in range(3)]

        def proj(p, r):
            pa, qa = {}, {}
            _fast_mm((S53 if r == 0 else S55)[1], hl, tile_dot(p, r), mh, pa, qa)
            n0 = 0 if r == 0 else RT + (r - 1) * GT
            for n in range(len(pa)):
                y, z, e = _fast_out(pa, qa, n, mh)
                idx = p * NT + n0 + n
                if full:
                    ring_ref[idx, pl.ds(wa, 8), :] = pk2(z[16:24], z[24:32])
                    y = _cat([y[0:M2], z[0:M2], y[M2:2 * M2]])
                else:
                    y = e
                    ring_ref[idx, pl.ds(wx, n_mem // 2), :] = pk2(y[0:8], y[8:16])[0:n_mem // 2]
                yt[p][n0 + n] = stash(p * 16 + (n0 + n) % 16, packed(p, (n0 + n) % 3, y))

        def ab(z8):
            return jnp.where(la8, z8, 0.0), jnp.where(la8, 0.0, z8)

        def packed(p, j, y):
            u2 = pk2(y[32:40], y[40:48])
            if p == 0 or j == 0:
                return [pk2(y[0:8], y[8:16]), pk2(y[16:24], y[24:32]), u2]
            if j == 2:
                return [pk2(y[8:16], y[0:8]), pk2(y[24:32], y[16:24]), u2]
            xa_a, xa_b = ab(y[8:16])
            out = [pk2(xa_b, xa_a), pk2(y[24:32], y[16:24]) & mask_b, pk2(y[16:24], y[24:32]) & mask_a, u2]
            if full:
                out += [pk2(*ab(y[0:8])), pk2(*ab(y[16:24]))]
            return out

        def stash(idx, parts):
            kv_ref[idx, 0:8 * len(parts), :] = _cat(parts)
            return lambda: [kv_ref[idx, 8 * e:8 * e + 8, :] for e in range(len(parts))]

        def pair(p, g):
            xs = [ring_ref[p * NT + 3 * g + j, pl.ds(rd, seg // 2), :] for j in range(3)] if full else None
            return [f() for f in yt[p][3 * g:3 * g + 3]], xs

        def q_rows(z, j):
            v0, v1, v2 = z[0][j]
            return [v0] + ([z[1][j]] if full else []) + [v1, v2]

        def kv_tiles(z):
            yt, x1 = z
            v0, v1, v2 = yt[0]
            t0 = [v0] + ([x1[0]] if full else [v1, v2]) + [v1, v2]
            w0, w1, w2 = yt[2]
            t2 = [w0, w1, w2] + ([x1[2]] if full else [w1, w2])
            if full:
                t0 += [v0, v1]
                t2 += [w0, w1]
            e1, mb, ma, u2 = yt[1][0:4]
            mid2 = [e1, mb, u2 & mask_b, ma, u2 & mask_a]
            mid1 = None
            if full:
                lo, hi = x1[1][0:8], x1[1][8:16]
                mid1 = [yt[1][4], lo & mask_a, hi & mask_a, lo & mask_b, hi & mask_b, e1, yt[1][5]]
            return t0, mid1, mid2, t2

        def mat(parts):
            return _upk(_cat(parts))

        def scores(q, k):
            k0, km1, km2, k2_ = kv_tiles(k)
            s_a = _nt(mat(q_rows(q, 0)), mat(k0))
            s_b = _nt(mat(q_rows(q, 2)), mat(k2_))
            qm = q_rows(q, 1)
            if full:
                s_m = _cat([_nt(mat(qm[0:2]), mat(km1)), _cat([_nt(mat(qm[2:4]), mat(km2)), jnp.zeros((seg, CW - R), F32)], axis=1)])
            else:
                s_m = _nt(mat(qm), mat(km2))
            out = []
            for e, sx in enumerate((s_a, s_b)):
                s = (sx + s_m) * scale + bias_ref[bidx + e, 0:RA, 0:CW]
                ex = jnp.exp2(s - jnp.max(s, axis=-1, keepdims=True))
                out.append(ex * _recip(jnp.sum(ex, axis=-1, keepdims=True)))
            return out

        def pv(p, v):
            v0, vm1, vm2, v2 = kv_tiles(v)
            o_a = _nn(p[0].astype(BF16), mat(v0))
            o_b = _nn(p[1].astype(BF16), mat(v2))
            p = p[0] + p[1]
            if full:
                o_m = _cat([_nn(p[0:M2 + seg].astype(BF16), mat(vm1)),
                            _nn(p[M2 + seg:R, 0:R].astype(BF16), mat(vm2))])
            else:
                o_m = _nn(p.astype(BF16), mat(vm2))
            return [o_a, o_m, o_b]

        ot = []
        pacc, qacc = {}, {}

        def add_o(r):
            n0 = 0 if r == 0 else RT + (r - 1) * GT
            oo = ot[n0:n0 + (RT if r == 0 else GT)]
            if full:
                gt = (lambda z: z) if (r >= TAILPV and not GT8) else functools.partial(gate, GO)
                us = [_cat([o[48:64], o[32:48]]) for o in oo]
                if LZ:
                    ops = _Operands([o[0:32] for o in oo], us, [o[64:80] for o in oo], gt)
                else:
                    ops = _Operands([o[0:32] for o in oo], [gt(z) for z in us], [o[64:80] for o in oo])
            else:
                ops = _Operands(None, None, oo)
            _fast_mm((S35 if r == 0 else S55)[1], ops, tile_dot(3, r), mh, pacc, qacc)

        bqkv = [None] * 3
        probs = []

        def do_pv():
            for g in range(len(ot) // 3, len(probs)):
                ot.extend(pv(probs[g], pair(2, g)))

        if full:
            an = pl.multiple_of(jnp.minimum(A0 + (s_ + 1) * AH, S - AH), AH)
            al = _ln(x_ref[pl.ds(an, AH), :].astype(F32))
            h_ref[RB:RB + AH, :] = al
            if LDA:
                dl.append((LDA, [al[e:e + 8, j * 128:(j + 1) * 128] for e in range(0, AH, 8) for j in range(3)]))
                dl.append((LDA + 2, [al[e:e + 8, j * 128:(j + 1) * 128] for e in range(0, AH, 8) for j in range(3, 5)]))

        for r in range(NG + 1):
            proj(2, r)
            proj(1, r)
            proj(0, r)
            if r == 0:
                blhs = _ln(b_in()).astype(BF16)
            if r < 3:
                bqkv[2 - r] = b_proj(blhs, 2 - r)
            if r == BAR:
                sink = []
                ob = b_attn(jobs, *bqkv, sink=sink)
                if BDL and full:
                    dl.extend((cnt[0] + BD0 + BDL * e, d) for e, d in enumerate(sink))
            if r == BOUT_R:
                zb = b_out(_cat(ob), b_in())
                x2_new = zb[0:seg]
                if full:
                    o_store(t - 1 - LAG, zb[seg:2 * seg])
                    nxt = x2_new
                else:
                    o_store(lb * (t_last - LAG - 1) - 1, x2_new)
                    nxt = jnp.where(t < LAG - 1, x_ref[seg:2 * seg, :].astype(F32), x2_new)
                sl = _ln(nxt)
                h_ref[n_mem:M2, :] = sl[0:n_mem]
                h_ref[M2 + n_mem:RB, :] = sl[n_mem:seg]
                if LD and full:
                    for j in range(nct):
                        dl.append((cnt[0] + LD + 2 * j, [sl[e:e + 8, j * 128:(j + 1) * 128] for e in range(0, seg, 8)]))
                    dl.sort(key=lambda e: e[0])
            if r in WSCHED:
                add_o(WSCHED[r])
            do_pv()
            for g in range(len(probs), (RT + r * GT) // 3):
                probs.append(scores(pair(0, g), pair(1, g)))
        for r in range(len(WSCHED), TAILPV):
            add_o(r)
        do_pv()
        for r in range(TAILPV, NG + 1):
            add_o(r)
        cols = []
        for n in range(nct):
            y, z, e = _fast_out(pacc, qacc, n, mh)
            cols.append(_cat([y, z[16:32], z[0:16], e]) if full else e)
        acc = _cat(cols, axis=1)

        y2 = x2_ref[...] + _cat([acc[n_mem:M2], acc[RA - seg + n_mem:RA]])
        mem2 = acc[RA - seg:RA - seg + n_mem]
        if full:
            x_cur = x_ref[pl.ds(pl.multiple_of(t * seg, seg), seg), :].astype(F32)
            xb_ref[0:seg, :] = x_cur + acc[M2:M2 + seg]
            xb_ref[seg:2 * seg, :] = y2
            m1n = acc[0:n_mem]
            m2n = mem2
        else:
            xb_ref[pl.ds(pl.multiple_of(jnp.where(t < LAG, 0, (t - n_seg + 2) * seg), seg), seg), :] = y2
            m1n = jnp.where(t < LAG - 1, h_ref[RB + AH:RB + AH + n_mem, :], mem2)
            m2n = jnp.where(t == LAG - 1, mem0_ref[...].astype(F32), mem2)
        x2_ref[...] = nxt
        return _cat([m1n, m2n])

    def single_body(t, c):
        @pl.when(t == n_seg)
        def _():
            out_copy(t - (LAG + 2)).start()
        return step(t, c, False)

    def full_body(t, c):
        @pl.when(t >= LAG + 2)
        def _():
            out_copy(t - (LAG + 2)).start()
        return step(t, c, True)

    def phase(ph, c):
        t0 = ph * n_seg
        c = lax.fori_loop(t0, t0 + LAG, single_body, c)

        @pl.when(ph == 0)
        def _():
            x_late.wait()
        return lax.fori_loop(LAG, jnp.where(ph == 0, n_seg, LAG), full_body, c)
    if not SKIPM:
      lax.fori_loop(0, 2, phase, _cat([h_ref[0:n_mem, :], h_ref[M2:M2 + n_mem, :]]))

    if SKIPM:
        def keep(i, c):
            z = (w_ref[i, pl.ds(pl.multiple_of(i * 8, 8), 8), :] + ring_ref[i, pl.ds(pl.multiple_of(i * 8, 8), 8), :]
                 + wr_ref[i & 3, pl.ds(pl.multiple_of(i * 8, 8), 8), :])
            xb_ref[2 * seg:2 * seg + 8, 0:128] = pltpu.bitcast(z, F32) + h_ref[pl.ds(pl.multiple_of((i & 7) * 8, 8), 8), 0:128] + x2_ref[0:8, 0:128]
            return c
        lax.fori_loop(0, 36, keep, 0)
    out_copy(n_seg - 3).start()
    res = xb_ref[2 * seg:4 * seg, :]
    blhs = _ln(res).astype(BF16)
    ob = b_attn([(1, n_seg - 2), (1, n_seg - 1)], *[b_proj(blhs, part) for part in range(3)])
    o_store(n_seg - 2, b_out(_cat(ob), res))
    out_copy(n_seg - 2).start()
    out_copy(n_seg - 1).start()
    pltpu.make_async_copy(o_ref.at[pl.ds(seg, S), :], out_hbm, sem_o).wait()


@functools.partial(jax.jit, static_argnames=("seg",))
def _run(A_x, A_mem0, A_Wq, A_Wk, A_Wv, A_Wo, B_wqkv, B_wo, *, seg):
    _, S, dm = A_x.shape
    n_heads, dh = A_Wq.shape[1], A_Wq.shape[2]
    n_mem = A_mem0.shape[1]
    n_seg = S // seg
    hd = n_heads * dh
    nct = dm // 128
    ng = (hd // 128 - RT) // GT
    assert (seg, n_seg, n_mem, dh, dm % 128, n_heads, LAG) == (32, 64, 8, 192, 0, 32, 2)

    x = A_x.reshape(S, dm)
    mem0 = A_mem0.reshape(n_mem, dm)
    wq = jnp.transpose(A_Wq, (1, 2, 0)).reshape(hd, dm)
    wk = jnp.transpose(A_Wk, (1, 2, 0)).reshape(hd, dm)
    wv = jnp.transpose(A_Wv, (1, 2, 0)).reshape(hd, dm)
    wo = A_Wo.reshape(hd, dm)
    _, _, _, _, rs, xc = _plan(seg, n_seg)

    kern = functools.partial(_kernel, seg=seg, n_seg=n_seg, n_mem=n_mem,
                             n_heads=n_heads, dh=dh, dm=dm)
    hbm = pl.BlockSpec(memory_space=pltpu.HBM)

    out = pl.pallas_call(
        kern,
        in_specs=[hbm] * 8,
        out_specs=hbm,
        out_shape=jax.ShapeDtypeStruct((S, dm), A_x.dtype),
        scratch_shapes=[
            pltpu.VMEM((S, dm), BF16),
            pltpu.VMEM((n_mem, dm), BF16),
            pltpu.VMEM((NSLOT, 4, GT * 128, dm), BF16),
            pltpu.VMEM((RT * 128, dm), BF16),
            pltpu.VMEM((4, len(S53[0]) * 64, 128), U32),
            pltpu.VMEM((4 * ng, len(S55[0]) * 64, 128), U32),
            pltpu.VMEM((dm, 4 * dm + 128), BF16),
            pltpu.VMEM((nct, 4 * dm + 32, 128), F32),
            pltpu.VMEM((4 * nct, dm // 2, 128), U32),
            pltpu.VMEM((len(KEYS_R), HC * xc // 4, 128), U32),
            pltpu.VMEM((len(KEYS_R), HC * xc // 4, 128), U32),
            pltpu.VMEM((len(KEYS) - len(KEYS_R), NXC * xc // 4, 128), U32),
            pltpu.VMEM((15, 8, 128), U32),
            pltpu.VMEM((3 * hd // 128, rs // 2 + 8, 128), U32),
            pltpu.VMEM((3 * n_mem + seg + AH, dm), F32),
            pltpu.VMEM((4 * seg, dm), F32),
            pltpu.VMEM((seg, dm), F32),
            pltpu.VMEM((2, nct, HIST + seg, 128), F32),
            pltpu.VMEM((2, nct, HIST + seg, 128), F32),
            pltpu.VMEM((S + seg, dm), A_x.dtype),
            pltpu.VMEM((4, 2 * n_mem + 2 * seg, 128), F32),
            pltpu.VMEM((48, 48, 128), U32),
            pltpu.SemaphoreType.DMA((NSLOT,)),
            pltpu.SemaphoreType.DMA((8 + NXC,)),
            pltpu.SemaphoreType.DMA((4,)),
            pltpu.SemaphoreType.DMA(()),
        ],
        compiler_params=pltpu.CompilerParams(
            vmem_limit_bytes=126 * 1024 * 1024,
            disable_bounds_checks=True,
        ),
    )(x, mem0, wq, wk, wv, wo, B_wqkv, B_wo)
    return out.reshape(1, S, dm)


def pallas_interleave_layers__memory_aug_recurrent_mem_tr__sliding_local_dilated__prompt_kernel(
    A_x: jax.Array,
    A_mem0: jax.Array,
    A_Wq: jax.Array,
    A_Wk: jax.Array,
    A_Wv: jax.Array,
    A_Wo: jax.Array,
    A_seg_len,
    B_x: jax.Array,
    B_wqkv: jax.Array,
    B_wo: jax.Array,
):
    del B_x
    seg = A_seg_len if isinstance(A_seg_len, int) else 32
    return _run(A_x, A_mem0, A_Wq, A_Wk, A_Wv, A_Wo, B_wqkv, B_wo, seg=seg)
```

```python
import functools

import jax
import jax.numpy as jnp
from jax import lax
import jax.experimental.pallas as pl
import jax.experimental.pallas.tpu as pltpu

F32 = jnp.float32
BF16 = jnp.bfloat16
U32 = jnp.uint32
NEG = -1000000000.0
LN_EPS = 1e-05
LOG2E = 1.4426950408889634
NEG2 = NEG * LOG2E

B_HEADS = 32
B_WIN = 8
B_DIL = 2
HIST = 16
SKIPM = int(0)
PACE = int(1)
BDL = int(0)
BD0 = int(40)
PB = int(60)
PB0 = int(100)
PC = int(0)
GO = int(40)
LZ = int(0)
GH = int(0)
GT8 = int(0)
LD = int(150)
LDA = int(0)
HS = int(1)
BF = '2'
GE = int(0)
BAR = int(3)
BO = int(5)
WS = '346789'
AH = 16
LAG = 2
NSLOT = 2
NXC = 6
HC = 3
WSCHED = dict((int(c), i) for i, c in enumerate(WS))
BOUT_R = BO
TAILPV = 8


def _ln(x):
    m = jnp.mean(x, axis=-1, keepdims=True)
    c = x - m
    v = jnp.mean(c * c, axis=-1, keepdims=True)
    return c * lax.rsqrt(v + LN_EPS)


def _recip(d):
    return pl.reciprocal(d, approx=True)


def _nt(a, b):
    return lax.dot_general(a, b, (((1,), (1,)), ((), ())), preferred_element_type=F32)


def _nn(a, b):
    return jnp.dot(a, b, preferred_element_type=F32)


def _cat(xs, axis=0):
    return xs[0] if len(xs) == 1 else jnp.concatenate(xs, axis=axis)


def _pk(z):
    return pltpu.bitcast(z, U32)


def _upk(z):
    return pltpu.bitcast(z, BF16)


LAM = (-1.5, -0.5, 0.0, 0.5, 1.5)


def _scheme(stars):
    tiles, prog = [], []
    for star in stars:
        if len(star) == 1:
            prog.append(("single", star[0], None, len(tiles)))
            tiles.append([star[0][:2]])
            continue
        left = [len(star) - 1] * len(star)
        for j in range(1, len(star)):
            for i in range(j):
                x, y = star[i], star[j]
                prog.append(("pair", x, y, len(tiles)))
                tiles += [[(x[0], y[1])], [(y[0], x[1])], [(x[0], y[1]), (y[0], x[1])]]
                for e in (i, j):
                    left[e] -= 1
                    if left[e] == 0:
                        z = star[e]
                        prog.append(("diag", z, None, len(tiles)))
                        tiles += [[z[:2]] + [(o[0], z[1]) for o in star if o is not z],
                                  [z[:2]] + [(z[0], o[1]) for o in star if o is not z]]
    return tiles, prog


S55 = _scheme([[(i, i, LAM[i]) for i in range(5)]])
S53 = _scheme([[(0, 0, LAM[0]), (2, 1, LAM[2]), (4, 2, LAM[4])], [(1, 0, LAM[1]), (3, 2, LAM[3])],
               [(1, 1, LAM[1])], [(3, 1, LAM[3])]])
S35 = _scheme([[(0, 0, LAM[0]), (1, 2, LAM[2]), (2, 4, LAM[4])], [(0, 1, LAM[1]), (2, 3, LAM[3])],
               [(1, 1, LAM[1])], [(1, 3, LAM[3])]])


def _spread(prog):
    pairs = [e for e in prog if e[0] != "diag"]
    diags = [e for e in prog if e[0] == "diag"]
    out, k = [], 0
    for i, e in enumerate(pairs):
        out.append(e)
        while k < len(diags) and (k + 0.5) * len(pairs) <= (i + 1) * len(diags):
            out.append(diags[k])
            k += 1
    return out + diags[k:]


def _op_keys(prog):
    keys = []
    for kind, x, y, _ in prog:
        if kind == "pair":
            new = [(nm, x[0], x[2], y[0], y[2]) for nm in ("l1", "l2", "A")]
        else:
            new = [("a", x[0], x[2]), ("b", x[0])]
        keys += [k for k in new if k not in keys]
    return keys


def _scaled(c, u):
    return u if c == 1.0 else c * u


class _Operands:
    def __init__(self, T, U, E, gate=None):
        if gate is not None:
            class Lazy:
                def __getitem__(lz, k):
                    return self._get(("u", k), lambda: gate(U[k]))
            self.U = Lazy()
        else:
            self.U = U
        self.T, self.E, self.memo = T, E, {}

    def _get(self, key, fn):
        if key not in self.memo:
            self.memo[key] = fn()
        return self.memo[key]

    def paired(self, key):
        T, U = self.T, self.U
        if key[0] == "b":
            return U[key[1]]
        if key[0] == "a":
            k, lam = key[1:]
            if lam == 0.0:
                return T[k]
            return self._get(("f",) + key, lambda: T[k] - _scaled(lam, U[k]) if lam > 0
                             else T[k] + _scaled(-lam, U[k]))
        kx, lx, ky, ly = key[1:]
        A = self._get(("f", "A") + key[1:],
                      lambda: self.paired(("a", kx, lx)) + self.paired(("a", ky, ly)))
        if key[0] == "A":
            return A
        return A - _scaled(ly - lx, U[kx]) if key[0] == "l1" else A + _scaled(ly - lx, U[ky])

    def extra(self, key):
        if key[0] == "a":
            return self.E[key[1]]
        return self._get(("e", key[1], key[3]), lambda: self.E[key[1]] + self.E[key[3]])

    def __call__(self, key):
        if self.T is None:
            ek = ("a", key[1]) if key[0] in ("a", "s") else ("l", key[1], 0, key[3])
            return self._get(ek, lambda: self.extra(ek).astype(BF16))

        def build():
            ak = ("a",) + key[1:] if key[0] == "s" else key
            parts = [self.paired(ak)]
            if self.E is not None and ak[0] in ("a", "l1", "l2"):
                parts.append(self.extra(ak))
            if key[0] == "s":
                parts.append(self.U[key[1]])
            return _cat(parts).astype(BF16)
        return self._get(key, build)


def _fast_mm(prog, op, dot, m, p, q):
    def add(d, key, val):
        d[key] = val if key not in d else d[key] + val

    for kind, x, y, i in prog:
        if kind == "pair":
            kk = (x[0], x[2], y[0], y[2])
            p1, p2 = dot(op(("l1",) + kk), i), dot(op(("l2",) + kk), i + 1)
            if m:
                r = _scaled(1.0 / (y[2] - x[2]), p2[0:m] - p1[0:m] + dot(op(("A",) + kk), i + 2))
                add(q, (x[1], x[2]), r)
                add(q, (y[1], y[2]), r)
            add(p, y[1], p1)
            add(p, x[1], p2)
        elif kind == "diag":
            add(p, x[1], dot(op(("a", x[0], x[2])), i))
            if m:
                add(q, (x[1], x[2]), dot(op(("b", x[0])), i + 1))
        else:
            r = dot(op(("s", x[0], x[2])), i)
            add(p, x[1], r[0:r.shape[0] - m])
            if m:
                add(q, (x[1], x[2]), r[r.shape[0] - m:])


def _fast_out(p, q, n, m):
    if not m:
        return None, None, p[n]
    y, z = p[n][0:m], None
    for (nn, lam), v in q.items():
        if nn == n:
            z = v if z is None else z + v
            if lam != 0.0:
                y = y + _scaled(lam, v) if lam > 0 else y - _scaled(-lam, v)
    return y, z, (p[n][m:] if p[n].shape[0] > m else None)


def _combo(tile, block):
    out = block(*tile[0])
    for kn in tile[1:]:
        out = out - block(*kn)
    return out


GT = 5
RT = 3
KEYS_R = _op_keys(S53[1])
KEYS = KEYS_R + [k for k in _op_keys(S55[1]) if k not in KEYS_R]


def _plan(seg, n_seg):
    S = seg * n_seg
    R0 = LAG * seg
    A0 = S - (n_seg - LAG) * AH
    NPRE = A0 - R0 - LAG * 8
    RS = -(-(A0 - R0 + AH) // seg) * seg
    XC = NPRE // NXC // 32 * 32
    assert XC * NXC + 16 == NPRE
    return S, R0, A0, NPRE, RS, XC


def _kernel(x_hbm, mem0_hbm, wq_hbm, wk_hbm, wv_hbm, wo_hbm, bqkv_hbm, bwo_hbm,
            out_hbm,
            x_ref, mem0_ref, stage_ref, stage0_ref, wr_ref, w_ref, bst_ref, btmp_ref, bw_ref,
            xla_ref, xlb_ref, xlc_ref, xe_ref, ring_ref, h_ref, xb_ref, x2_ref, kb_ref, vb_ref, o_ref, bias_ref, kv_ref, bwf_ref,
            sem_w, sem_m, sem_b, sem_o,
            *, seg, n_seg, n_mem, n_heads, dh, dm):
    S, R0, A0, NPRE, RS, XC = _plan(seg, n_seg)
    M2 = 2 * n_mem
    R = M2 + 2 * seg
    RB = M2 + seg
    PW = 2 * dh
    G = n_heads // 2
    nct = dm // 128
    bdh = dm // B_HEADS
    NT = n_heads * dh // 128
    NG = (NT - RT) // GT
    w_hbm = (wq_hbm, wk_hbm, wv_hbm, wo_hbm)

    def w_copy(p, g):
        slot = g & (NSLOT - 1)
        return pltpu.make_async_copy(w_hbm[p].at[pl.ds((RT + (g - 1) * GT) * 128, GT * 128), :],
                                     stage_ref.at[slot, p], sem_w.at[slot])

    def w0_copy(p):
        dst = stage0_ref if p == 3 else stage_ref.at[0, p, pl.ds(0, RT * 128)]
        return pltpu.make_async_copy(w_hbm[p].at[pl.ds(0, RT * 128), :], dst, sem_m.at[4 + p])

    NB1 = 3 * nct
    WO0 = 3 * dm
    XF = A0 + AH
    XH = XC // 2

    def rows_copy(r0, n, sem):
        return pltpu.make_async_copy(x_hbm.at[pl.ds(r0, n), :], x_ref.at[pl.ds(r0, n), :], sem)

    def x_copy(i):
        return rows_copy(pl.multiple_of(R0 + i * XC, 16), XC, sem_m.at[8 + i])

    small = [rows_copy(0, R0, sem_m.at[1]), rows_copy(R0 + NPRE - 16, XF - R0 - NPRE + 16, sem_m.at[2]),
             pltpu.make_async_copy(mem0_hbm, mem0_ref, sem_m.at[3])]
    x_late = rows_copy(XF, S - XF, sem_m.at[0])

    def bq_copy(part):
        c0 = pl.multiple_of(part * dm, 128)
        return pltpu.make_async_copy(bqkv_hbm.at[:, pl.ds(c0, dm)], bst_ref.at[:, pl.ds(c0, dm)], sem_b.at[part])

    bo_copy = pltpu.make_async_copy(bwo_hbm, bst_ref.at[:, pl.ds(3 * dm, dm)], sem_b.at[3])

    def bst_tile(c):
        return bst_ref[:, pl.ds(pl.multiple_of(c * 128, 128), 128)]

    def bias_tables(full):
        RA = R if full else M2 + seg
        CW = 128
        ri = lax.broadcasted_iota(jnp.int32, (RA, CW), 0)
        ci = lax.broadcasted_iota(jnp.int32, (RA, CW), 1)
        if not full:
            ri = jnp.where(ri >= M2, ri + seg, ri)

        def table(i, bounds, vals):
            out = vals[-1]
            for b, v in zip(reversed(bounds), reversed(vals[:-1])):
                out = jnp.where(i < b, v, out)
            return out
        qi = ri - table(ri, [16, 48, 56], [0, 8, 48, 40])
        g0 = (ci < 8) | ((ci >= 16) & (ci < 48))
        k2 = ci - table(ci, [8, 24, 32, 48, 56, 80, 88, 96, 104], [-8, 0, 24, 8, 48, 40, 72, 80, 96, 104])
        if full:
            k1 = ci - table(ci, [8, 48], [0, 8, 40])
            row_l2 = ((ri >= 8) & (ri < 16)) | (ri >= 48)
            row_xa = (ri >= 8) & (ri < 16)
            valid = (row_xa == (ci >= 80)) & (ci < 112)
            is_a = jnp.where(ci >= 80, ((ci >= 88) & (ci < 104)).astype(jnp.int32),
                             (g0 != row_l2).astype(jnp.int32)) > 0
            ki = jnp.where(row_l2, k2, k1)
            visible = valid & ((qi < n_mem) | (qi >= ki))
            fill = jnp.where(valid, NEG2, -jnp.inf)
        else:
            is_a = jnp.logical_not(g0)
            visible = (qi < n_mem) | (qi >= k2)
            fill = NEG2
        for e, mine in enumerate((is_a, jnp.logical_not(is_a))):
            bias_ref[(0 if full else 2) + e, 0:RA, :] = jnp.where(
                mine, jnp.where(visible, 0.0, fill), -jnp.inf)

    for i in range(HC):
        x_copy(i).start()

    def zero_body(j, c):
        btmp_ref[j, 0:dm, :] = jnp.zeros((dm, 128), F32)
        return c
    lax.fori_loop(0, nct, zero_body, 0)

    w0_copy(0).start()
    xb_ref[0:2 * seg, :] = jnp.zeros((2 * seg, dm), F32)
    kb_ref[...] = jnp.zeros(kb_ref.shape, F32)
    vb_ref[...] = jnp.zeros(vb_ref.shape, F32)
    bst_ref[:, 4 * dm:] = jnp.zeros((dm, 128), BF16)
    bias_tables(True)
    bias_tables(False)

    def ekey(key):
        return ("a", key[1]) if key[0] == "a" else ("l", key[1], 0, key[3])
    EKEYS = []
    for key in KEYS:
        if key[0] in ("a", "l1") and ekey(key) not in EKEYS:
            EKEYS.append(ekey(key))

    def e_ops():
        ye = _ln(x_ref[R0 + NPRE - 16:R0 + NPRE, :].astype(F32))
        eops = _Operands(None, None, [ye[:, k * 128:(k + 1) * 128] for k in range(nct)])
        for j, key in enumerate(EKEYS):
            xe_ref[j] = _pk(eops(key))

    NKR = len(KEYS_R)

    def xl(j, hf, i):
        if j >= NKR:
            ref, j, i = xlc_ref, j - NKR, hf * HC + i
        else:
            ref = (xla_ref, xlb_ref)[hf]
        r0 = i * (XH // 2)
        return ref.at[j, pl.ds(r0 if isinstance(r0, int) else pl.multiple_of(r0, 8), XH // 2)]

    def ln_ops(hf, i, lo, hi):
        y = _ln(x_ref[pl.ds(pl.multiple_of(R0 + (hf * HC + i) * XC, 16), XC), :].astype(F32))
        ops = _Operands([y[0:XH, k * 128:(k + 1) * 128] for k in range(nct)],
                        [y[XH:XC, k * 128:(k + 1) * 128] for k in range(nct)], None)
        for j in range(lo, hi):
            xl(j, hf, i)[...] = _pk(ops(KEYS[j]))

    def ln_body(i, c):
        x_copy(i).wait()

        @pl.when(i == 0)
        def _():
            x_copy(HC).start()

        @pl.when(i == 1)
        def _():
            w0_copy(1).start()
            w0_copy(2).start()

        @pl.when(i == 2)
        def _():
            x_copy(HC + 1).start()
            x_copy(HC + 2).start()
            for cp in small:
                cp.start()
        ln_ops(0, i, 0, len(KEYS_R))
        return c
    lax.fori_loop(0, HC, ln_body, 0)

    def prep(scheme, w, dst):
        raw = lambda k, n: w[n * 128:(n + 1) * 128, k * 128:(k + 1) * 128]
        tb = []
        for i, tl in enumerate(scheme[0]):
            tb.append(raw(*tl[0]) if len(tl) == 1
                      else _combo(tl, lambda k, n: raw(k, n).astype(F32)).astype(BF16))
            tt = _pk(tb[i].T)
            dst[i * 64:(i + 1) * 64, :] = tt
            if len(tl) > 1:
                tdeps.append([tt[56:64]])
        return tb

    pcnt, pdl, tdeps = [0], [], []

    def pre_chunk(scheme, w, dst, n0, chunks, never=None, tb=None):
        tiles, prog = scheme
        prog = _spread(prog)
        dot = lambda a, i: _nn(a, _upk(dst[i * 64:(i + 1) * 64, :]))
        if w is not None:
            if tb is None:
                tb = prep(scheme, w, dst)
            dot = lambda a, i: _nt(a, tb[i])

        for c in chunks:
            def op(key):
                def ld(kk):
                    v = xl(KEYS.index(kk), c // HC, c % HC)[...]
                    if c == NXC - 1 and kk[0] in ("a", "l1", "l2"):
                        v = _cat([v, xe_ref[EKEYS.index(ekey(kk))]])
                    return v
                if key[0] == "s":
                    return _upk(_cat([ld(("a",) + key[1:]), ld(("b", key[1]))]))
                v = ld(key)
                pcnt[0] += 1
                pdl.sort(key=lambda e: e[0])
                if pdl and pcnt[0] >= pdl[0][0]:
                    deps = pdl.pop(0)[1]
                    v = _cat([jnp.where(never, d, v[8 * e:8 * e + 8]) for e, d in enumerate(deps)]
                             + ([v[8 * len(deps):]] if v.shape[0] > 8 * len(deps) else []))
                return _upk(v)
            p, q = {}, {}
            _fast_mm(prog, op, dot, XH, p, q)
            for n in range(len(p)):
                y, z, e = _fast_out(p, q, n, XH)
                ring_ref[n0 + n, c * XH:c * XH + XH // 2, :] = _pk(y.astype(BF16))
                ring_ref[n0 + n, c * XH + XH // 2:(c + 1) * XH, :] = _pk(z.astype(BF16))
                if e is not None:
                    ring_ref[n0 + n, NXC * XH:NXC * XH + 8, :] = _pk(e.astype(BF16))

    def init_rows():
        x0 = x_ref[0:seg, :].astype(F32)
        sl = _ln(x0)
        xt = _ln(x_ref[R0 + NPRE:XF, :].astype(F32))
        h_ref[0:n_mem, :] = xt[0:n_mem]
        h_ref[n_mem:M2, :] = sl[0:n_mem]
        h_ref[M2:M2 + n_mem, :] = mem0_ref[...].astype(F32)
        h_ref[M2 + n_mem:RB, :] = sl[n_mem:seg]
        h_ref[RB:RB + AH, :] = xt[M2:M2 + AH]
        h_ref[RB + AH:RB + AH + n_mem, :] = xt[n_mem:M2]
        x2_ref[...] = x0

    def first_a(p, c):
        buf = stage_ref.at[0, p, pl.ds(0, RT * 128)]
        pltpu.make_async_copy(buf, buf, sem_m.at[4 + p]).wait()
        x_copy(HC + p).wait()

        @pl.when(p == 0)
        def _():
            for pp in range(4):
                w_copy(pp, 1).start()

        @pl.when(p == 2)
        def _():
            bq_copy(0).start()
        ln_ops(1, p, 0, len(KEYS))
        pre_chunk(S53, buf, wr_ref.at[p], p * NT, range(HC))
        return c
    lax.fori_loop(0, 3, first_a, 0)
    for cp in small:
        cp.wait()

    def first_b(p, c):
        e_ops()
        init_rows()
        ln_ops(0, p, len(KEYS_R), len(KEYS))
        pre_chunk(S53, None, wr_ref.at[p], p * NT, range(HC, NXC))
        return c
    lax.fori_loop(0, 3, first_b, 0)

    dpt = 128 // B_HEADS

    def b_stage1(u):
        uc = jnp.clip(u, 0, NB1 - 1)
        tr = bst_tile(jnp.where(u >= 0, uc, NB1 + nct)).astype(F32).T
        r0 = pl.multiple_of(uc * 128, 128)
        for j in range(nct):
            btmp_ref[j, pl.ds(r0, 128), :] = tr[:, j * 128:(j + 1) * 128]
        return [pltpu.bitcast(tr[120:128, j * 128:(j + 1) * 128], U32) for j in range(nct)]

    def b_stage1_wo(u):
        uc = jnp.clip(u, 0, nct - 1)
        btmp_ref[uc, WO0:WO0 + dm, :] = bst_tile(jnp.where(u >= 0, NB1 + uc, NB1 + nct)).astype(F32)

    def b_stage2(u):
        uc = jnp.clip(u, 0, NB1 - 1)
        part = (uc >= nct).astype(jnp.int32) + (uc >= 2 * nct).astype(jnp.int32)
        r0 = part * dm + (uc - part * nct) * dpt
        rows = _cat([_cat([btmp_ref[j, pl.ds(r0 + dd, B_HEADS, stride=bdh), :]
                           for j in range(nct)], axis=1) for dd in range(dpt)])
        val = _pk(rows.T.astype(BF16))
        bw_ref[uc] = val
        return [val[64 * j + 56:64 * j + 64] for j in range(nct)]

    def b_stage2_wo(u):
        uc = jnp.clip(u, 0, nct - 1)
        r0 = jnp.where(u >= 0, WO0, 0)
        bw_ref[NB1 + uc] = _pk(
            _cat([btmp_ref[uc, pl.ds(r0 + d, B_HEADS, stride=bdh), :] for d in range(bdh)]).astype(BF16))

    def wo_store(scheme, w, dst, never=None):
        if scheme is S55:
            rawt = lambda k, n: w[k * 128:(k + 1) * 128, n * 128:(n + 1) * 128]
            plain = [i for i, tl in enumerate(scheme[0]) if len(tl) == 1]
            for i, tl in enumerate(scheme[0]):
                if len(tl) > 1:
                    val = _combo(tl, lambda k, n: rawt(k, n).astype(F32)).astype(BF16)
                    val = _pk(_upk(_pk(val.T)).T)
                    dst[i * 64:(i + 1) * 64, :] = val
                    j = plain.pop()
                    pv_ = _pk(rawt(*scheme[0][j][0]))
                    dst[j * 64:(j + 1) * 64, :] = jnp.where(never, val, pv_) if PACE else pv_
            return
        for r in range(0, 128, 16):
            memo = {}

            def raw(k, n):
                return w[k * 128 + r:k * 128 + r + 16, n * 128:(n + 1) * 128]

            def block(k, n):
                if (k, n) not in memo:
                    memo[k, n] = raw(k, n).astype(F32)
                return memo[k, n]
            for i, tl in enumerate(scheme[0]):
                val = raw(*tl[0]) if len(tl) == 1 else _combo(tl, block).astype(BF16)
                dst[i * 64 + r // 2:i * 64 + r // 2 + 8, :] = _pk(val)

    def pre_body(g, c):
        slot = g & (NSLOT - 1)
        buf = stage_ref.at[slot]
        pltpu.make_async_copy(buf, buf, sem_w.at[slot]).wait()

        @pl.when((g >= 2) & (g <= 4))
        def _():
            bq_copy(g - 2).wait()

        @pl.when(g == 4)
        def _():
            bo_copy.wait()

        @pl.when(g <= 2)
        def _():
            bq_copy(g).start()

        @pl.when(g == 2)
        def _():
            bo_copy.start()

        @pl.when(g + 1 <= NG)
        def _():
            for p in range(4):
                w_copy(p, g + 1).start()

        @pl.when(g == NG - 1)
        def _():
            w0_copy(3).start()
            x_late.start()

        wo_store(S55, stage_ref.at[slot, 3], w_ref.at[3 * NG + g - 1], g > NG + 5)
        deps = [b_stage2(3 * (g - 5) + e) for e in range(3)]
        b_stage2_wo(g - 5)
        deps += [b_stage1(3 * (g - 2) + e) for e in range(3)]
        b_stage1_wo(g - 4)
        pcnt[0] = 0
        if PB:
            pdl.extend((PB0 + PB * e, d) for e, d in enumerate(deps))
        tbs = [prep(S55, stage_ref.at[slot, 0], w_ref.at[g - 1])]
        for p in range(3):
            if p < 2:
                del tdeps[:]
                tbs.append(prep(S55, stage_ref.at[slot, p + 1], w_ref.at[(p + 1) * NG + g - 1]))
                if PC:
                    pdl.extend((pcnt[0] + 60 + PC * e, d) for e, d in enumerate(tdeps))
            pre_chunk(S55, stage_ref.at[slot, p], w_ref.at[p * NG + g - 1], p * NT + RT + (g - 1) * GT, range(NXC),
                      g > NG + 5, tbs[p])
        return c
    lax.fori_loop(1, NG + 1, pre_body, 0)
    w0_copy(3).wait()

    def bprep(part, c):
        for r in range(0, 64, 8):
            memo = {}

            def raw(k, n):
                return bw_ref[part * nct + n, k * 64 + r:k * 64 + r + 8, :]

            def block(k, n):
                if (k, n) not in memo:
                    memo[k, n] = _upk(raw(k, n)).astype(F32)
                return memo[k, n]
            for i, tl in enumerate(S55[0]):
                val = raw(*tl[0]) if len(tl) == 1 else _pk(_combo(tl, block).astype(BF16))
                bwf_ref[part - int(BF[0]), i * 64 + r:i * 64 + r + 8, :] = val
        return c
    lax.fori_loop(int(BF[0]), int(BF[-1]) + 1, bprep, 0)

    bscale = float(bdh) ** (-0.5) * LOG2E

    bops = {}

    def b_fmm(z, part):
        kt = lambda a: [a[:, k * 128:(k + 1) * 128] for k in range(nct)]
        if id(z) not in bops:
            bops[id(z)] = (z, _Operands(kt(z[0:seg]), kt(z[seg:2 * seg]), None))
        ops = bops[id(z)][1]
        p, q = {}, {}
        _fast_mm(S55[1], ops, lambda a, i: _nn(a, _upk(bwf_ref[part - int(BF[0]), i * 64:(i + 1) * 64, :])), seg, p, q)
        return _cat([_cat(_fast_out(p, q, n, seg)[0:2]) for n in range(nct)], axis=1)

    def b_proj(lhs, part):
        if str(part) in BF and lhs.shape[0] == 2 * seg:
            return b_fmm(lhs, part)
        lhs = lhs.astype(BF16)
        return _nn(lhs, _cat([_upk(bw_ref[part * nct + j]) for j in range(nct)], axis=1))

    def b_attn(jobs, q, k, v, sink=None):
        row = lax.broadcasted_iota(jnp.int32, (seg, 128), 0)
        outs = []
        for i, (l, sidx) in enumerate(jobs):
            r0 = i * seg
            pos = row + sidx * seg
            for j in range(nct if HS else 0):
                kb_ref[l, j, 0:HIST, :] = kb_ref[l, j, seg:seg + HIST, :]
                vb_ref[l, j, 0:HIST, :] = vb_ref[l, j, seg:seg + HIST, :]
            for j in range(nct):
                kb_ref[l, j, HIST:HIST + seg, :] = k[r0:r0 + seg, j * 128:(j + 1) * 128]
                vb_ref[l, j, HIST:HIST + seg, :] = v[r0:r0 + seg, j * 128:(j + 1) * 128]
            logits = []
            for w in range(B_WIN):
                o = HIST - w * B_DIL
                acc = None
                for j in range(nct):
                    p = q[r0:r0 + seg, j * 128:(j + 1) * 128] * kb_ref[l, j, o:o + seg, :]
                    acc = p if acc is None else acc + p
                acc = acc + pltpu.roll(acc, 64, 1)
                acc = acc + pltpu.roll(acc, 32, 1)
                lg = acc * bscale
                if w > 0:
                    lg = jnp.where(pos >= w * B_DIL, lg, NEG2)
                logits.append(lg)
            m = logits[0]
            for w in range(1, B_WIN):
                m = jnp.maximum(m, logits[w])
            es = [jnp.exp2(lg - m) for lg in logits]
            den = es[0]
            for w in range(1, B_WIN):
                den = den + es[w]
            inv = _recip(den)
            cols = []
            for j in range(nct):
                acc = None
                for w in range(B_WIN):
                    o = HIST - w * B_DIL
                    p = es[w] * vb_ref[l, j, o:o + seg, :]
                    acc = p if acc is None else acc + p
                cols.append(acc * inv)
            outs.append(_cat(cols, axis=1) if '3' in BF else _cat(cols, axis=1).astype(BF16))
            if sink is not None:
                for rg in range(0, seg, 8):
                    sink.append([c[rg:rg + 8] for c in cols])
            for j in range(0 if HS else nct):
                kb_ref[l, j, 0:HIST, :] = k[r0 + seg - HIST:r0 + seg, j * 128:(j + 1) * 128]
                vb_ref[l, j, 0:HIST, :] = v[r0 + seg - HIST:r0 + seg, j * 128:(j + 1) * 128]
        return outs

    def b_out(ob, res):
        return res + b_proj(ob, 3)

    def o_store(b, val):
        ro = pl.multiple_of((b + 1) * seg, seg)
        o_ref[pl.ds(ro, val.shape[0]), :] = val.astype(o_ref.dtype)

    def out_copy(b):
        ro = pl.multiple_of(b * seg, seg)
        return pltpu.make_async_copy(o_ref.at[pl.ds(ro + seg, seg), :], out_hbm.at[pl.ds(ro, seg), :], sem_o)

    def step(t, hc, full):
        t_last = n_seg + LAG - 1
        if full:
            jobs = [(0, t - 1), (1, t - 1 - LAG)]

            def b_in():
                return xb_ref[0:2 * seg, :]
        else:
            lb = (t == t_last).astype(jnp.int32)
            jobs = [(lb, t - 1 - lb * (LAG + 1))]

            def b_in():
                return xb_ref[pl.ds(pl.multiple_of(lb * seg, seg), seg), :]
        v0r = _cat([hc[0:n_mem], h_ref[n_mem:M2, :]])
        v1r = _cat([hc[n_mem:M2], h_ref[M2 + n_mem:2 * M2, :]])

        hist = []
        never = t > 4 * n_seg

        def gate(back, z):
            if not back or len(hist) < back:
                return z
            gv = hist[-back]
            return _cat([jnp.where(never, gv, z[e:e + 8]) for e in range(0, z.shape[0], 8)])

        def ktiles(z):
            return [z[:, k * 128:(k + 1) * 128] for k in range(z.shape[1] // 128)]
        if full:
            hl = _Operands(ktiles(_cat([v0r, h_ref[2 * M2:RB, :]])), ktiles(_cat([v1r, h_ref[RB:RB + AH, :]])), None)
        else:
            hl = _Operands(None, None, ktiles(_cat([v0r, v1r, h_ref[2 * M2:RB, :]])))
        mh = 2 * M2 if full else 0

        def tile_dot(p, r):
            src = wr_ref.at[p] if r == 0 else w_ref.at[p * NG + r - 1]

            def dot(a, i):
                wt = src[i * 64:(i + 1) * 64, :]
                cnt[0] += 1
                if dl and cnt[0] >= dl[0][0]:
                    deps = dl.pop(0)[1]
                    wt = _cat([jnp.where(never, pltpu.bitcast(d, U32), wt[8 * e:8 * e + 8])
                               for e, d in enumerate(deps)] + [wt[8 * len(deps):]])
                res_ = _nn(a, _upk(wt))
                hist.append(res_[0:8])
                return res_
            return dot
        cnt, dl = [0], []
        scale = float(dh) ** (-0.5) * LOG2E
        if full:
            s_ = t - LAG
            rd = pl.multiple_of(lax.rem(s_ * (seg // 2), RS // 2), seg // 2)
            wa = pl.multiple_of(lax.rem((A0 - R0 + s_ * AH) // 2, RS // 2), 8)
        else:
            wx = pl.multiple_of(jnp.where(t < LAG, NPRE // 2 + t * (n_mem // 2), RS // 2), n_mem // 2)
            wo_store(S35, stage0_ref, wr_ref.at[3])

        RA = R if full else M2 + seg
        CW = R + 2 * M2 if full else R
        bidx = 0 if full else 2
        half = dh - 128
        la8 = lax.broadcasted_iota(jnp.int32, (n_mem, 128), 1) < half
        ones = jnp.full((n_mem, 128), 0xFFFFFFFF, U32)
        zero = jnp.zeros((n_mem, 128), U32)
        mask_a = jnp.where(la8, ones, zero)
        mask_b = jnp.where(la8, zero, ones)

        def pk2(a, b):
            return _pk(_cat([a, b]).astype(BF16))

        yt = [[None] * NT for _ in range(3)]

        def proj(p, r):
            pa, qa = {}, {}
            _fast_mm((S53 if r == 0 else S55)[1], hl, tile_dot(p, r), mh, pa, qa)
            n0 = 0 if r == 0 else RT + (r - 1) * GT
            for n in range(len(pa)):
                y, z, e = _fast_out(pa, qa, n, mh)
                idx = p * NT + n0 + n
                if full:
                    ring_ref[idx, pl.ds(wa, 8), :] = pk2(z[16:24], z[24:32])
                    y = _cat([y[0:M2], z[0:M2], y[M2:2 * M2]])
                else:
                    y = e
                    ring_ref[idx, pl.ds(wx, n_mem // 2), :] = pk2(y[0:8], y[8:16])[0:n_mem // 2]
                yt[p][n0 + n] = stash(p * 16 + (n0 + n) % 16, packed(p, (n0 + n) % 3, y))

        def ab(z8):
            return jnp.where(la8, z8, 0.0), jnp.where(la8, 0.0, z8)

        def packed(p, j, y):
            u2 = pk2(y[32:40], y[40:48])
            if p == 0 or j == 0:
                return [pk2(y[0:8], y[8:16]), pk2(y[16:24], y[24:32]), u2]
            if j == 2:
                return [pk2(y[8:16], y[0:8]), pk2(y[24:32], y[16:24]), u2]
            xa_a, xa_b = ab(y[8:16])
            out = [pk2(xa_b, xa_a), pk2(y[24:32], y[16:24]) & mask_b, pk2(y[16:24], y[24:32]) & mask_a, u2]
            if full:
                out += [pk2(*ab(y[0:8])), pk2(*ab(y[16:24]))]
            return out

        def stash(idx, parts):
            kv_ref[idx, 0:8 * len(parts), :] = _cat(parts)
            return lambda: [kv_ref[idx, 8 * e:8 * e + 8, :] for e in range(len(parts))]

        def pair(p, g):
            xs = [ring_ref[p * NT + 3 * g + j, pl.ds(rd, seg // 2), :] for j in range(3)] if full else None
            return [f() for f in yt[p][3 * g:3 * g + 3]], xs

        def q_rows(z, j):
            v0, v1, v2 = z[0][j]
            return [v0] + ([z[1][j]] if full else []) + [v1, v2]

        def kv_tiles(z):
            yt, x1 = z
            v0, v1, v2 = yt[0]
            t0 = [v0] + ([x1[0]] if full else [v1, v2]) + [v1, v2]
            w0, w1, w2 = yt[2]
            t2 = [w0, w1, w2] + ([x1[2]] if full else [w1, w2])
            if full:
                t0 += [v0, v1]
                t2 += [w0, w1]
            e1, mb, ma, u2 = yt[1][0:4]
            mid2 = [e1, mb, u2 & mask_b, ma, u2 & mask_a]
            mid1 = None
            if full:
                lo, hi = x1[1][0:8], x1[1][8:16]
                mid1 = [yt[1][4], lo & mask_a, hi & mask_a, lo & mask_b, hi & mask_b, e1, yt[1][5]]
            return t0, mid1, mid2, t2

        def mat(parts):
            return _upk(_cat(parts))

        def scores(q, k):
            k0, km1, km2, k2_ = kv_tiles(k)
            s_a = _nt(mat(q_rows(q, 0)), mat(k0))
            s_b = _nt(mat(q_rows(q, 2)), mat(k2_))
            qm = q_rows(q, 1)
            if full:
                s_m = _cat([_nt(mat(qm[0:2]), mat(km1)), _cat([_nt(mat(qm[2:4]), mat(km2)), jnp.zeros((seg, CW - R), F32)], axis=1)])
            else:
                s_m = _nt(mat(qm), mat(km2))
            out = []
            for e, sx in enumerate((s_a, s_b)):
                s = (sx + s_m) * scale + bias_ref[bidx + e, 0:RA, 0:CW]
                ex = jnp.exp2(s - jnp.max(s, axis=-1, keepdims=True))
                out.append(ex * _recip(jnp.sum(ex, axis=-1, keepdims=True)))
            return out

        def pv(p, v):
            v0, vm1, vm2, v2 = kv_tiles(v)
            o_a = _nn(p[0].astype(BF16), mat(v0))
            o_b = _nn(p[1].astype(BF16), mat(v2))
            p = p[0] + p[1]
            if full:
                o_m = _cat([_nn(p[0:M2 + seg].astype(BF16), mat(vm1)),
                            _nn(p[M2 + seg:R, 0:R].astype(BF16), mat(vm2))])
            else:
                o_m = _nn(p.astype(BF16), mat(vm2))
            return [o_a, o_m, o_b]

        ot = []
        pacc, qacc = {}, {}

        def add_o(r):
            n0 = 0 if r == 0 else RT + (r - 1) * GT
            oo = ot[n0:n0 + (RT if r == 0 else GT)]
            if full:
                gt = (lambda z: z) if (r >= TAILPV and not GT8) else functools.partial(gate, GO)
                us = [_cat([o[48:64], o[32:48]]) for o in oo]
                if LZ:
                    ops = _Operands([o[0:32] for o in oo], us, [o[64:80] for o in oo], gt)
                else:
                    ops = _Operands([o[0:32] for o in oo], [gt(z) for z in us], [o[64:80] for o in oo])
            else:
                ops = _Operands(None, None, oo)
            _fast_mm((S35 if r == 0 else S55)[1], ops, tile_dot(3, r), mh, pacc, qacc)

        bqkv = [None] * 3
        probs = []

        def do_pv():
            for g in range(len(ot) // 3, len(probs)):
                ot.extend(pv(probs[g], pair(2, g)))

        if full:
            an = pl.multiple_of(jnp.minimum(A0 + (s_ + 1) * AH, S - AH), AH)
            al = _ln(x_ref[pl.ds(an, AH), :].astype(F32))
            h_ref[RB:RB + AH, :] = al
            if LDA:
                dl.append((LDA, [al[e:e + 8, j * 128:(j + 1) * 128] for e in range(0, AH, 8) for j in range(3)]))
                dl.append((LDA + 2, [al[e:e + 8, j * 128:(j + 1) * 128] for e in range(0, AH, 8) for j in range(3, 5)]))

        for r in range(NG + 1):
            proj(2, r)
            proj(1, r)
            proj(0, r)
            if r == 0:
                blhs = _ln(b_in())
            if r < 3:
                bqkv[2 - r] = b_proj(blhs, 2 - r)
            if r == BAR:
                sink = []
                ob = b_attn(jobs, *bqkv, sink=sink)
                if BDL and full:
                    dl.extend((cnt[0] + BD0 + BDL * e, d) for e, d in enumerate(sink))
            if r == BOUT_R:
                zb = b_out(_cat(ob), b_in())
                x2_new = zb[0:seg]
                if full:
                    o_store(t - 1 - LAG, zb[seg:2 * seg])
                    nxt = x2_new
                else:
                    o_store(lb * (t_last - LAG - 1) - 1, x2_new)
                    nxt = jnp.where(t < LAG - 1, x_ref[seg:2 * seg, :].astype(F32), x2_new)
                sl = _ln(nxt)
                h_ref[n_mem:M2, :] = sl[0:n_mem]
                h_ref[M2 + n_mem:RB, :] = sl[n_mem:seg]
                if LD and full:
                    for j in range(nct):
                        dl.append((cnt[0] + LD + 2 * j, [sl[e:e + 8, j * 128:(j + 1) * 128] for e in range(0, seg, 8)]))
                    dl.sort(key=lambda e: e[0])
            if r in WSCHED:
                add_o(WSCHED[r])
            do_pv()
            for g in range(len(probs), (RT + r * GT) // 3):
                probs.append(scores(pair(0, g), pair(1, g)))
        for r in range(len(WSCHED), TAILPV):
            add_o(r)
        do_pv()
        for r in range(TAILPV, NG + 1):
            add_o(r)
        cols = []
        for n in range(nct):
            y, z, e = _fast_out(pacc, qacc, n, mh)
            cols.append(_cat([y, z[16:32], z[0:16], e]) if full else e)
        acc = _cat(cols, axis=1)

        y2 = x2_ref[...] + _cat([acc[n_mem:M2], acc[RA - seg + n_mem:RA]])
        mem2 = acc[RA - seg:RA - seg + n_mem]
        if full:
            x_cur = x_ref[pl.ds(pl.multiple_of(t * seg, seg), seg), :].astype(F32)
            xb_ref[0:seg, :] = x_cur + acc[M2:M2 + seg]
            xb_ref[seg:2 * seg, :] = y2
            m1n = acc[0:n_mem]
            m2n = mem2
        else:
            xb_ref[pl.ds(pl.multiple_of(jnp.where(t < LAG, 0, (t - n_seg + 2) * seg), seg), seg), :] = y2
            m1n = jnp.where(t < LAG - 1, h_ref[RB + AH:RB + AH + n_mem, :], mem2)
            m2n = jnp.where(t == LAG - 1, mem0_ref[...].astype(F32), mem2)
        x2_ref[...] = nxt
        return _cat([m1n, m2n])

    def single_body(t, c):
        @pl.when(t == n_seg)
        def _():
            out_copy(t - (LAG + 2)).start()
        return step(t, c, False)

    def full_body(t, c):
        @pl.when(t >= LAG + 2)
        def _():
            out_copy(t - (LAG + 2)).start()
        return step(t, c, True)

    def phase(ph, c):
        t0 = ph * n_seg
        c = lax.fori_loop(t0, t0 + LAG, single_body, c)

        @pl.when(ph == 0)
        def _():
            x_late.wait()
        return lax.fori_loop(LAG, jnp.where(ph == 0, n_seg, LAG), full_body, c)
    if not SKIPM:
      lax.fori_loop(0, 2, phase, _cat([h_ref[0:n_mem, :], h_ref[M2:M2 + n_mem, :]]))

    if SKIPM:
        def keep(i, c):
            z = (w_ref[i, pl.ds(pl.multiple_of(i * 8, 8), 8), :] + ring_ref[i, pl.ds(pl.multiple_of(i * 8, 8), 8), :]
                 + wr_ref[i & 3, pl.ds(pl.multiple_of(i * 8, 8), 8), :])
            xb_ref[2 * seg:2 * seg + 8, 0:128] = pltpu.bitcast(z, F32) + h_ref[pl.ds(pl.multiple_of((i & 7) * 8, 8), 8), 0:128] + x2_ref[0:8, 0:128]
            return c
        lax.fori_loop(0, 36, keep, 0)
    out_copy(n_seg - 3).start()
    res = xb_ref[2 * seg:4 * seg, :]
    blhs = _ln(res)
    ob = b_attn([(1, n_seg - 2), (1, n_seg - 1)], *[b_proj(blhs, part) for part in range(3)])
    o_store(n_seg - 2, b_out(_cat(ob), res))
    out_copy(n_seg - 2).start()
    out_copy(n_seg - 1).start()
    pltpu.make_async_copy(o_ref.at[pl.ds(seg, S), :], out_hbm, sem_o).wait()


@functools.partial(jax.jit, static_argnames=("seg",))
def _run(A_x, A_mem0, A_Wq, A_Wk, A_Wv, A_Wo, B_wqkv, B_wo, *, seg):
    _, S, dm = A_x.shape
    n_heads, dh = A_Wq.shape[1], A_Wq.shape[2]
    n_mem = A_mem0.shape[1]
    n_seg = S // seg
    hd = n_heads * dh
    nct = dm // 128
    ng = (hd // 128 - RT) // GT
    assert (seg, n_seg, n_mem, dh, dm % 128, n_heads, LAG) == (32, 64, 8, 192, 0, 32, 2)

    x = A_x.reshape(S, dm)
    mem0 = A_mem0.reshape(n_mem, dm)
    wq = jnp.transpose(A_Wq, (1, 2, 0)).reshape(hd, dm)
    wk = jnp.transpose(A_Wk, (1, 2, 0)).reshape(hd, dm)
    wv = jnp.transpose(A_Wv, (1, 2, 0)).reshape(hd, dm)
    wo = A_Wo.reshape(hd, dm)
    _, _, _, _, rs, xc = _plan(seg, n_seg)

    kern = functools.partial(_kernel, seg=seg, n_seg=n_seg, n_mem=n_mem,
                             n_heads=n_heads, dh=dh, dm=dm)
    hbm = pl.BlockSpec(memory_space=pltpu.HBM)

    out = pl.pallas_call(
        kern,
        in_specs=[hbm] * 8,
        out_specs=hbm,
        out_shape=jax.ShapeDtypeStruct((S, dm), A_x.dtype),
        scratch_shapes=[
            pltpu.VMEM((S, dm), BF16),
            pltpu.VMEM((n_mem, dm), BF16),
            pltpu.VMEM((NSLOT, 4, GT * 128, dm), BF16),
            pltpu.VMEM((RT * 128, dm), BF16),
            pltpu.VMEM((4, len(S53[0]) * 64, 128), U32),
            pltpu.VMEM((4 * ng, len(S55[0]) * 64, 128), U32),
            pltpu.VMEM((dm, 4 * dm + 128), BF16),
            pltpu.VMEM((nct, 4 * dm + 32, 128), F32),
            pltpu.VMEM((4 * nct, dm // 2, 128), U32),
            pltpu.VMEM((len(KEYS_R), HC * xc // 4, 128), U32),
            pltpu.VMEM((len(KEYS_R), HC * xc // 4, 128), U32),
            pltpu.VMEM((len(KEYS) - len(KEYS_R), NXC * xc // 4, 128), U32),
            pltpu.VMEM((15, 8, 128), U32),
            pltpu.VMEM((3 * hd // 128, rs // 2 + 8, 128), U32),
            pltpu.VMEM((3 * n_mem + seg + AH, dm), F32),
            pltpu.VMEM((4 * seg, dm), F32),
            pltpu.VMEM((seg, dm), F32),
            pltpu.VMEM((2, nct, HIST + seg, 128), F32),
            pltpu.VMEM((2, nct, HIST + seg, 128), F32),
            pltpu.VMEM((S + seg, dm), A_x.dtype),
            pltpu.VMEM((4, 2 * n_mem + 2 * seg, 128), F32),
            pltpu.VMEM((48, 48, 128), U32),
            pltpu.VMEM((len(BF), 40 * 64, 128), U32),
            pltpu.SemaphoreType.DMA((NSLOT,)),
            pltpu.SemaphoreType.DMA((8 + NXC,)),
            pltpu.SemaphoreType.DMA((4,)),
            pltpu.SemaphoreType.DMA(()),
        ],
        compiler_params=pltpu.CompilerParams(
            vmem_limit_bytes=128 * 1024 * 1024,
            disable_bounds_checks=True,
        ),
    )(x, mem0, wq, wk, wv, wo, B_wqkv, B_wo)
    return out.reshape(1, S, dm)


def pallas_interleave_layers__memory_aug_recurrent_mem_tr__sliding_local_dilated__prompt_kernel(
    A_x: jax.Array,
    A_mem0: jax.Array,
    A_Wq: jax.Array,
    A_Wk: jax.Array,
    A_Wv: jax.Array,
    A_Wo: jax.Array,
    A_seg_len,
    B_x: jax.Array,
    B_wqkv: jax.Array,
    B_wo: jax.Array,
):
    del B_x
    seg = A_seg_len if isinstance(A_seg_len, int) else 32
    return _run(A_x, A_mem0, A_Wq, A_Wk, A_Wv, A_Wo, B_wqkv, B_wo, seg=seg)
```

```python
import functools

import jax
import jax.numpy as jnp
from jax import lax
import jax.experimental.pallas as pl
import jax.experimental.pallas.tpu as pltpu

F32 = jnp.float32
BF16 = jnp.bfloat16
U32 = jnp.uint32
NEG = -1000000000.0
LN_EPS = 1e-05
LOG2E = 1.4426950408889634
NEG2 = NEG * LOG2E

B_HEADS = 32
B_WIN = 8
B_DIL = 2
HIST = 16
AH = 16
LAG = 2
NSLOT = 2
NXC = 6
HC = 3
WSCHED = {3: 0, 4: 1, 6: 2, 7: 3, 8: 4, 9: 5}
BOUT_R = 5
TAILPV = 8
GATE_O = 30
DUE_LN = 150
DUE_B0, DUE_B = 100, 60


def _ln(x):
    m = jnp.mean(x, axis=-1, keepdims=True)
    c = x - m
    v = jnp.mean(c * c, axis=-1, keepdims=True)
    return c * lax.rsqrt(v + LN_EPS)


def _recip(d):
    return pl.reciprocal(d, approx=True)


def _nt(a, b):
    return lax.dot_general(a, b, (((1,), (1,)), ((), ())), preferred_element_type=F32)


def _nn(a, b):
    return jnp.dot(a, b, preferred_element_type=F32)


def _cat(xs, axis=0):
    return xs[0] if len(xs) == 1 else jnp.concatenate(xs, axis=axis)


def _pk(z):
    return pltpu.bitcast(z, U32)


def _upk(z):
    return pltpu.bitcast(z, BF16)


LAM = (-1.5, -0.5, 0.0, 0.5, 1.5)


def _scheme(stars):
    tiles, prog = [], []
    for star in stars:
        if len(star) == 1:
            prog.append(("single", star[0], None, len(tiles)))
            tiles.append([star[0][:2]])
            continue
        left = [len(star) - 1] * len(star)
        for j in range(1, len(star)):
            for i in range(j):
                x, y = star[i], star[j]
                prog.append(("pair", x, y, len(tiles)))
                tiles += [[(x[0], y[1])], [(y[0], x[1])], [(x[0], y[1]), (y[0], x[1])]]
                for e in (i, j):
                    left[e] -= 1
                    if left[e] == 0:
                        z = star[e]
                        prog.append(("diag", z, None, len(tiles)))
                        tiles += [[z[:2]] + [(o[0], z[1]) for o in star if o is not z],
                                  [z[:2]] + [(z[0], o[1]) for o in star if o is not z]]
    return tiles, prog


S55 = _scheme([[(i, i, LAM[i]) for i in range(5)]])
S53 = _scheme([[(0, 0, LAM[0]), (2, 1, LAM[2]), (4, 2, LAM[4])], [(1, 0, LAM[1]), (3, 2, LAM[3])],
               [(1, 1, LAM[1])], [(3, 1, LAM[3])]])
S35 = _scheme([[(0, 0, LAM[0]), (1, 2, LAM[2]), (2, 4, LAM[4])], [(0, 1, LAM[1]), (2, 3, LAM[3])],
               [(1, 1, LAM[1])], [(1, 3, LAM[3])]])


def _spread(prog):
    pairs = [e for e in prog if e[0] != "diag"]
    diags = [e for e in prog if e[0] == "diag"]
    out, k = [], 0
    for i, e in enumerate(pairs):
        out.append(e)
        while k < len(diags) and (k + 0.5) * len(pairs) <= (i + 1) * len(diags):
            out.append(diags[k])
            k += 1
    return out + diags[k:]


def _op_keys(prog):
    keys = []
    for kind, x, y, _ in prog:
        if kind == "pair":
            new = [(nm, x[0], x[2], y[0], y[2]) for nm in ("l1", "l2", "A")]
        else:
            new = [("a", x[0], x[2]), ("b", x[0])]
        keys += [k for k in new if k not in keys]
    return keys


def _scaled(c, u):
    return u if c == 1.0 else c * u


class _Operands:
    def __init__(self, T, U, E):
        self.T, self.U, self.E, self.memo = T, U, E, {}

    def _get(self, key, fn):
        if key not in self.memo:
            self.memo[key] = fn()
        return self.memo[key]

    def paired(self, key):
        T, U = self.T, self.U
        if key[0] == "b":
            return U[key[1]]
        if key[0] == "a":
            k, lam = key[1:]
            if lam == 0.0:
                return T[k]
            return self._get(("f",) + key, lambda: T[k] - _scaled(lam, U[k]) if lam > 0
                             else T[k] + _scaled(-lam, U[k]))
        kx, lx, ky, ly = key[1:]
        A = self._get(("f", "A") + key[1:],
                      lambda: self.paired(("a", kx, lx)) + self.paired(("a", ky, ly)))
        if key[0] == "A":
            return A
        return A - _scaled(ly - lx, U[kx]) if key[0] == "l1" else A + _scaled(ly - lx, U[ky])

    def extra(self, key):
        if key[0] == "a":
            return self.E[key[1]]
        return self._get(("e", key[1], key[3]), lambda: self.E[key[1]] + self.E[key[3]])

    def __call__(self, key):
        if self.T is None:
            ek = ("a", key[1]) if key[0] in ("a", "s") else ("l", key[1], 0, key[3])
            return self._get(ek, lambda: self.extra(ek).astype(BF16))

        def build():
            ak = ("a",) + key[1:] if key[0] == "s" else key
            parts = [self.paired(ak)]
            if self.E is not None and ak[0] in ("a", "l1", "l2"):
                parts.append(self.extra(ak))
            if key[0] == "s":
                parts.append(self.U[key[1]])
            return _cat(parts).astype(BF16)
        return self._get(key, build)


def _fast_mm(prog, op, dot, m, p, q):
    def add(d, key, val):
        d[key] = val if key not in d else d[key] + val

    for kind, x, y, i in prog:
        if kind == "pair":
            kk = (x[0], x[2], y[0], y[2])
            p1, p2 = dot(op(("l1",) + kk), i), dot(op(("l2",) + kk), i + 1)
            if m:
                r = _scaled(1.0 / (y[2] - x[2]), p2[0:m] - p1[0:m] + dot(op(("A",) + kk), i + 2))
                add(q, (x[1], x[2]), r)
                add(q, (y[1], y[2]), r)
            add(p, y[1], p1)
            add(p, x[1], p2)
        elif kind == "diag":
            add(p, x[1], dot(op(("a", x[0], x[2])), i))
            if m:
                add(q, (x[1], x[2]), dot(op(("b", x[0])), i + 1))
        else:
            r = dot(op(("s", x[0], x[2])), i)
            add(p, x[1], r[0:r.shape[0] - m])
            if m:
                add(q, (x[1], x[2]), r[r.shape[0] - m:])


def _fast_out(p, q, n, m):
    if not m:
        return None, None, p[n]
    y, z = p[n][0:m], None
    for (nn, lam), v in q.items():
        if nn == n:
            z = v if z is None else z + v
            if lam != 0.0:
                y = y + _scaled(lam, v) if lam > 0 else y - _scaled(-lam, v)
    return y, z, (p[n][m:] if p[n].shape[0] > m else None)


def _combo(tile, block):
    out = block(*tile[0])
    for kn in tile[1:]:
        out = out - block(*kn)
    return out


GT = 5
RT = 3
KEYS_R = _op_keys(S53[1])
KEYS = KEYS_R + [k for k in _op_keys(S55[1]) if k not in KEYS_R]


def _plan(seg, n_seg):
    S = seg * n_seg
    R0 = LAG * seg
    A0 = S - (n_seg - LAG) * AH
    NPRE = A0 - R0 - LAG * 8
    RS = -(-(A0 - R0 + AH) // seg) * seg
    XC = NPRE // NXC // 32 * 32
    assert XC * NXC + 16 == NPRE
    return S, R0, A0, NPRE, RS, XC


def _kernel(x_hbm, mem0_hbm, wq_hbm, wk_hbm, wv_hbm, wo_hbm, bqkv_hbm, bwo_hbm,
            out_hbm,
            x_ref, mem0_ref, stage_ref, stage0_ref, wr_ref, w_ref, bst_ref, btmp_ref, bw_ref,
            xla_ref, xlb_ref, xlc_ref, xe_ref, ring_ref, h_ref, xb_ref, x2_ref, kb_ref, vb_ref, o_ref, bias_ref, kv_ref, bwf_ref,
            sem_w, sem_m, sem_b, sem_o,
            *, seg, n_seg, n_mem, n_heads, dh, dm):
    S, R0, A0, NPRE, RS, XC = _plan(seg, n_seg)
    M2 = 2 * n_mem
    R = M2 + 2 * seg
    RB = M2 + seg
    PW = 2 * dh
    G = n_heads // 2
    nct = dm // 128
    bdh = dm // B_HEADS
    NT = n_heads * dh // 128
    NG = (NT - RT) // GT
    w_hbm = (wq_hbm, wk_hbm, wv_hbm, wo_hbm)

    def w_copy(p, g):
        slot = g & (NSLOT - 1)
        return pltpu.make_async_copy(w_hbm[p].at[pl.ds((RT + (g - 1) * GT) * 128, GT * 128), :],
                                     stage_ref.at[slot, p], sem_w.at[slot])

    def w0_copy(p):
        dst = stage0_ref if p == 3 else stage_ref.at[0, p, pl.ds(0, RT * 128)]
        return pltpu.make_async_copy(w_hbm[p].at[pl.ds(0, RT * 128), :], dst, sem_m.at[4 + p])

    NB1 = 3 * nct
    WO0 = 3 * dm
    XF = A0 + AH
    XH = XC // 2

    def rows_copy(r0, n, sem):
        return pltpu.make_async_copy(x_hbm.at[pl.ds(r0, n), :], x_ref.at[pl.ds(r0, n), :], sem)

    def x_copy(i):
        return rows_copy(pl.multiple_of(R0 + i * XC, 16), XC, sem_m.at[8 + i])

    small = [rows_copy(0, R0, sem_m.at[1]), rows_copy(R0 + NPRE - 16, XF - R0 - NPRE + 16, sem_m.at[2]),
             pltpu.make_async_copy(mem0_hbm, mem0_ref, sem_m.at[3])]
    x_late = rows_copy(XF, S - XF, sem_m.at[0])

    def bq_copy(part):
        c0 = pl.multiple_of(part * dm, 128)
        return pltpu.make_async_copy(bqkv_hbm.at[:, pl.ds(c0, dm)], bst_ref.at[:, pl.ds(c0, dm)], sem_b.at[part])

    bo_copy = pltpu.make_async_copy(bwo_hbm, bst_ref.at[:, pl.ds(3 * dm, dm)], sem_b.at[3])

    def bst_tile(c):
        return bst_ref[:, pl.ds(pl.multiple_of(c * 128, 128), 128)]

    def bias_tables(full):
        RA = R if full else M2 + seg
        CW = 128
        ri = lax.broadcasted_iota(jnp.int32, (RA, CW), 0)
        ci = lax.broadcasted_iota(jnp.int32, (RA, CW), 1)
        if not full:
            ri = jnp.where(ri >= M2, ri + seg, ri)

        def table(i, bounds, vals):
            out = vals[-1]
            for b, v in zip(reversed(bounds), reversed(vals[:-1])):
                out = jnp.where(i < b, v, out)
            return out
        qi = ri - table(ri, [16, 48, 56], [0, 8, 48, 40])
        g0 = (ci < 8) | ((ci >= 16) & (ci < 48))
        k2 = ci - table(ci, [8, 24, 32, 48, 56, 80, 88, 96, 104], [-8, 0, 24, 8, 48, 40, 72, 80, 96, 104])
        if full:
            k1 = ci - table(ci, [8, 48], [0, 8, 40])
            row_l2 = ((ri >= 8) & (ri < 16)) | (ri >= 48)
            row_xa = (ri >= 8) & (ri < 16)
            valid = (row_xa == (ci >= 80)) & (ci < 112)
            is_a = jnp.where(ci >= 80, ((ci >= 88) & (ci < 104)).astype(jnp.int32),
                             (g0 != row_l2).astype(jnp.int32)) > 0
            ki = jnp.where(row_l2, k2, k1)
            visible = valid & ((qi < n_mem) | (qi >= ki))
            fill = jnp.where(valid, NEG2, -jnp.inf)
        else:
            is_a = jnp.logical_not(g0)
            visible = (qi < n_mem) | (qi >= k2)
            fill = NEG2
        for e, mine in enumerate((is_a, jnp.logical_not(is_a))):
            bias_ref[(0 if full else 2) + e, 0:RA, :] = jnp.where(
                mine, jnp.where(visible, 0.0, fill), -jnp.inf)

    for i in range(HC):
        x_copy(i).start()

    def zero_body(j, c):
        btmp_ref[j, 0:dm, :] = jnp.zeros((dm, 128), F32)
        return c
    lax.fori_loop(0, nct, zero_body, 0)

    w0_copy(0).start()
    xb_ref[0:2 * seg, :] = jnp.zeros((2 * seg, dm), F32)
    kb_ref[...] = jnp.zeros(kb_ref.shape, F32)
    vb_ref[...] = jnp.zeros(vb_ref.shape, F32)
    bst_ref[:, 4 * dm:] = jnp.zeros((dm, 128), BF16)
    bias_tables(True)
    bias_tables(False)

    def ekey(key):
        return ("a", key[1]) if key[0] == "a" else ("l", key[1], 0, key[3])
    EKEYS = []
    for key in KEYS:
        if key[0] in ("a", "l1") and ekey(key) not in EKEYS:
            EKEYS.append(ekey(key))

    def e_ops():
        ye = _ln(x_ref[R0 + NPRE - 16:R0 + NPRE, :].astype(F32))
        eops = _Operands(None, None, [ye[:, k * 128:(k + 1) * 128] for k in range(nct)])
        for j, key in enumerate(EKEYS):
            xe_ref[j] = _pk(eops(key))

    NKR = len(KEYS_R)

    def xl(j, hf, i):
        if j >= NKR:
            ref, j, i = xlc_ref, j - NKR, hf * HC + i
        else:
            ref = (xla_ref, xlb_ref)[hf]
        r0 = i * (XH // 2)
        return ref.at[j, pl.ds(r0 if isinstance(r0, int) else pl.multiple_of(r0, 8), XH // 2)]

    def ln_ops(hf, i, lo, hi):
        y = _ln(x_ref[pl.ds(pl.multiple_of(R0 + (hf * HC + i) * XC, 16), XC), :].astype(F32))
        ops = _Operands([y[0:XH, k * 128:(k + 1) * 128] for k in range(nct)],
                        [y[XH:XC, k * 128:(k + 1) * 128] for k in range(nct)], None)
        for j in range(lo, hi):
            xl(j, hf, i)[...] = _pk(ops(KEYS[j]))

    def ln_body(i, c):
        x_copy(i).wait()

        @pl.when(i == 0)
        def _():
            x_copy(HC).start()

        @pl.when(i == 1)
        def _():
            w0_copy(1).start()
            w0_copy(2).start()

        @pl.when(i == 2)
        def _():
            x_copy(HC + 1).start()
            x_copy(HC + 2).start()
            for cp in small:
                cp.start()
        ln_ops(0, i, 0, len(KEYS_R))
        return c
    lax.fori_loop(0, HC, ln_body, 0)

    def prep(scheme, w, dst):
        raw = lambda k, n: w[n * 128:(n + 1) * 128, k * 128:(k + 1) * 128]
        tb = []
        for i, tl in enumerate(scheme[0]):
            tb.append(raw(*tl[0]) if len(tl) == 1
                      else _combo(tl, lambda k, n: raw(k, n).astype(F32)).astype(BF16))
            dst[i * 64:(i + 1) * 64, :] = _pk(tb[i].T)
        return tb

    pcnt, pdl = [0], []

    def pre_chunk(scheme, w, dst, n0, chunks, never=None, tb=None):
        tiles, prog = scheme
        prog = _spread(prog)
        dot = lambda a, i: _nn(a, _upk(dst[i * 64:(i + 1) * 64, :]))
        if w is not None:
            if tb is None:
                tb = prep(scheme, w, dst)
            dot = lambda a, i: _nt(a, tb[i])

        for c in chunks:
            def op(key):
                def ld(kk):
                    v = xl(KEYS.index(kk), c // HC, c % HC)[...]
                    if c == NXC - 1 and kk[0] in ("a", "l1", "l2"):
                        v = _cat([v, xe_ref[EKEYS.index(ekey(kk))]])
                    return v
                if key[0] == "s":
                    return _upk(_cat([ld(("a",) + key[1:]), ld(("b", key[1]))]))
                v = ld(key)
                pcnt[0] += 1
                if pdl and pcnt[0] >= pdl[0][0]:
                    deps = pdl.pop(0)[1]
                    v = _cat([jnp.where(never, d, v[8 * e:8 * e + 8]) for e, d in enumerate(deps)]
                             + ([v[8 * len(deps):]] if v.shape[0] > 8 * len(deps) else []))
                return _upk(v)
            p, q = {}, {}
            _fast_mm(prog, op, dot, XH, p, q)
            for n in range(len(p)):
                y, z, e = _fast_out(p, q, n, XH)
                ring_ref[n0 + n, c * XH:c * XH + XH // 2, :] = _pk(y.astype(BF16))
                ring_ref[n0 + n, c * XH + XH // 2:(c + 1) * XH, :] = _pk(z.astype(BF16))
                if e is not None:
                    ring_ref[n0 + n, NXC * XH:NXC * XH + 8, :] = _pk(e.astype(BF16))

    def init_rows():
        x0 = x_ref[0:seg, :].astype(F32)
        sl = _ln(x0)
        xt = _ln(x_ref[R0 + NPRE:XF, :].astype(F32))
        h_ref[0:n_mem, :] = xt[0:n_mem]
        h_ref[n_mem:M2, :] = sl[0:n_mem]
        h_ref[M2:M2 + n_mem, :] = mem0_ref[...].astype(F32)
        h_ref[M2 + n_mem:RB, :] = sl[n_mem:seg]
        h_ref[RB:RB + AH, :] = xt[M2:M2 + AH]
        h_ref[RB + AH:RB + AH + n_mem, :] = xt[n_mem:M2]
        x2_ref[...] = x0

    def first_a(p, c):
        buf = stage_ref.at[0, p, pl.ds(0, RT * 128)]
        pltpu.make_async_copy(buf, buf, sem_m.at[4 + p]).wait()
        x_copy(HC + p).wait()

        @pl.when(p == 0)
        def _():
            for pp in range(4):
                w_copy(pp, 1).start()

        @pl.when(p == 2)
        def _():
            bq_copy(0).start()
        ln_ops(1, p, 0, len(KEYS))
        pre_chunk(S53, buf, wr_ref.at[p], p * NT, range(HC))
        return c
    lax.fori_loop(0, 3, first_a, 0)
    for cp in small:
        cp.wait()

    def first_b(p, c):
        e_ops()
        init_rows()
        ln_ops(0, p, len(KEYS_R), len(KEYS))
        pre_chunk(S53, None, wr_ref.at[p], p * NT, range(HC, NXC))
        return c
    lax.fori_loop(0, 3, first_b, 0)

    dpt = 128 // B_HEADS

    def b_stage1(u):
        uc = jnp.clip(u, 0, NB1 - 1)
        tr = bst_tile(jnp.where(u >= 0, uc, NB1 + nct)).astype(F32).T
        r0 = pl.multiple_of(uc * 128, 128)
        for j in range(nct):
            btmp_ref[j, pl.ds(r0, 128), :] = tr[:, j * 128:(j + 1) * 128]
        return [pltpu.bitcast(tr[120:128, j * 128:(j + 1) * 128], U32) for j in range(nct)]

    def b_stage1_wo(u):
        uc = jnp.clip(u, 0, nct - 1)
        btmp_ref[uc, WO0:WO0 + dm, :] = bst_tile(jnp.where(u >= 0, NB1 + uc, NB1 + nct)).astype(F32)

    def b_stage2(u):
        uc = jnp.clip(u, 0, NB1 - 1)
        part = (uc >= nct).astype(jnp.int32) + (uc >= 2 * nct).astype(jnp.int32)
        r0 = part * dm + (uc - part * nct) * dpt
        rows = _cat([_cat([btmp_ref[j, pl.ds(r0 + dd, B_HEADS, stride=bdh), :]
                           for j in range(nct)], axis=1) for dd in range(dpt)])
        val = _pk(rows.T.astype(BF16))
        bw_ref[uc] = val
        return [val[64 * j + 56:64 * j + 64] for j in range(nct)]

    def b_stage2_wo(u):
        uc = jnp.clip(u, 0, nct - 1)
        r0 = jnp.where(u >= 0, WO0, 0)
        bw_ref[NB1 + uc] = _pk(
            _cat([btmp_ref[uc, pl.ds(r0 + d, B_HEADS, stride=bdh), :] for d in range(bdh)]).astype(BF16))

    def wo_store(scheme, w, dst, never=None):
        if scheme is S55:
            rawt = lambda k, n: w[k * 128:(k + 1) * 128, n * 128:(n + 1) * 128]
            plain = [i for i, tl in enumerate(scheme[0]) if len(tl) == 1]
            for i, tl in enumerate(scheme[0]):
                if len(tl) > 1:
                    val = _combo(tl, lambda k, n: rawt(k, n).astype(F32)).astype(BF16)
                    val = _pk(_upk(_pk(val.T)).T)
                    dst[i * 64:(i + 1) * 64, :] = val
                    j = plain.pop()
                    pv_ = _pk(rawt(*scheme[0][j][0]))
                    dst[j * 64:(j + 1) * 64, :] = jnp.where(never, val, pv_)
            return
        for r in range(0, 128, 16):
            memo = {}

            def raw(k, n):
                return w[k * 128 + r:k * 128 + r + 16, n * 128:(n + 1) * 128]

            def block(k, n):
                if (k, n) not in memo:
                    memo[k, n] = raw(k, n).astype(F32)
                return memo[k, n]
            for i, tl in enumerate(scheme[0]):
                val = raw(*tl[0]) if len(tl) == 1 else _combo(tl, block).astype(BF16)
                dst[i * 64 + r // 2:i * 64 + r // 2 + 8, :] = _pk(val)

    def pre_body(g, c):
        slot = g & (NSLOT - 1)
        buf = stage_ref.at[slot]
        pltpu.make_async_copy(buf, buf, sem_w.at[slot]).wait()

        @pl.when((g >= 2) & (g <= 4))
        def _():
            bq_copy(g - 2).wait()

        @pl.when(g == 4)
        def _():
            bo_copy.wait()

        @pl.when(g <= 2)
        def _():
            bq_copy(g).start()

        @pl.when(g == 2)
        def _():
            bo_copy.start()

        @pl.when(g + 1 <= NG)
        def _():
            for p in range(4):
                w_copy(p, g + 1).start()

        @pl.when(g == NG - 1)
        def _():
            w0_copy(3).start()
            x_late.start()

        wo_store(S55, stage_ref.at[slot, 3], w_ref.at[3 * NG + g - 1], g > NG + 5)
        deps = [b_stage2(3 * (g - 5) + e) for e in range(3)]
        b_stage2_wo(g - 5)
        deps += [b_stage1(3 * (g - 2) + e) for e in range(3)]
        b_stage1_wo(g - 4)
        pcnt[0] = 0
        pdl.extend((DUE_B0 + DUE_B * e, d) for e, d in enumerate(deps))
        tbs = [prep(S55, stage_ref.at[slot, 0], w_ref.at[g - 1])]
        for p in range(3):
            if p < 2:
                tbs.append(prep(S55, stage_ref.at[slot, p + 1], w_ref.at[(p + 1) * NG + g - 1]))
            pre_chunk(S55, stage_ref.at[slot, p], w_ref.at[p * NG + g - 1], p * NT + RT + (g - 1) * GT, range(NXC),
                      g > NG + 5, tbs[p])
        return c
    lax.fori_loop(1, NG + 1, pre_body, 0)
    w0_copy(3).wait()

    for r in range(0, 64, 8):
        def raw(k, n):
            return bw_ref[2 * nct + n, k * 64 + r:k * 64 + r + 8, :]
        blocks = {(k, n): _upk(raw(k, n)).astype(F32) for k in range(nct) for n in range(nct)}
        for i, tl in enumerate(S55[0]):
            val = raw(*tl[0]) if len(tl) == 1 else _pk(_combo(tl, lambda k, n: blocks[k, n]).astype(BF16))
            bwf_ref[i * 64 + r:i * 64 + r + 8, :] = val

    bscale = float(bdh) ** (-0.5) * LOG2E

    def b_proj(lhs, part):
        if part == 2 and lhs.shape[0] == 2 * seg:
            kt = lambda a: [a[:, k * 128:(k + 1) * 128] for k in range(nct)]
            ops = _Operands(kt(lhs[0:seg]), kt(lhs[seg:2 * seg]), None)
            p, q = {}, {}
            _fast_mm(S55[1], ops, lambda a, i: _nn(a, _upk(bwf_ref[i * 64:(i + 1) * 64, :])), seg, p, q)
            return _cat([_cat(_fast_out(p, q, n, seg)[0:2]) for n in range(nct)], axis=1)
        return _nn(lhs.astype(BF16), _cat([_upk(bw_ref[part * nct + j]) for j in range(nct)], axis=1))

    def b_attn(jobs, q, k, v):
        row = lax.broadcasted_iota(jnp.int32, (seg, 128), 0)
        outs = []
        for i, (l, sidx) in enumerate(jobs):
            r0 = i * seg
            pos = row + sidx * seg
            for j in range(nct):
                kb_ref[l, j, 0:HIST, :] = kb_ref[l, j, seg:seg + HIST, :]
                vb_ref[l, j, 0:HIST, :] = vb_ref[l, j, seg:seg + HIST, :]
            for j in range(nct):
                kb_ref[l, j, HIST:HIST + seg, :] = k[r0:r0 + seg, j * 128:(j + 1) * 128]
                vb_ref[l, j, HIST:HIST + seg, :] = v[r0:r0 + seg, j * 128:(j + 1) * 128]
            logits = []
            for w in range(B_WIN):
                o = HIST - w * B_DIL
                acc = None
                for j in range(nct):
                    p = q[r0:r0 + seg, j * 128:(j + 1) * 128] * kb_ref[l, j, o:o + seg, :]
                    acc = p if acc is None else acc + p
                acc = acc + pltpu.roll(acc, 64, 1)
                acc = acc + pltpu.roll(acc, 32, 1)
                lg = acc * bscale
                if w > 0:
                    lg = jnp.where(pos >= w * B_DIL, lg, NEG2)
                logits.append(lg)
            m = logits[0]
            for w in range(1, B_WIN):
                m = jnp.maximum(m, logits[w])
            es = [jnp.exp2(lg - m) for lg in logits]
            den = es[0]
            for w in range(1, B_WIN):
                den = den + es[w]
            inv = _recip(den)
            cols = []
            for j in range(nct):
                acc = None
                for w in range(B_WIN):
                    o = HIST - w * B_DIL
                    p = es[w] * vb_ref[l, j, o:o + seg, :]
                    acc = p if acc is None else acc + p
                cols.append(acc * inv)
            outs.append(_cat(cols, axis=1).astype(BF16))
        return outs

    def b_out(ob, res):
        return res + b_proj(ob, 3)

    def o_store(b, val):
        ro = pl.multiple_of((b + 1) * seg, seg)
        o_ref[pl.ds(ro, val.shape[0]), :] = val.astype(o_ref.dtype)

    def out_copy(b):
        ro = pl.multiple_of(b * seg, seg)
        return pltpu.make_async_copy(o_ref.at[pl.ds(ro + seg, seg), :], out_hbm.at[pl.ds(ro, seg), :], sem_o)

    def step(t, hc, full):
        t_last = n_seg + LAG - 1
        if full:
            jobs = [(0, t - 1), (1, t - 1 - LAG)]

            def b_in():
                return xb_ref[0:2 * seg, :]
        else:
            lb = (t == t_last).astype(jnp.int32)
            jobs = [(lb, t - 1 - lb * (LAG + 1))]

            def b_in():
                return xb_ref[pl.ds(pl.multiple_of(lb * seg, seg), seg), :]
        v0r = _cat([hc[0:n_mem], h_ref[n_mem:M2, :]])
        v1r = _cat([hc[n_mem:M2], h_ref[M2 + n_mem:2 * M2, :]])

        hist = []
        never = t > 4 * n_seg

        def gate(back, z):
            gv = hist[-back]
            return _cat([jnp.where(never, gv, z[e:e + 8]) for e in range(0, z.shape[0], 8)])

        def ktiles(z):
            return [z[:, k * 128:(k + 1) * 128] for k in range(z.shape[1] // 128)]
        if full:
            hl = _Operands(ktiles(_cat([v0r, h_ref[2 * M2:RB, :]])), ktiles(_cat([v1r, h_ref[RB:RB + AH, :]])), None)
        else:
            hl = _Operands(None, None, ktiles(_cat([v0r, v1r, h_ref[2 * M2:RB, :]])))
        mh = 2 * M2 if full else 0

        def tile_dot(p, r):
            src = wr_ref.at[p] if r == 0 else w_ref.at[p * NG + r - 1]

            def dot(a, i):
                wt = src[i * 64:(i + 1) * 64, :]
                cnt[0] += 1
                if dl and cnt[0] >= dl[0][0]:
                    deps = dl.pop(0)[1]
                    wt = _cat([jnp.where(never, pltpu.bitcast(d, U32), wt[8 * e:8 * e + 8])
                               for e, d in enumerate(deps)] + [wt[8 * len(deps):]])
                res_ = _nn(a, _upk(wt))
                hist.append(res_[0:8])
                return res_
            return dot
        cnt, dl = [0], []
        scale = float(dh) ** (-0.5) * LOG2E
        if full:
            s_ = t - LAG
            rd = pl.multiple_of(lax.rem(s_ * (seg // 2), RS // 2), seg // 2)
            wa = pl.multiple_of(lax.rem((A0 - R0 + s_ * AH) // 2, RS // 2), 8)
        else:
            wx = pl.multiple_of(jnp.where(t < LAG, NPRE // 2 + t * (n_mem // 2), RS // 2), n_mem // 2)
            wo_store(S35, stage0_ref, wr_ref.at[3])

        RA = R if full else M2 + seg
        CW = R + 2 * M2 if full else R
        bidx = 0 if full else 2
        half = dh - 128
        la8 = lax.broadcasted_iota(jnp.int32, (n_mem, 128), 1) < half
        ones = jnp.full((n_mem, 128), 0xFFFFFFFF, U32)
        zero = jnp.zeros((n_mem, 128), U32)
        mask_a = jnp.where(la8, ones, zero)
        mask_b = jnp.where(la8, zero, ones)

        def pk2(a, b):
            return _pk(_cat([a, b]).astype(BF16))

        yt = [[None] * NT for _ in range(3)]

        def proj(p, r):
            pa, qa = {}, {}
            _fast_mm((S53 if r == 0 else S55)[1], hl, tile_dot(p, r), mh, pa, qa)
            n0 = 0 if r == 0 else RT + (r - 1) * GT
            for n in range(len(pa)):
                y, z, e = _fast_out(pa, qa, n, mh)
                idx = p * NT + n0 + n
                if full:
                    ring_ref[idx, pl.ds(wa, 8), :] = pk2(z[16:24], z[24:32])
                    y = _cat([y[0:M2], z[0:M2], y[M2:2 * M2]])
                else:
                    y = e
                    ring_ref[idx, pl.ds(wx, n_mem // 2), :] = pk2(y[0:8], y[8:16])[0:n_mem // 2]
                yt[p][n0 + n] = stash(p * 16 + (n0 + n) % 16, packed(p, (n0 + n) % 3, y))

        def ab(z8):
            return jnp.where(la8, z8, 0.0), jnp.where(la8, 0.0, z8)

        def packed(p, j, y):
            u2 = pk2(y[32:40], y[40:48])
            if p == 0 or j == 0:
                return [pk2(y[0:8], y[8:16]), pk2(y[16:24], y[24:32]), u2]
            if j == 2:
                return [pk2(y[8:16], y[0:8]), pk2(y[24:32], y[16:24]), u2]
            xa_a, xa_b = ab(y[8:16])
            out = [pk2(xa_b, xa_a), pk2(y[24:32], y[16:24]) & mask_b, pk2(y[16:24], y[24:32]) & mask_a, u2]
            if full:
                out += [pk2(*ab(y[0:8])), pk2(*ab(y[16:24]))]
            return out

        def stash(idx, parts):
            kv_ref[idx, 0:8 * len(parts), :] = _cat(parts)
            return lambda: [kv_ref[idx, 8 * e:8 * e + 8, :] for e in range(len(parts))]

        def pair(p, g):
            xs = [ring_ref[p * NT + 3 * g + j, pl.ds(rd, seg // 2), :] for j in range(3)] if full else None
            return [f() for f in yt[p][3 * g:3 * g + 3]], xs

        def q_rows(z, j):
            v0, v1, v2 = z[0][j]
            return [v0] + ([z[1][j]] if full else []) + [v1, v2]

        def kv_tiles(z):
            yt, x1 = z
            v0, v1, v2 = yt[0]
            t0 = [v0] + ([x1[0]] if full else [v1, v2]) + [v1, v2]
            w0, w1, w2 = yt[2]
            t2 = [w0, w1, w2] + ([x1[2]] if full else [w1, w2])
            if full:
                t0 += [v0, v1]
                t2 += [w0, w1]
            e1, mb, ma, u2 = yt[1][0:4]
            mid2 = [e1, mb, u2 & mask_b, ma, u2 & mask_a]
            mid1 = None
            if full:
                lo, hi = x1[1][0:8], x1[1][8:16]
                mid1 = [yt[1][4], lo & mask_a, hi & mask_a, lo & mask_b, hi & mask_b, e1, yt[1][5]]
            return t0, mid1, mid2, t2

        def mat(parts):
            return _upk(_cat(parts))

        def scores(q, k):
            k0, km1, km2, k2_ = kv_tiles(k)
            s_a = _nt(mat(q_rows(q, 0)), mat(k0))
            s_b = _nt(mat(q_rows(q, 2)), mat(k2_))
            qm = q_rows(q, 1)
            if full:
                s_m = _cat([_nt(mat(qm[0:2]), mat(km1)), _cat([_nt(mat(qm[2:4]), mat(km2)), jnp.zeros((seg, CW - R), F32)], axis=1)])
            else:
                s_m = _nt(mat(qm), mat(km2))
            out = []
            for e, sx in enumerate((s_a, s_b)):
                s = (sx + s_m) * scale + bias_ref[bidx + e, 0:RA, 0:CW]
                ex = jnp.exp2(s - jnp.max(s, axis=-1, keepdims=True))
                out.append(ex * _recip(jnp.sum(ex, axis=-1, keepdims=True)))
            return out

        def pv(p, v):
            v0, vm1, vm2, v2 = kv_tiles(v)
            o_a = _nn(p[0].astype(BF16), mat(v0))
            o_b = _nn(p[1].astype(BF16), mat(v2))
            p = p[0] + p[1]
            if full:
                o_m = _cat([_nn(p[0:M2 + seg].astype(BF16), mat(vm1)),
                            _nn(p[M2 + seg:R, 0:R].astype(BF16), mat(vm2))])
            else:
                o_m = _nn(p.astype(BF16), mat(vm2))
            return [o_a, o_m, o_b]

        ot = []
        pacc, qacc = {}, {}

        def add_o(r):
            n0 = 0 if r == 0 else RT + (r - 1) * GT
            oo = ot[n0:n0 + (RT if r == 0 else GT)]
            if full:
                us = [_cat([o[48:64], o[32:48]]) for o in oo]
                if r < TAILPV:
                    us = [gate(GATE_O, z) for z in us]
                ops = _Operands([o[0:32] for o in oo], us, [o[64:80] for o in oo])
            else:
                ops = _Operands(None, None, oo)
            _fast_mm((S35 if r == 0 else S55)[1], ops, tile_dot(3, r), mh, pacc, qacc)

        bqkv = [None] * 3
        probs = []

        def do_pv():
            for g in range(len(ot) // 3, len(probs)):
                ot.extend(pv(probs[g], pair(2, g)))

        if full:
            an = pl.multiple_of(jnp.minimum(A0 + (s_ + 1) * AH, S - AH), AH)
            h_ref[RB:RB + AH, :] = _ln(x_ref[pl.ds(an, AH), :].astype(F32))

        for r in range(NG + 1):
            proj(2, r)
            proj(1, r)
            proj(0, r)
            if r == 0:
                blhs = _ln(b_in())
            if r < 3:
                bqkv[2 - r] = b_proj(blhs, 2 - r)
            if r == 3:
                ob = b_attn(jobs, *bqkv)
            if r == BOUT_R:
                zb = b_out(_cat(ob), b_in())
                x2_new = zb[0:seg]
                if full:
                    o_store(t - 1 - LAG, zb[seg:2 * seg])
                    nxt = x2_new
                else:
                    o_store(lb * (t_last - LAG - 1) - 1, x2_new)
                    nxt = jnp.where(t < LAG - 1, x_ref[seg:2 * seg, :].astype(F32), x2_new)
                sl = _ln(nxt)
                h_ref[n_mem:M2, :] = sl[0:n_mem]
                h_ref[M2 + n_mem:RB, :] = sl[n_mem:seg]
                if full:
                    for j in range(nct):
                        dl.append((cnt[0] + DUE_LN + 2 * j, [sl[e:e + 8, j * 128:(j + 1) * 128] for e in range(0, seg, 8)]))
            if r in WSCHED:
                add_o(WSCHED[r])
            do_pv()
            for g in range(len(probs), (RT + r * GT) // 3):
                probs.append(scores(pair(0, g), pair(1, g)))
        for r in range(len(WSCHED), TAILPV):
            add_o(r)
        do_pv()
        for r in range(TAILPV, NG + 1):
            add_o(r)
        cols = []
        for n in range(nct):
            y, z, e = _fast_out(pacc, qacc, n, mh)
            cols.append(_cat([y, z[16:32], z[0:16], e]) if full else e)
        acc = _cat(cols, axis=1)

        y2 = x2_ref[...] + _cat([acc[n_mem:M2], acc[RA - seg + n_mem:RA]])
        mem2 = acc[RA - seg:RA - seg + n_mem]
        if full:
            x_cur = x_ref[pl.ds(pl.multiple_of(t * seg, seg), seg), :].astype(F32)
            xb_ref[0:seg, :] = x_cur + acc[M2:M2 + seg]
            xb_ref[seg:2 * seg, :] = y2
            m1n = acc[0:n_mem]
            m2n = mem2
        else:
            xb_ref[pl.ds(pl.multiple_of(jnp.where(t < LAG, 0, (t - n_seg + 2) * seg), seg), seg), :] = y2
            m1n = jnp.where(t < LAG - 1, h_ref[RB + AH:RB + AH + n_mem, :], mem2)
            m2n = jnp.where(t == LAG - 1, mem0_ref[...].astype(F32), mem2)
        x2_ref[...] = nxt
        return _cat([m1n, m2n])

    def single_body(t, c):
        @pl.when(t == n_seg)
        def _():
            out_copy(t - (LAG + 2)).start()
        return step(t, c, False)

    def full_body(t, c):
        @pl.when(t >= LAG + 2)
        def _():
            out_copy(t - (LAG + 2)).start()
        return step(t, c, True)

    def phase(ph, c):
        t0 = ph * n_seg
        c = lax.fori_loop(t0, t0 + LAG, single_body, c)

        @pl.when(ph == 0)
        def _():
            x_late.wait()
        return lax.fori_loop(LAG, jnp.where(ph == 0, n_seg, LAG), full_body, c)
    lax.fori_loop(0, 2, phase, _cat([h_ref[0:n_mem, :], h_ref[M2:M2 + n_mem, :]]))

    out_copy(n_seg - 3).start()
    res = xb_ref[2 * seg:4 * seg, :]
    blhs = _ln(res)
    ob = b_attn([(1, n_seg - 2), (1, n_seg - 1)], *[b_proj(blhs, part) for part in range(3)])
    o_store(n_seg - 2, b_out(_cat(ob), res))
    out_copy(n_seg - 2).start()
    out_copy(n_seg - 1).start()
    pltpu.make_async_copy(o_ref.at[pl.ds(seg, S), :], out_hbm, sem_o).wait()


@functools.partial(jax.jit, static_argnames=("seg",))
def _run(A_x, A_mem0, A_Wq, A_Wk, A_Wv, A_Wo, B_wqkv, B_wo, *, seg):
    _, S, dm = A_x.shape
    n_heads, dh = A_Wq.shape[1], A_Wq.shape[2]
    n_mem = A_mem0.shape[1]
    n_seg = S // seg
    hd = n_heads * dh
    nct = dm // 128
    ng = (hd // 128 - RT) // GT
    assert (seg, n_seg, n_mem, dh, dm % 128, n_heads, LAG) == (32, 64, 8, 192, 0, 32, 2)

    x = A_x.reshape(S, dm)
    mem0 = A_mem0.reshape(n_mem, dm)
    wq = jnp.transpose(A_Wq, (1, 2, 0)).reshape(hd, dm)
    wk = jnp.transpose(A_Wk, (1, 2, 0)).reshape(hd, dm)
    wv = jnp.transpose(A_Wv, (1, 2, 0)).reshape(hd, dm)
    wo = A_Wo.reshape(hd, dm)
    _, _, _, _, rs, xc = _plan(seg, n_seg)

    kern = functools.partial(_kernel, seg=seg, n_seg=n_seg, n_mem=n_mem,
                             n_heads=n_heads, dh=dh, dm=dm)
    hbm = pl.BlockSpec(memory_space=pltpu.HBM)

    out = pl.pallas_call(
        kern,
        in_specs=[hbm] * 8,
        out_specs=hbm,
        out_shape=jax.ShapeDtypeStruct((S, dm), A_x.dtype),
        scratch_shapes=[
            pltpu.VMEM((S, dm), BF16),
            pltpu.VMEM((n_mem, dm), BF16),
            pltpu.VMEM((NSLOT, 4, GT * 128, dm), BF16),
            pltpu.VMEM((RT * 128, dm), BF16),
            pltpu.VMEM((4, len(S53[0]) * 64, 128), U32),
            pltpu.VMEM((4 * ng, len(S55[0]) * 64, 128), U32),
            pltpu.VMEM((dm, 4 * dm + 128), BF16),
            pltpu.VMEM((nct, 4 * dm + 32, 128), F32),
            pltpu.VMEM((4 * nct, dm // 2, 128), U32),
            pltpu.VMEM((len(KEYS_R), HC * xc // 4, 128), U32),
            pltpu.VMEM((len(KEYS_R), HC * xc // 4, 128), U32),
            pltpu.VMEM((len(KEYS) - len(KEYS_R), NXC * xc // 4, 128), U32),
            pltpu.VMEM((15, 8, 128), U32),
            pltpu.VMEM((3 * hd // 128, rs // 2 + 8, 128), U32),
            pltpu.VMEM((3 * n_mem + seg + AH, dm), F32),
            pltpu.VMEM((4 * seg, dm), F32),
            pltpu.VMEM((seg, dm), F32),
            pltpu.VMEM((2, nct, HIST + seg, 128), F32),
            pltpu.VMEM((2, nct, HIST + seg, 128), F32),
            pltpu.VMEM((S + seg, dm), A_x.dtype),
            pltpu.VMEM((4, 2 * n_mem + 2 * seg, 128), F32),
            pltpu.VMEM((48, 48, 128), U32),
            pltpu.VMEM((len(S55[0]) * 64, 128), U32),
            pltpu.SemaphoreType.DMA((NSLOT,)),
            pltpu.SemaphoreType.DMA((8 + NXC,)),
            pltpu.SemaphoreType.DMA((4,)),
            pltpu.SemaphoreType.DMA(()),
        ],
        compiler_params=pltpu.CompilerParams(
            vmem_limit_bytes=127 * 1024 * 1024,
            disable_bounds_checks=True,
        ),
    )(x, mem0, wq, wk, wv, wo, B_wqkv, B_wo)
    return out.reshape(1, S, dm)


def pallas_interleave_layers__memory_aug_recurrent_mem_tr__sliding_local_dilated__prompt_kernel(
    A_x: jax.Array,
    A_mem0: jax.Array,
    A_Wq: jax.Array,
    A_Wk: jax.Array,
    A_Wv: jax.Array,
    A_Wo: jax.Array,
    A_seg_len,
    B_x: jax.Array,
    B_wqkv: jax.Array,
    B_wo: jax.Array,
):
    del B_x
    seg = A_seg_len if isinstance(A_seg_len, int) else 32
    return _run(A_x, A_mem0, A_Wq, A_Wk, A_Wv, A_Wo, B_wqkv, B_wo, seg=seg)
```

```python
import functools

import jax
import jax.numpy as jnp
from jax import lax
import jax.experimental.pallas as pl
import jax.experimental.pallas.tpu as pltpu

F32 = jnp.float32
BF16 = jnp.bfloat16
U32 = jnp.uint32
NEG = -1000000000.0
LN_EPS = 1e-05
LOG2E = 1.4426950408889634
NEG2 = NEG * LOG2E

B_HEADS = 32
B_WIN = 8
B_DIL = 2
HIST = 16
AH = 16
LAG = 2
NSLOT = 2
NXC = 6
HC = 3
WSCHED = {3: 0, 4: 1, 6: 2, 7: 3, 8: 4, 9: 5}
BOUT_R = 5
TAILPV = 8
GATE_O = 30
DUE_LN = 150
DUE_X = 24
DUE_B0, DUE_B = 100, 60


def _ln(x):
    m = jnp.mean(x, axis=-1, keepdims=True)
    c = x - m
    v = jnp.mean(c * c, axis=-1, keepdims=True)
    return c * lax.rsqrt(v + LN_EPS)


def _recip(d):
    return pl.reciprocal(d, approx=True)


def _nt(a, b):
    return lax.dot_general(a, b, (((1,), (1,)), ((), ())), preferred_element_type=F32)


def _nn(a, b):
    return jnp.dot(a, b, preferred_element_type=F32)


def _cat(xs, axis=0):
    return xs[0] if len(xs) == 1 else jnp.concatenate(xs, axis=axis)


def _pk(z):
    return pltpu.bitcast(z, U32)


def _upk(z):
    return pltpu.bitcast(z, BF16)


LAM = (-1.5, -0.5, 0.0, 0.5, 1.5)


def _scheme(stars):
    tiles, prog = [], []
    for star in stars:
        if len(star) == 1:
            prog.append(("single", star[0], None, len(tiles)))
            tiles.append([star[0][:2]])
            continue
        left = [len(star) - 1] * len(star)
        for j in range(1, len(star)):
            for i in range(j):
                x, y = star[i], star[j]
                prog.append(("pair", x, y, len(tiles)))
                tiles += [[(x[0], y[1])], [(y[0], x[1])], [(x[0], y[1]), (y[0], x[1])]]
                for e in (i, j):
                    left[e] -= 1
                    if left[e] == 0:
                        z = star[e]
                        prog.append(("diag", z, None, len(tiles)))
                        tiles += [[z[:2]] + [(o[0], z[1]) for o in star if o is not z],
                                  [z[:2]] + [(z[0], o[1]) for o in star if o is not z]]
    return tiles, prog


S55 = _scheme([[(i, i, LAM[i]) for i in range(5)]])
S53 = _scheme([[(0, 0, LAM[0]), (2, 1, LAM[2]), (4, 2, LAM[4])], [(1, 0, LAM[1]), (3, 2, LAM[3])],
               [(1, 1, LAM[1])], [(3, 1, LAM[3])]])
S35 = _scheme([[(0, 0, LAM[0]), (1, 2, LAM[2]), (2, 4, LAM[4])], [(0, 1, LAM[1]), (2, 3, LAM[3])],
               [(1, 1, LAM[1])], [(1, 3, LAM[3])]])


def _spread(prog):
    pairs = [e for e in prog if e[0] != "diag"]
    diags = [e for e in prog if e[0] == "diag"]
    out, k = [], 0
    for i, e in enumerate(pairs):
        out.append(e)
        while k < len(diags) and (k + 0.5) * len(pairs) <= (i + 1) * len(diags):
            out.append(diags[k])
            k += 1
    return out + diags[k:]


def _op_keys(prog):
    keys = []
    for kind, x, y, _ in prog:
        if kind == "pair":
            new = [(nm, x[0], x[2], y[0], y[2]) for nm in ("l1", "l2", "A")]
        else:
            new = [("a", x[0], x[2]), ("b", x[0])]
        keys += [k for k in new if k not in keys]
    return keys


def _scaled(c, u):
    return u if c == 1.0 else c * u


class _Operands:
    def __init__(self, T, U, E):
        self.T, self.U, self.E, self.memo = T, U, E, {}

    def _get(self, key, fn):
        if key not in self.memo:
            self.memo[key] = fn()
        return self.memo[key]

    def paired(self, key):
        T, U = self.T, self.U
        if key[0] == "b":
            return U[key[1]]
        if key[0] == "a":
            k, lam = key[1:]
            if lam == 0.0:
                return T[k]
            return self._get(("f",) + key, lambda: T[k] - _scaled(lam, U[k]) if lam > 0
                             else T[k] + _scaled(-lam, U[k]))
        kx, lx, ky, ly = key[1:]
        A = self._get(("f", "A") + key[1:],
                      lambda: self.paired(("a", kx, lx)) + self.paired(("a", ky, ly)))
        if key[0] == "A":
            return A
        return A - _scaled(ly - lx, U[kx]) if key[0] == "l1" else A + _scaled(ly - lx, U[ky])

    def extra(self, key):
        if key[0] == "a":
            return self.E[key[1]]
        return self._get(("e", key[1], key[3]), lambda: self.E[key[1]] + self.E[key[3]])

    def __call__(self, key):
        if self.T is None:
            ek = ("a", key[1]) if key[0] in ("a", "s") else ("l", key[1], 0, key[3])
            return self._get(ek, lambda: self.extra(ek).astype(BF16))

        def build():
            ak = ("a",) + key[1:] if key[0] == "s" else key
            parts = [self.paired(ak)]
            if self.E is not None and ak[0] in ("a", "l1", "l2"):
                parts.append(self.extra(ak))
            if key[0] == "s":
                parts.append(self.U[key[1]])
            return _cat(parts).astype(BF16)
        return self._get(key, build)


def _fast_mm(prog, op, dot, m, p, q):
    def add(d, key, val):
        d[key] = val if key not in d else d[key] + val

    for kind, x, y, i in prog:
        if kind == "pair":
            kk = (x[0], x[2], y[0], y[2])
            p1, p2 = dot(op(("l1",) + kk), i), dot(op(("l2",) + kk), i + 1)
            if m:
                r = _scaled(1.0 / (y[2] - x[2]), p2[0:m] - p1[0:m] + dot(op(("A",) + kk), i + 2))
                add(q, (x[1], x[2]), r)
                add(q, (y[1], y[2]), r)
            add(p, y[1], p1)
            add(p, x[1], p2)
        elif kind == "diag":
            add(p, x[1], dot(op(("a", x[0], x[2])), i))
            if m:
                add(q, (x[1], x[2]), dot(op(("b", x[0])), i + 1))
        else:
            r = dot(op(("s", x[0], x[2])), i)
            add(p, x[1], r[0:r.shape[0] - m])
            if m:
                add(q, (x[1], x[2]), r[r.shape[0] - m:])


def _fast_out(p, q, n, m):
    if not m:
        return None, None, p[n]
    y, z = p[n][0:m], None
    for (nn, lam), v in q.items():
        if nn == n:
            z = v if z is None else z + v
            if lam != 0.0:
                y = y + _scaled(lam, v) if lam > 0 else y - _scaled(-lam, v)
    return y, z, (p[n][m:] if p[n].shape[0] > m else None)


def _combo(tile, block):
    out = block(*tile[0])
    for kn in tile[1:]:
        out = out - block(*kn)
    return out


GT = 5
RT = 3
KEYS_R = _op_keys(S53[1])
KEYS = KEYS_R + [k for k in _op_keys(S55[1]) if k not in KEYS_R]


def _plan(seg, n_seg):
    S = seg * n_seg
    R0 = LAG * seg
    A0 = S - (n_seg - LAG) * AH
    NPRE = A0 - R0 - LAG * 8
    RS = -(-(A0 - R0 + AH) // seg) * seg
    XC = NPRE // NXC // 32 * 32
    assert XC * NXC + 16 == NPRE
    return S, R0, A0, NPRE, RS, XC


def _kernel(x_hbm, mem0_hbm, wq_hbm, wk_hbm, wv_hbm, wo_hbm, bqkv_hbm, bwo_hbm,
            out_hbm,
            x_ref, mem0_ref, stage_ref, stage0_ref, wr_ref, w_ref, bst_ref, btmp_ref, bw_ref,
            xla_ref, xlb_ref, xlc_ref, xe_ref, ring_ref, h_ref, xb_ref, x2_ref, kb_ref, vb_ref, o_ref, bias_ref, kv_ref, bwf_ref,
            sem_w, sem_m, sem_b, sem_o,
            *, seg, n_seg, n_mem, n_heads, dh, dm):
    S, R0, A0, NPRE, RS, XC = _plan(seg, n_seg)
    M2 = 2 * n_mem
    R = M2 + 2 * seg
    RB = M2 + seg
    nct = dm // 128
    bdh = dm // B_HEADS
    NT = n_heads * dh // 128
    NG = (NT - RT) // GT
    w_hbm = (wq_hbm, wk_hbm, wv_hbm, wo_hbm)

    def w_copy(p, g):
        slot = g & (NSLOT - 1)
        return pltpu.make_async_copy(w_hbm[p].at[pl.ds((RT + (g - 1) * GT) * 128, GT * 128), :],
                                     stage_ref.at[slot, p], sem_w.at[slot])

    def w0_copy(p):
        dst = stage0_ref if p == 3 else stage_ref.at[0, p, pl.ds(0, RT * 128)]
        return pltpu.make_async_copy(w_hbm[p].at[pl.ds(0, RT * 128), :], dst, sem_m.at[4 + p])

    NB1 = 3 * nct
    WO0 = 3 * dm
    XF = A0 + AH
    XH = XC // 2

    def rows_copy(r0, n, sem):
        return pltpu.make_async_copy(x_hbm.at[pl.ds(r0, n), :], x_ref.at[pl.ds(r0, n), :], sem)

    def x_copy(i):
        return rows_copy(pl.multiple_of(R0 + i * XC, 16), XC, sem_m.at[8 + i])

    small = [rows_copy(0, R0, sem_m.at[1]), rows_copy(R0 + NPRE - 16, XF - R0 - NPRE + 16, sem_m.at[2]),
             pltpu.make_async_copy(mem0_hbm, mem0_ref, sem_m.at[3])]
    x_late = rows_copy(XF, S - XF, sem_m.at[0])

    def bq_copy(part):
        c0 = pl.multiple_of(part * dm, 128)
        return pltpu.make_async_copy(bqkv_hbm.at[:, pl.ds(c0, dm)], bst_ref.at[:, pl.ds(c0, dm)], sem_b.at[part])

    bo_copy = pltpu.make_async_copy(bwo_hbm, bst_ref.at[:, pl.ds(3 * dm, dm)], sem_b.at[3])

    def bst_tile(c):
        return bst_ref[:, pl.ds(pl.multiple_of(c * 128, 128), 128)]

    def bias_tables(full):
        RA = R if full else M2 + seg
        CW = 128
        ri = lax.broadcasted_iota(jnp.int32, (RA, CW), 0)
        ci = lax.broadcasted_iota(jnp.int32, (RA, CW), 1)
        if not full:
            ri = jnp.where(ri >= M2, ri + seg, ri)

        def table(i, bounds, vals):
            out = vals[-1]
            for b, v in zip(reversed(bounds), reversed(vals[:-1])):
                out = jnp.where(i < b, v, out)
            return out
        qi = ri - table(ri, [16, 48, 56], [0, 8, 48, 40])
        g0 = (ci < 8) | ((ci >= 16) & (ci < 48))
        k2 = ci - table(ci, [8, 24, 32, 48, 56, 80, 88, 96, 104], [-8, 0, 24, 8, 48, 40, 72, 80, 96, 104])
        if full:
            k1 = ci - table(ci, [8, 48], [0, 8, 40])
            row_l2 = ((ri >= 8) & (ri < 16)) | (ri >= 48)
            row_xa = (ri >= 8) & (ri < 16)
            valid = (row_xa == (ci >= 80)) & (ci < 112)
            is_a = jnp.where(ci >= 80, ((ci >= 88) & (ci < 104)).astype(jnp.int32),
                             (g0 != row_l2).astype(jnp.int32)) > 0
            ki = jnp.where(row_l2, k2, k1)
            visible = valid & ((qi < n_mem) | (qi >= ki))
            fill = jnp.where(valid, NEG2, -jnp.inf)
        else:
            is_a = jnp.logical_not(g0)
            visible = (qi < n_mem) | (qi >= k2)
            fill = NEG2
        for e, mine in enumerate((is_a, jnp.logical_not(is_a))):
            bias_ref[(0 if full else 2) + e, 0:RA, :] = jnp.where(
                mine, jnp.where(visible, 0.0, fill), -jnp.inf)

    for i in range(HC):
        x_copy(i).start()

    def zero_body(j, c):
        btmp_ref[j, 0:dm, :] = jnp.zeros((dm, 128), F32)
        return c
    lax.fori_loop(0, nct, zero_body, 0)

    w0_copy(0).start()
    xb_ref[0:2 * seg, :] = jnp.zeros((2 * seg, dm), F32)
    kb_ref[...] = jnp.zeros(kb_ref.shape, F32)
    vb_ref[...] = jnp.zeros(vb_ref.shape, F32)
    bst_ref[:, 4 * dm:] = jnp.zeros((dm, 128), BF16)
    bias_tables(True)
    bias_tables(False)

    def ekey(key):
        return ("a", key[1]) if key[0] == "a" else ("l", key[1], 0, key[3])
    EKEYS = []
    for key in KEYS:
        if key[0] in ("a", "l1") and ekey(key) not in EKEYS:
            EKEYS.append(ekey(key))

    def e_ops():
        ye = _ln(x_ref[R0 + NPRE - 16:R0 + NPRE, :].astype(F32))
        eops = _Operands(None, None, [ye[:, k * 128:(k + 1) * 128] for k in range(nct)])
        for j, key in enumerate(EKEYS):
            xe_ref[j] = _pk(eops(key))

    NKR = len(KEYS_R)

    def xl(j, hf, i):
        if j >= NKR:
            ref, j, i = xlc_ref, j - NKR, hf * HC + i
        else:
            ref = (xla_ref, xlb_ref)[hf]
        r0 = i * (XH // 2)
        return ref.at[j, pl.ds(r0 if isinstance(r0, int) else pl.multiple_of(r0, 8), XH // 2)]

    def ln_ops(hf, i, lo, hi):
        y = _ln(x_ref[pl.ds(pl.multiple_of(R0 + (hf * HC + i) * XC, 16), XC), :].astype(F32))
        ops = _Operands([y[0:XH, k * 128:(k + 1) * 128] for k in range(nct)],
                        [y[XH:XC, k * 128:(k + 1) * 128] for k in range(nct)], None)
        vals = []
        for j in range(lo, hi):
            v = _pk(ops(KEYS[j]))
            xl(j, hf, i)[...] = v
            vals.append([v[e:e + 8] for e in range(0, XH // 2, 8)])
        return vals

    def ln_body(i, c):
        x_copy(i).wait()

        @pl.when(i == 0)
        def _():
            x_copy(HC).start()

        @pl.when(i == 1)
        def _():
            w0_copy(1).start()
            w0_copy(2).start()

        @pl.when(i == 2)
        def _():
            x_copy(HC + 1).start()
            x_copy(HC + 2).start()
            for cp in small:
                cp.start()
        ln_ops(0, i, 0, len(KEYS_R))
        return c
    lax.fori_loop(0, HC, ln_body, 0)

    def prep(scheme, w, dst):
        raw = lambda k, n: w[n * 128:(n + 1) * 128, k * 128:(k + 1) * 128]
        tb = []
        for i, tl in enumerate(scheme[0]):
            tb.append(raw(*tl[0]) if len(tl) == 1
                      else _combo(tl, lambda k, n: raw(k, n).astype(F32)).astype(BF16))
            dst[i * 64:(i + 1) * 64, :] = _pk(tb[i].T)
        return tb

    pcnt, pdl = [0], []

    def pre_chunk(scheme, w, dst, n0, chunks, never=None, tb=None):
        tiles, prog = scheme
        prog = _spread(prog)
        dot = lambda a, i: _nn(a, _upk(dst[i * 64:(i + 1) * 64, :]))
        if w is not None:
            if tb is None:
                tb = prep(scheme, w, dst)
            dot = lambda a, i: _nt(a, tb[i])

        for cs in chunks:
            def op(key):
                def ld(kk):
                    v = [xl(KEYS.index(kk), c // HC, c % HC)[...] for c in cs]
                    if NXC - 1 in cs and kk[0] in ("a", "l1", "l2"):
                        v.append(xe_ref[EKEYS.index(ekey(kk))])
                    return _cat(v)
                if key[0] == "s":
                    return _upk(_cat([ld(("a",) + key[1:]), ld(("b", key[1]))]))
                v = ld(key)
                pcnt[0] += len(cs)
                if pdl and pcnt[0] >= pdl[0][0]:
                    deps = pdl.pop(0)[1]
                    v = _cat([jnp.where(never, d, v[8 * e:8 * e + 8]) for e, d in enumerate(deps)]
                             + ([v[8 * len(deps):]] if v.shape[0] > 8 * len(deps) else []))
                return _upk(v)
            p, q = {}, {}
            m = XH * len(cs)
            _fast_mm(prog, op, dot, m, p, q)
            for n in range(len(p)):
                y, z, e = _fast_out(p, q, n, m)
                for ic, c in enumerate(cs):
                    ring_ref[n0 + n, c * XH:c * XH + XH // 2, :] = _pk(y[ic * XH:(ic + 1) * XH].astype(BF16))
                    ring_ref[n0 + n, c * XH + XH // 2:(c + 1) * XH, :] = _pk(z[ic * XH:(ic + 1) * XH].astype(BF16))
                if e is not None:
                    ring_ref[n0 + n, NXC * XH:NXC * XH + 8, :] = _pk(e.astype(BF16))

    def init_rows():
        x0 = x_ref[0:seg, :].astype(F32)
        sl = _ln(x0)
        xt = _ln(x_ref[R0 + NPRE:XF, :].astype(F32))
        h_ref[0:n_mem, :] = xt[0:n_mem]
        h_ref[n_mem:M2, :] = sl[0:n_mem]
        h_ref[M2:M2 + n_mem, :] = mem0_ref[...].astype(F32)
        h_ref[M2 + n_mem:RB, :] = sl[n_mem:seg]
        h_ref[RB:RB + AH, :] = xt[M2:M2 + AH]
        h_ref[RB + AH:RB + AH + n_mem, :] = xt[n_mem:M2]
        x2_ref[...] = x0

    def first_a(p, c):
        buf = stage_ref.at[0, p, pl.ds(0, RT * 128)]
        pltpu.make_async_copy(buf, buf, sem_m.at[4 + p]).wait()
        x_copy(HC + p).wait()

        @pl.when(p == 0)
        def _():
            for pp in range(4):
                w_copy(pp, 1).start()

        @pl.when(p == 2)
        def _():
            bq_copy(0).start()
        vals = ln_ops(1, p, 0, len(KEYS))
        pcnt[0] = 0
        pdl.extend((DUE_X + e, d) for e, d in enumerate(vals))
        pre_chunk(S53, buf, wr_ref.at[p], p * NT, [[c] for c in range(HC)], p > 9)
        del pdl[:]
        return c
    lax.fori_loop(0, 3, first_a, 0)
    for cp in small:
        cp.wait()

    def first_b(p, c):
        e_ops()
        init_rows()
        vals = ln_ops(0, p, len(KEYS_R), len(KEYS))
        pcnt[0] = 0
        pdl.extend((DUE_X + 2 * e, d) for e, d in enumerate(vals))
        pre_chunk(S53, None, wr_ref.at[p], p * NT, [[c] for c in range(HC, NXC)], p > 9)
        del pdl[:]
        return c
    lax.fori_loop(0, 3, first_b, 0)

    dpt = 128 // B_HEADS

    def b_stage1(u):
        uc = jnp.clip(u, 0, NB1 - 1)
        tr = bst_tile(jnp.where(u >= 0, uc, NB1 + nct)).astype(F32).T
        r0 = pl.multiple_of(uc * 128, 128)
        for j in range(nct):
            btmp_ref[j, pl.ds(r0, 128), :] = tr[:, j * 128:(j + 1) * 128]
        return [pltpu.bitcast(tr[120:128, j * 128:(j + 1) * 128], U32) for j in range(nct)]

    def b_stage1_wo(u):
        uc = jnp.clip(u, 0, nct - 1)
        btmp_ref[uc, WO0:WO0 + dm, :] = bst_tile(jnp.where(u >= 0, NB1 + uc, NB1 + nct)).astype(F32)

    def b_stage2(u):
        uc = jnp.clip(u, 0, NB1 - 1)
        part = (uc >= nct).astype(jnp.int32) + (uc >= 2 * nct).astype(jnp.int32)
        r0 = part * dm + (uc - part * nct) * dpt
        rows = _cat([_cat([btmp_ref[j, pl.ds(r0 + dd, B_HEADS, stride=bdh), :]
                           for j in range(nct)], axis=1) for dd in range(dpt)])
        val = _pk(rows.T.astype(BF16))
        bw_ref[uc] = val
        return [val[64 * j + 56:64 * j + 64] for j in range(nct)]

    def b_stage2_wo(u):
        uc = jnp.clip(u, 0, nct - 1)
        r0 = jnp.where(u >= 0, WO0, 0)
        bw_ref[NB1 + uc] = _pk(
            _cat([btmp_ref[uc, pl.ds(r0 + d, B_HEADS, stride=bdh), :] for d in range(bdh)]).astype(BF16))

    def wo_store(scheme, w, dst, never=None):
        if scheme is S55:
            rawt = lambda k, n: w[k * 128:(k + 1) * 128, n * 128:(n + 1) * 128]
            plain = [i for i, tl in enumerate(scheme[0]) if len(tl) == 1]
            for i, tl in enumerate(scheme[0]):
                if len(tl) > 1:
                    val = _combo(tl, lambda k, n: rawt(k, n).astype(F32)).astype(BF16)
                    val = _pk(_upk(_pk(val.T)).T)
                    dst[i * 64:(i + 1) * 64, :] = val
                    j = plain.pop()
                    pv_ = _pk(rawt(*scheme[0][j][0]))
                    dst[j * 64:(j + 1) * 64, :] = jnp.where(never, val, pv_)
            return
        for r in range(0, 128, 16):
            memo = {}

            def raw(k, n):
                return w[k * 128 + r:k * 128 + r + 16, n * 128:(n + 1) * 128]

            def block(k, n):
                if (k, n) not in memo:
                    memo[k, n] = raw(k, n).astype(F32)
                return memo[k, n]
            for i, tl in enumerate(scheme[0]):
                val = raw(*tl[0]) if len(tl) == 1 else _combo(tl, block).astype(BF16)
                dst[i * 64 + r // 2:i * 64 + r // 2 + 8, :] = _pk(val)

    def pre_body(g, c):
        slot = g & (NSLOT - 1)
        buf = stage_ref.at[slot]
        pltpu.make_async_copy(buf, buf, sem_w.at[slot]).wait()

        @pl.when((g >= 2) & (g <= 4))
        def _():
            bq_copy(g - 2).wait()

        @pl.when(g == 4)
        def _():
            bo_copy.wait()

        @pl.when(g <= 2)
        def _():
            bq_copy(g).start()

        @pl.when(g == 2)
        def _():
            bo_copy.start()

        @pl.when(g + 1 <= NG)
        def _():
            for p in range(4):
                w_copy(p, g + 1).start()

        @pl.when(g == NG - 1)
        def _():
            w0_copy(3).start()
            x_late.start()

        wo_store(S55, stage_ref.at[slot, 3], w_ref.at[3 * NG + g - 1], g > NG + 5)
        deps = [b_stage2(3 * (g - 5) + e) for e in range(3)]
        b_stage2_wo(g - 5)
        deps += [b_stage1(3 * (g - 2) + e) for e in range(3)]
        b_stage1_wo(g - 4)
        pcnt[0] = 0
        pdl.extend((DUE_B0 + DUE_B * e, d) for e, d in enumerate(deps))
        tbs = [prep(S55, stage_ref.at[slot, 0], w_ref.at[g - 1])]
        for p in range(3):
            if p < 2:
                tbs.append(prep(S55, stage_ref.at[slot, p + 1], w_ref.at[(p + 1) * NG + g - 1]))
            pre_chunk(S55, stage_ref.at[slot, p], w_ref.at[p * NG + g - 1], p * NT + RT + (g - 1) * GT, [[0, 1, 2], [3], [4], [5]],
                      g > NG + 5, tbs[p])
        return c
    lax.fori_loop(1, NG + 1, pre_body, 0)
    w0_copy(3).wait()
    wo_store(S35, stage0_ref, wr_ref.at[3])

    for r in range(0, 64, 8):
        def raw(k, n):
            return bw_ref[2 * nct + n, k * 64 + r:k * 64 + r + 8, :]
        blocks = {(k, n): _upk(raw(k, n)).astype(F32) for k in range(nct) for n in range(nct)}
        for i, tl in enumerate(S55[0]):
            val = raw(*tl[0]) if len(tl) == 1 else _pk(_combo(tl, lambda k, n: blocks[k, n]).astype(BF16))
            bwf_ref[i * 64 + r:i * 64 + r + 8, :] = val

    bscale = float(bdh) ** (-0.5) * LOG2E

    def b_proj(lhs, part):
        if part == 2 and lhs.shape[0] == 2 * seg:
            kt = lambda a: [a[:, k * 128:(k + 1) * 128] for k in range(nct)]
            ops = _Operands(kt(lhs[0:seg]), kt(lhs[seg:2 * seg]), None)
            p, q = {}, {}
            _fast_mm(S55[1], ops, lambda a, i: _nn(a, _upk(bwf_ref[i * 64:(i + 1) * 64, :])), seg, p, q)
            return _cat([_cat(_fast_out(p, q, n, seg)[0:2]) for n in range(nct)], axis=1)
        return _nn(lhs.astype(BF16), _cat([_upk(bw_ref[part * nct + j]) for j in range(nct)], axis=1))

    def b_attn(jobs, q, k, v):
        row = lax.broadcasted_iota(jnp.int32, (seg, 128), 0)
        outs = []
        for i, (l, sidx) in enumerate(jobs):
            r0 = i * seg
            pos = row + sidx * seg
            for j in range(nct):
                kb_ref[l, j, 0:HIST, :] = kb_ref[l, j, seg:seg + HIST, :]
                vb_ref[l, j, 0:HIST, :] = vb_ref[l, j, seg:seg + HIST, :]
            for j in range(nct):
                kb_ref[l, j, HIST:HIST + seg, :] = k[r0:r0 + seg, j * 128:(j + 1) * 128]
                vb_ref[l, j, HIST:HIST + seg, :] = v[r0:r0 + seg, j * 128:(j + 1) * 128]
            logits = []
            for w in range(B_WIN):
                o = HIST - w * B_DIL
                acc = None
                for j in range(nct):
                    p = q[r0:r0 + seg, j * 128:(j + 1) * 128] * kb_ref[l, j, o:o + seg, :]
                    acc = p if acc is None else acc + p
                acc = acc + pltpu.roll(acc, 64, 1)
                acc = acc + pltpu.roll(acc, 32, 1)
                lg = acc * bscale
                if w > 0:
                    lg = jnp.where(pos >= w * B_DIL, lg, NEG2)
                logits.append(lg)
            m = logits[0]
            for w in range(1, B_WIN):
                m = jnp.maximum(m, logits[w])
            es = [jnp.exp2(lg - m) for lg in logits]
            den = es[0]
            for w in range(1, B_WIN):
                den = den + es[w]
            inv = _recip(den)
            cols = []
            for j in range(nct):
                acc = None
                for w in range(B_WIN):
                    o = HIST - w * B_DIL
                    p = es[w] * vb_ref[l, j, o:o + seg, :]
                    acc = p if acc is None else acc + p
                cols.append(acc * inv)
            outs.append(_cat(cols, axis=1).astype(BF16))
        return outs

    def b_out(ob, res):
        return res + b_proj(ob, 3)

    def o_store(b, val):
        ro = pl.multiple_of((b + 1) * seg, seg)
        o_ref[pl.ds(ro, val.shape[0]), :] = val.astype(o_ref.dtype)

    def out_copy(b):
        ro = pl.multiple_of(b * seg, seg)
        return pltpu.make_async_copy(o_ref.at[pl.ds(ro + seg, seg), :], out_hbm.at[pl.ds(ro, seg), :], sem_o)

    def step(t, hc, full):
        t_last = n_seg + LAG - 1
        if full:
            jobs = [(0, t - 1), (1, t - 1 - LAG)]

            def b_in():
                return xb_ref[0:2 * seg, :]
        else:
            lb = (t == t_last).astype(jnp.int32)
            jobs = [(lb, t - 1 - lb * (LAG + 1))]

            def b_in():
                return xb_ref[pl.ds(pl.multiple_of(lb * seg, seg), seg), :]
        v0r = _cat([hc[0:n_mem], h_ref[n_mem:M2, :]])
        v1r = _cat([hc[n_mem:M2], h_ref[M2 + n_mem:2 * M2, :]])

        hist = []
        never = t > 4 * n_seg

        def gate(back, z):
            gv = hist[-back]
            return _cat([jnp.where(never, gv, z[e:e + 8]) for e in range(0, z.shape[0], 8)])

        def ktiles(z):
            return [z[:, k * 128:(k + 1) * 128] for k in range(z.shape[1] // 128)]
        if full:
            hl = _Operands(ktiles(_cat([v0r, h_ref[2 * M2:RB, :]])), ktiles(_cat([v1r, h_ref[RB:RB + AH, :]])), None)
        else:
            hl = _Operands(None, None, ktiles(_cat([v0r, v1r, h_ref[2 * M2:RB, :]])))
        mh = 2 * M2 if full else 0

        def tile_dot(p, r):
            src = wr_ref.at[p] if r == 0 else w_ref.at[p * NG + r - 1]

            def dot(a, i):
                wt = src[i * 64:(i + 1) * 64, :]
                cnt[0] += 1
                if dl and cnt[0] >= dl[0][0]:
                    deps = dl.pop(0)[1]
                    wt = _cat([jnp.where(never, pltpu.bitcast(d, U32), wt[8 * e:8 * e + 8])
                               for e, d in enumerate(deps)] + [wt[8 * len(deps):]])
                res_ = _nn(a, _upk(wt))
                hist.append(res_[0:8])
                return res_
            return dot
        cnt, dl = [0], []
        scale = float(dh) ** (-0.5) * LOG2E
        if full:
            s_ = t - LAG
            rd = pl.multiple_of(lax.rem(s_ * (seg // 2), RS // 2), seg // 2)
            wa = pl.multiple_of(lax.rem((A0 - R0 + s_ * AH) // 2, RS // 2), 8)
        else:
            wx = pl.multiple_of(jnp.where(t < LAG, NPRE // 2 + t * (n_mem // 2), RS // 2), n_mem // 2)

        RA = R if full else M2 + seg
        CW = R + 2 * M2 if full else R
        bidx = 0 if full else 2
        half = dh - 128
        la8 = lax.broadcasted_iota(jnp.int32, (n_mem, 128), 1) < half
        ones = jnp.full((n_mem, 128), 0xFFFFFFFF, U32)
        zero = jnp.zeros((n_mem, 128), U32)
        mask_a = jnp.where(la8, ones, zero)
        mask_b = jnp.where(la8, zero, ones)

        def pk2(a, b):
            return _pk(_cat([a, b]).astype(BF16))

        yt = [[None] * NT for _ in range(3)]

        def proj(p, r):
            pa, qa = {}, {}
            _fast_mm((S53 if r == 0 else S55)[1], hl, tile_dot(p, r), mh, pa, qa)
            n0 = 0 if r == 0 else RT + (r - 1) * GT
            for n in range(len(pa)):
                y, z, e = _fast_out(pa, qa, n, mh)
                idx = p * NT + n0 + n
                if full:
                    ring_ref[idx, pl.ds(wa, 8), :] = pk2(z[16:24], z[24:32])
                    y = _cat([y[0:M2], z[0:M2], y[M2:2 * M2]])
                else:
                    y = e
                    ring_ref[idx, pl.ds(wx, n_mem // 2), :] = pk2(y[0:8], y[8:16])[0:n_mem // 2]
                yt[p][n0 + n] = stash(p * 16 + (n0 + n) % 16, packed(p, (n0 + n) % 3, y))

        def ab(z8):
            return jnp.where(la8, z8, 0.0), jnp.where(la8, 0.0, z8)

        def packed(p, j, y):
            u2 = pk2(y[32:40], y[40:48])
            if p == 0 or j == 0:
                return [pk2(y[0:8], y[8:16]), pk2(y[16:24], y[24:32]), u2]
            if j == 2:
                return [pk2(y[8:16], y[0:8]), pk2(y[24:32], y[16:24]), u2]
            xa_a, xa_b = ab(y[8:16])
            out = [pk2(xa_b, xa_a), pk2(y[24:32], y[16:24]) & mask_b, pk2(y[16:24], y[24:32]) & mask_a, u2]
            if full:
                out += [pk2(*ab(y[0:8])), pk2(*ab(y[16:24]))]
            return out

        def stash(idx, parts):
            kv_ref[idx, 0:8 * len(parts), :] = _cat(parts)
            return lambda: [kv_ref[idx, 8 * e:8 * e + 8, :] for e in range(len(parts))]

        def pair(p, g):
            xs = [ring_ref[p * NT + 3 * g + j, pl.ds(rd, seg // 2), :] for j in range(3)] if full else None
            return [f() for f in yt[p][3 * g:3 * g + 3]], xs

        def q_rows(z, j):
            v0, v1, v2 = z[0][j]
            return [v0] + ([z[1][j]] if full else []) + [v1, v2]

        def kv_tiles(z):
            yt, x1 = z
            v0, v1, v2 = yt[0]
            t0 = [v0] + ([x1[0]] if full else [v1, v2]) + [v1, v2]
            w0, w1, w2 = yt[2]
            t2 = [w0, w1, w2] + ([x1[2]] if full else [w1, w2])
            if full:
                t0 += [v0, v1]
                t2 += [w0, w1]
            e1, mb, ma, u2 = yt[1][0:4]
            mid2 = [e1, mb, u2 & mask_b, ma, u2 & mask_a]
            mid1 = None
            if full:
                lo, hi = x1[1][0:8], x1[1][8:16]
                mid1 = [yt[1][4], lo & mask_a, hi & mask_a, lo & mask_b, hi & mask_b, e1, yt[1][5]]
            return t0, mid1, mid2, t2

        def mat(parts):
            return _upk(_cat(parts))

        def scores(q, k):
            k0, km1, km2, k2_ = kv_tiles(k)
            s_a = _nt(mat(q_rows(q, 0)), mat(k0))
            s_b = _nt(mat(q_rows(q, 2)), mat(k2_))
            qm = q_rows(q, 1)
            if full:
                s_m = _cat([_nt(mat(qm[0:2]), mat(km1)), _cat([_nt(mat(qm[2:4]), mat(km2)), jnp.zeros((seg, CW - R), F32)], axis=1)])
            else:
                s_m = _nt(mat(qm), mat(km2))
            out = []
            for e, sx in enumerate((s_a, s_b)):
                s = (sx + s_m) * scale + bias_ref[bidx + e, 0:RA, 0:CW]
                ex = jnp.exp2(s - jnp.max(s, axis=-1, keepdims=True))
                out.append(ex * _recip(jnp.sum(ex, axis=-1, keepdims=True)))
            return out

        def pv(p, v):
            v0, vm1, vm2, v2 = kv_tiles(v)
            o_a = _nn(p[0].astype(BF16), mat(v0))
            o_b = _nn(p[1].astype(BF16), mat(v2))
            p = p[0] + p[1]
            if full:
                o_m = _cat([_nn(p[0:M2 + seg].astype(BF16), mat(vm1)),
                            _nn(p[M2 + seg:R, 0:R].astype(BF16), mat(vm2))])
            else:
                o_m = _nn(p.astype(BF16), mat(vm2))
            return [o_a, o_m, o_b]

        ot = []
        pacc, qacc = {}, {}

        def add_o(r):
            n0 = 0 if r == 0 else RT + (r - 1) * GT
            oo = ot[n0:n0 + (RT if r == 0 else GT)]
            if full:
                us = [_cat([o[48:64], o[32:48]]) for o in oo]
                if r < TAILPV:
                    us = [gate(GATE_O, z) for z in us]
                ops = _Operands([o[0:32] for o in oo], us, [o[64:80] for o in oo])
            else:
                ops = _Operands(None, None, oo)
            _fast_mm((S35 if r == 0 else S55)[1], ops, tile_dot(3, r), mh, pacc, qacc)

        bqkv = [None] * 3
        probs = []

        def do_pv():
            for g in range(len(ot) // 3, len(probs)):
                ot.extend(pv(probs[g], pair(2, g)))

        if full:
            an = pl.multiple_of(jnp.minimum(A0 + (s_ + 1) * AH, S - AH), AH)
            h_ref[RB:RB + AH, :] = _ln(x_ref[pl.ds(an, AH), :].astype(F32))

        for r in range(NG + 1):
            proj(2, r)
            proj(1, r)
            proj(0, r)
            if r == 0:
                blhs = _ln(b_in())
            if r < 3:
                bqkv[2 - r] = b_proj(blhs, 2 - r)
            if r == 3:
                ob = b_attn(jobs, *bqkv)
            if r == BOUT_R:
                zb = b_out(_cat(ob), b_in())
                x2_new = zb[0:seg]
                if full:
                    o_store(t - 1 - LAG, zb[seg:2 * seg])
                    nxt = x2_new
                else:
                    o_store(lb * (t_last - LAG - 1) - 1, x2_new)
                    nxt = jnp.where(t < LAG - 1, x_ref[seg:2 * seg, :].astype(F32), x2_new)
                sl = _ln(nxt)
                h_ref[n_mem:M2, :] = sl[0:n_mem]
                h_ref[M2 + n_mem:RB, :] = sl[n_mem:seg]
                if full:
                    for j in range(nct):
                        dl.append((cnt[0] + DUE_LN + 2 * j, [sl[e:e + 8, j * 128:(j + 1) * 128] for e in range(0, seg, 8)]))
            if r in WSCHED:
                add_o(WSCHED[r])
            do_pv()
            for g in range(len(probs), (RT + r * GT) // 3):
                probs.append(scores(pair(0, g), pair(1, g)))
        for r in range(len(WSCHED), TAILPV):
            add_o(r)
        do_pv()
        for r in range(TAILPV, NG + 1):
            add_o(r)
        cols = []
        for n in range(nct):
            y, z, e = _fast_out(pacc, qacc, n, mh)
            cols.append(_cat([y, z[16:32], z[0:16], e]) if full else e)
        acc = _cat(cols, axis=1)

        y2 = x2_ref[...] + _cat([acc[n_mem:M2], acc[RA - seg + n_mem:RA]])
        mem2 = acc[RA - seg:RA - seg + n_mem]
        if full:
            x_cur = x_ref[pl.ds(pl.multiple_of(t * seg, seg), seg), :].astype(F32)
            xb_ref[0:seg, :] = x_cur + acc[M2:M2 + seg]
            xb_ref[seg:2 * seg, :] = y2
            m1n = acc[0:n_mem]
            m2n = mem2
        else:
            xb_ref[pl.ds(pl.multiple_of(jnp.where(t < LAG, 0, (t - n_seg + 2) * seg), seg), seg), :] = y2
            m1n = jnp.where(t < LAG - 1, h_ref[RB + AH:RB + AH + n_mem, :], mem2)
            m2n = jnp.where(t == LAG - 1, mem0_ref[...].astype(F32), mem2)
        x2_ref[...] = nxt
        return _cat([m1n, m2n])

    def single_body(t, c):
        @pl.when(t == n_seg)
        def _():
            out_copy(t - (LAG + 2)).start()
        return step(t, c, False)

    def full_body(t, c):
        @pl.when(t >= LAG + 2)
        def _():
            out_copy(t - (LAG + 2)).start()
        return step(t, c, True)

    def phase(ph, c):
        t0 = ph * n_seg
        c = lax.fori_loop(t0, t0 + LAG, single_body, c)

        @pl.when(ph == 0)
        def _():
            x_late.wait()
        return lax.fori_loop(LAG, jnp.where(ph == 0, n_seg, LAG), full_body, c)
    lax.fori_loop(0, 2, phase, _cat([h_ref[0:n_mem, :], h_ref[M2:M2 + n_mem, :]]))

    out_copy(n_seg - 3).start()
    res = xb_ref[2 * seg:4 * seg, :]
    blhs = _ln(res)
    ob = b_attn([(1, n_seg - 2), (1, n_seg - 1)], *[b_proj(blhs, part) for part in range(3)])
    o_store(n_seg - 2, b_out(_cat(ob), res))
    out_copy(n_seg - 2).start()
    out_copy(n_seg - 1).start()
    pltpu.make_async_copy(o_ref.at[pl.ds(seg, S), :], out_hbm, sem_o).wait()


@functools.partial(jax.jit, static_argnames=("seg",))
def _run(A_x, A_mem0, A_Wq, A_Wk, A_Wv, A_Wo, B_wqkv, B_wo, *, seg):
    _, S, dm = A_x.shape
    n_heads, dh = A_Wq.shape[1], A_Wq.shape[2]
    n_mem = A_mem0.shape[1]
    n_seg = S // seg
    hd = n_heads * dh
    nct = dm // 128
    ng = (hd // 128 - RT) // GT
    assert (seg, n_seg, n_mem, dh, dm % 128, n_heads, LAG) == (32, 64, 8, 192, 0, 32, 2)

    x = A_x.reshape(S, dm)
    mem0 = A_mem0.reshape(n_mem, dm)
    wq = jnp.transpose(A_Wq, (1, 2, 0)).reshape(hd, dm)
    wk = jnp.transpose(A_Wk, (1, 2, 0)).reshape(hd, dm)
    wv = jnp.transpose(A_Wv, (1, 2, 0)).reshape(hd, dm)
    wo = A_Wo.reshape(hd, dm)
    _, _, _, _, rs, xc = _plan(seg, n_seg)

    kern = functools.partial(_kernel, seg=seg, n_seg=n_seg, n_mem=n_mem,
                             n_heads=n_heads, dh=dh, dm=dm)
    hbm = pl.BlockSpec(memory_space=pltpu.HBM)

    out = pl.pallas_call(
        kern,
        in_specs=[hbm] * 8,
        out_specs=hbm,
        out_shape=jax.ShapeDtypeStruct((S, dm), A_x.dtype),
        scratch_shapes=[
            pltpu.VMEM((S, dm), BF16),
            pltpu.VMEM((n_mem, dm), BF16),
            pltpu.VMEM((NSLOT, 4, GT * 128, dm), BF16),
            pltpu.VMEM((RT * 128, dm), BF16),
            pltpu.VMEM((4, len(S53[0]) * 64, 128), U32),
            pltpu.VMEM((4 * ng, len(S55[0]) * 64, 128), U32),
            pltpu.VMEM((dm, 4 * dm + 128), BF16),
            pltpu.VMEM((nct, 4 * dm + 32, 128), F32),
            pltpu.VMEM((4 * nct, dm // 2, 128), U32),
            pltpu.VMEM((len(KEYS_R), HC * xc // 4, 128), U32),
            pltpu.VMEM((len(KEYS_R), HC * xc // 4, 128), U32),
            pltpu.VMEM((len(KEYS) - len(KEYS_R), NXC * xc // 4, 128), U32),
            pltpu.VMEM((15, 8, 128), U32),
            pltpu.VMEM((3 * hd // 128, rs // 2 + 8, 128), U32),
            pltpu.VMEM((3 * n_mem + seg + AH, dm), F32),
            pltpu.VMEM((4 * seg, dm), F32),
            pltpu.VMEM((seg, dm), F32),
            pltpu.VMEM((2, nct, HIST + seg, 128), F32),
            pltpu.VMEM((2, nct, HIST + seg, 128), F32),
            pltpu.VMEM((S + seg, dm), A_x.dtype),
            pltpu.VMEM((4, 2 * n_mem + 2 * seg, 128), F32),
            pltpu.VMEM((48, 48, 128), U32),
            pltpu.VMEM((len(S55[0]) * 64, 128), U32),
            pltpu.SemaphoreType.DMA((NSLOT,)),
            pltpu.SemaphoreType.DMA((8 + NXC,)),
            pltpu.SemaphoreType.DMA((4,)),
            pltpu.SemaphoreType.DMA(()),
        ],
        compiler_params=pltpu.CompilerParams(
            vmem_limit_bytes=127 * 1024 * 1024,
            disable_bounds_checks=True,
        ),
    )(x, mem0, wq, wk, wv, wo, B_wqkv, B_wo)
    return out.reshape(1, S, dm)


def pallas_interleave_layers__memory_aug_recurrent_mem_tr__sliding_local_dilated__prompt_kernel(
    A_x: jax.Array,
    A_mem0: jax.Array,
    A_Wq: jax.Array,
    A_Wk: jax.Array,
    A_Wv: jax.Array,
    A_Wo: jax.Array,
    A_seg_len,
    B_x: jax.Array,
    B_wqkv: jax.Array,
    B_wo: jax.Array,
):
    del B_x
    seg = A_seg_len if isinstance(A_seg_len, int) else 32
    return _run(A_x, A_mem0, A_Wq, A_Wk, A_Wv, A_Wo, B_wqkv, B_wo, seg=seg)
```

```python
import functools

import jax
import jax.numpy as jnp
from jax import lax
import jax.experimental.pallas as pl
import jax.experimental.pallas.tpu as pltpu

F32 = jnp.float32
BF16 = jnp.bfloat16
U32 = jnp.uint32
NEG = -1000000000.0
LN_EPS = 1e-05
LOG2E = 1.4426950408889634
NEG2 = NEG * LOG2E

B_HEADS = 32
B_WIN = 8
B_DIL = 2
HIST = 16
WF = int(1)
PF = int(0)
BLF = int(0)
AH = 16
LAG = 2
NSLOT = 2
NXC = 6
HC = 3
WSCHED = {3: 0, 4: 1, 6: 2, 7: 3, 8: 4, 9: 5}
BOUT_R = 5
TAILPV = int(8)
GATE_O = int(50)
DUE_LN = 150
DUE_X = 24
DUE_B0, DUE_B = 100, 60


def _ln(x):
    m = jnp.mean(x, axis=-1, keepdims=True)
    c = x - m
    v = jnp.mean(c * c, axis=-1, keepdims=True)
    return c * lax.rsqrt(v + LN_EPS)


def _recip(d):
    return pl.reciprocal(d, approx=True)


def _nt(a, b):
    return lax.dot_general(a, b, (((1,), (1,)), ((), ())), preferred_element_type=F32)


def _nn(a, b):
    return lax.dot_general(a, b, (((1,), (0,)), ((), ())), preferred_element_type=F32)


def _cat(xs, axis=0):
    return xs[0] if len(xs) == 1 else jnp.concatenate(xs, axis=axis)


def _pk(z):
    return pltpu.bitcast(z, U32)


def _upk(z):
    return pltpu.bitcast(z, BF16)


LAM = (-1.5, -0.5, 0.0, 0.5, 1.5)


def _scheme(stars):
    tiles, prog = [], []
    for star in stars:
        if len(star) == 1:
            prog.append(("single", star[0], None, len(tiles)))
            tiles.append([star[0][:2]])
            continue
        left = [len(star) - 1] * len(star)
        for j in range(1, len(star)):
            for i in range(j):
                x, y = star[i], star[j]
                prog.append(("pair", x, y, len(tiles)))
                tiles += [[(x[0], y[1])], [(y[0], x[1])], [(x[0], y[1]), (y[0], x[1])]]
                for e in (i, j):
                    left[e] -= 1
                    if left[e] == 0:
                        z = star[e]
                        prog.append(("diag", z, None, len(tiles)))
                        tiles += [[z[:2]] + [(o[0], z[1]) for o in star if o is not z],
                                  [z[:2]] + [(z[0], o[1]) for o in star if o is not z]]
    return tiles, prog


S55 = _scheme([[(i, i, LAM[i]) for i in range(5)]])
S53 = _scheme([[(0, 0, LAM[0]), (2, 1, LAM[2]), (4, 2, LAM[4])], [(1, 0, LAM[1]), (3, 2, LAM[3])],
               [(1, 1, LAM[1])], [(3, 1, LAM[3])]])
S35 = _scheme([[(0, 0, LAM[0]), (1, 2, LAM[2]), (2, 4, LAM[4])], [(0, 1, LAM[1]), (2, 3, LAM[3])],
               [(1, 1, LAM[1])], [(1, 3, LAM[3])]])


def _spread(prog):
    pairs = [e for e in prog if e[0] != "diag"]
    diags = [e for e in prog if e[0] == "diag"]
    out, k = [], 0
    for i, e in enumerate(pairs):
        out.append(e)
        while k < len(diags) and (k + 0.5) * len(pairs) <= (i + 1) * len(diags):
            out.append(diags[k])
            k += 1
    return out + diags[k:]


def _op_keys(prog):
    keys = []
    for kind, x, y, _ in prog:
        if kind == "pair":
            new = [(nm, x[0], x[2], y[0], y[2]) for nm in ("l1", "l2", "A")]
        else:
            new = [("a", x[0], x[2]), ("b", x[0])]
        keys += [k for k in new if k not in keys]
    return keys


def _scaled(c, u):
    return u if c == 1.0 else c * u


class _Operands:
    def __init__(self, T, U, E, dtype=BF16):
        self.T, self.U, self.E, self.memo, self.dtype = T, U, E, {}, dtype

    def _get(self, key, fn):
        if key not in self.memo:
            self.memo[key] = fn()
        return self.memo[key]

    def paired(self, key):
        T, U = self.T, self.U
        if key[0] == "b":
            return U[key[1]]
        if key[0] == "a":
            k, lam = key[1:]
            if lam == 0.0:
                return T[k]
            return self._get(("f",) + key, lambda: T[k] - _scaled(lam, U[k]) if lam > 0
                             else T[k] + _scaled(-lam, U[k]))
        kx, lx, ky, ly = key[1:]
        A = self._get(("f", "A") + key[1:],
                      lambda: self.paired(("a", kx, lx)) + self.paired(("a", ky, ly)))
        if key[0] == "A":
            return A
        return A - _scaled(ly - lx, U[kx]) if key[0] == "l1" else A + _scaled(ly - lx, U[ky])

    def extra(self, key):
        if key[0] == "a":
            return self.E[key[1]]
        return self._get(("e", key[1], key[3]), lambda: self.E[key[1]] + self.E[key[3]])

    def __call__(self, key):
        if self.T is None:
            ek = ("a", key[1]) if key[0] in ("a", "s") else ("l", key[1], 0, key[3])
            return self._get(ek, lambda: self.extra(ek).astype(self.dtype))

        def build():
            ak = ("a",) + key[1:] if key[0] == "s" else key
            parts = [self.paired(ak)]
            if self.E is not None and ak[0] in ("a", "l1", "l2"):
                parts.append(self.extra(ak))
            if key[0] == "s":
                parts.append(self.U[key[1]])
            return _cat(parts).astype(self.dtype)
        return self._get(key, build)


def _fast_mm(prog, op, dot, m, p, q):
    def add(d, key, val):
        d[key] = val if key not in d else d[key] + val

    for kind, x, y, i in prog:
        if kind == "pair":
            kk = (x[0], x[2], y[0], y[2])
            p1, p2 = dot(op(("l1",) + kk), i), dot(op(("l2",) + kk), i + 1)
            if m:
                r = _scaled(1.0 / (y[2] - x[2]), p2[0:m] - p1[0:m] + dot(op(("A",) + kk), i + 2))
                add(q, (x[1], x[2]), r)
                add(q, (y[1], y[2]), r)
            add(p, y[1], p1)
            add(p, x[1], p2)
        elif kind == "diag":
            add(p, x[1], dot(op(("a", x[0], x[2])), i))
            if m:
                add(q, (x[1], x[2]), dot(op(("b", x[0])), i + 1))
        else:
            r = dot(op(("s", x[0], x[2])), i)
            add(p, x[1], r[0:r.shape[0] - m])
            if m:
                add(q, (x[1], x[2]), r[r.shape[0] - m:])


def _fast_out(p, q, n, m):
    if not m:
        return None, None, p[n]
    y, z = p[n][0:m], None
    for (nn, lam), v in q.items():
        if nn == n:
            z = v if z is None else z + v
            if lam != 0.0:
                y = y + _scaled(lam, v) if lam > 0 else y - _scaled(-lam, v)
    return y, z, (p[n][m:] if p[n].shape[0] > m else None)


def _combo(tile, block):
    out = block(*tile[0])
    for kn in tile[1:]:
        out = out - block(*kn)
    return out


GT = 5
RT = 3
KEYS_R = _op_keys(S53[1])
KEYS = KEYS_R + [k for k in _op_keys(S55[1]) if k not in KEYS_R]


def _plan(seg, n_seg):
    S = seg * n_seg
    R0 = LAG * seg
    A0 = S - (n_seg - LAG) * AH
    NPRE = A0 - R0 - LAG * 8
    RS = -(-(A0 - R0 + AH) // seg) * seg
    XC = NPRE // NXC // 32 * 32
    assert XC * NXC + 16 == NPRE
    return S, R0, A0, NPRE, RS, XC


def _kernel(x_hbm, mem0_hbm, wq_hbm, wk_hbm, wv_hbm, wo_hbm, bqkv_hbm, bwo_hbm,
            out_hbm,
            x_ref, mem0_ref, stage_ref, stage0_ref, wr_ref, w_ref, bst_ref, btmp_ref, bw_ref,
            xla_ref, xlb_ref, xlc_ref, xe_ref, ring_ref, h_ref, xb_ref, x2_ref, kb_ref, vb_ref, o_ref, bias_ref, kv_ref, bwf_ref,
            sem_w, sem_m, sem_b, sem_o,
            *, seg, n_seg, n_mem, n_heads, dh, dm):
    S, R0, A0, NPRE, RS, XC = _plan(seg, n_seg)
    M2 = 2 * n_mem
    R = M2 + 2 * seg
    RB = M2 + seg
    nct = dm // 128
    bdh = dm // B_HEADS
    NT = n_heads * dh // 128
    NG = (NT - RT) // GT
    w_hbm = (wq_hbm, wk_hbm, wv_hbm, wo_hbm)

    def w_copy(p, g):
        slot = g & (NSLOT - 1)
        return pltpu.make_async_copy(w_hbm[p].at[pl.ds((RT + (g - 1) * GT) * 128, GT * 128), :],
                                     stage_ref.at[slot, p], sem_w.at[slot])

    def w0_copy(p):
        dst = stage0_ref if p == 3 else stage_ref.at[0, p, pl.ds(0, RT * 128)]
        return pltpu.make_async_copy(w_hbm[p].at[pl.ds(0, RT * 128), :], dst, sem_m.at[4 + p])

    NB1 = 3 * nct
    WO0 = 3 * dm
    XF = A0 + AH
    XH = XC // 2

    def rows_copy(r0, n, sem):
        return pltpu.make_async_copy(x_hbm.at[pl.ds(r0, n), :], x_ref.at[pl.ds(r0, n), :], sem)

    def x_copy(i):
        return rows_copy(pl.multiple_of(R0 + i * XC, 16), XC, sem_m.at[8 + i])

    small = [rows_copy(0, R0, sem_m.at[1]), rows_copy(R0 + NPRE - 16, XF - R0 - NPRE + 16, sem_m.at[2]),
             pltpu.make_async_copy(mem0_hbm, mem0_ref, sem_m.at[3])]
    x_late = rows_copy(XF, S - XF, sem_m.at[0])

    def bq_copy(part):
        c0 = pl.multiple_of(part * dm, 128)
        return pltpu.make_async_copy(bqkv_hbm.at[:, pl.ds(c0, dm)], bst_ref.at[:, pl.ds(c0, dm)], sem_b.at[part])

    bo_copy = pltpu.make_async_copy(bwo_hbm, bst_ref.at[:, pl.ds(3 * dm, dm)], sem_b.at[3])

    def bst_tile(c):
        return bst_ref[:, pl.ds(pl.multiple_of(c * 128, 128), 128)]

    def bias_tables(full):
        RA = R if full else M2 + seg
        CW = 128
        ri = lax.broadcasted_iota(jnp.int32, (RA, CW), 0)
        ci = lax.broadcasted_iota(jnp.int32, (RA, CW), 1)
        if not full:
            ri = jnp.where(ri >= M2, ri + seg, ri)

        def table(i, bounds, vals):
            out = vals[-1]
            for b, v in zip(reversed(bounds), reversed(vals[:-1])):
                out = jnp.where(i < b, v, out)
            return out
        qi = ri - table(ri, [16, 48, 56], [0, 8, 48, 40])
        g0 = (ci < 8) | ((ci >= 16) & (ci < 48))
        k2 = ci - table(ci, [8, 24, 32, 48, 56], [-8, 0, 24, 8, 48, 40])
        if full:
            k1 = ci - table(ci, [8, 48], [0, 8, 40])
            row_l2 = ((ri >= 8) & (ri < 16)) | (ri >= 48)
            is_a = g0 != row_l2
            ki = jnp.where(row_l2, k2, k1)
        else:
            is_a = jnp.logical_not(g0)
            ki = k2
        visible = (qi < n_mem) | (qi >= ki)
        fill = NEG2
        for e, mine in enumerate((is_a, jnp.logical_not(is_a))):
            bias_ref[(0 if full else 2) + e, 0:RA, :] = jnp.where(
                mine, jnp.where(visible, 0.0, fill), -jnp.inf)

    for i in range(HC):
        x_copy(i).start()

    def zero_body(j, c):
        btmp_ref[j, 0:dm, :] = jnp.zeros((dm, 128), F32)
        return c
    lax.fori_loop(0, nct, zero_body, 0)

    w0_copy(0).start()
    xb_ref[0:2 * seg, :] = jnp.zeros((2 * seg, dm), F32)
    kb_ref[...] = jnp.zeros(kb_ref.shape, F32)
    vb_ref[...] = jnp.zeros(vb_ref.shape, F32)
    bst_ref[:, 4 * dm:] = jnp.zeros((dm, 128), BF16)
    bias_tables(True)
    bias_tables(False)

    def ekey(key):
        return ("a", key[1]) if key[0] == "a" else ("l", key[1], 0, key[3])
    EKEYS = []
    for key in KEYS:
        if key[0] in ("a", "l1") and ekey(key) not in EKEYS:
            EKEYS.append(ekey(key))

    def e_ops():
        ye = _ln(x_ref[R0 + NPRE - 16:R0 + NPRE, :].astype(F32))
        eops = _Operands(None, None, [ye[:, k * 128:(k + 1) * 128] for k in range(nct)])
        for j, key in enumerate(EKEYS):
            xe_ref[j] = _pk(eops(key))

    NKR = len(KEYS_R)

    def xl(j, hf, i):
        if j >= NKR:
            ref, j, i = xlc_ref, j - NKR, hf * HC + i
        else:
            ref = (xla_ref, xlb_ref)[hf]
        r0 = i * (XH // 2)
        return ref.at[j, pl.ds(r0 if isinstance(r0, int) else pl.multiple_of(r0, 8), XH // 2)]

    def ln_ops(hf, i, lo, hi):
        y = _ln(x_ref[pl.ds(pl.multiple_of(R0 + (hf * HC + i) * XC, 16), XC), :].astype(F32))
        ops = _Operands([y[0:XH, k * 128:(k + 1) * 128] for k in range(nct)],
                        [y[XH:XC, k * 128:(k + 1) * 128] for k in range(nct)], None)
        vals = []
        for j in range(lo, hi):
            v = _pk(ops(KEYS[j]))
            xl(j, hf, i)[...] = v
            vals.append([v[e:e + 8] for e in range(0, XH // 2, 8)])
        return vals

    def ln_body(i, c):
        x_copy(i).wait()

        @pl.when(i == 0)
        def _():
            x_copy(HC).start()

        @pl.when(i == 1)
        def _():
            w0_copy(1).start()
            w0_copy(2).start()

        @pl.when(i == 2)
        def _():
            x_copy(HC + 1).start()
            x_copy(HC + 2).start()
            for cp in small:
                cp.start()
        ln_ops(0, i, 0, len(KEYS_R))
        return c
    lax.fori_loop(0, HC, ln_body, 0)

    def prep(scheme, w, dst):
        raw = lambda k, n: w[n * 128:(n + 1) * 128, k * 128:(k + 1) * 128]
        tb = []
        for i, tl in enumerate(scheme[0]):
            tb.append(raw(*tl[0]) if len(tl) == 1
                      else _combo(tl, lambda k, n: raw(k, n).astype(F32)).astype(BF16))
            dst[i * 64:(i + 1) * 64, :] = _pk(tb[i].T)
        return tb

    pcnt, pdl = [0], []

    def pre_chunk(scheme, w, dst, n0, chunks, never=None, tb=None):
        tiles, prog = scheme
        prog = _spread(prog)
        dot = lambda a, i: _nn(a, _upk(dst[i * 64:(i + 1) * 64, :]))
        if w is not None:
            if tb is None:
                tb = prep(scheme, w, dst)
            dot = lambda a, i: _nt(a, tb[i])

        for cs in chunks:
            def op(key):
                def ld(kk):
                    v = [xl(KEYS.index(kk), c // HC, c % HC)[...] for c in cs]
                    if NXC - 1 in cs and kk[0] in ("a", "l1", "l2"):
                        v.append(xe_ref[EKEYS.index(ekey(kk))])
                    return _cat(v)
                if key[0] == "s":
                    return _upk(_cat([ld(("a",) + key[1:]), ld(("b", key[1]))]))
                v = ld(key)
                pcnt[0] += len(cs)
                if pdl and pcnt[0] >= pdl[0][0]:
                    deps = pdl.pop(0)[1]
                    v = _cat([jnp.where(never, d, v[8 * e:8 * e + 8]) for e, d in enumerate(deps)]
                             + ([v[8 * len(deps):]] if v.shape[0] > 8 * len(deps) else []))
                return _upk(v)
            p, q = {}, {}
            m = XH * len(cs)
            _fast_mm(prog, op, dot, m, p, q)
            for n in range(len(p)):
                y, z, e = _fast_out(p, q, n, m)
                for ic, c in enumerate(cs):
                    ring_ref[n0 + n, c * XH:c * XH + XH // 2, :] = _pk(y[ic * XH:(ic + 1) * XH].astype(BF16))
                    ring_ref[n0 + n, c * XH + XH // 2:(c + 1) * XH, :] = _pk(z[ic * XH:(ic + 1) * XH].astype(BF16))
                if e is not None:
                    ring_ref[n0 + n, NXC * XH:NXC * XH + 8, :] = _pk(e.astype(BF16))

    def init_rows():
        x0 = x_ref[0:seg, :].astype(F32)
        sl = _ln(x0)
        xt = _ln(x_ref[R0 + NPRE:XF, :].astype(F32))
        h_ref[0:n_mem, :] = xt[0:n_mem]
        h_ref[n_mem:M2, :] = sl[0:n_mem]
        h_ref[M2:M2 + n_mem, :] = mem0_ref[...].astype(F32)
        h_ref[M2 + n_mem:RB, :] = sl[n_mem:seg]
        h_ref[RB:RB + AH, :] = xt[M2:M2 + AH]
        h_ref[RB + AH:RB + AH + n_mem, :] = xt[n_mem:M2]
        x2_ref[...] = x0

    def first_a(p, c):
        buf = stage_ref.at[0, p, pl.ds(0, RT * 128)]
        pltpu.make_async_copy(buf, buf, sem_m.at[4 + p]).wait()
        x_copy(HC + p).wait()

        @pl.when(p == 0)
        def _():
            for pp in range(4):
                w_copy(pp, 1).start()

        @pl.when(p == 2)
        def _():
            bq_copy(0).start()
        vals = ln_ops(1, p, 0, len(KEYS))
        pcnt[0] = 0
        pdl.extend((DUE_X + e, d) for e, d in enumerate(vals))
        pre_chunk(S53, buf, wr_ref.at[p], p * NT, [[c] for c in range(HC)], p > 9)
        del pdl[:]
        return c
    lax.fori_loop(0, 3, first_a, 0)
    for cp in small:
        cp.wait()

    def first_b(p, c):
        e_ops()
        init_rows()
        vals = ln_ops(0, p, len(KEYS_R), len(KEYS))
        pcnt[0] = 0
        pdl.extend((DUE_X + 2 * e, d) for e, d in enumerate(vals))
        pre_chunk(S53, None, wr_ref.at[p], p * NT, [[c] for c in range(HC, NXC)], p > 9)
        del pdl[:]
        return c
    lax.fori_loop(0, 3, first_b, 0)

    dpt = 128 // B_HEADS

    def b_stage1(u):
        uc = jnp.clip(u, 0, NB1 - 1)
        tr = bst_tile(jnp.where(u >= 0, uc, NB1 + nct)).astype(F32).T
        r0 = pl.multiple_of(uc * 128, 128)
        for j in range(nct):
            btmp_ref[j, pl.ds(r0, 128), :] = tr[:, j * 128:(j + 1) * 128]
        return [pltpu.bitcast(tr[120:128, j * 128:(j + 1) * 128], U32) for j in range(nct)]

    def b_stage1_wo(u):
        uc = jnp.clip(u, 0, nct - 1)
        btmp_ref[uc, WO0:WO0 + dm, :] = bst_tile(jnp.where(u >= 0, NB1 + uc, NB1 + nct)).astype(F32)

    def b_stage2(u):
        uc = jnp.clip(u, 0, NB1 - 1)
        part = (uc >= nct).astype(jnp.int32) + (uc >= 2 * nct).astype(jnp.int32)
        r0 = part * dm + (uc - part * nct) * dpt
        rows = _cat([_cat([btmp_ref[j, pl.ds(r0 + dd, B_HEADS, stride=bdh), :]
                           for j in range(nct)], axis=1) for dd in range(dpt)])
        val = _pk(rows.T.astype(BF16))
        bw_ref[uc] = val
        return [val[64 * j + 56:64 * j + 64] for j in range(nct)]

    def b_stage2_wo(u):
        uc = jnp.clip(u, 0, nct - 1)
        r0 = jnp.where(u >= 0, WO0, 0)
        bw_ref[NB1 + uc] = _pk(
            _cat([btmp_ref[uc, pl.ds(r0 + d, B_HEADS, stride=bdh), :] for d in range(bdh)]).astype(BF16))

    def wo_store(scheme, w, dst, never=None):
        if scheme is S55:
            rawt = lambda k, n: w[k * 128:(k + 1) * 128, n * 128:(n + 1) * 128]
            plain = [i for i, tl in enumerate(scheme[0]) if len(tl) == 1]
            for i, tl in enumerate(scheme[0]):
                if len(tl) > 1:
                    val = _combo(tl, lambda k, n: rawt(k, n).astype(F32)).astype(BF16)
                    val = _pk(_upk(_pk(val.T)).T)
                    dst[i * 64:(i + 1) * 64, :] = val
                    j = plain.pop()
                    pv_ = _pk(rawt(*scheme[0][j][0]))
                    dst[j * 64:(j + 1) * 64, :] = jnp.where(never, val, pv_)
            return
        for r in range(0, 128, 16):
            memo = {}

            def raw(k, n):
                return w[k * 128 + r:k * 128 + r + 16, n * 128:(n + 1) * 128]

            def block(k, n):
                if (k, n) not in memo:
                    memo[k, n] = raw(k, n).astype(F32)
                return memo[k, n]
            for i, tl in enumerate(scheme[0]):
                val = raw(*tl[0]) if len(tl) == 1 else _combo(tl, block).astype(BF16)
                dst[i * 64 + r // 2:i * 64 + r // 2 + 8, :] = _pk(val)

    def pre_body(g, c):
        slot = g & (NSLOT - 1)
        buf = stage_ref.at[slot]
        pltpu.make_async_copy(buf, buf, sem_w.at[slot]).wait()

        @pl.when((g >= 2) & (g <= 4))
        def _():
            bq_copy(g - 2).wait()

        @pl.when(g == 4)
        def _():
            bo_copy.wait()

        @pl.when(g <= 2)
        def _():
            bq_copy(g).start()

        @pl.when(g == 2)
        def _():
            bo_copy.start()

        @pl.when(g + 1 <= NG)
        def _():
            for p in range(4):
                w_copy(p, g + 1).start()

        @pl.when(g == NG - 1)
        def _():
            w0_copy(3).start()
            x_late.start()

        wo_store(S55, stage_ref.at[slot, 3], w_ref.at[3 * NG + g - 1], g > NG + 5)
        deps = [b_stage2(3 * (g - 5) + e) for e in range(3)]
        b_stage2_wo(g - 5)
        deps += [b_stage1(3 * (g - 2) + e) for e in range(3)]
        b_stage1_wo(g - 4)
        pcnt[0] = 0
        pdl.extend((DUE_B0 + DUE_B * e, d) for e, d in enumerate(deps))
        tbs = [prep(S55, stage_ref.at[slot, 0], w_ref.at[g - 1])]
        for p in range(3):
            if p < 2:
                tbs.append(prep(S55, stage_ref.at[slot, p + 1], w_ref.at[(p + 1) * NG + g - 1]))
            pre_chunk(S55, stage_ref.at[slot, p], w_ref.at[p * NG + g - 1], p * NT + RT + (g - 1) * GT, [[0, 1, 2], [3], [4], [5]],
                      g > NG + 5, tbs[p])
        return c
    lax.fori_loop(1, NG + 1, pre_body, 0)
    w0_copy(3).wait()
    wo_store(S35, stage0_ref, wr_ref.at[3])

    for r in range(0, 64, 8):
        def raw(k, n):
            return bw_ref[2 * nct + n, k * 64 + r:k * 64 + r + 8, :]
        blocks = {(k, n): _upk(raw(k, n)).astype(F32) for k in range(nct) for n in range(nct)}
        for i, tl in enumerate(S55[0]):
            val = raw(*tl[0]) if len(tl) == 1 else _pk(_combo(tl, lambda k, n: blocks[k, n]).astype(BF16))
            bwf_ref[i * 64 + r:i * 64 + r + 8, :] = val

    bscale = float(bdh) ** (-0.5) * LOG2E

    def b_proj(lhs, part):
        if part == 2 and lhs.shape[0] == 2 * seg:
            kt = lambda a: [a[:, k * 128:(k + 1) * 128] for k in range(nct)]
            ops = _Operands(kt(lhs[0:seg]), kt(lhs[seg:2 * seg]), None, F32 if BLF else BF16)
            p, q = {}, {}
            _fast_mm(S55[1], ops, lambda a, i: _nn(a, _upk(bwf_ref[i * 64:(i + 1) * 64, :])), seg, p, q)
            return _cat([_cat(_fast_out(p, q, n, seg)[0:2]) for n in range(nct)], axis=1)
        return _nn(lhs.astype(BF16), _cat([_upk(bw_ref[part * nct + j]) for j in range(nct)], axis=1))

    def b_attn(jobs, q, k, v):
        row = lax.broadcasted_iota(jnp.int32, (seg, 128), 0)
        outs = []
        for i, (l, sidx) in enumerate(jobs):
            r0 = i * seg
            pos = row + sidx * seg
            for j in range(nct):
                kb_ref[l, j, 0:HIST, :] = kb_ref[l, j, seg:seg + HIST, :]
                vb_ref[l, j, 0:HIST, :] = vb_ref[l, j, seg:seg + HIST, :]
            for j in range(nct):
                kb_ref[l, j, HIST:HIST + seg, :] = k[r0:r0 + seg, j * 128:(j + 1) * 128]
                vb_ref[l, j, HIST:HIST + seg, :] = v[r0:r0 + seg, j * 128:(j + 1) * 128]
            logits = []
            for w in range(B_WIN):
                o = HIST - w * B_DIL
                acc = None
                for j in range(nct):
                    p = q[r0:r0 + seg, j * 128:(j + 1) * 128] * kb_ref[l, j, o:o + seg, :]
                    acc = p if acc is None else acc + p
                acc = acc + pltpu.roll(acc, 64, 1)
                acc = acc + pltpu.roll(acc, 32, 1)
                lg = acc * bscale
                if w > 0:
                    lg = jnp.where(pos >= w * B_DIL, lg, NEG2)
                logits.append(lg)
            m = logits[0]
            for w in range(1, B_WIN):
                m = jnp.maximum(m, logits[w])
            es = [jnp.exp2(lg - m) for lg in logits]
            den = es[0]
            for w in range(1, B_WIN):
                den = den + es[w]
            inv = _recip(den)
            cols = []
            for j in range(nct):
                acc = None
                for w in range(B_WIN):
                    o = HIST - w * B_DIL
                    p = es[w] * vb_ref[l, j, o:o + seg, :]
                    acc = p if acc is None else acc + p
                cols.append(acc * inv)
            outs.append(_cat(cols, axis=1).astype(BF16))
        return outs

    def b_out(ob, res):
        return res + b_proj(ob, 3)

    def o_store(b, val):
        ro = pl.multiple_of((b + 1) * seg, seg)
        o_ref[pl.ds(ro, val.shape[0]), :] = val.astype(o_ref.dtype)

    def out_copy(b):
        ro = pl.multiple_of(b * seg, seg)
        return pltpu.make_async_copy(o_ref.at[pl.ds(ro + seg, seg), :], out_hbm.at[pl.ds(ro, seg), :], sem_o)

    def step(t, hc, full):
        t_last = n_seg + LAG - 1
        if full:
            jobs = [(0, t - 1), (1, t - 1 - LAG)]

            def b_in():
                return xb_ref[0:2 * seg, :]
        else:
            lb = (t == t_last).astype(jnp.int32)
            jobs = [(lb, t - 1 - lb * (LAG + 1))]

            def b_in():
                return xb_ref[pl.ds(pl.multiple_of(lb * seg, seg), seg), :]
        v0r = _cat([hc[0:n_mem], h_ref[n_mem:M2, :]])
        v1r = _cat([hc[n_mem:M2], h_ref[M2 + n_mem:2 * M2, :]])

        hist = []
        never = t > 4 * n_seg

        def gate(back, z):
            gv = hist[-back]
            return _cat([jnp.where(never, gv, z[e:e + 8]) for e in range(0, z.shape[0], 8)])

        def ktiles(z):
            return [z[:, k * 128:(k + 1) * 128] for k in range(z.shape[1] // 128)]
        if full:
            hl = _Operands(ktiles(_cat([v0r, h_ref[2 * M2:RB, :]])), ktiles(_cat([v1r, h_ref[RB:RB + AH, :]])), None)
        else:
            hl = _Operands(None, None, ktiles(_cat([v0r, v1r, h_ref[2 * M2:RB, :]])))
        mh = 2 * M2 if full else 0

        def tile_dot(p, r):
            src = wr_ref.at[p] if r == 0 else w_ref.at[p * NG + r - 1]

            def dot(a, i):
                wt = src[i * 64:(i + 1) * 64, :]
                cnt[0] += 1
                if dl and cnt[0] >= dl[0][0]:
                    deps = dl.pop(0)[1]
                    wt = _cat([jnp.where(never, pltpu.bitcast(d, U32), wt[8 * e:8 * e + 8])
                               for e, d in enumerate(deps)] + [wt[8 * len(deps):]])
                res_ = _nn(a, _upk(wt))
                hist.append(res_[0:8])
                return res_
            return dot
        cnt, dl = [0], []
        scale = float(dh) ** (-0.5) * LOG2E
        if full:
            s_ = t - LAG
            rd = pl.multiple_of(lax.rem(s_ * (seg // 2), RS // 2), seg // 2)
            wa = pl.multiple_of(lax.rem((A0 - R0 + s_ * AH) // 2, RS // 2), 8)
        else:
            wx = pl.multiple_of(jnp.where(t < LAG, NPRE // 2 + t * (n_mem // 2), RS // 2), n_mem // 2)

        RA = R if full else M2 + seg
        CW = R
        bidx = 0 if full else 2
        half = dh - 128
        la8 = lax.broadcasted_iota(jnp.int32, (n_mem, 128), 1) < half
        ones = jnp.full((n_mem, 128), 0xFFFFFFFF, U32)
        zero = jnp.zeros((n_mem, 128), U32)
        mask_a = jnp.where(la8, ones, zero)
        mask_b = jnp.where(la8, zero, ones)

        def pk2(a, b):
            return _pk(_cat([a, b]).astype(BF16))

        yt = [[None] * NT for _ in range(3)]

        def proj(p, r):
            pa, qa = {}, {}
            _fast_mm((S53 if r == 0 else S55)[1], hl, tile_dot(p, r), mh, pa, qa)
            n0 = 0 if r == 0 else RT + (r - 1) * GT
            for n in range(len(pa)):
                y, z, e = _fast_out(pa, qa, n, mh)
                idx = p * NT + n0 + n
                if full:
                    ring_ref[idx, pl.ds(wa, 8), :] = pk2(z[16:24], z[24:32])
                    y = _cat([y[0:M2], z[0:M2], y[M2:2 * M2]])
                else:
                    y = e
                    ring_ref[idx, pl.ds(wx, n_mem // 2), :] = pk2(y[0:8], y[8:16])[0:n_mem // 2]
                yt[p][n0 + n] = stash(p * 16 + (n0 + n) % 16, packed(p, (n0 + n) % 3, y))

        def ab(z8):
            return jnp.where(la8, z8, 0.0), jnp.where(la8, 0.0, z8)

        def packed(p, j, y):
            if p == 0 and j == 1 and full:
                return [pltpu.bitcast(y[e:e + 8], U32) for e in range(0, RB, 8)]
            u2 = pk2(y[32:40], y[40:48])
            if p == 0 or j == 0:
                return [pk2(y[0:8], y[8:16]), pk2(y[16:24], y[24:32]), u2]
            if j == 2:
                return [pk2(y[8:16], y[0:8]), pk2(y[24:32], y[16:24]), u2]
            xa_a, xa_b = ab(y[8:16])
            out = [pk2(xa_b, xa_a), pk2(y[24:32], y[16:24]) & mask_b, pk2(y[16:24], y[24:32]) & mask_a, u2]
            if full:
                out += [pk2(*ab(y[0:8]))]
            return out

        def stash(idx, parts):
            kv_ref[idx, 0:8 * len(parts), :] = _cat(parts)
            return lambda: [kv_ref[idx, 8 * e:8 * e + 8, :] for e in range(len(parts))]

        def pair(p, g):
            xs = [ring_ref[p * NT + 3 * g + j, pl.ds(rd, seg // 2), :] for j in range(3)] if full else None
            return [f() for f in yt[p][3 * g:3 * g + 3]], xs

        def q_rows(z, j):
            v0, v1, v2 = z[0][j]
            return [v0] + ([z[1][j]] if full else []) + [v1, v2]

        def kv_tiles(z):
            yt, x1 = z
            v0, v1, v2 = yt[0]
            t0 = [v0] + ([x1[0]] if full else [v1, v2]) + [v1, v2]
            w0, w1, w2 = yt[2]
            t2 = [w0, w1, w2] + ([x1[2]] if full else [w1, w2])
            e1, mb, ma, u2 = yt[1][0:4]
            mid2 = [e1, mb, u2 & mask_b, ma, u2 & mask_a]
            mid1 = None
            if full:
                lo, hi = x1[1][0:8], x1[1][8:16]
                mid1 = [yt[1][4], lo & mask_a, hi & mask_a, lo & mask_b, hi & mask_b]
            return t0, mid1, mid2, t2

        def mat(parts):
            return _upk(_cat(parts))

        def merge(y1, y2):
            return _cat([y1[0:8], y2[0:8], y1[8:40], y2[8:40]])

        def scores(q, k):
            k0, km1, km2, k2_ = kv_tiles(k)
            s_a = _nt(mat(q_rows(q, 0)), mat(k0))
            s_b = _nt(mat(q_rows(q, 2)), mat(k2_))
            if full:
                f = [pltpu.bitcast(z, F32) for z in q[0][1]]
                s_m = merge(_nt(_cat([f[0], _upk(q[1][1]).astype(F32)]), mat(km1)),
                            _nt(_cat(f[1:]), mat(km2)))
            else:
                s_m = _nt(mat(q_rows(q, 1)), mat(km2))
            out = []
            for e, sx in enumerate((s_a, s_b)):
                s = (sx + s_m) * scale + bias_ref[bidx + e, 0:RA, 0:CW]
                ex = jnp.exp2(s - jnp.max(s, axis=-1, keepdims=True))
                out.append(ex * _recip(jnp.sum(ex, axis=-1, keepdims=True)))
            return out

        def pv(p, v):
            PD = F32 if PF else BF16
            v0, vm1, vm2, v2 = kv_tiles(v)
            o_a = _nn(p[0].astype(PD), mat(v0))
            o_b = _nn(p[1].astype(PD), mat(v2))
            p = p[0] + p[1]
            if full:
                o_m = merge(_nn(_cat([p[0:8], p[16:48]]), mat(vm1)), _nn(_cat([p[8:16], p[48:80]]), mat(vm2)))
            else:
                o_m = _nn(p.astype(PD), mat(vm2))
            return [o_a, o_m, o_b]

        ot = []
        pacc, qacc = {}, {}
        mo = n_mem + seg if (full and WF) else mh

        def add_o(r):
            n0 = 0 if r == 0 else RT + (r - 1) * GT
            oo = ot[n0:n0 + (RT if r == 0 else GT)]
            if full and WF:
                us = [_cat([o[48:56], o[8:16], o[56:80]]) for o in oo]
                if r < TAILPV and GATE_O:
                    us = [gate(GATE_O, z) for z in us]
                ops = _Operands([_cat([o[0:8], o[16:48]]) for o in oo], us, None, F32)
            elif full:
                us = [_cat([o[48:64], o[32:48]]) for o in oo]
                if r < TAILPV:
                    us = [gate(GATE_O, z) for z in us]
                ops = _Operands([o[0:32] for o in oo], us, [o[64:80] for o in oo])
            else:
                ops = _Operands(None, None, oo)
            _fast_mm((S35 if r == 0 else S55)[1], ops, tile_dot(3, r), mo, pacc, qacc)

        bqkv = [None] * 3
        probs = []

        def do_pv():
            for g in range(len(ot) // 3, len(probs)):
                ot.extend(pv(probs[g], pair(2, g)))

        if full:
            an = pl.multiple_of(jnp.minimum(A0 + (s_ + 1) * AH, S - AH), AH)
            h_ref[RB:RB + AH, :] = _ln(x_ref[pl.ds(an, AH), :].astype(F32))

        for r in range(NG + 1):
            proj(2, r)
            proj(1, r)
            proj(0, r)
            if r == 0:
                blhs = _ln(b_in())
            if r < 3:
                bqkv[2 - r] = b_proj(blhs, 2 - r)
            if r == 3:
                ob = b_attn(jobs, *bqkv)
            if r == BOUT_R:
                zb = b_out(_cat(ob), b_in())
                x2_new = zb[0:seg]
                if full:
                    o_store(t - 1 - LAG, zb[seg:2 * seg])
                    nxt = x2_new
                else:
                    o_store(lb * (t_last - LAG - 1) - 1, x2_new)
                    nxt = jnp.where(t < LAG - 1, x_ref[seg:2 * seg, :].astype(F32), x2_new)
                sl = _ln(nxt)
                h_ref[n_mem:M2, :] = sl[0:n_mem]
                h_ref[M2 + n_mem:RB, :] = sl[n_mem:seg]
                if full:
                    for j in range(nct):
                        dl.append((cnt[0] + DUE_LN + 2 * j, [sl[e:e + 8, j * 128:(j + 1) * 128] for e in range(0, seg, 8)]))
            if r in WSCHED:
                add_o(WSCHED[r])
            do_pv()
            for g in range(len(probs), (RT + r * GT) // 3):
                probs.append(scores(pair(0, g), pair(1, g)))
        for r in range(len(WSCHED), TAILPV):
            add_o(r)
        do_pv()
        for r in range(TAILPV, NG + 1):
            add_o(r)
        cols = []
        for n in range(nct):
            y, z, e = _fast_out(pacc, qacc, n, mo)
            if full and WF:
                cols.append(_cat([y[0:8], z[8:16], y[8:40], z[0:8], z[16:40]]))
            else:
                cols.append(_cat([y, z[16:32], z[0:16], e]) if full else e)
        acc = _cat(cols, axis=1)

        y2 = x2_ref[...] + _cat([acc[n_mem:M2], acc[RA - seg + n_mem:RA]])
        mem2 = acc[RA - seg:RA - seg + n_mem]
        if full:
            x_cur = x_ref[pl.ds(pl.multiple_of(t * seg, seg), seg), :].astype(F32)
            xb_ref[0:seg, :] = x_cur + acc[M2:M2 + seg]
            xb_ref[seg:2 * seg, :] = y2
            m1n = acc[0:n_mem]
            m2n = mem2
        else:
            xb_ref[pl.ds(pl.multiple_of(jnp.where(t < LAG, 0, (t - n_seg + 2) * seg), seg), seg), :] = y2
            m1n = jnp.where(t < LAG - 1, h_ref[RB + AH:RB + AH + n_mem, :], mem2)
            m2n = jnp.where(t == LAG - 1, mem0_ref[...].astype(F32), mem2)
        x2_ref[...] = nxt
        return _cat([m1n, m2n])

    def single_body(t, c):
        @pl.when(t == n_seg)
        def _():
            out_copy(t - (LAG + 2)).start()
        return step(t, c, False)

    def full_body(t, c):
        @pl.when(t >= LAG + 2)
        def _():
            out_copy(t - (LAG + 2)).start()
        return step(t, c, True)

    def phase(ph, c):
        t0 = ph * n_seg
        c = lax.fori_loop(t0, t0 + LAG, single_body, c)

        @pl.when(ph == 0)
        def _():
            x_late.wait()
        return lax.fori_loop(LAG, jnp.where(ph == 0, n_seg, LAG), full_body, c)
    lax.fori_loop(0, 2, phase, _cat([h_ref[0:n_mem, :], h_ref[M2:M2 + n_mem, :]]))

    out_copy(n_seg - 3).start()
    res = xb_ref[2 * seg:4 * seg, :]
    blhs = _ln(res)
    ob = b_attn([(1, n_seg - 2), (1, n_seg - 1)], *[b_proj(blhs, part) for part in range(3)])
    o_store(n_seg - 2, b_out(_cat(ob), res))
    out_copy(n_seg - 2).start()
    out_copy(n_seg - 1).start()
    pltpu.make_async_copy(o_ref.at[pl.ds(seg, S), :], out_hbm, sem_o).wait()


@functools.partial(jax.jit, static_argnames=("seg",))
def _run(A_x, A_mem0, A_Wq, A_Wk, A_Wv, A_Wo, B_wqkv, B_wo, *, seg):
    _, S, dm = A_x.shape
    n_heads, dh = A_Wq.shape[1], A_Wq.shape[2]
    n_mem = A_mem0.shape[1]
    n_seg = S // seg
    hd = n_heads * dh
    nct = dm // 128
    ng = (hd // 128 - RT) // GT
    assert (seg, n_seg, n_mem, dh, dm % 128, n_heads, LAG) == (32, 64, 8, 192, 0, 32, 2)

    x = A_x.reshape(S, dm)
    mem0 = A_mem0.reshape(n_mem, dm)
    wq = jnp.transpose(A_Wq, (1, 2, 0)).reshape(hd, dm)
    wk = jnp.transpose(A_Wk, (1, 2, 0)).reshape(hd, dm)
    wv = jnp.transpose(A_Wv, (1, 2, 0)).reshape(hd, dm)
    wo = A_Wo.reshape(hd, dm)
    _, _, _, _, rs, xc = _plan(seg, n_seg)

    kern = functools.partial(_kernel, seg=seg, n_seg=n_seg, n_mem=n_mem,
                             n_heads=n_heads, dh=dh, dm=dm)
    hbm = pl.BlockSpec(memory_space=pltpu.HBM)

    out = pl.pallas_call(
        kern,
        in_specs=[hbm] * 8,
        out_specs=hbm,
        out_shape=jax.ShapeDtypeStruct((S, dm), A_x.dtype),
        scratch_shapes=[
            pltpu.VMEM((S, dm), BF16),
            pltpu.VMEM((n_mem, dm), BF16),
            pltpu.VMEM((NSLOT, 4, GT * 128, dm), BF16),
            pltpu.VMEM((RT * 128, dm), BF16),
            pltpu.VMEM((4, len(S53[0]) * 64, 128), U32),
            pltpu.VMEM((4 * ng, len(S55[0]) * 64, 128), U32),
            pltpu.VMEM((dm, 4 * dm + 128), BF16),
            pltpu.VMEM((nct, 4 * dm + 32, 128), F32),
            pltpu.VMEM((4 * nct, dm // 2, 128), U32),
            pltpu.VMEM((len(KEYS_R), HC * xc // 4, 128), U32),
            pltpu.VMEM((len(KEYS_R), HC * xc // 4, 128), U32),
            pltpu.VMEM((len(KEYS) - len(KEYS_R), NXC * xc // 4, 128), U32),
            pltpu.VMEM((15, 8, 128), U32),
            pltpu.VMEM((3 * hd // 128, rs // 2 + 8, 128), U32),
            pltpu.VMEM((3 * n_mem + seg + AH, dm), F32),
            pltpu.VMEM((4 * seg, dm), F32),
            pltpu.VMEM((seg, dm), F32),
            pltpu.VMEM((2, nct, HIST + seg, 128), F32),
            pltpu.VMEM((2, nct, HIST + seg, 128), F32),
            pltpu.VMEM((S + seg, dm), A_x.dtype),
            pltpu.VMEM((4, 2 * n_mem + 2 * seg, 128), F32),
            pltpu.VMEM((48, 48, 128), U32),
            pltpu.VMEM((len(S55[0]) * 64, 128), U32),
            pltpu.SemaphoreType.DMA((NSLOT,)),
            pltpu.SemaphoreType.DMA((8 + NXC,)),
            pltpu.SemaphoreType.DMA((4,)),
            pltpu.SemaphoreType.DMA(()),
        ],
        compiler_params=pltpu.CompilerParams(
            vmem_limit_bytes=127 * 1024 * 1024,
            disable_bounds_checks=True,
        ),
    )(x, mem0, wq, wk, wv, wo, B_wqkv, B_wo)
    return out.reshape(1, S, dm)


def pallas_interleave_layers__memory_aug_recurrent_mem_tr__sliding_local_dilated__prompt_kernel(
    A_x: jax.Array,
    A_mem0: jax.Array,
    A_Wq: jax.Array,
    A_Wk: jax.Array,
    A_Wv: jax.Array,
    A_Wo: jax.Array,
    A_seg_len,
    B_x: jax.Array,
    B_wqkv: jax.Array,
    B_wo: jax.Array,
):
    del B_x
    seg = A_seg_len if isinstance(A_seg_len, int) else 32
    return _run(A_x, A_mem0, A_Wq, A_Wk, A_Wv, A_Wo, B_wqkv, B_wo, seg=seg)
```

```python
import functools

import jax
import jax.numpy as jnp
from jax import lax
import jax.experimental.pallas as pl
import jax.experimental.pallas.tpu as pltpu

F32 = jnp.float32
BF16 = jnp.bfloat16
U32 = jnp.uint32
NEG = -1000000000.0
LN_EPS = 1e-05
LOG2E = 1.4426950408889634
NEG2 = NEG * LOG2E

B_HEADS = 32
B_WIN = 8
B_DIL = 2
HIST = 16
WF = int(1)
PF = int(0)
BLF = int(0)
AH = 16
LAG = 2
NSLOT = 2
NXC = 6
HC = 3
WSCHED = {3: 0, 4: 1, 6: 2, 7: 3, 8: 4, 9: 5}
BOUT_R = 5
TAILPV = int(8)
GATE_O = int(50)
DUE_LN = 150
DUE_X = 24
DUE_B0, DUE_B = 100, 60


def _ln(x):
    m = jnp.mean(x, axis=-1, keepdims=True)
    c = x - m
    v = jnp.mean(c * c, axis=-1, keepdims=True)
    return c * lax.rsqrt(v + LN_EPS)


def _recip(d):
    return pl.reciprocal(d, approx=True)


def _nt(a, b):
    return lax.dot_general(a, b, (((1,), (1,)), ((), ())), preferred_element_type=F32)


def _nn(a, b):
    return lax.dot_general(a, b, (((1,), (0,)), ((), ())), preferred_element_type=F32)


def _cat(xs, axis=0):
    return xs[0] if len(xs) == 1 else jnp.concatenate(xs, axis=axis)


def _pk(z):
    return pltpu.bitcast(z, U32)


def _upk(z):
    return pltpu.bitcast(z, BF16)


LAM = (-1.5, -0.5, 0.0, 0.5, 1.5)


def _scheme(stars):
    tiles, prog = [], []
    for star in stars:
        if len(star) == 1:
            prog.append(("single", star[0], None, len(tiles)))
            tiles.append([star[0][:2]])
            continue
        left = [len(star) - 1] * len(star)
        for j in range(1, len(star)):
            for i in range(j):
                x, y = star[i], star[j]
                prog.append(("pair", x, y, len(tiles)))
                tiles += [[(x[0], y[1])], [(y[0], x[1])], [(x[0], y[1]), (y[0], x[1])]]
                for e in (i, j):
                    left[e] -= 1
                    if left[e] == 0:
                        z = star[e]
                        prog.append(("diag", z, None, len(tiles)))
                        tiles += [[z[:2]] + [(o[0], z[1]) for o in star if o is not z],
                                  [z[:2]] + [(z[0], o[1]) for o in star if o is not z]]
    return tiles, prog


S55 = _scheme([[(i, i, LAM[i]) for i in range(5)]])
S53 = _scheme([[(0, 0, LAM[0]), (2, 1, LAM[2]), (4, 2, LAM[4])], [(1, 0, LAM[1]), (3, 2, LAM[3])],
               [(1, 1, LAM[1])], [(3, 1, LAM[3])]])
S35 = _scheme([[(0, 0, LAM[0]), (1, 2, LAM[2]), (2, 4, LAM[4])], [(0, 1, LAM[1]), (2, 3, LAM[3])],
               [(1, 1, LAM[1])], [(1, 3, LAM[3])]])


def _spread(prog):
    pairs = [e for e in prog if e[0] != "diag"]
    diags = [e for e in prog if e[0] == "diag"]
    out, k = [], 0
    for i, e in enumerate(pairs):
        out.append(e)
        while k < len(diags) and (k + 0.5) * len(pairs) <= (i + 1) * len(diags):
            out.append(diags[k])
            k += 1
    return out + diags[k:]


def _op_keys(prog):
    keys = []
    for kind, x, y, _ in prog:
        if kind == "pair":
            new = [(nm, x[0], x[2], y[0], y[2]) for nm in ("l1", "l2", "A")]
        else:
            new = [("a", x[0], x[2]), ("b", x[0])]
        keys += [k for k in new if k not in keys]
    return keys


def _scaled(c, u):
    return u if c == 1.0 else c * u


class _Operands:
    def __init__(self, T, U, E, dtype=BF16):
        self.T, self.U, self.E, self.memo, self.dtype = T, U, E, {}, dtype

    def _get(self, key, fn):
        if key not in self.memo:
            self.memo[key] = fn()
        return self.memo[key]

    def paired(self, key):
        T, U = self.T, self.U
        if key[0] == "b":
            return U[key[1]]
        if key[0] == "a":
            k, lam = key[1:]
            if lam == 0.0:
                return T[k]
            return self._get(("f",) + key, lambda: T[k] - _scaled(lam, U[k]) if lam > 0
                             else T[k] + _scaled(-lam, U[k]))
        kx, lx, ky, ly = key[1:]
        A = self._get(("f", "A") + key[1:],
                      lambda: self.paired(("a", kx, lx)) + self.paired(("a", ky, ly)))
        if key[0] == "A":
            return A
        return A - _scaled(ly - lx, U[kx]) if key[0] == "l1" else A + _scaled(ly - lx, U[ky])

    def extra(self, key):
        if key[0] == "a":
            return self.E[key[1]]
        return self._get(("e", key[1], key[3]), lambda: self.E[key[1]] + self.E[key[3]])

    def __call__(self, key):
        if self.T is None:
            ek = ("a", key[1]) if key[0] in ("a", "s") else ("l", key[1], 0, key[3])
            return self._get(ek, lambda: self.extra(ek).astype(self.dtype))

        def build():
            ak = ("a",) + key[1:] if key[0] == "s" else key
            parts = [self.paired(ak)]
            if self.E is not None and ak[0] in ("a", "l1", "l2"):
                parts.append(self.extra(ak))
            if key[0] == "s":
                parts.append(self.U[key[1]])
            return _cat(parts).astype(self.dtype)
        return self._get(key, build)


def _fast_mm(prog, op, dot, m, p, q):
    def add(d, key, val):
        d[key] = val if key not in d else d[key] + val

    for kind, x, y, i in prog:
        if kind == "pair":
            kk = (x[0], x[2], y[0], y[2])
            p1, p2 = dot(op(("l1",) + kk), i), dot(op(("l2",) + kk), i + 1)
            if m:
                r = _scaled(1.0 / (y[2] - x[2]), p2[0:m] - p1[0:m] + dot(op(("A",) + kk), i + 2))
                add(q, (x[1], x[2]), r)
                add(q, (y[1], y[2]), r)
            add(p, y[1], p1)
            add(p, x[1], p2)
        elif kind == "diag":
            add(p, x[1], dot(op(("a", x[0], x[2])), i))
            if m:
                add(q, (x[1], x[2]), dot(op(("b", x[0])), i + 1))
        else:
            r = dot(op(("s", x[0], x[2])), i)
            add(p, x[1], r[0:r.shape[0] - m])
            if m:
                add(q, (x[1], x[2]), r[r.shape[0] - m:])


def _fast_out(p, q, n, m):
    if not m:
        return None, None, p[n]
    y, z = p[n][0:m], None
    for (nn, lam), v in q.items():
        if nn == n:
            z = v if z is None else z + v
            if lam != 0.0:
                y = y + _scaled(lam, v) if lam > 0 else y - _scaled(-lam, v)
    return y, z, (p[n][m:] if p[n].shape[0] > m else None)


def _combo(tile, block):
    out = block(*tile[0])
    for kn in tile[1:]:
        out = out - block(*kn)
    return out


GT = 5
RT = 3
KEYS_R = _op_keys(S53[1])
KEYS = KEYS_R + [k for k in _op_keys(S55[1]) if k not in KEYS_R]


def _plan(seg, n_seg):
    S = seg * n_seg
    R0 = LAG * seg
    A0 = S - (n_seg - LAG) * AH
    NPRE = A0 - R0
    RS = -(-(A0 - R0 + AH) // seg) * seg
    XC = NPRE // NXC // 32 * 32
    assert XC * NXC + 32 == NPRE
    return S, R0, A0, NPRE, RS, XC


def _kernel(x_hbm, mem0_hbm, wq_hbm, wk_hbm, wv_hbm, wo_hbm, bqkv_hbm, bwo_hbm,
            out_hbm,
            x_ref, mem0_ref, stage_ref, stage0_ref, wr_ref, w_ref, bst_ref, btmp_ref, bw_ref,
            xla_ref, xlb_ref, xlc_ref, xe_ref, ring_ref, h_ref, xb_ref, x2_ref, kb_ref, vb_ref, o_ref, bias_ref, kv_ref, bwf_ref,
            sem_w, sem_m, sem_b, sem_o,
            *, seg, n_seg, n_mem, n_heads, dh, dm):
    S, R0, A0, NPRE, RS, XC = _plan(seg, n_seg)
    M2 = 2 * n_mem
    R = M2 + 2 * seg
    RB = M2 + seg
    nct = dm // 128
    bdh = dm // B_HEADS
    NT = n_heads * dh // 128
    NG = (NT - RT) // GT
    w_hbm = (wq_hbm, wk_hbm, wv_hbm, wo_hbm)

    def w_copy(p, g):
        slot = g & (NSLOT - 1)
        return pltpu.make_async_copy(w_hbm[p].at[pl.ds((RT + (g - 1) * GT) * 128, GT * 128), :],
                                     stage_ref.at[slot, p], sem_w.at[slot])

    def w0_copy(p):
        dst = stage0_ref if p == 3 else stage_ref.at[0, p, pl.ds(0, RT * 128)]
        return pltpu.make_async_copy(w_hbm[p].at[pl.ds(0, RT * 128), :], dst, sem_m.at[4 + p])

    NB1 = 3 * nct
    WO0 = 3 * dm
    XF = A0 + AH
    XH = XC // 2

    def rows_copy(r0, n, sem):
        return pltpu.make_async_copy(x_hbm.at[pl.ds(r0, n), :], x_ref.at[pl.ds(r0, n), :], sem)

    def x_copy(i):
        return rows_copy(pl.multiple_of(R0 + i * XC, 16), XC, sem_m.at[8 + i])

    small = [rows_copy(0, R0, sem_m.at[1]), rows_copy(R0 + NPRE - 32, XF - R0 - NPRE + 32, sem_m.at[2]),
             pltpu.make_async_copy(mem0_hbm, mem0_ref, sem_m.at[3])]
    x_late = rows_copy(XF, S - XF, sem_m.at[0])

    def bq_copy(part):
        c0 = pl.multiple_of(part * dm, 128)
        return pltpu.make_async_copy(bqkv_hbm.at[:, pl.ds(c0, dm)], bst_ref.at[:, pl.ds(c0, dm)], sem_b.at[part])

    bo_copy = pltpu.make_async_copy(bwo_hbm, bst_ref.at[:, pl.ds(3 * dm, dm)], sem_b.at[3])

    def bst_tile(c):
        return bst_ref[:, pl.ds(pl.multiple_of(c * 128, 128), 128)]

    def bias_tables(full):
        RA = R if full else n_mem + seg
        CW = 128
        ri = lax.broadcasted_iota(jnp.int32, (RA, CW), 0)
        ci = lax.broadcasted_iota(jnp.int32, (RA, CW), 1)
        if not full:
            ri = jnp.where(ri >= n_mem, ri + n_mem + seg, ri + n_mem)

        def table(i, bounds, vals):
            out = vals[-1]
            for b, v in zip(reversed(bounds), reversed(vals[:-1])):
                out = jnp.where(i < b, v, out)
            return out
        qi = ri - table(ri, [16, 48, 56], [0, 8, 48, 40])
        g0 = (ci < 8) | ((ci >= 16) & (ci < 48))
        k2 = ci - table(ci, [8, 24, 32, 48, 56], [-8, 0, 24, 8, 48, 40])
        if full:
            k1 = ci - table(ci, [8, 48], [0, 8, 40])
            row_l2 = ((ri >= 8) & (ri < 16)) | (ri >= 48)
            is_a = g0 != row_l2
            ki = jnp.where(row_l2, k2, k1)
        else:
            is_a = jnp.logical_not(g0)
            ki = k2
        visible = (qi < n_mem) | (qi >= ki)
        fill = NEG2
        for e, mine in enumerate((is_a, jnp.logical_not(is_a))):
            bias_ref[(0 if full else 2) + e, 0:RA, :] = jnp.where(
                mine, jnp.where(visible, 0.0, fill), -jnp.inf)

    for i in range(HC):
        x_copy(i).start()

    def zero_body(j, c):
        btmp_ref[j, 0:dm, :] = jnp.zeros((dm, 128), F32)
        return c
    lax.fori_loop(0, nct, zero_body, 0)

    w0_copy(0).start()
    xb_ref[0:2 * seg, :] = jnp.zeros((2 * seg, dm), F32)
    kb_ref[...] = jnp.zeros(kb_ref.shape, F32)
    vb_ref[...] = jnp.zeros(vb_ref.shape, F32)
    bst_ref[:, 4 * dm:] = jnp.zeros((dm, 128), BF16)
    bias_tables(True)
    bias_tables(False)

    def e_ops():
        ye = _ln(x_ref[R0 + NPRE - 32:R0 + NPRE, :].astype(F32))
        eops = _Operands([ye[0:16, k * 128:(k + 1) * 128] for k in range(nct)],
                         [ye[16:32, k * 128:(k + 1) * 128] for k in range(nct)], None)
        for j, key in enumerate(KEYS):
            xe_ref[j] = _pk(eops(key))

    NKR = len(KEYS_R)

    def xl(j, hf, i):
        if j >= NKR:
            ref, j, i = xlc_ref, j - NKR, hf * HC + i
        else:
            ref = (xla_ref, xlb_ref)[hf]
        r0 = i * (XH // 2)
        return ref.at[j, pl.ds(r0 if isinstance(r0, int) else pl.multiple_of(r0, 8), XH // 2)]

    def ln_ops(hf, i, lo, hi):
        y = _ln(x_ref[pl.ds(pl.multiple_of(R0 + (hf * HC + i) * XC, 16), XC), :].astype(F32))
        ops = _Operands([y[0:XH, k * 128:(k + 1) * 128] for k in range(nct)],
                        [y[XH:XC, k * 128:(k + 1) * 128] for k in range(nct)], None)
        vals = []
        for j in range(lo, hi):
            v = _pk(ops(KEYS[j]))
            xl(j, hf, i)[...] = v
            vals.append([v[e:e + 8] for e in range(0, XH // 2, 8)])
        return vals

    def ln_body(i, c):
        x_copy(i).wait()

        @pl.when(i == 0)
        def _():
            x_copy(HC).start()

        @pl.when(i == 1)
        def _():
            w0_copy(1).start()
            w0_copy(2).start()

        @pl.when(i == 2)
        def _():
            x_copy(HC + 1).start()
            x_copy(HC + 2).start()
            for cp in small:
                cp.start()
        ln_ops(0, i, 0, len(KEYS_R))
        return c
    lax.fori_loop(0, HC, ln_body, 0)

    def prep(scheme, w, dst):
        raw = lambda k, n: w[n * 128:(n + 1) * 128, k * 128:(k + 1) * 128]
        tb = []
        for i, tl in enumerate(scheme[0]):
            tb.append(raw(*tl[0]) if len(tl) == 1
                      else _combo(tl, lambda k, n: raw(k, n).astype(F32)).astype(BF16))
            dst[i * 64:(i + 1) * 64, :] = _pk(tb[i].T)
        return tb

    pcnt, pdl = [0], []

    def pre_chunk(scheme, w, dst, n0, chunks, never=None, tb=None):
        tiles, prog = scheme
        prog = _spread(prog)
        dot = lambda a, i: _nn(a, _upk(dst[i * 64:(i + 1) * 64, :]))
        if w is not None:
            if tb is None:
                tb = prep(scheme, w, dst)
            dot = lambda a, i: _nt(a, tb[i])

        for cs in chunks:
            def op(key):
                def ld(kk):
                    v = [xl(KEYS.index(kk), c // HC, c % HC)[...] for c in cs]
                    if NXC - 1 in cs:
                        v.append(xe_ref[KEYS.index(kk)])
                    return _cat(v)
                if key[0] == "s":
                    return _upk(_cat([ld(("a",) + key[1:]), ld(("b", key[1]))]))
                v = ld(key)
                pcnt[0] += len(cs)
                if pdl and pcnt[0] >= pdl[0][0]:
                    deps = pdl.pop(0)[1]
                    v = _cat([jnp.where(never, d, v[8 * e:8 * e + 8]) for e, d in enumerate(deps)]
                             + ([v[8 * len(deps):]] if v.shape[0] > 8 * len(deps) else []))
                return _upk(v)
            p, q = {}, {}
            m = XH * len(cs) + (16 if NXC - 1 in cs else 0)
            _fast_mm(prog, op, dot, m, p, q)
            for n in range(len(p)):
                y, z, e = _fast_out(p, q, n, m)
                for ic, c in enumerate(cs):
                    ring_ref[n0 + n, c * XH:c * XH + XH // 2, :] = _pk(y[ic * XH:(ic + 1) * XH].astype(BF16))
                    ring_ref[n0 + n, c * XH + XH // 2:(c + 1) * XH, :] = _pk(z[ic * XH:(ic + 1) * XH].astype(BF16))
                if NXC - 1 in cs:
                    ring_ref[n0 + n, NXC * XH:NXC * XH + 16, :] = _pk(_cat([y[m - 16:m], z[m - 16:m]]).astype(BF16))

    def init_rows():
        x0 = x_ref[0:seg, :].astype(F32)
        sl = _ln(x0)
        xt = _ln(x_ref[R0 + NPRE:XF, :].astype(F32))
        h_ref[n_mem:M2, :] = sl[0:n_mem]
        h_ref[M2 + n_mem:RB, :] = sl[n_mem:seg]
        h_ref[RB:RB + AH, :] = xt
        x2_ref[...] = x0

    def first_a(p, c):
        buf = stage_ref.at[0, p, pl.ds(0, RT * 128)]
        pltpu.make_async_copy(buf, buf, sem_m.at[4 + p]).wait()
        x_copy(HC + p).wait()

        @pl.when(p == 0)
        def _():
            for pp in range(4):
                w_copy(pp, 1).start()

        @pl.when(p == 2)
        def _():
            bq_copy(0).start()
        vals = ln_ops(1, p, 0, len(KEYS))
        pcnt[0] = 0
        pdl.extend((DUE_X + e, d) for e, d in enumerate(vals))
        pre_chunk(S53, buf, wr_ref.at[p], p * NT, [[c] for c in range(HC)], p > 9)
        del pdl[:]
        return c
    lax.fori_loop(0, 3, first_a, 0)
    for cp in small:
        cp.wait()

    def first_b(p, c):
        e_ops()
        init_rows()
        vals = ln_ops(0, p, len(KEYS_R), len(KEYS))
        pcnt[0] = 0
        pdl.extend((DUE_X + 2 * e, d) for e, d in enumerate(vals))
        pre_chunk(S53, None, wr_ref.at[p], p * NT, [[c] for c in range(HC, NXC)], p > 9)
        del pdl[:]
        return c
    lax.fori_loop(0, 3, first_b, 0)

    dpt = 128 // B_HEADS

    def b_stage1(u):
        uc = jnp.clip(u, 0, NB1 - 1)
        tr = bst_tile(jnp.where(u >= 0, uc, NB1 + nct)).astype(F32).T
        r0 = pl.multiple_of(uc * 128, 128)
        for j in range(nct):
            btmp_ref[j, pl.ds(r0, 128), :] = tr[:, j * 128:(j + 1) * 128]
        return [pltpu.bitcast(tr[120:128, j * 128:(j + 1) * 128], U32) for j in range(nct)]

    def b_stage1_wo(u):
        uc = jnp.clip(u, 0, nct - 1)
        btmp_ref[uc, WO0:WO0 + dm, :] = bst_tile(jnp.where(u >= 0, NB1 + uc, NB1 + nct)).astype(F32)

    def b_stage2(u):
        uc = jnp.clip(u, 0, NB1 - 1)
        part = (uc >= nct).astype(jnp.int32) + (uc >= 2 * nct).astype(jnp.int32)
        r0 = part * dm + (uc - part * nct) * dpt
        rows = _cat([_cat([btmp_ref[j, pl.ds(r0 + dd, B_HEADS, stride=bdh), :]
                           for j in range(nct)], axis=1) for dd in range(dpt)])
        val = _pk(rows.T.astype(BF16))
        bw_ref[uc] = val
        return [val[64 * j + 56:64 * j + 64] for j in range(nct)]

    def b_stage2_wo(u):
        uc = jnp.clip(u, 0, nct - 1)
        r0 = jnp.where(u >= 0, WO0, 0)
        bw_ref[NB1 + uc] = _pk(
            _cat([btmp_ref[uc, pl.ds(r0 + d, B_HEADS, stride=bdh), :] for d in range(bdh)]).astype(BF16))

    def wo_store(scheme, w, dst, never=None):
        if scheme is S55:
            rawt = lambda k, n: w[k * 128:(k + 1) * 128, n * 128:(n + 1) * 128]
            plain = [i for i, tl in enumerate(scheme[0]) if len(tl) == 1]
            for i, tl in enumerate(scheme[0]):
                if len(tl) > 1:
                    val = _combo(tl, lambda k, n: rawt(k, n).astype(F32)).astype(BF16)
                    val = _pk(_upk(_pk(val.T)).T)
                    dst[i * 64:(i + 1) * 64, :] = val
                    j = plain.pop()
                    pv_ = _pk(rawt(*scheme[0][j][0]))
                    dst[j * 64:(j + 1) * 64, :] = jnp.where(never, val, pv_)
            return
        for r in range(0, 128, 16):
            memo = {}

            def raw(k, n):
                return w[k * 128 + r:k * 128 + r + 16, n * 128:(n + 1) * 128]

            def block(k, n):
                if (k, n) not in memo:
                    memo[k, n] = raw(k, n).astype(F32)
                return memo[k, n]
            for i, tl in enumerate(scheme[0]):
                val = raw(*tl[0]) if len(tl) == 1 else _combo(tl, block).astype(BF16)
                dst[i * 64 + r // 2:i * 64 + r // 2 + 8, :] = _pk(val)

    def pre_body(g, c):
        slot = g & (NSLOT - 1)
        buf = stage_ref.at[slot]
        pltpu.make_async_copy(buf, buf, sem_w.at[slot]).wait()

        @pl.when((g >= 2) & (g <= 4))
        def _():
            bq_copy(g - 2).wait()

        @pl.when(g == 4)
        def _():
            bo_copy.wait()

        @pl.when(g <= 2)
        def _():
            bq_copy(g).start()

        @pl.when(g == 2)
        def _():
            bo_copy.start()

        @pl.when(g + 1 <= NG)
        def _():
            for p in range(4):
                w_copy(p, g + 1).start()

        @pl.when(g == NG - 1)
        def _():
            w0_copy(3).start()
            x_late.start()

        wo_store(S55, stage_ref.at[slot, 3], w_ref.at[3 * NG + g - 1], g > NG + 5)
        deps = [b_stage2(3 * (g - 5) + e) for e in range(3)]
        b_stage2_wo(g - 5)
        deps += [b_stage1(3 * (g - 2) + e) for e in range(3)]
        b_stage1_wo(g - 4)
        pcnt[0] = 0
        pdl.extend((DUE_B0 + DUE_B * e, d) for e, d in enumerate(deps))
        tbs = [prep(S55, stage_ref.at[slot, 0], w_ref.at[g - 1])]
        for p in range(3):
            if p < 2:
                tbs.append(prep(S55, stage_ref.at[slot, p + 1], w_ref.at[(p + 1) * NG + g - 1]))
            pre_chunk(S55, stage_ref.at[slot, p], w_ref.at[p * NG + g - 1], p * NT + RT + (g - 1) * GT, [[0, 1, 2], [3], [4], [5]],
                      g > NG + 5, tbs[p])
        return c
    lax.fori_loop(1, NG + 1, pre_body, 0)
    w0_copy(3).wait()
    wo_store(S35, stage0_ref, wr_ref.at[3])

    for r in range(0, 64, 8):
        def raw(k, n):
            return bw_ref[2 * nct + n, k * 64 + r:k * 64 + r + 8, :]
        blocks = {(k, n): _upk(raw(k, n)).astype(F32) for k in range(nct) for n in range(nct)}
        for i, tl in enumerate(S55[0]):
            val = raw(*tl[0]) if len(tl) == 1 else _pk(_combo(tl, lambda k, n: blocks[k, n]).astype(BF16))
            bwf_ref[i * 64 + r:i * 64 + r + 8, :] = val

    bscale = float(bdh) ** (-0.5) * LOG2E

    def b_proj(lhs, part):
        if part == 2 and lhs.shape[0] == 2 * seg:
            kt = lambda a: [a[:, k * 128:(k + 1) * 128] for k in range(nct)]
            ops = _Operands(kt(lhs[0:seg]), kt(lhs[seg:2 * seg]), None, F32 if BLF else BF16)
            p, q = {}, {}
            _fast_mm(S55[1], ops, lambda a, i: _nn(a, _upk(bwf_ref[i * 64:(i + 1) * 64, :])), seg, p, q)
            return _cat([_cat(_fast_out(p, q, n, seg)[0:2]) for n in range(nct)], axis=1)
        return _nn(lhs.astype(BF16), _cat([_upk(bw_ref[part * nct + j]) for j in range(nct)], axis=1))

    def b_attn(jobs, q, k, v):
        row = lax.broadcasted_iota(jnp.int32, (seg, 128), 0)
        outs = []
        for i, (l, sidx) in enumerate(jobs):
            r0 = i * seg
            pos = row + sidx * seg
            for j in range(nct):
                kb_ref[l, j, 0:HIST, :] = kb_ref[l, j, seg:seg + HIST, :]
                vb_ref[l, j, 0:HIST, :] = vb_ref[l, j, seg:seg + HIST, :]
            for j in range(nct):
                kb_ref[l, j, HIST:HIST + seg, :] = k[r0:r0 + seg, j * 128:(j + 1) * 128]
                vb_ref[l, j, HIST:HIST + seg, :] = v[r0:r0 + seg, j * 128:(j + 1) * 128]
            logits = []
            for w in range(B_WIN):
                o = HIST - w * B_DIL
                acc = None
                for j in range(nct):
                    p = q[r0:r0 + seg, j * 128:(j + 1) * 128] * kb_ref[l, j, o:o + seg, :]
                    acc = p if acc is None else acc + p
                acc = acc + pltpu.roll(acc, 64, 1)
                acc = acc + pltpu.roll(acc, 32, 1)
                lg = acc * bscale
                if w > 0:
                    lg = jnp.where(pos >= w * B_DIL, lg, NEG2)
                logits.append(lg)
            m = logits[0]
            for w in range(1, B_WIN):
                m = jnp.maximum(m, logits[w])
            es = [jnp.exp2(lg - m) for lg in logits]
            den = es[0]
            for w in range(1, B_WIN):
                den = den + es[w]
            inv = _recip(den)
            cols = []
            for j in range(nct):
                acc = None
                for w in range(B_WIN):
                    o = HIST - w * B_DIL
                    p = es[w] * vb_ref[l, j, o:o + seg, :]
                    acc = p if acc is None else acc + p
                cols.append(acc * inv)
            outs.append(_cat(cols, axis=1).astype(BF16))
        return outs

    def b_out(ob, res):
        return res + b_proj(ob, 3)

    def o_store(b, val):
        ro = pl.multiple_of((b + 1) * seg, seg)
        o_ref[pl.ds(ro, val.shape[0]), :] = val.astype(o_ref.dtype)

    def out_copy(b):
        ro = pl.multiple_of(b * seg, seg)
        return pltpu.make_async_copy(o_ref.at[pl.ds(ro + seg, seg), :], out_hbm.at[pl.ds(ro, seg), :], sem_o)

    def step(t, hc, full):
        t_last = n_seg + LAG - 1
        if full:
            jobs = [(0, t - 1), (1, t - 1 - LAG)]

            def b_in():
                return xb_ref[0:2 * seg, :]
        else:
            lb = (t == t_last).astype(jnp.int32)
            jobs = [(lb, t - 1 - lb * (LAG + 1))]

            def b_in():
                return xb_ref[pl.ds(pl.multiple_of(lb * seg, seg), seg), :]
        v0r = _cat([hc[0:n_mem], h_ref[n_mem:M2, :]])
        v1r = _cat([hc[n_mem:M2], h_ref[M2 + n_mem:2 * M2, :]])

        hist = []
        never = t > 4 * n_seg

        def gate(back, z):
            gv = hist[-back]
            return _cat([jnp.where(never, gv, z[e:e + 8]) for e in range(0, z.shape[0], 8)])

        def ktiles(z):
            return [z[:, k * 128:(k + 1) * 128] for k in range(z.shape[1] // 128)]
        if full:
            hl = _Operands(ktiles(_cat([v0r, h_ref[2 * M2:RB, :]])), ktiles(_cat([v1r, h_ref[RB:RB + AH, :]])), None)
        else:
            hl = _Operands(None, None, ktiles(_cat([h_ref[n_mem:M2, :], v1r, h_ref[2 * M2:RB, :]])), F32)
        mh = 2 * M2 if full else 0

        def tile_dot(p, r):
            src = wr_ref.at[p] if r == 0 else w_ref.at[p * NG + r - 1]

            def dot(a, i):
                wt = src[i * 64:(i + 1) * 64, :]
                cnt[0] += 1
                if dl and cnt[0] >= dl[0][0]:
                    deps = dl.pop(0)[1]
                    wt = _cat([jnp.where(never, pltpu.bitcast(d, U32), wt[8 * e:8 * e + 8])
                               for e, d in enumerate(deps)] + [wt[8 * len(deps):]])
                res_ = _nn(a, _upk(wt))
                hist.append(res_[0:8])
                return res_
            return dot
        cnt, dl = [0], []
        scale = float(dh) ** (-0.5) * LOG2E
        if full:
            s_ = t - LAG
            rd = pl.multiple_of(lax.rem(s_ * (seg // 2), RS // 2), seg // 2)
            wa = pl.multiple_of(lax.rem((A0 - R0 + s_ * AH) // 2, RS // 2), 8)

        RA = R if full else n_mem + seg
        CW = R
        bidx = 0 if full else 2
        half = dh - 128
        la8 = lax.broadcasted_iota(jnp.int32, (n_mem, 128), 1) < half
        ones = jnp.full((n_mem, 128), 0xFFFFFFFF, U32)
        zero = jnp.zeros((n_mem, 128), U32)
        mask_a = jnp.where(la8, ones, zero)
        mask_b = jnp.where(la8, zero, ones)

        def pk2(a, b):
            return _pk(_cat([a, b]).astype(BF16))

        yt = [[None] * NT for _ in range(3)]

        def proj(p, r):
            pa, qa = {}, {}
            _fast_mm((S53 if r == 0 else S55)[1], hl, tile_dot(p, r), mh, pa, qa)
            n0 = 0 if r == 0 else RT + (r - 1) * GT
            for n in range(len(pa)):
                y, z, e = _fast_out(pa, qa, n, mh)
                idx = p * NT + n0 + n
                if full:
                    ring_ref[idx, pl.ds(wa, 8), :] = pk2(z[16:24], z[24:32])
                    y = _cat([y[0:M2], z[0:M2], y[M2:2 * M2]])
                else:
                    y = _cat([e[0:8], e])
                yt[p][n0 + n] = stash(p * 16 + (n0 + n) % 16, packed(p, (n0 + n) % 3, y))

        def ab(z8):
            return jnp.where(la8, z8, 0.0), jnp.where(la8, 0.0, z8)

        def packed(p, j, y):
            if p == 0 and (j == 1 or not full):
                return [pltpu.bitcast(y[e:e + 8], U32) for e in range(0 if full else 8, RB, 8)]
            u2 = pk2(y[32:40], y[40:48])
            if p == 0 or j == 0:
                return [pk2(y[0:8], y[8:16]), pk2(y[16:24], y[24:32]), u2]
            if j == 2:
                return [pk2(y[8:16], y[0:8]), pk2(y[24:32], y[16:24]), u2]
            xa_a, xa_b = ab(y[8:16])
            out = [pk2(xa_b, xa_a), pk2(y[24:32], y[16:24]) & mask_b, pk2(y[16:24], y[24:32]) & mask_a, u2]
            if full:
                out += [pk2(*ab(y[0:8]))]
            return out

        def stash(idx, parts):
            kv_ref[idx, 0:8 * len(parts), :] = _cat(parts)
            return lambda: [kv_ref[idx, 8 * e:8 * e + 8, :] for e in range(len(parts))]

        def pair(p, g):
            xs = [ring_ref[p * NT + 3 * g + j, pl.ds(rd, seg // 2), :] for j in range(3)] if full else None
            return [f() for f in yt[p][3 * g:3 * g + 3]], xs

        def q_rows(z, j):
            if not full:
                return pltpu.bitcast(_cat(z[0][j]), F32)
            v0, v1, v2 = z[0][j]
            return mat([v0, z[1][j], v1, v2])

        def kv_tiles(z):
            yt, x1 = z
            v0, v1, v2 = yt[0]
            t0 = [v0] + ([x1[0]] if full else [v1, v2]) + [v1, v2]
            w0, w1, w2 = yt[2]
            t2 = [w0, w1, w2] + ([x1[2]] if full else [w1, w2])
            e1, mb, ma, u2 = yt[1][0:4]
            mid2 = [e1, mb, u2 & mask_b, ma, u2 & mask_a]
            mid1 = None
            if full:
                lo, hi = x1[1][0:8], x1[1][8:16]
                mid1 = [yt[1][4], lo & mask_a, hi & mask_a, lo & mask_b, hi & mask_b]
            return t0, mid1, mid2, t2

        def mat(parts):
            return _upk(_cat(parts))

        def merge(y1, y2):
            return _cat([y1[0:8], y2[0:8], y1[8:40], y2[8:40]])

        def scores(q, k):
            k0, km1, km2, k2_ = kv_tiles(k)
            s_a = _nt(q_rows(q, 0), mat(k0))
            s_b = _nt(q_rows(q, 2), mat(k2_))
            if full:
                f = [pltpu.bitcast(z, F32) for z in q[0][1]]
                s_m = merge(_nt(_cat([f[0], _upk(q[1][1]).astype(F32)]), mat(km1)),
                            _nt(_cat(f[1:]), mat(km2)))
            else:
                s_m = _nt(q_rows(q, 1), mat(km2))
            out = []
            for e, sx in enumerate((s_a, s_b)):
                s = (sx + s_m) * scale + bias_ref[bidx + e, 0:RA, 0:CW]
                ex = jnp.exp2(s - jnp.max(s, axis=-1, keepdims=True))
                out.append(ex * _recip(jnp.sum(ex, axis=-1, keepdims=True)))
            return out

        def pv(p, v):
            PD = F32 if (PF or not full) else BF16
            v0, vm1, vm2, v2 = kv_tiles(v)
            o_a = _nn(p[0].astype(PD), mat(v0))
            o_b = _nn(p[1].astype(PD), mat(v2))
            p = p[0] + p[1]
            if full:
                o_m = merge(_nn(_cat([p[0:8], p[16:48]]), mat(vm1)), _nn(_cat([p[8:16], p[48:80]]), mat(vm2)))
            else:
                o_m = _nn(p.astype(PD), mat(vm2))
            return [o_a, o_m, o_b]

        ot = []
        pacc, qacc = {}, {}
        mo = n_mem + seg if (full and WF) else mh

        def add_o(r):
            n0 = 0 if r == 0 else RT + (r - 1) * GT
            oo = ot[n0:n0 + (RT if r == 0 else GT)]
            if full and WF:
                us = [_cat([o[48:56], o[8:16], o[56:80]]) for o in oo]
                if r < TAILPV and GATE_O:
                    us = [gate(GATE_O, z) for z in us]
                ops = _Operands([_cat([o[0:8], o[16:48]]) for o in oo], us, None, F32)
            elif full:
                us = [_cat([o[48:64], o[32:48]]) for o in oo]
                if r < TAILPV:
                    us = [gate(GATE_O, z) for z in us]
                ops = _Operands([o[0:32] for o in oo], us, [o[64:80] for o in oo])
            else:
                ops = _Operands(None, None, oo, F32)
            _fast_mm((S35 if r == 0 else S55)[1], ops, tile_dot(3, r), mo, pacc, qacc)

        bqkv = [None] * 3
        probs = []

        def do_pv():
            for g in range(len(ot) // 3, len(probs)):
                ot.extend(pv(probs[g], pair(2, g)))

        if full:
            an = pl.multiple_of(jnp.minimum(A0 + (s_ + 1) * AH, S - AH), AH)
            h_ref[RB:RB + AH, :] = _ln(x_ref[pl.ds(an, AH), :].astype(F32))

        for r in range(NG + 1):
            proj(2, r)
            proj(1, r)
            proj(0, r)
            if r == 0:
                blhs = _ln(b_in())
            if r < 3:
                bqkv[2 - r] = b_proj(blhs, 2 - r)
            if r == 3:
                ob = b_attn(jobs, *bqkv)
            if r == BOUT_R:
                zb = b_out(_cat(ob), b_in())
                x2_new = zb[0:seg]
                if full:
                    o_store(t - 1 - LAG, zb[seg:2 * seg])
                    nxt = x2_new
                else:
                    o_store(lb * (t_last - LAG - 1) - 1, x2_new)
                    nxt = jnp.where(t < LAG - 1, x_ref[seg:2 * seg, :].astype(F32), x2_new)
                sl = _ln(nxt)
                h_ref[n_mem:M2, :] = sl[0:n_mem]
                h_ref[M2 + n_mem:RB, :] = sl[n_mem:seg]
                if full:
                    for j in range(nct):
                        dl.append((cnt[0] + DUE_LN + 2 * j, [sl[e:e + 8, j * 128:(j + 1) * 128] for e in range(0, seg, 8)]))
            if r in WSCHED:
                add_o(WSCHED[r])
            do_pv()
            for g in range(len(probs), (RT + r * GT) // 3):
                probs.append(scores(pair(0, g), pair(1, g)))
        for r in range(len(WSCHED), TAILPV):
            add_o(r)
        do_pv()
        for r in range(TAILPV, NG + 1):
            add_o(r)
        cols = []
        for n in range(nct):
            y, z, e = _fast_out(pacc, qacc, n, mo)
            if full and WF:
                cols.append(_cat([y[0:8], z[8:16], y[8:40], z[0:8], z[16:40]]))
            else:
                cols.append(_cat([y, z[16:32], z[0:16], e]) if full else e)
        acc = _cat(cols, axis=1)

        xa0 = n_mem if full else 0
        y2 = x2_ref[...] + _cat([acc[xa0:xa0 + n_mem], acc[RA - seg + n_mem:RA]])
        mem2 = acc[RA - seg:RA - seg + n_mem]
        if full:
            x_cur = x_ref[pl.ds(pl.multiple_of(t * seg, seg), seg), :].astype(F32)
            xb_ref[0:seg, :] = x_cur + acc[M2:M2 + seg]
            xb_ref[seg:2 * seg, :] = y2
            m1n = acc[0:n_mem]
            m2n = mem2
        else:
            xb_ref[pl.ds(pl.multiple_of(jnp.where(t < LAG, 0, (t - n_seg + 2) * seg), seg), seg), :] = y2
            m1n = mem2
            m2n = jnp.where(t == LAG - 1, mem0_ref[...].astype(F32), mem2)
        x2_ref[...] = nxt
        return _cat([m1n, m2n])

    def single_body(t, c):
        @pl.when(t == n_seg)
        def _():
            out_copy(t - (LAG + 2)).start()
        return step(t, c, False)

    def full_body(t, c):
        @pl.when(t >= LAG + 2)
        def _():
            out_copy(t - (LAG + 2)).start()
        return step(t, c, True)

    def phase(ph, c):
        t0 = ph * n_seg
        c = lax.fori_loop(t0, t0 + LAG, single_body, c)

        @pl.when(ph == 0)
        def _():
            x_late.wait()
        return lax.fori_loop(LAG, jnp.where(ph == 0, n_seg, LAG), full_body, c)
    lax.fori_loop(0, 2, phase, _cat([mem0_ref[...].astype(F32)] * 2))

    out_copy(n_seg - 3).start()
    res = xb_ref[2 * seg:4 * seg, :]
    blhs = _ln(res)
    ob = b_attn([(1, n_seg - 2), (1, n_seg - 1)], *[b_proj(blhs, part) for part in range(3)])
    o_store(n_seg - 2, b_out(_cat(ob), res))
    out_copy(n_seg - 2).start()
    out_copy(n_seg - 1).start()
    pltpu.make_async_copy(o_ref.at[pl.ds(seg, S), :], out_hbm, sem_o).wait()


@functools.partial(jax.jit, static_argnames=("seg",))
def _run(A_x, A_mem0, A_Wq, A_Wk, A_Wv, A_Wo, B_wqkv, B_wo, *, seg):
    _, S, dm = A_x.shape
    n_heads, dh = A_Wq.shape[1], A_Wq.shape[2]
    n_mem = A_mem0.shape[1]
    n_seg = S // seg
    hd = n_heads * dh
    nct = dm // 128
    ng = (hd // 128 - RT) // GT
    assert (seg, n_seg, n_mem, dh, dm % 128, n_heads, LAG) == (32, 64, 8, 192, 0, 32, 2)

    x = A_x.reshape(S, dm)
    mem0 = A_mem0.reshape(n_mem, dm)
    wq = jnp.transpose(A_Wq, (1, 2, 0)).reshape(hd, dm)
    wk = jnp.transpose(A_Wk, (1, 2, 0)).reshape(hd, dm)
    wv = jnp.transpose(A_Wv, (1, 2, 0)).reshape(hd, dm)
    wo = A_Wo.reshape(hd, dm)
    _, _, _, _, rs, xc = _plan(seg, n_seg)

    kern = functools.partial(_kernel, seg=seg, n_seg=n_seg, n_mem=n_mem,
                             n_heads=n_heads, dh=dh, dm=dm)
    hbm = pl.BlockSpec(memory_space=pltpu.HBM)

    out = pl.pallas_call(
        kern,
        in_specs=[hbm] * 8,
        out_specs=hbm,
        out_shape=jax.ShapeDtypeStruct((S, dm), A_x.dtype),
        scratch_shapes=[
            pltpu.VMEM((S, dm), BF16),
            pltpu.VMEM((n_mem, dm), BF16),
            pltpu.VMEM((NSLOT, 4, GT * 128, dm), BF16),
            pltpu.VMEM((RT * 128, dm), BF16),
            pltpu.VMEM((4, len(S53[0]) * 64, 128), U32),
            pltpu.VMEM((4 * ng, len(S55[0]) * 64, 128), U32),
            pltpu.VMEM((dm, 4 * dm + 128), BF16),
            pltpu.VMEM((nct, 4 * dm + 32, 128), F32),
            pltpu.VMEM((4 * nct, dm // 2, 128), U32),
            pltpu.VMEM((len(KEYS_R), HC * xc // 4, 128), U32),
            pltpu.VMEM((len(KEYS_R), HC * xc // 4, 128), U32),
            pltpu.VMEM((len(KEYS) - len(KEYS_R), NXC * xc // 4, 128), U32),
            pltpu.VMEM((len(KEYS), 8, 128), U32),
            pltpu.VMEM((3 * hd // 128, rs // 2, 128), U32),
            pltpu.VMEM((2 * n_mem + seg + AH, dm), F32),
            pltpu.VMEM((4 * seg, dm), F32),
            pltpu.VMEM((seg, dm), F32),
            pltpu.VMEM((2, nct, HIST + seg, 128), F32),
            pltpu.VMEM((2, nct, HIST + seg, 128), F32),
            pltpu.VMEM((S + seg, dm), A_x.dtype),
            pltpu.VMEM((4, 2 * n_mem + 2 * seg, 128), F32),
            pltpu.VMEM((48, 48, 128), U32),
            pltpu.VMEM((len(S55[0]) * 64, 128), U32),
            pltpu.SemaphoreType.DMA((NSLOT,)),
            pltpu.SemaphoreType.DMA((8 + NXC,)),
            pltpu.SemaphoreType.DMA((4,)),
            pltpu.SemaphoreType.DMA(()),
        ],
        compiler_params=pltpu.CompilerParams(
            vmem_limit_bytes=127 * 1024 * 1024,
            disable_bounds_checks=True,
        ),
    )(x, mem0, wq, wk, wv, wo, B_wqkv, B_wo)
    return out.reshape(1, S, dm)


def pallas_interleave_layers__memory_aug_recurrent_mem_tr__sliding_local_dilated__prompt_kernel(
    A_x: jax.Array,
    A_mem0: jax.Array,
    A_Wq: jax.Array,
    A_Wk: jax.Array,
    A_Wv: jax.Array,
    A_Wo: jax.Array,
    A_seg_len,
    B_x: jax.Array,
    B_wqkv: jax.Array,
    B_wo: jax.Array,
):
    del B_x
    seg = A_seg_len if isinstance(A_seg_len, int) else 32
    return _run(A_x, A_mem0, A_Wq, A_Wk, A_Wv, A_Wo, B_wqkv, B_wo, seg=seg)
```

```python
import functools

import jax
import jax.numpy as jnp
from jax import lax
import jax.experimental.pallas as pl
import jax.experimental.pallas.tpu as pltpu

F32 = jnp.float32
BF16 = jnp.bfloat16
U32 = jnp.uint32
NEG = -1000000000.0
LN_EPS = 1e-05
LOG2E = 1.4426950408889634
NEG2 = NEG * LOG2E

B_HEADS = 32
B_WIN = 8
B_DIL = 2
HIST = 16
AH = 16
LAG = 2
NSLOT = 2
NXC = 6
HC = 3
WSCHED = {3: 0, 4: 1, 6: 2, 7: 3, 8: 4, 9: 5}
BOUT_R = 5
TAILPV = 8
GATE_O = 50
DUE_LN = 150
DUE_X = 24
DUE_B0, DUE_B = 100, 60


def _ln(x):
    m = jnp.mean(x, axis=-1, keepdims=True)
    c = x - m
    v = jnp.mean(c * c, axis=-1, keepdims=True)
    return c * lax.rsqrt(v + LN_EPS)


def _recip(d):
    return pl.reciprocal(d, approx=True)


def _nt(a, b):
    return lax.dot_general(a, b, (((1,), (1,)), ((), ())), preferred_element_type=F32)


def _nn(a, b):
    return lax.dot_general(a, b, (((1,), (0,)), ((), ())), preferred_element_type=F32)


def _cat(xs, axis=0):
    return xs[0] if len(xs) == 1 else jnp.concatenate(xs, axis=axis)


def _pk(z):
    return pltpu.bitcast(z, U32)


def _upk(z):
    return pltpu.bitcast(z, BF16)


LAM = (-1.5, -0.5, 0.0, 0.5, 1.5)


def _scheme(stars):
    tiles, prog = [], []
    for star in stars:
        if len(star) == 1:
            prog.append(("single", star[0], None, len(tiles)))
            tiles.append([star[0][:2]])
            continue
        left = [len(star) - 1] * len(star)
        for j in range(1, len(star)):
            for i in range(j):
                x, y = star[i], star[j]
                prog.append(("pair", x, y, len(tiles)))
                tiles += [[(x[0], y[1])], [(y[0], x[1])], [(x[0], y[1]), (y[0], x[1])]]
                for e in (i, j):
                    left[e] -= 1
                    if left[e] == 0:
                        z = star[e]
                        prog.append(("diag", z, None, len(tiles)))
                        tiles += [[z[:2]] + [(o[0], z[1]) for o in star if o is not z],
                                  [z[:2]] + [(z[0], o[1]) for o in star if o is not z]]
    return tiles, prog


S55 = _scheme([[(i, i, LAM[i]) for i in range(5)]])
S53 = _scheme([[(0, 0, LAM[0]), (2, 1, LAM[2]), (4, 2, LAM[4])], [(1, 0, LAM[1]), (3, 2, LAM[3])],
               [(1, 1, LAM[1])], [(3, 1, LAM[3])]])
S35 = _scheme([[(0, 0, LAM[0]), (1, 2, LAM[2]), (2, 4, LAM[4])], [(0, 1, LAM[1]), (2, 3, LAM[3])],
               [(1, 1, LAM[1])], [(1, 3, LAM[3])]])


def _spread(prog):
    pairs = [e for e in prog if e[0] != "diag"]
    diags = [e for e in prog if e[0] == "diag"]
    out, k = [], 0
    for i, e in enumerate(pairs):
        out.append(e)
        while k < len(diags) and (k + 0.5) * len(pairs) <= (i + 1) * len(diags):
            out.append(diags[k])
            k += 1
    return out + diags[k:]


def _op_keys(prog):
    keys = []
    for kind, x, y, _ in prog:
        if kind == "pair":
            new = [(nm, x[0], x[2], y[0], y[2]) for nm in ("l1", "l2", "A")]
        else:
            new = [("a", x[0], x[2]), ("b", x[0])]
        keys += [k for k in new if k not in keys]
    return keys


def _scaled(c, u):
    return u if c == 1.0 else c * u


class _Operands:
    def __init__(self, T, U, E, dtype=BF16):
        self.T, self.U, self.E, self.memo, self.dtype = T, U, E, {}, dtype

    def _get(self, key, fn):
        if key not in self.memo:
            self.memo[key] = fn()
        return self.memo[key]

    def paired(self, key):
        T, U = self.T, self.U
        if key[0] == "b":
            return U[key[1]]
        if key[0] == "a":
            k, lam = key[1:]
            if lam == 0.0:
                return T[k]
            return self._get(("f",) + key, lambda: T[k] - _scaled(lam, U[k]) if lam > 0
                             else T[k] + _scaled(-lam, U[k]))
        kx, lx, ky, ly = key[1:]
        A = self._get(("f", "A") + key[1:],
                      lambda: self.paired(("a", kx, lx)) + self.paired(("a", ky, ly)))
        if key[0] == "A":
            return A
        return A - _scaled(ly - lx, U[kx]) if key[0] == "l1" else A + _scaled(ly - lx, U[ky])

    def extra(self, key):
        if key[0] == "a":
            return self.E[key[1]]
        return self._get(("e", key[1], key[3]), lambda: self.E[key[1]] + self.E[key[3]])

    def __call__(self, key):
        if self.T is None:
            ek = ("a", key[1]) if key[0] in ("a", "s") else ("l", key[1], 0, key[3])
            return self._get(ek, lambda: self.extra(ek).astype(self.dtype))

        def build():
            ak = ("a",) + key[1:] if key[0] == "s" else key
            parts = [self.paired(ak)]
            if self.E is not None and ak[0] in ("a", "l1", "l2"):
                parts.append(self.extra(ak))
            if key[0] == "s":
                parts.append(self.U[key[1]])
            return _cat(parts).astype(self.dtype)
        return self._get(key, build)


def _fast_mm(prog, op, dot, m, p, q):
    def add(d, key, val):
        d[key] = val if key not in d else d[key] + val

    for kind, x, y, i in prog:
        if kind == "pair":
            kk = (x[0], x[2], y[0], y[2])
            p1, p2 = dot(op(("l1",) + kk), i), dot(op(("l2",) + kk), i + 1)
            if m:
                r = _scaled(1.0 / (y[2] - x[2]), p2[0:m] - p1[0:m] + dot(op(("A",) + kk), i + 2))
                add(q, (x[1], x[2]), r)
                add(q, (y[1], y[2]), r)
            add(p, y[1], p1)
            add(p, x[1], p2)
        elif kind == "diag":
            add(p, x[1], dot(op(("a", x[0], x[2])), i))
            if m:
                add(q, (x[1], x[2]), dot(op(("b", x[0])), i + 1))
        else:
            r = dot(op(("s", x[0], x[2])), i)
            add(p, x[1], r[0:r.shape[0] - m])
            if m:
                add(q, (x[1], x[2]), r[r.shape[0] - m:])


def _fast_out(p, q, n, m):
    if not m:
        return None, None, p[n]
    y, z = p[n][0:m], None
    for (nn, lam), v in q.items():
        if nn == n:
            z = v if z is None else z + v
            if lam != 0.0:
                y = y + _scaled(lam, v) if lam > 0 else y - _scaled(-lam, v)
    return y, z, (p[n][m:] if p[n].shape[0] > m else None)


def _combo(tile, block):
    out = block(*tile[0])
    for kn in tile[1:]:
        out = out - block(*kn)
    return out


GT = 5
RT = 3
KEYS_R = _op_keys(S53[1])
KEYS = KEYS_R + [k for k in _op_keys(S55[1]) if k not in KEYS_R]


def _plan(seg, n_seg):
    S = seg * n_seg
    R0 = LAG * seg
    A0 = S - (n_seg - LAG) * AH
    NPRE = A0 - R0
    RS = -(-(A0 - R0 + AH) // seg) * seg
    XC = NPRE // NXC // 32 * 32
    assert XC * NXC + 32 == NPRE
    return S, R0, A0, NPRE, RS, XC


def _kernel(x_hbm, mem0_hbm, wq_hbm, wk_hbm, wv_hbm, wo_hbm, bqkv_hbm, bwo_hbm,
            out_hbm,
            x_ref, mem0_ref, stage_ref, stage0_ref, wr_ref, w_ref, bst_ref, btmp_ref, bw_ref,
            xla_ref, xlb_ref, xlc_ref, xe_ref, ring_ref, h_ref, xb_ref, x2_ref, kb_ref, vb_ref, o_ref, bias_ref, kv_ref, bwf_ref,
            sem_w, sem_m, sem_b, sem_o,
            *, seg, n_seg, n_mem, n_heads, dh, dm):
    S, R0, A0, NPRE, RS, XC = _plan(seg, n_seg)
    M2 = 2 * n_mem
    R = M2 + 2 * seg
    RB = M2 + seg
    nct = dm // 128
    bdh = dm // B_HEADS
    NT = n_heads * dh // 128
    NG = (NT - RT) // GT
    w_hbm = (wq_hbm, wk_hbm, wv_hbm, wo_hbm)

    def w_copy(p, g):
        slot = g & (NSLOT - 1)
        return pltpu.make_async_copy(w_hbm[p].at[pl.ds((RT + (g - 1) * GT) * 128, GT * 128), :],
                                     stage_ref.at[slot, p], sem_w.at[slot])

    def w0_copy(p):
        dst = stage0_ref if p == 3 else stage_ref.at[0, p, pl.ds(0, RT * 128)]
        return pltpu.make_async_copy(w_hbm[p].at[pl.ds(0, RT * 128), :], dst, sem_m.at[4 + p])

    NB1 = 3 * nct
    WO0 = 3 * dm
    XF = A0 + AH
    XH = XC // 2

    def rows_copy(r0, n, sem):
        return pltpu.make_async_copy(x_hbm.at[pl.ds(r0, n), :], x_ref.at[pl.ds(r0, n), :], sem)

    def x_copy(i):
        return rows_copy(pl.multiple_of(R0 + i * XC, 16), XC, sem_m.at[8 + i])

    small = [rows_copy(0, R0, sem_m.at[1]), rows_copy(R0 + NPRE - 32, XF - R0 - NPRE + 32, sem_m.at[2]),
             pltpu.make_async_copy(mem0_hbm, mem0_ref, sem_m.at[3])]
    x_late = rows_copy(XF, S - XF, sem_m.at[0])

    def bq_copy(part):
        c0 = pl.multiple_of(part * dm, 128)
        return pltpu.make_async_copy(bqkv_hbm.at[:, pl.ds(c0, dm)], bst_ref.at[:, pl.ds(c0, dm)], sem_b.at[part])

    bo_copy = pltpu.make_async_copy(bwo_hbm, bst_ref.at[:, pl.ds(3 * dm, dm)], sem_b.at[3])

    def bst_tile(c):
        return bst_ref[:, pl.ds(pl.multiple_of(c * 128, 128), 128)]

    def bias_tables(full):
        RA = R if full else n_mem + seg
        CW = 128
        ri = lax.broadcasted_iota(jnp.int32, (RA, CW), 0)
        ci = lax.broadcasted_iota(jnp.int32, (RA, CW), 1)
        if not full:
            ri = jnp.where(ri >= n_mem, ri + n_mem + seg, ri + n_mem)

        def table(i, bounds, vals):
            out = vals[-1]
            for b, v in zip(reversed(bounds), reversed(vals[:-1])):
                out = jnp.where(i < b, v, out)
            return out
        qi = ri - table(ri, [16, 48, 56], [0, 8, 48, 40])
        g0 = (ci < 8) | ((ci >= 16) & (ci < 48))
        k2 = ci - table(ci, [8, 24, 32, 48, 56], [-8, 0, 24, 8, 48, 40])
        if full:
            k1 = ci - table(ci, [8, 48], [0, 8, 40])
            row_l2 = ((ri >= 8) & (ri < 16)) | (ri >= 48)
            is_a = g0 != row_l2
            ki = jnp.where(row_l2, k2, k1)
        else:
            is_a = jnp.logical_not(g0)
            ki = k2
        visible = (qi < n_mem) | (qi >= ki)
        fill = NEG2
        for e, mine in enumerate((is_a, jnp.logical_not(is_a))):
            bias_ref[(0 if full else 2) + e, 0:RA, :] = jnp.where(
                mine, jnp.where(visible, 0.0, fill), -jnp.inf)

    for i in range(HC):
        x_copy(i).start()

    def zero_body(j, c):
        btmp_ref[j, 0:dm, :] = jnp.zeros((dm, 128), F32)
        return c
    lax.fori_loop(0, nct, zero_body, 0)

    w0_copy(0).start()
    xb_ref[0:2 * seg, :] = jnp.zeros((2 * seg, dm), F32)
    kb_ref[...] = jnp.zeros(kb_ref.shape, F32)
    vb_ref[...] = jnp.zeros(vb_ref.shape, F32)
    bst_ref[:, 4 * dm:] = jnp.zeros((dm, 128), BF16)
    bias_tables(True)
    bias_tables(False)

    def e_ops():
        ye = _ln(x_ref[R0 + NPRE - 32:R0 + NPRE, :].astype(F32))
        eops = _Operands([ye[0:16, k * 128:(k + 1) * 128] for k in range(nct)],
                         [ye[16:32, k * 128:(k + 1) * 128] for k in range(nct)], None)
        for j, key in enumerate(KEYS):
            xe_ref[j] = _pk(eops(key))

    NKR = len(KEYS_R)

    def xl(j, hf, i):
        if j >= NKR:
            ref, j, i = xlc_ref, j - NKR, hf * HC + i
        else:
            ref = (xla_ref, xlb_ref)[hf]
        r0 = i * (XH // 2)
        return ref.at[j, pl.ds(r0 if isinstance(r0, int) else pl.multiple_of(r0, 8), XH // 2)]

    def ln_ops(hf, i, lo, hi):
        y = _ln(x_ref[pl.ds(pl.multiple_of(R0 + (hf * HC + i) * XC, 16), XC), :].astype(F32))
        ops = _Operands([y[0:XH, k * 128:(k + 1) * 128] for k in range(nct)],
                        [y[XH:XC, k * 128:(k + 1) * 128] for k in range(nct)], None)
        vals = []
        for j in range(lo, hi):
            v = _pk(ops(KEYS[j]))
            xl(j, hf, i)[...] = v
            vals.append([v[e:e + 8] for e in range(0, XH // 2, 8)])
        return vals

    def ln_body(i, c):
        x_copy(i).wait()

        @pl.when(i == 0)
        def _():
            x_copy(HC).start()

        @pl.when(i == 1)
        def _():
            w0_copy(1).start()
            w0_copy(2).start()

        @pl.when(i == 2)
        def _():
            x_copy(HC + 1).start()
            x_copy(HC + 2).start()
            for cp in small:
                cp.start()
        ln_ops(0, i, 0, len(KEYS_R))
        return c
    lax.fori_loop(0, HC, ln_body, 0)

    def prep(scheme, w, dst):
        raw = lambda k, n: w[n * 128:(n + 1) * 128, k * 128:(k + 1) * 128]
        tb = []
        for i, tl in enumerate(scheme[0]):
            tb.append(raw(*tl[0]) if len(tl) == 1
                      else _combo(tl, lambda k, n: raw(k, n).astype(F32)).astype(BF16))
            dst[i * 64:(i + 1) * 64, :] = _pk(tb[i].T)
        return tb

    pcnt, pdl = [0], []

    def pre_chunk(scheme, w, dst, n0, chunks, never=None, tb=None):
        tiles, prog = scheme
        prog = _spread(prog)
        dot = lambda a, i: _nn(a, _upk(dst[i * 64:(i + 1) * 64, :]))
        if w is not None:
            if tb is None:
                tb = prep(scheme, w, dst)
            dot = lambda a, i: _nt(a, tb[i])

        for cs in chunks:
            def op(key):
                def ld(kk):
                    v = [xl(KEYS.index(kk), c // HC, c % HC)[...] for c in cs]
                    if NXC - 1 in cs:
                        v.append(xe_ref[KEYS.index(kk)])
                    return _cat(v)
                if key[0] == "s":
                    return _upk(_cat([ld(("a",) + key[1:]), ld(("b", key[1]))]))
                v = ld(key)
                pcnt[0] += len(cs)
                if pdl and pcnt[0] >= pdl[0][0]:
                    deps = pdl.pop(0)[1]
                    v = _cat([jnp.where(never, d, v[8 * e:8 * e + 8]) for e, d in enumerate(deps)]
                             + ([v[8 * len(deps):]] if v.shape[0] > 8 * len(deps) else []))
                return _upk(v)
            p, q = {}, {}
            m = XH * len(cs) + (16 if NXC - 1 in cs else 0)
            _fast_mm(prog, op, dot, m, p, q)
            for n in range(len(p)):
                y, z, e = _fast_out(p, q, n, m)
                for ic, c in enumerate(cs):
                    ring_ref[n0 + n, c * XH:c * XH + XH // 2, :] = _pk(y[ic * XH:(ic + 1) * XH].astype(BF16))
                    ring_ref[n0 + n, c * XH + XH // 2:(c + 1) * XH, :] = _pk(z[ic * XH:(ic + 1) * XH].astype(BF16))
                if NXC - 1 in cs:
                    ring_ref[n0 + n, NXC * XH:NXC * XH + 16, :] = _pk(_cat([y[m - 16:m], z[m - 16:m]]).astype(BF16))

    def init_rows():
        x0 = x_ref[0:seg, :].astype(F32)
        sl = _ln(x0)
        xt = _ln(x_ref[R0 + NPRE:XF, :].astype(F32))
        h_ref[n_mem:M2, :] = sl[0:n_mem]
        h_ref[M2 + n_mem:RB, :] = sl[n_mem:seg]
        h_ref[RB:RB + AH, :] = xt
        x2_ref[...] = x0

    def first_a(p, c):
        buf = stage_ref.at[0, p, pl.ds(0, RT * 128)]
        pltpu.make_async_copy(buf, buf, sem_m.at[4 + p]).wait()
        x_copy(HC + p).wait()

        @pl.when(p == 0)
        def _():
            for pp in range(4):
                w_copy(pp, 1).start()

        @pl.when(p == 2)
        def _():
            bq_copy(0).start()
        vals = ln_ops(1, p, 0, len(KEYS))
        pcnt[0] = 0
        pdl.extend((DUE_X + e, d) for e, d in enumerate(vals))
        pre_chunk(S53, buf, wr_ref.at[p], p * NT, [[c] for c in range(HC)], p > 9)
        del pdl[:]
        return c
    lax.fori_loop(0, 3, first_a, 0)
    for cp in small:
        cp.wait()

    def first_b(p, c):
        e_ops()
        init_rows()
        vals = ln_ops(0, p, len(KEYS_R), len(KEYS))
        pcnt[0] = 0
        pdl.extend((DUE_X + 2 * e, d) for e, d in enumerate(vals))
        pre_chunk(S53, None, wr_ref.at[p], p * NT, [[c] for c in range(HC, NXC)], p > 9)
        del pdl[:]
        return c
    lax.fori_loop(0, 3, first_b, 0)

    dpt = 128 // B_HEADS

    def b_stage1(u):
        uc = jnp.clip(u, 0, NB1 - 1)
        tr = bst_tile(jnp.where(u >= 0, uc, NB1 + nct)).astype(F32).T
        r0 = pl.multiple_of(uc * 128, 128)
        for j in range(nct):
            btmp_ref[j, pl.ds(r0, 128), :] = tr[:, j * 128:(j + 1) * 128]
        return [pltpu.bitcast(tr[120:128, j * 128:(j + 1) * 128], U32) for j in range(nct)]

    def b_stage1_wo(u):
        uc = jnp.clip(u, 0, nct - 1)
        btmp_ref[uc, WO0:WO0 + dm, :] = bst_tile(jnp.where(u >= 0, NB1 + uc, NB1 + nct)).astype(F32)

    def b_stage2(u):
        uc = jnp.clip(u, 0, NB1 - 1)
        part = (uc >= nct).astype(jnp.int32) + (uc >= 2 * nct).astype(jnp.int32)
        r0 = part * dm + (uc - part * nct) * dpt
        rows = _cat([_cat([btmp_ref[j, pl.ds(r0 + dd, B_HEADS, stride=bdh), :]
                           for j in range(nct)], axis=1) for dd in range(dpt)])
        val = _pk(rows.T.astype(BF16))
        bw_ref[uc] = val
        return [val[64 * j + 56:64 * j + 64] for j in range(nct)]

    def b_stage2_wo(u):
        uc = jnp.clip(u, 0, nct - 1)
        r0 = jnp.where(u >= 0, WO0, 0)
        bw_ref[NB1 + uc] = _pk(
            _cat([btmp_ref[uc, pl.ds(r0 + d, B_HEADS, stride=bdh), :] for d in range(bdh)]).astype(BF16))

    def wo_store(scheme, w, dst, never=None):
        if scheme is S55:
            rawt = lambda k, n: w[k * 128:(k + 1) * 128, n * 128:(n + 1) * 128]
            plain = [i for i, tl in enumerate(scheme[0]) if len(tl) == 1]
            for i, tl in enumerate(scheme[0]):
                if len(tl) > 1:
                    val = _combo(tl, lambda k, n: rawt(k, n).astype(F32)).astype(BF16)
                    val = _pk(_upk(_pk(val.T)).T)
                    dst[i * 64:(i + 1) * 64, :] = val
                    j = plain.pop()
                    pv_ = _pk(rawt(*scheme[0][j][0]))
                    dst[j * 64:(j + 1) * 64, :] = jnp.where(never, val, pv_)
            return
        for r in range(0, 128, 16):
            memo = {}

            def raw(k, n):
                return w[k * 128 + r:k * 128 + r + 16, n * 128:(n + 1) * 128]

            def block(k, n):
                if (k, n) not in memo:
                    memo[k, n] = raw(k, n).astype(F32)
                return memo[k, n]
            for i, tl in enumerate(scheme[0]):
                val = raw(*tl[0]) if len(tl) == 1 else _combo(tl, block).astype(BF16)
                dst[i * 64 + r // 2:i * 64 + r // 2 + 8, :] = _pk(val)

    def pre_body(g, c):
        slot = g & (NSLOT - 1)
        buf = stage_ref.at[slot]
        pltpu.make_async_copy(buf, buf, sem_w.at[slot]).wait()

        @pl.when((g >= 2) & (g <= 4))
        def _():
            bq_copy(g - 2).wait()

        @pl.when(g == 4)
        def _():
            bo_copy.wait()

        @pl.when(g <= 2)
        def _():
            bq_copy(g).start()

        @pl.when(g == 2)
        def _():
            bo_copy.start()

        @pl.when(g + 1 <= NG)
        def _():
            for p in range(4):
                w_copy(p, g + 1).start()

        @pl.when(g == NG - 1)
        def _():
            w0_copy(3).start()
            x_late.start()

        wo_store(S55, stage_ref.at[slot, 3], w_ref.at[3 * NG + g - 1], g > NG + 5)
        deps = [b_stage2(3 * (g - 5) + e) for e in range(3)]
        b_stage2_wo(g - 5)
        deps += [b_stage1(3 * (g - 2) + e) for e in range(3)]
        b_stage1_wo(g - 4)
        pcnt[0] = 0
        pdl.extend((DUE_B0 + DUE_B * e, d) for e, d in enumerate(deps))
        tbs = [prep(S55, stage_ref.at[slot, 0], w_ref.at[g - 1])]
        for p in range(3):
            if p < 2:
                tbs.append(prep(S55, stage_ref.at[slot, p + 1], w_ref.at[(p + 1) * NG + g - 1]))
            pre_chunk(S55, stage_ref.at[slot, p], w_ref.at[p * NG + g - 1], p * NT + RT + (g - 1) * GT, [[0, 1, 2], [3], [4], [5]],
                      g > NG + 5, tbs[p])
        return c
    lax.fori_loop(1, NG + 1, pre_body, 0)
    w0_copy(3).wait()
    wo_store(S35, stage0_ref, wr_ref.at[3])

    for r in range(0, 64, 8):
        def raw(k, n):
            return bw_ref[2 * nct + n, k * 64 + r:k * 64 + r + 8, :]
        blocks = {(k, n): _upk(raw(k, n)).astype(F32) for k in range(nct) for n in range(nct)}
        for i, tl in enumerate(S55[0]):
            val = raw(*tl[0]) if len(tl) == 1 else _pk(_combo(tl, lambda k, n: blocks[k, n]).astype(BF16))
            bwf_ref[i * 64 + r:i * 64 + r + 8, :] = val

    bscale = float(bdh) ** (-0.5) * LOG2E

    def b_proj(lhs, part):
        if part == 2 and lhs.shape[0] == 2 * seg:
            kt = lambda a: [a[:, k * 128:(k + 1) * 128] for k in range(nct)]
            ops = _Operands(kt(lhs[0:seg]), kt(lhs[seg:2 * seg]), None, F32)
            p, q = {}, {}
            _fast_mm(S55[1], ops, lambda a, i: _nn(a, _upk(bwf_ref[i * 64:(i + 1) * 64, :])), seg, p, q)
            return _cat([_cat(_fast_out(p, q, n, seg)[0:2]) for n in range(nct)], axis=1)
        return _nn(lhs.astype(BF16), _cat([_upk(bw_ref[part * nct + j]) for j in range(nct)], axis=1))

    def b_attn(jobs, q, k, v):
        row = lax.broadcasted_iota(jnp.int32, (seg, 128), 0)
        outs = []
        for i, (l, sidx) in enumerate(jobs):
            r0 = i * seg
            pos = row + sidx * seg
            for j in range(nct):
                kb_ref[l, j, 0:HIST, :] = kb_ref[l, j, seg:seg + HIST, :]
                vb_ref[l, j, 0:HIST, :] = vb_ref[l, j, seg:seg + HIST, :]
            for j in range(nct):
                kb_ref[l, j, HIST:HIST + seg, :] = k[r0:r0 + seg, j * 128:(j + 1) * 128]
                vb_ref[l, j, HIST:HIST + seg, :] = v[r0:r0 + seg, j * 128:(j + 1) * 128]
            logits = []
            for w in range(B_WIN):
                o = HIST - w * B_DIL
                acc = None
                for j in range(nct):
                    p = q[r0:r0 + seg, j * 128:(j + 1) * 128] * kb_ref[l, j, o:o + seg, :]
                    acc = p if acc is None else acc + p
                acc = acc + pltpu.roll(acc, 64, 1)
                acc = acc + pltpu.roll(acc, 32, 1)
                lg = acc * bscale
                if w > 0:
                    lg = jnp.where(pos >= w * B_DIL, lg, NEG2)
                logits.append(lg)
            m = logits[0]
            for w in range(1, B_WIN):
                m = jnp.maximum(m, logits[w])
            es = [jnp.exp2(lg - m) for lg in logits]
            den = es[0]
            for w in range(1, B_WIN):
                den = den + es[w]
            inv = _recip(den)
            cols = []
            for j in range(nct):
                acc = None
                for w in range(B_WIN):
                    o = HIST - w * B_DIL
                    p = es[w] * vb_ref[l, j, o:o + seg, :]
                    acc = p if acc is None else acc + p
                cols.append(acc * inv)
            outs.append(_cat(cols, axis=1).astype(BF16))
        return outs

    def b_out(ob, res):
        return res + b_proj(ob, 3)

    def o_store(b, val):
        ro = pl.multiple_of((b + 1) * seg, seg)
        o_ref[pl.ds(ro, val.shape[0]), :] = val.astype(o_ref.dtype)

    def out_copy(b):
        ro = pl.multiple_of(b * seg, seg)
        return pltpu.make_async_copy(o_ref.at[pl.ds(ro + seg, seg), :], out_hbm.at[pl.ds(ro, seg), :], sem_o)

    def step(t, hc, full):
        t_last = n_seg + LAG - 1
        if full:
            jobs = [(0, t - 1), (1, t - 1 - LAG)]

            def b_in():
                return xb_ref[0:2 * seg, :]
        else:
            lb = (t == t_last).astype(jnp.int32)
            jobs = [(lb, t - 1 - lb * (LAG + 1))]

            def b_in():
                return xb_ref[pl.ds(pl.multiple_of(lb * seg, seg), seg), :]
        v0r = _cat([hc[0:n_mem], h_ref[n_mem:M2, :]])
        v1r = _cat([hc[n_mem:M2], h_ref[M2 + n_mem:2 * M2, :]])

        hist = []
        never = t > 4 * n_seg

        def gate(back, z):
            gv = hist[-back]
            return _cat([jnp.where(never, gv, z[e:e + 8]) for e in range(0, z.shape[0], 8)])

        def ktiles(z):
            return [z[:, k * 128:(k + 1) * 128] for k in range(z.shape[1] // 128)]
        if full:
            hl = _Operands(ktiles(_cat([v0r, h_ref[2 * M2:RB, :]])), ktiles(_cat([v1r, h_ref[RB:RB + AH, :]])), None)
        else:
            hl = _Operands(None, None, ktiles(_cat([h_ref[n_mem:M2, :], v1r, h_ref[2 * M2:RB, :]])), F32)
        mh = 2 * M2 if full else 0

        def tile_dot(p, r):
            src = wr_ref.at[p] if r == 0 else w_ref.at[p * NG + r - 1]

            def dot(a, i):
                wt = src[i * 64:(i + 1) * 64, :]
                cnt[0] += 1
                if dl and cnt[0] >= dl[0][0]:
                    deps = dl.pop(0)[1]
                    wt = _cat([jnp.where(never, pltpu.bitcast(d, U32), wt[8 * e:8 * e + 8])
                               for e, d in enumerate(deps)] + [wt[8 * len(deps):]])
                res_ = _nn(a, _upk(wt))
                hist.append(res_[0:8])
                return res_
            return dot
        cnt, dl = [0], []
        scale = float(dh) ** (-0.5) * LOG2E
        if full:
            s_ = t - LAG
            rd = pl.multiple_of(lax.rem(s_ * (seg // 2), RS // 2), seg // 2)
            wa = pl.multiple_of(lax.rem((A0 - R0 + s_ * AH) // 2, RS // 2), 8)

        RA = R if full else n_mem + seg
        CW = R
        bidx = 0 if full else 2
        half = dh - 128
        la8 = lax.broadcasted_iota(jnp.int32, (n_mem, 128), 1) < half
        ones = jnp.full((n_mem, 128), 0xFFFFFFFF, U32)
        zero = jnp.zeros((n_mem, 128), U32)
        mask_a = jnp.where(la8, ones, zero)
        mask_b = jnp.where(la8, zero, ones)

        def pk2(a, b):
            return _pk(_cat([a, b]).astype(BF16))

        yt = [[None] * NT for _ in range(3)]

        def proj(p, r):
            pa, qa = {}, {}
            _fast_mm((S53 if r == 0 else S55)[1], hl, tile_dot(p, r), mh, pa, qa)
            n0 = 0 if r == 0 else RT + (r - 1) * GT
            for n in range(len(pa)):
                y, z, e = _fast_out(pa, qa, n, mh)
                idx = p * NT + n0 + n
                if full:
                    ring_ref[idx, pl.ds(wa, 8), :] = pk2(z[16:24], z[24:32])
                    y = _cat([y[0:M2], z[0:M2], y[M2:2 * M2]])
                else:
                    y = _cat([e[0:8], e])
                yt[p][n0 + n] = stash(p * 16 + (n0 + n) % 16, packed(p, (n0 + n) % 3, y))

        def ab(z8):
            return jnp.where(la8, z8, 0.0), jnp.where(la8, 0.0, z8)

        def packed(p, j, y):
            if p == 0:
                return [pltpu.bitcast(y[e:e + 8], U32) for e in range(0 if full else 8, RB, 8)]
            u2 = pk2(y[32:40], y[40:48])
            if j == 0:
                return [pk2(y[0:8], y[8:16]), pk2(y[16:24], y[24:32]), u2]
            if j == 2:
                return [pk2(y[8:16], y[0:8]), pk2(y[24:32], y[16:24]), u2]
            xa_a, xa_b = ab(y[8:16])
            out = [pk2(xa_b, xa_a), pk2(y[24:32], y[16:24]) & mask_b, pk2(y[16:24], y[24:32]) & mask_a, u2]
            if full:
                out += [pk2(*ab(y[0:8]))]
            return out

        def stash(idx, parts):
            kv_ref[idx, 0:8 * len(parts), :] = _cat(parts)
            return lambda: [kv_ref[idx, 8 * e:8 * e + 8, :] for e in range(len(parts))]

        def pair(p, g):
            xs = [ring_ref[p * NT + 3 * g + j, pl.ds(rd, seg // 2), :] for j in range(3)] if full else None
            return [f() for f in yt[p][3 * g:3 * g + 3]], xs

        def q_rows(z, j):
            if not full:
                return pltpu.bitcast(_cat(z[0][j]), F32)
            f = [pltpu.bitcast(e, F32) for e in z[0][j]]
            return _cat(f[0:2] + [_upk(z[1][j]).astype(F32)] + f[2:])

        def kv_tiles(z):
            yt, x1 = z
            v0, v1, v2 = yt[0]
            t0 = [v0] + ([x1[0]] if full else [v1, v2]) + [v1, v2]
            w0, w1, w2 = yt[2]
            t2 = [w0, w1, w2] + ([x1[2]] if full else [w1, w2])
            e1, mb, ma, u2 = yt[1][0:4]
            mid2 = [e1, mb, u2 & mask_b, ma, u2 & mask_a]
            mid1 = None
            if full:
                lo, hi = x1[1][0:8], x1[1][8:16]
                mid1 = [yt[1][4], lo & mask_a, hi & mask_a, lo & mask_b, hi & mask_b]
            return t0, mid1, mid2, t2

        def mat(parts):
            return _upk(_cat(parts))

        def merge(y1, y2):
            return _cat([y1[0:8], y2[0:8], y1[8:40], y2[8:40]])

        def scores(q, k):
            k0, km1, km2, k2_ = kv_tiles(k)
            s_a = _nt(q_rows(q, 0), mat(k0))
            s_b = _nt(q_rows(q, 2), mat(k2_))
            if full:
                f = [pltpu.bitcast(z, F32) for z in q[0][1]]
                s_m = merge(_nt(_cat([f[0], _upk(q[1][1]).astype(F32)]), mat(km1)),
                            _nt(_cat(f[1:]), mat(km2)))
            else:
                s_m = _nt(q_rows(q, 1), mat(km2))
            out = []
            for e, sx in enumerate((s_a, s_b)):
                s = (sx + s_m) * scale + bias_ref[bidx + e, 0:RA, 0:CW]
                ex = jnp.exp2(s - jnp.max(s, axis=-1, keepdims=True))
                out.append(ex * _recip(jnp.sum(ex, axis=-1, keepdims=True)))
            return out

        def pv(p, v):
            PD = BF16 if full else F32
            v0, vm1, vm2, v2 = kv_tiles(v)
            o_a = _nn(p[0].astype(PD), mat(v0))
            o_b = _nn(p[1].astype(PD), mat(v2))
            p = p[0] + p[1]
            if full:
                o_m = merge(_nn(_cat([p[0:8], p[16:48]]), mat(vm1)), _nn(_cat([p[8:16], p[48:80]]), mat(vm2)))
            else:
                o_m = _nn(p.astype(PD), mat(vm2))
            return [o_a, o_m, o_b]

        ot = []
        pacc, qacc = {}, {}
        mo = n_mem + seg if full else 0

        def add_o(r):
            n0 = 0 if r == 0 else RT + (r - 1) * GT
            oo = ot[n0:n0 + (RT if r == 0 else GT)]
            if full:
                us = [_cat([o[48:56], o[8:16], o[56:80]]) for o in oo]
                if r < TAILPV:
                    us = [gate(GATE_O, z) for z in us]
                ops = _Operands([_cat([o[0:8], o[16:48]]) for o in oo], us, None, F32)
            else:
                ops = _Operands(None, None, oo, F32)
            _fast_mm((S35 if r == 0 else S55)[1], ops, tile_dot(3, r), mo, pacc, qacc)

        bqkv = [None] * 3
        probs = []

        def do_pv():
            for g in range(len(ot) // 3, len(probs)):
                ot.extend(pv(probs[g], pair(2, g)))

        if full:
            an = pl.multiple_of(jnp.minimum(A0 + (s_ + 1) * AH, S - AH), AH)
            h_ref[RB:RB + AH, :] = _ln(x_ref[pl.ds(an, AH), :].astype(F32))

        for r in range(NG + 1):
            for pp in (2, 1, 0):
                proj(pp, r)
            if r == 0:
                blhs = _ln(b_in())
            if r < 3:
                bqkv[2 - r] = b_proj(blhs, 2 - r)
            if r == 3:
                ob = b_attn(jobs, *bqkv)
            if r == BOUT_R:
                zb = b_out(_cat(ob), b_in())
                x2_new = zb[0:seg]
                if full:
                    o_store(t - 1 - LAG, zb[seg:2 * seg])
                    nxt = x2_new
                else:
                    o_store(lb * (t_last - LAG - 1) - 1, x2_new)
                    nxt = jnp.where(t < LAG - 1, x_ref[seg:2 * seg, :].astype(F32), x2_new)
                sl = _ln(nxt)
                h_ref[n_mem:M2, :] = sl[0:n_mem]
                h_ref[M2 + n_mem:RB, :] = sl[n_mem:seg]
                if full:
                    for j in range(nct):
                        dl.append((cnt[0] + DUE_LN + 2 * j, [sl[e:e + 8, j * 128:(j + 1) * 128] for e in range(0, seg, 8)]))
            if r in WSCHED:
                add_o(WSCHED[r])
            do_pv()
            for g in range(len(probs), (RT + r * GT) // 3):
                probs.append(scores(pair(0, g), pair(1, g)))
        for r in range(len(WSCHED), TAILPV):
            add_o(r)
        do_pv()
        for r in range(TAILPV, NG + 1):
            add_o(r)
        cols = []
        for n in range(nct):
            y, z, e = _fast_out(pacc, qacc, n, mo)
            cols.append(_cat([y[0:8], z[8:16], y[8:40], z[0:8], z[16:40]]) if full else e)
        acc = _cat(cols, axis=1)

        xa0 = n_mem if full else 0
        y2 = x2_ref[...] + _cat([acc[xa0:xa0 + n_mem], acc[RA - seg + n_mem:RA]])
        mem2 = acc[RA - seg:RA - seg + n_mem]
        if full:
            x_cur = x_ref[pl.ds(pl.multiple_of(t * seg, seg), seg), :].astype(F32)
            xb_ref[0:seg, :] = x_cur + acc[M2:M2 + seg]
            xb_ref[seg:2 * seg, :] = y2
            m1n = acc[0:n_mem]
            m2n = mem2
        else:
            xb_ref[pl.ds(pl.multiple_of(jnp.where(t < LAG, 0, (t - n_seg + 2) * seg), seg), seg), :] = y2
            m1n = mem2
            m2n = jnp.where(t == LAG - 1, mem0_ref[...].astype(F32), mem2)
        x2_ref[...] = nxt
        return _cat([m1n, m2n])

    def single_body(t, c):
        @pl.when(t == n_seg)
        def _():
            out_copy(t - (LAG + 2)).start()
        return step(t, c, False)

    def full_body(t, c):
        @pl.when(t >= LAG + 2)
        def _():
            out_copy(t - (LAG + 2)).start()
        return step(t, c, True)

    def phase(ph, c):
        t0 = ph * n_seg
        c = lax.fori_loop(t0, t0 + LAG, single_body, c)

        @pl.when(ph == 0)
        def _():
            x_late.wait()
        return lax.fori_loop(LAG, jnp.where(ph == 0, n_seg, LAG), full_body, c)
    lax.fori_loop(0, 2, phase, _cat([mem0_ref[...].astype(F32)] * 2))

    out_copy(n_seg - 3).start()
    res = xb_ref[2 * seg:4 * seg, :]
    blhs = _ln(res)
    ob = b_attn([(1, n_seg - 2), (1, n_seg - 1)], *[b_proj(blhs, part) for part in range(3)])
    o_store(n_seg - 2, b_out(_cat(ob), res))
    out_copy(n_seg - 2).start()
    out_copy(n_seg - 1).start()
    pltpu.make_async_copy(o_ref.at[pl.ds(seg, S), :], out_hbm, sem_o).wait()


@functools.partial(jax.jit, static_argnames=("seg",))
def _run(A_x, A_mem0, A_Wq, A_Wk, A_Wv, A_Wo, B_wqkv, B_wo, *, seg):
    _, S, dm = A_x.shape
    n_heads, dh = A_Wq.shape[1], A_Wq.shape[2]
    n_mem = A_mem0.shape[1]
    n_seg = S // seg
    hd = n_heads * dh
    nct = dm // 128
    ng = (hd // 128 - RT) // GT
    assert (seg, n_seg, n_mem, dh, dm % 128, n_heads, LAG) == (32, 64, 8, 192, 0, 32, 2)

    x = A_x.reshape(S, dm)
    mem0 = A_mem0.reshape(n_mem, dm)
    wq = jnp.transpose(A_Wq, (1, 2, 0)).reshape(hd, dm)
    wk = jnp.transpose(A_Wk, (1, 2, 0)).reshape(hd, dm)
    wv = jnp.transpose(A_Wv, (1, 2, 0)).reshape(hd, dm)
    wo = A_Wo.reshape(hd, dm)
    _, _, _, _, rs, xc = _plan(seg, n_seg)

    kern = functools.partial(_kernel, seg=seg, n_seg=n_seg, n_mem=n_mem,
                             n_heads=n_heads, dh=dh, dm=dm)
    hbm = pl.BlockSpec(memory_space=pltpu.HBM)

    out = pl.pallas_call(
        kern,
        in_specs=[hbm] * 8,
        out_specs=hbm,
        out_shape=jax.ShapeDtypeStruct((S, dm), A_x.dtype),
        scratch_shapes=[
            pltpu.VMEM((S, dm), BF16),
            pltpu.VMEM((n_mem, dm), BF16),
            pltpu.VMEM((NSLOT, 4, GT * 128, dm), BF16),
            pltpu.VMEM((RT * 128, dm), BF16),
            pltpu.VMEM((4, len(S53[0]) * 64, 128), U32),
            pltpu.VMEM((4 * ng, len(S55[0]) * 64, 128), U32),
            pltpu.VMEM((dm, 4 * dm + 128), BF16),
            pltpu.VMEM((nct, 4 * dm + 32, 128), F32),
            pltpu.VMEM((4 * nct, dm // 2, 128), U32),
            pltpu.VMEM((len(KEYS_R), HC * xc // 4, 128), U32),
            pltpu.VMEM((len(KEYS_R), HC * xc // 4, 128), U32),
            pltpu.VMEM((len(KEYS) - len(KEYS_R), NXC * xc // 4, 128), U32),
            pltpu.VMEM((len(KEYS), 8, 128), U32),
            pltpu.VMEM((3 * hd // 128, rs // 2, 128), U32),
            pltpu.VMEM((2 * n_mem + seg + AH, dm), F32),
            pltpu.VMEM((4 * seg, dm), F32),
            pltpu.VMEM((seg, dm), F32),
            pltpu.VMEM((2, nct, HIST + seg, 128), F32),
            pltpu.VMEM((2, nct, HIST + seg, 128), F32),
            pltpu.VMEM((S + seg, dm), A_x.dtype),
            pltpu.VMEM((4, 2 * n_mem + 2 * seg, 128), F32),
            pltpu.VMEM((48, 48, 128), U32),
            pltpu.VMEM((len(S55[0]) * 64, 128), U32),
            pltpu.SemaphoreType.DMA((NSLOT,)),
            pltpu.SemaphoreType.DMA((8 + NXC,)),
            pltpu.SemaphoreType.DMA((4,)),
            pltpu.SemaphoreType.DMA(()),
        ],
        compiler_params=pltpu.CompilerParams(
            vmem_limit_bytes=127 * 1024 * 1024,
            disable_bounds_checks=True,
        ),
    )(x, mem0, wq, wk, wv, wo, B_wqkv, B_wo)
    return out.reshape(1, S, dm)


def pallas_interleave_layers__memory_aug_recurrent_mem_tr__sliding_local_dilated__prompt_kernel(
    A_x: jax.Array,
    A_mem0: jax.Array,
    A_Wq: jax.Array,
    A_Wk: jax.Array,
    A_Wv: jax.Array,
    A_Wo: jax.Array,
    A_seg_len,
    B_x: jax.Array,
    B_wqkv: jax.Array,
    B_wo: jax.Array,
):
    del B_x
    seg = A_seg_len if isinstance(A_seg_len, int) else 32
    return _run(A_x, A_mem0, A_Wq, A_Wk, A_Wv, A_Wo, B_wqkv, B_wo, seg=seg)
```
